```python
import jax
import jax.numpy as jnp

def _softmax(x, axis=-1):
    return jax.nn.softmax(x, axis=axis)
def _gelu(x):
    return jax.nn.gelu(x, approximate=True)
def _silu(x):
    return jax.nn.silu(x)
def _sigmoid(x):
    return jax.nn.sigmoid(x)
def _layernorm(x, axis=-1, eps=1e-5):
    m = jnp.mean(x, axis=axis, keepdims=True)
    v = jnp.var(x, axis=axis, keepdims=True)
    return (x - m) / jnp.sqrt(v + eps)
def _scatter_add(tgt, idx, src, axis=0):
    return tgt.at[idx].add(src)
def _segment_sum(src, seg, n):
    return jax.ops.segment_sum(src, seg, n)
class _Rng:
    def __init__(self, key):
        self._k = key
    def _next(self):
        self._k, sub = jax.random.split(self._k)
        return sub
    def normal(self, shape):
        return jax.random.normal(self._next(), shape, dtype=jnp.bfloat16)
    def randint(self, lo, hi, shape):
        return jax.random.randint(self._next(), shape, lo, hi, dtype=jnp.int32)
    def uniform(self, shape, lo=0.0, hi=1.0):
        return jax.random.uniform(self._next(), shape, jnp.bfloat16, lo, hi)
    def permutation(self, n):
        return jax.random.permutation(self._next(), n)


kernel_name = 'parallel_sum__linear_attn_block__moe_arch_mod__prompt'

def setup_inputs():
    _rng = _Rng(jax.random.key(int.from_bytes(__import__("os").urandom(4), "little")))
    _w = (lambda a: (lambda t: t.astype(jnp.bfloat16) if jnp.issubdtype(t.dtype, jnp.floating) else t)(jnp.asarray(a)))
    def _A_setup():
        B, S, D = 1, 2048, 1024
        return {
            "x": _w((lambda *s: _rng.normal(s) * 0.05)(B, S, D)),
            "wqkv": _w((lambda *s: _rng.normal(s) * 0.05)(D, 3 * D)),
            "wo": _w((lambda *s: _rng.normal(s) * 0.05)(D, D)),
        }
    _A_in = _A_setup()

    def _B_setup():
        B, S, D, F, C = 1, 2048, 1024, 3584, 1
        return {
            "x": _w((lambda *s: _rng.normal(s) * 0.05)(B, S, D)),
            "w_r": _w((lambda *s: _rng.normal(s) * 0.05)(D)),
            "w_gate": _w((lambda *s: _rng.normal(s) * 0.05)(D, F)),
            "w_up": _w((lambda *s: _rng.normal(s) * 0.05)(D, F)),
            "w_down": _w((lambda *s: _rng.normal(s) * 0.05)(F, D)),
        }
    _B_in = _B_setup()

    return {
        "A_x": _A_in["x"],
        "A_wqkv": _A_in["wqkv"],
        "A_wo": _A_in["wo"],
        "B_x": _B_in["x"],
        "B_w_r": _B_in["w_r"],
        "B_w_gate": _B_in["w_gate"],
        "B_w_up": _B_in["w_up"],
        "B_w_down": _B_in["w_down"],
    }

def reference(A_x, A_wqkv, A_wo, B_x, B_w_r, B_w_gate, B_w_up, B_w_down):
    def _A_ref(x, wqkv, wo):
        B, S, D = x.shape
        H = 32; Dh = D // H
        qkv = (lambda x, *d: x.transpose(*d))((x @ wqkv).reshape(B, S, 3, H, Dh), 2, 0, 3, 1, 4)
        q, k, v = qkv[0], qkv[1], qkv[2]
        phi = lambda t: jnp.where(t > 0, t + 1, jnp.exp(t)) + 1e-6
        pq, pk = phi(q), phi(k)
        kv = jnp.einsum("bhsd,bhse->bhde", pk, v)
        z = jnp.einsum("bhsd->bhd", pk)
        num = jnp.einsum("bhqd,bhde->bhqe", pq, kv)
        den = jnp.einsum("bhqd,bhd->bhq", pq, z)[..., None] + 1e-6
        o = num / den
        return (lambda x, *d: x.transpose(*d))(o, 0, 2, 1, 3).reshape(B, S, D) @ wo

    def _B_ref(x, w_r, w_gate, w_up, w_down):
        B, S, D = x.shape
        C = 1
        r = x @ w_r
        idx = jnp.argsort(-r, axis=-1)[:, :C]
        idx_e = jnp.repeat(idx.reshape(B, C, 1), D, axis=2)
        x_sel = jnp.take_along_axis(x, idx_e, axis=1)
        g = _silu(x_sel @ w_gate)
        u = x_sel @ w_up
        y = (g * u) @ w_down
        r_sel = _sigmoid(jnp.take_along_axis(r, idx, axis=1))
        y = y * r_sel.reshape(B, C, 1)
        b_off = (jnp.arange(B) * S).reshape(B, 1)
        flat_idx = (idx + b_off).reshape(B * C)
        zero = (x * 0.0).reshape(B * S, D)
        upd = _scatter_add(zero, flat_idx, y.reshape(B * C, D), axis=0)
        return x + upd.reshape(B, S, D)

    x = A_x
    xn = _layernorm(x, axis=-1)
    return x + _A_ref(xn, A_wqkv, A_wo) + _B_ref(xn, B_w_r, B_w_gate, B_w_up, B_w_down)
```

```python
import jax
import jax.numpy as jnp
from jax import lax
import jax.experimental.pallas as pl
import jax.experimental.pallas.tpu as pltpu

bf16, f32, u32, i32 = jnp.bfloat16, jnp.float32, jnp.uint32, jnp.int32

S = 2048
D = 1024
F = 3584
HP = S // 2
HD = D // 2
R = 256
NT = HP // R
FW = 512
NF = F // FW

L_ORD = (2, 3, 0, 1, 4, 5, 6)
R_ORD = (2, 0, 6, 5, 1, 4, 3)

NN = (((1,), (0,)), ((), ()))
NT_ = (((1,), (1,)), ((), ()))
TN = (((0,), (0,)), ((), ()))


def _dot(a, b, dims):
    return lax.dot_general(a, b, dims, preferred_element_type=f32)


def _pack(v):
    return pltpu.bitcast(v.astype(bf16), u32)


def _unpack(v):
    return pltpu.bitcast(v, bf16)


def _combine(m):
    m1, m2, m3, m4, m5, m6, m7 = m
    return m1 + m4 - m5 + m7, m3 + m5, m2 + m4, m1 - m2 + m3 + m6


def _lform(a11, a12, a21, a22):
    return (a11 + a22, a21 + a22, a11, a22, a11 + a12, a21 - a11, a12 - a22)


def _rform(b11, b12, b21, b22):
    return (b11 + b22, b11, b12 - b22, b21 - b11, b22, b11 + b12, b21 + b22)


def _phi(t):
    return jnp.where(t > 0, t + 1.0, jnp.exp(t)) + 1e-6


def _rbf(v):
    return v.astype(bf16).astype(f32)


def _layernorm_rows(xv):
    mf = jnp.sum(xv, axis=1, keepdims=True) * (1.0 / D)
    mb = _rbf(mf)
    d = xv - mb
    dm = mf - mb
    var = jnp.sum(d * d, axis=1, keepdims=True) * (1.0 / D) - dm * dm
    var = jnp.maximum(var, 0.0)
    sd = _rbf(jnp.sqrt(_rbf(_rbf(var) + 1e-5)))
    return d * (1.0 / sd)


def _kernel(x_hbm, wqkv_hbm, wo_hbm, wr_hbm, wg_hbm, wu_hbm, wd_hbm, out_hbm,
            x_buf, wk_buf, wq_buf, wv_buf, wo_buf, wr_buf, wg_buf, wu_buf, wd_buf,
            xs, ps, qs, wks, wqs, ms, res, rbuf, zacc, zp, tscr, pq_buf,
            xb, yacc, rsel, out_buf, idx_s,
            sem_x, sem_w, sem_f, sem_o):

    def cp_x(t, h):
        r0 = h * HP + t * R
        return pltpu.make_async_copy(x_hbm.at[0, pl.ds(r0, R), :], x_buf.at[pl.ds(r0, R), :],
                                     sem_x.at[2 * t + h])

    cp_wk = pltpu.make_async_copy(wqkv_hbm.at[:, pl.ds(D, D)], wk_buf, sem_w.at[0])
    cp_wq = pltpu.make_async_copy(wqkv_hbm.at[:, pl.ds(0, D)], wq_buf, sem_w.at[1])
    cp_wo = pltpu.make_async_copy(wo_hbm, wo_buf, sem_w.at[2])
    cp_wr = pltpu.make_async_copy(wr_hbm, wr_buf, sem_w.at[3])
    cp_wv = [pltpu.make_async_copy(wqkv_hbm.at[:, pl.ds(2 * D + 128 * g, 128)], wv_buf.at[g],
                                   sem_w.at[4 + g]) for g in range(8)]

    def cp_ffn(c):
        return (pltpu.make_async_copy(wg_hbm.at[:, pl.ds(c * FW, FW)], wg_buf.at[c], sem_f.at[3 * c]),
                pltpu.make_async_copy(wu_hbm.at[:, pl.ds(c * FW, FW)], wu_buf.at[c], sem_f.at[3 * c + 1]),
                pltpu.make_async_copy(wd_hbm.at[pl.ds(c * FW, FW), :], wd_buf.at[c], sem_f.at[3 * c + 2]))

    def wait_ffn(c):
        pltpu.make_async_copy(wg_buf.at[c], wg_buf.at[c], sem_f.at[3 * c]).wait()
        pltpu.make_async_copy(wu_buf.at[c], wu_buf.at[c], sem_f.at[3 * c + 1]).wait()
        pltpu.make_async_copy(wd_buf.at[c], wd_buf.at[c], sem_f.at[3 * c + 2]).wait()

    def cp_out(t, h):
        r0 = h * HP + t * R
        if not isinstance(r0, int):
            r0 = pl.multiple_of(r0, R)
        return pltpu.make_async_copy(out_buf.at[pl.ds(r0, R), :], out_hbm.at[0, pl.ds(r0, R), :],
                                     sem_o.at[2 * t + h])

    def ln_tile(t):
        wr = wr_buf[...].reshape(1, D).astype(f32)
        for c in range(R // 16):
            p0 = t * R + c * 16
            halves = []
            for h in range(2):
                r0 = h * HP + p0
                xv = x_buf[r0:r0 + 16, :].astype(f32)
                xn = _layernorm_rows(xv)
                res[r0:r0 + 16, :] = xv + xn
                rbuf[r0:r0 + 16, :] = _rbf(jnp.sum(_rbf(xn) * wr, axis=1, keepdims=True))
                halves.append(xn)
            x11, x12 = halves[0][:, :HD], halves[0][:, HD:]
            x21, x22 = halves[1][:, :HD], halves[1][:, HD:]
            ops = (x11, x22, x11 + x22, x21 + x22, x11 + x12, x21 - x11, x12 - x22)
            for k in range(7):
                xs[k, p0 // 2:p0 // 2 + 8, :] = _pack(ops[k])

    def wk_prep():
        for c in range(HD // 16):
            r0 = c * 16
            top = wk_buf[r0:r0 + 16, :].astype(f32)
            bot = wk_buf[HD + r0:HD + r0 + 16, :].astype(f32)
            ops = _rform(top[:, :HD], top[:, HD:], bot[:, :HD], bot[:, HD:])
            for k in range(7):
                wks[k, r0 // 2:r0 // 2 + 8, :] = _pack(ops[k])

    def wq_prep():
        for g in range(8):
            wt = _pack(wq_buf[:, g * 128:(g + 1) * 128].T)
            for ct in range(8):
                tscr[ct] = wt[:, ct * 128:(ct + 1) * 128]
            for j in range(4):
                def rows(jj):
                    return _unpack(jnp.concatenate(
                        [tscr[ct, pl.ds(jj, 8, stride=8), :] for ct in range(8)], axis=1)).astype(f32)
                top, bot = rows(j), rows(j + 4)
                w11, w12, w21, w22 = top[:, :HD], top[:, HD:], bot[:, :HD], bot[:, HD:]
                ops = _rform(w11, w21, w12, w22)
                for k in range(7):
                    wqs[k, j * 64 + g * 8:j * 64 + g * 8 + 8, :] = _pack(ops[k])

    def kproj_tile(t):
        pr = pl.ds(t * (R // 2), R // 2)
        for c in range(4):
            cs = slice(c * 128, (c + 1) * 128)
            m = [_dot(_unpack(xs[L_ORD[k], pr, :]), _unpack(wks[k, :, cs]), NN) for k in range(7)]
            k11, k12, k21, k22 = [_phi(v) for v in _combine(m)]
            zl = (k11 + k21).reshape(R // 8, 8, 128).sum(axis=0)
            zr = (k12 + k22).reshape(R // 8, 8, 128).sum(axis=0)
            zacc[:, cs] += zl
            zacc[:, HD + c * 128:HD + (c + 1) * 128] += zr
            ops = _lform(k11, k21, k12, k22)
            for k in range(7):
                ps[k, c, pr, :] = _pack(ops[k])

    def z_prep():
        z = jnp.sum(zacc[...], axis=0, keepdims=True)
        zt = _pack(jnp.broadcast_to(z, (128, D)).astype(bf16).T)
        for g in range(8):
            tscr[g] = zt[g * 64:(g + 1) * 64, :]
        for j in range(8):
            blk = jnp.concatenate([tscr[g, pl.ds(j, 8, stride=8), :] for g in range(8)], axis=0)
            zp[:, j * 128:(j + 1) * 128] = _unpack(blk).T[0:8, :].astype(f32)

    def route():
        rv = rbuf[...]
        rmax = jnp.max(rv)
        idx = jnp.min(jnp.where(rv == rmax, lax.broadcasted_iota(i32, rv.shape, 0), S - 1))
        idx_s[0] = idx
        rsel[...] = jnp.full(rsel.shape, rmax, f32)
        b0 = pl.multiple_of((idx // 16) * 16, 16)
        xn = _rbf(_layernorm_rows(x_buf[pl.ds(b0, 16), :].astype(f32)))
        sel = lax.broadcasted_iota(i32, xn.shape, 0) == idx - b0
        row = jnp.sum(jnp.where(sel, xn, 0.0), axis=0, keepdims=True)
        xb[...] = jnp.broadcast_to(row, (128, D)).T
        yacc[...] = jnp.zeros(yacc.shape, f32)

    def g_chunk(j):
        m = [_dot(_unpack(ps[k, j]), _unpack(xs[R_ORD[k]]), TN) for k in range(7)]
        g11, g12, g21, g22 = _combine(m)
        hm = (lax.broadcasted_iota(i32, (128, 128), 0) // 32
              == lax.broadcasted_iota(i32, (128, 128), 1) // 32)
        for half, (ga, gb) in enumerate(((g11, g12), (g21, g22))):
            g = j + 4 * half
            gg = jnp.concatenate([ga, gb], axis=1).astype(bf16)
            kv = jnp.where(hm, _dot(gg, wv_buf[g], NN), 0.0)
            tscr[half] = _pack(kv)
            kvp = _unpack(jnp.concatenate(
                [tscr[half, pl.ds(jj, 8, stride=8), :] for jj in range(8)], axis=0))
            mg = _dot(kvp, wo_buf[pl.ds(pl.multiple_of(g * 128, 128), 128), :], NN)
            ops = _rform(mg[:64, :HD], mg[:64, HD:], mg[64:, :HD], mg[64:, HD:])
            for k in range(7):
                pk_ = _pack(ops[k])
                for jj in range(4):
                    ms[k, pl.ds(pl.multiple_of(jj * 64 + g * 8, 8), 8), :] = pk_[jj * 8:(jj + 1) * 8]

    def qproj_tile(t):
        pr = pl.ds(pl.multiple_of(t * (R // 2), R // 2), R // 2)
        dt = jnp.zeros((R, 128), f32)
        db = jnp.zeros((R, 128), f32)
        for c in range(4):
            m = [_dot(_unpack(xs[L_ORD[k], pr, :]), _unpack(wqs[k, c * 64:(c + 1) * 64, :]), NT_)
                 for k in range(7)]
            q11, q12, q21, q22 = [_phi(v) for v in _combine(m)]
            zl = zp[0:1, c * 128:(c + 1) * 128]
            zr = zp[0:1, HD + c * 128:HD + (c + 1) * 128]
            dt = dt + q11 * zl + q12 * zr
            db = db + q21 * zl + q22 * zr
            pq_buf[0, :, c * 128:(c + 1) * 128] = q11
            pq_buf[0, :, HD + c * 128:HD + (c + 1) * 128] = q12
            pq_buf[1, :, c * 128:(c + 1) * 128] = q21
            pq_buf[1, :, HD + c * 128:HD + (c + 1) * 128] = q22
        lane = lax.broadcasted_iota(i32, (R, 128), 1)
        recs = []
        for d in (dt, db):
            d = d + jnp.where(lane % 2 == 0, pltpu.roll(d, 127, 1), pltpu.roll(d, 1, 1))
            d = d + jnp.where(lane % 4 < 2, pltpu.roll(d, 126, 1), pltpu.roll(d, 2, 1))
            recs.append(1.0 / (d + 1e-6))
        for c in range(R // 16):
            rs = slice(c * 16, (c + 1) * 16)
            top = pq_buf[0, rs, :] * jnp.concatenate([recs[0][rs]] * 8, axis=1)
            bot = pq_buf[1, rs, :] * jnp.concatenate([recs[1][rs]] * 8, axis=1)
            ops = _lform(top[:, :HD], top[:, HD:], bot[:, :HD], bot[:, HD:])
            p2 = pl.ds(pl.multiple_of(t * (R // 2) + c * 8, 8), 8)
            for k in range(7):
                qs[k, p2, :] = _pack(ops[k])

    def out_tile(t):
        pr = pl.ds(pl.multiple_of(t * (R // 2), R // 2), R // 2)
        rt = pl.ds(pl.multiple_of(t * R, R), R)
        rb = pl.ds(pl.multiple_of(HP + t * R, R), R)
        for c in range(2):
            cl = slice(c * 256, (c + 1) * 256)
            cr = slice(HD + c * 256, HD + (c + 1) * 256)
            m = [_dot(_unpack(qs[k, pr, :]), _unpack(ms[k, :, cl]), NN) for k in range(7)]
            o11, o12, o21, o22 = _combine(m)
            out_buf[rt, cl] = (res[rt, cl] + o11).astype(bf16)
            out_buf[rt, cr] = (res[rt, cr] + o12).astype(bf16)
            out_buf[rb, cl] = (res[rb, cl] + o21).astype(bf16)
            out_buf[rb, cr] = (res[rb, cr] + o22).astype(bf16)

    def ffn_chunk(c):
        ag = jnp.zeros((8, FW), f32)
        au = jnp.zeros((8, FW), f32)
        for kg in range(D // 8):
            xv = jnp.concatenate([xb[8 * kg:8 * kg + 8, :]] * (FW // 128), axis=1)
            ag = ag + wg_buf[c, 8 * kg:8 * kg + 8, :].astype(f32) * xv
            au = au + wu_buf[c, 8 * kg:8 * kg + 8, :].astype(f32) * xv
        g = _rbf(jnp.sum(ag, axis=0, keepdims=True))
        u = _rbf(jnp.sum(au, axis=0, keepdims=True))
        h = _rbf(_rbf(g * jax.nn.sigmoid(g)) * u)
        hb = jnp.broadcast_to(h, (128, FW)).T
        acc = yacc[...]
        for kg in range(FW // 8):
            hv = jnp.concatenate([hb[8 * kg:8 * kg + 8, :]] * (D // 128), axis=1)
            acc = acc + wd_buf[c, 8 * kg:8 * kg + 8, :].astype(f32) * hv
        yacc[...] = acc

    cp_wr.start()
    cp_x(0, 0).start()
    cp_x(0, 1).start()
    cp_wk.start()
    for t in range(1, NT):
        cp_x(t, 0).start()
        cp_x(t, 1).start()
    zacc[...] = jnp.zeros(zacc.shape, f32)
    cp_wr.wait()
    cp_x(0, 0).wait()
    cp_x(0, 1).wait()
    ln_tile(0)
    cp_wk.wait()
    cp_wq.start()
    for c in cp_wv:
        c.start()
    cp_wo.start()
    for c in range(NF):
        for d in cp_ffn(c):
            d.start()
    wk_prep()
    for t in range(NT):
        if t + 1 < NT:
            cp_x(t + 1, 0).wait()
            cp_x(t + 1, 1).wait()
            kproj_tile(t)
            ln_tile(t + 1)
        else:
            cp_wq.wait()
            kproj_tile(t)
            wq_prep()
            route()
    z_prep()
    for c in cp_wv:
        c.wait()
    cp_wo.wait()

    def b_body(j, carry):
        wait_ffn(j)
        g_chunk(j)
        qproj_tile(j)
        ffn_chunk(j)
        return carry

    lax.fori_loop(0, NT, b_body, 0)

    def c_body(t, carry):
        wait_ffn(NT + t)
        out_tile(t)
        ffn_chunk(NT + t)
        cp_out(t, 0).start()
        cp_out(t, 1).start()
        return carry

    lax.fori_loop(0, NT - 1, c_body, 0)
    out_tile(NT - 1)

    for t in range(NT - 1):
        cp_out(t, 0).wait()
        cp_out(t, 1).wait()
    idx = idx_s[0]
    y = _rbf(jnp.sum(yacc[...], axis=0, keepdims=True))
    y = _rbf(y * _rbf(jax.nn.sigmoid(rsel[...])))
    b0 = pl.multiple_of((idx // 16) * 16, 16)
    blk = out_buf[pl.ds(b0, 16), :].astype(f32)
    sel = lax.broadcasted_iota(i32, blk.shape, 0) == idx - b0
    out_buf[pl.ds(b0, 16), :] = (blk + jnp.where(sel, y, 0.0)).astype(bf16)
    cp_out(NT - 1, 0).start()
    cp_out(NT - 1, 1).start()

    @pl.when(idx % HP < (NT - 1) * R)
    def _():
        cp = pltpu.make_async_copy(out_buf.at[pl.ds(b0, 16), :], out_hbm.at[0, pl.ds(b0, 16), :],
                                   sem_o.at[0])
        cp.start()
        cp.wait()

    cp_out(NT - 1, 0).wait()
    cp_out(NT - 1, 1).wait()


@jax.jit
def pallas_parallel_sum__linear_attn_block__moe_arch_mod__prompt_kernel(
    A_x: jax.Array,
    A_wqkv: jax.Array,
    A_wo: jax.Array,
    B_x: jax.Array,
    B_w_r: jax.Array,
    B_w_gate: jax.Array,
    B_w_up: jax.Array,
    B_w_down: jax.Array,
):
    del B_x
    V = pltpu.VMEM
    scratch = [
        V((S, D), bf16),
        V((D, D), bf16),
        V((D, D), bf16),
        V((8, D, 128), bf16),
        V((D, D), bf16),
        V((D,), bf16),
        V((NF, D, FW), bf16),
        V((NF, D, FW), bf16),
        V((NF, FW, D), bf16),
        V((7, HP // 2, HD), u32),
        V((7, 4, HP // 2, 128), u32),
        V((7, HP // 2, HD), u32),
        V((7, HD // 2, HD), u32),
        V((7, HD // 2, HD), u32),
        V((7, HD // 2, HD), u32),
        V((S, D), f32),
        V((S, 1), f32),
        V((8, D), f32),
        V((8, D), f32),
        V((8, 64, 128), u32),
        V((2, R, D), f32),
        V((D, 128), f32),
        V((8, D), f32),
        V((1, D), f32),
        V((S, D), bf16),
        pltpu.SMEM((1,), i32),
        pltpu.SemaphoreType.DMA((2 * NT,)),
        pltpu.SemaphoreType.DMA((12,)),
        pltpu.SemaphoreType.DMA((3 * NF,)),
        pltpu.SemaphoreType.DMA((2 * NT,)),
    ]
    return pl.pallas_call(
        _kernel,
        out_shape=jax.ShapeDtypeStruct((1, S, D), bf16),
        in_specs=[pl.BlockSpec(memory_space=pl.ANY)] * 7,
        out_specs=pl.BlockSpec(memory_space=pl.ANY),
        scratch_shapes=scratch,
        compiler_params=pltpu.CompilerParams(vmem_limit_bytes=110 * 1024 * 1024),
    )(A_x, A_wqkv, A_wo, B_w_r, B_w_gate, B_w_up, B_w_down)
```

```python
import contextlib

import jax
import jax.numpy as jnp
from jax import lax
import jax.experimental.pallas as pl
import jax.experimental.pallas.tpu as pltpu

bf16, f32, u32, i32 = jnp.bfloat16, jnp.float32, jnp.uint32, jnp.int32

S = 2048
D = 1024
F = 3584
HP = S // 2
HD = D // 2
R = 256
NT = HP // R
FW = 896
NF = F // FW
QLAG = 768

L_ORD = (2, 3, 0, 1, 4, 5, 6)
R_ORD = (2, 0, 6, 5, 1, 4, 3)

NN = (((1,), (0,)), ((), ()))
NT_ = (((1,), (1,)), ((), ()))
TN = (((0,), (0,)), ((), ()))


SCOPES = False


def _scope(name):
    return jax.named_scope(name) if SCOPES else contextlib.nullcontext()


def _dot(a, b, dims):
    return lax.dot_general(a, b, dims, preferred_element_type=f32)


def _pack(v):
    return pltpu.bitcast(v.astype(bf16), u32)


def _unpack(v):
    return pltpu.bitcast(v, bf16)


def _combine(m):
    m1, m2, m3, m4, m5, m6, m7 = m
    return m1 + m4 - m5 + m7, m3 + m5, m2 + m4, m1 - m2 + m3 + m6


def _lform(a11, a12, a21, a22):
    return (a11 + a22, a21 + a22, a11, a22, a11 + a12, a21 - a11, a12 - a22)


def _rform(b11, b12, b21, b22):
    return (b11 + b22, b11, b12 - b22, b21 - b11, b22, b11 + b12, b21 + b22)


def _phi(t):
    return jnp.where(t > 0, t + 1.0, jnp.exp(t)) + 1e-6


def _rbf(v):
    return v.astype(bf16).astype(f32)


def _layernorm_rows(xv):
    mf = jnp.sum(xv, axis=1, keepdims=True) * (1.0 / D)
    mb = _rbf(mf)
    d = xv - mb
    dm = mf - mb
    var = jnp.sum(d * d, axis=1, keepdims=True) * (1.0 / D) - dm * dm
    var = jnp.maximum(var, 0.0)
    sd = _rbf(jnp.sqrt(_rbf(_rbf(var) + 1e-5)))
    return d * (1.0 / sd)


def _kernel(x_hbm, wqkv_hbm, wo_hbm, wr_hbm, wg_hbm, wu_hbm, wd_hbm, out_hbm,
            x_buf, wk_buf, wq_buf, wv_buf, wo_buf, wr_buf, wg_buf, wu_buf, wd_buf,
            xs, ps, qs, wks, wqs, ms, sa, sb, stats, zacc, zp, tscr, tscr2, pq_buf,
            xb, yacc, rsel, out_buf, zero_buf, idx_s, sem):

    SEM_X, SEM_WK, SEM_WQ, SEM_B, SEM_O, SEM_Z = 0, NT, NT + 1, NT + 2, 2 * NT + 2, 2 * NT + 3

    def cp(src, dst, s):
        return pltpu.make_async_copy(src, dst, sem.at[s])

    def cp_x(t):
        return [cp(x_hbm.at[0, pl.ds(h * HP + t * R, R), :], x_buf.at[pl.ds(h * HP + t * R, R), :],
                   SEM_X + t) for h in range(2)]

    cp_wr = cp(wr_hbm, wr_buf, SEM_X)
    cp_wk = cp(wqkv_hbm.at[:, pl.ds(D, D)], wk_buf, SEM_WK)
    cp_wq = cp(wqkv_hbm.at[:, pl.ds(0, D)], wq_buf, SEM_WQ)

    def cp_b(j, wait_only=False):
        def off(v, m):
            return v if isinstance(v, int) else pl.multiple_of(v, m)
        out = []
        for g in (j, j + 4):
            c0 = off(g * 128, 128)
            dst = wv_buf.at[:, pl.ds(c0, 128)]
            out.append(cp(dst if wait_only else wqkv_hbm.at[:, pl.ds(2 * D + c0, 128)], dst, SEM_B + j))
            dst = wo_buf.at[pl.ds(c0, 128), :]
            out.append(cp(dst if wait_only else wo_hbm.at[pl.ds(c0, 128), :], dst, SEM_B + j))
        f0 = off(j * FW, 128)
        for src, dst in ((wg_hbm.at[:, pl.ds(f0, FW)], wg_buf.at[j]),
                         (wu_hbm.at[:, pl.ds(f0, FW)], wu_buf.at[j]),
                         (wd_hbm.at[pl.ds(f0, FW), :], wd_buf.at[j])):
            out.append(cp(dst if wait_only else src, dst, SEM_B + j))
        return out

    def cp_out(t, h):
        r0 = h * HP + t * R
        if not isinstance(r0, int):
            r0 = pl.multiple_of(r0, R)
        return cp(out_buf.at[pl.ds(r0, R), :], out_hbm.at[0, pl.ds(r0, R), :], SEM_O)

    clock = [0]
    toks = []
    sides = []

    def emit_tok(vals, stamp=None):
        t = None
        for v in vals:
            v = pltpu.bitcast(v, u32) if v.dtype != u32 else v
            t = v if t is None else t | v
        toks.append((clock[0] if stamp is None else stamp, t & zero_buf[0]))

    def add_side(gen_fn, n, t0, t1):
        st = {"i": 0, "n": n, "t0": clock[0] + t0, "t1": clock[0] + t1}
        st["g"] = gen_fn(lambda vals: emit_tok(
            vals, st["t0"] + (st["i"] + 1) * (st["t1"] - st["t0"]) // st["n"]))
        sides.append(st)

    def advance(until):
        for st in sides:
            while st["i"] < st["n"] and st["t0"] + st["i"] * (st["t1"] - st["t0"]) // st["n"] < until:
                next(st["g"], None)
                st["i"] += 1

    def finish():
        for st in sides:
            for _ in st["g"]:
                pass
        sides.clear()
        toks.clear()

    def mm(lhs, rhs, dims, cycles, nseg=1):
        advance(clock[0] + cycles)
        segs = []
        w = rhs.shape[1] // nseg
        for s in range(nseg):
            now = clock[0] + s * cycles // nseg
            due = [t for (c, t) in toks if c <= now]
            toks[:] = [(c, t) for (c, t) in toks if c > now]
            head = rhs[0:8, s * w:s * w + 128]
            for t in due:
                head = head | t
            segs.append(head)
            if w > 128:
                segs.append(rhs[0:8, s * w + 128:(s + 1) * w])
        rhs = jnp.concatenate([jnp.concatenate(segs, axis=1), rhs[8:]], axis=0)
        clock[0] += cycles
        return _dot(lhs, _unpack(rhs), dims)

    def ln_tile(t, tok):
        wr = wr_buf[...].reshape(1, D).astype(f32)
        lane = lax.broadcasted_iota(i32, (16, 128), 1)
        for c in range(R // 16):
            p0 = t * R + c * 16
            halves = []
            deps = []
            for h in range(2):
                r0 = h * HP + p0
                xv = x_buf[r0:r0 + 16, :].astype(f32)
                mf = jnp.sum(xv, axis=1, keepdims=True) * (1.0 / D)
                d = xv - mf
                var = jnp.sum(d * d, axis=1, keepdims=True) * (1.0 / D)
                tr = jnp.sum(d * wr, axis=1, keepdims=True)
                rs = lax.rsqrt(var + 1e-5)
                halves.append(d * rs)
                rs = jnp.broadcast_to(rs, (16, 128))
                mf = jnp.broadcast_to(mf, (16, 128))
                sa[r0:r0 + 16, :] = 1.0 + rs
                sb[r0:r0 + 16, :] = mf * rs
                st = jnp.where(lane == 0, mf, jnp.where(lane == 1, jnp.broadcast_to(var, (16, 128)),
                                                        jnp.broadcast_to(tr, (16, 128))))
                stats[r0:r0 + 16, :] = st
                deps += [rs[0:8], rs[8:16], st[0:8], st[8:16]]
            tok(deps)
            x11, x12 = halves[0][:, :HD], halves[0][:, HD:]
            x21, x22 = halves[1][:, :HD], halves[1][:, HD:]
            ops = (x11, x22, x11 + x22, x21 + x22, x11 + x12, x21 - x11, x12 - x22)
            for k in range(7):
                xs.at[k][p0 // 2:p0 // 2 + 8, :] = _pack(ops[k])
            yield

    def wk_prep():
        for c in range(HD // 16):
            r0 = c * 16
            top = wk_buf[r0:r0 + 16, :].astype(f32)
            bot = wk_buf[HD + r0:HD + r0 + 16, :].astype(f32)
            ops = _rform(top[:, :HD], top[:, HD:], bot[:, :HD], bot[:, HD:])
            for k in range(7):
                wks.at[k][r0 // 2:r0 // 2 + 8, :] = _pack(ops[k])

    def wq_prep(tok):
        for g in range(8):
            wt = _pack(wq_buf[:, g * 128:(g + 1) * 128].T)
            for ct in range(8):
                tscr.at[ct][...] = wt[:, ct * 128:(ct + 1) * 128]
            deps = []
            for j in range(4):
                def rows(jj):
                    return _unpack(jnp.concatenate(
                        [tscr[ct, pl.ds(jj, 8, stride=8), :] for ct in range(8)], axis=1)).astype(f32)
                top, bot = rows(j), rows(j + 4)
                w11, w12, w21, w22 = top[:, :HD], top[:, HD:], bot[:, :HD], bot[:, HD:]
                ops = _rform(w11, w21, w12, w22)
                for k in range(7):
                    wqs.at[k][j * 64 + g * 8:j * 64 + g * 8 + 8, :] = _pack(ops[k])
                deps += [ops[5][0:8, 384:512], ops[6][0:8, 384:512]]
            tok(deps)
            yield

    def kproj_tile(t):
        pr = pl.ds(t * (R // 2), R // 2)
        for c in range(4):
            cs = slice(c * 128, (c + 1) * 128)
            m = [mm(_unpack(xs[L_ORD[k], pr, :]), wks[k, :, cs], NN, R) for k in range(7)]
            k11, k12, k21, k22 = [_phi(v) for v in _combine(m)]
            zl = (k11 + k21).reshape(R // 8, 8, 128).sum(axis=0)
            zr = (k12 + k22).reshape(R // 8, 8, 128).sum(axis=0)
            zacc[:, cs] += zl
            zacc[:, HD + c * 128:HD + (c + 1) * 128] += zr
            ops = _lform(k11, k21, k12, k22)
            for k in range(7):
                ps.at[k][pr, cs] = _pack(ops[k])

    def z_prep():
        z = jnp.sum(zacc[...], axis=0, keepdims=True)
        zt = _pack(jnp.broadcast_to(z, (128, D)).astype(bf16).T)
        for g in range(8):
            tscr.at[g][...] = zt[g * 64:(g + 1) * 64, :]
        for j in range(8):
            blk = jnp.concatenate([tscr[g, pl.ds(j, 8, stride=8), :] for g in range(8)], axis=0)
            zp[:, j * 128:(j + 1) * 128] = _unpack(blk).T[0:8, :].astype(f32)

    def route(tok):
        rows = [stats[b * 128:(b + 1) * 128, :].T[0:8, :] for b in range(S // 128)]
        mf = jnp.concatenate([v[0:1] for v in rows], axis=0)
        var = jnp.concatenate([v[1:2] for v in rows], axis=0)
        tr = jnp.concatenate([v[2:3] for v in rows], axis=0)
        wsum = jnp.sum(wr_buf[...].reshape(1, D).astype(f32), axis=1, keepdims=True)
        sd = _rbf(jnp.sqrt(_rbf(_rbf(var) + 1e-5)))
        rv = _rbf((tr + (mf - _rbf(mf)) * wsum) / sd)
        rmax = jnp.max(rv)
        pos = (lax.broadcasted_iota(i32, rv.shape, 0) * 128 + lax.broadcasted_iota(i32, rv.shape, 1))
        idx = jnp.min(jnp.where(rv == rmax, pos, S - 1))
        idx_s[0] = idx
        rsel[...] = jnp.full(rsel.shape, rmax, f32)
        b0 = pl.multiple_of((idx // 16) * 16, 16)
        xn = _rbf(_layernorm_rows(x_buf[pl.ds(b0, 16), :].astype(f32)))
        sel = lax.broadcasted_iota(i32, xn.shape, 0) == idx - b0
        row = jnp.sum(jnp.where(sel, xn, 0.0), axis=0, keepdims=True)
        xbv = jnp.broadcast_to(row, (128, D)).T
        xb[...] = xbv
        yacc[...] = jnp.zeros(yacc.shape, f32)
        tok([xbv[b * 128 + 120:(b + 1) * 128] for b in range(8)])
        yield

    def b_tile(j):
        jc = pl.ds(pl.multiple_of(j * 128, 128), 128)
        pr = pl.ds(pl.multiple_of(j * (R // 2), R // 2), R // 2)
        pq = pq_buf.at[j % 2]
        z_prep()
        m = [mm(_unpack(ps[k, :, jc]), xs[R_ORD[k]], TN, 1024, 4) for k in range(7)]
        g11, g12, g21, g22 = _combine(m)
        hm = (lax.broadcasted_iota(i32, (128, 128), 0) // 32
              == lax.broadcasted_iota(i32, (128, 128), 1) // 32)
        den = [jnp.zeros((R, 128), f32), jnp.zeros((R, 128), f32)]

        def q_chunk(c):
            m = [mm(_unpack(xs[L_ORD[k], pr, :]), wqs[k, c * 64:(c + 1) * 64, :], NT_, R)
                 for k in range(7)]
            q11, q12, q21, q22 = [_phi(v) for v in _combine(m)]
            cl = slice(c * 128, (c + 1) * 128)
            cr = slice(HD + c * 128, HD + (c + 1) * 128)
            zl, zr = zp[0:1, cl], zp[0:1, cr]
            den[0] = den[0] + q11 * zl + q12 * zr
            den[1] = den[1] + q21 * zl + q22 * zr
            pq.at[0][:, cl] = q11
            pq.at[0][:, cr] = q12
            pq.at[1][:, cl] = q21
            pq.at[1][:, cr] = q22
            if c < 3:
                emit_tok([d[i * 8:(i + 1) * 8] for d in den for i in range(R // 8)], clock[0] + QLAG)

        q_chunk(0)
        kvps = []
        for half, (ga, gb) in enumerate(((g11, g12), (g21, g22))):
            gc = pl.ds(pl.multiple_of((j + 4 * half) * 128, 128), 128)
            gg = jnp.concatenate([ga, gb], axis=1).astype(bf16)
            advance(clock[0] + 256)
            clock[0] += 256
            kv = jnp.where(hm, _dot(gg, wv_buf[:, gc], NN), 0.0)
            tscr2.at[half][...] = _pack(kv)
            kvps.append(_unpack(jnp.concatenate(
                [tscr2[half, pl.ds(jj, 8, stride=8), :] for jj in range(8)], axis=0)))
        for c in range(1, 4):
            q_chunk(c)
        for half in range(2):
            g = j + 4 * half
            advance(clock[0] + 256)
            clock[0] += 256
            mg = _dot(kvps[half], wo_buf[pl.ds(pl.multiple_of(g * 128, 128), 128), :], NN)
            ops = _rform(mg[:64, :HD], mg[:64, HD:], mg[64:, :HD], mg[64:, HD:])
            for k in range(7):
                for jj in range(4):
                    ms.at[k][pl.ds(pl.multiple_of(jj * 64 + g * 8, 8), 8), :] = _pack(
                        ops[k][jj * 16:(jj + 1) * 16])
        lane = lax.broadcasted_iota(i32, (R, 128), 1)
        recs = []
        for d in den:
            d = d + jnp.where(lane % 2 == 0, pltpu.roll(d, 127, 1), pltpu.roll(d, 1, 1))
            d = d + jnp.where(lane % 4 < 2, pltpu.roll(d, 126, 1), pltpu.roll(d, 2, 1))
            recs.append(1.0 / (d + 1e-6))
        for c in range(R // 16):
            rs = slice(c * 16, (c + 1) * 16)
            top = pq[0, rs, :] * jnp.concatenate([recs[0][rs]] * 8, axis=1)
            bot = pq[1, rs, :] * jnp.concatenate([recs[1][rs]] * 8, axis=1)
            ops = _lform(top[:, :HD], top[:, HD:], bot[:, :HD], bot[:, HD:])
            p2 = pl.ds(pl.multiple_of(j * (R // 2) + c * 8, 8), 8)
            for k in range(7):
                qs.at[k][p2, :] = _pack(ops[k])

    def out_tile(t, y):
        pr = pl.ds(pl.multiple_of(t * (R // 2), R // 2), R // 2)
        rt = pl.ds(pl.multiple_of(t * R, R), R)
        rb = pl.ds(pl.multiple_of(HP + t * R, R), R)
        row = lax.broadcasted_iota(i32, (R, 256), 0) + t * R
        hit = (row == idx_s[0], row + HP == idx_s[0])
        for c in range(2):
            cl = slice(c * 256, (c + 1) * 256)
            cr = slice(HD + c * 256, HD + (c + 1) * 256)
            m = [_dot(_unpack(qs[k, pr, :]), _unpack(ms[k, :, cl]), NN) for k in range(7)]
            o11, o12, o21, o22 = _combine(m)
            for h, cc, o in ((0, cl, o11), (0, cr, o12), (1, cl, o21), (1, cr, o22)):
                rr = (rt, rb)[h]
                a = jnp.concatenate([sa[rr, :]] * 2, axis=1)
                b = jnp.concatenate([sb[rr, :]] * 2, axis=1)
                o = o + jnp.where(hit[h], y[:, cc], 0.0)
                out_buf[rr, cc] = (x_buf[rr, cc].astype(f32) * a - b + o).astype(bf16)

    def ffn_chunk(c, tok):
        nl = FW // 128
        ag = jnp.zeros((8, FW), f32)
        au = jnp.zeros((8, FW), f32)
        for kg in range(D // 8):
            xv = jnp.concatenate([xb[8 * kg:8 * kg + 8, :]] * nl, axis=1)
            ag = ag + wg_buf[c, 8 * kg:8 * kg + 8, :].astype(f32) * xv
            au = au + wu_buf[c, 8 * kg:8 * kg + 8, :].astype(f32) * xv
            if kg % 4 == 3:
                tok([a[:, i * 128:(i + 1) * 128] for a in (ag, au) for i in range(nl)])
                yield
        g = _rbf(jnp.sum(ag, axis=0, keepdims=True))
        u = _rbf(jnp.sum(au, axis=0, keepdims=True))
        h = _rbf(_rbf(g * jax.nn.sigmoid(g)) * u)
        hb = jnp.broadcast_to(h, (128, FW)).T
        yield
        acc = yacc[...]
        for kg in range(FW // 8):
            hv = jnp.concatenate([hb[8 * kg:8 * kg + 8, :]] * (D // 128), axis=1)
            acc = acc + wd_buf[c, 8 * kg:8 * kg + 8, :].astype(f32) * hv
            if kg % 7 == 6:
                tok([acc[:, i * 128:(i + 1) * 128] for i in range(D // 128)])
                yield
        yacc[...] = acc

    with _scope("p0_issue"):
        cp_wr.start()
        for c in cp_x(0):
            c.start()
        cp_wk.start()
        for t in range(1, NT):
            for c in cp_x(t):
                c.start()
        cp_wq.start()
        for j in range(NT):
            for c in cp_b(j):
                c.start()
        zacc[...] = jnp.zeros(zacc.shape, f32)
        zero_buf[1] = jnp.zeros((8, 128), u32)
        cp_zero = cp(zero_buf.at[1], zero_buf.at[0], SEM_Z)
        cp_zero.start()
        cp_zero.wait()
        cp_wr.wait()
        for c in cp_x(0):
            c.wait()
    with _scope("p1_ln0"):
        for _ in ln_tile(0, lambda v: None):
            pass
    with _scope("p2_waitwk"):
        cp_wk.wait()
    with _scope("p3_wkprep"):
        wk_prep()
    for t in range(NT):
        with _scope("a_wait%d" % t):
            for c in (cp_x(t + 1) if t + 1 < NT else [cp_wq]):
                c.wait()
        with _scope("a_tile%d" % t):
            if t + 1 < NT:
                add_side(lambda tok, t=t: ln_tile(t + 1, tok), R // 16, 300, 28 * R + 300)
            else:
                add_side(wq_prep, 8, 300, 24 * R)
                add_side(route, 1, 0, 10 * R)
            kproj_tile(t)
            finish()

    def b_body(j, carry):
        with _scope("b_wait"):
            for c in cp_b(j, wait_only=True):
                c.wait()
        with _scope("b_body"):
            add_side(lambda tok: ffn_chunk(j, tok), 32 + 1 + 16, 200, 14000)
            b_tile(j)
            finish()
        return carry

    lax.fori_loop(0, NT, b_body, 0)

    def c_body(t, carry):
        with _scope("c_body"):
            y = _rbf(jnp.sum(yacc[...], axis=0, keepdims=True))
            y = _rbf(y * _rbf(jax.nn.sigmoid(rsel[...])))
            out_tile(t, y)
            cp_out(t, 0).start()
            cp_out(t, 1).start()
        return carry

    lax.fori_loop(0, NT, c_body, 0)
    with _scope("tail"):
        for t in range(NT):
            cp_out(t, 0).wait()
            cp_out(t, 1).wait()


@jax.jit
def pallas_parallel_sum__linear_attn_block__moe_arch_mod__prompt_kernel(
    A_x: jax.Array,
    A_wqkv: jax.Array,
    A_wo: jax.Array,
    B_x: jax.Array,
    B_w_r: jax.Array,
    B_w_gate: jax.Array,
    B_w_up: jax.Array,
    B_w_down: jax.Array,
):
    del B_x
    V = pltpu.VMEM
    scratch = [
        V((S, D), bf16),
        V((D, D), bf16),
        V((D, D), bf16),
        V((D, D), bf16),
        V((D, D), bf16),
        V((D,), bf16),
        V((NF, D, FW), bf16),
        V((NF, D, FW), bf16),
        V((NF, FW, D), bf16),
        V((7, HP // 2, HD), u32),
        V((7, HP // 2, HD), u32),
        V((7, HP // 2, HD), u32),
        V((7, HD // 2, HD), u32),
        V((7, HD // 2, HD), u32),
        V((7, HD // 2, HD), u32),
        V((S, 128), f32),
        V((S, 128), f32),
        V((S, 128), f32),
        V((8, D), f32),
        V((8, D), f32),
        V((8, 64, 128), u32),
        V((2, 64, 128), u32),
        V((2, 2, R, D), f32),
        V((D, 128), f32),
        V((8, D), f32),
        V((1, D), f32),
        V((S, D), bf16),
        V((2, 8, 128), u32),
        pltpu.SMEM((1,), i32),
        pltpu.SemaphoreType.DMA((2 * NT + 4,)),
    ]
    return pl.pallas_call(
        _kernel,
        out_shape=jax.ShapeDtypeStruct((1, S, D), bf16),
        in_specs=[pl.BlockSpec(memory_space=pl.ANY)] * 7,
        out_specs=pl.BlockSpec(memory_space=pl.ANY),
        scratch_shapes=scratch,
        compiler_params=pltpu.CompilerParams(vmem_limit_bytes=110 * 1024 * 1024),
    )(A_x, A_wqkv, A_wo, B_w_r, B_w_gate, B_w_up, B_w_down)
```

```python
import contextlib

import jax
import jax.numpy as jnp
from jax import lax
import jax.experimental.pallas as pl
import jax.experimental.pallas.tpu as pltpu

bf16, f32, u32, i32 = jnp.bfloat16, jnp.float32, jnp.uint32, jnp.int32

S = 2048
D = 1024
F = 3584
HP = S // 2
HD = D // 2
R = 256
NT = HP // R
FW = 896
NF = F // FW
QLAG = 768
QA = 192
CR = 128

L_ORD = (2, 3, 0, 1, 4, 5, 6)
R_ORD = (2, 0, 6, 5, 1, 4, 3)

NN = (((1,), (0,)), ((), ()))
NT_ = (((1,), (1,)), ((), ()))
TN = (((0,), (0,)), ((), ()))


SCOPES = False


def _scope(name):
    return jax.named_scope(name) if SCOPES else contextlib.nullcontext()


def _dot(a, b, dims):
    return lax.dot_general(a, b, dims, preferred_element_type=f32)


def _pack(v):
    return pltpu.bitcast(v.astype(bf16), u32)


def _unpack(v):
    return pltpu.bitcast(v, bf16)


def _combine(m):
    m1, m2, m3, m4, m5, m6, m7 = m
    return m1 + m4 - m5 + m7, m3 + m5, m2 + m4, m1 - m2 + m3 + m6


def _lform(a11, a12, a21, a22):
    return (a11 + a22, a21 + a22, a11, a22, a11 + a12, a21 - a11, a12 - a22)


def _rform(b11, b12, b21, b22):
    return (b11 + b22, b11, b12 - b22, b21 - b11, b22, b11 + b12, b21 + b22)


def _phi(t):
    return jnp.where(t > 0, t + 1.0, jnp.exp(t)) + 1e-6


def _rbf(v):
    return v.astype(bf16).astype(f32)


def _layernorm_rows(xv):
    mf = jnp.sum(xv, axis=1, keepdims=True) * (1.0 / D)
    mb = _rbf(mf)
    d = xv - mb
    dm = mf - mb
    var = jnp.sum(d * d, axis=1, keepdims=True) * (1.0 / D) - dm * dm
    var = jnp.maximum(var, 0.0)
    sd = _rbf(jnp.sqrt(_rbf(_rbf(var) + 1e-5)))
    return d * (1.0 / sd)


def _kernel(x_hbm, wqkv_hbm, wo_hbm, wr_hbm, wg_hbm, wu_hbm, wd_hbm, out_hbm,
            x_buf, wk_buf, wq_buf, wv_buf, wo_buf, wr_buf, wg_buf, wu_buf, wd_buf,
            xs, ps, qs, wks, wqs, ms, sa, sb, stats, zacc, zp, tscr, tscr2, pq_buf,
            xb, yacc, rsel, out_buf, zero_buf, idx_s, sem):

    SEM_X, SEM_WK, SEM_WQ, SEM_B, SEM_O, SEM_Z = 0, NT, NT + 1, NT + 2, 2 * NT + 2, 2 * NT + 3

    def cp(src, dst, s):
        return pltpu.make_async_copy(src, dst, sem.at[s])

    def cp_x(t):
        return [cp(x_hbm.at[0, pl.ds(h * HP + t * R, R), :], x_buf.at[pl.ds(h * HP + t * R, R), :],
                   SEM_X + t) for h in range(2)]

    cp_wr = cp(wr_hbm, wr_buf, SEM_X)
    cp_wk = cp(wqkv_hbm.at[:, pl.ds(D, D)], wk_buf, SEM_WK)
    cp_wq = cp(wqkv_hbm.at[:, pl.ds(0, D)], wq_buf, SEM_WQ)

    def cp_b(j, wait_only=False):
        def off(v, m):
            return v if isinstance(v, int) else pl.multiple_of(v, m)
        out = []
        for g in (j, j + 4):
            c0 = off(g * 128, 128)
            dst = wv_buf.at[:, pl.ds(c0, 128)]
            out.append(cp(dst if wait_only else wqkv_hbm.at[:, pl.ds(2 * D + c0, 128)], dst, SEM_B + j))
            dst = wo_buf.at[pl.ds(c0, 128), :]
            out.append(cp(dst if wait_only else wo_hbm.at[pl.ds(c0, 128), :], dst, SEM_B + j))
        f0 = off(j * FW, 128)
        for src, dst in ((wg_hbm.at[:, pl.ds(f0, FW)], wg_buf.at[j]),
                         (wu_hbm.at[:, pl.ds(f0, FW)], wu_buf.at[j]),
                         (wd_hbm.at[pl.ds(f0, FW), :], wd_buf.at[j])):
            out.append(cp(dst if wait_only else src, dst, SEM_B + j))
        return out

    clock = [0]
    toks = []
    sides = []

    def emit_tok(vals, stamp=None):
        t = None
        for v in vals:
            v = pltpu.bitcast(v, u32) if v.dtype != u32 else v
            t = v if t is None else t | v
        toks.append((clock[0] if stamp is None else stamp, t & zero_buf[0]))

    def add_side(gen_fn, n, t0, t1):
        st = {"i": 0, "n": n, "t0": clock[0] + t0, "t1": clock[0] + t1}
        st["g"] = gen_fn(lambda vals: emit_tok(
            vals, st["t0"] + (st["i"] + 1) * (st["t1"] - st["t0"]) // st["n"]))
        sides.append(st)

    def advance(until):
        for st in sides:
            while st["i"] < st["n"] and st["t0"] + st["i"] * (st["t1"] - st["t0"]) // st["n"] < until:
                next(st["g"], None)
                st["i"] += 1

    def finish():
        for st in sides:
            for _ in st["g"]:
                pass
        sides.clear()
        toks.clear()

    def mm(lhs, rhs, dims, cycles, nseg=1):
        advance(clock[0] + cycles)
        segs = []
        w = rhs.shape[1] // nseg
        for s in range(nseg):
            now = clock[0] + s * cycles // nseg
            due = [t for (c, t) in toks if c <= now]
            toks[:] = [(c, t) for (c, t) in toks if c > now]
            head = rhs[0:8, s * w:s * w + 128]
            for t in due:
                head = head | t
            segs.append(head)
            if w > 128:
                segs.append(rhs[0:8, s * w + 128:(s + 1) * w])
        rhs = jnp.concatenate([jnp.concatenate(segs, axis=1), rhs[8:]], axis=0)
        clock[0] += cycles
        return _dot(lhs, _unpack(rhs), dims)

    def ln_tile(t, tok):
        wr = wr_buf[...].reshape(1, D).astype(f32)
        lane = lax.broadcasted_iota(i32, (16, 128), 1)
        for c in range(R // 16):
            p0 = t * R + c * 16
            halves = []
            deps = []
            for h in range(2):
                r0 = h * HP + p0
                xv = x_buf[r0:r0 + 16, :].astype(f32)
                mf = jnp.sum(xv, axis=1, keepdims=True) * (1.0 / D)
                d = xv - mf
                var = jnp.sum(d * d, axis=1, keepdims=True) * (1.0 / D)
                tr = jnp.sum(d * wr, axis=1, keepdims=True)
                rs = lax.rsqrt(var + 1e-5)
                halves.append(d * rs)
                rs = jnp.broadcast_to(rs, (16, 128))
                mf = jnp.broadcast_to(mf, (16, 128))
                sa[r0:r0 + 16, :] = 1.0 + rs
                sb[r0:r0 + 16, :] = mf * rs
                st = jnp.where(lane == 0, mf, jnp.where(lane == 1, jnp.broadcast_to(var, (16, 128)),
                                                        jnp.broadcast_to(tr, (16, 128))))
                stats[r0:r0 + 16, :] = st
                deps += [rs[0:8], rs[8:16], st[0:8], st[8:16]]
            tok(deps)
            x11, x12 = halves[0][:, :HD], halves[0][:, HD:]
            x21, x22 = halves[1][:, :HD], halves[1][:, HD:]
            ops = (x11, x22, x11 + x22, x21 + x22, x11 + x12, x21 - x11, x12 - x22)
            for k in range(7):
                xs.at[k][p0 // 2:p0 // 2 + 8, :] = _pack(ops[k])
            yield

    def wk_prep():
        for c in range(HD // 16):
            r0 = c * 16
            top = wk_buf[r0:r0 + 16, :].astype(f32)
            bot = wk_buf[HD + r0:HD + r0 + 16, :].astype(f32)
            ops = _rform(top[:, :HD], top[:, HD:], bot[:, :HD], bot[:, HD:])
            for k in range(7):
                wks.at[k][r0 // 2:r0 // 2 + 8, :] = _pack(ops[k])

    def wq_prep(tok):
        for g in range(8):
            wt = _pack(wq_buf[:, g * 128:(g + 1) * 128].T)
            for ct in range(8):
                tscr.at[ct][...] = wt[:, ct * 128:(ct + 1) * 128]
            deps = []
            for j in range(4):
                def rows(jj):
                    return _unpack(jnp.concatenate(
                        [tscr[ct, pl.ds(jj, 8, stride=8), :] for ct in range(8)], axis=1)).astype(f32)
                top, bot = rows(j), rows(j + 4)
                w11, w12, w21, w22 = top[:, :HD], top[:, HD:], bot[:, :HD], bot[:, HD:]
                ops = _rform(w11, w21, w12, w22)
                for k in range(7):
                    wqs.at[k][j * 64 + g * 8:j * 64 + g * 8 + 8, :] = _pack(ops[k])
                deps += [ops[5][0:8, 384:512], ops[6][0:8, 384:512]]
            tok(deps)
            yield

    def kproj_tile(t):
        pr = pl.ds(t * (R // 2), R // 2)
        for c in range(4):
            cs = slice(c * 128, (c + 1) * 128)
            m = [mm(_unpack(xs[L_ORD[k], pr, :]), wks[k, :, cs], NN, R) for k in range(7)]
            k11, k12, k21, k22 = [_phi(v) for v in _combine(m)]
            zl = (k11 + k21).reshape(R // 8, 8, 128).sum(axis=0)
            zr = (k12 + k22).reshape(R // 8, 8, 128).sum(axis=0)
            zacc[:, cs] += zl
            zacc[:, HD + c * 128:HD + (c + 1) * 128] += zr
            ops = _lform(k11, k21, k12, k22)
            for k in range(7):
                ps.at[k][pr, cs] = _pack(ops[k])

    def z_prep():
        z = jnp.sum(zacc[...], axis=0, keepdims=True)
        zt = _pack(jnp.broadcast_to(z, (128, D)).astype(bf16).T)
        for g in range(8):
            tscr.at[g][...] = zt[g * 64:(g + 1) * 64, :]
        for j in range(8):
            blk = jnp.concatenate([tscr[g, pl.ds(j, 8, stride=8), :] for g in range(8)], axis=0)
            zp[:, j * 128:(j + 1) * 128] = _unpack(blk).T[0:8, :].astype(f32)

    def route(tok):
        rows = [stats[b * 128:(b + 1) * 128, :].T[0:8, :] for b in range(S // 128)]
        mf = jnp.concatenate([v[0:1] for v in rows], axis=0)
        var = jnp.concatenate([v[1:2] for v in rows], axis=0)
        tr = jnp.concatenate([v[2:3] for v in rows], axis=0)
        wsum = jnp.sum(wr_buf[...].reshape(1, D).astype(f32), axis=1, keepdims=True)
        sd = _rbf(jnp.sqrt(_rbf(_rbf(var) + 1e-5)))
        rv = _rbf((tr + (mf - _rbf(mf)) * wsum) / sd)
        rmax = jnp.max(rv)
        pos = (lax.broadcasted_iota(i32, rv.shape, 0) * 128 + lax.broadcasted_iota(i32, rv.shape, 1))
        idx = jnp.min(jnp.where(rv == rmax, pos, S - 1))
        idx_s[0] = idx
        rsel[...] = jnp.full(rsel.shape, rmax, f32)
        b0 = pl.multiple_of((idx // 16) * 16, 16)
        xn = _rbf(_layernorm_rows(x_buf[pl.ds(b0, 16), :].astype(f32)))
        sel = lax.broadcasted_iota(i32, xn.shape, 0) == idx - b0
        row = jnp.sum(jnp.where(sel, xn, 0.0), axis=0, keepdims=True)
        xbv = jnp.broadcast_to(row, (128, D)).T
        xb[...] = xbv
        yacc[...] = jnp.zeros(yacc.shape, f32)
        tok([xbv[b * 128 + 120:(b + 1) * 128] for b in range(8)])
        yield

    def q_part(j, r0, nr):
        pr = pl.ds(pl.multiple_of((j * R + r0) // 2, 8), nr // 2)
        pq = pq_buf.at[j % 2]
        rr = slice(r0, r0 + nr)
        den = [None, None]
        for c in range(4):
            m = [mm(_unpack(xs[L_ORD[k], pr, :]), wqs[k, c * 64:(c + 1) * 64, :], NT_, nr)
                 for k in range(7)]
            q11, q12, q21, q22 = [_phi(v) for v in _combine(m)]
            cl = slice(c * 128, (c + 1) * 128)
            cr = slice(HD + c * 128, HD + (c + 1) * 128)
            zl, zr = zp[0:1, cl], zp[0:1, cr]
            dt, db = q11 * zl + q12 * zr, q21 * zl + q22 * zr
            den = [dt, db] if c == 0 else [den[0] + dt, den[1] + db]
            pq.at[0][rr, cl] = q11
            pq.at[0][rr, cr] = q12
            pq.at[1][rr, cl] = q21
            pq.at[1][rr, cr] = q22
            if c < 3:
                emit_tok([d[i * 8:(i + 1) * 8] for d in den for i in range(nr // 8)], clock[0] + QLAG)
                yield
        lane = lax.broadcasted_iota(i32, (nr, 128), 1)
        recs = []
        for d in den:
            d = d + jnp.where(lane % 2 == 0, pltpu.roll(d, 127, 1), pltpu.roll(d, 1, 1))
            d = d + jnp.where(lane % 4 < 2, pltpu.roll(d, 126, 1), pltpu.roll(d, 2, 1))
            recs.append(1.0 / (d + 1e-6))
        for c in range(nr // 16):
            rs = slice(c * 16, (c + 1) * 16)
            rq = slice(r0 + c * 16, r0 + (c + 1) * 16)
            top = pq[0, rq, :] * jnp.concatenate([recs[0][rs]] * 8, axis=1)
            bot = pq[1, rq, :] * jnp.concatenate([recs[1][rs]] * 8, axis=1)
            ops = _lform(top[:, :HD], top[:, HD:], bot[:, :HD], bot[:, HD:])
            p2 = pl.ds(pl.multiple_of((j * R + r0) // 2 + c * 8, 8), 8)
            for k in range(7):
                qs.at[k][p2, :] = _pack(ops[k])
            emit_tok([ops[0][0:8, 0:128], ops[0][8:16, 0:128]], clock[0] + QLAG + 128 * c)
        yield

    def b_tile(j):
        jc = pl.ds(pl.multiple_of(j * 128, 128), 128)
        z_prep()
        for _ in q_part(j, 0, QA):
            pass
        m = [mm(_unpack(ps[k, :, jc]), xs[R_ORD[k]], TN, 1024, 4) for k in range(7)]
        g11, g12, g21, g22 = _combine(m)
        hm = (lax.broadcasted_iota(i32, (128, 128), 0) // 32
              == lax.broadcasted_iota(i32, (128, 128), 1) // 32)
        qb = q_part(j, QA, R - QA)
        next(qb)
        kvps = []
        for half, (ga, gb) in enumerate(((g11, g12), (g21, g22))):
            gc = pl.ds(pl.multiple_of((j + 4 * half) * 128, 128), 128)
            gg = jnp.concatenate([ga, gb], axis=1).astype(bf16)
            advance(clock[0] + 256)
            clock[0] += 256
            kv = jnp.where(hm, _dot(gg, wv_buf[:, gc], NN), 0.0)
            tscr2.at[half][...] = _pack(kv)
            kvps.append(_unpack(jnp.concatenate(
                [tscr2[half, pl.ds(jj, 8, stride=8), :] for jj in range(8)], axis=0)))
        for _ in qb:
            pass
        for half in range(2):
            g = j + 4 * half
            advance(clock[0] + 256)
            clock[0] += 256
            mg = _dot(kvps[half], wo_buf[pl.ds(pl.multiple_of(g * 128, 128), 128), :], NN)
            ops = _rform(mg[:64, :HD], mg[:64, HD:], mg[64:, :HD], mg[64:, HD:])
            for k in range(7):
                for jj in range(4):
                    ms.at[k][pl.ds(pl.multiple_of(jj * 64 + g * 8, 8), 8), :] = _pack(
                        ops[k][jj * 16:(jj + 1) * 16])

    def out_part(p0, nr, y):
        pr = pl.ds(pl.multiple_of(p0 // 2, 8), nr // 2)
        rows = (pl.ds(pl.multiple_of(p0, 16), nr), pl.ds(pl.multiple_of(HP + p0, 16), nr))
        row = lax.broadcasted_iota(i32, (nr, 256), 0) + p0
        hit = (row == idx_s[0], row + HP == idx_s[0])
        for c in range(2):
            cl = pl.ds(c * 256, 256)
            cr = pl.ds(HD + c * 256, 256)
            m = [_dot(_unpack(qs[k, pr, :]), _unpack(ms[k, :, cl]), NN) for k in range(7)]
            o11, o12, o21, o22 = _combine(m)
            for h, cc, o in ((1, cr, o22), (1, cl, o21), (0, cr, o12), (0, cl, o11)):
                rr = rows[h]
                a = jnp.concatenate([sa[rr, :]] * 2, axis=1)
                b = jnp.concatenate([sb[rr, :]] * 2, axis=1)
                o = o + jnp.where(hit[h], y[:, cc.start:cc.start + 256], 0.0)
                out_buf[rr, cc] = (x_buf[rr, cc].astype(f32) * a - b + o).astype(bf16)
                cp(out_buf.at[rr, cc], out_hbm.at[0, rr, cc], SEM_O).start()

    def ffn_chunk(c, tok):
        nl = FW // 128
        ag = jnp.zeros((8, FW), f32)
        au = jnp.zeros((8, FW), f32)
        for kg in range(D // 8):
            xv = jnp.concatenate([xb[8 * kg:8 * kg + 8, :]] * nl, axis=1)
            ag = ag + wg_buf[c, 8 * kg:8 * kg + 8, :].astype(f32) * xv
            au = au + wu_buf[c, 8 * kg:8 * kg + 8, :].astype(f32) * xv
            if kg % 4 == 3:
                tok([a[:, i * 128:(i + 1) * 128] for a in (ag, au) for i in range(nl)])
                yield
        g = _rbf(jnp.sum(ag, axis=0, keepdims=True))
        u = _rbf(jnp.sum(au, axis=0, keepdims=True))
        h = _rbf(_rbf(g * jax.nn.sigmoid(g)) * u)
        hb = jnp.broadcast_to(h, (128, FW)).T
        yield
        acc = yacc[...]
        for kg in range(FW // 8):
            hv = jnp.concatenate([hb[8 * kg:8 * kg + 8, :]] * (D // 128), axis=1)
            acc = acc + wd_buf[c, 8 * kg:8 * kg + 8, :].astype(f32) * hv
            if kg % 7 == 6:
                tok([acc[:, i * 128:(i + 1) * 128] for i in range(D // 128)])
                yield
        yacc[...] = acc

    with _scope("p0_issue"):
        cp_wr.start()
        for c in cp_x(0):
            c.start()
        cp_wk.start()
        for t in range(1, NT):
            for c in cp_x(t):
                c.start()
        cp_wq.start()
        for j in range(NT):
            for c in cp_b(j):
                c.start()
        zacc[...] = jnp.zeros(zacc.shape, f32)
        zero_buf[1] = jnp.zeros((8, 128), u32)
        cp_zero = cp(zero_buf.at[1], zero_buf.at[0], SEM_Z)
        cp_zero.start()
        cp_zero.wait()
        cp_wr.wait()
        for c in cp_x(0):
            c.wait()
    with _scope("p1_ln0"):
        for _ in ln_tile(0, lambda v: None):
            pass
    with _scope("p2_waitwk"):
        cp_wk.wait()
    with _scope("p3_wkprep"):
        wk_prep()
    for t in range(NT):
        with _scope("a_wait%d" % t):
            for c in (cp_x(t + 1) if t + 1 < NT else [cp_wq]):
                c.wait()
        with _scope("a_tile%d" % t):
            if t + 1 < NT:
                add_side(lambda tok, t=t: ln_tile(t + 1, tok), R // 16, 300, 28 * R + 300)
            else:
                add_side(wq_prep, 8, 300, 24 * R)
                add_side(route, 1, 0, 10 * R)
            kproj_tile(t)
            finish()

    def b_body(j, carry):
        with _scope("b_wait"):
            for c in cp_b(j, wait_only=True):
                c.wait()
        with _scope("b_body"):
            add_side(lambda tok: ffn_chunk(j, tok), 32 + 1 + 16, 200, 14000)
            b_tile(j)
            finish()
        return carry

    lax.fori_loop(0, NT, b_body, 0)

    def c_body(t, carry):
        with _scope("c_body"):
            y = _rbf(jnp.sum(yacc[...], axis=0, keepdims=True))
            y = _rbf(y * _rbf(jax.nn.sigmoid(rsel[...])))
            for p in range(R // CR):
                out_part(t * R + p * CR, CR, y)
        return carry

    lax.fori_loop(0, NT, c_body, 0)
    with _scope("tail"):
        cp(out_buf, out_hbm.at[0], SEM_O).wait()


@jax.jit
def pallas_parallel_sum__linear_attn_block__moe_arch_mod__prompt_kernel(
    A_x: jax.Array,
    A_wqkv: jax.Array,
    A_wo: jax.Array,
    B_x: jax.Array,
    B_w_r: jax.Array,
    B_w_gate: jax.Array,
    B_w_up: jax.Array,
    B_w_down: jax.Array,
):
    del B_x
    V = pltpu.VMEM
    scratch = [
        V((S, D), bf16),
        V((D, D), bf16),
        V((D, D), bf16),
        V((D, D), bf16),
        V((D, D), bf16),
        V((D,), bf16),
        V((NF, D, FW), bf16),
        V((NF, D, FW), bf16),
        V((NF, FW, D), bf16),
        V((7, HP // 2, HD), u32),
        V((7, HP // 2, HD), u32),
        V((7, HP // 2, HD), u32),
        V((7, HD // 2, HD), u32),
        V((7, HD // 2, HD), u32),
        V((7, HD // 2, HD), u32),
        V((S, 128), f32),
        V((S, 128), f32),
        V((S, 128), f32),
        V((8, D), f32),
        V((8, D), f32),
        V((8, 64, 128), u32),
        V((2, 64, 128), u32),
        V((2, 2, R, D), f32),
        V((D, 128), f32),
        V((8, D), f32),
        V((1, D), f32),
        V((S, D), bf16),
        V((2, 8, 128), u32),
        pltpu.SMEM((1,), i32),
        pltpu.SemaphoreType.DMA((2 * NT + 4,)),
    ]
    return pl.pallas_call(
        _kernel,
        out_shape=jax.ShapeDtypeStruct((1, S, D), bf16),
        in_specs=[pl.BlockSpec(memory_space=pl.ANY)] * 7,
        out_specs=pl.BlockSpec(memory_space=pl.ANY),
        scratch_shapes=scratch,
        compiler_params=pltpu.CompilerParams(vmem_limit_bytes=110 * 1024 * 1024,
                                             disable_bounds_checks=True,
                                             disable_semaphore_checks=True),
    )(A_x, A_wqkv, A_wo, B_w_r, B_w_gate, B_w_up, B_w_down)
```

```python
import contextlib

import jax
import jax.numpy as jnp
from jax import lax
import jax.experimental.pallas as pl
import jax.experimental.pallas.tpu as pltpu

bf16, f32, u32, i32 = jnp.bfloat16, jnp.float32, jnp.uint32, jnp.int32

S = 2048
D = 1024
F = 3584
HP = S // 2
HD = D // 2
R = 256
NT = HP // R
FW = 896
NF = F // FW
QLAG = 768
QA = 192
FSTEP = 2
CR = 128

L_ORD = (2, 3, 0, 1, 4, 5, 6)
R_ORD = (2, 0, 6, 5, 1, 4, 3)

NN = (((1,), (0,)), ((), ()))
NT_ = (((1,), (1,)), ((), ()))
TN = (((0,), (0,)), ((), ()))


SCOPES = False


def _scope(name):
    return jax.named_scope(name) if SCOPES else contextlib.nullcontext()


def _dot(a, b, dims):
    return lax.dot_general(a, b, dims, preferred_element_type=f32)


def _pack(v):
    return pltpu.bitcast(v.astype(bf16), u32)


def _unpack(v):
    return pltpu.bitcast(v, bf16)


def _combine(m):
    m1, m2, m3, m4, m5, m6, m7 = m
    return m1 + m4 - m5 + m7, m3 + m5, m2 + m4, m1 - m2 + m3 + m6


def _lform(a11, a12, a21, a22):
    return (a11 + a22, a21 + a22, a11, a22, a11 + a12, a21 - a11, a12 - a22)


def _rform(b11, b12, b21, b22):
    return (b11 + b22, b11, b12 - b22, b21 - b11, b22, b11 + b12, b21 + b22)


def _phi(t):
    return jnp.where(t > 0, t + 1.0, jnp.exp(t)) + 1e-6


def _rbf(v):
    return v.astype(bf16).astype(f32)


def _layernorm_rows(xv):
    mf = jnp.sum(xv, axis=1, keepdims=True) * (1.0 / D)
    mb = _rbf(mf)
    d = xv - mb
    dm = mf - mb
    var = jnp.sum(d * d, axis=1, keepdims=True) * (1.0 / D) - dm * dm
    var = jnp.maximum(var, 0.0)
    sd = _rbf(jnp.sqrt(_rbf(_rbf(var) + 1e-5)))
    return d * (1.0 / sd)


def _kernel(x_hbm, wqkv_hbm, wo_hbm, wr_hbm, wg_hbm, wu_hbm, wd_hbm, out_hbm,
            x_buf, wk_buf, wq_buf, wv_buf, wo_buf, wr_buf, wg_buf, wu_buf, wd_buf,
            xs, ps, qs, wks, wqs, ms, sa, sb, stats, zacc, zp, tscr, tscr2, pq_buf,
            xb, hb_buf, yacc, rsel, out_buf, zero_buf, idx_s, sem):

    SEM_X, SEM_WK, SEM_WQ, SEM_B, SEM_O, SEM_Z = 0, NT, NT + 1, NT + 2, 2 * NT + 2, 2 * NT + 3

    def cp(src, dst, s):
        return pltpu.make_async_copy(src, dst, sem.at[s])

    def cp_x(t):
        return [cp(x_hbm.at[0, pl.ds(h * HP + t * R, R), :], x_buf.at[pl.ds(h * HP + t * R, R), :],
                   SEM_X + t) for h in range(2)]

    cp_wr = cp(wr_hbm, wr_buf, SEM_X)
    cp_wk = cp(wqkv_hbm.at[:, pl.ds(D, D)], wk_buf, SEM_WK)
    cp_wq = cp(wqkv_hbm.at[:, pl.ds(0, D)], wq_buf, SEM_WQ)

    def cp_b(j, wait_only=False):
        def off(v, m):
            return v if isinstance(v, int) else pl.multiple_of(v, m)
        out = []
        for g in (j, j + 4):
            c0 = off(g * 128, 128)
            dst = wv_buf.at[:, pl.ds(c0, 128)]
            out.append(cp(dst if wait_only else wqkv_hbm.at[:, pl.ds(2 * D + c0, 128)], dst, SEM_B + j))
            dst = wo_buf.at[pl.ds(c0, 128), :]
            out.append(cp(dst if wait_only else wo_hbm.at[pl.ds(c0, 128), :], dst, SEM_B + j))
        f0 = off(j * FW, 128)
        for src, dst in ((wg_hbm.at[:, pl.ds(f0, FW)], wg_buf.at[j]),
                         (wu_hbm.at[:, pl.ds(f0, FW)], wu_buf.at[j]),
                         (wd_hbm.at[pl.ds(f0, FW), :], wd_buf.at[j])):
            out.append(cp(dst if wait_only else src, dst, SEM_B + j))
        return out

    clock = [0]
    toks = []
    sides = []
    fwd = [None]

    def emit_tok(vals, stamp=None):
        t = None
        for v in vals:
            v = pltpu.bitcast(v, u32) if v.dtype != u32 else v
            t = v if t is None else t | v
        toks.append((clock[0] if stamp is None else stamp, t & zero_buf[0]))

    def gate(v):
        if fwd[0] is None:
            return v
        if fwd[0][1] is None:
            fwd[0][1] = pltpu.bitcast(fwd[0][0](), u32) & zero_buf[0]
        return pltpu.bitcast(pltpu.bitcast(v, u32) | fwd[0][1], f32)

    def add_side(gen_fn, n, t0, t1, lag=None):
        st = {"i": 0, "n": n, "t0": clock[0] + t0, "t1": clock[0] + t1}

        def tok(vals):
            if lag is not None:
                emit_tok(vals, st["t0"] + (st["i"] + 1) * (st["t1"] - st["t0"]) // st["n"] + lag)
        st["g"] = gen_fn(tok)
        sides.append(st)

    def advance(until):
        for st in sides:
            while st["i"] < st["n"] and st["t0"] + st["i"] * (st["t1"] - st["t0"]) // st["n"] < until:
                next(st["g"], None)
                st["i"] += 1

    def finish():
        for st in sides:
            for _ in st["g"]:
                pass
        sides.clear()
        toks.clear()
        fwd[0] = None

    def mm(lhs, rhs, dims, cycles, nseg=1):
        due = [t for (c, t) in toks if c <= clock[0]]
        toks[:] = [(c, t) for (c, t) in toks if c > clock[0]]
        if due:
            head = rhs[0:8, 0:128]
            for t in due:
                head = head | t
            if rhs.shape[1] > 128:
                head = jnp.concatenate([head, rhs[0:8, 128:]], axis=1)
            rhs = jnp.concatenate([head, rhs[8:]], axis=0)
        res = _dot(lhs, _unpack(rhs), dims)
        ngr = res.shape[0] // 16
        for sg in range(nseg):
            for i in range(ngr):
                fwd[0] = [lambda sg=sg, i=i: res[i * 16:i * 16 + 8, sg * 128:(sg + 1) * 128], None]
                clock[0] += cycles // nseg // ngr
                advance(clock[0])
        return res

    def ln_tile(t, tok):
        wr = wr_buf[...].reshape(1, D).astype(f32)
        lane = lax.broadcasted_iota(i32, (16, 128), 1)
        for c in range(R // 16):
            p0 = t * R + c * 16
            halves = []
            deps = []
            for h in range(2):
                r0 = h * HP + p0
                xv = x_buf[r0:r0 + 16, :].astype(f32)
                xg = jnp.concatenate(
                    [jnp.concatenate([gate(xv[0:8, 0:128]), gate(xv[8:16, 0:128])], axis=0), xv[:, 128:]],
                    axis=1)
                mf = jnp.sum(xg, axis=1, keepdims=True) * (1.0 / D)
                d = xv - mf
                var = jnp.sum(d * d, axis=1, keepdims=True) * (1.0 / D)
                tr = jnp.sum(d * wr, axis=1, keepdims=True)
                rs = lax.rsqrt(var + 1e-5)
                halves.append(d * rs)
                rs = jnp.broadcast_to(rs, (16, 128))
                mf = jnp.broadcast_to(mf, (16, 128))
                sa[r0:r0 + 16, :] = 1.0 + rs
                sb[r0:r0 + 16, :] = mf * rs
                st = jnp.where(lane == 0, mf, jnp.where(lane == 1, jnp.broadcast_to(var, (16, 128)),
                                                        jnp.broadcast_to(tr, (16, 128))))
                stats[r0:r0 + 16, :] = st
                deps += [rs[0:8], rs[8:16], st[0:8], st[8:16]]
            tok(deps)
            x11, x12 = halves[0][:, :HD], halves[0][:, HD:]
            x21, x22 = halves[1][:, :HD], halves[1][:, HD:]
            ops = (x11, x22, x11 + x22, x21 + x22, x11 + x12, x21 - x11, x12 - x22)
            for k in range(7):
                xs.at[k][p0 // 2:p0 // 2 + 8, :] = _pack(ops[k])
            yield

    def wk_prep():
        for c in range(HD // 16):
            r0 = c * 16
            top = wk_buf[r0:r0 + 16, :].astype(f32)
            bot = wk_buf[HD + r0:HD + r0 + 16, :].astype(f32)
            ops = _rform(top[:, :HD], top[:, HD:], bot[:, :HD], bot[:, HD:])
            for k in range(7):
                wks.at[k][r0 // 2:r0 // 2 + 8, :] = _pack(ops[k])

    def wq_prep(tok):
        for g in range(8):
            wt = _pack(wq_buf[:, g * 128:(g + 1) * 128].T)
            for ct in range(8):
                tscr.at[ct][...] = wt[:, ct * 128:(ct + 1) * 128]
            deps = []
            for j in range(4):
                def rows(jj):
                    return _unpack(jnp.concatenate(
                        [tscr[ct, pl.ds(jj, 8, stride=8), :] for ct in range(8)], axis=1)).astype(f32)
                top, bot = rows(j), rows(j + 4)
                w11, w12, w21, w22 = top[:, :HD], top[:, HD:], bot[:, :HD], bot[:, HD:]
                ops = _rform(w11, w21, w12, w22)
                for k in range(7):
                    wqs.at[k][j * 64 + g * 8:j * 64 + g * 8 + 8, :] = _pack(ops[k])
                deps += [ops[5][0:8, 384:512], ops[6][0:8, 384:512]]
            tok(deps)
            yield

    def kproj_tile(t):
        pr = pl.ds(t * (R // 2), R // 2)
        for c in range(4):
            cs = slice(c * 128, (c + 1) * 128)
            m = [mm(_unpack(xs[L_ORD[k], pr, :]), wks[k, :, cs], NN, R) for k in range(7)]
            k11, k12, k21, k22 = [_phi(v) for v in _combine(m)]
            zl = (k11 + k21).reshape(R // 8, 8, 128).sum(axis=0)
            zr = (k12 + k22).reshape(R // 8, 8, 128).sum(axis=0)
            zacc[:, cs] += zl
            zacc[:, HD + c * 128:HD + (c + 1) * 128] += zr
            ops = _lform(k11, k21, k12, k22)
            for k in range(7):
                ps.at[k][pr, cs] = _pack(ops[k])

    def z_prep():
        z = jnp.sum(zacc[...], axis=0, keepdims=True)
        zt = _pack(jnp.broadcast_to(z, (128, D)).astype(bf16).T)
        for g in range(8):
            tscr.at[g][...] = zt[g * 64:(g + 1) * 64, :]
        for j in range(8):
            blk = jnp.concatenate([tscr[g, pl.ds(j, 8, stride=8), :] for g in range(8)], axis=0)
            zp[:, j * 128:(j + 1) * 128] = _unpack(blk).T[0:8, :].astype(f32)

    def route(tok):
        rows = [stats[b * 128:(b + 1) * 128, :].T[0:8, :] for b in range(S // 128)]
        mf = jnp.concatenate([v[0:1] for v in rows], axis=0)
        var = jnp.concatenate([v[1:2] for v in rows], axis=0)
        tr = jnp.concatenate([v[2:3] for v in rows], axis=0)
        wsum = jnp.sum(wr_buf[...].reshape(1, D).astype(f32), axis=1, keepdims=True)
        sd = _rbf(jnp.sqrt(_rbf(_rbf(var) + 1e-5)))
        rv = _rbf((tr + (mf - _rbf(mf)) * wsum) / sd)
        rmax = jnp.max(rv)
        pos = (lax.broadcasted_iota(i32, rv.shape, 0) * 128 + lax.broadcasted_iota(i32, rv.shape, 1))
        idx = jnp.min(jnp.where(rv == rmax, pos, S - 1))
        idx_s[0] = idx
        rsel[...] = jnp.full(rsel.shape, rmax, f32)
        b0 = pl.multiple_of((idx // 16) * 16, 16)
        xn = _rbf(_layernorm_rows(x_buf[pl.ds(b0, 16), :].astype(f32)))
        sel = lax.broadcasted_iota(i32, xn.shape, 0) == idx - b0
        row = jnp.sum(jnp.where(sel, xn, 0.0), axis=0, keepdims=True)
        xbv = jnp.broadcast_to(row, (128, D)).T
        xb[...] = xbv
        yacc[...] = jnp.zeros(yacc.shape, f32)
        tok([xbv[b * 128 + 120:(b + 1) * 128] for b in range(8)])
        yield

    def q_part(j, r0, nr, spread=0):
        pr = pl.ds(pl.multiple_of((j * R + r0) // 2, 8), nr // 2)
        pq = pq_buf.at[j % 2]
        rr = slice(r0, r0 + nr)
        den = [None, None]
        for c in range(4):
            m = [mm(_unpack(xs[L_ORD[k], pr, :]), wqs[k, c * 64:(c + 1) * 64, :], NT_, nr)
                 for k in range(7)]
            q11, q12, q21, q22 = [_phi(v) for v in _combine(m)]
            cl = slice(c * 128, (c + 1) * 128)
            cr = slice(HD + c * 128, HD + (c + 1) * 128)
            zl, zr = zp[0:1, cl], zp[0:1, cr]
            dt, db = q11 * zl + q12 * zr, q21 * zl + q22 * zr
            den = [dt, db] if c == 0 else [den[0] + dt, den[1] + db]
            pq.at[0][rr, cl] = q11
            pq.at[0][rr, cr] = q12
            pq.at[1][rr, cl] = q21
            pq.at[1][rr, cr] = q22
            if c < 3:
                emit_tok([d[i * 8:(i + 1) * 8] for d in den for i in range(nr // 8)], clock[0] + QLAG)
                yield
        lane = lax.broadcasted_iota(i32, (16, 128), 1)

        def normalise(tok):
            for c in range(nr // 16):
                recs = []
                for d in den:
                    d = d[c * 16:(c + 1) * 16]
                    if spread:
                        d = jnp.concatenate([gate(d[0:8]), gate(d[8:16])], axis=0)
                    d = d + jnp.where(lane % 2 == 0, pltpu.roll(d, 127, 1), pltpu.roll(d, 1, 1))
                    d = d + jnp.where(lane % 4 < 2, pltpu.roll(d, 126, 1), pltpu.roll(d, 2, 1))
                    recs.append(1.0 / (d + 1e-6))
                rq = slice(r0 + c * 16, r0 + (c + 1) * 16)
                p2 = pl.ds(pl.multiple_of((j * R + r0) // 2 + c * 8, 8), 8)
                yield
                yield
                for ct in range(4):
                    cl = slice(ct * 128, (ct + 1) * 128)
                    cr = slice(HD + ct * 128, HD + (ct + 1) * 128)
                    rc = recs
                    if spread:
                        rc = [jnp.concatenate([gate(r[0:8]), gate(r[8:16])], axis=0) for r in recs]
                    ops = _lform(pq[0, rq, cl] * rc[0], pq[0, rq, cr] * rc[0],
                                 pq[1, rq, cl] * rc[1], pq[1, rq, cr] * rc[1])
                    for k in range(7):
                        qs.at[k][p2, cl] = _pack(ops[k])
                    yield

        if spread:
            emit_tok([d[i * 8:(i + 1) * 8] for d in den for i in range(nr // 8)], clock[0] + QLAG)
            add_side(normalise, 6 * (nr // 16), 256, spread)
        else:
            for _ in normalise(None):
                pass
        yield

    def b_tile(j):
        jc = pl.ds(pl.multiple_of(j * 128, 128), 128)
        z_prep()
        for _ in q_part(j, 0, QA, 6000):
            pass
        m = [mm(_unpack(ps[k, :, jc]), xs[R_ORD[k]], TN, 1024, 4) for k in range(7)]
        g11, g12, g21, g22 = _combine(m)
        hm = (lax.broadcasted_iota(i32, (128, 128), 0) // 32
              == lax.broadcasted_iota(i32, (128, 128), 1) // 32)
        qb = q_part(j, QA, R - QA)
        next(qb)
        kvps = []
        for half, (ga, gb) in enumerate(((g11, g12), (g21, g22))):
            gc = pl.ds(pl.multiple_of((j + 4 * half) * 128, 128), 128)
            gg = jnp.concatenate([ga, gb], axis=1).astype(bf16)
            clock[0] += 256
            kv = jnp.where(hm, _dot(gg, wv_buf[:, gc], NN), 0.0)
            tscr2.at[half][...] = _pack(kv)
            kvps.append(_unpack(jnp.concatenate(
                [tscr2[half, pl.ds(jj, 8, stride=8), :] for jj in (0, 4, 1, 5, 2, 6, 3, 7)], axis=0)))
        for _ in qb:
            pass
        for half in range(2):
            g = j + 4 * half
            gr = pl.ds(pl.multiple_of(g * 128, 128), 128)
            for c in range(2):
                cl = slice(c * 256, (c + 1) * 256)
                wo2 = jnp.concatenate([wo_buf[gr, cl], wo_buf[gr, HD + c * 256:HD + (c + 1) * 256]], axis=1)
                clock[0] += 128
                mg = _dot(kvps[half], wo2, NN)
                for jj in range(4):
                    top, bot = mg[jj * 32:jj * 32 + 16], mg[jj * 32 + 16:(jj + 1) * 32]
                    ops = _rform(top[:, :256], top[:, 256:], bot[:, :256], bot[:, 256:])
                    for k in range(7):
                        ms.at[k][pl.ds(pl.multiple_of(jj * 64 + g * 8, 8), 8), cl] = _pack(ops[k])

    def out_part(p0, nr, y):
        pr = pl.ds(pl.multiple_of(p0 // 2, 8), nr // 2)
        rows = (pl.ds(pl.multiple_of(p0, 16), nr), pl.ds(pl.multiple_of(HP + p0, 16), nr))
        row = lax.broadcasted_iota(i32, (nr, 256), 0) + p0
        hit = (row == idx_s[0], row + HP == idx_s[0])
        for c in range(2):
            cl = pl.ds(c * 256, 256)
            cr = pl.ds(HD + c * 256, 256)
            m = [_dot(_unpack(qs[k, pr, :]), _unpack(ms[k, :, cl]), NN) for k in range(7)]
            o11, o12, o21, o22 = _combine(m)
            for h, cc, o in ((1, cr, o22), (1, cl, o21), (0, cr, o12), (0, cl, o11)):
                rr = rows[h]
                a = jnp.concatenate([sa[rr, :]] * 2, axis=1)
                b = jnp.concatenate([sb[rr, :]] * 2, axis=1)
                o = o + jnp.where(hit[h], y[:, cc.start:cc.start + 256], 0.0)
                out_buf[rr, cc] = (x_buf[rr, cc].astype(f32) * a - b + o).astype(bf16)
                cp(out_buf.at[rr, cc], out_hbm.at[0, rr, cc], SEM_O).start()

    def ffn_chunk(c, tok):
        hs = []
        for f0 in range(0, FW, 256):
            w = min(256, FW - f0)
            fs = slice(f0, f0 + w)
            ag = jnp.zeros((8, w), f32)
            au = jnp.zeros((8, w), f32)
            step = FSTEP * 256 // w
            for kg in range(D // 8):
                xv = jnp.concatenate([gate(xb[8 * kg:8 * kg + 8, :])] * (w // 128), axis=1)
                ag = ag + wg_buf[c, 8 * kg:8 * kg + 8, fs].astype(f32) * xv
                au = au + wu_buf[c, 8 * kg:8 * kg + 8, fs].astype(f32) * xv
                if kg % step == step - 1:
                    tok([a[:, i * 128:(i + 1) * 128] for a in (ag, au) for i in range(w // 128)])
                    yield
            g = _rbf(jnp.sum(ag, axis=0, keepdims=True))
            u = _rbf(jnp.sum(au, axis=0, keepdims=True))
            h = _rbf(_rbf(g * jax.nn.sigmoid(g)) * u)
            hb_buf.at[c % 2][fs, :] = jnp.broadcast_to(h, (128, w)).T
        for d0 in range(0, D, 512):
            ds_ = slice(d0, d0 + 512)
            acc = yacc[:, ds_]
            for kg in range(FW // 8):
                hv = jnp.concatenate([gate(hb_buf[c % 2, 8 * kg:8 * kg + 8, :])] * 4, axis=1)
                acc = acc + wd_buf[c, 8 * kg:8 * kg + 8, ds_].astype(f32) * hv
                if kg % FSTEP == FSTEP - 1:
                    tok([acc[:, i * 128:(i + 1) * 128] for i in range(4)])
                    yield
            yacc[:, ds_] = acc

    with _scope("p0_issue"):
        cp_wr.start()
        for c in cp_x(0):
            c.start()
        cp_wk.start()
        for t in range(1, NT):
            for c in cp_x(t):
                c.start()
        cp_wq.start()
        for j in range(NT):
            for c in cp_b(j):
                c.start()
        zacc[...] = jnp.zeros(zacc.shape, f32)
        zero_buf[1] = jnp.zeros((8, 128), u32)
        cp_zero = cp(zero_buf.at[1], zero_buf.at[0], SEM_Z)
        cp_zero.start()
        cp_zero.wait()
        cp_wr.wait()
        for c in cp_x(0):
            c.wait()
    with _scope("p1_ln0"):
        for _ in ln_tile(0, lambda v: None):
            pass
    with _scope("p2_waitwk"):
        cp_wk.wait()
    with _scope("p3_wkprep"):
        wk_prep()
    for t in range(NT):
        with _scope("a_wait%d" % t):
            for c in (cp_x(t + 1) if t + 1 < NT else [cp_wq]):
                c.wait()
        with _scope("a_tile%d" % t):
            if t + 1 < NT:
                add_side(lambda tok, t=t: ln_tile(t + 1, tok), R // 16, 0, 26 * R)
            else:
                add_side(wq_prep, 8, 300, 24 * R, 0)
                add_side(route, 1, 0, 10 * R, 0)
            kproj_tile(t)
            finish()

    def b_body(j, carry):
        with _scope("b_wait"):
            for c in cp_b(j, wait_only=True):
                c.wait()
        with _scope("b_body"):
            add_side(lambda tok: ffn_chunk(j, tok), (56 + 28) * 8 // FSTEP, 0, 13500)
            b_tile(j)
            finish()
        return carry

    lax.fori_loop(0, NT, b_body, 0)

    def c_body(t, carry):
        with _scope("c_body"):
            y = _rbf(jnp.sum(yacc[...], axis=0, keepdims=True))
            y = _rbf(y * _rbf(jax.nn.sigmoid(rsel[...])))
            for p in range(R // CR):
                out_part(t * R + p * CR, CR, y)
        return carry

    lax.fori_loop(0, NT, c_body, 0)
    with _scope("tail"):
        cp(out_buf, out_hbm.at[0], SEM_O).wait()


@jax.jit
def pallas_parallel_sum__linear_attn_block__moe_arch_mod__prompt_kernel(
    A_x: jax.Array,
    A_wqkv: jax.Array,
    A_wo: jax.Array,
    B_x: jax.Array,
    B_w_r: jax.Array,
    B_w_gate: jax.Array,
    B_w_up: jax.Array,
    B_w_down: jax.Array,
):
    del B_x
    V = pltpu.VMEM
    scratch = [
        V((S, D), bf16),
        V((D, D), bf16),
        V((D, D), bf16),
        V((D, D), bf16),
        V((D, D), bf16),
        V((D,), bf16),
        V((NF, D, FW), bf16),
        V((NF, D, FW), bf16),
        V((NF, FW, D), bf16),
        V((7, HP // 2, HD), u32),
        V((7, HP // 2, HD), u32),
        V((7, HP // 2, HD), u32),
        V((7, HD // 2, HD), u32),
        V((7, HD // 2, HD), u32),
        V((7, HD // 2, HD), u32),
        V((S, 128), f32),
        V((S, 128), f32),
        V((S, 128), f32),
        V((8, D), f32),
        V((8, D), f32),
        V((8, 64, 128), u32),
        V((2, 64, 128), u32),
        V((2, 2, R, D), f32),
        V((D, 128), f32),
        V((2, FW, 128), f32),
        V((8, D), f32),
        V((1, D), f32),
        V((S, D), bf16),
        V((2, 8, 128), u32),
        pltpu.SMEM((1,), i32),
        pltpu.SemaphoreType.DMA((2 * NT + 4,)),
    ]
    return pl.pallas_call(
        _kernel,
        out_shape=jax.ShapeDtypeStruct((1, S, D), bf16),
        in_specs=[pl.BlockSpec(memory_space=pl.ANY)] * 7,
        out_specs=pl.BlockSpec(memory_space=pl.ANY),
        scratch_shapes=scratch,
        compiler_params=pltpu.CompilerParams(vmem_limit_bytes=110 * 1024 * 1024,
                                             disable_bounds_checks=True,
                                             disable_semaphore_checks=True),
    )(A_x, A_wqkv, A_wo, B_w_r, B_w_gate, B_w_up, B_w_down)
```

```python
import contextlib

import jax
import jax.numpy as jnp
from jax import lax
import jax.experimental.pallas as pl
import jax.experimental.pallas.tpu as pltpu

bf16, f32, u32, i32 = jnp.bfloat16, jnp.float32, jnp.uint32, jnp.int32

S = 2048
D = 1024
F = 3584
HP = S // 2
HD = D // 2
R = 256
NT = HP // R
FW = 896
NF = F // FW
QLAG = 768
QA = 192
FSTEP = 2
CR = 128

L_ORD = (2, 3, 0, 1, 4, 5, 6)
R_ORD = (2, 0, 6, 5, 1, 4, 3)

K_SEQ = (1, 4, 0, 2, 3, 5, 6)

NN = (((1,), (0,)), ((), ()))
NT_ = (((1,), (1,)), ((), ()))
TN = (((0,), (0,)), ((), ()))


SCOPES = False


def _scope(name):
    return jax.named_scope(name) if SCOPES else contextlib.nullcontext()


def _dot(a, b, dims):
    return lax.dot_general(a, b, dims, preferred_element_type=f32)


def _pack(v):
    return pltpu.bitcast(v.astype(bf16), u32)


def _unpack(v):
    return pltpu.bitcast(v, bf16)


def _combine(m):
    m1, m2, m3, m4, m5, m6, m7 = m
    return m1 + m4 - m5 + m7, m3 + m5, m2 + m4, m1 - m2 + m3 + m6


def _lform(a11, a12, a21, a22):
    return (a11 + a22, a21 + a22, a11, a22, a11 + a12, a21 - a11, a12 - a22)


def _rform(b11, b12, b21, b22):
    return (b11 + b22, b11, b12 - b22, b21 - b11, b22, b11 + b12, b21 + b22)


def _phi(t):
    return jnp.where(t > 0, t + 1.0, jnp.exp(t)) + 1e-6


def _rbf(v):
    return v.astype(bf16).astype(f32)


def _layernorm_rows(xv):
    mf = jnp.sum(xv, axis=1, keepdims=True) * (1.0 / D)
    mb = _rbf(mf)
    d = xv - mb
    dm = mf - mb
    var = jnp.sum(d * d, axis=1, keepdims=True) * (1.0 / D) - dm * dm
    var = jnp.maximum(var, 0.0)
    sd = _rbf(jnp.sqrt(_rbf(_rbf(var) + 1e-5)))
    return d * (1.0 / sd)


def _kernel(x_hbm, wqkv_hbm, wo_hbm, wr_hbm, wg_hbm, wu_hbm, wd_hbm, out_hbm,
            x_buf, wk_buf, wq_buf, wv_buf, wo_buf, wr_buf, wg_buf, wu_buf, wd_buf,
            xs, ps, qs, wks, wqs, ms, sa, sb, stats, zacc, zp, tscr, tscr2, wqt, pq_buf,
            xb, hb_buf, yacc, rsel, out_buf, zero_buf, idx_s, sem):

    SEM_B, SEM_O, SEM_Z, SEM_A = 0, NT, NT + 1, NT + 2

    def cp(src, dst, s):
        return pltpu.make_async_copy(src, dst, sem.at[s])

    def cp_x(p0, n, s):
        return [cp(x_hbm.at[0, pl.ds(h * HP + p0, n), :], x_buf.at[pl.ds(h * HP + p0, n), :], s)
                for h in range(2)]

    def cp_wk(c, s):
        return [cp(wqkv_hbm.at[:, pl.ds(D + h * HD + c * 128, 128)],
                   wk_buf.at[c, :, pl.ds(h * 128, 128)], s) for h in range(2)]

    a_groups = [
        [cp(wr_hbm, wr_buf, SEM_A)] + cp_x(0, 128, SEM_A),
        cp_x(128, 128, SEM_A + 1),
        cp_wk(0, SEM_A + 2),
        cp_wk(1, SEM_A + 3),
        cp_wk(2, SEM_A + 4) + cp_x(256, 128, SEM_A + 4) + cp_wk(3, SEM_A + 4),
        cp_x(384, 384, SEM_A + 5),
        cp_x(768, 256, SEM_A + 6) + [cp(wqkv_hbm.at[:, pl.ds(0, D)], wq_buf, SEM_A + 6)],
    ]

    def cp_b(j, wait_only=False):
        def off(v, m):
            return v if isinstance(v, int) else pl.multiple_of(v, m)
        out = []
        for g in (j, j + 4):
            c0 = off(g * 128, 128)
            dst = wv_buf.at[:, pl.ds(c0, 128)]
            out.append(cp(dst if wait_only else wqkv_hbm.at[:, pl.ds(2 * D + c0, 128)], dst, SEM_B + j))
            dst = wo_buf.at[pl.ds(c0, 128), :]
            out.append(cp(dst if wait_only else wo_hbm.at[pl.ds(c0, 128), :], dst, SEM_B + j))
        f0 = off(j * FW, 128)
        for src, dst in ((wg_hbm.at[:, pl.ds(f0, FW)], wg_buf.at[j]),
                         (wu_hbm.at[:, pl.ds(f0, FW)], wu_buf.at[j]),
                         (wd_hbm.at[pl.ds(f0, FW), :], wd_buf.at[j])):
            out.append(cp(dst if wait_only else src, dst, SEM_B + j))
        return out

    clock = [0]
    toks = []
    sides = []
    fwd = [None]

    def emit_tok(vals, stamp=None):
        t = None
        for v in vals:
            v = pltpu.bitcast(v, u32) if v.dtype != u32 else v
            t = v if t is None else t | v
        toks.append((clock[0] if stamp is None else stamp, t & zero_buf[0]))

    def gate(v):
        if fwd[0] is None:
            return v
        if fwd[0][1] is None:
            fwd[0][1] = pltpu.bitcast(fwd[0][0](), u32) & zero_buf[0]
        head = pltpu.bitcast(pltpu.bitcast(v[0:8], u32) | fwd[0][1], v.dtype)
        return head if v.shape[0] == 8 else jnp.concatenate([head, v[8:]], axis=0)

    def add_side(gen_fn, n, t0, t1, lag=None):
        st = {"i": 0, "n": n, "t0": clock[0] + t0, "t1": clock[0] + t1}

        def tok(vals):
            if lag is not None:
                emit_tok(vals, st["t0"] + (st["i"] + 1) * (st["t1"] - st["t0"]) // st["n"] + lag)
        st["g"] = gen_fn(tok)
        sides.append(st)

    def advance(until):
        for st in sides:
            while st["i"] < st["n"] and st["t0"] + st["i"] * (st["t1"] - st["t0"]) // st["n"] < until:
                next(st["g"], None)
                st["i"] += 1

    def finish():
        for st in sides:
            for _ in st["g"]:
                pass
        sides.clear()
        toks.clear()
        fwd[0] = None

    def mm(lhs, rhs, dims, cycles, nseg=1):
        due = [t for (c, t) in toks if c <= clock[0]]
        toks[:] = [(c, t) for (c, t) in toks if c > clock[0]]
        if due:
            head = rhs[0:8, 0:128]
            for t in due:
                head = head | t
            if rhs.shape[1] > 128:
                head = jnp.concatenate([head, rhs[0:8, 128:]], axis=1)
            rhs = jnp.concatenate([head, rhs[8:]], axis=0)
        res = _dot(lhs, _unpack(rhs), dims)
        ngr = res.shape[0] // 16
        for sg in range(nseg):
            for i in range(ngr):
                fwd[0] = [lambda sg=sg, i=i: res[i * 16:i * 16 + 8, sg * 128:(sg + 1) * 128], None]
                clock[0] += cycles // nseg // ngr
                advance(clock[0])
        return res

    def ln_rows(p_start, n_rows, tok):
        wr = wr_buf[...].reshape(1, D).astype(f32)
        lane = lax.broadcasted_iota(i32, (8, 128), 1)
        for c in range(n_rows // 16):
            p0 = p_start + c * 16
            ds_, rss = [], []
            for r0 in (p0, p0 + 8, HP + p0, HP + p0 + 8):
                xv = x_buf[r0:r0 + 8, :].astype(f32)
                xg = jnp.concatenate([gate(xv[:, 0:128]), xv[:, 128:]], axis=1)
                mf = jnp.sum(xg, axis=1, keepdims=True) * (1.0 / D)
                d = xv - mf
                var = jnp.sum(d * d, axis=1, keepdims=True) * (1.0 / D)
                tr = jnp.sum(d * wr, axis=1, keepdims=True)
                rs = jnp.broadcast_to(lax.rsqrt(var + 1e-5), (8, 128))
                mf = jnp.broadcast_to(mf, (8, 128))
                sa[r0:r0 + 8, :] = 1.0 + rs
                sb[r0:r0 + 8, :] = mf * rs
                stats[r0:r0 + 8, :] = jnp.where(
                    lane == 0, mf, jnp.where(lane == 1, jnp.broadcast_to(var, (8, 128)),
                                             jnp.broadcast_to(tr, (8, 128))))
                ds_.append(d)
                rss.append(rs)
                yield
            pend.append((p0, ds_, rss))
            if len(pend) > 1:
                yield from ln_finish(*pend.pop(0))
        while pend:
            yield from ln_finish(*pend.pop(0))

    pend = []

    def ln_finish(p0, ds_, rss):
        for ct in range(4):
            cl = slice(ct * 128, (ct + 1) * 128)
            cr = slice(HD + ct * 128, HD + (ct + 1) * 128)
            rg = [gate(r) for r in rss]
            x11, x12, x21, x22 = [
                jnp.concatenate([ds_[i][:, cc] * rg[i], ds_[i + 1][:, cc] * rg[i + 1]], axis=0)
                for i, cc in ((0, cl), (0, cr), (2, cl), (2, cr))]
            ops = (x11, x22, x11 + x22, x21 + x22, x11 + x12, x21 - x11, x12 - x22)
            for k in range(7):
                xs.at[k][p0 // 2:p0 // 2 + 8, cl] = _pack(ops[k])
            yield

    def wk_prep(c, tok=None):
        for i in range(HD // 16):
            r0 = i * 16
            top = wk_buf[c, r0:r0 + 16, :].astype(f32)
            bot = wk_buf[c, HD + r0:HD + r0 + 16, :].astype(f32)
            ops = _rform(gate(top[:, :128]), top[:, 128:], bot[:, :128], gate(bot[:, 128:]))
            for k in range(7):
                wks.at[k][r0 // 2:r0 // 2 + 8, c * 128:(c + 1) * 128] = _pack(ops[k])
            yield

    def wq_prep(tok):
        def transpose(g):
            for ct in range(8):
                tile = gate(pltpu.bitcast(wq_buf[ct * 128:(ct + 1) * 128, g * 128:(g + 1) * 128], u32))
                wqt.at[g * 8 + ct][...] = pltpu.bitcast(_unpack(tile).T, u32)
                yield

        def combine(g):
            for j in range(4):
                for ct in range(4):
                    w11, w12, w21, w22 = [
                        _unpack(gate(wqt[g * 8 + cc, pl.ds(jj, 8, stride=8), :])).astype(f32)
                        for jj, cc in ((j, ct), (j, ct + 4), (j + 4, ct), (j + 4, ct + 4))]
                    ops = _rform(w11, w21, w12, w22)
                    for k in range(7):
                        wqs.at[k][j * 64 + g * 8:j * 64 + g * 8 + 8, ct * 128:(ct + 1) * 128] = _pack(ops[k])
                    yield

        for g in range(9):
            if g < 8:
                yield from transpose(g)
            if g > 0:
                yield from combine(g - 1)

    def kproj(p0, n, chunks=range(4)):
        pr = pl.ds(p0 // 2, n // 2)
        for c in chunks:
            cs = slice(c * 128, (c + 1) * 128)
            m = [None] * 7
            for k in K_SEQ:
                m[k] = mm(_unpack(xs[L_ORD[k], pr, :]), wks[k, :, cs], NN, n)
            k11, k12, k21, k22 = [_phi(v) for v in _combine(m)]
            zl = (k11 + k21).reshape(n // 8, 8, 128).sum(axis=0)
            zr = (k12 + k22).reshape(n // 8, 8, 128).sum(axis=0)
            zacc[:, cs] += zl
            zacc[:, HD + c * 128:HD + (c + 1) * 128] += zr
            ops = _lform(k11, k21, k12, k22)
            for k in range(7):
                ps.at[k][pr, cs] = _pack(ops[k])

    def z_prep():
        z = jnp.sum(zacc[...], axis=0, keepdims=True)
        zt = _pack(jnp.broadcast_to(z, (128, D)).astype(bf16).T)
        for g in range(8):
            tscr.at[g][...] = zt[g * 64:(g + 1) * 64, :]
        for j in range(8):
            blk = jnp.concatenate([tscr[g, pl.ds(j, 8, stride=8), :] for g in range(8)], axis=0)
            zp[:, j * 128:(j + 1) * 128] = _unpack(blk).T[0:8, :].astype(f32)

    def route(tok):
        rows = []
        for b in range(S // 128):
            rows.append(gate(stats[b * 128:(b + 1) * 128, :]).T[0:8, :])
            yield
        mf = jnp.concatenate([v[0:1] for v in rows], axis=0)
        var = jnp.concatenate([v[1:2] for v in rows], axis=0)
        tr = jnp.concatenate([v[2:3] for v in rows], axis=0)
        wsum = jnp.sum(wr_buf[...].reshape(1, D).astype(f32), axis=1, keepdims=True)
        sd = _rbf(jnp.sqrt(_rbf(_rbf(var) + 1e-5)))
        rv = _rbf((tr + (mf - _rbf(mf)) * wsum) / sd)
        rmax = jnp.max(rv)
        pos = (lax.broadcasted_iota(i32, rv.shape, 0) * 128 + lax.broadcasted_iota(i32, rv.shape, 1))
        idx = jnp.min(jnp.where(rv == rmax, pos, S - 1))
        idx_s[0] = idx
        rsel[...] = jnp.full(rsel.shape, rmax, f32)
        b0 = pl.multiple_of((idx // 16) * 16, 16)
        xn = _rbf(_layernorm_rows(x_buf[pl.ds(b0, 16), :].astype(f32)))
        sel = lax.broadcasted_iota(i32, xn.shape, 0) == idx - b0
        row = jnp.sum(jnp.where(sel, xn, 0.0), axis=0, keepdims=True)
        xbv = jnp.broadcast_to(row, (128, D)).T
        xb[...] = xbv
        yacc[...] = jnp.zeros(yacc.shape, f32)
        tok([xbv[b * 128 + 120:(b + 1) * 128] for b in range(8)])
        yield

    def q_part(j, r0, nr, spread=0):
        pr = pl.ds(pl.multiple_of((j * R + r0) // 2, 8), nr // 2)
        pq = pq_buf.at[j % 2]
        rr = slice(r0, r0 + nr)
        den = [None, None]
        for c in range(4):
            m = [mm(_unpack(xs[L_ORD[k], pr, :]), wqs[k, c * 64:(c + 1) * 64, :], NT_, nr)
                 for k in range(7)]
            q11, q12, q21, q22 = [_phi(v) for v in _combine(m)]
            cl = slice(c * 128, (c + 1) * 128)
            cr = slice(HD + c * 128, HD + (c + 1) * 128)
            zl, zr = zp[0:1, cl], zp[0:1, cr]
            dt, db = q11 * zl + q12 * zr, q21 * zl + q22 * zr
            den = [dt, db] if c == 0 else [den[0] + dt, den[1] + db]
            pq.at[0][rr, cl] = q11
            pq.at[0][rr, cr] = q12
            pq.at[1][rr, cl] = q21
            pq.at[1][rr, cr] = q22
            if c < 3:
                emit_tok([d[i * 8:(i + 1) * 8] for d in den for i in range(nr // 8)], clock[0] + QLAG)
                yield
        lane = lax.broadcasted_iota(i32, (16, 128), 1)

        def normalise(tok):
            for c in range(nr // 16):
                recs = []
                for d in den:
                    d = d[c * 16:(c + 1) * 16]
                    if spread:
                        d = jnp.concatenate([gate(d[0:8]), gate(d[8:16])], axis=0)
                    d = d + jnp.where(lane % 2 == 0, pltpu.roll(d, 127, 1), pltpu.roll(d, 1, 1))
                    d = d + jnp.where(lane % 4 < 2, pltpu.roll(d, 126, 1), pltpu.roll(d, 2, 1))
                    recs.append(1.0 / (d + 1e-6))
                rq = slice(r0 + c * 16, r0 + (c + 1) * 16)
                p2 = pl.ds(pl.multiple_of((j * R + r0) // 2 + c * 8, 8), 8)
                yield
                yield
                for ct in range(4):
                    cl = slice(ct * 128, (ct + 1) * 128)
                    cr = slice(HD + ct * 128, HD + (ct + 1) * 128)
                    rc = recs
                    if spread:
                        rc = [jnp.concatenate([gate(r[0:8]), gate(r[8:16])], axis=0) for r in recs]
                    ops = _lform(pq[0, rq, cl] * rc[0], pq[0, rq, cr] * rc[0],
                                 pq[1, rq, cl] * rc[1], pq[1, rq, cr] * rc[1])
                    for k in range(7):
                        qs.at[k][p2, cl] = _pack(ops[k])
                    yield

        if spread:
            emit_tok([d[i * 8:(i + 1) * 8] for d in den for i in range(nr // 8)], clock[0] + QLAG)
            add_side(normalise, 6 * (nr // 16), 256, spread)
        else:
            for _ in normalise(None):
                pass
        yield

    def b_tile(j):
        jc = pl.ds(pl.multiple_of(j * 128, 128), 128)
        z_prep()
        for _ in q_part(j, 0, QA, 6000):
            pass
        m = [mm(_unpack(ps[k, :, jc]), xs[R_ORD[k]], TN, 1024, 4) for k in range(7)]
        g11, g12, g21, g22 = _combine(m)
        hm = (lax.broadcasted_iota(i32, (128, 128), 0) // 32
              == lax.broadcasted_iota(i32, (128, 128), 1) // 32)
        qb = q_part(j, QA, R - QA)
        next(qb)
        kvps = []
        for half, (ga, gb) in enumerate(((g11, g12), (g21, g22))):
            gc = pl.ds(pl.multiple_of((j + 4 * half) * 128, 128), 128)
            gg = jnp.concatenate([ga, gb], axis=1).astype(bf16)
            clock[0] += 256
            kv = jnp.where(hm, _dot(gg, wv_buf[:, gc], NN), 0.0)
            tscr2.at[half][...] = _pack(kv)
            kvps.append(_unpack(jnp.concatenate(
                [tscr2[half, pl.ds(jj, 8, stride=8), :] for jj in (0, 4, 1, 5, 2, 6, 3, 7)], axis=0)))
        for _ in qb:
            pass
        for half in range(2):
            g = j + 4 * half
            gr = pl.ds(pl.multiple_of(g * 128, 128), 128)
            for c in range(2):
                cl = slice(c * 256, (c + 1) * 256)
                wo2 = jnp.concatenate([wo_buf[gr, cl], wo_buf[gr, HD + c * 256:HD + (c + 1) * 256]], axis=1)
                clock[0] += 128
                mg = _dot(kvps[half], wo2, NN)
                for jj in range(4):
                    top, bot = mg[jj * 32:jj * 32 + 16], mg[jj * 32 + 16:(jj + 1) * 32]
                    ops = _rform(top[:, :256], top[:, 256:], bot[:, :256], bot[:, 256:])
                    for k in range(7):
                        ms.at[k][pl.ds(pl.multiple_of(jj * 64 + g * 8, 8), 8), cl] = _pack(ops[k])

    def out_part(p0, nr, y):
        pr = pl.ds(pl.multiple_of(p0 // 2, 8), nr // 2)
        rows = (pl.ds(pl.multiple_of(p0, 16), nr), pl.ds(pl.multiple_of(HP + p0, 16), nr))
        row = lax.broadcasted_iota(i32, (nr, 256), 0) + p0
        hit = (row == idx_s[0], row + HP == idx_s[0])
        for c in range(2):
            cl = pl.ds(c * 256, 256)
            cr = pl.ds(HD + c * 256, 256)
            m = [_dot(_unpack(qs[k, pr, :]), _unpack(ms[k, :, cl]), NN) for k in range(7)]
            o11, o12, o21, o22 = _combine(m)
            for h, cc, o in ((1, cr, o22), (1, cl, o21), (0, cr, o12), (0, cl, o11)):
                rr = rows[h]
                a = jnp.concatenate([sa[rr, :]] * 2, axis=1)
                b = jnp.concatenate([sb[rr, :]] * 2, axis=1)
                o = o + jnp.where(hit[h], y[:, cc.start:cc.start + 256], 0.0)
                out_buf[rr, cc] = (x_buf[rr, cc].astype(f32) * a - b + o).astype(bf16)
                cp(out_buf.at[rr, cc], out_hbm.at[0, rr, cc], SEM_O).start()

    def ffn_chunk(c, tok):
        hs = []
        for f0 in range(0, FW, 256):
            w = min(256, FW - f0)
            fs = slice(f0, f0 + w)
            ag = jnp.zeros((8, w), f32)
            au = jnp.zeros((8, w), f32)
            step = FSTEP * 256 // w
            for kg in range(D // 8):
                xv = jnp.concatenate([gate(xb[8 * kg:8 * kg + 8, :])] * (w // 128), axis=1)
                ag = ag + wg_buf[c, 8 * kg:8 * kg + 8, fs].astype(f32) * xv
                au = au + wu_buf[c, 8 * kg:8 * kg + 8, fs].astype(f32) * xv
                if kg % step == step - 1:
                    tok([a[:, i * 128:(i + 1) * 128] for a in (ag, au) for i in range(w // 128)])
                    yield
            g = _rbf(jnp.sum(ag, axis=0, keepdims=True))
            u = _rbf(jnp.sum(au, axis=0, keepdims=True))
            h = _rbf(_rbf(g * jax.nn.sigmoid(g)) * u)
            hb_buf.at[c % 2][fs, :] = jnp.broadcast_to(h, (128, w)).T
        for d0 in range(0, D, 512):
            ds_ = slice(d0, d0 + 512)
            acc = yacc[:, ds_]
            for kg in range(FW // 8):
                hv = jnp.concatenate([gate(hb_buf[c % 2, 8 * kg:8 * kg + 8, :])] * 4, axis=1)
                acc = acc + wd_buf[c, 8 * kg:8 * kg + 8, ds_].astype(f32) * hv
                if kg % FSTEP == FSTEP - 1:
                    tok([acc[:, i * 128:(i + 1) * 128] for i in range(4)])
                    yield
            yacc[:, ds_] = acc

    def wait_group(i):
        with _scope("a_wait%d" % i):
            for c in a_groups[i]:
                c.wait()

    def run_all(gen):
        for _ in gen:
            pass

    def ln_side(p0, n, t0, t1):
        add_side(lambda tok: ln_rows(p0, n, tok), n // 2, t0, t1)

    with _scope("p0_issue"):
        for grp in a_groups:
            for c in grp:
                c.start()
        for j in range(NT):
            for c in cp_b(j):
                c.start()
        zacc[...] = jnp.zeros(zacc.shape, f32)
        zero_buf[1] = jnp.zeros((8, 128), u32)
        cp_zero = cp(zero_buf.at[1], zero_buf.at[0], SEM_Z)
        cp_zero.start()
        cp_zero.wait()
    wait_group(0)
    with _scope("a0"):
        run_all(ln_rows(0, 128, None))
    wait_group(1)
    with _scope("a1"):
        run_all(ln_rows(128, 128, None))
    wait_group(2)
    with _scope("a2"):
        run_all(wk_prep(0))
        kproj(0, 256, [0])
        finish()
    wait_group(3)
    with _scope("a3"):
        run_all(wk_prep(1))
        kproj(0, 256, [1])
        finish()
    wait_group(4)
    with _scope("a4"):
        run_all(wk_prep(2))
        add_side(lambda tok: wk_prep(3), 32, 300, 1500)
        ln_side(256, 128, 0, 3300)
        kproj(0, 256, [2, 3])
        finish()
    wait_group(5)
    with _scope("a5"):
        for p0 in (256, 384, 512):
            ln_side(p0 + 128, 128, 0, 3200)
            kproj(p0, 128)
        finish()
    wait_group(6)
    with _scope("a6"):
        add_side(wq_prep, 8 * 24, 0, 10000)
        for p0 in (640, 768):
            ln_side(p0 + 128, 128, 0, 3200)
            kproj(p0, 128)
        add_side(route, 17, 0, 800)
        kproj(896, 128)
        finish()

    def b_body(j, carry):
        with _scope("b_wait"):
            for c in cp_b(j, wait_only=True):
                c.wait()
        with _scope("b_body"):
            add_side(lambda tok: ffn_chunk(j, tok), (56 + 28) * 8 // FSTEP, 0, 13500)
            b_tile(j)
            finish()
        return carry

    lax.fori_loop(0, NT, b_body, 0)

    def c_body(t, carry):
        with _scope("c_body"):
            y = _rbf(jnp.sum(yacc[...], axis=0, keepdims=True))
            y = _rbf(y * _rbf(jax.nn.sigmoid(rsel[...])))
            for p in range(R // CR):
                out_part(t * R + p * CR, CR, y)
        return carry

    lax.fori_loop(0, NT, c_body, 0)
    with _scope("tail"):
        cp(out_buf, out_hbm.at[0], SEM_O).wait()


@jax.jit
def pallas_parallel_sum__linear_attn_block__moe_arch_mod__prompt_kernel(
    A_x: jax.Array,
    A_wqkv: jax.Array,
    A_wo: jax.Array,
    B_x: jax.Array,
    B_w_r: jax.Array,
    B_w_gate: jax.Array,
    B_w_up: jax.Array,
    B_w_down: jax.Array,
):
    del B_x
    V = pltpu.VMEM
    scratch = [
        V((S, D), bf16),
        V((4, D, 256), bf16),
        V((D, D), bf16),
        V((D, D), bf16),
        V((D, D), bf16),
        V((D,), bf16),
        V((NF, D, FW), bf16),
        V((NF, D, FW), bf16),
        V((NF, FW, D), bf16),
        V((7, HP // 2, HD), u32),
        V((7, HP // 2, HD), u32),
        V((7, HP // 2, HD), u32),
        V((7, HD // 2, HD), u32),
        V((7, HD // 2, HD), u32),
        V((7, HD // 2, HD), u32),
        V((S, 128), f32),
        V((S, 128), f32),
        V((S, 128), f32),
        V((8, D), f32),
        V((8, D), f32),
        V((8, 64, 128), u32),
        V((2, 64, 128), u32),
        V((64, 64, 128), u32),
        V((2, 2, R, D), f32),
        V((D, 128), f32),
        V((2, FW, 128), f32),
        V((8, D), f32),
        V((1, D), f32),
        V((S, D), bf16),
        V((2, 8, 128), u32),
        pltpu.SMEM((1,), i32),
        pltpu.SemaphoreType.DMA((NT + 9,)),
    ]
    return pl.pallas_call(
        _kernel,
        out_shape=jax.ShapeDtypeStruct((1, S, D), bf16),
        in_specs=[pl.BlockSpec(memory_space=pl.ANY)] * 7,
        out_specs=pl.BlockSpec(memory_space=pl.ANY),
        scratch_shapes=scratch,
        compiler_params=pltpu.CompilerParams(vmem_limit_bytes=110 * 1024 * 1024,
                                             disable_bounds_checks=True,
                                             disable_semaphore_checks=True),
    )(A_x, A_wqkv, A_wo, B_w_r, B_w_gate, B_w_up, B_w_down)
```

```python
import contextlib

import jax
import jax.numpy as jnp
from jax import lax
import jax.experimental.pallas as pl
import jax.experimental.pallas.tpu as pltpu

bf16, f32, u32, i32 = jnp.bfloat16, jnp.float32, jnp.uint32, jnp.int32

S = 2048
D = 1024
F = 3584
HP = S // 2
HD = D // 2
R = 256
NT = HP // R
FW = 896
NF = F // FW
QLAG = 768
UNROLL_B = False
QA = 192
SLAG = 400
FSTEP = 2
CR = 128

L_ORD = (2, 3, 0, 1, 4, 5, 6)
R_ORD = (2, 0, 6, 5, 1, 4, 3)

K_SEQ = (1, 4, 0, 2, 3, 5, 6)

NN = (((1,), (0,)), ((), ()))
NT_ = (((1,), (1,)), ((), ()))
TN = (((0,), (0,)), ((), ()))


SCOPES = False


def _scope(name):
    return jax.named_scope(name) if SCOPES else contextlib.nullcontext()


def _mo(v, m):
    return v if isinstance(v, int) else pl.multiple_of(v, m)


def _dot(a, b, dims):
    return lax.dot_general(a, b, dims, preferred_element_type=f32)


def _pack(v):
    return pltpu.bitcast(v.astype(bf16), u32)


def _unpack(v):
    return pltpu.bitcast(v, bf16)


def _combine(m):
    m1, m2, m3, m4, m5, m6, m7 = m
    return m1 + m4 - m5 + m7, m3 + m5, m2 + m4, m1 - m2 + m3 + m6


def _lform(a11, a12, a21, a22):
    return (a11 + a22, a21 + a22, a11, a22, a11 + a12, a21 - a11, a12 - a22)


def _rform(b11, b12, b21, b22):
    return (b11 + b22, b11, b12 - b22, b21 - b11, b22, b11 + b12, b21 + b22)


def _phi(t):
    return jnp.where(t > 0, t + 1.0, jnp.exp(t)) + 1e-6


def _rbf(v):
    return v.astype(bf16).astype(f32)


def _layernorm_rows(xv):
    mf = jnp.sum(xv, axis=1, keepdims=True) * (1.0 / D)
    mb = _rbf(mf)
    d = xv - mb
    dm = mf - mb
    var = jnp.sum(d * d, axis=1, keepdims=True) * (1.0 / D) - dm * dm
    var = jnp.maximum(var, 0.0)
    sd = _rbf(jnp.sqrt(_rbf(_rbf(var) + 1e-5)))
    return d * (1.0 / sd)


def _kernel(x_hbm, wqkv_hbm, wo_hbm, wr_hbm, wg_hbm, wu_hbm, wd_hbm, out_hbm,
            x_buf, wk_buf, wq_buf, wv_buf, wo_buf, wr_buf, wg_buf, wu_buf, wd_buf,
            xs, ps, qs, wks, wqs, ms, sa, sb, stats, zacc, zp, tscr, tscr2, wqt, pq_buf,
            xb, hb_buf, yacc, rsel, out_buf, zero_buf, idx_s, sem):

    SEM_B, SEM_O, SEM_Z, SEM_A = 0, NT, NT + 1, NT + 2

    def cp(src, dst, s):
        return pltpu.make_async_copy(src, dst, sem.at[s])

    def cp_x(p0, n, s):
        return [cp(x_hbm.at[0, pl.ds(h * HP + p0, n), :], x_buf.at[pl.ds(h * HP + p0, n), :], s)
                for h in range(2)]

    def cp_wk(c, s):
        return [cp(wqkv_hbm.at[:, pl.ds(D + h * HD + c * 128, 128)],
                   wk_buf.at[c, :, pl.ds(h * 128, 128)], s) for h in range(2)]

    a_groups = [
        [cp(wr_hbm, wr_buf, SEM_A)] + cp_x(0, 128, SEM_A),
        cp_x(128, 128, SEM_A + 1),
        cp_wk(0, SEM_A + 2),
        cp_wk(1, SEM_A + 3),
        cp_wk(2, SEM_A + 4) + cp_x(256, 128, SEM_A + 4) + cp_wk(3, SEM_A + 4),
        cp_x(384, 384, SEM_A + 5),
        cp_x(768, 256, SEM_A + 6) + [cp(wqkv_hbm.at[:, pl.ds(0, D)], wq_buf, SEM_A + 6)],
    ]

    def cp_b(j, wait_only=False):
        def off(v, m):
            return v if isinstance(v, int) else _mo(v, m)
        out = []
        for g in (j, j + 4):
            c0 = off(g * 128, 128)
            dst = wv_buf.at[:, pl.ds(c0, 128)]
            out.append(cp(dst if wait_only else wqkv_hbm.at[:, pl.ds(2 * D + c0, 128)], dst, SEM_B + j))
            dst = wo_buf.at[pl.ds(c0, 128), :]
            out.append(cp(dst if wait_only else wo_hbm.at[pl.ds(c0, 128), :], dst, SEM_B + j))
        f0 = off(j * FW, 128)
        for src, dst in ((wg_hbm.at[:, pl.ds(f0, FW)], wg_buf.at[j]),
                         (wu_hbm.at[:, pl.ds(f0, FW)], wu_buf.at[j]),
                         (wd_hbm.at[pl.ds(f0, FW), :], wd_buf.at[j])):
            out.append(cp(dst if wait_only else src, dst, SEM_B + j))
        return out

    clock = [0]
    toks = []
    sides = []
    fwd = [None]

    def emit_tok(vals, stamp=None):
        t = None
        for v in vals:
            v = pltpu.bitcast(v, u32) if v.dtype != u32 else v
            t = v if t is None else t | v
        toks.append((clock[0] if stamp is None else stamp, t & zero_buf[0]))

    def gate(v):
        if fwd[0] is None:
            return v
        if fwd[0][1] is None:
            fwd[0][1] = pltpu.bitcast(fwd[0][0](), u32) & zero_buf[0]
        head = pltpu.bitcast(pltpu.bitcast(v[0:8], u32) | fwd[0][1], v.dtype)
        return head if v.shape[0] == 8 else jnp.concatenate([head, v[8:]], axis=0)

    def add_side(gen_fn, n, t0, t1, lag=None):
        st = {"i": 0, "n": n, "t0": clock[0] + t0, "t1": clock[0] + t1}

        def tok(vals):
            if lag is not None:
                emit_tok(vals, st["t0"] + (st["i"] + 1) * (st["t1"] - st["t0"]) // st["n"] + lag)
        st["g"] = gen_fn(tok)
        sides.append(st)

    def advance(until):
        for st in sides:
            while st["i"] < st["n"] and st["t0"] + st["i"] * (st["t1"] - st["t0"]) // st["n"] < until:
                next(st["g"], None)
                st["i"] += 1

    def finish():
        for st in sides:
            for _ in st["g"]:
                pass
        sides.clear()
        toks.clear()
        fwd[0] = None

    def mm(lhs, rhs, dims, cycles, nseg=1):
        due = [t for (c, t) in toks if c <= clock[0]]
        toks[:] = [(c, t) for (c, t) in toks if c > clock[0]]
        if due:
            head = rhs[0:8, 0:128]
            for t in due:
                head = head | t
            if rhs.shape[1] > 128:
                head = jnp.concatenate([head, rhs[0:8, 128:]], axis=1)
            rhs = jnp.concatenate([head, rhs[8:]], axis=0)
        res = _dot(lhs, _unpack(rhs), dims)
        ngr = res.shape[0] // 16
        for sg in range(nseg):
            for i in range(ngr):
                fwd[0] = [lambda sg=sg, i=i: res[i * 16:i * 16 + 8, sg * 128:(sg + 1) * 128], None]
                clock[0] += cycles // nseg // ngr
                advance(clock[0])
        return res

    def ln_rows(p_start, n_rows, tok):
        wr = wr_buf[...].reshape(1, D).astype(f32)
        lane = lax.broadcasted_iota(i32, (8, 128), 1)
        for c in range(n_rows // 16):
            p0 = p_start + c * 16
            ds_, rss, sts = [], [], []
            for r0 in (p0, p0 + 8, HP + p0, HP + p0 + 8):
                xv = x_buf[r0:r0 + 8, :].astype(f32)
                xg = jnp.concatenate([gate(xv[:, 0:128]), xv[:, 128:]], axis=1)
                mf = jnp.sum(xg, axis=1, keepdims=True) * (1.0 / D)
                d = xv - mf
                var = jnp.sum(d * d, axis=1, keepdims=True) * (1.0 / D)
                tr = jnp.sum(d * wr, axis=1, keepdims=True)
                rs = jnp.broadcast_to(lax.rsqrt(var + 1e-5), (8, 128))
                mf = jnp.broadcast_to(mf, (8, 128))
                sa[r0:r0 + 8, :] = 1.0 + rs
                sb[r0:r0 + 8, :] = mf * rs
                st = jnp.where(lane == 0, mf, jnp.where(lane == 1, jnp.broadcast_to(var, (8, 128)),
                                                        jnp.broadcast_to(tr, (8, 128))))
                stats[r0:r0 + 8, :] = st
                ds_.append(d)
                rss.append(rs)
                sts.append(st)
                yield
            pend.append((p0, ds_, rss, sts))
            if len(pend) > 1:
                yield from ln_finish(tok, *pend.pop(0))
        while pend:
            yield from ln_finish(tok, *pend.pop(0))

    pend = []

    def ln_finish(tok, p0, ds_, rss, sts):
        for ct in range(4):
            cl = slice(ct * 128, (ct + 1) * 128)
            cr = slice(HD + ct * 128, HD + (ct + 1) * 128)
            rg = [gate(r) for r in rss]
            x11, x12, x21, x22 = [
                jnp.concatenate([ds_[i][:, cc] * rg[i], ds_[i + 1][:, cc] * rg[i + 1]], axis=0)
                for i, cc in ((0, cl), (0, cr), (2, cl), (2, cr))]
            ops = (x11, x22, x11 + x22, x21 + x22, x11 + x12, x21 - x11, x12 - x22)
            for k in range(7):
                xs.at[k][p0 // 2:p0 // 2 + 8, cl] = _pack(ops[k])
            if tok is not None:
                tok([ops[3][0:8], ops[3][8:16], ops[4][0:8], ops[4][8:16], sts[ct]])
            yield

    def wk_prep(c, tok=None):
        for i in range(HD // 16):
            r0 = i * 16
            top = wk_buf[c, r0:r0 + 16, :].astype(f32)
            bot = wk_buf[c, HD + r0:HD + r0 + 16, :].astype(f32)
            ops = _rform(gate(top[:, :128]), top[:, 128:], bot[:, :128], gate(bot[:, 128:]))
            for k in range(7):
                wks.at[k][r0 // 2:r0 // 2 + 8, c * 128:(c + 1) * 128] = _pack(ops[k])
            yield

    def wq_prep(tok):
        def transpose(g):
            for ct in range(8):
                tile = gate(pltpu.bitcast(wq_buf[ct * 128:(ct + 1) * 128, g * 128:(g + 1) * 128], u32))
                wqt.at[g * 8 + ct][...] = pltpu.bitcast(_unpack(tile).T, u32)
                yield

        def combine(g):
            for j in range(4):
                for ct in range(4):
                    w11, w12, w21, w22 = [
                        _unpack(gate(wqt[g * 8 + cc, pl.ds(jj, 8, stride=8), :])).astype(f32)
                        for jj, cc in ((j, ct), (j, ct + 4), (j + 4, ct), (j + 4, ct + 4))]
                    ops = _rform(w11, w21, w12, w22)
                    for k in range(7):
                        wqs.at[k][j * 64 + g * 8:j * 64 + g * 8 + 8, ct * 128:(ct + 1) * 128] = _pack(ops[k])
                    tok([ops[5][0:8], ops[6][0:8]])
                    yield

        for g in range(9):
            if g < 8:
                yield from transpose(g)
            if g > 0:
                yield from combine(g - 1)

    def kproj(p0, n, chunks=range(4)):
        pr = pl.ds(p0 // 2, n // 2)
        for c in chunks:
            cs = slice(c * 128, (c + 1) * 128)
            m = [None] * 7
            for k in K_SEQ:
                m[k] = mm(_unpack(xs[L_ORD[k], pr, :]), wks[k, :, cs], NN, n)
            k11, k12, k21, k22 = [_phi(v) for v in _combine(m)]
            zl = (k11 + k21).reshape(n // 8, 8, 128).sum(axis=0)
            zr = (k12 + k22).reshape(n // 8, 8, 128).sum(axis=0)
            zacc[:, cs] += zl
            zacc[:, HD + c * 128:HD + (c + 1) * 128] += zr
            ops = _lform(k11, k21, k12, k22)
            for k in range(7):
                ps.at[k][pr, cs] = _pack(ops[k])

    def z_prep():
        z = jnp.sum(zacc[...], axis=0, keepdims=True)
        zt = _pack(jnp.broadcast_to(z, (128, D)).astype(bf16).T)
        for g in range(8):
            tscr.at[g][...] = zt[g * 64:(g + 1) * 64, :]
        for j in range(8):
            blk = jnp.concatenate([tscr[g, pl.ds(j, 8, stride=8), :] for g in range(8)], axis=0)
            zp[:, j * 128:(j + 1) * 128] = _unpack(blk).T[0:8, :].astype(f32)

    def route(tok):
        rows = []
        for b in range(S // 128):
            rows.append(gate(stats[b * 128:(b + 1) * 128, :]).T[0:8, :])
            yield
        mf = jnp.concatenate([v[0:1] for v in rows], axis=0)
        var = jnp.concatenate([v[1:2] for v in rows], axis=0)
        tr = jnp.concatenate([v[2:3] for v in rows], axis=0)
        wsum = jnp.sum(wr_buf[...].reshape(1, D).astype(f32), axis=1, keepdims=True)
        sd = _rbf(jnp.sqrt(_rbf(_rbf(var) + 1e-5)))
        rv = _rbf((tr + (mf - _rbf(mf)) * wsum) / sd)
        rmax = jnp.max(rv)
        pos = (lax.broadcasted_iota(i32, rv.shape, 0) * 128 + lax.broadcasted_iota(i32, rv.shape, 1))
        idx = jnp.min(jnp.where(rv == rmax, pos, S - 1))
        idx_s[0] = idx
        rsel[...] = jnp.full(rsel.shape, rmax, f32)
        b0 = _mo((idx // 16) * 16, 16)
        xn = _rbf(_layernorm_rows(x_buf[pl.ds(b0, 16), :].astype(f32)))
        sel = lax.broadcasted_iota(i32, xn.shape, 0) == idx - b0
        row = jnp.sum(jnp.where(sel, xn, 0.0), axis=0, keepdims=True)
        xbv = jnp.broadcast_to(row, (128, D)).T
        xb[...] = xbv
        yacc[...] = jnp.zeros(yacc.shape, f32)
        tok([xbv[b * 128 + 120:(b + 1) * 128] for b in range(8)])
        yield

    def q_part(j, r0, nr, spread=0):
        pr = pl.ds(_mo((j * R + r0) // 2, 8), nr // 2)
        pq = pq_buf.at[j % 2]
        rr = slice(r0, r0 + nr)
        den = [None, None]
        for c in range(4):
            m = [mm(_unpack(xs[L_ORD[k], pr, :]), wqs[k, c * 64:(c + 1) * 64, :], NT_, nr)
                 for k in range(7)]
            q11, q12, q21, q22 = [_phi(v) for v in _combine(m)]
            cl = slice(c * 128, (c + 1) * 128)
            cr = slice(HD + c * 128, HD + (c + 1) * 128)
            zl, zr = zp[0:1, cl], zp[0:1, cr]
            dt, db = q11 * zl + q12 * zr, q21 * zl + q22 * zr
            den = [dt, db] if c == 0 else [den[0] + dt, den[1] + db]
            pq.at[0][rr, cl] = q11
            pq.at[0][rr, cr] = q12
            pq.at[1][rr, cl] = q21
            pq.at[1][rr, cr] = q22
            if c < 3:
                emit_tok([d[i * 8:(i + 1) * 8] for d in den for i in range(nr // 8)], clock[0] + QLAG)
                yield
        lane = lax.broadcasted_iota(i32, (16, 128), 1)

        def normalise(tok):
            for c in range(nr // 16):
                recs = []
                for d in den:
                    d = d[c * 16:(c + 1) * 16]
                    if spread:
                        d = jnp.concatenate([gate(d[0:8]), gate(d[8:16])], axis=0)
                    d = d + jnp.where(lane % 2 == 0, pltpu.roll(d, 127, 1), pltpu.roll(d, 1, 1))
                    d = d + jnp.where(lane % 4 < 2, pltpu.roll(d, 126, 1), pltpu.roll(d, 2, 1))
                    recs.append(1.0 / (d + 1e-6))
                rq = slice(r0 + c * 16, r0 + (c + 1) * 16)
                p2 = pl.ds(_mo((j * R + r0) // 2 + c * 8, 8), 8)
                yield
                yield
                for ct in range(4):
                    cl = slice(ct * 128, (ct + 1) * 128)
                    cr = slice(HD + ct * 128, HD + (ct + 1) * 128)
                    rc = recs
                    if spread:
                        rc = [jnp.concatenate([gate(r[0:8]), gate(r[8:16])], axis=0) for r in recs]
                    ops = _lform(pq[0, rq, cl] * rc[0], pq[0, rq, cr] * rc[0],
                                 pq[1, rq, cl] * rc[1], pq[1, rq, cr] * rc[1])
                    for k in range(7):
                        qs.at[k][p2, cl] = _pack(ops[k])
                    yield

        if spread:
            emit_tok([d[i * 8:(i + 1) * 8] for d in den for i in range(nr // 8)], clock[0] + QLAG)
            add_side(normalise, 6 * (nr // 16), 256, spread)
        else:
            for _ in normalise(None):
                pass
        yield

    def b_tile(j):
        jc = pl.ds(_mo(j * 128, 128), 128)
        z_prep()
        for _ in q_part(j, 0, QA, 6000):
            pass
        m = [mm(_unpack(ps[k, :, jc]), xs[R_ORD[k]], TN, 1024, 4) for k in range(7)]
        g11, g12, g21, g22 = _combine(m)
        hm = (lax.broadcasted_iota(i32, (128, 128), 0) // 32
              == lax.broadcasted_iota(i32, (128, 128), 1) // 32)
        qb = q_part(j, QA, R - QA)
        next(qb)
        kvps = []
        for half, (ga, gb) in enumerate(((g11, g12), (g21, g22))):
            gc = pl.ds(_mo((j + 4 * half) * 128, 128), 128)
            gg = jnp.concatenate([ga, gb], axis=1).astype(bf16)
            clock[0] += 256
            kv = jnp.where(hm, _dot(gg, wv_buf[:, gc], NN), 0.0)
            tscr2.at[half][...] = _pack(kv)
            kvps.append(_unpack(jnp.concatenate(
                [tscr2[half, pl.ds(jj, 8, stride=8), :] for jj in (0, 4, 1, 5, 2, 6, 3, 7)], axis=0)))
        for _ in qb:
            pass
        for half in range(2):
            g = j + 4 * half
            gr = pl.ds(_mo(g * 128, 128), 128)
            for c in range(2):
                cl = slice(c * 256, (c + 1) * 256)
                wo2 = jnp.concatenate([wo_buf[gr, cl], wo_buf[gr, HD + c * 256:HD + (c + 1) * 256]], axis=1)
                clock[0] += 128
                mg = _dot(kvps[half], wo2, NN)
                for jj in range(4):
                    top, bot = mg[jj * 32:jj * 32 + 16], mg[jj * 32 + 16:(jj + 1) * 32]
                    ops = _rform(top[:, :256], top[:, 256:], bot[:, :256], bot[:, 256:])
                    for k in range(7):
                        ms.at[k][pl.ds(_mo(jj * 64 + g * 8, 8), 8), cl] = _pack(ops[k])

    def out_part(p0, nr, y):
        pr = pl.ds(_mo(p0 // 2, 8), nr // 2)
        rows = (pl.ds(_mo(p0, 16), nr), pl.ds(_mo(HP + p0, 16), nr))
        row = lax.broadcasted_iota(i32, (nr, 256), 0) + p0
        hit = (row == idx_s[0], row + HP == idx_s[0])
        for c in range(2):
            cl = pl.ds(c * 256, 256)
            cr = pl.ds(HD + c * 256, 256)
            m = [_dot(_unpack(qs[k, pr, :]), _unpack(ms[k, :, cl]), NN) for k in range(7)]
            o11, o12, o21, o22 = _combine(m)
            for h, cc, o in ((1, cr, o22), (1, cl, o21), (0, cr, o12), (0, cl, o11)):
                rr = rows[h]
                a = jnp.concatenate([sa[rr, :]] * 2, axis=1)
                b = jnp.concatenate([sb[rr, :]] * 2, axis=1)
                o = o + jnp.where(hit[h], y[:, cc.start:cc.start + 256], 0.0)
                out_buf[rr, cc] = (x_buf[rr, cc].astype(f32) * a - b + o).astype(bf16)
                cp(out_buf.at[rr, cc], out_hbm.at[0, rr, cc], SEM_O).start()

    def ffn_chunk(c, tok):
        hs = []
        for f0 in range(0, FW, 256):
            w = min(256, FW - f0)
            fs = slice(f0, f0 + w)
            ag = jnp.zeros((8, w), f32)
            au = jnp.zeros((8, w), f32)
            step = FSTEP * 256 // w
            for kg in range(D // 8):
                xv = jnp.concatenate([gate(xb[8 * kg:8 * kg + 8, :])] * (w // 128), axis=1)
                ag = ag + wg_buf[c, 8 * kg:8 * kg + 8, fs].astype(f32) * xv
                au = au + wu_buf[c, 8 * kg:8 * kg + 8, fs].astype(f32) * xv
                if kg % step == step - 1:
                    tok([a[:, i * 128:(i + 1) * 128] for a in (ag, au) for i in range(w // 128)])
                    yield
            g = _rbf(jnp.sum(ag, axis=0, keepdims=True))
            u = _rbf(jnp.sum(au, axis=0, keepdims=True))
            h = _rbf(_rbf(g * jax.nn.sigmoid(g)) * u)
            hb_buf.at[c % 2][fs, :] = jnp.broadcast_to(h, (128, w)).T
        for d0 in range(0, D, 512):
            ds_ = slice(d0, d0 + 512)
            acc = yacc[:, ds_]
            for kg in range(FW // 8):
                hv = jnp.concatenate([gate(hb_buf[c % 2, 8 * kg:8 * kg + 8, :])] * 4, axis=1)
                acc = acc + wd_buf[c, 8 * kg:8 * kg + 8, ds_].astype(f32) * hv
                if kg % FSTEP == FSTEP - 1:
                    tok([acc[:, i * 128:(i + 1) * 128] for i in range(4)])
                    yield
            yacc[:, ds_] = acc

    def wait_group(i):
        with _scope("a_wait%d" % i):
            for c in a_groups[i]:
                c.wait()

    def run_all(gen):
        for _ in gen:
            pass

    def ln_side(p0, n, t0, t1):
        add_side(lambda tok: ln_rows(p0, n, tok), n // 2, t0, t1, SLAG)

    with _scope("p0_issue"):
        for grp in a_groups:
            for c in grp:
                c.start()
        for j in range(NT):
            for c in cp_b(j):
                c.start()
        zacc[...] = jnp.zeros(zacc.shape, f32)
        zero_buf[1] = jnp.zeros((8, 128), u32)
        cp_zero = cp(zero_buf.at[1], zero_buf.at[0], SEM_Z)
        cp_zero.start()
        cp_zero.wait()
    wait_group(0)
    with _scope("a0"):
        run_all(ln_rows(0, 128, None))
    wait_group(1)
    with _scope("a1"):
        run_all(ln_rows(128, 128, None))
    wait_group(2)
    with _scope("a2"):
        run_all(wk_prep(0))
        kproj(0, 256, [0])
        finish()
    wait_group(3)
    with _scope("a3"):
        run_all(wk_prep(1))
        kproj(0, 256, [1])
        finish()
    wait_group(4)
    with _scope("a4"):
        run_all(wk_prep(2))
        add_side(lambda tok: wk_prep(3), 32, 300, 1500)
        ln_side(256, 128, 0, 3300)
        kproj(0, 256, [2, 3])
        finish()
    wait_group(5)
    with _scope("a5"):
        for p0 in (256, 384, 512):
            ln_side(p0 + 128, 128, 0, 3200)
            kproj(p0, 128)
        finish()
    wait_group(6)
    with _scope("a6"):
        add_side(wq_prep, 8 * 24, 0, 10000, SLAG)
        for p0 in (640, 768):
            ln_side(p0 + 128, 128, 0, 3200)
            kproj(p0, 128)
        add_side(route, 17, 0, 800)
        kproj(896, 128)
        finish()

    def b_body(j, carry):
        with _scope("b_wait"):
            for c in cp_b(j, wait_only=True):
                c.wait()
        with _scope("b_body"):
            add_side(lambda tok: ffn_chunk(j, tok), (56 + 28) * 8 // FSTEP, 0, 13500)
            b_tile(j)
            finish()
        return carry

    if UNROLL_B:
        for j in range(NT):
            b_body(j, 0)
    else:
        lax.fori_loop(0, NT, b_body, 0)

    def c_body(t, carry):
        with _scope("c_body"):
            y = _rbf(jnp.sum(yacc[...], axis=0, keepdims=True))
            y = _rbf(y * _rbf(jax.nn.sigmoid(rsel[...])))
            for p in range(R // CR):
                out_part(t * R + p * CR, CR, y)
        return carry

    lax.fori_loop(0, NT, c_body, 0)
    with _scope("tail"):
        cp(out_buf, out_hbm.at[0], SEM_O).wait()


@jax.jit
def pallas_parallel_sum__linear_attn_block__moe_arch_mod__prompt_kernel(
    A_x: jax.Array,
    A_wqkv: jax.Array,
    A_wo: jax.Array,
    B_x: jax.Array,
    B_w_r: jax.Array,
    B_w_gate: jax.Array,
    B_w_up: jax.Array,
    B_w_down: jax.Array,
):
    del B_x
    V = pltpu.VMEM
    scratch = [
        V((S, D), bf16),
        V((4, D, 256), bf16),
        V((D, D), bf16),
        V((D, D), bf16),
        V((D, D), bf16),
        V((D,), bf16),
        V((NF, D, FW), bf16),
        V((NF, D, FW), bf16),
        V((NF, FW, D), bf16),
        V((7, HP // 2, HD), u32),
        V((7, HP // 2, HD), u32),
        V((7, HP // 2, HD), u32),
        V((7, HD // 2, HD), u32),
        V((7, HD // 2, HD), u32),
        V((7, HD // 2, HD), u32),
        V((S, 128), f32),
        V((S, 128), f32),
        V((S, 128), f32),
        V((8, D), f32),
        V((8, D), f32),
        V((8, 64, 128), u32),
        V((2, 64, 128), u32),
        V((64, 64, 128), u32),
        V((2, 2, R, D), f32),
        V((D, 128), f32),
        V((2, FW, 128), f32),
        V((8, D), f32),
        V((1, D), f32),
        V((S, D), bf16),
        V((2, 8, 128), u32),
        pltpu.SMEM((1,), i32),
        pltpu.SemaphoreType.DMA((NT + 9,)),
    ]
    return pl.pallas_call(
        _kernel,
        out_shape=jax.ShapeDtypeStruct((1, S, D), bf16),
        in_specs=[pl.BlockSpec(memory_space=pl.ANY)] * 7,
        out_specs=pl.BlockSpec(memory_space=pl.ANY),
        scratch_shapes=scratch,
        compiler_params=pltpu.CompilerParams(vmem_limit_bytes=110 * 1024 * 1024,
                                             disable_bounds_checks=True,
                                             disable_semaphore_checks=True),
    )(A_x, A_wqkv, A_wo, B_w_r, B_w_gate, B_w_up, B_w_down)
```

```python
import contextlib

import jax
import jax.numpy as jnp
from jax import lax
import jax.experimental.pallas as pl
import jax.experimental.pallas.tpu as pltpu

bf16, f32, u32, i32 = jnp.bfloat16, jnp.float32, jnp.uint32, jnp.int32

S = 2048
D = 1024
F = 3584
HP = S // 2
HD = D // 2
R = 256
NT = HP // R
HQ = S // 4
RQ = HQ // NT
FW = 896
NF = F // FW
QLAG = 768
UNROLL_B = False
QA = 96
NOFFN = False
SLAG = 400
FSTEP = 2
CR = 32

L_ORD = (2, 3, 0, 1, 4, 5, 6)
R_ORD = (2, 0, 6, 5, 1, 4, 3)

K_SEQ = (1, 4, 0, 2, 3, 5, 6)

NN = (((1,), (0,)), ((), ()))
NT_ = (((1,), (1,)), ((), ()))
TN = (((0,), (0,)), ((), ()))


SCOPES = False


def _scope(name):
    return jax.named_scope(name) if SCOPES else contextlib.nullcontext()


def _mo(v, m):
    return v if isinstance(v, int) else pl.multiple_of(v, m)


def _dot(a, b, dims):
    return lax.dot_general(a, b, dims, preferred_element_type=f32)


def _pack(v):
    return pltpu.bitcast(v.astype(bf16), u32)


def _unpack(v):
    return pltpu.bitcast(v, bf16)


def _combine(m):
    m1, m2, m3, m4, m5, m6, m7 = m
    return m1 + m4 - m5 + m7, m3 + m5, m2 + m4, m1 - m2 + m3 + m6


def _lform(a11, a12, a21, a22):
    return (a11 + a22, a21 + a22, a11, a22, a11 + a12, a21 - a11, a12 - a22)


def _rform(b11, b12, b21, b22):
    return (b11 + b22, b11, b12 - b22, b21 - b11, b22, b11 + b12, b21 + b22)


def _form2(form, blk):
    lvl1 = [form(blk[r][c], blk[r][c + 2], blk[r + 2][c], blk[r + 2][c + 2])
            for r in range(2) for c in range(2)]
    return [v for k1 in range(7) for v in form(*[lvl1[i][k1] for i in range(4)])]


class _Sym:
    def __init__(self, t):
        self.t = t

    def __add__(self, o):
        return _Sym({**self.t, **o.t})

    def __sub__(self, o):
        return _Sym({**self.t, **{k: -v for k, v in o.t.items()}})


def _phi(t):
    return jnp.where(t > 0, t + 1.0, jnp.exp(t)) + 1e-6


def _rbf(v):
    return v.astype(bf16).astype(f32)


def _layernorm_rows(xv):
    mf = jnp.sum(xv, axis=1, keepdims=True) * (1.0 / D)
    mb = _rbf(mf)
    d = xv - mb
    dm = mf - mb
    var = jnp.sum(d * d, axis=1, keepdims=True) * (1.0 / D) - dm * dm
    var = jnp.maximum(var, 0.0)
    sd = _rbf(jnp.sqrt(_rbf(_rbf(var) + 1e-5)))
    return d * (1.0 / sd)


def _kernel(x_hbm, wqkv_hbm, wo_hbm, wr_hbm, wg_hbm, wu_hbm, wd_hbm, out_hbm,
            x_buf, wk_buf, wq_buf, wv_buf, wo_buf, wr_buf, wg_buf, wu_buf, wd_buf,
            xs, ps, qs, wks, wqs, ms, sa, sb, stats, zacc, zp, tscr, tscr2, wqt, pq_buf, den_buf, mg_buf,
            xb, hb_buf, yacc, rsel, out_buf, zero_buf, idx_s, sem):

    SEM_B, SEM_O, SEM_Z, SEM_A = 0, NT, NT + 1, NT + 2

    def cp(src, dst, s):
        return pltpu.make_async_copy(src, dst, sem.at[s])

    def cp_x(p0, n, s):
        return [cp(x_hbm.at[0, pl.ds(h * HP + p0, n), :], x_buf.at[pl.ds(h * HP + p0, n), :], s)
                for h in range(2)]

    def cp_wk(c, s):
        return [cp(wqkv_hbm.at[:, pl.ds(D + h * HD + c * 128, 128)],
                   wk_buf.at[c, :, pl.ds(h * 128, 128)], s) for h in range(2)]

    a_groups = [
        [cp(wr_hbm, wr_buf, SEM_A)] + cp_x(0, 128, SEM_A),
        cp_x(128, 128, SEM_A + 1),
        cp_wk(0, SEM_A + 2),
        cp_wk(1, SEM_A + 3),
        cp_wk(2, SEM_A + 4) + cp_x(256, 128, SEM_A + 4) + cp_wk(3, SEM_A + 4),
        cp_x(384, 384, SEM_A + 5),
        cp_x(768, 256, SEM_A + 6) + [cp(wqkv_hbm.at[:, pl.ds(0, D)], wq_buf, SEM_A + 6)],
    ]

    def cp_b(j, wait_only=False):
        def off(v, m):
            return v if isinstance(v, int) else _mo(v, m)
        out = []
        for hh, g in enumerate((j, j + 4)):
            c0 = off(g * 128, 128)
            dst = wv_buf.at[j, :, pl.ds(hh * 128, 128)]
            out.append(cp(dst if wait_only else wqkv_hbm.at[:, pl.ds(2 * D + c0, 128)], dst, SEM_B + j))
            dst = wo_buf.at[pl.ds(c0, 128), :]
            out.append(cp(dst if wait_only else wo_hbm.at[pl.ds(c0, 128), :], dst, SEM_B + j))
        f0 = off(j * FW, 128)
        for src, dst in ((wg_hbm.at[:, pl.ds(f0, FW)], wg_buf.at[j, :, pl.ds(0, FW)]),
                         (wu_hbm.at[:, pl.ds(f0, FW)], wu_buf.at[j, :, pl.ds(0, FW)]),
                         (wd_hbm.at[pl.ds(f0, FW), :], wd_buf.at[j, pl.ds(0, FW), :])):
            out.append(cp(dst if wait_only else src, dst, SEM_B + j))
        return out

    clock = [0]
    toks = []
    sides = []
    fwd = [None]

    def emit_tok(vals, stamp=None):
        t = None
        for v in vals:
            v = pltpu.bitcast(v, u32) if v.dtype != u32 else v
            t = v if t is None else t | v
        toks.append((clock[0] if stamp is None else stamp, t & zero_buf[0]))

    def gate(v):
        if fwd[0] is None:
            return v
        if fwd[0][1] is None:
            fwd[0][1] = pltpu.bitcast(fwd[0][0](), u32) & zero_buf[0]
        head = pltpu.bitcast(pltpu.bitcast(v[0:8], u32) | fwd[0][1], v.dtype)
        return head if v.shape[0] == 8 else jnp.concatenate([head, v[8:]], axis=0)

    def add_side(gen_fn, n, t0, t1, lag=None):
        st = {"i": 0, "n": n, "t0": clock[0] + t0, "t1": clock[0] + t1}

        def tok(vals):
            if lag is not None:
                emit_tok(vals, st["t0"] + (st["i"] + 1) * (st["t1"] - st["t0"]) // st["n"] + lag)
        st["g"] = gen_fn(tok)
        sides.append(st)

    def advance(until):
        for st in sides:
            while st["i"] < st["n"] and st["t0"] + st["i"] * (st["t1"] - st["t0"]) // st["n"] < until:
                next(st["g"], None)
                st["i"] += 1

    def finish():
        for st in sides:
            for _ in st["g"]:
                pass
        sides.clear()
        toks.clear()
        fwd[0] = None

    def mm(lhs, rhs, dims, cycles, nseg=1):
        due = [t for (c, t) in toks if c <= clock[0]]
        toks[:] = [(c, t) for (c, t) in toks if c > clock[0]]
        if due:
            head = rhs[0:8, 0:128]
            for t in due:
                head = head | t
            if rhs.shape[1] > 128:
                head = jnp.concatenate([head, rhs[0:8, 128:]], axis=1)
            rhs = jnp.concatenate([head, rhs[8:]], axis=0)
        res = _dot(lhs, _unpack(rhs), dims)
        ngr = res.shape[0] // 16
        for sg in range(nseg):
            for i in range(ngr):
                fwd[0] = [lambda sg=sg, i=i: res[i * 16:i * 16 + 8, sg * 128:(sg + 1) * 128], None]
                clock[0] += cycles // nseg // ngr
                advance(clock[0])
        return res

    def ln_rows(p_start, n_rows, tok):
        wr = wr_buf[...].reshape(1, D).astype(f32)
        lane = lax.broadcasted_iota(i32, (8, 128), 1)
        for c in range(n_rows // 16):
            p0 = p_start + c * 16
            ds_, rss, sts = [], [], []
            for r0 in (p0, p0 + 8, HP + p0, HP + p0 + 8):
                xv = x_buf[r0:r0 + 8, :].astype(f32)
                xg = jnp.concatenate([gate(xv[:, 0:128]), xv[:, 128:]], axis=1)
                mf = jnp.sum(xg, axis=1, keepdims=True) * (1.0 / D)
                d = xv - mf
                var = jnp.sum(d * d, axis=1, keepdims=True) * (1.0 / D)
                tr = jnp.sum(d * wr, axis=1, keepdims=True)
                rs = jnp.broadcast_to(lax.rsqrt(var + 1e-5), (8, 128))
                mf = jnp.broadcast_to(mf, (8, 128))
                sa[r0:r0 + 8, :] = 1.0 + rs
                sb[r0:r0 + 8, :] = mf * rs
                st = jnp.where(lane == 0, mf, jnp.where(lane == 1, jnp.broadcast_to(var, (8, 128)),
                                                        jnp.broadcast_to(tr, (8, 128))))
                stats[r0:r0 + 8, :] = st
                ds_.append(d)
                rss.append(rs)
                sts.append(st)
                yield
            pend.append((p0, ds_, rss, sts))
            if len(pend) > 1:
                yield from ln_finish(tok, *pend.pop(0))
        while pend:
            yield from ln_finish(tok, *pend.pop(0))

    pend = []

    def ln_finish(tok, p0, ds_, rss, sts):
        for ct in range(4):
            cl = slice(ct * 128, (ct + 1) * 128)
            cr = slice(HD + ct * 128, HD + (ct + 1) * 128)
            rg = [gate(r) for r in rss]
            x11, x12, x21, x22 = [
                jnp.concatenate([ds_[i][:, cc] * rg[i], ds_[i + 1][:, cc] * rg[i + 1]], axis=0)
                for i, cc in ((0, cl), (0, cr), (2, cl), (2, cr))]
            ops = (x11, x22, x11 + x22, x21 + x22, x11 + x12, x21 - x11, x12 - x22)
            for k in range(7):
                xs.at[k][p0 // 2:p0 // 2 + 8, cl] = _pack(ops[k])
            if tok is not None:
                tok([ops[3][0:8], ops[3][8:16], ops[4][0:8], ops[4][8:16]])
            yield

    def wk_prep(c, tok=None):
        for i in range(HD // 16):
            r0 = i * 16
            top = wk_buf[c, r0:r0 + 16, :].astype(f32)
            bot = wk_buf[c, HD + r0:HD + r0 + 16, :].astype(f32)
            ops = _rform(gate(top[:, :128]), top[:, 128:], bot[:, :128], gate(bot[:, 128:]))
            for k in range(7):
                wks.at[k][r0 // 2:r0 // 2 + 8, c * 128:(c + 1) * 128] = _pack(ops[k])
            yield

    def wq_prep(tok):
        def transpose(g):
            for ct in range(8):
                tile = gate(pltpu.bitcast(wq_buf[ct * 128:(ct + 1) * 128, g * 128:(g + 1) * 128], u32))
                wqt.at[g * 8 + ct][...] = pltpu.bitcast(_unpack(tile).T, u32)
                yield

        def combine(g):
            for j in range(4):
                for ct in range(4):
                    w11, w12, w21, w22 = [
                        _unpack(gate(wqt[g * 8 + cc, pl.ds(jj, 8, stride=8), :])).astype(f32)
                        for jj, cc in ((j, ct), (j, ct + 4), (j + 4, ct), (j + 4, ct + 4))]
                    ops = _rform(w11, w21, w12, w22)
                    for k in range(7):
                        wqs.at[k][j * 64 + g * 8:j * 64 + g * 8 + 8, ct * 128:(ct + 1) * 128] = _pack(ops[k])
                    tok([ops[5][0:8], ops[6][0:8]])
                    yield

        for g in range(9):
            if g < 8:
                yield from transpose(g)
            if g > 0:
                yield from combine(g - 1)

    def kproj(p0, n, chunks=range(4)):
        pr = pl.ds(p0 // 2, n // 2)
        for c in chunks:
            cs = slice(c * 128, (c + 1) * 128)
            m = [None] * 7
            for k in K_SEQ:
                m[k] = mm(_unpack(xs[L_ORD[k], pr, :]), wks[k, :, cs], NN, n)
            k11, k12, k21, k22 = [_phi(v) for v in _combine(m)]
            zl = (k11 + k21).reshape(n // 8, 8, 128).sum(axis=0)
            zr = (k12 + k22).reshape(n // 8, 8, 128).sum(axis=0)
            zacc[:, cs] += zl
            zacc[:, HD + c * 128:HD + (c + 1) * 128] += zr
            ops = _lform(k11, k21, k12, k22)
            for k in range(7):
                ps.at[c][pr, k * 128:(k + 1) * 128] = _pack(ops[k])

    def z_prep():
        z = jnp.sum(zacc[...], axis=0, keepdims=True)
        zt = _pack(jnp.broadcast_to(z, (128, D)).astype(bf16).T)
        for g in range(8):
            tscr.at[g][...] = zt[g * 64:(g + 1) * 64, :]
        for j in range(8):
            blk = jnp.concatenate([tscr[g, pl.ds(j, 8, stride=8), :] for g in range(8)], axis=0)
            zp[:, j * 128:(j + 1) * 128] = _unpack(blk).T[0:8, :].astype(f32)

    def route(tok):
        rows = []
        for b in range(S // 128):
            rows.append(gate(stats[b * 128:(b + 1) * 128, :]).T[0:8, :])
            yield
        mf = jnp.concatenate([v[0:1] for v in rows], axis=0)
        var = jnp.concatenate([v[1:2] for v in rows], axis=0)
        tr = jnp.concatenate([v[2:3] for v in rows], axis=0)
        wsum = jnp.sum(wr_buf[...].reshape(1, D).astype(f32), axis=1, keepdims=True)
        sd = _rbf(jnp.sqrt(_rbf(_rbf(var) + 1e-5)))
        rv = _rbf((tr + (mf - _rbf(mf)) * wsum) / sd)
        rmax = jnp.max(rv)
        pos = (lax.broadcasted_iota(i32, rv.shape, 0) * 128 + lax.broadcasted_iota(i32, rv.shape, 1))
        idx = jnp.min(jnp.where(rv == rmax, pos, S - 1))
        idx_s[0] = idx
        rsel[...] = jnp.full(rsel.shape, rmax, f32)
        b0 = _mo((idx // 16) * 16, 16)
        xn = _rbf(_layernorm_rows(x_buf[pl.ds(b0, 16), :].astype(f32)))
        sel = lax.broadcasted_iota(i32, xn.shape, 0) == idx - b0
        row = jnp.sum(jnp.where(sel, xn, 0.0), axis=0, keepdims=True)
        xbv = jnp.broadcast_to(row, (128, D)).T
        xb[...] = xbv
        yacc[...] = jnp.zeros(yacc.shape, f32)
        tok([xbv[b * 128 + 120:(b + 1) * 128] for b in range(8)])
        yield

    def form2_steps(form, get, put):
        terms = form(*[_Sym({i: 1}) for i in range(4)])
        for k1 in range(7):
            sub = []
            for r in range(2):
                for c in range(2):
                    v = None
                    for i, sg in sorted(terms[k1].t.items(), key=lambda e: -e[1]):
                        b = get(r + 2 * (i // 2), c + 2 * (i % 2))
                        if v is None:
                            v = gate16(b) if r == c else b
                        else:
                            v = v + b if sg > 0 else v - b
                    sub.append(v)
            for k2, v in enumerate(form(*sub)):
                put(k1 * 7 + k2, _pack(v))
            yield

    def gate16(v):
        return jnp.concatenate([gate(v[0:8]), gate(v[8:16])], axis=0)

    def q_part(j, r0, nr):
        prs = [pl.ds(_mo((h * HQ + j * RQ + r0) // 2, 8), nr // 2) for h in range(2)]
        pq = pq_buf.at[j % 2]
        rr = slice(r0, r0 + nr)
        den = [None, None]
        for c in range(4):
            m = [mm(_unpack(jnp.concatenate([xs[L_ORD[k], pr, :] for pr in prs], axis=0)),
                    wqs[k, c * 64:(c + 1) * 64, :], NT_, 2 * nr) for k in range(7)]
            q11, q12, q21, q22 = [_phi(v) for v in _combine(m)]
            cl = slice(c * 128, (c + 1) * 128)
            cr = slice(HD + c * 128, HD + (c + 1) * 128)
            zl, zr = zp[0:1, cl], zp[0:1, cr]
            dt, db = q11 * zl + q12 * zr, q21 * zl + q22 * zr
            den = [dt, db] if c == 0 else [den[0] + dt, den[1] + db]
            for h in range(2):
                hs = slice(h * nr, (h + 1) * nr)
                pq.at[h][rr, cl] = q11[hs]
                pq.at[h][rr, cr] = q12[hs]
                pq.at[2 + h][rr, cl] = q21[hs]
                pq.at[2 + h][rr, cr] = q22[hs]
            emit_tok([d[i * 8:(i + 1) * 8] for d in den for i in range(nr // 4)], clock[0] + QLAG)
            if c == 3:
                for q in range(4):
                    den_buf.at[j % 2, q][rr, :] = den[q // 2][(q % 2) * nr:(q % 2 + 1) * nr]
            yield

    def normalise(j, r0, nr, jq):
        pq = pq_buf.at[j % 2]
        lane = lax.broadcasted_iota(i32, (16, 128), 1)

        def recips(c):
            rq = slice(r0 + c * 16, r0 + (c + 1) * 16)
            recs = []
            for q in range(4):
                d = gate16(den_buf[j % 2, q, rq, :])
                d = d + jnp.where(lane % 2 == 0, pltpu.roll(d, 127, 1), pltpu.roll(d, 1, 1))
                d = d + jnp.where(lane % 4 < 2, pltpu.roll(d, 126, 1), pltpu.roll(d, 2, 1))
                recs.append(1.0 / (d + 1e-6))
            return recs

        nxt = recips(0)
        for _ in range(4):
            yield
        for c in range(nr // 16):
            rq = slice(r0 + c * 16, r0 + (c + 1) * 16)
            p2 = pl.ds(_mo((jq * RQ + r0) // 2 + c * 8, 8), 8)
            recs = nxt
            for q in range(4):
                for hf in range(2):
                    cs = slice(hf * HD, (hf + 1) * HD)
                    pq.at[q][rq, cs] = pq[q, rq, cs] * jnp.concatenate([gate16(recs[q])] * 4, axis=1)
                    yield
            if c + 1 < nr // 16:
                nxt = recips(c + 1)
            yield
            for ct in range(2):
                def put(k, v):
                    qs.at[k][p2, ct * 128:(ct + 1) * 128] = v
                yield from form2_steps(
                    _lform, lambda q, u: pq[q, rq, u * 256 + ct * 128:u * 256 + (ct + 1) * 128], put)

    def b_tile(j):
        jc = pl.ds(_mo(j * 128, 128), 128)
        z_prep()
        nb = RQ - QA
        add_side(lambda tok: normalise(j + 1, QA, nb, (j + 3) % 4), 4 + 23 * (nb // 16), 0, 14 * QA * 4)
        for _ in q_part(j, 0, QA):
            pass
        add_side(lambda tok: normalise(j, 0, QA, j), 4 + 23 * (QA // 16), 400, 7000)
        m = [mm(_unpack(ps[j, :, k * 128:(k + 1) * 128]), xs[R_ORD[k]], TN, 1024, 4) for k in range(7)]
        g11, g12, g21, g22 = _combine(m)
        hm = (lax.broadcasted_iota(i32, (128, 128), 0) // 32
              == lax.broadcasted_iota(i32, (128, 128), 1) // 32)
        qb = q_part(j, QA, nb)
        next(qb)
        kvps = []
        for half, (ga, gb) in enumerate(((g11, g12), (g21, g22))):
            gc = pl.ds(_mo((j + 4 * half) * 128, 128), 128)
            gg = jnp.concatenate([ga, gb], axis=1).astype(bf16)
            clock[0] += 256
            kv = jnp.where(hm, _dot(gg, wv_buf[j, :, half * 128:(half + 1) * 128], NN), 0.0)
            tscr2.at[half][...] = _pack(kv)
            kvps.append(_unpack(jnp.concatenate(
                [tscr2[half, pl.ds(jj, 8, stride=8), :] for jj in range(8)], axis=0)))
        next(qb)
        mg = mg_buf.at[j % 2]
        for half in range(2):
            gr = pl.ds(_mo((j + 4 * half) * 128, 128), 128)
            clock[0] += 256
            mg.at[half][...] = _dot(kvps[half], wo_buf[gr, :], NN)

        def m_form(tok):
            for half in range(2):
                g = j + 4 * half
                for jj in range(2):
                    for ct in range(2):
                        def put(k, v):
                            ms.at[k][pl.ds(_mo(jj * 64 + g * 8, 8), 8), ct * 128:(ct + 1) * 128] = v
                        yield from form2_steps(
                            _rform, lambda q, u: mg[half, (2 * q + jj) * 16:(2 * q + jj + 1) * 16,
                                                    u * 256 + ct * 128:u * 256 + (ct + 1) * 128], put)

        add_side(m_form, 56, 0, 28 * nb - 100)
        for _ in qb:
            pass

    def out_part(p0, nr, y):
        pr = pl.ds(_mo(p0 // 2, 8), nr // 2)
        rows = [pl.ds(_mo(q * HQ + p0, 16), nr) for q in range(4)]
        row = lax.broadcasted_iota(i32, (nr, 256), 0) + p0
        m1 = []
        for k1 in range(7):
            m2 = [_dot(_unpack(qs[k1 * 7 + k2, pr, :]), _unpack(ms[k1 * 7 + k2]), NN) for k2 in range(7)]
            m1.append(_combine(m2))
        for s2 in range(4):
            outs = _combine([m1[k1][s2] for k1 in range(7)])
            for s1 in range(4):
                q = (s1 // 2) * 2 + s2 // 2
                u = (s1 % 2) * 2 + s2 % 2
                rr, cc = rows[q], pl.ds(u * 256, 256)
                a = jnp.concatenate([sa[rr, :]] * 2, axis=1)
                b = jnp.concatenate([sb[rr, :]] * 2, axis=1)
                o = outs[s1] + jnp.where(row + q * HQ == idx_s[0], y[:, u * 256:(u + 1) * 256], 0.0)
                out_buf[rr, cc] = (x_buf[rr, cc].astype(f32) * a - b + o).astype(bf16)
        for q in range(4):
            cp(out_buf.at[rows[q], :], out_hbm.at[0, rows[q], :], SEM_O).start()

    def ffn_chunk(c, tok):
        hs = []
        for f0 in range(0, FW, 256):
            w = min(256, FW - f0)
            fs = slice(f0, f0 + w)
            ag = jnp.zeros((8, w), f32)
            au = jnp.zeros((8, w), f32)
            step = FSTEP * 256 // w
            for kg in range(D // 8):
                xv = jnp.concatenate([gate(xb[8 * kg:8 * kg + 8, :])] * (w // 128), axis=1)
                ag = ag + wg_buf[c, 8 * kg:8 * kg + 8, fs].astype(f32) * xv
                au = au + wu_buf[c, 8 * kg:8 * kg + 8, fs].astype(f32) * xv
                if kg % step == step - 1:
                    tok([a[:, i * 128:(i + 1) * 128] for a in (ag, au) for i in range(w // 128)])
                    yield
            g = _rbf(jnp.sum(ag, axis=0, keepdims=True))
            u = _rbf(jnp.sum(au, axis=0, keepdims=True))
            h = _rbf(_rbf(g * jax.nn.sigmoid(g)) * u)
            hb_buf.at[c % 2][fs, :] = jnp.broadcast_to(h, (128, w)).T
        for d0 in range(0, D, 512):
            ds_ = slice(d0, d0 + 512)
            acc = yacc[:, ds_]
            for kg in range(FW // 8):
                hv = jnp.concatenate([gate(hb_buf[c % 2, 8 * kg:8 * kg + 8, :])] * 4, axis=1)
                acc = acc + wd_buf[c, 8 * kg:8 * kg + 8, ds_].astype(f32) * hv
                if kg % FSTEP == FSTEP - 1:
                    tok([acc[:, i * 128:(i + 1) * 128] for i in range(4)])
                    yield
            yacc[:, ds_] = acc

    def wait_group(i):
        with _scope("a_wait%d" % i):
            for c in a_groups[i]:
                c.wait()

    def run_all(gen):
        for _ in gen:
            pass

    def ln_side(p0, n, t0, t1):
        add_side(lambda tok: ln_rows(p0, n, tok), n // 2, t0, t1, SLAG)

    with _scope("p0_issue"):
        for grp in a_groups:
            for c in grp:
                c.start()
        for j in range(NT):
            for c in cp_b(j):
                c.start()
        zacc[...] = jnp.zeros(zacc.shape, f32)
        pq_buf[1, :, QA:RQ, :] = jnp.ones((4, RQ - QA, D), f32)
        den_buf[1, :, QA:RQ, :] = jnp.ones((4, RQ - QA, 128), f32)
        zero_buf[1] = jnp.zeros((8, 128), u32)
        cp_zero = cp(zero_buf.at[1], zero_buf.at[0], SEM_Z)
        cp_zero.start()
        cp_zero.wait()
    wait_group(0)
    with _scope("a0"):
        run_all(ln_rows(0, 128, None))
    wait_group(1)
    with _scope("a1"):
        run_all(ln_rows(128, 128, None))
    wait_group(2)
    with _scope("a2"):
        run_all(wk_prep(0))
        kproj(0, 256, [0])
        finish()
    wait_group(3)
    with _scope("a3"):
        run_all(wk_prep(1))
        kproj(0, 256, [1])
        finish()
    wait_group(4)
    with _scope("a4"):
        run_all(wk_prep(2))
        add_side(lambda tok: wk_prep(3), 32, 300, 1500)
        ln_side(256, 128, 0, 3300)
        kproj(0, 256, [2, 3])
        finish()
    wait_group(5)
    with _scope("a5"):
        for p0 in (256, 384, 512):
            ln_side(p0 + 128, 128, 0, 3200)
            kproj(p0, 128)
        finish()
    wait_group(6)
    with _scope("a6"):
        add_side(wq_prep, 8 * 24, 0, 10000, SLAG)
        for p0 in (640, 768):
            ln_side(p0 + 128, 128, 0, 3200)
            kproj(p0, 128)
        add_side(route, 17, 0, 800)
        kproj(896, 128)
        finish()

    def b_body(j, carry):
        with _scope("b_wait"):
            for c in cp_b(j, wait_only=True):
                c.wait()
        with _scope("b_body"):
            if not NOFFN:
              add_side(lambda tok: ffn_chunk(j, tok), (56 + 28) * 8 // FSTEP, 0, 13500)
            b_tile(j)
            finish()
        return carry

    if UNROLL_B:
        for j in range(NT):
            b_body(j, 0)
    else:
        lax.fori_loop(0, NT, b_body, 0)

    with _scope("bc"):
        run_all(normalise(NT - 1, QA, RQ - QA, NT - 1))

    def c_body(t, carry):
        with _scope("c_body"):
            y = _rbf(jnp.sum(yacc[...], axis=0, keepdims=True))
            y = _rbf(y * _rbf(jax.nn.sigmoid(rsel[...])))
            for p in range(RQ // CR):
                out_part(t * RQ + p * CR, CR, y)
        return carry

    lax.fori_loop(0, NT, c_body, 0)
    with _scope("tail"):
        cp(out_buf, out_hbm.at[0], SEM_O).wait()


@jax.jit
def pallas_parallel_sum__linear_attn_block__moe_arch_mod__prompt_kernel(
    A_x: jax.Array,
    A_wqkv: jax.Array,
    A_wo: jax.Array,
    B_x: jax.Array,
    B_w_r: jax.Array,
    B_w_gate: jax.Array,
    B_w_up: jax.Array,
    B_w_down: jax.Array,
):
    del B_x
    V = pltpu.VMEM
    scratch = [
        V((S, D), bf16),
        V((4, D, 256), bf16),
        V((D, D), bf16),
        V((4, D, 256), bf16),
        V((D, D), bf16),
        V((D,), bf16),
        V((NF, D, 1024), bf16),
        V((NF, D, 1024), bf16),
        V((NF, 1024, D), bf16),
        V((7, HP // 2, HD), u32),
        V((4, HP // 2, 1024), u32),
        V((49, HQ // 2, 256), u32),
        V((7, HD // 2, HD), u32),
        V((7, HD // 2, HD), u32),
        V((49, 128, 256), u32),
        V((S, 128), f32),
        V((S, 128), f32),
        V((S, 128), f32),
        V((8, D), f32),
        V((8, D), f32),
        V((8, 64, 128), u32),
        V((2, 64, 128), u32),
        V((64, 64, 128), u32),
        V((2, 4, RQ, D), f32),
        V((2, 4, RQ, 128), f32),
        V((2, 2, 128, D), f32),
        V((D, 128), f32),
        V((2, 1024, 128), f32),
        V((8, D), f32),
        V((1, D), f32),
        V((S, D), bf16),
        V((2, 8, 128), u32),
        pltpu.SMEM((1,), i32),
        pltpu.SemaphoreType.DMA((NT + 9,)),
    ]
    return pl.pallas_call(
        _kernel,
        out_shape=jax.ShapeDtypeStruct((1, S, D), bf16),
        in_specs=[pl.BlockSpec(memory_space=pl.ANY)] * 7,
        out_specs=pl.BlockSpec(memory_space=pl.ANY),
        scratch_shapes=scratch,
        compiler_params=pltpu.CompilerParams(vmem_limit_bytes=110 * 1024 * 1024,
                                             disable_bounds_checks=True,
                                             disable_semaphore_checks=True),
    )(A_x, A_wqkv, A_wo, B_w_r, B_w_gate, B_w_up, B_w_down)
```

```python
import contextlib

import jax
import jax.numpy as jnp
from jax import lax
import jax.experimental.pallas as pl
import jax.experimental.pallas.tpu as pltpu

bf16, f32, u32, i32 = jnp.bfloat16, jnp.float32, jnp.uint32, jnp.int32

S = 2048
D = 1024
F = 3584
HP = S // 2
HD = D // 2
R = 256
NT = HP // R
HQ = S // 4
RQ = HQ // NT
FW = 896
NF = F // FW
QLAG = 768
UNROLL_B = False
KW = (16, 16, 16, 16, 16, 16, 16)
CU = 1
QA = 96
NOFFN = False
SLAG = 400
FSTEP = 2
CR = 32

L_ORD = (2, 3, 0, 1, 4, 5, 6)
R_ORD = (2, 0, 6, 5, 1, 4, 3)

K_SEQ = (1, 4, 0, 2, 3, 5, 6)
K_SEQ2 = (0, 1, 2, 5, 3, 4, 6)

NN = (((1,), (0,)), ((), ()))
NT_ = (((1,), (1,)), ((), ()))
TN = (((0,), (0,)), ((), ()))


SCOPES = False


def _scope(name):
    return jax.named_scope(name) if SCOPES else contextlib.nullcontext()


def _mo(v, m):
    return v if isinstance(v, int) else pl.multiple_of(v, m)


def _dot(a, b, dims):
    return lax.dot_general(a, b, dims, preferred_element_type=f32)


def _pack(v):
    return pltpu.bitcast(v.astype(bf16), u32)


def _unpack(v):
    return pltpu.bitcast(v, bf16)


def _combine(m):
    m1, m2, m3, m4, m5, m6, m7 = m
    return m1 + m4 - m5 + m7, m3 + m5, m2 + m4, m1 - m2 + m3 + m6


def _lform(a11, a12, a21, a22):
    return (a11 + a22, a21 + a22, a11, a22, a11 + a12, a21 - a11, a12 - a22)


def _rform(b11, b12, b21, b22):
    return (b11 + b22, b11, b12 - b22, b21 - b11, b22, b11 + b12, b21 + b22)


def _form2(form, blk):
    lvl1 = [form(blk[r][c], blk[r][c + 2], blk[r + 2][c], blk[r + 2][c + 2])
            for r in range(2) for c in range(2)]
    return [v for k1 in range(7) for v in form(*[lvl1[i][k1] for i in range(4)])]


class _Sym:
    def __init__(self, t):
        self.t = t

    def __add__(self, o):
        return _Sym({**self.t, **o.t})

    def __sub__(self, o):
        return _Sym({**self.t, **{k: -v for k, v in o.t.items()}})


def _phi(t):
    return jnp.where(t > 0, t + 1.0, jnp.exp(t)) + 1e-6


def _rbf(v):
    return v.astype(bf16).astype(f32)


def _layernorm_rows(xv):
    mf = jnp.sum(xv, axis=1, keepdims=True) * (1.0 / D)
    mb = _rbf(mf)
    d = xv - mb
    dm = mf - mb
    var = jnp.sum(d * d, axis=1, keepdims=True) * (1.0 / D) - dm * dm
    var = jnp.maximum(var, 0.0)
    sd = _rbf(jnp.sqrt(_rbf(_rbf(var) + 1e-5)))
    return d * (1.0 / sd)


def _kernel(x_hbm, wqkv_hbm, wo_hbm, wr_hbm, wg_hbm, wu_hbm, wd_hbm, out_hbm,
            x_buf, wk_buf, wq_buf, wv_buf, wo_buf, wr_buf, wg_buf, wu_buf, wd_buf,
            xs, ps, qs, wks, wqs, ms, sa, sb, stats, zacc, zp, tscr, tscr2, wqt, pq_buf, den_buf, pqb_buf, denb_buf, qsb, mg_buf,
            xb, hb_buf, yacc, rsel, out_buf, zero_buf, idx_s, sem):

    SEM_B, SEM_O, SEM_Z, SEM_A = 0, NT, NT + 1, NT + 2

    def cp(src, dst, s):
        return pltpu.make_async_copy(src, dst, sem.at[s])

    def cp_x(p0, n, s):
        return [cp(x_hbm.at[0, pl.ds(h * HP + p0, n), :], x_buf.at[pl.ds(h * HP + p0, n), :], s)
                for h in range(2)]

    def cp_wk(c, s):
        return [cp(wqkv_hbm.at[:, pl.ds(D + h * HD + c * 128, 128)],
                   wk_buf.at[c, :, pl.ds(h * 128, 128)], s) for h in range(2)]

    a_groups = [
        [cp(wr_hbm, wr_buf, SEM_A)] + cp_x(0, 128, SEM_A),
        cp_x(128, 128, SEM_A + 1),
        cp_wk(0, SEM_A + 2),
        cp_wk(1, SEM_A + 3),
        cp_wk(2, SEM_A + 4) + cp_x(256, 128, SEM_A + 4) + cp_wk(3, SEM_A + 4),
        cp_x(384, 384, SEM_A + 5),
        cp_x(768, 256, SEM_A + 6) + [cp(wqkv_hbm.at[:, pl.ds(0, D)], wq_buf, SEM_A + 6)],
    ]

    def cp_b(j, wait_only=False):
        def off(v, m):
            return v if isinstance(v, int) else _mo(v, m)
        out = []
        for hh, g in enumerate((j, j + 4)):
            c0 = off(g * 128, 128)
            dst = wv_buf.at[j, :, pl.ds(hh * 128, 128)]
            out.append(cp(dst if wait_only else wqkv_hbm.at[:, pl.ds(2 * D + c0, 128)], dst, SEM_B + j))
            dst = wo_buf.at[pl.ds(c0, 128), :]
            out.append(cp(dst if wait_only else wo_hbm.at[pl.ds(c0, 128), :], dst, SEM_B + j))
        f0 = off(j * FW, 128)
        for src, dst in ((wg_hbm.at[:, pl.ds(f0, FW)], wg_buf.at[j, :, pl.ds(0, FW)]),
                         (wu_hbm.at[:, pl.ds(f0, FW)], wu_buf.at[j, :, pl.ds(0, FW)]),
                         (wd_hbm.at[pl.ds(f0, FW), :], wd_buf.at[j, pl.ds(0, FW), :])):
            out.append(cp(dst if wait_only else src, dst, SEM_B + j))
        return out

    clock = [0]
    toks = []
    sides = []
    fwd = [None]

    def emit_tok(vals, stamp=None):
        t = None
        for v in vals:
            v = pltpu.bitcast(v, u32) if v.dtype != u32 else v
            t = v if t is None else t | v
        toks.append((clock[0] if stamp is None else stamp, t & zero_buf[0]))

    def gate(v):
        if fwd[0] is None:
            return v
        if fwd[0][1] is None:
            fwd[0][1] = pltpu.bitcast(fwd[0][0](), u32) & zero_buf[0]
        head = pltpu.bitcast(pltpu.bitcast(v[0:8], u32) | fwd[0][1], v.dtype)
        return head if v.shape[0] == 8 else jnp.concatenate([head, v[8:]], axis=0)

    def add_side(gen_fn, n, t0, t1, lag=None):
        st = {"i": 0, "n": n, "t0": clock[0] + t0, "t1": clock[0] + t1}

        def tok(vals):
            if lag is not None:
                emit_tok(vals, st["t0"] + (st["i"] + 1) * (st["t1"] - st["t0"]) // st["n"] + lag)
        st["g"] = gen_fn(tok)
        sides.append(st)

    def advance(until):
        for st in sides:
            while st["i"] < st["n"] and st["t0"] + st["i"] * (st["t1"] - st["t0"]) // st["n"] < until:
                next(st["g"], None)
                st["i"] += 1

    def finish():
        for st in sides:
            for _ in st["g"]:
                pass
        sides.clear()
        toks.clear()
        fwd[0] = None

    def mm(lhs, rhs, dims, cycles, nseg=1):
        due = [t for (c, t) in toks if c <= clock[0]]
        toks[:] = [(c, t) for (c, t) in toks if c > clock[0]]
        if due:
            head = rhs[0:8, 0:128]
            for t in due:
                head = head | t
            if rhs.shape[1] > 128:
                head = jnp.concatenate([head, rhs[0:8, 128:]], axis=1)
            rhs = jnp.concatenate([head, rhs[8:]], axis=0)
        res = _dot(lhs, _unpack(rhs), dims)
        ngr = res.shape[0] // 16
        for sg in range(nseg):
            for i in range(ngr):
                fwd[0] = [lambda sg=sg, i=i: res[i * 16:i * 16 + 8, sg * 128:(sg + 1) * 128], None]
                clock[0] += cycles // nseg // ngr
                advance(clock[0])
        return res

    def ln_rows(p_start, n_rows, tok):
        wr = wr_buf[...].reshape(1, D).astype(f32)
        lane = lax.broadcasted_iota(i32, (8, 128), 1)
        for c in range(n_rows // 16):
            p0 = p_start + c * 16
            ds_, rss, sts = [], [], []
            for r0 in (p0, p0 + 8, HP + p0, HP + p0 + 8):
                xv = x_buf[r0:r0 + 8, :].astype(f32)
                xg = jnp.concatenate([gate(xv[:, 0:128]), xv[:, 128:]], axis=1)
                mf = jnp.sum(xg, axis=1, keepdims=True) * (1.0 / D)
                d = xv - mf
                var = jnp.sum(d * d, axis=1, keepdims=True) * (1.0 / D)
                tr = jnp.sum(d * wr, axis=1, keepdims=True)
                rs = jnp.broadcast_to(lax.rsqrt(var + 1e-5), (8, 128))
                mf = jnp.broadcast_to(mf, (8, 128))
                sa[r0:r0 + 8, :] = 1.0 + rs
                sb[r0:r0 + 8, :] = mf * rs
                st = jnp.where(lane == 0, mf, jnp.where(lane == 1, jnp.broadcast_to(var, (8, 128)),
                                                        jnp.broadcast_to(tr, (8, 128))))
                stats[r0:r0 + 8, :] = st
                ds_.append(d)
                rss.append(rs)
                sts.append(st)
                yield
            pend.append((p0, ds_, rss, sts))
            if len(pend) > 1:
                yield from ln_finish(tok, *pend.pop(0))
        while pend:
            yield from ln_finish(tok, *pend.pop(0))

    pend = []

    def ln_finish(tok, p0, ds_, rss, sts):
        for ct in range(4):
            cl = slice(ct * 128, (ct + 1) * 128)
            cr = slice(HD + ct * 128, HD + (ct + 1) * 128)
            rg = [gate(r) for r in rss]
            x11, x12, x21, x22 = [
                jnp.concatenate([ds_[i][:, cc] * rg[i], ds_[i + 1][:, cc] * rg[i + 1]], axis=0)
                for i, cc in ((0, cl), (0, cr), (2, cl), (2, cr))]
            ops = (x11, x22, x11 + x22, x21 + x22, x11 + x12, x21 - x11, x12 - x22)
            for k in range(7):
                xs.at[k][p0 // 2:p0 // 2 + 8, cl] = _pack(ops[k])
            if tok is not None:
                tok([ops[3][0:8], ops[3][8:16], ops[4][0:8], ops[4][8:16]])
            yield

    def wk_prep(c, tok=None):
        for i in range(HD // 16):
            r0 = i * 16
            top = wk_buf[c, r0:r0 + 16, :].astype(f32)
            bot = wk_buf[c, HD + r0:HD + r0 + 16, :].astype(f32)
            ops = _rform(gate(top[:, :128]), top[:, 128:], bot[:, :128], gate(bot[:, 128:]))
            for k in range(7):
                wks.at[k][r0 // 2:r0 // 2 + 8, c * 128:(c + 1) * 128] = _pack(ops[k])
            yield

    def wq_prep(tok):
        def transpose(g):
            for ct in range(8):
                tile = gate(pltpu.bitcast(wq_buf[ct * 128:(ct + 1) * 128, g * 128:(g + 1) * 128], u32))
                wqt.at[g * 8 + ct][...] = pltpu.bitcast(_unpack(tile).T, u32)
                yield

        def combine(g):
            for j in range(4):
                for ct in range(4):
                    w11, w12, w21, w22 = [
                        _unpack(gate(wqt[g * 8 + cc, pl.ds(jj, 8, stride=8), :])).astype(f32)
                        for jj, cc in ((j, ct), (j, ct + 4), (j + 4, ct), (j + 4, ct + 4))]
                    ops = _rform(w11, w21, w12, w22)
                    for k in range(7):
                        wqs.at[k][j * 64 + g * 8:j * 64 + g * 8 + 8, ct * 128:(ct + 1) * 128] = _pack(ops[k])
                    tok([ops[5][0:8], ops[6][0:8]])
                    yield

        for g in range(9):
            if g < 8:
                yield from transpose(g)
            if g > 0:
                yield from combine(g - 1)

    def kproj(p0, n, chunks=range(4)):
        pr = pl.ds(p0 // 2, n // 2)
        for c in chunks:
            cs = slice(c * 128, (c + 1) * 128)
            m = [None] * 7
            for i, k in enumerate(K_SEQ):
                m[k] = mm(_unpack(xs[L_ORD[k], pr, :]), wks[k, :, cs], NN, n * KW[i] // 16)
            k11, k12, k21, k22 = [_phi(v) for v in _combine(m)]
            zl = (k11 + k21).reshape(n // 8, 8, 128).sum(axis=0)
            zr = (k12 + k22).reshape(n // 8, 8, 128).sum(axis=0)
            zacc[:, cs] += zl
            zacc[:, HD + c * 128:HD + (c + 1) * 128] += zr
            ops = _lform(k11, k21, k12, k22)
            for k in range(7):
                ps.at[c][pr, k * 128:(k + 1) * 128] = _pack(ops[k])

    def z_prep():
        z = jnp.sum(zacc[...], axis=0, keepdims=True)
        zt = _pack(jnp.broadcast_to(z, (128, D)).astype(bf16).T)
        for g in range(8):
            tscr.at[g][...] = zt[g * 64:(g + 1) * 64, :]
        for j in range(8):
            blk = jnp.concatenate([tscr[g, pl.ds(j, 8, stride=8), :] for g in range(8)], axis=0)
            zp[:, j * 128:(j + 1) * 128] = _unpack(blk).T[0:8, :].astype(f32)

    def route(tok):
        rows = []
        for b in range(S // 128):
            rows.append(gate(stats[b * 128:(b + 1) * 128, :]).T[0:8, :])
            yield
        mf = jnp.concatenate([v[0:1] for v in rows], axis=0)
        var = jnp.concatenate([v[1:2] for v in rows], axis=0)
        tr = jnp.concatenate([v[2:3] for v in rows], axis=0)
        wsum = jnp.sum(wr_buf[...].reshape(1, D).astype(f32), axis=1, keepdims=True)
        sd = _rbf(jnp.sqrt(_rbf(_rbf(var) + 1e-5)))
        rv = _rbf((tr + (mf - _rbf(mf)) * wsum) / sd)
        rmax = jnp.max(rv)
        pos = (lax.broadcasted_iota(i32, rv.shape, 0) * 128 + lax.broadcasted_iota(i32, rv.shape, 1))
        idx = jnp.min(jnp.where(rv == rmax, pos, S - 1))
        idx_s[0] = idx
        rsel[...] = jnp.full(rsel.shape, rmax, f32)
        b0 = _mo((idx // 16) * 16, 16)
        xn = _rbf(_layernorm_rows(x_buf[pl.ds(b0, 16), :].astype(f32)))
        sel = lax.broadcasted_iota(i32, xn.shape, 0) == idx - b0
        row = jnp.sum(jnp.where(sel, xn, 0.0), axis=0, keepdims=True)
        xbv = jnp.broadcast_to(row, (128, D)).T
        xb[...] = xbv
        yacc[...] = jnp.zeros(yacc.shape, f32)
        tok([xbv[b * 128 + 120:(b + 1) * 128] for b in range(8)])
        yield

    def form2_steps(form, get, put, tok=None):
        terms = form(*[_Sym({i: 1}) for i in range(4)])
        for k1 in range(7):
            sub = []
            for r in range(2):
                for c in range(2):
                    v = None
                    for i, sg in sorted(terms[k1].t.items(), key=lambda e: -e[1]):
                        b = get(r + 2 * (i // 2), c + 2 * (i % 2))
                        if v is None:
                            v = gate16(b) if r == c else b
                        else:
                            v = v + b if sg > 0 else v - b
                    sub.append(v)
            vals = form(*sub)
            for k2, v in enumerate(vals):
                put(k1 * 7 + k2, _pack(v))
            if tok is not None:
                tok([v[o:o + 8] for v in vals[-2:] for o in (0, 8)])
            yield

    def gate16(v):
        return jnp.concatenate([gate(v[0:8]), gate(v[8:16])], axis=0)

    def q_part(j, r0, nr, pq, dn):
        prs = [pl.ds(_mo(j * (RQ // 2) + (h * HQ + r0) // 2, 8), nr // 2) for h in range(2)]
        den = [None, None]
        for c in range(4):
            m = [mm(_unpack(jnp.concatenate([xs[L_ORD[k], pr, :] for pr in prs], axis=0)),
                    wqs[k, c * 64:(c + 1) * 64, :], NT_, 2 * nr) for k in range(7)]
            q11, q12, q21, q22 = [_phi(v) for v in _combine(m)]
            cl = slice(c * 128, (c + 1) * 128)
            cr = slice(HD + c * 128, HD + (c + 1) * 128)
            zl, zr = zp[0:1, cl], zp[0:1, cr]
            dt, db = q11 * zl + q12 * zr, q21 * zl + q22 * zr
            den = [dt, db] if c == 0 else [den[0] + dt, den[1] + db]
            for h in range(2):
                hs = slice(h * nr, (h + 1) * nr)
                pq.at[h][0:nr, cl] = q11[hs]
                pq.at[h][0:nr, cr] = q12[hs]
                pq.at[2 + h][0:nr, cl] = q21[hs]
                pq.at[2 + h][0:nr, cr] = q22[hs]
            emit_tok([d[i * 8:(i + 1) * 8] for d in den for i in range(nr // 4)], clock[0] + QLAG)
            if c == 3:
                for q in range(4):
                    dn.at[q][0:nr, :] = den[q // 2][(q % 2) * nr:(q % 2 + 1) * nr]
            yield

    def normalise(pq, dn, nr, dst, p0, tok=None):
        lane = lax.broadcasted_iota(i32, (16, 128), 1)

        def recips(c):
            recs = []
            for q in range(4):
                d = gate16(dn[q, c * 16:(c + 1) * 16, :])
                d = d + jnp.where(lane % 2 == 0, pltpu.roll(d, 127, 1), pltpu.roll(d, 1, 1))
                d = d + jnp.where(lane % 4 < 2, pltpu.roll(d, 126, 1), pltpu.roll(d, 2, 1))
                recs.append(1.0 / (d + 1e-6))
            return recs

        nxt = recips(0)
        for _ in range(4):
            yield
        for c in range(nr // 16):
            rq = slice(c * 16, (c + 1) * 16)
            p2 = pl.ds(_mo(p0 + c * 8, 8), 8)
            recs = nxt
            for q in range(4):
                for hf in range(2):
                    cs = slice(hf * HD, (hf + 1) * HD)
                    pq.at[q][rq, cs] = pq[q, rq, cs] * jnp.concatenate([gate16(recs[q])] * 4, axis=1)
                    yield
            if c + 1 < nr // 16:
                nxt = recips(c + 1)
            yield
            for ct in range(2):
                def put(k, v):
                    dst.at[k][p2, ct * 128:(ct + 1) * 128] = v
                yield from form2_steps(
                    _lform, lambda q, u: pq[q, rq, u * 256 + ct * 128:u * 256 + (ct + 1) * 128], put, tok)

    def b_tile(j):
        jc = pl.ds(_mo(j * 128, 128), 128)
        z_prep()
        nb = RQ - QA
        j2 = j & 1
        for _ in q_part(j, 0, QA, pq_buf.at[j2], den_buf.at[j2]):
            pass
        add_side(lambda tok: normalise(pq_buf.at[j2], den_buf.at[j2], QA, qs, j * (RQ // 2)),
                 4 + 23 * (QA // 16), 400, 7000)
        m = [mm(_unpack(ps[j, :, k * 128:(k + 1) * 128]), xs[R_ORD[k]], TN, 1024, 4) for k in range(7)]
        g11, g12, g21, g22 = _combine(m)
        hm = (lax.broadcasted_iota(i32, (128, 128), 0) // 32
              == lax.broadcasted_iota(i32, (128, 128), 1) // 32)
        qb = q_part(j, QA, nb, pqb_buf.at[j], denb_buf.at[j])
        next(qb)
        kvps = []
        for half, (ga, gb) in enumerate(((g11, g12), (g21, g22))):
            gc = pl.ds(_mo((j + 4 * half) * 128, 128), 128)
            gg = jnp.concatenate([ga, gb], axis=1).astype(bf16)
            clock[0] += 256
            kv = jnp.where(hm, _dot(gg, wv_buf[j, :, half * 128:(half + 1) * 128], NN), 0.0)
            tscr2.at[half][...] = _pack(kv)
            kvps.append(_unpack(jnp.concatenate(
                [tscr2[half, pl.ds(jj, 8, stride=8), :] for jj in range(8)], axis=0)))
        next(qb)
        mg = mg_buf.at[j2]
        for half in range(2):
            gr = pl.ds(_mo((j + 4 * half) * 128, 128), 128)
            clock[0] += 256
            mg.at[half][...] = _dot(kvps[half], wo_buf[gr, :], NN)

        def m_form(tok):
            for half in range(2):
                g = j + 4 * half
                for jj in range(2):
                    for ct in range(2):
                        def put(k, v):
                            ms.at[k][pl.ds(_mo(jj * 64 + g * 8, 8), 8), ct * 128:(ct + 1) * 128] = v
                        yield from form2_steps(
                            _rform, lambda q, u: mg[half, (2 * q + jj) * 16:(2 * q + jj + 1) * 16,
                                                    u * 256 + ct * 128:u * 256 + (ct + 1) * 128], put)

        add_side(m_form, 56, 0, 28 * nb - 100)
        for _ in qb:
            pass

    def out_part(p0, nr, y, src, pr0):
        pr = pl.ds(_mo(pr0, 8), nr // 2)
        rows = [pl.ds(_mo(q * HQ + p0, 16), nr) for q in range(4)]
        row = lax.broadcasted_iota(i32, (nr, 256), 0) + p0
        m1 = [None] * 7
        for k1 in K_SEQ2:
            m2 = [None] * 7
            for k2 in K_SEQ2:
                m2[k2] = mm(_unpack(src[k1 * 7 + k2, pr, :]), ms[k1 * 7 + k2], NN, nr)
            m1[k1] = _combine(m2)
        outs = [_combine([m1[k1][s2] for k1 in range(7)]) for s2 in range(4)]
        for s1 in (3, 2, 1, 0):
            for s2 in range(4):
                q = (s1 // 2) * 2 + s2 // 2
                u = (s1 % 2) * 2 + s2 % 2
                rr, cc = rows[q], pl.ds(u * 256, 256)
                a = jnp.concatenate([sa[rr, :]] * 2, axis=1)
                b = jnp.concatenate([sb[rr, :]] * 2, axis=1)
                o = outs[s2][s1] + jnp.where(row + q * HQ == idx_s[0], y[:, u * 256:(u + 1) * 256], 0.0)
                out_buf[rr, cc] = (x_buf[rr, cc].astype(f32) * a - b + o).astype(bf16)
                if s2 % 2 == 1:
                    ch = pl.ds((s1 % 2) * HD, HD)
                    cp(out_buf.at[rr, ch], out_hbm.at[0, rr, ch], SEM_O).start()

    def ffn_chunk(c, tok):
        hs = []
        for f0 in range(0, FW, 256):
            w = min(256, FW - f0)
            fs = slice(f0, f0 + w)
            ag = jnp.zeros((8, w), f32)
            au = jnp.zeros((8, w), f32)
            step = FSTEP * 256 // w
            for kg in range(D // 8):
                xv = jnp.concatenate([gate(xb[8 * kg:8 * kg + 8, :])] * (w // 128), axis=1)
                ag = ag + wg_buf[c, 8 * kg:8 * kg + 8, fs].astype(f32) * xv
                au = au + wu_buf[c, 8 * kg:8 * kg + 8, fs].astype(f32) * xv
                if kg % step == step - 1:
                    tok([a[:, i * 128:(i + 1) * 128] for a in (ag, au) for i in range(w // 128)])
                    yield
            g = _rbf(jnp.sum(ag, axis=0, keepdims=True))
            u = _rbf(jnp.sum(au, axis=0, keepdims=True))
            h = _rbf(_rbf(g * jax.nn.sigmoid(g)) * u)
            hb_buf.at[c & 1][fs, :] = jnp.broadcast_to(h, (128, w)).T
        for d0 in range(0, D, 512):
            ds_ = slice(d0, d0 + 512)
            acc = yacc[:, ds_]
            for kg in range(FW // 8):
                hv = jnp.concatenate([gate(hb_buf[c & 1, 8 * kg:8 * kg + 8, :])] * 4, axis=1)
                acc = acc + wd_buf[c, 8 * kg:8 * kg + 8, ds_].astype(f32) * hv
                if kg % FSTEP == FSTEP - 1:
                    tok([acc[:, i * 128:(i + 1) * 128] for i in range(4)])
                    yield
            yacc[:, ds_] = acc

    def wait_group(i):
        with _scope("a_wait%d" % i):
            for c in a_groups[i]:
                c.wait()

    def run_all(gen):
        for _ in gen:
            pass

    def ln_side(p0, n, t0, t1):
        add_side(lambda tok: ln_rows(p0, n, tok), n // 2, t0, t1, SLAG)

    with _scope("p0_issue"):
        for grp in a_groups:
            for c in grp:
                c.start()
        for j in range(NT):
            for c in cp_b(j):
                c.start()
        zacc[...] = jnp.zeros(zacc.shape, f32)
        zero_buf[1] = jnp.zeros((8, 128), u32)
        cp_zero = cp(zero_buf.at[1], zero_buf.at[0], SEM_Z)
        cp_zero.start()
        cp_zero.wait()
    wait_group(0)
    with _scope("a0"):
        run_all(ln_rows(0, 128, None))
    wait_group(1)
    with _scope("a1"):
        run_all(ln_rows(128, 128, None))
    wait_group(2)
    with _scope("a2"):
        run_all(wk_prep(0))
        kproj(0, 256, [0])
        finish()
    wait_group(3)
    with _scope("a3"):
        run_all(wk_prep(1))
        kproj(0, 256, [1])
        finish()
    wait_group(4)
    with _scope("a4"):
        run_all(wk_prep(2))
        add_side(lambda tok: wk_prep(3), 32, 300, 1500)
        ln_side(256, 128, 0, 3300)
        kproj(0, 256, [2, 3])
        finish()
    wait_group(5)
    with _scope("a5"):
        for p0 in (256, 384, 512):
            ln_side(p0 + 128, 128, 0, 3200)
            kproj(p0, 128)
        finish()
    wait_group(6)
    with _scope("a6"):
        add_side(wq_prep, 8 * 24, 0, 10000, SLAG)
        for p0 in (640, 768):
            ln_side(p0 + 128, 128, 0, 3200)
            kproj(p0, 128)
        add_side(route, 17, 0, 800)
        kproj(896, 128)
        finish()

    def b_body(j, carry):
        with _scope("b_wait"):
            for c in cp_b(j, wait_only=True):
                c.wait()
        with _scope("b_body"):
            if not NOFFN:
              add_side(lambda tok: ffn_chunk(j, tok), (56 + 28) * 8 // FSTEP, 0, 13500)
            b_tile(j)
            finish()
        return carry

    if UNROLL_B:
        for j in range(NT):
            b_body(j, 0)
    else:
        lax.fori_loop(0, NT, b_body, 0)

    def c_body(t, carry):
        with _scope("c_body"):
            y = _rbf(jnp.sum(yacc[...], axis=0, keepdims=True))
            y = _rbf(y * _rbf(jax.nn.sigmoid(rsel[...])))
            nb = RQ - QA
            for i in range(CU):
                tt = t * CU + i
                add_side(lambda tok, tt=tt, i=i: normalise(pqb_buf.at[tt], denb_buf.at[tt], nb, qsb,
                                                          i * (nb // 2), tok),
                         4 + 23 * (nb // 16), 0, 49 * QA - 800, SLAG)
                for p in range(QA // CR):
                    out_part(tt * RQ + p * CR, CR, y, qs, tt * (RQ // 2) + p * (CR // 2))
                out_part(tt * RQ + QA, nb, y, qsb, i * (nb // 2))
            finish()
        return carry

    lax.fori_loop(0, NT // CU, c_body, 0)
    with _scope("tail"):
        cp(out_buf, out_hbm.at[0], SEM_O).wait()


@jax.jit
def pallas_parallel_sum__linear_attn_block__moe_arch_mod__prompt_kernel(
    A_x: jax.Array,
    A_wqkv: jax.Array,
    A_wo: jax.Array,
    B_x: jax.Array,
    B_w_r: jax.Array,
    B_w_gate: jax.Array,
    B_w_up: jax.Array,
    B_w_down: jax.Array,
):
    del B_x
    V = pltpu.VMEM
    scratch = [
        V((S, D), bf16),
        V((4, D, 256), bf16),
        V((D, D), bf16),
        V((4, D, 256), bf16),
        V((D, D), bf16),
        V((D,), bf16),
        V((NF, D, 1024), bf16),
        V((NF, D, 1024), bf16),
        V((NF, 1024, D), bf16),
        V((7, HP // 2, HD), u32),
        V((4, HP // 2, 1024), u32),
        V((49, HQ // 2, 256), u32),
        V((7, HD // 2, HD), u32),
        V((7, HD // 2, HD), u32),
        V((49, 128, 256), u32),
        V((S, 128), f32),
        V((S, 128), f32),
        V((S, 128), f32),
        V((8, D), f32),
        V((8, D), f32),
        V((8, 64, 128), u32),
        V((2, 64, 128), u32),
        V((64, 64, 128), u32),
        V((2, 4, RQ, D), f32),
        V((2, 4, RQ, 128), f32),
        V((4, 4, RQ - QA, D), f32),
        V((4, 4, RQ - QA, 128), f32),
        V((49, CU * (RQ - QA) // 2, 256), u32),
        V((2, 2, 128, D), f32),
        V((D, 128), f32),
        V((2, 1024, 128), f32),
        V((8, D), f32),
        V((1, D), f32),
        V((S, D), bf16),
        V((2, 8, 128), u32),
        pltpu.SMEM((1,), i32),
        pltpu.SemaphoreType.DMA((NT + 9,)),
    ]
    return pl.pallas_call(
        _kernel,
        out_shape=jax.ShapeDtypeStruct((1, S, D), bf16),
        in_specs=[pl.BlockSpec(memory_space=pl.ANY)] * 7,
        out_specs=pl.BlockSpec(memory_space=pl.ANY),
        scratch_shapes=scratch,
        compiler_params=pltpu.CompilerParams(vmem_limit_bytes=110 * 1024 * 1024,
                                             disable_bounds_checks=True,
                                             disable_semaphore_checks=True),
    )(A_x, A_wqkv, A_wo, B_w_r, B_w_gate, B_w_up, B_w_down)
```

```python
import contextlib

import jax
import jax.numpy as jnp
from jax import lax
import jax.experimental.pallas as pl
import jax.experimental.pallas.tpu as pltpu

bf16, f32, u32, i32 = jnp.bfloat16, jnp.float32, jnp.uint32, jnp.int32

S = 2048
D = 1024
F = 3584
HP = S // 2
HD = D // 2
R = 256
NT = HP // R
HQ = S // 4
RQ = HQ // NT
FW = 896
NF = F // FW
QLAG = 768
UNROLL_B = False
KW = (16, 16, 16, 16, 16, 16, 16)
CU = 1
APLAN = 1
A4N = 64
QA = 96
NOFFN = False
SLAG = 400
FSTEP = 2
CR = 32

L_ORD = (2, 3, 0, 1, 4, 5, 6)
R_ORD = (2, 0, 6, 5, 1, 4, 3)

K_SEQ = (1, 4, 0, 2, 3, 5, 6)
K_SEQ2 = (0, 1, 2, 5, 3, 4, 6)

NN = (((1,), (0,)), ((), ()))
NT_ = (((1,), (1,)), ((), ()))
TN = (((0,), (0,)), ((), ()))


SCOPES = False


def _scope(name):
    return jax.named_scope(name) if SCOPES else contextlib.nullcontext()


def _mo(v, m):
    return v if isinstance(v, int) else pl.multiple_of(v, m)


def _dot(a, b, dims):
    return lax.dot_general(a, b, dims, preferred_element_type=f32)


def _pack(v):
    return pltpu.bitcast(v.astype(bf16), u32)


def _unpack(v):
    return pltpu.bitcast(v, bf16)


def _combine(m):
    m1, m2, m3, m4, m5, m6, m7 = m
    return m1 + m4 - m5 + m7, m3 + m5, m2 + m4, m1 - m2 + m3 + m6


def _lform(a11, a12, a21, a22):
    return (a11 + a22, a21 + a22, a11, a22, a11 + a12, a21 - a11, a12 - a22)


def _rform(b11, b12, b21, b22):
    return (b11 + b22, b11, b12 - b22, b21 - b11, b22, b11 + b12, b21 + b22)


def _form2(form, blk):
    lvl1 = [form(blk[r][c], blk[r][c + 2], blk[r + 2][c], blk[r + 2][c + 2])
            for r in range(2) for c in range(2)]
    return [v for k1 in range(7) for v in form(*[lvl1[i][k1] for i in range(4)])]


class _Sym:
    def __init__(self, t):
        self.t = t

    def __add__(self, o):
        return _Sym({**self.t, **o.t})

    def __sub__(self, o):
        return _Sym({**self.t, **{k: -v for k, v in o.t.items()}})


def _phi(t):
    return jnp.where(t > 0, t + 1.0, jnp.exp(t)) + 1e-6


def _rbf(v):
    return v.astype(bf16).astype(f32)


def _layernorm_rows(xv):
    mf = jnp.sum(xv, axis=1, keepdims=True) * (1.0 / D)
    mb = _rbf(mf)
    d = xv - mb
    dm = mf - mb
    var = jnp.sum(d * d, axis=1, keepdims=True) * (1.0 / D) - dm * dm
    var = jnp.maximum(var, 0.0)
    sd = _rbf(jnp.sqrt(_rbf(_rbf(var) + 1e-5)))
    return d * (1.0 / sd)


def _kernel(x_hbm, wqkv_hbm, wo_hbm, wr_hbm, wg_hbm, wu_hbm, wd_hbm, out_hbm,
            x_buf, wk_buf, wq_buf, wv_buf, wo_buf, wr_buf, wg_buf, wu_buf, wd_buf,
            xs, ps, qs, wks, wqs, ms, sa, sb, stats, zacc, zp, tscr, tscr2, wqt, pq_buf, den_buf, pqb_buf, denb_buf, qsb, mg_buf,
            xb, hb_buf, yacc, rsel, out_buf, zero_buf, idx_s, sem):

    SEM_B, SEM_O, SEM_Z, SEM_A = 0, NT, NT + 1, NT + 2

    def cp(src, dst, s):
        return pltpu.make_async_copy(src, dst, sem.at[s])

    def cp_x(p0, n, s):
        return [cp(x_hbm.at[0, pl.ds(h * HP + p0, n), :], x_buf.at[pl.ds(h * HP + p0, n), :], s)
                for h in range(2)]

    def cp_wk(c, s):
        return [cp(wqkv_hbm.at[:, pl.ds(D + c * 256, 256)], wk_buf.at[c], s)]

    cp_wq = lambda s_: [cp(wqkv_hbm.at[:, pl.ds(0, D)], wq_buf, s_)]
    if APLAN == 0:
        a_groups = [
            [cp(wr_hbm, wr_buf, SEM_A)] + cp_x(0, 128, SEM_A),
            cp_x(128, 128, SEM_A + 1),
            cp_wk(0, SEM_A + 2),
            cp_wk(1, SEM_A + 3),
            cp_wk(2, SEM_A + 4) + cp_x(256, 128, SEM_A + 4) + cp_wk(3, SEM_A + 4),
            cp_x(384, 384, SEM_A + 5),
            cp_x(768, 256, SEM_A + 6) + cp_wq(SEM_A + 6),
        ]
    else:
        a_groups = [
            [cp(wr_hbm, wr_buf, SEM_A)] + cp_x(0, 128, SEM_A),
            cp_x(128, 128, SEM_A + 1),
            cp_wk(0, SEM_A + 2),
            cp_wk(1, SEM_A + 3) + cp_wk(2, SEM_A + 3),
            cp_x(256, 128, SEM_A + 4),
            cp_wk(3, SEM_A + 5) + cp_x(384, 256, SEM_A + 5),
            cp_x(640, 384, SEM_A + 6) + cp_wq(SEM_A + 6),
        ]

    def cp_b(j, wait_only=False):
        def off(v, m):
            return v if isinstance(v, int) else _mo(v, m)
        out = []
        c0 = off(j * 256, 256)
        dst = wv_buf.at[j]
        out.append(cp(dst if wait_only else wqkv_hbm.at[:, pl.ds(2 * D + c0, 256)], dst, SEM_B + j))
        dst = wo_buf.at[pl.ds(c0, 256), :]
        out.append(cp(dst if wait_only else wo_hbm.at[pl.ds(c0, 256), :], dst, SEM_B + j))
        f0 = off(j * FW, 128)
        for src, dst in ((wg_hbm.at[:, pl.ds(f0, FW)], wg_buf.at[j, :, pl.ds(0, FW)]),
                         (wu_hbm.at[:, pl.ds(f0, FW)], wu_buf.at[j, :, pl.ds(0, FW)]),
                         (wd_hbm.at[pl.ds(f0, FW), :], wd_buf.at[j, pl.ds(0, FW), :])):
            out.append(cp(dst if wait_only else src, dst, SEM_B + j))
        return out

    clock = [0]
    toks = []
    sides = []
    fwd = [None]

    def emit_tok(vals, stamp=None):
        t = None
        for v in vals:
            v = pltpu.bitcast(v, u32) if v.dtype != u32 else v
            t = v if t is None else t | v
        toks.append((clock[0] if stamp is None else stamp, t & zero_buf[0]))

    def gate(v):
        if fwd[0] is None:
            return v
        if fwd[0][1] is None:
            fwd[0][1] = pltpu.bitcast(fwd[0][0](), u32) & zero_buf[0]
        head = pltpu.bitcast(pltpu.bitcast(v[0:8], u32) | fwd[0][1], v.dtype)
        return head if v.shape[0] == 8 else jnp.concatenate([head, v[8:]], axis=0)

    def add_side(gen_fn, n, t0, t1, lag=None):
        st = {"i": 0, "n": n, "t0": clock[0] + t0, "t1": clock[0] + t1}

        def tok(vals):
            if lag is not None:
                emit_tok(vals, st["t0"] + (st["i"] + 1) * (st["t1"] - st["t0"]) // st["n"] + lag)
        st["g"] = gen_fn(tok)
        sides.append(st)

    def advance(until):
        for st in sides:
            while st["i"] < st["n"] and st["t0"] + st["i"] * (st["t1"] - st["t0"]) // st["n"] < until:
                next(st["g"], None)
                st["i"] += 1

    def finish():
        for st in sides:
            for _ in st["g"]:
                pass
        sides.clear()
        toks.clear()
        fwd[0] = None

    def mm(lhs, rhs, dims, cycles, nseg=1):
        due = [t for (c, t) in toks if c <= clock[0]]
        toks[:] = [(c, t) for (c, t) in toks if c > clock[0]]
        if due:
            head = rhs[0:8, 0:128]
            for t in due:
                head = head | t
            if rhs.shape[1] > 128:
                head = jnp.concatenate([head, rhs[0:8, 128:]], axis=1)
            rhs = jnp.concatenate([head, rhs[8:]], axis=0)
        res = _dot(lhs, _unpack(rhs), dims)
        ngr = res.shape[0] // 16
        for sg in range(nseg):
            for i in range(ngr):
                fwd[0] = [lambda sg=sg, i=i: res[i * 16:i * 16 + 8, sg * 128:(sg + 1) * 128], None]
                clock[0] += cycles // nseg // ngr
                advance(clock[0])
        return res

    def ln_rows(p_start, n_rows, tok):
        wr = wr_buf[...].reshape(1, D).astype(f32)
        lane = lax.broadcasted_iota(i32, (8, 128), 1)
        for c in range(n_rows // 16):
            p0 = p_start + c * 16
            ds_, rss, sts = [], [], []
            for r0 in (p0, p0 + 8, HP + p0, HP + p0 + 8):
                xv = x_buf[r0:r0 + 8, :].astype(f32)
                xg = jnp.concatenate([gate(xv[:, 0:128]), xv[:, 128:]], axis=1)
                mf = jnp.sum(xg, axis=1, keepdims=True) * (1.0 / D)
                d = xv - mf
                var = jnp.sum(d * d, axis=1, keepdims=True) * (1.0 / D)
                tr = jnp.sum(d * wr, axis=1, keepdims=True)
                rs = jnp.broadcast_to(lax.rsqrt(var + 1e-5), (8, 128))
                mf = jnp.broadcast_to(mf, (8, 128))
                sa[r0:r0 + 8, :] = 1.0 + rs
                sb[r0:r0 + 8, :] = mf * rs
                st = jnp.where(lane == 0, mf, jnp.where(lane == 1, jnp.broadcast_to(var, (8, 128)),
                                                        jnp.broadcast_to(tr, (8, 128))))
                stats[r0:r0 + 8, :] = st
                ds_.append(d)
                rss.append(rs)
                sts.append(st)
                yield
            pend.append((p0, ds_, rss, sts))
            if len(pend) > 1:
                yield from ln_finish(tok, *pend.pop(0))
        while pend:
            yield from ln_finish(tok, *pend.pop(0))

    pend = []

    def ln_finish(tok, p0, ds_, rss, sts):
        for ct in range(4):
            cl = slice(ct * 128, (ct + 1) * 128)
            cr = slice(HD + ct * 128, HD + (ct + 1) * 128)
            rg = [gate(r) for r in rss]
            x11, x12, x21, x22 = [
                jnp.concatenate([ds_[i][:, cc] * rg[i], ds_[i + 1][:, cc] * rg[i + 1]], axis=0)
                for i, cc in ((0, cl), (0, cr), (2, cl), (2, cr))]
            ops = (x11, x22, x11 + x22, x21 + x22, x11 + x12, x21 - x11, x12 - x22)
            for k in range(7):
                xs.at[k][p0 // 2:p0 // 2 + 8, cl] = _pack(ops[k])
            if tok is not None:
                tok([ops[3][0:8], ops[3][8:16], ops[4][0:8], ops[4][8:16]])
            yield

    def wk_prep(c, tok=None):
        for i in range(HD // 16):
            r0 = i * 16
            top = wk_buf[c, r0:r0 + 16, :].astype(f32)
            bot = wk_buf[c, HD + r0:HD + r0 + 16, :].astype(f32)
            ops = _rform(gate(top[:, :128]), top[:, 128:], bot[:, :128], gate(bot[:, 128:]))
            for k in range(7):
                wks.at[k][r0 // 2:r0 // 2 + 8, c * 128:(c + 1) * 128] = _pack(ops[k])
            yield

    def wq_prep(tok):
        def transpose(g):
            for ct in range(8):
                tile = gate(pltpu.bitcast(wq_buf[ct * 128:(ct + 1) * 128, g * 128:(g + 1) * 128], u32))
                wqt.at[g * 8 + ct][...] = pltpu.bitcast(_unpack(tile).T, u32)
                yield

        def combine(g):
            for j in range(4):
                for ct in range(4):
                    w11, w12, w21, w22 = [
                        _unpack(gate(wqt[g * 8 + cc, pl.ds(jj, 8, stride=8), :])).astype(f32)
                        for jj, cc in ((j, ct), (j, ct + 4), (j + 4, ct), (j + 4, ct + 4))]
                    ops = _rform(w11, w21, w12, w22)
                    for k in range(7):
                        wqs.at[k][j * 64 + g * 8:j * 64 + g * 8 + 8, ct * 128:(ct + 1) * 128] = _pack(ops[k])
                    tok([ops[5][0:8], ops[6][0:8]])
                    yield

        for g in range(9):
            if g < 8:
                yield from transpose(g)
            if g > 0:
                yield from combine(g - 1)

    def kproj(p0, n, chunks=range(4)):
        pr = pl.ds(p0 // 2, n // 2)
        for c in chunks:
            cs = slice(c * 128, (c + 1) * 128)
            m = [None] * 7
            for i, k in enumerate(K_SEQ):
                m[k] = mm(_unpack(xs[L_ORD[k], pr, :]), wks[k, :, cs], NN, n * KW[i] // 16)
            k11, k12, k21, k22 = [_phi(v) for v in _combine(m)]
            zl = (k11 + k21).reshape(n // 8, 8, 128).sum(axis=0)
            zr = (k12 + k22).reshape(n // 8, 8, 128).sum(axis=0)
            zacc[:, c * 256:c * 256 + 128] += zl
            zacc[:, c * 256 + 128:(c + 1) * 256] += zr
            ops = _lform(k11, k21, k12, k22)
            for k in range(7):
                ps.at[c][pr, k * 128:(k + 1) * 128] = _pack(ops[k])

    def z_prep():
        z = jnp.sum(zacc[...], axis=0, keepdims=True)
        zt = _pack(jnp.broadcast_to(z, (128, D)).astype(bf16).T)
        for g in range(8):
            tscr.at[g][...] = zt[g * 64:(g + 1) * 64, :]
        for j in range(8):
            blk = jnp.concatenate([tscr[g, pl.ds(j, 8, stride=8), :] for g in range(8)], axis=0)
            zp[:, j * 128:(j + 1) * 128] = _unpack(blk).T[0:8, :].astype(f32)

    def route(tok):
        rows = []
        for b in range(S // 128):
            rows.append(gate(stats[b * 128:(b + 1) * 128, :]).T[0:8, :])
            yield
        mf = jnp.concatenate([v[0:1] for v in rows], axis=0)
        var = jnp.concatenate([v[1:2] for v in rows], axis=0)
        tr = jnp.concatenate([v[2:3] for v in rows], axis=0)
        wsum = jnp.sum(wr_buf[...].reshape(1, D).astype(f32), axis=1, keepdims=True)
        sd = _rbf(jnp.sqrt(_rbf(_rbf(var) + 1e-5)))
        rv = _rbf((tr + (mf - _rbf(mf)) * wsum) / sd)
        rmax = jnp.max(rv)
        pos = (lax.broadcasted_iota(i32, rv.shape, 0) * 128 + lax.broadcasted_iota(i32, rv.shape, 1))
        idx = jnp.min(jnp.where(rv == rmax, pos, S - 1))
        idx_s[0] = idx
        rsel[...] = jnp.full(rsel.shape, rmax, f32)
        b0 = _mo((idx // 16) * 16, 16)
        xn = _rbf(_layernorm_rows(x_buf[pl.ds(b0, 16), :].astype(f32)))
        sel = lax.broadcasted_iota(i32, xn.shape, 0) == idx - b0
        row = jnp.sum(jnp.where(sel, xn, 0.0), axis=0, keepdims=True)
        xbv = jnp.broadcast_to(row, (128, D)).T
        xb[...] = xbv
        yacc[...] = jnp.zeros(yacc.shape, f32)
        tok([xbv[b * 128 + 120:(b + 1) * 128] for b in range(8)])
        yield

    def form2_steps(form, get, put, tok=None):
        terms = form(*[_Sym({i: 1}) for i in range(4)])
        for k1 in range(7):
            sub = []
            for r in range(2):
                for c in range(2):
                    v = None
                    for i, sg in sorted(terms[k1].t.items(), key=lambda e: -e[1]):
                        b = get(r + 2 * (i // 2), c + 2 * (i % 2))
                        if v is None:
                            v = gate16(b) if r == c else b
                        else:
                            v = v + b if sg > 0 else v - b
                    sub.append(v)
            vals = form(*sub)
            for k2, v in enumerate(vals):
                put(k1 * 7 + k2, _pack(v))
            if tok is not None:
                tok([v[o:o + 8] for v in vals[-2:] for o in (0, 8)])
            yield

    def gate16(v):
        return jnp.concatenate([gate(v[0:8]), gate(v[8:16])], axis=0)

    def q_part(j, r0, nr, pq, dn):
        prs = [pl.ds(_mo(j * (RQ // 2) + (h * HQ + r0) // 2, 8), nr // 2) for h in range(2)]
        den = [None, None]
        for c in range(4):
            m = [mm(_unpack(jnp.concatenate([xs[L_ORD[k], pr, :] for pr in prs], axis=0)),
                    wqs[k, c * 64:(c + 1) * 64, :], NT_, 2 * nr) for k in range(7)]
            q11, q12, q21, q22 = [_phi(v) for v in _combine(m)]
            cl = slice(c * 128, (c + 1) * 128)
            cr = slice(HD + c * 128, HD + (c + 1) * 128)
            zl, zr = zp[0:1, cl], zp[0:1, cr]
            dt, db = q11 * zl + q12 * zr, q21 * zl + q22 * zr
            den = [dt, db] if c == 0 else [den[0] + dt, den[1] + db]
            for h in range(2):
                hs = slice(h * nr, (h + 1) * nr)
                pq.at[h][0:nr, cl] = q11[hs]
                pq.at[h][0:nr, cr] = q12[hs]
                pq.at[2 + h][0:nr, cl] = q21[hs]
                pq.at[2 + h][0:nr, cr] = q22[hs]
            emit_tok([d[i * 8:(i + 1) * 8] for d in den for i in range(nr // 4)], clock[0] + QLAG)
            if c == 3:
                for q in range(4):
                    dn.at[q][0:nr, :] = den[q // 2][(q % 2) * nr:(q % 2 + 1) * nr]
            yield

    def normalise(pq, dn, nr, dst, p0, tok=None):
        lane = lax.broadcasted_iota(i32, (16, 128), 1)

        def recips(c):
            recs = []
            for q in range(4):
                d = gate16(dn[q, c * 16:(c + 1) * 16, :])
                d = d + jnp.where(lane % 2 == 0, pltpu.roll(d, 127, 1), pltpu.roll(d, 1, 1))
                d = d + jnp.where(lane % 4 < 2, pltpu.roll(d, 126, 1), pltpu.roll(d, 2, 1))
                recs.append(1.0 / (d + 1e-6))
            return recs

        nxt = recips(0)
        for _ in range(4):
            yield
        for c in range(nr // 16):
            rq = slice(c * 16, (c + 1) * 16)
            p2 = pl.ds(_mo(p0 + c * 8, 8), 8)
            recs = nxt
            for q in range(4):
                for hf in range(2):
                    cs = slice(hf * HD, (hf + 1) * HD)
                    pq.at[q][rq, cs] = pq[q, rq, cs] * jnp.concatenate([gate16(recs[q])] * 4, axis=1)
                    yield
            if c + 1 < nr // 16:
                nxt = recips(c + 1)
            yield
            for ct in range(2):
                def put(k, v):
                    dst.at[k][p2, ct * 128:(ct + 1) * 128] = v
                yield from form2_steps(
                    _lform, lambda q, u: pq[q, rq, u * 256 + ct * 128:u * 256 + (ct + 1) * 128], put, tok)

    def b_tile(j):
        jc = pl.ds(_mo(j * 128, 128), 128)
        z_prep()
        nb = RQ - QA
        j2 = j & 1
        for _ in q_part(j, 0, QA, pq_buf.at[j2], den_buf.at[j2]):
            pass
        add_side(lambda tok: normalise(pq_buf.at[j2], den_buf.at[j2], QA, qs, j * (RQ // 2)),
                 4 + 23 * (QA // 16), 400, 7000)
        m = [mm(_unpack(ps[j, :, k * 128:(k + 1) * 128]), xs[R_ORD[k]], TN, 1024, 4) for k in range(7)]
        g11, g12, g21, g22 = _combine(m)
        hm = (lax.broadcasted_iota(i32, (128, 128), 0) // 32
              == lax.broadcasted_iota(i32, (128, 128), 1) // 32)
        qb = q_part(j, QA, nb, pqb_buf.at[j], denb_buf.at[j])
        next(qb)
        kvps = []
        for half, (ga, gb) in enumerate(((g11, g12), (g21, g22))):
            gg = jnp.concatenate([ga, gb], axis=1).astype(bf16)
            clock[0] += 256
            kv = jnp.where(hm, _dot(gg, wv_buf[j, :, half * 128:(half + 1) * 128], NN), 0.0)
            tscr2.at[half][...] = _pack(kv)
            kvps.append(_unpack(jnp.concatenate(
                [tscr2[half, pl.ds(jj, 8, stride=8), :] for jj in range(8)], axis=0)))
        next(qb)
        mg = mg_buf.at[j2]
        for half in range(2):
            gr = pl.ds(_mo(j * 256 + half * 128, 128), 128)
            clock[0] += 256
            mg.at[half][...] = _dot(kvps[half], wo_buf[gr, :], NN)

        def m_form(tok):
            for half in range(2):
                g = 2 * j + half
                for jj in range(2):
                    for ct in range(2):
                        def put(k, v):
                            ms.at[k][pl.ds(_mo(jj * 64 + g * 8, 8), 8), ct * 128:(ct + 1) * 128] = v
                        yield from form2_steps(
                            _rform, lambda q, u: mg[half, (2 * q + jj) * 16:(2 * q + jj + 1) * 16,
                                                    u * 256 + ct * 128:u * 256 + (ct + 1) * 128], put)

        add_side(m_form, 56, 0, 28 * nb - 100)
        for _ in qb:
            pass

    def out_part(p0, nr, y, src, pr0):
        pr = pl.ds(_mo(pr0, 8), nr // 2)
        rows = [pl.ds(_mo(q * HQ + p0, 16), nr) for q in range(4)]
        row = lax.broadcasted_iota(i32, (nr, 256), 0) + p0
        m1 = [None] * 7
        for k1 in K_SEQ2:
            m2 = [None] * 7
            for k2 in K_SEQ2:
                m2[k2] = mm(_unpack(src[k1 * 7 + k2, pr, :]), ms[k1 * 7 + k2], NN, nr)
            m1[k1] = _combine(m2)
        outs = [_combine([m1[k1][s2] for k1 in range(7)]) for s2 in range(4)]
        for s1 in (3, 2, 1, 0):
            for s2 in range(4):
                q = (s1 // 2) * 2 + s2 // 2
                u = (s1 % 2) * 2 + s2 % 2
                rr, cc = rows[q], pl.ds(u * 256, 256)
                a = jnp.concatenate([sa[rr, :]] * 2, axis=1)
                b = jnp.concatenate([sb[rr, :]] * 2, axis=1)
                o = outs[s2][s1] + jnp.where(row + q * HQ == idx_s[0], y[:, u * 256:(u + 1) * 256], 0.0)
                out_buf[rr, cc] = (x_buf[rr, cc].astype(f32) * a - b + o).astype(bf16)
                if s2 % 2 == 1:
                    ch = pl.ds((s1 % 2) * HD, HD)
                    cp(out_buf.at[rr, ch], out_hbm.at[0, rr, ch], SEM_O).start()

    def ffn_chunk(c, tok):
        hs = []
        for f0 in range(0, FW, 256):
            w = min(256, FW - f0)
            fs = slice(f0, f0 + w)
            ag = jnp.zeros((8, w), f32)
            au = jnp.zeros((8, w), f32)
            step = FSTEP * 256 // w
            for kg in range(D // 8):
                xv = jnp.concatenate([gate(xb[8 * kg:8 * kg + 8, :])] * (w // 128), axis=1)
                ag = ag + wg_buf[c, 8 * kg:8 * kg + 8, fs].astype(f32) * xv
                au = au + wu_buf[c, 8 * kg:8 * kg + 8, fs].astype(f32) * xv
                if kg % step == step - 1:
                    tok([a[:, i * 128:(i + 1) * 128] for a in (ag, au) for i in range(w // 128)])
                    yield
            g = _rbf(jnp.sum(ag, axis=0, keepdims=True))
            u = _rbf(jnp.sum(au, axis=0, keepdims=True))
            h = _rbf(_rbf(g * jax.nn.sigmoid(g)) * u)
            hb_buf.at[c & 1][fs, :] = jnp.broadcast_to(h, (128, w)).T
        for d0 in range(0, D, 512):
            ds_ = slice(d0, d0 + 512)
            acc = yacc[:, ds_]
            for kg in range(FW // 8):
                hv = jnp.concatenate([gate(hb_buf[c & 1, 8 * kg:8 * kg + 8, :])] * 4, axis=1)
                acc = acc + wd_buf[c, 8 * kg:8 * kg + 8, ds_].astype(f32) * hv
                if kg % FSTEP == FSTEP - 1:
                    tok([acc[:, i * 128:(i + 1) * 128] for i in range(4)])
                    yield
            yacc[:, ds_] = acc

    def wait_group(i):
        with _scope("a_wait%d" % i):
            for c in a_groups[i]:
                c.wait()

    def run_all(gen):
        for _ in gen:
            pass

    def ln_side(p0, n, t0, t1):
        add_side(lambda tok: ln_rows(p0, n, tok), n // 2, t0, t1, SLAG)

    with _scope("p0_issue"):
        for grp in a_groups:
            for c in grp:
                c.start()
        for j in range(NT):
            for c in cp_b(j):
                c.start()
        zacc[...] = jnp.zeros(zacc.shape, f32)
        zero_buf[1] = jnp.zeros((8, 128), u32)
        cp_zero = cp(zero_buf.at[1], zero_buf.at[0], SEM_Z)
        cp_zero.start()
        cp_zero.wait()
    wait_group(0)
    with _scope("a0"):
        run_all(ln_rows(0, 128, None))
    wait_group(1)
    with _scope("a1"):
        run_all(ln_rows(128, 128, None))
    wait_group(2)
    with _scope("a2"):
        run_all(wk_prep(0))
        kproj(0, 256, [0])
        finish()
    if APLAN == 0:
        wait_group(3)
        with _scope("a3"):
            run_all(wk_prep(1))
            kproj(0, 256, [1])
            finish()
        wait_group(4)
        with _scope("a4"):
            run_all(wk_prep(2))
            add_side(lambda tok: wk_prep(3), 32, 300, 1500)
            ln_side(256, 128, 0, 3300)
            kproj(0, 256, [2, 3])
            finish()
        wait_group(5)
        with _scope("a5"):
            for p0 in (256, 384, 512):
                ln_side(p0 + 128, 128, 0, 3200)
                kproj(p0, 128)
            finish()
        wait_group(6)
        with _scope("a6"):
            add_side(wq_prep, 8 * 24, 0, 10000, SLAG)
            for p0 in (640, 768):
                ln_side(p0 + 128, 128, 0, 3200)
                kproj(p0, 128)
            add_side(route, 17, 0, 800)
            kproj(896, 128)
            finish()
    else:
        wait_group(3)
        with _scope("a3"):
            run_all(wk_prep(1))
            add_side(lambda tok: wk_prep(2), 32, 300, 1500)
            kproj(0, 256, [1])
            finish()
        wait_group(4)
        with _scope("a4"):
            ln_side(256, A4N, 0, 1500)
            kproj(0, 256, [2])
            finish()
        wait_group(5)
        with _scope("a5"):
            run_all(wk_prep(3))
            ln_side(256 + A4N, 128 - A4N, 0, 1400)
            kproj(0, 256, [3])
            for p0 in (256, 384):
                ln_side(p0 + 128, 128, 0, 3200)
                kproj(p0, 128)
            finish()
        wait_group(6)
        with _scope("a6"):
            add_side(wq_prep, 8 * 24, 0, 13500, SLAG)
            for p0 in (512, 640, 768):
                ln_side(p0 + 128, 128, 0, 3200)
                kproj(p0, 128)
            add_side(route, 17, 0, 800)
            kproj(896, 128)
            finish()

    def b_body(j, carry):
        with _scope("b_wait"):
            for c in cp_b(j, wait_only=True):
                c.wait()
        with _scope("b_body"):
            if not NOFFN:
              add_side(lambda tok: ffn_chunk(j, tok), (56 + 28) * 8 // FSTEP, 0, 13500)
            b_tile(j)
            finish()
        return carry

    if UNROLL_B:
        for j in range(NT):
            b_body(j, 0)
    else:
        lax.fori_loop(0, NT, b_body, 0)

    def c_body(t, carry):
        with _scope("c_body"):
            y = _rbf(jnp.sum(yacc[...], axis=0, keepdims=True))
            y = _rbf(y * _rbf(jax.nn.sigmoid(rsel[...])))
            nb = RQ - QA
            for i in range(CU):
                tt = t * CU + i
                add_side(lambda tok, tt=tt, i=i: normalise(pqb_buf.at[tt], denb_buf.at[tt], nb, qsb,
                                                          i * (nb // 2), tok),
                         4 + 23 * (nb // 16), 0, 49 * QA - 800, SLAG)
                for p in range(QA // CR):
                    out_part(tt * RQ + p * CR, CR, y, qs, tt * (RQ // 2) + p * (CR // 2))
                out_part(tt * RQ + QA, nb, y, qsb, i * (nb // 2))
            finish()
        return carry

    lax.fori_loop(0, NT // CU, c_body, 0)
    with _scope("tail"):
        cp(out_buf, out_hbm.at[0], SEM_O).wait()


@jax.jit
def pallas_parallel_sum__linear_attn_block__moe_arch_mod__prompt_kernel(
    A_x: jax.Array,
    A_wqkv: jax.Array,
    A_wo: jax.Array,
    B_x: jax.Array,
    B_w_r: jax.Array,
    B_w_gate: jax.Array,
    B_w_up: jax.Array,
    B_w_down: jax.Array,
):
    del B_x
    V = pltpu.VMEM
    scratch = [
        V((S, D), bf16),
        V((4, D, 256), bf16),
        V((D, D), bf16),
        V((4, D, 256), bf16),
        V((D, D), bf16),
        V((D,), bf16),
        V((NF, D, 1024), bf16),
        V((NF, D, 1024), bf16),
        V((NF, 1024, D), bf16),
        V((7, HP // 2, HD), u32),
        V((4, HP // 2, 1024), u32),
        V((49, HQ // 2, 256), u32),
        V((7, HD // 2, HD), u32),
        V((7, HD // 2, HD), u32),
        V((49, 128, 256), u32),
        V((S, 128), f32),
        V((S, 128), f32),
        V((S, 128), f32),
        V((8, D), f32),
        V((8, D), f32),
        V((8, 64, 128), u32),
        V((2, 64, 128), u32),
        V((64, 64, 128), u32),
        V((2, 4, RQ, D), f32),
        V((2, 4, RQ, 128), f32),
        V((4, 4, RQ - QA, D), f32),
        V((4, 4, RQ - QA, 128), f32),
        V((49, CU * (RQ - QA) // 2, 256), u32),
        V((2, 2, 128, D), f32),
        V((D, 128), f32),
        V((2, 1024, 128), f32),
        V((8, D), f32),
        V((1, D), f32),
        V((S, D), bf16),
        V((2, 8, 128), u32),
        pltpu.SMEM((1,), i32),
        pltpu.SemaphoreType.DMA((NT + 9,)),
    ]
    return pl.pallas_call(
        _kernel,
        out_shape=jax.ShapeDtypeStruct((1, S, D), bf16),
        in_specs=[pl.BlockSpec(memory_space=pl.ANY)] * 7,
        out_specs=pl.BlockSpec(memory_space=pl.ANY),
        scratch_shapes=scratch,
        compiler_params=pltpu.CompilerParams(vmem_limit_bytes=110 * 1024 * 1024,
                                             disable_bounds_checks=True,
                                             disable_semaphore_checks=True),
    )(A_x, A_wqkv, A_wo, B_w_r, B_w_gate, B_w_up, B_w_down)
```

```python
import contextlib

import jax
import jax.numpy as jnp
from jax import lax
import jax.experimental.pallas as pl
import jax.experimental.pallas.tpu as pltpu

bf16, f32, u32, i32 = jnp.bfloat16, jnp.float32, jnp.uint32, jnp.int32

S = 2048
D = 1024
F = 3584
HP = S // 2
HD = D // 2
R = 256
NT = HP // R
HQ = S // 4
RQ = HQ // NT
FW = 896
NF = F // FW
QLAG = 768
UNROLL_B = False
KW = (16, 16, 16, 16, 16, 16, 16)
CU = 1
APLAN = 1
A4N = 64
ZOUT = False
QA = 96
NOFFN = False
SLAG = 400
FSTEP = 2
CR = 32

L_ORD = (2, 3, 0, 1, 4, 5, 6)
R_ORD = (2, 0, 6, 5, 1, 4, 3)

K_SEQ = (1, 4, 0, 2, 3, 5, 6)
K_SEQ2 = (0, 1, 2, 5, 3, 4, 6)

NN = (((1,), (0,)), ((), ()))
NT_ = (((1,), (1,)), ((), ()))
TN = (((0,), (0,)), ((), ()))


SCOPES = False


def _scope(name):
    return jax.named_scope(name) if SCOPES else contextlib.nullcontext()


def _mo(v, m):
    return v if isinstance(v, int) else pl.multiple_of(v, m)


def _dot(a, b, dims):
    return lax.dot_general(a, b, dims, preferred_element_type=f32)


def _pack(v):
    return pltpu.bitcast(v.astype(bf16), u32)


def _unpack(v):
    return pltpu.bitcast(v, bf16)


def _combine(m):
    m1, m2, m3, m4, m5, m6, m7 = m
    return m1 + m4 - m5 + m7, m3 + m5, m2 + m4, m1 - m2 + m3 + m6


def _lform(a11, a12, a21, a22):
    return (a11 + a22, a21 + a22, a11, a22, a11 + a12, a21 - a11, a12 - a22)


def _rform(b11, b12, b21, b22):
    return (b11 + b22, b11, b12 - b22, b21 - b11, b22, b11 + b12, b21 + b22)


def _form2(form, blk):
    lvl1 = [form(blk[r][c], blk[r][c + 2], blk[r + 2][c], blk[r + 2][c + 2])
            for r in range(2) for c in range(2)]
    return [v for k1 in range(7) for v in form(*[lvl1[i][k1] for i in range(4)])]


class _Sym:
    def __init__(self, t):
        self.t = t

    def __add__(self, o):
        return _Sym({**self.t, **o.t})

    def __sub__(self, o):
        return _Sym({**self.t, **{k: -v for k, v in o.t.items()}})


def _phi(t):
    return jnp.where(t > 0, t + 1.0, jnp.exp(t)) + 1e-6


def _rbf(v):
    return v.astype(bf16).astype(f32)


def _layernorm_rows(xv):
    mf = jnp.sum(xv, axis=1, keepdims=True) * (1.0 / D)
    mb = _rbf(mf)
    d = xv - mb
    dm = mf - mb
    var = jnp.sum(d * d, axis=1, keepdims=True) * (1.0 / D) - dm * dm
    var = jnp.maximum(var, 0.0)
    sd = _rbf(jnp.sqrt(_rbf(_rbf(var) + 1e-5)))
    return d * (1.0 / sd)


def _kernel(x_hbm, wqkv_hbm, wo_hbm, wr_hbm, wg_hbm, wu_hbm, wd_hbm, out_hbm,
            x_buf, wk_buf, wq_buf, wv_buf, wo_buf, wr_buf, wg_buf, wu_buf, wd_buf,
            xs, ps, qs, wks, wqs, ms, sa, sb, stats, zacc, zp, tscr, tscr2, wqt, pq_buf, den_buf, pqb_buf, denb_buf, qsb, mg_buf,
            xb, hb_buf, yacc, rsel, out_buf, zero_buf, idx_s, sem):

    SEM_B, SEM_O, SEM_Z, SEM_A = 0, NT, NT + 1, NT + 2

    def cp(src, dst, s):
        return pltpu.make_async_copy(src, dst, sem.at[s])

    def cp_x(p0, n, s):
        return [cp(x_hbm.at[0, pl.ds(h * HP + p0, n), :], x_buf.at[pl.ds(h * HP + p0, n), :], s)
                for h in range(2)]

    def cp_wk(c, s):
        return [cp(wqkv_hbm.at[:, pl.ds(D + c * 256, 256)], wk_buf.at[c], s)]

    cp_wq = lambda s_: [cp(wqkv_hbm.at[:, pl.ds(0, D)], wq_buf, s_)]
    if APLAN == 0:
        a_groups = [
            [cp(wr_hbm, wr_buf.at[pl.ds(0, D)], SEM_A)] + cp_x(0, 128, SEM_A),
            cp_x(128, 128, SEM_A + 1),
            cp_wk(0, SEM_A + 2),
            cp_wk(1, SEM_A + 3),
            cp_wk(2, SEM_A + 4) + cp_x(256, 128, SEM_A + 4) + cp_wk(3, SEM_A + 4),
            cp_x(384, 384, SEM_A + 5),
            cp_x(768, 256, SEM_A + 6) + cp_wq(SEM_A + 6),
        ]
    else:
        a_groups = [
            [cp(wr_hbm, wr_buf.at[pl.ds(0, D)], SEM_A)] + cp_x(0, 128, SEM_A),
            cp_x(128, 128, SEM_A + 1),
            cp_wk(0, SEM_A + 2),
            cp_wk(1, SEM_A + 3) + cp_wk(2, SEM_A + 3),
            cp_x(256, 128, SEM_A + 4),
            cp_wk(3, SEM_A + 5) + cp_x(384, 256, SEM_A + 5),
            cp_x(640, 384, SEM_A + 6) + cp_wq(SEM_A + 6),
        ]

    def cp_b(j, wait_only=False):
        def off(v, m):
            return v if isinstance(v, int) else _mo(v, m)
        out = []
        c0 = off(j * 256, 256)
        dst = wv_buf.at[j]
        out.append(cp(dst if wait_only else wqkv_hbm.at[:, pl.ds(2 * D + c0, 256)], dst, SEM_B + j))
        dst = wo_buf.at[pl.ds(c0, 256), :]
        out.append(cp(dst if wait_only else wo_hbm.at[pl.ds(c0, 256), :], dst, SEM_B + j))
        f0 = off(j * FW, 128)
        for src, dst in ((wg_hbm.at[:, pl.ds(f0, FW)], wg_buf.at[j, :, pl.ds(0, FW)]),
                         (wu_hbm.at[:, pl.ds(f0, FW)], wu_buf.at[j, :, pl.ds(0, FW)]),
                         (wd_hbm.at[pl.ds(f0, FW), :], wd_buf.at[j, pl.ds(0, FW), :])):
            out.append(cp(dst if wait_only else src, dst, SEM_B + j))
        return out

    clock = [0]
    toks = []
    sides = []
    fwd = [None]

    def emit_tok(vals, stamp=None):
        t = None
        for v in vals:
            v = pltpu.bitcast(v, u32) if v.dtype != u32 else v
            t = v if t is None else t | v
        toks.append((clock[0] if stamp is None else stamp, t & zero_buf[0]))

    def gate(v):
        if fwd[0] is None:
            return v
        if fwd[0][1] is None:
            fwd[0][1] = pltpu.bitcast(fwd[0][0](), u32) & zero_buf[0]
        head = pltpu.bitcast(pltpu.bitcast(v[0:8], u32) | fwd[0][1], v.dtype)
        return head if v.shape[0] == 8 else jnp.concatenate([head, v[8:]], axis=0)

    def add_side(gen_fn, n, t0, t1, lag=None):
        st = {"i": 0, "n": n, "t0": clock[0] + t0, "t1": clock[0] + t1}

        def tok(vals):
            if lag is not None:
                emit_tok(vals, st["t0"] + (st["i"] + 1) * (st["t1"] - st["t0"]) // st["n"] + lag)
        st["g"] = gen_fn(tok)
        sides.append(st)

    def advance(until):
        for st in sides:
            while st["i"] < st["n"] and st["t0"] + st["i"] * (st["t1"] - st["t0"]) // st["n"] < until:
                next(st["g"], None)
                st["i"] += 1

    def finish():
        for st in sides:
            for _ in st["g"]:
                pass
        sides.clear()
        toks.clear()
        fwd[0] = None

    def mm(lhs, rhs, dims, cycles, nseg=1):
        due = [t for (c, t) in toks if c <= clock[0]]
        toks[:] = [(c, t) for (c, t) in toks if c > clock[0]]
        if due:
            head = rhs[0:8, 0:128]
            for t in due:
                head = head | t
            if rhs.shape[1] > 128:
                head = jnp.concatenate([head, rhs[0:8, 128:]], axis=1)
            rhs = jnp.concatenate([head, rhs[8:]], axis=0)
        res = _dot(lhs, _unpack(rhs), dims)
        ngr = res.shape[0] // 16
        for sg in range(nseg):
            for i in range(ngr):
                fwd[0] = [lambda sg=sg, i=i: res[i * 16:i * 16 + 8, sg * 128:(sg + 1) * 128], None]
                clock[0] += cycles // nseg // ngr
                advance(clock[0])
        return res

    def ln_rows(p_start, n_rows, tok):
        wr = wr_buf[0:D].reshape(1, D).astype(f32)
        lane = lax.broadcasted_iota(i32, (8, 128), 1)
        for c in range(n_rows // 16):
            p0 = p_start + c * 16
            ds_, rss, sts = [], [], []
            for r0 in (p0, p0 + 8, HP + p0, HP + p0 + 8):
                xv = x_buf[r0:r0 + 8, :].astype(f32)
                xg = jnp.concatenate([gate(xv[:, 0:128]), xv[:, 128:]], axis=1)
                mf = jnp.sum(xg, axis=1, keepdims=True) * (1.0 / D)
                d = xv - mf
                var = jnp.sum(d * d, axis=1, keepdims=True) * (1.0 / D)
                tr = jnp.sum(d * wr, axis=1, keepdims=True)
                rs = jnp.broadcast_to(lax.rsqrt(var + 1e-5), (8, 128))
                mf = jnp.broadcast_to(mf, (8, 128))
                sa[r0:r0 + 8, :] = 1.0 + rs
                sb[r0:r0 + 8, :] = mf * rs
                st = jnp.where(lane == 0, mf, jnp.where(lane == 1, jnp.broadcast_to(var, (8, 128)),
                                                        jnp.broadcast_to(tr, (8, 128))))
                stats[r0:r0 + 8, :] = st
                ds_.append(d)
                rss.append(rs)
                sts.append(st)
                yield
            pend.append((p0, ds_, rss, sts))
            if len(pend) > 1:
                yield from ln_finish(tok, *pend.pop(0))
        while pend:
            yield from ln_finish(tok, *pend.pop(0))

    pend = []

    def ln_finish(tok, p0, ds_, rss, sts):
        for ct in range(4):
            cl = slice(ct * 128, (ct + 1) * 128)
            cr = slice(HD + ct * 128, HD + (ct + 1) * 128)
            rg = [gate(r) for r in rss]
            x11, x12, x21, x22 = [
                jnp.concatenate([ds_[i][:, cc] * rg[i], ds_[i + 1][:, cc] * rg[i + 1]], axis=0)
                for i, cc in ((0, cl), (0, cr), (2, cl), (2, cr))]
            ops = (x11, x22, x11 + x22, x21 + x22, x11 + x12, x21 - x11, x12 - x22)
            for k in range(7):
                xs.at[k][p0 // 2:p0 // 2 + 8, cl] = _pack(ops[k])
            if tok is not None:
                tok([ops[3][0:8], ops[3][8:16], ops[4][0:8], ops[4][8:16]])
            yield

    def wk_prep(c, tok=None):
        for i in range(HD // 16):
            r0 = i * 16
            top = wk_buf[c, r0:r0 + 16, :].astype(f32)
            bot = wk_buf[c, HD + r0:HD + r0 + 16, :].astype(f32)
            ops = _rform(gate(top[:, :128]), top[:, 128:], bot[:, :128], gate(bot[:, 128:]))
            for k in range(7):
                wks.at[k][r0 // 2:r0 // 2 + 8, c * 128:(c + 1) * 128] = _pack(ops[k])
            yield

    def wq_prep(tok):
        def transpose(g):
            for ct in range(8):
                tile = gate(pltpu.bitcast(wq_buf[ct * 128:(ct + 1) * 128, g * 128:(g + 1) * 128], u32))
                wqt.at[g * 8 + ct][...] = pltpu.bitcast(_unpack(tile).T, u32)
                yield

        def combine(g):
            for j in range(4):
                for ct in range(4):
                    w11, w12, w21, w22 = [
                        _unpack(gate(wqt[g * 8 + cc, pl.ds(jj, 8, stride=8), :])).astype(f32)
                        for jj, cc in ((j, ct), (j, ct + 4), (j + 4, ct), (j + 4, ct + 4))]
                    ops = _rform(w11, w21, w12, w22)
                    for k in range(7):
                        wqs.at[k][j * 64 + g * 8:j * 64 + g * 8 + 8, ct * 128:(ct + 1) * 128] = _pack(ops[k])
                    tok([ops[5][0:8], ops[6][0:8]])
                    yield

        for g in range(9):
            if g < 8:
                yield from transpose(g)
            if g > 0:
                yield from combine(g - 1)

    def kproj(p0, n, chunks=range(4)):
        pr = pl.ds(p0 // 2, n // 2)
        for c in chunks:
            cs = slice(c * 128, (c + 1) * 128)
            m = [None] * 7
            for i, k in enumerate(K_SEQ):
                m[k] = mm(_unpack(xs[L_ORD[k], pr, :]), wks[k, :, cs], NN, n * KW[i] // 16)
            k11, k12, k21, k22 = [_phi(v) for v in _combine(m)]
            zl = (k11 + k21).reshape(n // 8, 8, 128).sum(axis=0)
            zr = (k12 + k22).reshape(n // 8, 8, 128).sum(axis=0)
            zacc[:, c * 256:c * 256 + 128] += zl
            zacc[:, c * 256 + 128:(c + 1) * 256] += zr
            ops = _lform(k11, k21, k12, k22)
            for k in range(7):
                ps.at[c][pr, k * 128:(k + 1) * 128] = _pack(ops[k])

    def z_prep():
        z = jnp.sum(zacc[...], axis=0, keepdims=True)
        zt = _pack(jnp.broadcast_to(z, (128, D)).astype(bf16).T)
        for g in range(8):
            tscr.at[g][...] = zt[g * 64:(g + 1) * 64, :]
        for j in range(8):
            blk = jnp.concatenate([tscr[g, pl.ds(j, 8, stride=8), :] for g in range(8)], axis=0)
            zp[:, j * 128:(j + 1) * 128] = _unpack(blk).T[0:8, :].astype(f32)

    def route(tok):
        rows = []
        for b in range(S // 128):
            rows.append(gate(stats[b * 128:(b + 1) * 128, :]).T[0:8, :])
            yield
        mf = jnp.concatenate([v[0:1] for v in rows], axis=0)
        var = jnp.concatenate([v[1:2] for v in rows], axis=0)
        tr = jnp.concatenate([v[2:3] for v in rows], axis=0)
        wsum = jnp.sum(wr_buf[0:D].reshape(1, D).astype(f32), axis=1, keepdims=True)
        sd = _rbf(jnp.sqrt(_rbf(_rbf(var) + 1e-5)))
        rv = _rbf((tr + (mf - _rbf(mf)) * wsum) / sd)
        rmax = jnp.max(rv)
        pos = (lax.broadcasted_iota(i32, rv.shape, 0) * 128 + lax.broadcasted_iota(i32, rv.shape, 1))
        idx = jnp.min(jnp.where(rv == rmax, pos, S - 1))
        idx_s[0] = idx
        rsel[...] = jnp.full(rsel.shape, rmax, f32)
        b0 = _mo((idx // 16) * 16, 16)
        xn = _rbf(_layernorm_rows(x_buf[pl.ds(b0, 16), :].astype(f32)))
        sel = lax.broadcasted_iota(i32, xn.shape, 0) == idx - b0
        row = jnp.sum(jnp.where(sel, xn, 0.0), axis=0, keepdims=True)
        xbv = jnp.broadcast_to(row, (128, D)).T
        xb[...] = xbv
        yacc[...] = jnp.zeros(yacc.shape, f32)
        tok([xbv[b * 128 + 120:(b + 1) * 128] for b in range(8)])
        yield

    def form2_steps(form, get, put, tok=None):
        terms = form(*[_Sym({i: 1}) for i in range(4)])
        for k1 in range(7):
            sub = []
            for r in range(2):
                for c in range(2):
                    v = None
                    for i, sg in sorted(terms[k1].t.items(), key=lambda e: -e[1]):
                        b = get(r + 2 * (i // 2), c + 2 * (i % 2))
                        if v is None:
                            v = gate16(b) if r == c else b
                        else:
                            v = v + b if sg > 0 else v - b
                    sub.append(v)
            vals = form(*sub)
            for k2, v in enumerate(vals):
                put(k1 * 7 + k2, _pack(v))
            if tok is not None:
                tok([v[o:o + 8] for v in vals[-2:] for o in (0, 8)])
            yield

    def gate16(v):
        return jnp.concatenate([gate(v[0:8]), gate(v[8:16])], axis=0)

    def q_part(j, r0, nr, pq, dn):
        prs = [pl.ds(_mo(j * (RQ // 2) + (h * HQ + r0) // 2, 8), nr // 2) for h in range(2)]
        den = [None, None]
        for c in range(4):
            m = [mm(_unpack(jnp.concatenate([xs[L_ORD[k], pr, :] for pr in prs], axis=0)),
                    wqs[k, c * 64:(c + 1) * 64, :], NT_, 2 * nr) for k in range(7)]
            q11, q12, q21, q22 = [_phi(v) for v in _combine(m)]
            cl = slice(c * 128, (c + 1) * 128)
            cr = slice(HD + c * 128, HD + (c + 1) * 128)
            zl, zr = zp[0:1, cl], zp[0:1, cr]
            dt, db = q11 * zl + q12 * zr, q21 * zl + q22 * zr
            den = [dt, db] if c == 0 else [den[0] + dt, den[1] + db]
            for h in range(2):
                hs = slice(h * nr, (h + 1) * nr)
                pq.at[h][0:nr, cl] = q11[hs]
                pq.at[h][0:nr, cr] = q12[hs]
                pq.at[2 + h][0:nr, cl] = q21[hs]
                pq.at[2 + h][0:nr, cr] = q22[hs]
            emit_tok([d[i * 8:(i + 1) * 8] for d in den for i in range(nr // 4)], clock[0] + QLAG)
            if c == 3:
                for q in range(4):
                    dn.at[q][0:nr, :] = den[q // 2][(q % 2) * nr:(q % 2 + 1) * nr]
            yield

    def normalise(pq, dn, nr, dst, p0, tok=None):
        lane = lax.broadcasted_iota(i32, (16, 128), 1)

        def recips(c):
            recs = []
            for q in range(4):
                d = gate16(dn[q, c * 16:(c + 1) * 16, :])
                d = d + jnp.where(lane % 2 == 0, pltpu.roll(d, 127, 1), pltpu.roll(d, 1, 1))
                d = d + jnp.where(lane % 4 < 2, pltpu.roll(d, 126, 1), pltpu.roll(d, 2, 1))
                recs.append(1.0 / (d + 1e-6))
            return recs

        nxt = recips(0)
        for _ in range(4):
            yield
        for c in range(nr // 16):
            rq = slice(c * 16, (c + 1) * 16)
            p2 = pl.ds(_mo(p0 + c * 8, 8), 8)
            recs = nxt
            for q in range(4):
                for hf in range(2):
                    cs = slice(hf * HD, (hf + 1) * HD)
                    pq.at[q][rq, cs] = pq[q, rq, cs] * jnp.concatenate([gate16(recs[q])] * 4, axis=1)
                    yield
            if c + 1 < nr // 16:
                nxt = recips(c + 1)
            yield
            for ct in range(2):
                def put(k, v):
                    dst.at[k][p2, ct * 128:(ct + 1) * 128] = v
                yield from form2_steps(
                    _lform, lambda q, u: pq[q, rq, u * 256 + ct * 128:u * 256 + (ct + 1) * 128], put, tok)

    def b_tile(j):
        jc = pl.ds(_mo(j * 128, 128), 128)
        if not ZOUT:
            z_prep()
        nb = RQ - QA
        j2 = j & 1
        for _ in q_part(j, 0, QA, pq_buf.at[j2], den_buf.at[j2]):
            pass
        add_side(lambda tok: normalise(pq_buf.at[j2], den_buf.at[j2], QA, qs, j * (RQ // 2)),
                 4 + 23 * (QA // 16), 400, 7000)
        m = [mm(_unpack(ps[j, :, k * 128:(k + 1) * 128]), xs[R_ORD[k]], TN, 1024, 4) for k in range(7)]
        g11, g12, g21, g22 = _combine(m)
        hm = (lax.broadcasted_iota(i32, (128, 128), 0) // 32
              == lax.broadcasted_iota(i32, (128, 128), 1) // 32)
        qb = q_part(j, QA, nb, pqb_buf.at[j], denb_buf.at[j])
        next(qb)
        kvps = []
        for half, (ga, gb) in enumerate(((g11, g12), (g21, g22))):
            gg = jnp.concatenate([ga, gb], axis=1).astype(bf16)
            clock[0] += 256
            kv = jnp.where(hm, _dot(gg, wv_buf[j, :, half * 128:(half + 1) * 128], NN), 0.0)
            tscr2.at[half][...] = _pack(kv)
            kvps.append(_unpack(jnp.concatenate(
                [tscr2[half, pl.ds(jj, 8, stride=8), :] for jj in range(8)], axis=0)))
        next(qb)
        mg = mg_buf.at[j2]
        for half in range(2):
            gr = pl.ds(_mo(j * 256 + half * 128, 128), 128)
            clock[0] += 256
            mg.at[half][...] = _dot(kvps[half], wo_buf[gr, :], NN)

        def m_form(tok):
            for half in range(2):
                g = 2 * j + half
                for jj in range(2):
                    for ct in range(2):
                        def put(k, v):
                            ms.at[k][pl.ds(_mo(jj * 64 + g * 8, 8), 8), ct * 128:(ct + 1) * 128] = v
                        yield from form2_steps(
                            _rform, lambda q, u: mg[half, (2 * q + jj) * 16:(2 * q + jj + 1) * 16,
                                                    u * 256 + ct * 128:u * 256 + (ct + 1) * 128], put)

        add_side(m_form, 56, 0, 28 * nb - 100)
        for _ in qb:
            pass

    def out_part(p0, nr, y, src, pr0):
        pr = pl.ds(_mo(pr0, 8), nr // 2)
        rows = [pl.ds(_mo(q * HQ + p0, 16), nr) for q in range(4)]
        row = lax.broadcasted_iota(i32, (nr, 256), 0) + p0
        m1 = [None] * 7
        for k1 in K_SEQ2:
            m2 = [None] * 7
            for k2 in K_SEQ2:
                m2[k2] = mm(_unpack(src[k1 * 7 + k2, pr, :]), ms[k1 * 7 + k2], NN, nr)
            m1[k1] = _combine(m2)
        outs = [_combine([m1[k1][s2] for k1 in range(7)]) for s2 in range(4)]
        for s1 in (3, 2, 1, 0):
            for s2 in range(4):
                q = (s1 // 2) * 2 + s2 // 2
                u = (s1 % 2) * 2 + s2 % 2
                rr, cc = rows[q], pl.ds(u * 256, 256)
                a = jnp.concatenate([sa[rr, :]] * 2, axis=1)
                b = jnp.concatenate([sb[rr, :]] * 2, axis=1)
                o = outs[s2][s1] + jnp.where(row + q * HQ == idx_s[0], y[:, u * 256:(u + 1) * 256], 0.0)
                out_buf[rr, cc] = (x_buf[rr, cc].astype(f32) * a - b + o).astype(bf16)
                if s2 % 2 == 1:
                    ch = pl.ds((s1 % 2) * HD, HD)
                    cp(out_buf.at[rr, ch], out_hbm.at[0, rr, ch], SEM_O).start()

    def ffn_chunk(c, tok):
        hs = []
        for f0 in range(0, FW, 256):
            w = min(256, FW - f0)
            fs = slice(f0, f0 + w)
            ag = jnp.zeros((8, w), f32)
            au = jnp.zeros((8, w), f32)
            step = FSTEP * 256 // w
            for kg in range(D // 8):
                xv = jnp.concatenate([gate(xb[8 * kg:8 * kg + 8, :])] * (w // 128), axis=1)
                ag = ag + wg_buf[c, 8 * kg:8 * kg + 8, fs].astype(f32) * xv
                au = au + wu_buf[c, 8 * kg:8 * kg + 8, fs].astype(f32) * xv
                if kg % step == step - 1:
                    tok([a[:, i * 128:(i + 1) * 128] for a in (ag, au) for i in range(w // 128)])
                    yield
            g = _rbf(jnp.sum(ag, axis=0, keepdims=True))
            u = _rbf(jnp.sum(au, axis=0, keepdims=True))
            h = _rbf(_rbf(g * jax.nn.sigmoid(g)) * u)
            hb_buf.at[c & 1][fs, :] = jnp.broadcast_to(h, (128, w)).T
        for d0 in range(0, D, 512):
            ds_ = slice(d0, d0 + 512)
            acc = yacc[:, ds_]
            for kg in range(FW // 8):
                hv = jnp.concatenate([gate(hb_buf[c & 1, 8 * kg:8 * kg + 8, :])] * 4, axis=1)
                acc = acc + wd_buf[c, 8 * kg:8 * kg + 8, ds_].astype(f32) * hv
                if kg % FSTEP == FSTEP - 1:
                    tok([acc[:, i * 128:(i + 1) * 128] for i in range(4)])
                    yield
            yacc[:, ds_] = acc

    def wait_group(i):
        with _scope("a_wait%d" % i):
            for c in a_groups[i]:
                c.wait()

    def run_all(gen):
        for _ in gen:
            pass

    def ln_side(p0, n, t0, t1):
        add_side(lambda tok: ln_rows(p0, n, tok), n // 2, t0, t1, SLAG)

    with _scope("p0_issue"):
        for grp in a_groups:
            for c in grp:
                c.start()
        for j in range(NT):
            for c in cp_b(j):
                c.start()
        zacc[...] = jnp.zeros(zacc.shape, f32)
        zero_buf[1] = jnp.zeros((8, 128), u32)
        cp_zero = cp(zero_buf.at[1], zero_buf.at[0], SEM_Z)
        cp_zero.start()
        cp_zero.wait()
    wait_group(0)
    with _scope("a0"):
        run_all(ln_rows(0, 128, None))
    wait_group(1)
    with _scope("a1"):
        run_all(ln_rows(128, 128, None))
    wait_group(2)
    with _scope("a2"):
        run_all(wk_prep(0))
        kproj(0, 256, [0])
        finish()
    if APLAN == 0:
        wait_group(3)
        with _scope("a3"):
            run_all(wk_prep(1))
            kproj(0, 256, [1])
            finish()
        wait_group(4)
        with _scope("a4"):
            run_all(wk_prep(2))
            add_side(lambda tok: wk_prep(3), 32, 300, 1500)
            ln_side(256, 128, 0, 3300)
            kproj(0, 256, [2, 3])
            finish()
        wait_group(5)
        with _scope("a5"):
            for p0 in (256, 384, 512):
                ln_side(p0 + 128, 128, 0, 3200)
                kproj(p0, 128)
            finish()
        wait_group(6)
        with _scope("a6"):
            add_side(wq_prep, 8 * 24, 0, 10000, SLAG)
            for p0 in (640, 768):
                ln_side(p0 + 128, 128, 0, 3200)
                kproj(p0, 128)
            add_side(route, 17, 0, 800)
            kproj(896, 128)
            finish()
    else:
        wait_group(3)
        with _scope("a3"):
            run_all(wk_prep(1))
            add_side(lambda tok: wk_prep(2), 32, 300, 1500)
            kproj(0, 256, [1])
            finish()
        wait_group(4)
        with _scope("a4"):
            ln_side(256, A4N, 0, 1500)
            kproj(0, 256, [2])
            finish()
        wait_group(5)
        with _scope("a5"):
            run_all(wk_prep(3))
            ln_side(256 + A4N, 128 - A4N, 0, 1400)
            kproj(0, 256, [3])
            for p0 in (256, 384):
                ln_side(p0 + 128, 128, 0, 3200)
                kproj(p0, 128)
            finish()
        wait_group(6)
        with _scope("a6"):
            add_side(wq_prep, 8 * 24, 0, 13500, SLAG)
            for p0 in (512, 640, 768):
                ln_side(p0 + 128, 128, 0, 3200)
                kproj(p0, 128)
            add_side(route, 17, 0, 800)
            kproj(896, 128)
            finish()

    if ZOUT:
        z_prep()

    def b_body(j, carry):
        with _scope("b_wait"):
            for c in cp_b(j, wait_only=True):
                c.wait()
        with _scope("b_body"):
            if not NOFFN:
              add_side(lambda tok: ffn_chunk(j, tok), (56 + 28) * 8 // FSTEP, 0, 13500)
            b_tile(j)
            finish()
        return carry

    if UNROLL_B:
        for j in range(NT):
            b_body(j, 0)
    else:
        lax.fori_loop(0, NT, b_body, 0)

    def c_body(t, carry):
        with _scope("c_body"):
            y = _rbf(jnp.sum(yacc[...], axis=0, keepdims=True))
            y = _rbf(y * _rbf(jax.nn.sigmoid(rsel[0:1, :])))
            nb = RQ - QA
            for i in range(CU):
                tt = t * CU + i
                add_side(lambda tok, tt=tt, i=i: normalise(pqb_buf.at[tt], denb_buf.at[tt], nb, qsb,
                                                          i * (nb // 2), tok),
                         4 + 23 * (nb // 16), 0, 49 * QA - 800, SLAG)
                for p in range(QA // CR):
                    out_part(tt * RQ + p * CR, CR, y, qs, tt * (RQ // 2) + p * (CR // 2))
                out_part(tt * RQ + QA, nb, y, qsb, i * (nb // 2))
            finish()
        return carry

    lax.fori_loop(0, NT // CU, c_body, 0)
    with _scope("tail"):
        cp(out_buf, out_hbm.at[0], SEM_O).wait()


@jax.jit
def pallas_parallel_sum__linear_attn_block__moe_arch_mod__prompt_kernel(
    A_x: jax.Array,
    A_wqkv: jax.Array,
    A_wo: jax.Array,
    B_x: jax.Array,
    B_w_r: jax.Array,
    B_w_gate: jax.Array,
    B_w_up: jax.Array,
    B_w_down: jax.Array,
):
    del B_x
    V = pltpu.VMEM
    scratch = [
        V((S, D), bf16),
        V((4, D, 256), bf16),
        V((D, D), bf16),
        V((4, D, 256), bf16),
        V((D, D), bf16),
        V((8 * D,), bf16),
        V((NF, D, 1024), bf16),
        V((NF, D, 1024), bf16),
        V((NF, 1024, D), bf16),
        V((7, HP // 2, HD), u32),
        V((4, HP // 2, 1024), u32),
        V((49, HQ // 2, 256), u32),
        V((7, HD // 2, HD), u32),
        V((7, HD // 2, HD), u32),
        V((49, 128, 256), u32),
        V((S, 128), f32),
        V((S, 128), f32),
        V((S, 128), f32),
        V((8, D), f32),
        V((8, D), f32),
        V((8, 64, 128), u32),
        V((2, 64, 128), u32),
        V((64, 64, 128), u32),
        V((2, 4, RQ, D), f32),
        V((2, 4, RQ, 128), f32),
        V((4, 4, RQ - QA, D), f32),
        V((4, 4, RQ - QA, 128), f32),
        V((49, CU * (RQ - QA) // 2, 256), u32),
        V((2, 2, 128, D), f32),
        V((D, 128), f32),
        V((2, 1024, 128), f32),
        V((8, D), f32),
        V((8, D), f32),
        V((S, D), bf16),
        V((4, 8, 128), u32),
        pltpu.SMEM((1,), i32),
        pltpu.SemaphoreType.DMA((NT + 9,)),
    ]
    return pl.pallas_call(
        _kernel,
        out_shape=jax.ShapeDtypeStruct((1, S, D), bf16),
        in_specs=[pl.BlockSpec(memory_space=pl.ANY)] * 7,
        out_specs=pl.BlockSpec(memory_space=pl.ANY),
        scratch_shapes=scratch,
        compiler_params=pltpu.CompilerParams(vmem_limit_bytes=110 * 1024 * 1024,
                                             disable_bounds_checks=True,
                                             disable_semaphore_checks=True),
    )(A_x, A_wqkv, A_wo, B_w_r, B_w_gate, B_w_up, B_w_down)
```

```python
import contextlib

import jax
import jax.numpy as jnp
from jax import lax
import jax.experimental.pallas as pl
import jax.experimental.pallas.tpu as pltpu

bf16, f32, u32, i32 = jnp.bfloat16, jnp.float32, jnp.uint32, jnp.int32

S = 2048
D = 1024
F = 3584
HP = S // 2
HD = D // 2
HQ = S // 4
BQ = HQ // 2
FH = F // 2
F1 = 256
QB = 64
QN = 48
QW = (20, 28, 28, 12, 8, 8, 8)
A6 = (7500, 7000, 10000, 9000, 13800, 10500, None)
LNTOK = 0
GLAG = 0
RECQ = True
FUSE = False
QSPLIT = 6
SLAG = 400
FSTEP = 2
CR = 32
XN = 128
VMEM_MB = 120
CT = 128

L_ORD = (2, 3, 0, 1, 4, 5, 6)
R_ORD = (2, 0, 6, 5, 1, 4, 3)

K_SEQ = (1, 4, 0, 2, 3, 5, 6)
K_SEQ2 = (0, 1, 2, 5, 3, 4, 6)

NN = (((1,), (0,)), ((), ()))
NT_ = (((1,), (1,)), ((), ()))
TN = (((0,), (0,)), ((), ()))


SCOPES = False


def _scope(name):
    return jax.named_scope(name) if SCOPES else contextlib.nullcontext()


def _mo(v, m):
    return v if isinstance(v, int) else pl.multiple_of(v, m)


def _dot(a, b, dims):
    return lax.dot_general(a, b, dims, preferred_element_type=f32)


def _pack(v):
    return pltpu.bitcast(v.astype(bf16), u32)


def _unpack(v):
    return pltpu.bitcast(v, bf16)


def _combine(m):
    m1, m2, m3, m4, m5, m6, m7 = m
    return m1 + m4 - m5 + m7, m3 + m5, m2 + m4, m1 - m2 + m3 + m6


def _lform(a11, a12, a21, a22):
    return (a11 + a22, a21 + a22, a11, a22, a11 + a12, a21 - a11, a12 - a22)


def _rform(b11, b12, b21, b22):
    return (b11 + b22, b11, b12 - b22, b21 - b11, b22, b11 + b12, b21 + b22)


def _sform(x11, x12, x21, x22):
    return (x11, x22, x11 + x22, x21 + x22, x11 + x12, x21 - x11, x12 - x22)


class _Sym:
    def __init__(self, t):
        self.t = t

    def __add__(self, o):
        return _Sym({**self.t, **o.t})

    def __sub__(self, o):
        return _Sym({**self.t, **{k: -v for k, v in o.t.items()}})


def _phi(t):
    return jnp.where(t > 0, t + 1.0, jnp.exp(t)) + 1e-6


def _rbf(v):
    return v.astype(bf16).astype(f32)


def _layernorm_rows(xv):
    mf = jnp.sum(xv, axis=1, keepdims=True) * (1.0 / D)
    mb = _rbf(mf)
    d = xv - mb
    dm = mf - mb
    var = jnp.sum(d * d, axis=1, keepdims=True) * (1.0 / D) - dm * dm
    var = jnp.maximum(var, 0.0)
    sd = _rbf(jnp.sqrt(_rbf(_rbf(var) + 1e-5)))
    return d * (1.0 / sd)


def _kernel(x_hbm, wqkv_hbm, wo_hbm, wr_hbm, wg_hbm, wu_hbm, wd_hbm, out_hbm,
            x_buf, wv_buf, wo_buf, wr_buf, wg_buf, wu_buf, wd_buf,
            xs, wqs, sa, sb, zacc, zp, pk_buf, xb, yacc, rsel, zero_buf,
            wks, stats, wqt, ps_raw, qs, ms, tscr, tscr2, pq_raw, den_raw, pqb_buf, denb_buf, qsb,
            mg_raw, hb_raw, out_buf, idx_s, sem):
    wq_buf = out_buf.at[pl.ds(0, D), :]
    wk_buf = out_buf.at[pl.ds(D, D), :]

    SEM_B, SEM_O, SEM_Z, SEM_A = 0, 4, 5, 6

    def cp(src, dst, s):
        return pltpu.make_async_copy(src, dst, sem.at[s])

    def cp_x(r0, n, s):
        rows = [pl.ds(_mo(q * HQ + r0, 16), n) for q in range(4)]
        return [cp(x_hbm.at[0, r, :], x_buf.at[r, :], s) for r in rows]

    def cp_wk(c, s):
        return [cp(wqkv_hbm.at[:, pl.ds(_mo(D + h * HD + c * 128, 128), 128)],
                   wk_buf.at[:, pl.ds(_mo(c * 256 + h * 128, 128), 128)], s) for h in range(2)]

    cp_wr = cp(wr_hbm, wr_buf.at[pl.ds(0, D)], SEM_Z)

    def make_a_groups():
        return [
            cp_x(0, 64, SEM_A),
            cp_x(64, 64, SEM_A + 1),
            cp_wk(0, SEM_A + 2),
            cp_wk(1, SEM_A + 3),
            cp_wk(2, SEM_A + 4) + cp_x(128, 64, SEM_A + 4),
            cp_wk(3, SEM_A + 5) + cp_x(192, 128, SEM_A + 5),
            cp_x(320, 192, SEM_A + 6) + [cp(wqkv_hbm.at[:, pl.ds(0, D)], wq_buf, SEM_A + 6)],
        ]

    def cp_b(j, part, wait_only=False):
        pairs = []
        f0, fw = (0, F1) if part == 0 else (F1, FH - F1)
        fs = pl.ds(_mo(j * FH + f0, 128), fw)
        pairs += [(wg_hbm.at[:, fs], wg_buf.at[j, :, pl.ds(f0, fw)]),
                  (wu_hbm.at[:, fs], wu_buf.at[j, :, pl.ds(f0, fw)]),
                  (wd_hbm.at[fs, :], wd_buf.at[j, pl.ds(f0, fw), :])]
        if part == 1:
            for a in range(4):
                c0 = _mo((2 * a + j) * 128, 128)
                pairs += [(wqkv_hbm.at[:, pl.ds(2 * D + c0, 128)], wv_buf.at[j, :, pl.ds(a * 128, 128)]),
                          (wo_hbm.at[pl.ds(c0, 128), :], wo_buf.at[j, pl.ds(a * 128, 128), :])]
        return [cp(dst if wait_only else src, dst, SEM_B + 2 * j + part) for src, dst in pairs]

    clock = [0]
    toks = []
    sides = []
    fwd = [None]

    def emit_tok(vals, stamp=None):
        t = None
        for v in vals:
            v = pltpu.bitcast(v, u32) if v.dtype != u32 else v
            t = v if t is None else t | v
        toks.append((clock[0] if stamp is None else stamp, t & zero_buf[0]))

    def gate(v):
        if fwd[0] is None:
            return v
        if fwd[0][1] is None:
            fwd[0][1] = pltpu.bitcast(fwd[0][0](), u32) & zero_buf[0]
        head = pltpu.bitcast(pltpu.bitcast(v[0:8], u32) | fwd[0][1], v.dtype)
        return head if v.shape[0] == 8 else jnp.concatenate([head, v[8:]], axis=0)

    def add_side(gen_fn, n, t0, t1, lag=None):
        st = {"i": 0, "n": n, "t0": clock[0] + t0, "t1": clock[0] + t1}

        def tok(vals):
            if lag is not None:
                emit_tok(vals, st["t0"] + (st["i"] + 1) * (st["t1"] - st["t0"]) // st["n"] + lag)
        st["g"] = gen_fn(tok)
        sides.append(st)

    def advance(until):
        for st in sides:
            while st["i"] < st["n"] and st["t0"] + st["i"] * (st["t1"] - st["t0"]) // st["n"] < until:
                next(st["g"], None)
                st["i"] += 1

    def finish():
        for st in sides:
            for _ in st["g"]:
                pass
        sides.clear()
        toks.clear()
        fwd[0] = None

    def mm(lhs, rhs, dims, cycles, nseg=1):
        due = [t for (c, t) in toks if c <= clock[0]]
        toks[:] = [(c, t) for (c, t) in toks if c > clock[0]]
        if due:
            head = rhs[0:8, 0:128]
            for t in due:
                head = head | t
            if rhs.shape[1] > 128:
                head = jnp.concatenate([head, rhs[0:8, 128:]], axis=1)
            rhs = jnp.concatenate([head, rhs[8:]], axis=0)
        res = _dot(lhs, _unpack(rhs), dims)
        ngr = res.shape[0] // 16
        for sg in range(nseg):
            for i in range(ngr):
                fwd[0] = [lambda sg=sg, i=i: res[i * 16:i * 16 + 8, sg * 128:(sg + 1) * 128], None]
                clock[0] += cycles // nseg // ngr
                advance(clock[0])
        return res

    def gate16(v):
        return jnp.concatenate([gate(v[0:8]), gate(v[8:16])], axis=0)

    def form_steps(form, get, put, tok=None, inner=None, gated=False):
        terms = form(*[_Sym({i: 1}) for i in range(4)])
        for k1 in range(7):
            sub = []
            for r in range(2):
                for c in range(2):
                    v = None
                    for i, sg in sorted(terms[k1].t.items(), key=lambda e: -e[1]):
                        b = get(r + 2 * (i // 2), c + 2 * (i % 2))
                        if v is None:
                            v = gate16(b) if r == c and not gated else b
                        else:
                            v = v + b if sg > 0 else v - b
                    sub.append(v)
            vals = []
            for k2, v in (enumerate(form(*sub)) if inner is None else inner(sub)):
                vals.append(v)
                put(k1, k2, _pack(v))
            if tok is not None:
                tok([v[o:o + 8] for v in vals[-2:] for o in (0, 8)])
            yield

    def strassen2(lhs, rhs, dims, cycles, nseg=1, wts=(16,) * 7):
        m1 = [None] * 7
        for i1, k1 in enumerate(K_SEQ2):
            m2 = [None] * 7
            for k2 in K_SEQ2:
                m2[k2] = mm(lhs(k1, k2), rhs(k1, k2), dims, cycles * wts[i1] // 16, nseg)
                yield
            m1[k1] = _combine(m2)
        out = [[None] * 4 for _ in range(4)]
        for s2 in range(4):
            for s1, v in enumerate(_combine([m1[k1][s2] for k1 in range(7)])):
                out[(s1 // 2) * 2 + s2 // 2][(s1 % 2) * 2 + s2 % 2] = v
        return out

    def row_views(base):
        if isinstance(base, int) and base == 0:
            return x_buf, sa, sb, stats, xn_buf, xs
        b = _mo(base, 64)
        return ([r.at[pl.ds(b, S - 64), :] for r in (x_buf, sa, sb, stats)]
                + [xn_buf.at[:, pl.ds(b, 64), :], xs.at[:, pl.ds(_mo(base // 2, 32), 32), :]])

    def xs_form(r0, tok, which="all", base=0):
        xn_v, xs_v = row_views(base)[4:]
        rows = slice(r0 % XN, r0 % XN + 16)

        def inner(sub):
            full = list(enumerate(_sform(*sub))) + [(7, sub[1]), (8, sub[2])]
            return [full[e] for e in {"all": (0, 1, 7, 8, 2, 5, 6, 3, 4), "l1": (0, 1, 7, 8),
                                      "l2": (2, 5, 6, 3, 4)}[which]]
        for ct in range(2):
            def put(k1, k2, v):
                xs_v.at[k1 * 9 + k2][r0 // 2:r0 // 2 + 8, ct * 128:(ct + 1) * 128] = v
            yield from form_steps(
                _sform, lambda q, u: xn_v[q, rows, u * 256 + ct * 128:u * 256 + (ct + 1) * 128],
                put, tok, inner)

    def ln_rows(r_start, n_rows, tok, which="all", base=0):
        x_v, sa_v, sb_v, st_v, xn_v, _ = row_views(base)
        wr = wr_buf[0:D].reshape(1, D).astype(f32)
        lane = lax.broadcasted_iota(i32, (8, 128), 1)
        for c in range(n_rows // 16 + 1):
            r0 = r_start + c * 16
            form = xs_form(r0 - 16, tok, which, base) if c > 0 else iter(())
            for g in range(8 if c < n_rows // 16 else 0):
                q, o = g // 2, (g % 2) * 8
                rg = q * HQ + r0 + o
                xv = x_v[rg:rg + 8, :].astype(f32)
                xg = jnp.concatenate([gate(xv[:, 0:128]), xv[:, 128:]], axis=1)
                mf = jnp.sum(xg, axis=1, keepdims=True) * (1.0 / D)
                d = xv - mf
                var = jnp.sum(d * d, axis=1, keepdims=True) * (1.0 / D)
                tr = jnp.sum(d * wr, axis=1, keepdims=True)
                rs = lax.rsqrt(var + 1e-5)
                xn = d * rs
                xn_v.at[q][r0 % XN + o:r0 % XN + o + 8, :] = xn
                rs = jnp.broadcast_to(rs, (8, 128))
                mf = jnp.broadcast_to(mf, (8, 128))
                sa_v[rg:rg + 8, :] = 1.0 + rs
                sb_v[rg:rg + 8, :] = mf * rs
                st = jnp.where(lane == 0, mf, jnp.where(lane == 1, jnp.broadcast_to(var, (8, 128)),
                                                        jnp.broadcast_to(tr, (8, 128))))
                st_v[rg:rg + 8, :] = st
                if tok is not None and LNTOK:
                    tok([rs, st][:LNTOK])
                yield
                if g >= 2 and c > 0:
                    for _ in range(2):
                        next(form)
                        yield
            yield from form

    def wk_prep(c, tok=None):
        cs = pl.ds(_mo(c * 256, 256), 256)
        for i in range(HD // 16):
            r0 = i * 16
            top = wk_buf[r0:r0 + 16, cs].astype(f32)
            bot = wk_buf[HD + r0:HD + r0 + 16, cs].astype(f32)
            ops = _rform(gate(top[:, :128]), top[:, 128:], bot[:, :128], gate(bot[:, 128:]))
            for k in range(7):
                wks.at[c][r0 // 2:r0 // 2 + 8, k * 128:(k + 1) * 128] = _pack(ops[k])
            yield

    def wq_perm(tok):
        def permute(kt):
            for g in range(8):
                tile = gate(pltpu.bitcast(wq_buf[kt * 128:(kt + 1) * 128, g * 128:(g + 1) * 128], u32))
                wqt.at[kt * 8 + g][...] = pltpu.bitcast(_unpack(tile).T, u32)
                yield

        def back(kt):
            for j in range(8):
                tile = gate(jnp.concatenate([wqt[kt * 8 + g, pl.ds(j, 8, stride=8), :] for g in range(8)],
                                            axis=0))
                v = pltpu.bitcast(_unpack(tile).T, u32)
                ps[(kt % 4) * 64:(kt % 4 + 1) * 64, (kt // 4) * D + j * 128:(kt // 4) * D + (j + 1) * 128] = v
                tok([v[56:64]])
                yield

        order = (0, 2, 4, 6, 1, 3, 5, 7)
        for n in range(10):
            if n < 8:
                yield from permute(order[n])
            if n > 1:
                yield from back(order[n - 2])

    def wq_form(tok):
        for i in range(16):
            for ct in range(2):
                def put(k1, k2, v):
                    wqs.at[k1 * 7 + k2][i * 8:(i + 1) * 8, ct * 128:(ct + 1) * 128] = v
                yield from form_steps(
                    _rform, lambda r, c: _unpack(gate(
                        ps[(r % 2) * 128 + i * 8:(r % 2) * 128 + (i + 1) * 8,
                           (r // 2) * D + c * 256 + ct * 128:(r // 2) * D + c * 256 + (ct + 1) * 128]
                    )).astype(f32), put, tok,
                    gated=True)

    def kproj(r0, n, chunks=((0, 0), (0, 1), (1, 0), (1, 1))):
        pr = pl.ds(r0 // 2, n // 2)
        for ch, ct in chunks:
            c = 2 * ch + ct
            m = [None] * 7
            for k in K_SEQ:
                e11, e22, e12, e21 = [xs[L_ORD[k] * 9 + e, pr, :] for e in (0, 1, 7, 8)]
                lhs = jnp.concatenate([jnp.concatenate([e11, e12], axis=1),
                                       jnp.concatenate([e21, e22], axis=1)], axis=0)
                m[k] = mm(_unpack(lhs), wks[c, :, k * 128:(k + 1) * 128], NN, 2 * n)
            kk = [_phi(v) for v in _combine(m)]
            for h in range(2):
                zacc[:, pl.ds(_mo(h * HD + c * 128, 128), 128)] += (
                    (kk[h] + kk[2 + h]).reshape(n // 4, 8, 128).sum(axis=0))
            for s1 in range(4):
                u = (s1 % 2) * 2 + ch
                for h in range(2):
                    pk_buf.at[ct, (s1 // 2) * 2 + h][r0:r0 + n, u * 128:(u + 1) * 128] = (
                        kk[s1][h * n:(h + 1) * n])

    def z_prep():
        z = jnp.sum(zacc[...], axis=0, keepdims=True)
        zt = _pack(jnp.broadcast_to(z, (128, D)).astype(bf16).T)
        for g in range(8):
            tscr.at[g][...] = zt[g * 64:(g + 1) * 64, :]
        for j in range(8):
            blk = jnp.concatenate([tscr[g, pl.ds(j, 8, stride=8), :] for g in range(8)], axis=0)
            zp[:, j * 128:(j + 1) * 128] = _unpack(blk).T[0:8, :].astype(f32)

    def route(tok):
        rows = []
        for b in range(S // 128):
            rows.append(gate(stats[b * 128:(b + 1) * 128, :]).T[0:8, :])
            yield
        mf = jnp.concatenate([v[0:1] for v in rows], axis=0)
        var = jnp.concatenate([v[1:2] for v in rows], axis=0)
        tr = jnp.concatenate([v[2:3] for v in rows], axis=0)
        wsum = jnp.sum(wr_buf[0:D].reshape(1, D).astype(f32), axis=1, keepdims=True)
        sd = _rbf(jnp.sqrt(_rbf(_rbf(var) + 1e-5)))
        rv = _rbf((tr + (mf - _rbf(mf)) * wsum) / sd)
        rmax = jnp.max(rv)
        pos = (lax.broadcasted_iota(i32, rv.shape, 0) * 128 + lax.broadcasted_iota(i32, rv.shape, 1))
        idx = jnp.min(jnp.where(rv == rmax, pos, S - 1))
        idx_s[0] = idx
        rsel[...] = jnp.full(rsel.shape, rmax, f32)
        b0 = _mo((idx // 16) * 16, 16)
        xn = _rbf(_layernorm_rows(x_buf[pl.ds(b0, 16), :].astype(f32)))
        sel = lax.broadcasted_iota(i32, xn.shape, 0) == idx - b0
        row = jnp.sum(jnp.where(sel, xn, 0.0), axis=0, keepdims=True)
        xbv = jnp.broadcast_to(row, (128, D)).T
        xb[...] = xbv
        yacc[...] = jnp.zeros(yacc.shape, f32)
        tok([xbv[b * 128 + 120:(b + 1) * 128] for b in range(8)])
        yield

    def ps_form(j, tok):
        for c in range(HQ // 16):
            def put(k1, k2, v):
                k = k1 * 7 + k2
                ps[c * 8:(c + 1) * 8, k * 128:(k + 1) * 128] = v
            yield from form_steps(
                _lform, lambda r, q: pk_buf[j, q, c * 16:(c + 1) * 16, r * 128:(r + 1) * 128], put, tok)

    def q_rows(j, r0, n, pq, rc, d0, rec):
        xj = xs.at[:, pl.ds(_mo(j * (BQ // 2), BQ // 2), BQ // 2), :]
        pr = slice(r0 // 2, (r0 + n) // 2)
        blk = yield from strassen2(lambda k1, k2: _unpack(xj[L_ORD[k1] * 9 + L_ORD[k2], pr, :]),
                                   lambda k1, k2: wqs[k1 * 7 + k2], NN, n, 1, QW)
        lane = lax.broadcasted_iota(i32, (n, 128), 1)
        for q in range(4):
            d = None
            for u in (3, 2, 1, 0):
                v = _phi(blk[q][u])
                pq.at[q][d0:d0 + n, u * 256:(u + 1) * 256] = v
                t = v * zp[0:1, u * 256:(u + 1) * 256]
                t = t[:, :128] + t[:, 128:]
                d = t if d is None else d + t
            if rec:
                d = recip(d, lane)
            rc.at[q][d0:d0 + n, :] = d

    def recip(d, lane):
        d = d + jnp.where(lane % 2 == 0, pltpu.roll(d, 127, 1), pltpu.roll(d, 1, 1))
        d = d + jnp.where(lane % 4 < 2, pltpu.roll(d, 126, 1), pltpu.roll(d, 2, 1))
        return 1.0 / (d + 1e-6)

    def normalise(pq, rc, nr, dst, p0, raw, tok=None):
        lane = lax.broadcasted_iota(i32, (16, 128), 1)

        def fix(c):
            if c < nr // 16 and raw(c * 16):
                for q in range(4):
                    rq = slice(c * 16, (c + 1) * 16)
                    rc.at[q][rq, :] = recip(gate16(rc[q, rq, :]), lane)

        fix(0)
        if raw(0):
            for _ in range(4):
                yield
        for c in range(nr // 16):
            rq = slice(c * 16, (c + 1) * 16)
            p2 = pl.ds(_mo(p0 + c * 8, 8), 8)
            fix(c + 1)
            for q in range(4):
                for hf in range(2):
                    cs = slice(hf * HD, (hf + 1) * HD)
                    pq.at[q][rq, cs] = pq[q, rq, cs] * jnp.concatenate([gate16(rc[q, rq, :])] * 4, axis=1)
                    yield
            for ct in range(2):
                def put(k1, k2, v):
                    dst.at[k1 * 7 + k2][p2, ct * 128:(ct + 1) * 128] = v
                yield from form_steps(
                    _lform, lambda q, u: pq[q, rq, u * 256 + ct * 128:u * 256 + (ct + 1) * 128], put, tok)

    hist = []

    def g_lhs(k):
        v = ps[:, k * 128:(k + 1) * 128]
        hist.append(fwd[0])
        if GLAG and len(hist) > GLAG and hist[-1 - GLAG] is not None:
            cur = fwd[0]
            fwd[0] = hist[-1 - GLAG]
            v = jnp.concatenate([gate(v[i * 64:(i + 1) * 64]) for i in range(4)], axis=0)
            fwd[0] = cur
        return _unpack(v)

    def g_kvm(j):
        blk = yield from strassen2(
            lambda k1, k2: g_lhs(k1 * 7 + k2),
            lambda k1, k2: xs[R_ORD[k1] * 9 + R_ORD[k2]], TN, 256, 2)
        hm = (lax.broadcasted_iota(i32, (128, 128), 0) // 32
              == lax.broadcasted_iota(i32, (128, 128), 1) // 32)
        qb = q_rows(j, BQ - QB, QB, pqb_buf.at[j], denb_buf.at[j], 0, False)
        for _ in range(QSPLIT):
            next(qb)
        kvps = []
        for a in (3, 2, 1, 0):
            gg = jnp.concatenate(blk[a], axis=1).astype(bf16)
            clock[0] += 256
            kv = jnp.where(hm, _dot(gg, wv_buf[j, :, a * 128:(a + 1) * 128], NN), 0.0)
            tscr2.at[a][...] = _pack(kv)
            kvps.append(_unpack(jnp.concatenate(
                [tscr2[a, pl.ds(jj, 8, stride=8), :] for jj in range(8)], axis=0)))
        mg = mg_buf

        def m_form(tok):
            for a in (3, 2, 1, 0):
                for jl in range(2):
                    for ct in range(2):
                        def put(k1, k2, v):
                            ms.at[k1 * 7 + k2][pl.ds(_mo(jl * 64 + (2 * a + j) * 8, 8), 8),
                                               ct * 128:(ct + 1) * 128] = v
                        yield from form_steps(
                            _rform, lambda q, u: mg[a, (2 * q + jl) * 16:(2 * q + jl + 1) * 16,
                                                    u * 256 + ct * 128:u * 256 + (ct + 1) * 128], put)

        for i, a in enumerate((3, 2, 1, 0)):
            wo_u = pltpu.bitcast(wo_buf[j, a * 128:(a + 1) * 128, :], u32)
            res = mm(kvps[i], wo_u, NN, 256)
            mg.at[a][...] = res
            if i == 0:
                add_side(m_form, 112, 128, 768 + (49 - QSPLIT) * QB - 100)
        for _ in qb:
            pass

    def out_part(p0, nr, y, src, pr0):
        pr = pl.ds(_mo(pr0, 8), nr // 2)
        rows = [pl.ds(_mo(q * HQ + p0, 16), nr) for q in range(4)]
        row = lax.broadcasted_iota(i32, (nr, 256), 0) + p0
        blk = yield from strassen2(lambda k1, k2: _unpack(src[k1 * 7 + k2, pr, :]),
                                   lambda k1, k2: ms[k1 * 7 + k2], NN, nr)
        for s1 in (3, 2, 1, 0):
            for s2 in range(4):
                q = (s1 // 2) * 2 + s2 // 2
                u = (s1 % 2) * 2 + s2 % 2
                rr, cc = rows[q], pl.ds(u * 256, 256)
                a = jnp.concatenate([sa[rr, :]] * 2, axis=1)
                b = jnp.concatenate([sb[rr, :]] * 2, axis=1)
                o = blk[q][u] + jnp.where(row + q * HQ == idx_s[0], y[:, u * 256:(u + 1) * 256], 0.0)
                out_buf[rr, cc] = (x_buf[rr, cc].astype(f32) * a - b + o).astype(bf16)
                if s2 % 2 == 1:
                    ch = pl.ds((s1 % 2) * HD, HD)
                    cp(out_buf.at[rr, ch], out_hbm.at[0, rr, ch], SEM_O).start()

    def ffn_part(j, f_lo, f_hi):
        for f0 in range(f_lo, f_hi, 256):
            fs = slice(f0, f0 + 256)
            ag = jnp.zeros((8, 256), f32)
            au = jnp.zeros((8, 256), f32)
            for kg in range(D // 8):
                xv = jnp.concatenate([gate(xb[8 * kg:8 * kg + 8, :])] * 2, axis=1)
                ag = ag + wg_buf[j, 8 * kg:8 * kg + 8, fs].astype(f32) * xv
                au = au + wu_buf[j, 8 * kg:8 * kg + 8, fs].astype(f32) * xv
                if kg % FSTEP == FSTEP - 1:
                    yield
            g = _rbf(jnp.sum(ag, axis=0, keepdims=True))
            u = _rbf(jnp.sum(au, axis=0, keepdims=True))
            h = _rbf(_rbf(g * jax.nn.sigmoid(g)) * u)
            hb_buf[fs, :] = jnp.broadcast_to(h, (128, 256)).T
        for d0 in range(0, D, 512):
            ds_ = slice(d0, d0 + 512)
            acc = yacc[:, ds_]
            for kg in range(f_lo // 8, f_hi // 8):
                hv = jnp.concatenate([gate(hb_buf[8 * kg:8 * kg + 8, :])] * 4, axis=1)
                acc = acc + wd_buf[j, 8 * kg:8 * kg + 8, ds_].astype(f32) * hv
                if kg % FSTEP == FSTEP - 1:
                    yield
            yacc[:, ds_] = acc

    def wait_group(i):
        with _scope("a_wait%d" % i):
            for c in a_groups[i]:
                c.wait()

    def run_all(gen):
        for _ in gen:
            pass

    def ln_side(r0, n, t0, t1):
        add_side(lambda tok: ln_rows(r0, n, tok), 22 * n // 16, t0, t1, SLAG)

    def l2_side(base, n, t0, t1):
        def gen(tok):
            for r in range(0, n, 16):
                yield from xs_form(r, tok, "l2", base)
        add_side(gen, 14 * n // 16, t0, t1)

    a_groups = make_a_groups()
    with _scope("p0_issue"):
        cp_wr.start()
        for grp in a_groups:
            for c in grp:
                c.start()
        for j in range(2):
            for part in range(2):
                for c in cp_b(j, part):
                    c.start()
        zacc[...] = jnp.zeros(zacc.shape, f32)
        zero_buf[1] = jnp.zeros((8, 128), u32)
        cp_zero = cp(zero_buf.at[1], zero_buf.at[0], SEM_Z)
        cp_zero.start()
        cp_zero.wait()
        cp_wr.wait()
        z0 = jnp.max(pltpu.bitcast(zero_buf[0], i32))
        ps, pq_buf, den_buf, mg_buf, hb_buf = [r.at[z0] for r in (ps_raw, pq_raw, den_raw, mg_raw, hb_raw)]
        xn_buf = mg_buf

    def a01(i, carry):
        with _scope("a_wait01"):
            for c in cp_x(i * 64, 64, SEM_A + i):
                c.wait()
        with _scope("a01"):
            run_all(ln_rows(0, 64, None, "l1", i * 64))
        return carry

    lax.fori_loop(0, 2, a01, 0)

    def a23(i, carry):
        with _scope("a_wait23"):
            for c in cp_wk(i, SEM_A + 2 + i):
                c.wait()
        with _scope("a23"):
            run_all(wk_prep(i))
            l2_side(i * 64, 64, 300, 1500)
            kproj(0, 128, [(0, i)])
            finish()
        return carry

    lax.fori_loop(0, 2, a23, 0)
    wait_group(4)
    with _scope("a4"):
        run_all(wk_prep(2))
        ln_side(128, 32, 0, 1500)
        kproj(0, 128, [(1, 0)])
        finish()
    wait_group(5)
    with _scope("a5"):
        run_all(wk_prep(3))
        ln_side(160, 32, 0, 1400)
        kproj(0, 128, [(1, 1)])
        for r0 in (128, 192):
            ln_side(r0 + 64, 64, 0, 3200)
            kproj(r0, 64)
        finish()
    wait_group(6)
    with _scope("a6"):
        ln_side(320, 192, 0, A6[0])
        add_side(wq_perm, 128, A6[1], A6[2], A6[6])
        add_side(wq_form, 224, A6[3], A6[4], A6[6])
        add_side(route, 17, A6[5], A6[5] + 800)
        for r0 in (256, 320, 384, 448):
            kproj(r0, 64)
        finish()

    def b_body(j, carry):
        qa = BQ - QB
        with _scope("b_wait0"):
            for c in cp_b(j, 0, wait_only=True):
                c.wait()
        with _scope("b_r0"):
            z_prep()
            t1 = 49 * qa - 400
            add_side(lambda tok: ps_form(j, None), 7 * HQ // 16, 0, t1)
            add_side(lambda tok: ffn_part(j, 0, F1), F1 * 3 // (4 * FSTEP), 0, t1)
            for r0 in range(0, qa, QN):
                run_all(q_rows(j, r0, min(QN, qa - r0), pq_buf, den_buf, r0, r0 + QN < qa))
            finish()
        with _scope("b_wait1"):
            for c in cp_b(j, 1, wait_only=True):
                c.wait()
        with _scope("b_r1"):
            add_side(lambda tok: ffn_part(j, F1, FH), (FH - F1) * 3 // (4 * FSTEP), 0, 12800)
            add_side(lambda tok: normalise(pq_buf, den_buf, qa, qs, j * (qa // 2),
                                           lambda r: (r // QN + 1) * QN >= qa), 22 * (qa // 16), 0, 12800)
            run_all(g_kvm(j))
            finish()
        return carry

    lax.fori_loop(0, 2, b_body, 0)

    def c_body(t, carry):
        with _scope("c_body"):
            y = _rbf(jnp.sum(yacc[...], axis=0, keepdims=True))
            y = _rbf(y * _rbf(jax.nn.sigmoid(rsel[0:1, :])))
            j, h = t >> 1, t & 1
            na, nb = (BQ - QB) // 2, QB // 2
            hb = pl.ds(_mo(h * nb, 16), nb)
            add_side(lambda tok: normalise(pqb_buf.at[j, :, hb, :], denb_buf.at[j, :, hb, :], nb, qsb, 0,
                                           lambda r: True, tok),
                     4 + 22 * (nb // 16), 0, 49 * na - 800, SLAG)
            for p in range(0, na, CR):
                p0 = j * BQ + h * na + p
                run_all(out_part(p0, min(CR, na - p), y, qs, t * (na // 2) + p // 2))
            run_all(out_part(j * BQ + BQ - QB + h * nb, nb, y, qsb, 0))
            finish()
        return carry

    lax.fori_loop(0, 4, c_body, 0)
    with _scope("tail"):
        cp(out_buf, out_hbm.at[0], SEM_O).wait()


@jax.jit
def pallas_parallel_sum__linear_attn_block__moe_arch_mod__prompt_kernel(
    A_x: jax.Array,
    A_wqkv: jax.Array,
    A_wo: jax.Array,
    B_x: jax.Array,
    B_w_r: jax.Array,
    B_w_gate: jax.Array,
    B_w_up: jax.Array,
    B_w_down: jax.Array,
):
    del B_x
    V = pltpu.VMEM
    scratch = [
        V((S, D), bf16),
        V((2, D, 512), bf16),
        V((2, 512, D), bf16),
        V((8 * D,), bf16),
        V((2, D, FH), bf16),
        V((2, D, FH), bf16),
        V((2, FH, D), bf16),
        V((63, HQ // 2, 256), u32),
        V((49, 128, 256), u32),
        V((S, 128), f32),
        V((S, 128), f32),
        V((8, D), f32),
        V((8, D), f32),
        V((2, 4, HQ, 512), f32),
        V((D, 128), f32),
        V((8, D), f32),
        V((8, D), f32),
        V((4, 8, 128), u32),
        V((4, HD // 2, 7 * 128), u32),
        V((S, 128), f32),
        V((64, 64, 128), u32),
        V((1, HQ // 2, 49 * 128), u32),
        V((49, BQ - QB, 256), u32),
        V((49, 128, 256), u32),
        V((8, 64, 128), u32),
        V((4, 64, 128), u32),
        V((1, 4, BQ - QB, D), f32),
        V((1, 4, BQ - QB, 128), f32),
        V((2, 4, QB, D), f32),
        V((2, 4, QB, 128), f32),
        V((49, QB // 4, 256), u32),
        V((1, 4, 128, D), f32),
        V((1, FH, 128), f32),
        V((S, D), bf16),
        pltpu.SMEM((1,), i32),
        pltpu.SemaphoreType.DMA((13,)),
    ]
    return pl.pallas_call(
        _kernel,
        out_shape=jax.ShapeDtypeStruct((1, S, D), bf16),
        in_specs=[pl.BlockSpec(memory_space=pl.ANY)] * 7,
        out_specs=pl.BlockSpec(memory_space=pl.ANY),
        scratch_shapes=scratch,
        compiler_params=pltpu.CompilerParams(vmem_limit_bytes=VMEM_MB * 1024 * 1024,
                                             disable_bounds_checks=True,
                                             fuse_transposed_lhs_in_matmul=FUSE,
                                             disable_semaphore_checks=True),
    )(A_x, A_wqkv, A_wo, B_w_r, B_w_gate, B_w_up, B_w_down)
```

```python
import contextlib

import jax
import jax.numpy as jnp
from jax import lax
import jax.experimental.pallas as pl
import jax.experimental.pallas.tpu as pltpu

bf16, f32, u32, i32 = jnp.bfloat16, jnp.float32, jnp.uint32, jnp.int32

S = 2048
D = 1024
F = 3584
HP = S // 2
HD = D // 2
HQ = S // 4
BQ = HQ // 2
FH = F // 2
F1 = 256
QB = 64
QN = 48
QW = (20, 28, 28, 12, 8, 8, 8)
A6 = (7500, 7000, 10000, 9000, 13800, 10500, None)
LNTOK = 0
GLAG = 0
RECQ = True
FUSE = False
QSPLIT = 6
SLAG = 400
FSTEP = 2
CR = 32
XN = 128
VMEM_MB = 120
CT = 128

L_ORD = (2, 3, 0, 1, 4, 5, 6)
R_ORD = (2, 0, 6, 5, 1, 4, 3)

K_SEQ = (1, 4, 0, 2, 3, 5, 6)
K_SEQ2 = (0, 1, 2, 5, 3, 4, 6)

NN = (((1,), (0,)), ((), ()))
NT_ = (((1,), (1,)), ((), ()))
TN = (((0,), (0,)), ((), ()))


SCOPES = False


def _scope(name):
    return jax.named_scope(name) if SCOPES else contextlib.nullcontext()


def _mo(v, m):
    return v if isinstance(v, int) else pl.multiple_of(v, m)


def _dot(a, b, dims):
    return lax.dot_general(a, b, dims, preferred_element_type=f32)


def _pack(v):
    return pltpu.bitcast(v.astype(bf16), u32)


def _unpack(v):
    return pltpu.bitcast(v, bf16)


def _combine(m):
    m1, m2, m3, m4, m5, m6, m7 = m
    return m1 + m4 - m5 + m7, m3 + m5, m2 + m4, m1 - m2 + m3 + m6


def _lform(a11, a12, a21, a22):
    return (a11 + a22, a21 + a22, a11, a22, a11 + a12, a21 - a11, a12 - a22)


def _rform(b11, b12, b21, b22):
    return (b11 + b22, b11, b12 - b22, b21 - b11, b22, b11 + b12, b21 + b22)


def _sform(x11, x12, x21, x22):
    return (x11, x22, x11 + x22, x21 + x22, x11 + x12, x21 - x11, x12 - x22)


class _Sym:
    def __init__(self, t):
        self.t = t

    def __add__(self, o):
        return _Sym({**self.t, **o.t})

    def __sub__(self, o):
        return _Sym({**self.t, **{k: -v for k, v in o.t.items()}})


def _phi(t):
    return jnp.where(t > 0, t + 1.0, jnp.exp(t)) + 1e-6


def _rbf(v):
    return v.astype(bf16).astype(f32)


def _layernorm_rows(xv):
    mf = jnp.sum(xv, axis=1, keepdims=True) * (1.0 / D)
    mb = _rbf(mf)
    d = xv - mb
    dm = mf - mb
    var = jnp.sum(d * d, axis=1, keepdims=True) * (1.0 / D) - dm * dm
    var = jnp.maximum(var, 0.0)
    sd = _rbf(jnp.sqrt(_rbf(_rbf(var) + 1e-5)))
    return d * (1.0 / sd)


def _kernel(x_hbm, wqkv_hbm, wo_hbm, wr_hbm, wg_hbm, wu_hbm, wd_hbm, out_hbm,
            x_buf, wv_buf, wo_buf, wr_buf, wg_buf, wu_buf, wd_buf,
            xs1, xs2, wqs, sa, sb, zacc, zp, pk_buf, xb, yacc, rsel, zero_buf,
            wks, stats, wqt, ps_raw, qs, ms, tscr, tscr2, pq_raw, den_raw, pqb_buf, denb_buf, qsb,
            mg_raw, hb_raw, out_buf, idx_s, sem):
    wq_buf = out_buf.at[pl.ds(0, D), :]
    wk_buf = out_buf.at[pl.ds(D, D), :]

    def xs_at(k1, e, rows=None):
        r = xs1.at[k1 * 4 + (0, 1, 7, 8).index(e)] if e in (0, 1, 7, 8) else xs2.at[k1 * 5 + e - 2]
        return r if rows is None else r.at[rows, :]

    SEM_B, SEM_O, SEM_Z, SEM_A = 0, 4, 5, 6

    def cp(src, dst, s):
        return pltpu.make_async_copy(src, dst, sem.at[s])

    def cp_x(r0, n, s):
        rows = [pl.ds(_mo(q * HQ + r0, 16), n) for q in range(4)]
        return [cp(x_hbm.at[0, r, :], x_buf.at[r, :], s) for r in rows]

    def cp_wk(c, s):
        return [cp(wqkv_hbm.at[:, pl.ds(_mo(D + h * HD + c * 128, 128), 128)],
                   wk_buf.at[:, pl.ds(_mo(c * 256 + h * 128, 128), 128)], s) for h in range(2)]

    cp_wr = cp(wr_hbm, wr_buf.at[pl.ds(0, D)], SEM_Z)

    def make_a_groups():
        return [
            cp_x(0, 64, SEM_A),
            cp_x(64, 64, SEM_A + 1),
            cp_wk(0, SEM_A + 2),
            cp_wk(1, SEM_A + 3),
            cp_wk(2, SEM_A + 4) + cp_x(128, 64, SEM_A + 4),
            cp_wk(3, SEM_A + 5) + cp_x(192, 128, SEM_A + 5),
            cp_x(320, 192, SEM_A + 6) + [cp(wqkv_hbm.at[:, pl.ds(0, D)], wq_buf, SEM_A + 6)],
        ]

    def cp_b(j, part, wait_only=False):
        pairs = []
        f0, fw = (0, F1) if part == 0 else (F1, FH - F1)
        fs = pl.ds(_mo(j * FH + f0, 128), fw)
        pairs += [(wg_hbm.at[:, fs], wg_buf.at[j, :, pl.ds(f0, fw)]),
                  (wu_hbm.at[:, fs], wu_buf.at[j, :, pl.ds(f0, fw)]),
                  (wd_hbm.at[fs, :], wd_buf.at[j, pl.ds(f0, fw), :])]
        if part == 1:
            for a in range(4):
                c0 = _mo((2 * a + j) * 128, 128)
                pairs += [(wqkv_hbm.at[:, pl.ds(2 * D + c0, 128)], wv_buf.at[j, :, pl.ds(a * 128, 128)]),
                          (wo_hbm.at[pl.ds(c0, 128), :], wo_buf.at[j, pl.ds(a * 128, 128), :])]
        return [cp(dst if wait_only else src, dst, SEM_B + 2 * j + part) for src, dst in pairs]

    clock = [0]
    toks = []
    sides = []
    fwd = [None]

    def emit_tok(vals, stamp=None):
        t = None
        for v in vals:
            v = pltpu.bitcast(v, u32) if v.dtype != u32 else v
            t = v if t is None else t | v
        toks.append((clock[0] if stamp is None else stamp, t & zero_buf[0]))

    def gate(v):
        if fwd[0] is None:
            return v
        if fwd[0][1] is None:
            fwd[0][1] = pltpu.bitcast(fwd[0][0](), u32) & zero_buf[0]
        head = pltpu.bitcast(pltpu.bitcast(v[0:8], u32) | fwd[0][1], v.dtype)
        return head if v.shape[0] == 8 else jnp.concatenate([head, v[8:]], axis=0)

    def add_side(gen_fn, n, t0, t1, lag=None):
        st = {"i": 0, "n": n, "t0": clock[0] + t0, "t1": clock[0] + t1}

        def tok(vals):
            if lag is not None:
                emit_tok(vals, st["t0"] + (st["i"] + 1) * (st["t1"] - st["t0"]) // st["n"] + lag)
        st["g"] = gen_fn(tok)
        sides.append(st)

    def advance(until):
        for st in sides:
            while st["i"] < st["n"] and st["t0"] + st["i"] * (st["t1"] - st["t0"]) // st["n"] < until:
                next(st["g"], None)
                st["i"] += 1

    def finish():
        for st in sides:
            for _ in st["g"]:
                pass
        sides.clear()
        toks.clear()
        fwd[0] = None

    def mm(lhs, rhs, dims, cycles, nseg=1):
        due = [t for (c, t) in toks if c <= clock[0]]
        toks[:] = [(c, t) for (c, t) in toks if c > clock[0]]
        if due:
            head = rhs[0:8, 0:128]
            for t in due:
                head = head | t
            if rhs.shape[1] > 128:
                head = jnp.concatenate([head, rhs[0:8, 128:]], axis=1)
            rhs = jnp.concatenate([head, rhs[8:]], axis=0)
        res = _dot(lhs, _unpack(rhs), dims)
        ngr = res.shape[0] // 16
        for sg in range(nseg):
            for i in range(ngr):
                fwd[0] = [lambda sg=sg, i=i: res[i * 16:i * 16 + 8, sg * 128:(sg + 1) * 128], None]
                clock[0] += cycles // nseg // ngr
                advance(clock[0])
        return res

    def gate16(v):
        return jnp.concatenate([gate(v[0:8]), gate(v[8:16])], axis=0)

    def form_steps(form, get, put, tok=None, inner=None, gated=False):
        terms = form(*[_Sym({i: 1}) for i in range(4)])
        for k1 in range(7):
            sub = []
            for r in range(2):
                for c in range(2):
                    v = None
                    for i, sg in sorted(terms[k1].t.items(), key=lambda e: -e[1]):
                        b = get(r + 2 * (i // 2), c + 2 * (i % 2))
                        if v is None:
                            v = gate16(b) if r == c and not gated else b
                        else:
                            v = v + b if sg > 0 else v - b
                    sub.append(v)
            vals = []
            for k2, v in (enumerate(form(*sub)) if inner is None else inner(sub)):
                vals.append(v)
                put(k1, k2, _pack(v))
            if tok is not None:
                tok([v[o:o + 8] for v in vals[-2:] for o in (0, 8)])
            yield

    def strassen2(lhs, rhs, dims, cycles, nseg=1, wts=(16,) * 7):
        m1 = [None] * 7
        for i1, k1 in enumerate(K_SEQ2):
            m2 = [None] * 7
            for k2 in K_SEQ2:
                m2[k2] = mm(lhs(k1, k2), rhs(k1, k2), dims, cycles * wts[i1] // 16, nseg)
                yield
            m1[k1] = _combine(m2)
        out = [[None] * 4 for _ in range(4)]
        for s2 in range(4):
            for s1, v in enumerate(_combine([m1[k1][s2] for k1 in range(7)])):
                out[(s1 // 2) * 2 + s2 // 2][(s1 % 2) * 2 + s2 % 2] = v
        return out

    def row_views(base):
        if isinstance(base, int) and base == 0:
            return x_buf, sa, sb, stats, xn_buf, None
        b = _mo(base, 64)
        return ([r.at[pl.ds(b, S - 64), :] for r in (x_buf, sa, sb, stats)]
                + [xn_buf.at[:, pl.ds(b, 64), :], pl.ds(_mo(base // 2, 32), 32)])

    def xs_form(r0, tok, which="all", base=0):
        xn_v, xs_v = row_views(base)[4:]
        rows = slice(r0 % XN, r0 % XN + 16)

        def inner(sub):
            full = list(enumerate(_sform(*sub))) + [(7, sub[1]), (8, sub[2])]
            return [full[e] for e in {"all": (0, 1, 7, 8, 2, 5, 6, 3, 4), "l1": (0, 1, 7, 8),
                                      "l2": (2, 5, 6, 3, 4)}[which]]
        for ct in range(2):
            def put(k1, k2, v):
                xs_at(k1, k2, xs_v)[r0 // 2:r0 // 2 + 8, ct * 128:(ct + 1) * 128] = v
            yield from form_steps(
                _sform, lambda q, u: xn_v[q, rows, u * 256 + ct * 128:u * 256 + (ct + 1) * 128],
                put, tok, inner)

    def ln_rows(r_start, n_rows, tok, which="all", base=0):
        x_v, sa_v, sb_v, st_v, xn_v, _ = row_views(base)
        wr = wr_buf[0:D].reshape(1, D).astype(f32)
        lane = lax.broadcasted_iota(i32, (8, 128), 1)
        for c in range(n_rows // 16 + 1):
            r0 = r_start + c * 16
            form = xs_form(r0 - 16, tok, which, base) if c > 0 else iter(())
            for g in range(8 if c < n_rows // 16 else 0):
                q, o = g // 2, (g % 2) * 8
                rg = q * HQ + r0 + o
                xv = x_v[rg:rg + 8, :].astype(f32)
                xg = jnp.concatenate([gate(xv[:, 0:128]), xv[:, 128:]], axis=1)
                mf = jnp.sum(xg, axis=1, keepdims=True) * (1.0 / D)
                d = xv - mf
                var = jnp.sum(d * d, axis=1, keepdims=True) * (1.0 / D)
                tr = jnp.sum(d * wr, axis=1, keepdims=True)
                rs = lax.rsqrt(var + 1e-5)
                xn = d * rs
                xn_v.at[q][r0 % XN + o:r0 % XN + o + 8, :] = xn
                rs = jnp.broadcast_to(rs, (8, 128))
                mf = jnp.broadcast_to(mf, (8, 128))
                sa_v[rg:rg + 8, :] = 1.0 + rs
                sb_v[rg:rg + 8, :] = mf * rs
                st = jnp.where(lane == 0, mf, jnp.where(lane == 1, jnp.broadcast_to(var, (8, 128)),
                                                        jnp.broadcast_to(tr, (8, 128))))
                st_v[rg:rg + 8, :] = st
                if tok is not None and LNTOK:
                    tok([rs, st][:LNTOK])
                yield
                if g >= 2 and c > 0:
                    for _ in range(2):
                        next(form)
                        yield
            yield from form

    def wk_prep(c, tok=None):
        cs = pl.ds(_mo(c * 256, 256), 256)
        for i in range(HD // 16):
            r0 = i * 16
            top = wk_buf[r0:r0 + 16, cs].astype(f32)
            bot = wk_buf[HD + r0:HD + r0 + 16, cs].astype(f32)
            ops = _rform(gate(top[:, :128]), top[:, 128:], bot[:, :128], gate(bot[:, 128:]))
            for k in range(7):
                wks.at[c][r0 // 2:r0 // 2 + 8, k * 128:(k + 1) * 128] = _pack(ops[k])
            yield

    def wq_perm(tok):
        def permute(kt):
            for g in range(8):
                tile = gate(pltpu.bitcast(wq_buf[kt * 128:(kt + 1) * 128, g * 128:(g + 1) * 128], u32))
                wqt.at[kt * 8 + g][...] = pltpu.bitcast(_unpack(tile).T, u32)
                yield

        def back(kt):
            for j in range(8):
                tile = gate(jnp.concatenate([wqt[kt * 8 + g, pl.ds(j, 8, stride=8), :] for g in range(8)],
                                            axis=0))
                v = pltpu.bitcast(_unpack(tile).T, u32)
                ps[(kt % 4) * 64:(kt % 4 + 1) * 64, (kt // 4) * D + j * 128:(kt // 4) * D + (j + 1) * 128] = v
                tok([v[56:64]])
                yield

        order = (0, 2, 4, 6, 1, 3, 5, 7)
        for n in range(10):
            if n < 8:
                yield from permute(order[n])
            if n > 1:
                yield from back(order[n - 2])

    def wq_form(tok):
        for i in range(16):
            for ct in range(2):
                def put(k1, k2, v):
                    wqs.at[k1 * 7 + k2][i * 8:(i + 1) * 8, ct * 128:(ct + 1) * 128] = v
                yield from form_steps(
                    _rform, lambda r, c: _unpack(gate(
                        ps[(r % 2) * 128 + i * 8:(r % 2) * 128 + (i + 1) * 8,
                           (r // 2) * D + c * 256 + ct * 128:(r // 2) * D + c * 256 + (ct + 1) * 128]
                    )).astype(f32), put, tok,
                    gated=True)

    def kproj(r0, n, chunks=((0, 0), (0, 1), (1, 0), (1, 1))):
        pr = pl.ds(r0 // 2, n // 2)
        for ch, ct in chunks:
            c = 2 * ch + ct
            m = [None] * 7
            for k in K_SEQ:
                e11, e22, e12, e21 = [xs_at(L_ORD[k], e)[pr, :] for e in (0, 1, 7, 8)]
                lhs = jnp.concatenate([jnp.concatenate([e11, e12], axis=1),
                                       jnp.concatenate([e21, e22], axis=1)], axis=0)
                m[k] = mm(_unpack(lhs), wks[c, :, k * 128:(k + 1) * 128], NN, 2 * n)
            kk = [_phi(v) for v in _combine(m)]
            for h in range(2):
                zacc[:, pl.ds(_mo(h * HD + c * 128, 128), 128)] += (
                    (kk[h] + kk[2 + h]).reshape(n // 4, 8, 128).sum(axis=0))
            for s1 in range(4):
                u = (s1 % 2) * 2 + ch
                for h in range(2):
                    pk_buf.at[ct, (s1 // 2) * 2 + h][r0:r0 + n, u * 128:(u + 1) * 128] = (
                        kk[s1][h * n:(h + 1) * n])

    def z_prep():
        z = jnp.sum(zacc[...], axis=0, keepdims=True)
        zt = _pack(jnp.broadcast_to(z, (128, D)).astype(bf16).T)
        for g in range(8):
            tscr.at[g][...] = zt[g * 64:(g + 1) * 64, :]
        for j in range(8):
            blk = jnp.concatenate([tscr[g, pl.ds(j, 8, stride=8), :] for g in range(8)], axis=0)
            zp[:, j * 128:(j + 1) * 128] = _unpack(blk).T[0:8, :].astype(f32)

    def route(tok):
        rows = []
        for b in range(S // 128):
            rows.append(gate(stats[b * 128:(b + 1) * 128, :]).T[0:8, :])
            yield
        mf = jnp.concatenate([v[0:1] for v in rows], axis=0)
        var = jnp.concatenate([v[1:2] for v in rows], axis=0)
        tr = jnp.concatenate([v[2:3] for v in rows], axis=0)
        wsum = jnp.sum(wr_buf[0:D].reshape(1, D).astype(f32), axis=1, keepdims=True)
        sd = _rbf(jnp.sqrt(_rbf(_rbf(var) + 1e-5)))
        rv = _rbf((tr + (mf - _rbf(mf)) * wsum) / sd)
        rmax = jnp.max(rv)
        pos = (lax.broadcasted_iota(i32, rv.shape, 0) * 128 + lax.broadcasted_iota(i32, rv.shape, 1))
        idx = jnp.min(jnp.where(rv == rmax, pos, S - 1))
        idx_s[0] = idx
        rsel[...] = jnp.full(rsel.shape, rmax, f32)
        b0 = _mo((idx // 16) * 16, 16)
        xn = _rbf(_layernorm_rows(x_buf[pl.ds(b0, 16), :].astype(f32)))
        sel = lax.broadcasted_iota(i32, xn.shape, 0) == idx - b0
        row = jnp.sum(jnp.where(sel, xn, 0.0), axis=0, keepdims=True)
        xbv = jnp.broadcast_to(row, (128, D)).T
        xb[...] = xbv
        yacc[...] = jnp.zeros(yacc.shape, f32)
        tok([xbv[b * 128 + 120:(b + 1) * 128] for b in range(8)])
        yield

    def ps_form(j, tok):
        for c in range(HQ // 16):
            def put(k1, k2, v):
                k = k1 * 7 + k2
                ps[c * 8:(c + 1) * 8, k * 128:(k + 1) * 128] = v
            yield from form_steps(
                _lform, lambda r, q: pk_buf[j, q, c * 16:(c + 1) * 16, r * 128:(r + 1) * 128], put, tok)

    def q_rows(j, r0, n, pq, rc, d0, rec):
        xj = pl.ds(_mo(j * (BQ // 2), BQ // 2), BQ // 2)
        pr = slice(r0 // 2, (r0 + n) // 2)
        blk = yield from strassen2(lambda k1, k2: _unpack(xs_at(L_ORD[k1], L_ORD[k2], xj)[pr, :]),
                                   lambda k1, k2: wqs[k1 * 7 + k2], NN, n, 1, QW)
        lane = lax.broadcasted_iota(i32, (n, 128), 1)
        for q in range(4):
            d = None
            for u in (3, 2, 1, 0):
                v = _phi(blk[q][u])
                pq.at[q][d0:d0 + n, u * 256:(u + 1) * 256] = v
                t = v * zp[0:1, u * 256:(u + 1) * 256]
                t = t[:, :128] + t[:, 128:]
                d = t if d is None else d + t
            if rec:
                d = recip(d, lane)
            rc.at[q][d0:d0 + n, :] = d

    def recip(d, lane):
        d = d + jnp.where(lane % 2 == 0, pltpu.roll(d, 127, 1), pltpu.roll(d, 1, 1))
        d = d + jnp.where(lane % 4 < 2, pltpu.roll(d, 126, 1), pltpu.roll(d, 2, 1))
        return 1.0 / (d + 1e-6)

    def normalise(pq, rc, nr, dst, p0, raw, tok=None):
        lane = lax.broadcasted_iota(i32, (16, 128), 1)

        def fix(c):
            if c < nr // 16 and raw(c * 16):
                for q in range(4):
                    rq = slice(c * 16, (c + 1) * 16)
                    rc.at[q][rq, :] = recip(gate16(rc[q, rq, :]), lane)

        fix(0)
        if raw(0):
            for _ in range(4):
                yield
        for c in range(nr // 16):
            rq = slice(c * 16, (c + 1) * 16)
            p2 = pl.ds(_mo(p0 + c * 8, 8), 8)
            fix(c + 1)
            for q in range(4):
                for hf in range(2):
                    cs = slice(hf * HD, (hf + 1) * HD)
                    pq.at[q][rq, cs] = pq[q, rq, cs] * jnp.concatenate([gate16(rc[q, rq, :])] * 4, axis=1)
                    yield
            for ct in range(2):
                def put(k1, k2, v):
                    dst.at[k1 * 7 + k2][p2, ct * 128:(ct + 1) * 128] = v
                yield from form_steps(
                    _lform, lambda q, u: pq[q, rq, u * 256 + ct * 128:u * 256 + (ct + 1) * 128], put, tok)

    hist = []

    def g_lhs(k):
        v = ps[:, k * 128:(k + 1) * 128]
        hist.append(fwd[0])
        if GLAG and len(hist) > GLAG and hist[-1 - GLAG] is not None:
            cur = fwd[0]
            fwd[0] = hist[-1 - GLAG]
            v = jnp.concatenate([gate(v[i * 64:(i + 1) * 64]) for i in range(4)], axis=0)
            fwd[0] = cur
        return _unpack(v)

    def g_kvm(j):
        blk = yield from strassen2(
            lambda k1, k2: g_lhs(k1 * 7 + k2),
            lambda k1, k2: xs_at(R_ORD[k1], R_ORD[k2])[...], TN, 256, 2)
        hm = (lax.broadcasted_iota(i32, (128, 128), 0) // 32
              == lax.broadcasted_iota(i32, (128, 128), 1) // 32)
        qb = q_rows(j, BQ - QB, QB, pqb_buf.at[j], denb_buf.at[j], 0, False)
        for _ in range(QSPLIT):
            next(qb)
        kvps = []
        for a in (3, 2, 1, 0):
            gg = jnp.concatenate(blk[a], axis=1).astype(bf16)
            clock[0] += 256
            kv = jnp.where(hm, _dot(gg, wv_buf[j, :, a * 128:(a + 1) * 128], NN), 0.0)
            tscr2.at[a][...] = _pack(kv)
            kvps.append(_unpack(jnp.concatenate(
                [tscr2[a, pl.ds(jj, 8, stride=8), :] for jj in range(8)], axis=0)))
        mg = mg_buf

        def m_form(tok):
            for a in (3, 2, 1, 0):
                for jl in range(2):
                    for ct in range(2):
                        def put(k1, k2, v):
                            ms.at[k1 * 7 + k2][pl.ds(_mo(jl * 64 + (2 * a + j) * 8, 8), 8),
                                               ct * 128:(ct + 1) * 128] = v
                        yield from form_steps(
                            _rform, lambda q, u: mg[a, (2 * q + jl) * 16:(2 * q + jl + 1) * 16,
                                                    u * 256 + ct * 128:u * 256 + (ct + 1) * 128], put)

        for i, a in enumerate((3, 2, 1, 0)):
            wo_u = pltpu.bitcast(wo_buf[j, a * 128:(a + 1) * 128, :], u32)
            res = mm(kvps[i], wo_u, NN, 256)
            mg.at[a][...] = res
            if i == 0:
                add_side(m_form, 112, 128, 768 + (49 - QSPLIT) * QB - 100)
        for _ in qb:
            pass

    def out_part(p0, nr, y, src, pr0):
        pr = pl.ds(_mo(pr0, 8), nr // 2)
        rows = [pl.ds(_mo(q * HQ + p0, 16), nr) for q in range(4)]
        row = lax.broadcasted_iota(i32, (nr, 256), 0) + p0
        blk = yield from strassen2(lambda k1, k2: _unpack(src[k1 * 7 + k2, pr, :]),
                                   lambda k1, k2: ms[k1 * 7 + k2], NN, nr)
        for s1 in (3, 2, 1, 0):
            for s2 in range(4):
                q = (s1 // 2) * 2 + s2 // 2
                u = (s1 % 2) * 2 + s2 % 2
                rr, cc = rows[q], pl.ds(u * 256, 256)
                a = jnp.concatenate([sa[rr, :]] * 2, axis=1)
                b = jnp.concatenate([sb[rr, :]] * 2, axis=1)
                o = blk[q][u] + jnp.where(row + q * HQ == idx_s[0], y[:, u * 256:(u + 1) * 256], 0.0)
                out_buf[rr, cc] = (x_buf[rr, cc].astype(f32) * a - b + o).astype(bf16)
                if s2 % 2 == 1:
                    ch = pl.ds((s1 % 2) * HD, HD)
                    cp(out_buf.at[rr, ch], out_hbm.at[0, rr, ch], SEM_O).start()

    def ffn_part(j, f_lo, f_hi):
        for f0 in range(f_lo, f_hi, 256):
            fs = slice(f0, f0 + 256)
            ag = jnp.zeros((8, 256), f32)
            au = jnp.zeros((8, 256), f32)
            for kg in range(D // 8):
                xv = jnp.concatenate([gate(xb[8 * kg:8 * kg + 8, :])] * 2, axis=1)
                ag = ag + wg_buf[j, 8 * kg:8 * kg + 8, fs].astype(f32) * xv
                au = au + wu_buf[j, 8 * kg:8 * kg + 8, fs].astype(f32) * xv
                if kg % FSTEP == FSTEP - 1:
                    yield
            g = _rbf(jnp.sum(ag, axis=0, keepdims=True))
            u = _rbf(jnp.sum(au, axis=0, keepdims=True))
            h = _rbf(_rbf(g * jax.nn.sigmoid(g)) * u)
            hb_buf[fs, :] = jnp.broadcast_to(h, (128, 256)).T
        for d0 in range(0, D, 512):
            ds_ = slice(d0, d0 + 512)
            acc = yacc[:, ds_]
            for kg in range(f_lo // 8, f_hi // 8):
                hv = jnp.concatenate([gate(hb_buf[8 * kg:8 * kg + 8, :])] * 4, axis=1)
                acc = acc + wd_buf[j, 8 * kg:8 * kg + 8, ds_].astype(f32) * hv
                if kg % FSTEP == FSTEP - 1:
                    yield
            yacc[:, ds_] = acc

    def wait_group(i):
        with _scope("a_wait%d" % i):
            for c in a_groups[i]:
                c.wait()

    def run_all(gen):
        for _ in gen:
            pass

    def ln_side(r0, n, t0, t1):
        add_side(lambda tok: ln_rows(r0, n, tok), 22 * n // 16, t0, t1, SLAG)

    def l2_side(base, n, t0, t1):
        def gen(tok):
            for r in range(0, n, 16):
                yield from xs_form(r, tok, "l2", base)
        add_side(gen, 14 * n // 16, t0, t1)

    a_groups = make_a_groups()
    with _scope("p0_issue"):
        cp_wr.start()
        for grp in a_groups:
            for c in grp:
                c.start()
        for j in range(2):
            for part in range(2):
                for c in cp_b(j, part):
                    c.start()
        zacc[...] = jnp.zeros(zacc.shape, f32)
        zero_buf[1] = jnp.zeros((8, 128), u32)
        cp_zero = cp(zero_buf.at[1], zero_buf.at[0], SEM_Z)
        cp_zero.start()
        cp_zero.wait()
        cp_wr.wait()
        z0 = jnp.max(pltpu.bitcast(zero_buf[0], i32))
        ps, pq_buf, den_buf, mg_buf, hb_buf = [r.at[z0] for r in (ps_raw, pq_raw, den_raw, mg_raw, hb_raw)]
        xn_buf = mg_buf

    def a01(i, carry):
        with _scope("a_wait01"):
            for c in cp_x(i * 64, 64, SEM_A + i):
                c.wait()
        with _scope("a01"):
            run_all(ln_rows(0, 64, None, "l1", i * 64))
        return carry

    lax.fori_loop(0, 2, a01, 0)

    def a23(i, carry):
        with _scope("a_wait23"):
            for c in cp_wk(i, SEM_A + 2 + i):
                c.wait()
        with _scope("a23"):
            run_all(wk_prep(i))
            l2_side(i * 64, 64, 300, 1500)
            kproj(0, 128, [(0, i)])
            finish()
        return carry

    lax.fori_loop(0, 2, a23, 0)
    wait_group(4)
    with _scope("a4"):
        run_all(wk_prep(2))
        ln_side(128, 32, 0, 1500)
        kproj(0, 128, [(1, 0)])
        finish()
    wait_group(5)
    with _scope("a5"):
        run_all(wk_prep(3))
        ln_side(160, 32, 0, 1400)
        kproj(0, 128, [(1, 1)])
        for r0 in (128, 192):
            ln_side(r0 + 64, 64, 0, 3200)
            kproj(r0, 64)
        finish()
    wait_group(6)
    with _scope("a6"):
        ln_side(320, 192, 0, A6[0])
        add_side(wq_perm, 128, A6[1], A6[2], A6[6])
        add_side(wq_form, 224, A6[3], A6[4], A6[6])
        add_side(route, 17, A6[5], A6[5] + 800)
        for r0 in (256, 320, 384, 448):
            kproj(r0, 64)
        finish()

    def b_body(j, carry):
        qa = BQ - QB
        with _scope("b_wait0"):
            for c in cp_b(j, 0, wait_only=True):
                c.wait()
        with _scope("b_r0"):
            z_prep()
            t1 = 49 * qa - 400
            add_side(lambda tok: ps_form(j, None), 7 * HQ // 16, 0, t1)
            add_side(lambda tok: ffn_part(j, 0, F1), F1 * 3 // (4 * FSTEP), 0, t1)
            for r0 in range(0, qa, QN):
                run_all(q_rows(j, r0, min(QN, qa - r0), pq_buf, den_buf, r0, r0 + QN < qa))
            finish()
        with _scope("b_wait1"):
            for c in cp_b(j, 1, wait_only=True):
                c.wait()
        with _scope("b_r1"):
            add_side(lambda tok: ffn_part(j, F1, FH), (FH - F1) * 3 // (4 * FSTEP), 0, 12800)
            add_side(lambda tok: normalise(pq_buf, den_buf, qa, qs, j * (qa // 2),
                                           lambda r: (r // QN + 1) * QN >= qa), 22 * (qa // 16), 0, 12800)
            run_all(g_kvm(j))
            finish()
        return carry

    lax.fori_loop(0, 2, b_body, 0)

    def c_body(t, carry):
        with _scope("c_body"):
            y = _rbf(jnp.sum(yacc[...], axis=0, keepdims=True))
            y = _rbf(y * _rbf(jax.nn.sigmoid(rsel[0:1, :])))
            j, h = t >> 1, t & 1
            na, nb = (BQ - QB) // 2, QB // 2
            hb = pl.ds(_mo(h * nb, 16), nb)
            add_side(lambda tok: normalise(pqb_buf.at[j, :, hb, :], denb_buf.at[j, :, hb, :], nb, qsb, 0,
                                           lambda r: True, tok),
                     4 + 22 * (nb // 16), 0, 49 * na - 800, SLAG)
            for p in range(0, na, CR):
                p0 = j * BQ + h * na + p
                run_all(out_part(p0, min(CR, na - p), y, qs, t * (na // 2) + p // 2))
            run_all(out_part(j * BQ + BQ - QB + h * nb, nb, y, qsb, 0))
            finish()
        return carry

    lax.fori_loop(0, 4, c_body, 0)
    with _scope("tail"):
        cp(out_buf, out_hbm.at[0], SEM_O).wait()


@jax.jit
def pallas_parallel_sum__linear_attn_block__moe_arch_mod__prompt_kernel(
    A_x: jax.Array,
    A_wqkv: jax.Array,
    A_wo: jax.Array,
    B_x: jax.Array,
    B_w_r: jax.Array,
    B_w_gate: jax.Array,
    B_w_up: jax.Array,
    B_w_down: jax.Array,
):
    del B_x
    V = pltpu.VMEM
    scratch = [
        V((S, D), bf16),
        V((2, D, 512), bf16),
        V((2, 512, D), bf16),
        V((8 * D,), bf16),
        V((2, D, FH), bf16),
        V((2, D, FH), bf16),
        V((2, FH, D), bf16),
        V((28, HQ // 2, 256), u32),
        V((35, HQ // 2, 256), u32),
        V((49, 128, 256), u32),
        V((S, 128), f32),
        V((S, 128), f32),
        V((8, D), f32),
        V((8, D), f32),
        V((2, 4, HQ, 512), f32),
        V((D, 128), f32),
        V((8, D), f32),
        V((8, D), f32),
        V((4, 8, 128), u32),
        V((4, HD // 2, 7 * 128), u32),
        V((S, 128), f32),
        V((64, 64, 128), u32),
        V((1, HQ // 2, 49 * 128), u32),
        V((49, BQ - QB, 256), u32),
        V((49, 128, 256), u32),
        V((8, 64, 128), u32),
        V((4, 64, 128), u32),
        V((1, 4, BQ - QB, D), f32),
        V((1, 4, BQ - QB, 128), f32),
        V((2, 4, QB, D), f32),
        V((2, 4, QB, 128), f32),
        V((49, QB // 4, 256), u32),
        V((1, 4, 128, D), f32),
        V((1, FH, 128), f32),
        V((S, D), bf16),
        pltpu.SMEM((1,), i32),
        pltpu.SemaphoreType.DMA((13,)),
    ]
    return pl.pallas_call(
        _kernel,
        out_shape=jax.ShapeDtypeStruct((1, S, D), bf16),
        in_specs=[pl.BlockSpec(memory_space=pl.ANY)] * 7,
        out_specs=pl.BlockSpec(memory_space=pl.ANY),
        scratch_shapes=scratch,
        compiler_params=pltpu.CompilerParams(vmem_limit_bytes=VMEM_MB * 1024 * 1024,
                                             disable_bounds_checks=True,
                                             fuse_transposed_lhs_in_matmul=FUSE,
                                             disable_semaphore_checks=True),
    )(A_x, A_wqkv, A_wo, B_w_r, B_w_gate, B_w_up, B_w_down)
```

```python
import contextlib

import jax
import jax.numpy as jnp
from jax import lax
import jax.experimental.pallas as pl
import jax.experimental.pallas.tpu as pltpu

bf16, f32, u32, i32 = jnp.bfloat16, jnp.float32, jnp.uint32, jnp.int32

S = 2048
D = 1024
F = 3584
HP = S // 2
HD = D // 2
HQ = S // 4
BQ = HQ // 2
FH = F // 2
F1 = 256
QB = 64
QN = 48
QW = (20, 28, 28, 12, 8, 8, 8)
A6 = (8500, 8000, 10800, 9800, 13900, 11300, None)
TOKEV = 2
TRTOK = 1
LNPAD = 2
A5 = 8500
A4N = 32
A5K = ((128, 32), (160, 48), (208, 48))
LNTOK = 1
LNLAG = 300
LNG = 1
GLAG = 0
RECQ = True
FUSE = False
QSPLIT = 6
SLAG = 400
FSTEP = 2
CR = 32
XN = 128
VMEM_MB = 120
CT = 128

L_ORD = (2, 3, 0, 1, 4, 5, 6)
R_ORD = (2, 0, 6, 5, 1, 4, 3)

K_SEQ = (1, 4, 0, 2, 3, 5, 6)
K_SEQ2 = (0, 1, 2, 5, 3, 4, 6)

NN = (((1,), (0,)), ((), ()))
NT_ = (((1,), (1,)), ((), ()))
TN = (((0,), (0,)), ((), ()))


SCOPES = False


def _scope(name):
    return jax.named_scope(name) if SCOPES else contextlib.nullcontext()


def _mo(v, m):
    return v if isinstance(v, int) else pl.multiple_of(v, m)


def _dot(a, b, dims):
    return lax.dot_general(a, b, dims, preferred_element_type=f32)


def _pack(v):
    return pltpu.bitcast(v.astype(bf16), u32)


def _unpack(v):
    return pltpu.bitcast(v, bf16)


def _combine(m):
    m1, m2, m3, m4, m5, m6, m7 = m
    return m1 + m4 - m5 + m7, m3 + m5, m2 + m4, m1 - m2 + m3 + m6


def _lform(a11, a12, a21, a22):
    return (a11 + a22, a21 + a22, a11, a22, a11 + a12, a21 - a11, a12 - a22)


def _rform(b11, b12, b21, b22):
    return (b11 + b22, b11, b12 - b22, b21 - b11, b22, b11 + b12, b21 + b22)


def _sform(x11, x12, x21, x22):
    return (x11, x22, x11 + x22, x21 + x22, x11 + x12, x21 - x11, x12 - x22)


class _Sym:
    def __init__(self, t):
        self.t = t

    def __add__(self, o):
        return _Sym({**self.t, **o.t})

    def __sub__(self, o):
        return _Sym({**self.t, **{k: -v for k, v in o.t.items()}})


def _phi(t):
    return jnp.where(t > 0, t + 1.0, jnp.exp(t)) + 1e-6


def _rbf(v):
    return v.astype(bf16).astype(f32)


def _layernorm_rows(xv):
    mf = jnp.sum(xv, axis=1, keepdims=True) * (1.0 / D)
    mb = _rbf(mf)
    d = xv - mb
    dm = mf - mb
    var = jnp.sum(d * d, axis=1, keepdims=True) * (1.0 / D) - dm * dm
    var = jnp.maximum(var, 0.0)
    sd = _rbf(jnp.sqrt(_rbf(_rbf(var) + 1e-5)))
    return d * (1.0 / sd)


def _kernel(x_hbm, wqkv_hbm, wo_hbm, wr_hbm, wg_hbm, wu_hbm, wd_hbm, out_hbm,
            x_buf, wv_buf, wo_buf, wr_buf, wg_buf, wu_buf, wd_buf,
            xs1, xs2, wqs, sa, sb, zacc, zp, pk_buf, xb, yacc, rsel, wrb, zero_buf,
            wks, stats, wqt, ps_raw, qs, ms, tscr, tscr2, pq_raw, den_raw, pqb_buf, denb_buf, qsb,
            mg_raw, hb_raw, out_buf, idx_s, sem):
    wq_buf = out_buf.at[pl.ds(0, D), :]
    wk_buf = out_buf.at[pl.ds(D, D), :]

    def xs_at(k1, e, rows=None):
        r = xs1.at[k1 * 4 + (0, 1, 7, 8).index(e)] if e in (0, 1, 7, 8) else xs2.at[k1 * 5 + e - 2]
        return r if rows is None else r.at[rows, :]

    SEM_B, SEM_O, SEM_Z, SEM_A = 0, 4, 5, 6

    def cp(src, dst, s):
        return pltpu.make_async_copy(src, dst, sem.at[s])

    def cp_x(r0, n, s):
        rows = [pl.ds(_mo(q * HQ + r0, 16), n) for q in range(4)]
        return [cp(x_hbm.at[0, r, :], x_buf.at[r, :], s) for r in rows]

    def cp_wk(c, s):
        return [cp(wqkv_hbm.at[:, pl.ds(_mo(D + h * HD + c * 128, 128), 128)],
                   wk_buf.at[:, pl.ds(_mo(c * 256 + h * 128, 128), 128)], s) for h in range(2)]

    cp_wr = cp(wr_hbm, wr_buf.at[pl.ds(0, D)], SEM_Z)

    def make_a_groups():
        return [
            cp_x(0, 64, SEM_A),
            cp_x(64, 64, SEM_A + 1),
            cp_wk(0, SEM_A + 2),
            cp_wk(1, SEM_A + 3),
            cp_wk(2, SEM_A + 4) + cp_x(128, 64, SEM_A + 4),
            cp_wk(3, SEM_A + 5) + cp_x(192, 128, SEM_A + 5),
            cp_x(320, 192, SEM_A + 6) + [cp(wqkv_hbm.at[:, pl.ds(0, D)], wq_buf, SEM_A + 6)],
        ]

    def cp_b(j, part, wait_only=False):
        pairs = []
        f0, fw = (0, F1) if part == 0 else (F1, FH - F1)
        fs = pl.ds(_mo(j * FH + f0, 128), fw)
        pairs += [(wg_hbm.at[:, fs], wg_buf.at[j, :, pl.ds(f0, fw)]),
                  (wu_hbm.at[:, fs], wu_buf.at[j, :, pl.ds(f0, fw)]),
                  (wd_hbm.at[fs, :], wd_buf.at[j, pl.ds(f0, fw), :])]
        if part == 1:
            for a in range(4):
                c0 = _mo((2 * a + j) * 128, 128)
                pairs += [(wqkv_hbm.at[:, pl.ds(2 * D + c0, 128)], wv_buf.at[j, :, pl.ds(a * 128, 128)]),
                          (wo_hbm.at[pl.ds(c0, 128), :], wo_buf.at[j, pl.ds(a * 128, 128), :])]
        return [cp(dst if wait_only else src, dst, SEM_B + 2 * j + part) for src, dst in pairs]

    clock = [0]
    toks = []
    sides = []
    fwd = [None]

    def emit_tok(vals, stamp=None):
        t = None
        for v in vals:
            v = pltpu.bitcast(v, u32) if v.dtype != u32 else v
            t = v if t is None else t | v
        toks.append((clock[0] if stamp is None else stamp, t & zero_buf[0]))

    def gate(v):
        if fwd[0] is None:
            return v
        if fwd[0][1] is None:
            fwd[0][1] = pltpu.bitcast(fwd[0][0](), u32) & zero_buf[0]
        head = pltpu.bitcast(pltpu.bitcast(v[0:8], u32) | fwd[0][1], v.dtype)
        return head if v.shape[0] == 8 else jnp.concatenate([head, v[8:]], axis=0)

    def add_side(gen_fn, n, t0, t1, lag=None):
        st = {"i": 0, "n": n, "t0": clock[0] + t0, "t1": clock[0] + t1}

        def tok(vals, extra=0):
            if lag is not None:
                emit_tok(vals, st["t0"] + (st["i"] + 1) * (st["t1"] - st["t0"]) // st["n"] + lag + extra)
        st["g"] = gen_fn(tok)
        sides.append(st)

    def advance(until):
        for st in sides:
            while st["i"] < st["n"] and st["t0"] + st["i"] * (st["t1"] - st["t0"]) // st["n"] < until:
                next(st["g"], None)
                st["i"] += 1
                if st["i"] == st["n"]:
                    for _ in st["g"]:
                        pass

    def flush():
        for st in sides:
            for _ in st["g"]:
                pass
        sides.clear()

    def finish():
        flush()
        toks.clear()
        fwd[0] = None

    def mm(lhs, rhs, dims, cycles, nseg=1):
        due = [t for (c, t) in toks if c <= clock[0]]
        toks[:] = [(c, t) for (c, t) in toks if c > clock[0]]
        if due:
            head = rhs[0:8, 0:128]
            for t in due:
                head = head | t
            if rhs.shape[1] > 128:
                head = jnp.concatenate([head, rhs[0:8, 128:]], axis=1)
            rhs = jnp.concatenate([head, rhs[8:]], axis=0)
        res = _dot(lhs, _unpack(rhs), dims)
        ngr = res.shape[0] // 16
        for sg in range(nseg):
            for i in range(ngr):
                fwd[0] = [lambda sg=sg, i=i: res[i * 16:i * 16 + 8, sg * 128:(sg + 1) * 128], None]
                clock[0] += cycles // nseg // ngr
                advance(clock[0])
        return res

    def gate16(v):
        return jnp.concatenate([gate(v[0:8]), gate(v[8:16])], axis=0)

    def form_steps(form, get, put, tok=None, inner=None, gated=False):
        terms = form(*[_Sym({i: 1}) for i in range(4)])
        for k1 in range(7):
            sub = []
            for r in range(2):
                for c in range(2):
                    v = None
                    for i, sg in sorted(terms[k1].t.items(), key=lambda e: -e[1]):
                        b = get(r + 2 * (i // 2), c + 2 * (i % 2))
                        if v is None:
                            v = gate16(b) if r == c and not gated else b
                        else:
                            v = v + b if sg > 0 else v - b
                    sub.append(v)
            vals = []
            for k2, v in (enumerate(form(*sub)) if inner is None else inner(sub)):
                vals.append(v)
                put(k1, k2, _pack(v))
            if tok is not None and k1 % TOKEV == TOKEV - 1 - (6 % TOKEV != TOKEV - 1):
                tok([v[o:o + 8] for v in vals[-2:] for o in (0, 8)])
            yield

    def strassen2(lhs, rhs, dims, cycles, nseg=1, wts=(16,) * 7):
        m1 = [None] * 7
        for i1, k1 in enumerate(K_SEQ2):
            m2 = [None] * 7
            for k2 in K_SEQ2:
                m2[k2] = mm(lhs(k1, k2), rhs(k1, k2), dims, cycles * wts[i1] // 16, nseg)
                yield
            m1[k1] = _combine(m2)
        out = [[None] * 4 for _ in range(4)]
        for s2 in range(4):
            for s1, v in enumerate(_combine([m1[k1][s2] for k1 in range(7)])):
                out[(s1 // 2) * 2 + s2 // 2][(s1 % 2) * 2 + s2 % 2] = v
        return out

    made = set()

    def need(*keys):
        assert all(k in made for k in keys), keys

    def row_views(base):
        if isinstance(base, int) and base == 0:
            return x_buf, sa, sb, stats, xn_buf, None
        b = _mo(base, 64)
        return ([r.at[pl.ds(b, S - 64), :] for r in (x_buf, sa, sb, stats)]
                + [xn_buf.at[:, pl.ds(b, 64), :], pl.ds(_mo(base // 2, 32), 32)])

    def xs_form(r0, tok, which="all", base=0):
        xn_v, xs_v = row_views(base)[4:]
        rows = slice(r0 % XN, r0 % XN + 16)

        def inner(sub):
            full = list(enumerate(_sform(*sub))) + [(7, sub[1]), (8, sub[2])]
            return [full[e] for e in {"all": (0, 1, 7, 8, 2, 5, 6, 3, 4), "l1": (0, 1, 7, 8),
                                      "l2": (2, 5, 6, 3, 4)}[which]]
        for ct in range(2):
            def put(k1, k2, v):
                xs_at(k1, k2, xs_v)[r0 // 2:r0 // 2 + 8, ct * 128:(ct + 1) * 128] = v
            yield from form_steps(
                _sform, lambda q, u: xn_v[q, rows, u * 256 + ct * 128:u * 256 + (ct + 1) * 128],
                put, tok, inner)
        made.add(("xs", r0))

    def ln_rows(r_start, n_rows, tok, which="all", base=0):
        x_v, sa_v, sb_v, st_v, xn_v, _ = row_views(base)
        lane = lax.broadcasted_iota(i32, (8, 128), 1)

        def later(r0):
            form = xs_form(r0, tok, which, base)
            for g in range(8):
                q, o = g // 2, (g % 2) * 8
                t = None
                for ct in range(8):
                    cs = slice(ct * 128, (ct + 1) * 128)
                    v = xn_v[q, r0 % XN + o:r0 % XN + o + 8, cs] * wrb[:, cs]
                    t = gate(v) if t is None else t + v
                st_v[q * HQ + r0 + o:q * HQ + r0 + o + 8, 128:256] = t
                if tok is not None and TRTOK:
                    tok([t])
                yield
                for _ in range(2 if g < 7 else 0):
                    next(form)
                    yield
            next(form, None)
            made.add(("ln", r0))

        for c in range(n_rows // 16 + 1):
            r0 = r_start + c * 16
            rest = later(r0 - 16) if c > 0 else iter(())
            for g in range(8 if c < n_rows // 16 else 0):
                q, o = g // 2, (g % 2) * 8
                rg = q * HQ + r0 + o
                xv = x_v[rg:rg + 8, :].astype(f32)
                xg = jnp.concatenate([gate(xv[:, 0:128]), xv[:, 128:]], axis=1)
                mf = jnp.sum(xg, axis=1, keepdims=True) * (1.0 / D)
                d = xv - mf
                var = jnp.sum(d * d, axis=1, keepdims=True) * (1.0 / D)
                rs = lax.rsqrt(var + 1e-5)
                xn_v.at[q][r0 % XN + o:r0 % XN + o + 8, :] = d * rs
                rs = jnp.broadcast_to(rs, (8, 128))
                mf = jnp.broadcast_to(mf, (8, 128))
                sa_v[rg:rg + 8, :] = 1.0 + rs
                sb_v[rg:rg + 8, :] = mf * rs
                st_v[rg:rg + 8, 0:128] = jnp.where(lane == 0, mf, jnp.broadcast_to(var, (8, 128)))
                if tok is not None and LNTOK:
                    tok([rs], LNLAG)
                yield
                if g >= LNG and c > 0:
                    for _ in range(3):
                        next(rest)
                        yield
                elif c == 0:
                    for _ in range(LNPAD):
                        yield
            yield from rest

    def wk_prep(c, tok=None):
        cs = pl.ds(_mo(c * 256, 256), 256)
        for i in range(HD // 16):
            r0 = i * 16
            top = wk_buf[r0:r0 + 16, cs].astype(f32)
            bot = wk_buf[HD + r0:HD + r0 + 16, cs].astype(f32)
            ops = _rform(gate(top[:, :128]), top[:, 128:], bot[:, :128], gate(bot[:, 128:]))
            for k in range(7):
                wks.at[c][r0 // 2:r0 // 2 + 8, k * 128:(k + 1) * 128] = _pack(ops[k])
            yield

    def wq_perm(tok):
        def permute(kt):
            for g in range(8):
                tile = gate(pltpu.bitcast(wq_buf[kt * 128:(kt + 1) * 128, g * 128:(g + 1) * 128], u32))
                wqt.at[kt * 8 + g][...] = pltpu.bitcast(_unpack(tile).T, u32)
                yield

        def back(kt):
            for j in range(8):
                tile = gate(jnp.concatenate([wqt[kt * 8 + g, pl.ds(j, 8, stride=8), :] for g in range(8)],
                                            axis=0))
                v = pltpu.bitcast(_unpack(tile).T.astype(f32), u32)
                ps[(kt % 2) * 128:(kt % 2 + 1) * 128, (kt // 2) * D + j * 128:(kt // 2) * D + (j + 1) * 128] = v
                made.add(("wqp", kt, j))
                yield

        order = (0, 2, 4, 6, 1, 3, 5, 7)
        for n in range(10):
            if n < 8:
                yield from permute(order[n])
            if n > 1:
                yield from back(order[n - 2])

    def wq_form(tok):
        for i in range(16):
            need(*[("wqp", 2 * r + i // 8, j) for r in range(4) for j in range(8)])
            for ct in range(2):
                def put(k1, k2, v):
                    wqs.at[k1 * 7 + k2][i * 8:(i + 1) * 8, ct * 128:(ct + 1) * 128] = v
                yield from form_steps(
                    _rform, lambda r, c: pltpu.bitcast(
                        ps[i * 16:(i + 1) * 16, r * D + c * 256 + ct * 128:r * D + c * 256 + (ct + 1) * 128],
                        f32), put, tok)

    def kproj(r0, n, chunks=((0, 0), (0, 1), (1, 0), (1, 1))):
        pr = pl.ds(r0 // 2, n // 2)
        need(*[("xs", r) for r in range(max(r0, 128), r0 + n, 16)])
        for ch, ct in chunks:
            c = 2 * ch + ct
            m = [None] * 7
            for k in K_SEQ:
                e11, e22, e12, e21 = [xs_at(L_ORD[k], e)[pr, :] for e in (0, 1, 7, 8)]
                lhs = jnp.concatenate([jnp.concatenate([e11, e12], axis=1),
                                       jnp.concatenate([e21, e22], axis=1)], axis=0)
                m[k] = mm(_unpack(lhs), wks[c, :, k * 128:(k + 1) * 128], NN, 2 * n)
            kk = [_phi(v) for v in _combine(m)]
            for h in range(2):
                zacc[:, pl.ds(_mo(h * HD + c * 128, 128), 128)] += (
                    (kk[h] + kk[2 + h]).reshape(n // 4, 8, 128).sum(axis=0))
            for s1 in range(4):
                u = (s1 % 2) * 2 + ch
                for h in range(2):
                    pk_buf.at[ct, (s1 // 2) * 2 + h][r0:r0 + n, u * 128:(u + 1) * 128] = (
                        kk[s1][h * n:(h + 1) * n])

    def z_prep():
        z = jnp.sum(zacc[...], axis=0, keepdims=True)
        zt = _pack(jnp.broadcast_to(z, (128, D)).astype(bf16).T)
        for g in range(8):
            tscr.at[g][...] = zt[g * 64:(g + 1) * 64, :]
        for j in range(8):
            blk = jnp.concatenate([tscr[g, pl.ds(j, 8, stride=8), :] for g in range(8)], axis=0)
            zp[:, j * 128:(j + 1) * 128] = _unpack(blk).T[0:8, :].astype(f32)

    def route(tok):
        need(*[("ln", r) for r in range(128, HQ, 16)])
        rows, dots = [], []
        for b in range(S // 128):
            rows.append(gate(stats[b * 128:(b + 1) * 128, 0:128]).T[0:8, :])
            dots.append(jnp.sum(gate(stats[b * 128:(b + 1) * 128, 128:256]).T, axis=0, keepdims=True))
            yield
        mf = jnp.concatenate([v[0:1] for v in rows], axis=0)
        var = jnp.concatenate([v[1:2] for v in rows], axis=0)
        tr = jnp.concatenate(dots, axis=0) * jnp.sqrt(var + 1e-5)
        wsum = jnp.sum(wrb[0:1, :], axis=1, keepdims=True)
        sd = _rbf(jnp.sqrt(_rbf(_rbf(var) + 1e-5)))
        rv = _rbf((tr + (mf - _rbf(mf)) * wsum) / sd)
        rmax = jnp.max(rv)
        pos = (lax.broadcasted_iota(i32, rv.shape, 0) * 128 + lax.broadcasted_iota(i32, rv.shape, 1))
        idx = jnp.min(jnp.where(rv == rmax, pos, S - 1))
        idx_s[0] = idx
        rsel[...] = jnp.full(rsel.shape, rmax, f32)
        b0 = _mo((idx // 16) * 16, 16)
        xn = _rbf(_layernorm_rows(x_buf[pl.ds(b0, 16), :].astype(f32)))
        sel = lax.broadcasted_iota(i32, xn.shape, 0) == idx - b0
        row = jnp.sum(jnp.where(sel, xn, 0.0), axis=0, keepdims=True)
        xbv = jnp.broadcast_to(row, (128, D)).T
        xb[...] = xbv
        yacc[...] = jnp.zeros(yacc.shape, f32)
        tok([xbv[b * 128 + 120:(b + 1) * 128] for b in range(8)])
        yield

    def ps_form(j, tok):
        for c in range(HQ // 16):
            def put(k1, k2, v):
                k = k1 * 7 + k2
                ps[c * 8:(c + 1) * 8, k * 128:(k + 1) * 128] = v
            yield from form_steps(
                _lform, lambda r, q: pk_buf[j, q, c * 16:(c + 1) * 16, r * 128:(r + 1) * 128], put, tok)

    def q_rows(j, r0, n, pq, rc, d0, rec):
        xj = pl.ds(_mo(j * (BQ // 2), BQ // 2), BQ // 2)
        pr = slice(r0 // 2, (r0 + n) // 2)
        blk = yield from strassen2(lambda k1, k2: _unpack(xs_at(L_ORD[k1], L_ORD[k2], xj)[pr, :]),
                                   lambda k1, k2: wqs[k1 * 7 + k2], NN, n, 1, QW)
        lane = lax.broadcasted_iota(i32, (n, 128), 1)
        for q in range(4):
            d = None
            for u in (3, 2, 1, 0):
                v = _phi(blk[q][u])
                pq.at[q][d0:d0 + n, u * 256:(u + 1) * 256] = v
                t = v * zp[0:1, u * 256:(u + 1) * 256]
                t = t[:, :128] + t[:, 128:]
                d = t if d is None else d + t
            if rec:
                d = recip(d, lane)
            rc.at[q][d0:d0 + n, :] = d

    def recip(d, lane):
        d = d + jnp.where(lane % 2 == 0, pltpu.roll(d, 127, 1), pltpu.roll(d, 1, 1))
        d = d + jnp.where(lane % 4 < 2, pltpu.roll(d, 126, 1), pltpu.roll(d, 2, 1))
        return 1.0 / (d + 1e-6)

    def normalise(pq, rc, nr, dst, p0, raw, tok=None):
        lane = lax.broadcasted_iota(i32, (16, 128), 1)

        def fix(c):
            if c < nr // 16 and raw(c * 16):
                for q in range(4):
                    rq = slice(c * 16, (c + 1) * 16)
                    rc.at[q][rq, :] = recip(gate16(rc[q, rq, :]), lane)

        fix(0)
        if raw(0):
            for _ in range(4):
                yield
        for c in range(nr // 16):
            rq = slice(c * 16, (c + 1) * 16)
            p2 = pl.ds(_mo(p0 + c * 8, 8), 8)
            fix(c + 1)
            for q in range(4):
                for hf in range(2):
                    cs = slice(hf * HD, (hf + 1) * HD)
                    pq.at[q][rq, cs] = pq[q, rq, cs] * jnp.concatenate([gate16(rc[q, rq, :])] * 4, axis=1)
                    yield
            for ct in range(2):
                def put(k1, k2, v):
                    dst.at[k1 * 7 + k2][p2, ct * 128:(ct + 1) * 128] = v
                yield from form_steps(
                    _lform, lambda q, u: pq[q, rq, u * 256 + ct * 128:u * 256 + (ct + 1) * 128], put, tok)
        made.add(("qs", id(dst)))

    hist = []

    def g_lhs(k):
        v = ps[:, k * 128:(k + 1) * 128]
        hist.append(fwd[0])
        if GLAG and len(hist) > GLAG and hist[-1 - GLAG] is not None:
            cur = fwd[0]
            fwd[0] = hist[-1 - GLAG]
            v = jnp.concatenate([gate(v[i * 64:(i + 1) * 64]) for i in range(4)], axis=0)
            fwd[0] = cur
        return _unpack(v)

    def g_kvm(j):
        blk = yield from strassen2(
            lambda k1, k2: g_lhs(k1 * 7 + k2),
            lambda k1, k2: xs_at(R_ORD[k1], R_ORD[k2])[...], TN, 256, 2)
        hm = (lax.broadcasted_iota(i32, (128, 128), 0) // 32
              == lax.broadcasted_iota(i32, (128, 128), 1) // 32)
        qb = q_rows(j, BQ - QB, QB, pqb_buf.at[j], denb_buf.at[j], 0, False)
        for _ in range(QSPLIT):
            next(qb)
        kvps = []
        for a in (3, 2, 1, 0):
            gg = jnp.concatenate(blk[a], axis=1).astype(bf16)
            clock[0] += 256
            kv = jnp.where(hm, _dot(gg, wv_buf[j, :, a * 128:(a + 1) * 128], NN), 0.0)
            tscr2.at[a][...] = _pack(kv)
            kvps.append(_unpack(jnp.concatenate(
                [tscr2[a, pl.ds(jj, 8, stride=8), :] for jj in range(8)], axis=0)))
        mg = mg_buf

        def m_form(tok):
            for a in (3, 2, 1, 0):
                need(("mg", a))
                for jl in range(2):
                    for ct in range(2):
                        def put(k1, k2, v):
                            ms.at[k1 * 7 + k2][pl.ds(_mo(jl * 64 + (2 * a + j) * 8, 8), 8),
                                               ct * 128:(ct + 1) * 128] = v
                        yield from form_steps(
                            _rform, lambda q, u: mg[a, (2 * q + jl) * 16:(2 * q + jl + 1) * 16,
                                                    u * 256 + ct * 128:u * 256 + (ct + 1) * 128], put)

        for i, a in enumerate((3, 2, 1, 0)):
            wo_u = pltpu.bitcast(wo_buf[j, a * 128:(a + 1) * 128, :], u32)
            res = mm(kvps[i], wo_u, NN, 256)
            mg.at[a][...] = res
            made.add(("mg", a))
            if i == 0:
                add_side(m_form, 112, 128, 768 + (49 - QSPLIT) * QB - 100)
        for _ in qb:
            pass

    def out_part(p0, nr, y, src, pr0):
        pr = pl.ds(_mo(pr0, 8), nr // 2)
        rows = [pl.ds(_mo(q * HQ + p0, 16), nr) for q in range(4)]
        row = lax.broadcasted_iota(i32, (nr, 256), 0) + p0
        blk = yield from strassen2(lambda k1, k2: _unpack(src[k1 * 7 + k2, pr, :]),
                                   lambda k1, k2: ms[k1 * 7 + k2], NN, nr)
        for s1 in (3, 2, 1, 0):
            for s2 in range(4):
                q = (s1 // 2) * 2 + s2 // 2
                u = (s1 % 2) * 2 + s2 % 2
                rr, cc = rows[q], pl.ds(u * 256, 256)
                a = jnp.concatenate([sa[rr, :]] * 2, axis=1)
                b = jnp.concatenate([sb[rr, :]] * 2, axis=1)
                o = blk[q][u] + jnp.where(row + q * HQ == idx_s[0], y[:, u * 256:(u + 1) * 256], 0.0)
                out_buf[rr, cc] = (x_buf[rr, cc].astype(f32) * a - b + o).astype(bf16)
                if s2 % 2 == 1:
                    ch = pl.ds((s1 % 2) * HD, HD)
                    cp(out_buf.at[rr, ch], out_hbm.at[0, rr, ch], SEM_O).start()

    def ffn_part(j, f_lo, f_hi):
        for f0 in range(f_lo, f_hi, 256):
            fs = slice(f0, f0 + 256)
            ag = jnp.zeros((8, 256), f32)
            au = jnp.zeros((8, 256), f32)
            for kg in range(D // 8):
                xv = jnp.concatenate([gate(xb[8 * kg:8 * kg + 8, :])] * 2, axis=1)
                ag = ag + wg_buf[j, 8 * kg:8 * kg + 8, fs].astype(f32) * xv
                au = au + wu_buf[j, 8 * kg:8 * kg + 8, fs].astype(f32) * xv
                if kg % FSTEP == FSTEP - 1:
                    yield
            g = _rbf(jnp.sum(ag, axis=0, keepdims=True))
            u = _rbf(jnp.sum(au, axis=0, keepdims=True))
            h = _rbf(_rbf(g * jax.nn.sigmoid(g)) * u)
            hb_buf[fs, :] = jnp.broadcast_to(h, (128, 256)).T
        for d0 in range(0, D, 512):
            ds_ = slice(d0, d0 + 512)
            acc = yacc[:, ds_]
            for kg in range(f_lo // 8, f_hi // 8):
                hv = jnp.concatenate([gate(hb_buf[8 * kg:8 * kg + 8, :])] * 4, axis=1)
                acc = acc + wd_buf[j, 8 * kg:8 * kg + 8, ds_].astype(f32) * hv
                if kg % FSTEP == FSTEP - 1:
                    yield
            yacc[:, ds_] = acc

    def wait_group(i):
        with _scope("a_wait%d" % i):
            for c in a_groups[i]:
                c.wait()

    def run_all(gen):
        for _ in gen:
            pass

    def ln_side(r0, n, t0, t1):
        add_side(lambda tok: ln_rows(r0, n, tok), 30 * n // 16 + 8 * LNPAD, t0, t1, SLAG)

    def l2_side(base, n, t0, t1):
        def gen(tok):
            for r in range(0, n, 16):
                yield from xs_form(r, tok, "l2", base)
        add_side(gen, 14 * n // 16, t0, t1)

    a_groups = make_a_groups()
    with _scope("p0_issue"):
        cp_wr.start()
        for grp in a_groups:
            for c in grp:
                c.start()
        for j in range(2):
            for part in range(2):
                for c in cp_b(j, part):
                    c.start()
        zacc[...] = jnp.zeros(zacc.shape, f32)
        zero_buf[1] = jnp.zeros((8, 128), u32)
        cp_zero = cp(zero_buf.at[1], zero_buf.at[0], SEM_Z)
        cp_zero.start()
        cp_zero.wait()
        cp_wr.wait()
        wrb[...] = jnp.broadcast_to(wr_buf[0:D].reshape(1, D).astype(f32), (8, D))
        z0 = jnp.max(pltpu.bitcast(zero_buf[0], i32))
        ps, pq_buf, den_buf, mg_buf, hb_buf = [r.at[z0] for r in (ps_raw, pq_raw, den_raw, mg_raw, hb_raw)]
        xn_buf = mg_buf

    def a01(i, carry):
        with _scope("a_wait01"):
            for c in cp_x(i * 64, 64, SEM_A + i):
                c.wait()
        with _scope("a01"):
            run_all(ln_rows(0, 64, None, "l1", i * 64))
        return carry

    lax.fori_loop(0, 2, a01, 0)

    def a23(i, carry):
        with _scope("a_wait23"):
            for c in cp_wk(i, SEM_A + 2 + i):
                c.wait()
        with _scope("a23"):
            run_all(wk_prep(i))
            l2_side(i * 64, 64, 300, 1500)
            kproj(0, 128, [(0, i)])
            finish()
        return carry

    lax.fori_loop(0, 2, a23, 0)
    wait_group(4)
    with _scope("a4"):
        run_all(wk_prep(2))
        ln_side(128, A4N, 0, 1500)
        kproj(0, 128, [(1, 0)])
        finish()
    wait_group(5)
    with _scope("a5"):
        run_all(wk_prep(3))
        if A5 == 0:
            ln_side(160, 32, 0, 1400)
            kproj(0, 128, [(1, 1)])
            for r0 in (128, 192):
                ln_side(r0 + 64, 64, 0, 3200)
                kproj(r0, 64)
        else:
            ln_side(128 + A4N, 192 - A4N, 0, A5)
            kproj(0, 128, [(1, 1)])
            for r0, n in A5K:
                kproj(r0, n)
        finish()
    wait_group(6)
    with _scope("a6"):
        ln_side(320, 192, 0, A6[0])
        add_side(wq_perm, 128, A6[1], A6[2], A6[6])
        add_side(wq_form, 224, A6[3], A6[4], A6[6])
        add_side(route, 17, A6[5], A6[5] + 800)
        for r0 in (256, 320, 384, 448):
            kproj(r0, 64)
        finish()

    def b_body(j, carry):
        qa = BQ - QB
        with _scope("b_wait0"):
            for c in cp_b(j, 0, wait_only=True):
                c.wait()
        with _scope("b_r0"):
            z_prep()
            t1 = 49 * qa - 400
            add_side(lambda tok: ps_form(j, None), 7 * HQ // 16, 0, t1)
            add_side(lambda tok: ffn_part(j, 0, F1), F1 * 3 // (4 * FSTEP), 0, t1)
            for r0 in range(0, qa, QN):
                run_all(q_rows(j, r0, min(QN, qa - r0), pq_buf, den_buf, r0, r0 + QN < qa))
            finish()
        with _scope("b_wait1"):
            for c in cp_b(j, 1, wait_only=True):
                c.wait()
        with _scope("b_r1"):
            add_side(lambda tok: ffn_part(j, F1, FH), (FH - F1) * 3 // (4 * FSTEP), 0, 12800)
            add_side(lambda tok: normalise(pq_buf, den_buf, qa, qs, j * (qa // 2),
                                           lambda r: (r // QN + 1) * QN >= qa), 22 * (qa // 16), 0, 12800)
            run_all(g_kvm(j))
            finish()
        return carry

    lax.fori_loop(0, 2, b_body, 0)

    def c_body(t, carry):
        with _scope("c_body"):
            y = _rbf(jnp.sum(yacc[...], axis=0, keepdims=True))
            y = _rbf(y * _rbf(jax.nn.sigmoid(rsel[0:1, :])))
            j, h = t >> 1, t & 1
            na, nb = (BQ - QB) // 2, QB // 2
            hb = pl.ds(_mo(h * nb, 16), nb)
            add_side(lambda tok: normalise(pqb_buf.at[j, :, hb, :], denb_buf.at[j, :, hb, :], nb, qsb, 0,
                                           lambda r: True, tok),
                     4 + 22 * (nb // 16), 0, 49 * na - 800, SLAG)
            for p in range(0, na, CR):
                p0 = j * BQ + h * na + p
                run_all(out_part(p0, min(CR, na - p), y, qs, t * (na // 2) + p // 2))
            advance(clock[0] + 10 ** 6)
            flush()
            run_all(out_part(j * BQ + BQ - QB + h * nb, nb, y, qsb, 0))
            finish()
        return carry

    lax.fori_loop(0, 4, c_body, 0)
    with _scope("tail"):
        cp(out_buf, out_hbm.at[0], SEM_O).wait()


@jax.jit
def pallas_parallel_sum__linear_attn_block__moe_arch_mod__prompt_kernel(
    A_x: jax.Array,
    A_wqkv: jax.Array,
    A_wo: jax.Array,
    B_x: jax.Array,
    B_w_r: jax.Array,
    B_w_gate: jax.Array,
    B_w_up: jax.Array,
    B_w_down: jax.Array,
):
    del B_x
    V = pltpu.VMEM
    scratch = [
        V((S, D), bf16),
        V((2, D, 512), bf16),
        V((2, 512, D), bf16),
        V((8 * D,), bf16),
        V((2, D, FH), bf16),
        V((2, D, FH), bf16),
        V((2, FH, D), bf16),
        V((28, HQ // 2, 256), u32),
        V((35, HQ // 2, 256), u32),
        V((49, 128, 256), u32),
        V((S, 128), f32),
        V((S, 128), f32),
        V((8, D), f32),
        V((8, D), f32),
        V((2, 4, HQ, 512), f32),
        V((D, 128), f32),
        V((8, D), f32),
        V((8, D), f32),
        V((8, D), f32),
        V((4, 8, 128), u32),
        V((4, HD // 2, 7 * 128), u32),
        V((S, 256), f32),
        V((64, 64, 128), u32),
        V((1, HQ // 2, 49 * 128), u32),
        V((49, BQ - QB, 256), u32),
        V((49, 128, 256), u32),
        V((8, 64, 128), u32),
        V((4, 64, 128), u32),
        V((1, 4, BQ - QB, D), f32),
        V((1, 4, BQ - QB, 128), f32),
        V((2, 4, QB, D), f32),
        V((2, 4, QB, 128), f32),
        V((49, QB // 4, 256), u32),
        V((1, 4, 128, D), f32),
        V((1, FH, 128), f32),
        V((S, D), bf16),
        pltpu.SMEM((1,), i32),
        pltpu.SemaphoreType.DMA((13,)),
    ]
    return pl.pallas_call(
        _kernel,
        out_shape=jax.ShapeDtypeStruct((1, S, D), bf16),
        in_specs=[pl.BlockSpec(memory_space=pl.ANY)] * 7,
        out_specs=pl.BlockSpec(memory_space=pl.ANY),
        scratch_shapes=scratch,
        compiler_params=pltpu.CompilerParams(vmem_limit_bytes=VMEM_MB * 1024 * 1024,
                                             disable_bounds_checks=True,
                                             fuse_transposed_lhs_in_matmul=FUSE,
                                             disable_semaphore_checks=True),
    )(A_x, A_wqkv, A_wo, B_w_r, B_w_gate, B_w_up, B_w_down)
```

```python
import contextlib

import jax
import jax.numpy as jnp
from jax import lax
import jax.experimental.pallas as pl
import jax.experimental.pallas.tpu as pltpu

bf16, f32, u32, i32 = jnp.bfloat16, jnp.float32, jnp.uint32, jnp.int32

S = 2048
D = 1024
F = 3584
HP = S // 2
HD = D // 2
HQ = S // 4
BQ = HQ // 2
FH = F // 2
F1 = 256
QB = 64
QN = 48
QW = (20, 28, 28, 12, 8, 8, 8)
A6 = (8500, 8000, 10800, 9800, 13900, 11300, None)
TOKEV = 2
TRTOK = 1
LNPAD = 2
A5 = 8500
A4N = 32
A5K = ((128, 32), (160, 48), (208, 48))
LNTOK = 1
LNLAG = 300
LNG = 1
GLAG = 0
RECQ = True
FUSE = False
QSPLIT = 6
SLAG = 400
FSTEP = 2
CR = 32
XN = 128
VMEM_MB = 120
CT = 128

L_ORD = (2, 3, 0, 1, 4, 5, 6)
R_ORD = (2, 0, 6, 5, 1, 4, 3)

K_SEQ = (1, 4, 0, 2, 3, 5, 6)
K_SEQ2 = (0, 1, 2, 5, 3, 4, 6)

NN = (((1,), (0,)), ((), ()))
NT_ = (((1,), (1,)), ((), ()))
TN = (((0,), (0,)), ((), ()))


SCOPES = False


def _scope(name):
    return jax.named_scope(name) if SCOPES else contextlib.nullcontext()


def _mo(v, m):
    return v if isinstance(v, int) else pl.multiple_of(v, m)


def _dot(a, b, dims):
    return lax.dot_general(a, b, dims, preferred_element_type=f32)


def _pack(v):
    return pltpu.bitcast(v.astype(bf16), u32)


def _unpack(v):
    return pltpu.bitcast(v, bf16)


def _combine(m):
    m1, m2, m3, m4, m5, m6, m7 = m
    return m1 + m4 - m5 + m7, m3 + m5, m2 + m4, m1 - m2 + m3 + m6


def _lform(a11, a12, a21, a22):
    return (a11 + a22, a21 + a22, a11, a22, a11 + a12, a21 - a11, a12 - a22)


def _rform(b11, b12, b21, b22):
    return (b11 + b22, b11, b12 - b22, b21 - b11, b22, b11 + b12, b21 + b22)


def _sform(x11, x12, x21, x22):
    return (x11, x22, x11 + x22, x21 + x22, x11 + x12, x21 - x11, x12 - x22)


class _Sym:
    def __init__(self, t):
        self.t = t

    def __add__(self, o):
        return _Sym({**self.t, **o.t})

    def __sub__(self, o):
        return _Sym({**self.t, **{k: -v for k, v in o.t.items()}})


def _st(u, ct):
    return slice((4 * ct + u) * 128, (4 * ct + u + 1) * 128)


def _to_st(v):
    return jnp.concatenate([v[:, (2 * u + ct) * 128:(2 * u + ct + 1) * 128]
                            for ct in range(2) for u in range(4)], axis=1)


def _phi(t):
    return jnp.where(t > 0, t + 1.0, jnp.exp(t)) + 1e-6


def _rbf(v):
    return v.astype(bf16).astype(f32)


def _layernorm_rows(xv):
    mf = jnp.sum(xv, axis=1, keepdims=True) * (1.0 / D)
    mb = _rbf(mf)
    d = xv - mb
    dm = mf - mb
    var = jnp.sum(d * d, axis=1, keepdims=True) * (1.0 / D) - dm * dm
    var = jnp.maximum(var, 0.0)
    sd = _rbf(jnp.sqrt(_rbf(_rbf(var) + 1e-5)))
    return d * (1.0 / sd)


def _kernel(x_hbm, wqkv_hbm, wo_hbm, wr_hbm, wg_hbm, wu_hbm, wd_hbm, out_hbm,
            x_buf, wv_buf, wo_buf, wr_buf, wg_buf, wu_buf, wd_buf,
            xs1, xs2, wqs, sa, sb, zacc, zp, pk_buf, xb, yacc, rsel, wrb, zero_buf,
            wks, stats, wqt, ps_raw, qs, ms, tscr, tscr2, pq_raw, den_raw, pqb_buf, denb_buf, qsb,
            mg_raw, hb_raw, out_buf, idx_s, sem):
    wq_buf = out_buf.at[pl.ds(0, D), :]
    wk_buf = out_buf.at[pl.ds(D, D), :]

    def xs_at(k1, e, rows=None):
        r = xs1.at[k1 * 4 + (0, 1, 7, 8).index(e)] if e in (0, 1, 7, 8) else xs2.at[k1 * 5 + e - 2]
        return r if rows is None else r.at[rows, :]

    SEM_B, SEM_O, SEM_Z, SEM_A = 0, 4, 5, 6

    def cp(src, dst, s):
        return pltpu.make_async_copy(src, dst, sem.at[s])

    def cp_x(r0, n, s):
        rows = [pl.ds(_mo(q * HQ + r0, 16), n) for q in range(4)]
        return [cp(x_hbm.at[0, r, :], x_buf.at[r, :], s) for r in rows]

    def cp_wk(c, s):
        return [cp(wqkv_hbm.at[:, pl.ds(_mo(D + h * HD + c * 128, 128), 128)],
                   wk_buf.at[:, pl.ds(_mo(c * 256 + h * 128, 128), 128)], s) for h in range(2)]

    cp_wr = cp(wr_hbm, wr_buf.at[pl.ds(0, D)], SEM_Z)

    def make_a_groups():
        return [
            cp_x(0, 64, SEM_A),
            cp_x(64, 64, SEM_A + 1),
            cp_wk(0, SEM_A + 2),
            cp_wk(1, SEM_A + 3),
            cp_wk(2, SEM_A + 4) + cp_x(128, 64, SEM_A + 4),
            cp_wk(3, SEM_A + 5) + cp_x(192, 128, SEM_A + 5),
            cp_x(320, 192, SEM_A + 6) + [cp(wqkv_hbm.at[:, pl.ds(0, D)], wq_buf, SEM_A + 6)],
        ]

    def cp_b(j, part, wait_only=False):
        pairs = []
        f0, fw = (0, F1) if part == 0 else (F1, FH - F1)
        fs = pl.ds(_mo(j * FH + f0, 128), fw)
        pairs += [(wg_hbm.at[:, fs], wg_buf.at[j, :, pl.ds(f0, fw)]),
                  (wu_hbm.at[:, fs], wu_buf.at[j, :, pl.ds(f0, fw)]),
                  (wd_hbm.at[fs, :], wd_buf.at[j, pl.ds(f0, fw), :])]
        if part == 1:
            for a in range(4):
                c0 = _mo((2 * a + j) * 128, 128)
                pairs += [(wqkv_hbm.at[:, pl.ds(2 * D + c0, 128)], wv_buf.at[j, :, pl.ds(a * 128, 128)]),
                          (wo_hbm.at[pl.ds(c0, 128), :], wo_buf.at[j, pl.ds(a * 128, 128), :])]
        return [cp(dst if wait_only else src, dst, SEM_B + 2 * j + part) for src, dst in pairs]

    clock = [0]
    toks = []
    sides = []
    fwd = [None]

    def emit_tok(vals, stamp=None):
        t = None
        for v in vals:
            v = pltpu.bitcast(v, u32) if v.dtype != u32 else v
            t = v if t is None else t | v
        toks.append((clock[0] if stamp is None else stamp, t & zero_buf[0]))

    def gate(v):
        if fwd[0] is None:
            return v
        if fwd[0][1] is None:
            fwd[0][1] = pltpu.bitcast(fwd[0][0](), u32) & zero_buf[0]
        head = pltpu.bitcast(pltpu.bitcast(v[0:8], u32) | fwd[0][1], v.dtype)
        return head if v.shape[0] == 8 else jnp.concatenate([head, v[8:]], axis=0)

    def add_side(gen_fn, n, t0, t1, lag=None):
        st = {"i": 0, "n": n, "t0": clock[0] + t0, "t1": clock[0] + t1}

        def tok(vals, extra=0):
            if lag is not None:
                emit_tok(vals, st["t0"] + (st["i"] + 1) * (st["t1"] - st["t0"]) // st["n"] + lag + extra)
        st["g"] = gen_fn(tok)
        sides.append(st)

    def advance(until):
        for st in sides:
            while st["i"] < st["n"] and st["t0"] + st["i"] * (st["t1"] - st["t0"]) // st["n"] < until:
                next(st["g"], None)
                st["i"] += 1
                if st["i"] == st["n"]:
                    for _ in st["g"]:
                        pass

    def flush():
        for st in sides:
            for _ in st["g"]:
                pass
        sides.clear()

    def finish():
        flush()
        toks.clear()
        fwd[0] = None

    def mm(lhs, rhs, dims, cycles, nseg=1):
        due = [t for (c, t) in toks if c <= clock[0]]
        toks[:] = [(c, t) for (c, t) in toks if c > clock[0]]
        if due:
            head = rhs[0:8, 0:128]
            for t in due:
                head = head | t
            if rhs.shape[1] > 128:
                head = jnp.concatenate([head, rhs[0:8, 128:]], axis=1)
            rhs = jnp.concatenate([head, rhs[8:]], axis=0)
        res = _dot(lhs, _unpack(rhs), dims)
        ngr = res.shape[0] // 16
        for sg in range(nseg):
            for i in range(ngr):
                fwd[0] = [lambda sg=sg, i=i: res[i * 16:i * 16 + 8, sg * 128:(sg + 1) * 128], None]
                clock[0] += cycles // nseg // ngr
                advance(clock[0])
        return res

    def gate16(v):
        return jnp.concatenate([gate(v[0:8]), gate(v[8:16])], axis=0)

    def form_steps(form, get, put, tok=None, inner=None, gated=False):
        terms = form(*[_Sym({i: 1}) for i in range(4)])
        for k1 in range(7):
            sub = []
            for r in range(2):
                for c in range(2):
                    v = None
                    for i, sg in sorted(terms[k1].t.items(), key=lambda e: -e[1]):
                        b = get(r + 2 * (i // 2), c + 2 * (i % 2))
                        if v is None:
                            v = gate16(b) if r == c and not gated else b
                        else:
                            v = v + b if sg > 0 else v - b
                    sub.append(v)
            vals = []
            for k2, v in (enumerate(form(*sub)) if inner is None else inner(sub)):
                vals.append(v)
                put(k1, k2, _pack(v))
            if tok is not None and k1 % TOKEV == TOKEV - 1 - (6 % TOKEV != TOKEV - 1):
                tok([v[o:o + 8] for v in vals[-2:] for o in (0, 8)])
            yield

    def strassen2(lhs, rhs, dims, cycles, nseg=1, wts=(16,) * 7):
        m1 = [None] * 7
        for i1, k1 in enumerate(K_SEQ2):
            m2 = [None] * 7
            for k2 in K_SEQ2:
                m2[k2] = mm(lhs(k1, k2), rhs(k1, k2), dims, cycles * wts[i1] // 16, nseg)
                yield
            m1[k1] = _combine(m2)
        out = [[None] * 4 for _ in range(4)]
        for s2 in range(4):
            for s1, v in enumerate(_combine([m1[k1][s2] for k1 in range(7)])):
                out[(s1 // 2) * 2 + s2 // 2][(s1 % 2) * 2 + s2 % 2] = v
        return out

    made = set()

    def need(*keys):
        assert all(k in made for k in keys), keys

    def row_views(base):
        if isinstance(base, int) and base == 0:
            return x_buf, sa, sb, stats, xn_buf, None
        b = _mo(base, 64)
        return ([r.at[pl.ds(b, S - 64), :] for r in (x_buf, sa, sb, stats)]
                + [xn_buf.at[:, pl.ds(b, 64), :], pl.ds(_mo(base // 2, 32), 32)])

    def xs_form(r0, tok, which="all", base=0):
        xn_v, xs_v = row_views(base)[4:]
        rows = slice(r0 % XN, r0 % XN + 16)

        def inner(sub):
            full = list(enumerate(_sform(*sub))) + [(7, sub[1]), (8, sub[2])]
            return [full[e] for e in {"all": (0, 1, 7, 8, 2, 5, 6, 3, 4), "l1": (0, 1, 7, 8),
                                      "l2": (2, 5, 6, 3, 4)}[which]]
        for ct in range(2):
            def put(k1, k2, v):
                xs_at(k1, k2, xs_v)[r0 // 2:r0 // 2 + 8, ct * 128:(ct + 1) * 128] = v
            yield from form_steps(
                _sform, lambda q, u: xn_v[q, rows, _st(u, ct)],
                put, tok, inner)
        made.add(("xs", r0))

    def ln_rows(r_start, n_rows, tok, which="all", base=0):
        x_v, sa_v, sb_v, st_v, xn_v, _ = row_views(base)
        lane = lax.broadcasted_iota(i32, (8, 128), 1)

        def later(r0):
            form = xs_form(r0, tok, which, base)
            for g in range(8):
                q, o = g // 2, (g % 2) * 8
                t = None
                for ct in range(8):
                    cs = slice(ct * 128, (ct + 1) * 128)
                    v = xn_v[q, r0 % XN + o:r0 % XN + o + 8, _st(ct // 2, ct % 2)] * wrb[:, cs]
                    t = gate(v) if t is None else t + v
                st_v[q * HQ + r0 + o:q * HQ + r0 + o + 8, 128:256] = t
                if tok is not None and TRTOK:
                    tok([t])
                yield
                for _ in range(2 if g < 7 else 0):
                    next(form)
                    yield
            next(form, None)
            made.add(("ln", r0))

        for c in range(n_rows // 16 + 1):
            r0 = r_start + c * 16
            rest = later(r0 - 16) if c > 0 else iter(())
            for g in range(8 if c < n_rows // 16 else 0):
                q, o = g // 2, (g % 2) * 8
                rg = q * HQ + r0 + o
                xv = x_v[rg:rg + 8, :].astype(f32)
                xg = jnp.concatenate([gate(xv[:, 0:128]), xv[:, 128:]], axis=1)
                mf = jnp.sum(xg, axis=1, keepdims=True) * (1.0 / D)
                d = xv - mf
                var = jnp.sum(d * d, axis=1, keepdims=True) * (1.0 / D)
                rs = lax.rsqrt(var + 1e-5)
                xn_v.at[q][r0 % XN + o:r0 % XN + o + 8, :] = _to_st(d * rs)
                rs = jnp.broadcast_to(rs, (8, 128))
                mf = jnp.broadcast_to(mf, (8, 128))
                sa_v[rg:rg + 8, :] = 1.0 + rs
                sb_v[rg:rg + 8, :] = mf * rs
                st_v[rg:rg + 8, 0:128] = jnp.where(lane == 0, mf, jnp.broadcast_to(var, (8, 128)))
                if tok is not None and LNTOK:
                    tok([rs], LNLAG)
                yield
                if g >= LNG and c > 0:
                    for _ in range(3):
                        next(rest)
                        yield
                elif c == 0:
                    for _ in range(LNPAD):
                        yield
            yield from rest

    def wk_prep(c, tok=None):
        cs = pl.ds(_mo(c * 256, 256), 256)
        for i in range(HD // 16):
            r0 = i * 16
            top = wk_buf[r0:r0 + 16, cs].astype(f32)
            bot = wk_buf[HD + r0:HD + r0 + 16, cs].astype(f32)
            ops = _rform(gate(top[:, :128]), top[:, 128:], bot[:, :128], gate(bot[:, 128:]))
            for k in range(7):
                wks.at[c][r0 // 2:r0 // 2 + 8, k * 128:(k + 1) * 128] = _pack(ops[k])
            yield

    def wq_perm(tok):
        def permute(kt):
            for g in range(8):
                tile = gate(pltpu.bitcast(wq_buf[kt * 128:(kt + 1) * 128, g * 128:(g + 1) * 128], u32))
                wqt.at[kt * 8 + g][...] = pltpu.bitcast(_unpack(tile).T, u32)
                yield

        def back(kt):
            for j in range(8):
                tile = gate(jnp.concatenate([wqt[kt * 8 + g, pl.ds(j, 8, stride=8), :] for g in range(8)],
                                            axis=0))
                v = pltpu.bitcast(_unpack(tile).T.astype(f32), u32)
                c0 = (kt // 2) * D + _st(j // 2, j % 2).start
                ps[(kt % 2) * 128:(kt % 2 + 1) * 128, c0:c0 + 128] = v
                made.add(("wqp", kt, j))
                yield

        order = (0, 2, 4, 6, 1, 3, 5, 7)
        for n in range(10):
            if n < 8:
                yield from permute(order[n])
            if n > 1:
                yield from back(order[n - 2])

    def wq_form(tok):
        for i in range(16):
            need(*[("wqp", 2 * r + i // 8, j) for r in range(4) for j in range(8)])
            for ct in range(2):
                def put(k1, k2, v):
                    wqs.at[k1 * 7 + k2][i * 8:(i + 1) * 8, ct * 128:(ct + 1) * 128] = v
                yield from form_steps(
                    _rform, lambda r, c: pltpu.bitcast(
                        ps[i * 16:(i + 1) * 16, r * D + _st(c, ct).start:r * D + _st(c, ct).stop],
                        f32), put, tok)

    def kproj(r0, n, chunks=((0, 0), (0, 1), (1, 0), (1, 1))):
        pr = pl.ds(r0 // 2, n // 2)
        need(*[("xs", r) for r in range(max(r0, 128), r0 + n, 16)])
        for ch, ct in chunks:
            c = 2 * ch + ct
            m = [None] * 7
            for k in K_SEQ:
                e11, e22, e12, e21 = [xs_at(L_ORD[k], e)[pr, :] for e in (0, 1, 7, 8)]
                lhs = jnp.concatenate([jnp.concatenate([e11, e12], axis=1),
                                       jnp.concatenate([e21, e22], axis=1)], axis=0)
                m[k] = mm(_unpack(lhs), wks[c, :, k * 128:(k + 1) * 128], NN, 2 * n)
            kk = [_phi(v) for v in _combine(m)]
            for h in range(2):
                zacc[:, pl.ds(_mo(h * HD + c * 128, 128), 128)] += (
                    (kk[h] + kk[2 + h]).reshape(n // 4, 8, 128).sum(axis=0))
            for s1 in range(4):
                u = (s1 % 2) * 2 + ch
                for h in range(2):
                    pk_buf.at[ct, (s1 // 2) * 2 + h][r0:r0 + n, u * 128:(u + 1) * 128] = (
                        kk[s1][h * n:(h + 1) * n])

    def z_prep():
        z = jnp.sum(zacc[...], axis=0, keepdims=True)
        zt = _pack(jnp.broadcast_to(z, (128, D)).astype(bf16).T)
        for g in range(8):
            tscr.at[g][...] = zt[g * 64:(g + 1) * 64, :]
        for j in range(8):
            blk = jnp.concatenate([tscr[g, pl.ds(j, 8, stride=8), :] for g in range(8)], axis=0)
            zp[:, j * 128:(j + 1) * 128] = _unpack(blk).T[0:8, :].astype(f32)

    def route(tok):
        need(*[("ln", r) for r in range(128, HQ, 16)])
        rows, dots = [], []
        for b in range(S // 128):
            rows.append(gate(stats[b * 128:(b + 1) * 128, 0:128]).T[0:8, :])
            dots.append(jnp.sum(gate(stats[b * 128:(b + 1) * 128, 128:256]).T, axis=0, keepdims=True))
            yield
        mf = jnp.concatenate([v[0:1] for v in rows], axis=0)
        var = jnp.concatenate([v[1:2] for v in rows], axis=0)
        tr = jnp.concatenate(dots, axis=0) * jnp.sqrt(var + 1e-5)
        wsum = jnp.sum(wrb[0:1, :], axis=1, keepdims=True)
        sd = _rbf(jnp.sqrt(_rbf(_rbf(var) + 1e-5)))
        rv = _rbf((tr + (mf - _rbf(mf)) * wsum) / sd)
        rmax = jnp.max(rv)
        pos = (lax.broadcasted_iota(i32, rv.shape, 0) * 128 + lax.broadcasted_iota(i32, rv.shape, 1))
        idx = jnp.min(jnp.where(rv == rmax, pos, S - 1))
        idx_s[0] = idx
        rsel[...] = jnp.full(rsel.shape, rmax, f32)
        b0 = _mo((idx // 16) * 16, 16)
        xn = _rbf(_layernorm_rows(x_buf[pl.ds(b0, 16), :].astype(f32)))
        sel = lax.broadcasted_iota(i32, xn.shape, 0) == idx - b0
        row = jnp.sum(jnp.where(sel, xn, 0.0), axis=0, keepdims=True)
        xbv = jnp.broadcast_to(row, (128, D)).T
        xb[...] = xbv
        yacc[...] = jnp.zeros(yacc.shape, f32)
        tok([xbv[b * 128 + 120:(b + 1) * 128] for b in range(8)])
        yield

    def ps_form(j, tok):
        for c in range(HQ // 16):
            def put(k1, k2, v):
                k = k1 * 7 + k2
                ps[c * 8:(c + 1) * 8, k * 128:(k + 1) * 128] = v
            yield from form_steps(
                _lform, lambda r, q: pk_buf[j, q, c * 16:(c + 1) * 16, r * 128:(r + 1) * 128], put, tok)

    def q_rows(j, r0, n, pq, rc, d0, rec):
        xj = pl.ds(_mo(j * (BQ // 2), BQ // 2), BQ // 2)
        pr = slice(r0 // 2, (r0 + n) // 2)
        blk = yield from strassen2(lambda k1, k2: _unpack(xs_at(L_ORD[k1], L_ORD[k2], xj)[pr, :]),
                                   lambda k1, k2: wqs[k1 * 7 + k2], NN, n, 1, QW)
        lane = lax.broadcasted_iota(i32, (n, 128), 1)
        for q in range(4):
            d = None
            for u in (3, 2, 1, 0):
                v = _phi(blk[q][u])
                for ct in range(2):
                    pq.at[q][d0:d0 + n, _st(u, ct)] = v[:, ct * 128:(ct + 1) * 128]
                t = v * zp[0:1, u * 256:(u + 1) * 256]
                t = t[:, :128] + t[:, 128:]
                d = t if d is None else d + t
            if rec:
                d = recip(d, lane)
            rc.at[q][d0:d0 + n, :] = d

    def recip(d, lane):
        d = d + jnp.where(lane % 2 == 0, pltpu.roll(d, 127, 1), pltpu.roll(d, 1, 1))
        d = d + jnp.where(lane % 4 < 2, pltpu.roll(d, 126, 1), pltpu.roll(d, 2, 1))
        return 1.0 / (d + 1e-6)

    def normalise(pq, rc, nr, dst, p0, raw, tok=None):
        lane = lax.broadcasted_iota(i32, (16, 128), 1)

        def fix(c):
            if c < nr // 16 and raw(c * 16):
                for q in range(4):
                    rq = slice(c * 16, (c + 1) * 16)
                    rc.at[q][rq, :] = recip(gate16(rc[q, rq, :]), lane)

        def scale(c):
            rq = slice(c * 16, (c + 1) * 16)
            fix(c + 1)
            for hf in range(2):
                for q in range(4):
                    cs = slice(hf * HD, (hf + 1) * HD)
                    pq.at[q][rq, cs] = pq[q, rq, cs] * jnp.concatenate([gate16(rc[q, rq, :])] * 4, axis=1)
                    yield

        def form(c):
            rq = slice(c * 16, (c + 1) * 16)
            p2 = pl.ds(_mo(p0 + c * 8, 8), 8)
            for ct in range(2):
                def put(k1, k2, v):
                    dst.at[k1 * 7 + k2][p2, ct * 128:(ct + 1) * 128] = v
                yield from form_steps(_lform, lambda q, u: pq[q, rq, _st(u, ct)], put, tok)

        fix(0)
        if raw(0):
            for _ in range(4):
                yield
        yield from scale(0)
        for c in range(nr // 16):
            nxt = scale(c + 1) if c + 1 < nr // 16 else iter(())
            for i, _ in enumerate(form(c)):
                yield
                if i < 8 and c + 1 < nr // 16:
                    next(nxt)
                    yield
        made.add(("qs", id(dst)))

    hist = []

    def g_lhs(k):
        v = ps[:, k * 128:(k + 1) * 128]
        hist.append(fwd[0])
        if GLAG and len(hist) > GLAG and hist[-1 - GLAG] is not None:
            cur = fwd[0]
            fwd[0] = hist[-1 - GLAG]
            v = jnp.concatenate([gate(v[i * 64:(i + 1) * 64]) for i in range(4)], axis=0)
            fwd[0] = cur
        return _unpack(v)

    def g_kvm(j):
        blk = yield from strassen2(
            lambda k1, k2: g_lhs(k1 * 7 + k2),
            lambda k1, k2: xs_at(R_ORD[k1], R_ORD[k2])[...], TN, 256, 2)
        hm = (lax.broadcasted_iota(i32, (128, 128), 0) // 32
              == lax.broadcasted_iota(i32, (128, 128), 1) // 32)
        qb = q_rows(j, BQ - QB, QB, pqb_buf.at[j], denb_buf.at[j], 0, False)
        for _ in range(QSPLIT):
            next(qb)
        kvps = []
        for a in (3, 2, 1, 0):
            gg = jnp.concatenate(blk[a], axis=1).astype(bf16)
            clock[0] += 256
            kv = jnp.where(hm, _dot(gg, wv_buf[j, :, a * 128:(a + 1) * 128], NN), 0.0)
            tscr2.at[a][...] = _pack(kv)
            kvps.append(_unpack(jnp.concatenate(
                [tscr2[a, pl.ds(jj, 8, stride=8), :] for jj in range(8)], axis=0)))
        mg = mg_buf

        def m_form(tok):
            for a in (3, 2, 1, 0):
                need(("mg", a))
                for jl in range(2):
                    for ct in range(2):
                        def put(k1, k2, v):
                            ms.at[k1 * 7 + k2][pl.ds(_mo(jl * 64 + (2 * a + j) * 8, 8), 8),
                                               ct * 128:(ct + 1) * 128] = v
                        yield from form_steps(
                            _rform, lambda q, u: mg[a, (2 * q + jl) * 16:(2 * q + jl + 1) * 16, _st(u, ct)], put)

        for i, a in enumerate((3, 2, 1, 0)):
            wo_u = pltpu.bitcast(wo_buf[j, a * 128:(a + 1) * 128, :], u32)
            res = mm(kvps[i], wo_u, NN, 256)
            mg.at[a][...] = _to_st(res)
            made.add(("mg", a))
            if i == 0:
                add_side(m_form, 112, 128, 768 + (49 - QSPLIT) * QB - 100)
        for _ in qb:
            pass

    def out_part(p0, nr, y, src, pr0):
        pr = pl.ds(_mo(pr0, 8), nr // 2)
        rows = [pl.ds(_mo(q * HQ + p0, 16), nr) for q in range(4)]
        row = lax.broadcasted_iota(i32, (nr, 256), 0) + p0
        blk = yield from strassen2(lambda k1, k2: _unpack(src[k1 * 7 + k2, pr, :]),
                                   lambda k1, k2: ms[k1 * 7 + k2], NN, nr)
        for s1 in (3, 2, 1, 0):
            for s2 in range(4):
                q = (s1 // 2) * 2 + s2 // 2
                u = (s1 % 2) * 2 + s2 % 2
                rr, cc = rows[q], pl.ds(u * 256, 256)
                a = jnp.concatenate([sa[rr, :]] * 2, axis=1)
                b = jnp.concatenate([sb[rr, :]] * 2, axis=1)
                o = blk[q][u] + jnp.where(row + q * HQ == idx_s[0], y[:, u * 256:(u + 1) * 256], 0.0)
                out_buf[rr, cc] = (x_buf[rr, cc].astype(f32) * a - b + o).astype(bf16)
                if s2 % 2 == 1:
                    ch = pl.ds((s1 % 2) * HD, HD)
                    cp(out_buf.at[rr, ch], out_hbm.at[0, rr, ch], SEM_O).start()

    def ffn_part(j, f_lo, f_hi):
        for f0 in range(f_lo, f_hi, 256):
            fs = slice(f0, f0 + 256)
            ag = jnp.zeros((8, 256), f32)
            au = jnp.zeros((8, 256), f32)
            for kg in range(D // 8):
                xv = jnp.concatenate([gate(xb[8 * kg:8 * kg + 8, :])] * 2, axis=1)
                ag = ag + wg_buf[j, 8 * kg:8 * kg + 8, fs].astype(f32) * xv
                au = au + wu_buf[j, 8 * kg:8 * kg + 8, fs].astype(f32) * xv
                if kg % FSTEP == FSTEP - 1:
                    yield
            g = _rbf(jnp.sum(ag, axis=0, keepdims=True))
            u = _rbf(jnp.sum(au, axis=0, keepdims=True))
            h = _rbf(_rbf(g * jax.nn.sigmoid(g)) * u)
            hb_buf[fs, :] = jnp.broadcast_to(h, (128, 256)).T
        for d0 in range(0, D, 512):
            ds_ = slice(d0, d0 + 512)
            acc = yacc[:, ds_]
            for kg in range(f_lo // 8, f_hi // 8):
                hv = jnp.concatenate([gate(hb_buf[8 * kg:8 * kg + 8, :])] * 4, axis=1)
                acc = acc + wd_buf[j, 8 * kg:8 * kg + 8, ds_].astype(f32) * hv
                if kg % FSTEP == FSTEP - 1:
                    yield
            yacc[:, ds_] = acc

    def wait_group(i):
        with _scope("a_wait%d" % i):
            for c in a_groups[i]:
                c.wait()

    def run_all(gen):
        for _ in gen:
            pass

    def ln_side(r0, n, t0, t1):
        add_side(lambda tok: ln_rows(r0, n, tok), 30 * n // 16 + 8 * LNPAD, t0, t1, SLAG)

    def l2_side(base, n, t0, t1):
        def gen(tok):
            for r in range(0, n, 16):
                yield from xs_form(r, tok, "l2", base)
        add_side(gen, 14 * n // 16, t0, t1)

    a_groups = make_a_groups()
    with _scope("p0_issue"):
        cp_wr.start()
        for grp in a_groups:
            for c in grp:
                c.start()
        for j in range(2):
            for part in range(2):
                for c in cp_b(j, part):
                    c.start()
        zacc[...] = jnp.zeros(zacc.shape, f32)
        zero_buf[1] = jnp.zeros((8, 128), u32)
        cp_zero = cp(zero_buf.at[1], zero_buf.at[0], SEM_Z)
        cp_zero.start()
        cp_zero.wait()
        cp_wr.wait()
        wrb[...] = jnp.broadcast_to(wr_buf[0:D].reshape(1, D).astype(f32), (8, D))
        z0 = jnp.max(pltpu.bitcast(zero_buf[0], i32))
        ps, pq_buf, den_buf, mg_buf, hb_buf = [r.at[z0] for r in (ps_raw, pq_raw, den_raw, mg_raw, hb_raw)]
        xn_buf = mg_buf

    def a01(i, carry):
        with _scope("a_wait01"):
            for c in cp_x(i * 64, 64, SEM_A + i):
                c.wait()
        with _scope("a01"):
            run_all(ln_rows(0, 64, None, "l1", i * 64))
        return carry

    lax.fori_loop(0, 2, a01, 0)

    def a23(i, carry):
        with _scope("a_wait23"):
            for c in cp_wk(i, SEM_A + 2 + i):
                c.wait()
        with _scope("a23"):
            run_all(wk_prep(i))
            l2_side(i * 64, 64, 300, 1500)
            kproj(0, 128, [(0, i)])
            finish()
        return carry

    lax.fori_loop(0, 2, a23, 0)
    wait_group(4)
    with _scope("a4"):
        run_all(wk_prep(2))
        ln_side(128, A4N, 0, 1500)
        kproj(0, 128, [(1, 0)])
        finish()
    wait_group(5)
    with _scope("a5"):
        run_all(wk_prep(3))
        if A5 == 0:
            ln_side(160, 32, 0, 1400)
            kproj(0, 128, [(1, 1)])
            for r0 in (128, 192):
                ln_side(r0 + 64, 64, 0, 3200)
                kproj(r0, 64)
        else:
            ln_side(128 + A4N, 192 - A4N, 0, A5)
            kproj(0, 128, [(1, 1)])
            for r0, n in A5K:
                kproj(r0, n)
        finish()
    wait_group(6)
    with _scope("a6"):
        ln_side(320, 192, 0, A6[0])
        add_side(wq_perm, 128, A6[1], A6[2], A6[6])
        add_side(wq_form, 224, A6[3], A6[4], A6[6])
        add_side(route, 17, A6[5], A6[5] + 800)
        for r0 in (256, 320, 384, 448):
            kproj(r0, 64)
        finish()

    def b_body(j, carry):
        qa = BQ - QB
        with _scope("b_wait0"):
            for c in cp_b(j, 0, wait_only=True):
                c.wait()
        with _scope("b_r0"):
            z_prep()
            t1 = 49 * qa - 400
            add_side(lambda tok: ps_form(j, None), 7 * HQ // 16, 0, t1)
            add_side(lambda tok: ffn_part(j, 0, F1), F1 * 3 // (4 * FSTEP), 0, t1)
            for r0 in range(0, qa, QN):
                run_all(q_rows(j, r0, min(QN, qa - r0), pq_buf, den_buf, r0, r0 + QN < qa))
            finish()
        with _scope("b_wait1"):
            for c in cp_b(j, 1, wait_only=True):
                c.wait()
        with _scope("b_r1"):
            add_side(lambda tok: ffn_part(j, F1, FH), (FH - F1) * 3 // (4 * FSTEP), 0, 12800)
            add_side(lambda tok: normalise(pq_buf, den_buf, qa, qs, j * (qa // 2),
                                           lambda r: (r // QN + 1) * QN >= qa), 22 * (qa // 16), 0, 12800)
            run_all(g_kvm(j))
            finish()
        return carry

    lax.fori_loop(0, 2, b_body, 0)

    def c_body(t, carry):
        with _scope("c_body"):
            y = _rbf(jnp.sum(yacc[...], axis=0, keepdims=True))
            y = _rbf(y * _rbf(jax.nn.sigmoid(rsel[0:1, :])))
            j, h = t >> 1, t & 1
            na, nb = (BQ - QB) // 2, QB // 2
            hb = pl.ds(_mo(h * nb, 16), nb)
            add_side(lambda tok: normalise(pqb_buf.at[j, :, hb, :], denb_buf.at[j, :, hb, :], nb, qsb, 0,
                                           lambda r: True, tok),
                     4 + 22 * (nb // 16), 0, 49 * na - 800, SLAG)
            for p in range(0, na, CR):
                p0 = j * BQ + h * na + p
                run_all(out_part(p0, min(CR, na - p), y, qs, t * (na // 2) + p // 2))
            advance(clock[0] + 10 ** 6)
            flush()
            run_all(out_part(j * BQ + BQ - QB + h * nb, nb, y, qsb, 0))
            finish()
        return carry

    lax.fori_loop(0, 4, c_body, 0)
    with _scope("tail"):
        cp(out_buf, out_hbm.at[0], SEM_O).wait()


@jax.jit
def pallas_parallel_sum__linear_attn_block__moe_arch_mod__prompt_kernel(
    A_x: jax.Array,
    A_wqkv: jax.Array,
    A_wo: jax.Array,
    B_x: jax.Array,
    B_w_r: jax.Array,
    B_w_gate: jax.Array,
    B_w_up: jax.Array,
    B_w_down: jax.Array,
):
    del B_x
    V = pltpu.VMEM
    scratch = [
        V((S, D), bf16),
        V((2, D, 512), bf16),
        V((2, 512, D), bf16),
        V((8 * D,), bf16),
        V((2, D, FH), bf16),
        V((2, D, FH), bf16),
        V((2, FH, D), bf16),
        V((28, HQ // 2, 256), u32),
        V((35, HQ // 2, 256), u32),
        V((49, 128, 256), u32),
        V((S, 128), f32),
        V((S, 128), f32),
        V((8, D), f32),
        V((8, D), f32),
        V((2, 4, HQ, 512), f32),
        V((D, 128), f32),
        V((8, D), f32),
        V((8, D), f32),
        V((8, D), f32),
        V((4, 8, 128), u32),
        V((4, HD // 2, 7 * 128), u32),
        V((S, 256), f32),
        V((64, 64, 128), u32),
        V((1, HQ // 2, 49 * 128), u32),
        V((49, BQ - QB, 256), u32),
        V((49, 128, 256), u32),
        V((8, 64, 128), u32),
        V((4, 64, 128), u32),
        V((1, 4, BQ - QB, D), f32),
        V((1, 4, BQ - QB, 128), f32),
        V((2, 4, QB, D), f32),
        V((2, 4, QB, 128), f32),
        V((49, QB // 4, 256), u32),
        V((1, 4, 128, D), f32),
        V((1, FH, 128), f32),
        V((S, D), bf16),
        pltpu.SMEM((1,), i32),
        pltpu.SemaphoreType.DMA((13,)),
    ]
    return pl.pallas_call(
        _kernel,
        out_shape=jax.ShapeDtypeStruct((1, S, D), bf16),
        in_specs=[pl.BlockSpec(memory_space=pl.ANY)] * 7,
        out_specs=pl.BlockSpec(memory_space=pl.ANY),
        scratch_shapes=scratch,
        compiler_params=pltpu.CompilerParams(vmem_limit_bytes=VMEM_MB * 1024 * 1024,
                                             disable_bounds_checks=True,
                                             fuse_transposed_lhs_in_matmul=FUSE,
                                             disable_semaphore_checks=True),
    )(A_x, A_wqkv, A_wo, B_w_r, B_w_gate, B_w_up, B_w_down)
```

```python
import contextlib

import jax
import jax.numpy as jnp
from jax import lax
import jax.experimental.pallas as pl
import jax.experimental.pallas.tpu as pltpu

bf16, f32, u32, i32 = jnp.bfloat16, jnp.float32, jnp.uint32, jnp.int32

S = 2048
D = 1024
F = 3584
HP = S // 2
HD = D // 2
HQ = S // 4
BQ = HQ // 2
FH = F // 2
F1 = 0
QB = 64
QN = 48
QW = (28, 36, 36, 6, 2, 2, 2)
A6 = (8500, 8000, 10800, 9800, 13900, 11300, None)
TOKEV = 2
TRTOK = 1
LNPAD = 2
A5 = 8500
A4N = 32
A5K = ((128, 32), (160, 48), (208, 48))
LNTOK = 1
LNLAG = 300
LNG = 1
R1T = (12800, 12800)
GW = (16,) * 7
GLAG = 0
RECQ = True
FUSE = False
QSPLIT = 6
SLAG = 400
FSTEP = 2
CR = 32
XN = 128
VMEM_MB = 120
CT = 128

L_ORD = (2, 3, 0, 1, 4, 5, 6)
R_ORD = (2, 0, 6, 5, 1, 4, 3)

K_SEQ = (1, 4, 0, 2, 3, 5, 6)
K_SEQ2 = (0, 1, 2, 5, 3, 4, 6)

NN = (((1,), (0,)), ((), ()))
NT_ = (((1,), (1,)), ((), ()))
TN = (((0,), (0,)), ((), ()))


SCOPES = False


def _scope(name):
    return jax.named_scope(name) if SCOPES else contextlib.nullcontext()


def _mo(v, m):
    return v if isinstance(v, int) else pl.multiple_of(v, m)


def _dot(a, b, dims):
    return lax.dot_general(a, b, dims, preferred_element_type=f32)


def _pack(v):
    return pltpu.bitcast(v.astype(bf16), u32)


def _unpack(v):
    return pltpu.bitcast(v, bf16)


def _combine(m):
    m1, m2, m3, m4, m5, m6, m7 = m
    return m1 + m4 - m5 + m7, m3 + m5, m2 + m4, m1 - m2 + m3 + m6


def _lform(a11, a12, a21, a22):
    return (a11 + a22, a21 + a22, a11, a22, a11 + a12, a21 - a11, a12 - a22)


def _rform(b11, b12, b21, b22):
    return (b11 + b22, b11, b12 - b22, b21 - b11, b22, b11 + b12, b21 + b22)


def _sform(x11, x12, x21, x22):
    return (x11, x22, x11 + x22, x21 + x22, x11 + x12, x21 - x11, x12 - x22)


class _Sym:
    def __init__(self, t):
        self.t = t

    def __add__(self, o):
        return _Sym({**self.t, **o.t})

    def __sub__(self, o):
        return _Sym({**self.t, **{k: -v for k, v in o.t.items()}})


def _st(u, ct):
    return slice((4 * ct + u) * 128, (4 * ct + u + 1) * 128)


def _to_st(v):
    return jnp.concatenate([v[:, (2 * u + ct) * 128:(2 * u + ct + 1) * 128]
                            for ct in range(2) for u in range(4)], axis=1)


def _phi(t):
    return jnp.where(t > 0, t + 1.0, jnp.exp(t)) + 1e-6


def _rbf(v):
    return v.astype(bf16).astype(f32)


def _layernorm_rows(xv):
    mf = jnp.sum(xv, axis=1, keepdims=True) * (1.0 / D)
    mb = _rbf(mf)
    d = xv - mb
    dm = mf - mb
    var = jnp.sum(d * d, axis=1, keepdims=True) * (1.0 / D) - dm * dm
    var = jnp.maximum(var, 0.0)
    sd = _rbf(jnp.sqrt(_rbf(_rbf(var) + 1e-5)))
    return d * (1.0 / sd)


def _kernel(x_hbm, wqkv_hbm, wo_hbm, wr_hbm, wg_hbm, wu_hbm, wd_hbm, out_hbm,
            x_buf, wv_buf, wo_buf, wr_buf, wg_buf, wu_buf, wd_buf,
            xs1, xs2, wqs, sa, sb, zacc, zp, pk_buf, xb, yacc, rsel, wrb, zero_buf,
            wks, stats, wqt, ps_raw, qs, ms, tscr, tscr2, pq_raw, den_raw, pqb_buf, denb_buf, qsb,
            mg_raw, hb_raw, out_buf, idx_s, sem):
    wq_buf = out_buf.at[pl.ds(0, D), :]
    wk_buf = out_buf.at[pl.ds(D, D), :]

    def xs_at(k1, e, rows=None):
        r = xs1.at[k1 * 4 + (0, 1, 7, 8).index(e)] if e in (0, 1, 7, 8) else xs2.at[k1 * 5 + e - 2]
        return r if rows is None else r.at[rows, :]

    SEM_B, SEM_O, SEM_Z, SEM_A = 0, 4, 5, 6

    def cp(src, dst, s):
        return pltpu.make_async_copy(src, dst, sem.at[s])

    def cp_x(r0, n, s):
        rows = [pl.ds(_mo(q * HQ + r0, 16), n) for q in range(4)]
        return [cp(x_hbm.at[0, r, :], x_buf.at[r, :], s) for r in rows]

    def cp_wk(c, s):
        return [cp(wqkv_hbm.at[:, pl.ds(_mo(D + h * HD + c * 128, 128), 128)],
                   wk_buf.at[:, pl.ds(_mo(c * 256 + h * 128, 128), 128)], s) for h in range(2)]

    cp_wr = cp(wr_hbm, wr_buf.at[pl.ds(0, D)], SEM_Z)

    def make_a_groups():
        return [
            cp_x(0, 64, SEM_A),
            cp_x(64, 64, SEM_A + 1),
            cp_wk(0, SEM_A + 2),
            cp_wk(1, SEM_A + 3),
            cp_wk(2, SEM_A + 4) + cp_x(128, 64, SEM_A + 4),
            cp_wk(3, SEM_A + 5) + cp_x(192, 128, SEM_A + 5),
            cp_x(320, 192, SEM_A + 6) + [cp(wqkv_hbm.at[:, pl.ds(0, D)], wq_buf, SEM_A + 6)],
        ]

    def cp_b(j, part, wait_only=False):
        pairs = []
        f0, fw = (0, F1) if part == 0 else (F1, FH - F1)
        fs = pl.ds(_mo(j * FH + f0, 128), fw)
        if fw:
          pairs += [(wg_hbm.at[:, fs], wg_buf.at[j, :, pl.ds(f0, fw)]),
                  (wu_hbm.at[:, fs], wu_buf.at[j, :, pl.ds(f0, fw)]),
                  (wd_hbm.at[fs, :], wd_buf.at[j, pl.ds(f0, fw), :])]
        if part == 1:
            for a in range(4):
                c0 = _mo((2 * a + j) * 128, 128)
                pairs += [(wqkv_hbm.at[:, pl.ds(2 * D + c0, 128)], wv_buf.at[j, :, pl.ds(a * 128, 128)]),
                          (wo_hbm.at[pl.ds(c0, 128), :], wo_buf.at[j, pl.ds(a * 128, 128), :])]
        return [cp(dst if wait_only else src, dst, SEM_B + 2 * j + part) for src, dst in pairs]

    clock = [0]
    toks = []
    sides = []
    fwd = [None]

    def emit_tok(vals, stamp=None):
        t = None
        for v in vals:
            v = pltpu.bitcast(v, u32) if v.dtype != u32 else v
            t = v if t is None else t | v
        toks.append((clock[0] if stamp is None else stamp, t & zero_buf[0]))

    def gate(v):
        if fwd[0] is None:
            return v
        if fwd[0][1] is None:
            fwd[0][1] = pltpu.bitcast(fwd[0][0](), u32) & zero_buf[0]
        head = pltpu.bitcast(pltpu.bitcast(v[0:8], u32) | fwd[0][1], v.dtype)
        return head if v.shape[0] == 8 else jnp.concatenate([head, v[8:]], axis=0)

    def add_side(gen_fn, n, t0, t1, lag=None):
        st = {"i": 0, "n": n, "t0": clock[0] + t0, "t1": clock[0] + t1}

        def tok(vals, extra=0):
            if lag is not None:
                emit_tok(vals, st["t0"] + (st["i"] + 1) * (st["t1"] - st["t0"]) // st["n"] + lag + extra)
        st["g"] = gen_fn(tok)
        sides.append(st)

    def advance(until):
        for st in sides:
            while st["i"] < st["n"] and st["t0"] + st["i"] * (st["t1"] - st["t0"]) // st["n"] < until:
                next(st["g"], None)
                st["i"] += 1
                if st["i"] == st["n"]:
                    for _ in st["g"]:
                        pass

    def flush():
        for st in sides:
            for _ in st["g"]:
                pass
        sides.clear()

    def finish():
        flush()
        toks.clear()
        fwd[0] = None

    def mm(lhs, rhs, dims, cycles, nseg=1):
        due = [t for (c, t) in toks if c <= clock[0]]
        toks[:] = [(c, t) for (c, t) in toks if c > clock[0]]
        if due:
            head = rhs[0:8, 0:128]
            for t in due:
                head = head | t
            if rhs.shape[1] > 128:
                head = jnp.concatenate([head, rhs[0:8, 128:]], axis=1)
            rhs = jnp.concatenate([head, rhs[8:]], axis=0)
        res = _dot(lhs, _unpack(rhs), dims)
        ngr = res.shape[0] // 16
        for sg in range(nseg):
            for i in range(ngr):
                fwd[0] = [lambda sg=sg, i=i: res[i * 16:i * 16 + 8, sg * 128:(sg + 1) * 128], None]
                clock[0] += cycles // nseg // ngr
                advance(clock[0])
        return res

    def gate16(v):
        return jnp.concatenate([gate(v[0:8]), gate(v[8:16])], axis=0)

    def form_steps(form, get, put, tok=None, inner=None, gated=False):
        terms = form(*[_Sym({i: 1}) for i in range(4)])
        for k1 in range(7):
            sub = []
            for r in range(2):
                for c in range(2):
                    v = None
                    for i, sg in sorted(terms[k1].t.items(), key=lambda e: -e[1]):
                        b = get(r + 2 * (i // 2), c + 2 * (i % 2))
                        if v is None:
                            v = gate16(b) if r == c and not gated else b
                        else:
                            v = v + b if sg > 0 else v - b
                    sub.append(v)
            vals = []
            for k2, v in (enumerate(form(*sub)) if inner is None else inner(sub)):
                vals.append(v)
                put(k1, k2, _pack(v))
            if tok is not None and k1 % TOKEV == TOKEV - 1 - (6 % TOKEV != TOKEV - 1):
                tok([v[o:o + 8] for v in vals[-2:] for o in (0, 8)])
            yield

    def strassen2(lhs, rhs, dims, cycles, nseg=1, wts=(16,) * 7):
        m1 = [None] * 7
        for i1, k1 in enumerate(K_SEQ2):
            m2 = [None] * 7
            for k2 in K_SEQ2:
                m2[k2] = mm(lhs(k1, k2), rhs(k1, k2), dims, cycles * wts[i1] // 16, nseg)
                yield
            m1[k1] = _combine(m2)
        out = [[None] * 4 for _ in range(4)]
        for s2 in range(4):
            for s1, v in enumerate(_combine([m1[k1][s2] for k1 in range(7)])):
                out[(s1 // 2) * 2 + s2 // 2][(s1 % 2) * 2 + s2 % 2] = v
        return out

    made = set()

    def need(*keys):
        assert all(k in made for k in keys), keys

    def row_views(base):
        if isinstance(base, int) and base == 0:
            return x_buf, sa, sb, stats, xn_buf, None
        b = _mo(base, 64)
        return ([r.at[pl.ds(b, S - 64), :] for r in (x_buf, sa, sb, stats)]
                + [xn_buf.at[:, pl.ds(b, 64), :], pl.ds(_mo(base // 2, 32), 32)])

    def xs_form(r0, tok, which="all", base=0):
        xn_v, xs_v = row_views(base)[4:]
        rows = slice(r0 % XN, r0 % XN + 16)

        def inner(sub):
            full = list(enumerate(_sform(*sub))) + [(7, sub[1]), (8, sub[2])]
            return [full[e] for e in {"all": (0, 1, 7, 8, 2, 5, 6, 3, 4), "l1": (0, 1, 7, 8),
                                      "l2": (2, 5, 6, 3, 4)}[which]]
        for ct in range(2):
            def put(k1, k2, v):
                xs_at(k1, k2, xs_v)[r0 // 2:r0 // 2 + 8, ct * 128:(ct + 1) * 128] = v
            yield from form_steps(
                _sform, lambda q, u: xn_v[q, rows, _st(u, ct)],
                put, tok, inner)
        made.add(("xs", r0))

    def ln_rows(r_start, n_rows, tok, which="all", base=0):
        x_v, sa_v, sb_v, st_v, xn_v, _ = row_views(base)
        lane = lax.broadcasted_iota(i32, (8, 128), 1)

        def later(r0):
            form = xs_form(r0, tok, which, base)
            for g in range(8):
                q, o = g // 2, (g % 2) * 8
                t = None
                for ct in range(8):
                    cs = slice(ct * 128, (ct + 1) * 128)
                    v = xn_v[q, r0 % XN + o:r0 % XN + o + 8, _st(ct // 2, ct % 2)] * wrb[:, cs]
                    t = gate(v) if t is None else t + v
                st_v[q * HQ + r0 + o:q * HQ + r0 + o + 8, 128:256] = t
                if tok is not None and TRTOK:
                    tok([t])
                yield
                for _ in range(2 if g < 7 else 0):
                    next(form)
                    yield
            next(form, None)
            made.add(("ln", r0))

        for c in range(n_rows // 16 + 1):
            r0 = r_start + c * 16
            rest = later(r0 - 16) if c > 0 else iter(())
            for g in range(8 if c < n_rows // 16 else 0):
                q, o = g // 2, (g % 2) * 8
                rg = q * HQ + r0 + o
                xv = x_v[rg:rg + 8, :].astype(f32)
                xg = jnp.concatenate([gate(xv[:, 0:128]), xv[:, 128:]], axis=1)
                mf = jnp.sum(xg, axis=1, keepdims=True) * (1.0 / D)
                d = xv - mf
                var = jnp.sum(d * d, axis=1, keepdims=True) * (1.0 / D)
                rs = lax.rsqrt(var + 1e-5)
                xn_v.at[q][r0 % XN + o:r0 % XN + o + 8, :] = _to_st(d * rs)
                rs = jnp.broadcast_to(rs, (8, 128))
                mf = jnp.broadcast_to(mf, (8, 128))
                sa_v[rg:rg + 8, :] = 1.0 + rs
                sb_v[rg:rg + 8, :] = mf * rs
                st_v[rg:rg + 8, 0:128] = jnp.where(lane == 0, mf, jnp.broadcast_to(var, (8, 128)))
                if tok is not None and LNTOK:
                    tok([rs], LNLAG)
                yield
                if g >= LNG and c > 0:
                    for _ in range(3):
                        next(rest)
                        yield
                elif c == 0:
                    for _ in range(LNPAD):
                        yield
            yield from rest

    def wk_prep(c, tok=None):
        cs = pl.ds(_mo(c * 256, 256), 256)
        for i in range(HD // 16):
            r0 = i * 16
            top = wk_buf[r0:r0 + 16, cs].astype(f32)
            bot = wk_buf[HD + r0:HD + r0 + 16, cs].astype(f32)
            ops = _rform(gate(top[:, :128]), top[:, 128:], bot[:, :128], gate(bot[:, 128:]))
            for k in range(7):
                wks.at[c][r0 // 2:r0 // 2 + 8, k * 128:(k + 1) * 128] = _pack(ops[k])
            yield

    def wq_perm(tok):
        def permute(kt):
            for g in range(8):
                tile = gate(pltpu.bitcast(wq_buf[kt * 128:(kt + 1) * 128, g * 128:(g + 1) * 128], u32))
                wqt.at[kt * 8 + g][...] = pltpu.bitcast(_unpack(tile).T, u32)
                yield

        def back(kt):
            for j in range(8):
                tile = gate(jnp.concatenate([wqt[kt * 8 + g, pl.ds(j, 8, stride=8), :] for g in range(8)],
                                            axis=0))
                v = pltpu.bitcast(_unpack(tile).T.astype(f32), u32)
                c0 = (kt // 2) * D + _st(j // 2, j % 2).start
                ps[(kt % 2) * 128:(kt % 2 + 1) * 128, c0:c0 + 128] = v
                made.add(("wqp", kt, j))
                yield

        order = (0, 2, 4, 6, 1, 3, 5, 7)
        for n in range(10):
            if n < 8:
                yield from permute(order[n])
            if n > 1:
                yield from back(order[n - 2])

    def wq_form(tok):
        for i in range(16):
            need(*[("wqp", 2 * r + i // 8, j) for r in range(4) for j in range(8)])
            for ct in range(2):
                def put(k1, k2, v):
                    wqs.at[k1 * 7 + k2][i * 8:(i + 1) * 8, ct * 128:(ct + 1) * 128] = v
                yield from form_steps(
                    _rform, lambda r, c: pltpu.bitcast(
                        ps[i * 16:(i + 1) * 16, r * D + _st(c, ct).start:r * D + _st(c, ct).stop],
                        f32), put, tok)

    def kproj(r0, n, chunks=((0, 0), (0, 1), (1, 0), (1, 1))):
        pr = pl.ds(r0 // 2, n // 2)
        need(*[("xs", r) for r in range(max(r0, 128), r0 + n, 16)])
        for ch, ct in chunks:
            c = 2 * ch + ct
            m = [None] * 7
            for k in K_SEQ:
                e11, e22, e12, e21 = [xs_at(L_ORD[k], e)[pr, :] for e in (0, 1, 7, 8)]
                lhs = jnp.concatenate([jnp.concatenate([e11, e12], axis=1),
                                       jnp.concatenate([e21, e22], axis=1)], axis=0)
                m[k] = mm(_unpack(lhs), wks[c, :, k * 128:(k + 1) * 128], NN, 2 * n)
            kk = [_phi(v) for v in _combine(m)]
            for h in range(2):
                zacc[:, pl.ds(_mo(h * HD + c * 128, 128), 128)] += (
                    (kk[h] + kk[2 + h]).reshape(n // 4, 8, 128).sum(axis=0))
            for s1 in range(4):
                u = (s1 % 2) * 2 + ch
                for h in range(2):
                    pk_buf.at[ct, (s1 // 2) * 2 + h][r0:r0 + n, u * 128:(u + 1) * 128] = (
                        kk[s1][h * n:(h + 1) * n])

    def z_prep():
        z = jnp.sum(zacc[...], axis=0, keepdims=True)
        zt = _pack(jnp.broadcast_to(z, (128, D)).astype(bf16).T)
        for g in range(8):
            tscr.at[g][...] = zt[g * 64:(g + 1) * 64, :]
        for j in range(8):
            blk = jnp.concatenate([tscr[g, pl.ds(j, 8, stride=8), :] for g in range(8)], axis=0)
            zp[:, j * 128:(j + 1) * 128] = _unpack(blk).T[0:8, :].astype(f32)

    def route(tok):
        need(*[("ln", r) for r in range(128, HQ, 16)])
        rows, dots = [], []
        for b in range(S // 128):
            rows.append(gate(stats[b * 128:(b + 1) * 128, 0:128]).T[0:8, :])
            dots.append(jnp.sum(gate(stats[b * 128:(b + 1) * 128, 128:256]).T, axis=0, keepdims=True))
            yield
        mf = jnp.concatenate([v[0:1] for v in rows], axis=0)
        var = jnp.concatenate([v[1:2] for v in rows], axis=0)
        tr = jnp.concatenate(dots, axis=0) * jnp.sqrt(var + 1e-5)
        wsum = jnp.sum(wrb[0:1, :], axis=1, keepdims=True)
        sd = _rbf(jnp.sqrt(_rbf(_rbf(var) + 1e-5)))
        rv = _rbf((tr + (mf - _rbf(mf)) * wsum) / sd)
        rmax = jnp.max(rv)
        pos = (lax.broadcasted_iota(i32, rv.shape, 0) * 128 + lax.broadcasted_iota(i32, rv.shape, 1))
        idx = jnp.min(jnp.where(rv == rmax, pos, S - 1))
        idx_s[0] = idx
        rsel[...] = jnp.full(rsel.shape, rmax, f32)
        b0 = _mo((idx // 16) * 16, 16)
        xn = _rbf(_layernorm_rows(x_buf[pl.ds(b0, 16), :].astype(f32)))
        sel = lax.broadcasted_iota(i32, xn.shape, 0) == idx - b0
        row = jnp.sum(jnp.where(sel, xn, 0.0), axis=0, keepdims=True)
        xbv = jnp.broadcast_to(row, (128, D)).T
        xb[...] = xbv
        yacc[...] = jnp.zeros(yacc.shape, f32)
        tok([xbv[b * 128 + 120:(b + 1) * 128] for b in range(8)])
        yield

    def ps_form(j, tok):
        for c in range(HQ // 16):
            def put(k1, k2, v):
                k = k1 * 7 + k2
                ps[c * 8:(c + 1) * 8, k * 128:(k + 1) * 128] = v
            yield from form_steps(
                _lform, lambda r, q: pk_buf[j, q, c * 16:(c + 1) * 16, r * 128:(r + 1) * 128], put, tok)

    def q_rows(j, r0, n, pq, rc, d0, rec):
        xj = pl.ds(_mo(j * (BQ // 2), BQ // 2), BQ // 2)
        pr = slice(r0 // 2, (r0 + n) // 2)
        blk = yield from strassen2(lambda k1, k2: _unpack(xs_at(L_ORD[k1], L_ORD[k2], xj)[pr, :]),
                                   lambda k1, k2: wqs[k1 * 7 + k2], NN, n, 1, QW)
        lane = lax.broadcasted_iota(i32, (n, 128), 1)
        for q in range(4):
            d = None
            for u in (3, 2, 1, 0):
                v = _phi(blk[q][u])
                for ct in range(2):
                    pq.at[q][d0:d0 + n, _st(u, ct)] = v[:, ct * 128:(ct + 1) * 128]
                t = v * zp[0:1, u * 256:(u + 1) * 256]
                t = t[:, :128] + t[:, 128:]
                d = t if d is None else d + t
            if rec:
                d = recip(d, lane)
            rc.at[q][d0:d0 + n, :] = d

    def recip(d, lane):
        d = d + jnp.where(lane % 2 == 0, pltpu.roll(d, 127, 1), pltpu.roll(d, 1, 1))
        d = d + jnp.where(lane % 4 < 2, pltpu.roll(d, 126, 1), pltpu.roll(d, 2, 1))
        return 1.0 / (d + 1e-6)

    def normalise(pq, rc, nr, dst, p0, raw, tok=None):
        lane = lax.broadcasted_iota(i32, (16, 128), 1)

        def fix(c):
            if c < nr // 16 and raw(c * 16):
                for q in range(4):
                    rq = slice(c * 16, (c + 1) * 16)
                    rc.at[q][rq, :] = recip(gate16(rc[q, rq, :]), lane)

        def scale(c):
            rq = slice(c * 16, (c + 1) * 16)
            fix(c + 1)
            for hf in range(2):
                for q in range(4):
                    cs = slice(hf * HD, (hf + 1) * HD)
                    pq.at[q][rq, cs] = pq[q, rq, cs] * jnp.concatenate([gate16(rc[q, rq, :])] * 4, axis=1)
                    yield

        def form(c):
            rq = slice(c * 16, (c + 1) * 16)
            p2 = pl.ds(_mo(p0 + c * 8, 8), 8)
            for ct in range(2):
                def put(k1, k2, v):
                    dst.at[k1 * 7 + k2][p2, ct * 128:(ct + 1) * 128] = v
                yield from form_steps(_lform, lambda q, u: pq[q, rq, _st(u, ct)], put, tok)

        fix(0)
        if raw(0):
            for _ in range(4):
                yield
        yield from scale(0)
        for c in range(nr // 16):
            nxt = scale(c + 1) if c + 1 < nr // 16 else iter(())
            for i, _ in enumerate(form(c)):
                yield
                if i < 8 and c + 1 < nr // 16:
                    next(nxt)
                    yield
        made.add(("qs", id(dst)))

    hist = []

    def g_lhs(k):
        v = ps[:, k * 128:(k + 1) * 128]
        hist.append(fwd[0])
        if GLAG and len(hist) > GLAG and hist[-1 - GLAG] is not None:
            cur = fwd[0]
            fwd[0] = hist[-1 - GLAG]
            v = jnp.concatenate([gate(v[i * 64:(i + 1) * 64]) for i in range(4)], axis=0)
            fwd[0] = cur
        return _unpack(v)

    def g_kvm(j):
        blk = yield from strassen2(
            lambda k1, k2: g_lhs(k1 * 7 + k2),
            lambda k1, k2: xs_at(R_ORD[k1], R_ORD[k2])[...], TN, 256, 2, GW)
        hm = (lax.broadcasted_iota(i32, (128, 128), 0) // 32
              == lax.broadcasted_iota(i32, (128, 128), 1) // 32)
        qb = q_rows(j, BQ - QB, QB, pqb_buf.at[j], denb_buf.at[j], 0, False)
        for _ in range(QSPLIT):
            next(qb)
        kvps = []
        for a in (3, 2, 1, 0):
            gg = jnp.concatenate(blk[a], axis=1).astype(bf16)
            clock[0] += 256
            kv = jnp.where(hm, _dot(gg, wv_buf[j, :, a * 128:(a + 1) * 128], NN), 0.0)
            tscr2.at[a][...] = _pack(kv)
            kvps.append(_unpack(jnp.concatenate(
                [tscr2[a, pl.ds(jj, 8, stride=8), :] for jj in range(8)], axis=0)))
        mg = mg_buf

        def m_form(tok):
            for a in (3, 2, 1, 0):
                need(("mg", a))
                for jl in range(2):
                    for ct in range(2):
                        def put(k1, k2, v):
                            ms.at[k1 * 7 + k2][pl.ds(_mo(jl * 64 + (2 * a + j) * 8, 8), 8),
                                               ct * 128:(ct + 1) * 128] = v
                        yield from form_steps(
                            _rform, lambda q, u: mg[a, (2 * q + jl) * 16:(2 * q + jl + 1) * 16, _st(u, ct)], put)

        for i, a in enumerate((3, 2, 1, 0)):
            wo_u = pltpu.bitcast(wo_buf[j, a * 128:(a + 1) * 128, :], u32)
            res = mm(kvps[i], wo_u, NN, 256)
            mg.at[a][...] = _to_st(res)
            made.add(("mg", a))
            if i == 0:
                add_side(m_form, 112, 128, 768 + (49 - QSPLIT) * QB - 100)
        for _ in qb:
            pass

    def out_part(p0, nr, y, src, pr0):
        pr = pl.ds(_mo(pr0, 8), nr // 2)
        rows = [pl.ds(_mo(q * HQ + p0, 16), nr) for q in range(4)]
        row = lax.broadcasted_iota(i32, (nr, 256), 0) + p0
        blk = yield from strassen2(lambda k1, k2: _unpack(src[k1 * 7 + k2, pr, :]),
                                   lambda k1, k2: ms[k1 * 7 + k2], NN, nr)
        for s1 in (3, 2, 1, 0):
            for s2 in range(4):
                q = (s1 // 2) * 2 + s2 // 2
                u = (s1 % 2) * 2 + s2 % 2
                rr, cc = rows[q], pl.ds(u * 256, 256)
                a = jnp.concatenate([sa[rr, :]] * 2, axis=1)
                b = jnp.concatenate([sb[rr, :]] * 2, axis=1)
                o = blk[q][u] + jnp.where(row + q * HQ == idx_s[0], y[:, u * 256:(u + 1) * 256], 0.0)
                out_buf[rr, cc] = (x_buf[rr, cc].astype(f32) * a - b + o).astype(bf16)
                if s2 % 2 == 1:
                    ch = pl.ds((s1 % 2) * HD, HD)
                    cp(out_buf.at[rr, ch], out_hbm.at[0, rr, ch], SEM_O).start()

    def ffn_part(j, f_lo, f_hi):
        for f0 in range(f_lo, f_hi, 256):
            fs = slice(f0, f0 + 256)
            ag = jnp.zeros((8, 256), f32)
            au = jnp.zeros((8, 256), f32)
            for kg in range(D // 8):
                xv = jnp.concatenate([gate(xb[8 * kg:8 * kg + 8, :])] * 2, axis=1)
                ag = ag + wg_buf[j, 8 * kg:8 * kg + 8, fs].astype(f32) * xv
                au = au + wu_buf[j, 8 * kg:8 * kg + 8, fs].astype(f32) * xv
                if kg % FSTEP == FSTEP - 1:
                    yield
            g = _rbf(jnp.sum(ag, axis=0, keepdims=True))
            u = _rbf(jnp.sum(au, axis=0, keepdims=True))
            h = _rbf(_rbf(g * jax.nn.sigmoid(g)) * u)
            hb_buf[fs, :] = jnp.broadcast_to(h, (128, 256)).T
        for d0 in range(0, D, 512):
            ds_ = slice(d0, d0 + 512)
            acc = yacc[:, ds_]
            for kg in range(f_lo // 8, f_hi // 8):
                hv = jnp.concatenate([gate(hb_buf[8 * kg:8 * kg + 8, :])] * 4, axis=1)
                acc = acc + wd_buf[j, 8 * kg:8 * kg + 8, ds_].astype(f32) * hv
                if kg % FSTEP == FSTEP - 1:
                    yield
            yacc[:, ds_] = acc

    def wait_group(i):
        with _scope("a_wait%d" % i):
            for c in a_groups[i]:
                c.wait()

    def run_all(gen):
        for _ in gen:
            pass

    def ln_side(r0, n, t0, t1):
        add_side(lambda tok: ln_rows(r0, n, tok), 30 * n // 16 + 8 * LNPAD, t0, t1, SLAG)

    def l2_side(base, n, t0, t1):
        def gen(tok):
            for r in range(0, n, 16):
                yield from xs_form(r, tok, "l2", base)
        add_side(gen, 14 * n // 16, t0, t1)

    a_groups = make_a_groups()
    with _scope("p0_issue"):
        cp_wr.start()
        for grp in a_groups:
            for c in grp:
                c.start()
        for j in range(2):
            for part in range(2):
                for c in cp_b(j, part):
                    c.start()
        zacc[...] = jnp.zeros(zacc.shape, f32)
        zero_buf[1] = jnp.zeros((8, 128), u32)
        cp_zero = cp(zero_buf.at[1], zero_buf.at[0], SEM_Z)
        cp_zero.start()
        cp_zero.wait()
        cp_wr.wait()
        wrb[...] = jnp.broadcast_to(wr_buf[0:D].reshape(1, D).astype(f32), (8, D))
        z0 = jnp.max(pltpu.bitcast(zero_buf[0], i32))
        ps, pq_buf, den_buf, mg_buf, hb_buf = [r.at[z0] for r in (ps_raw, pq_raw, den_raw, mg_raw, hb_raw)]
        xn_buf = mg_buf

    def a01(i, carry):
        with _scope("a_wait01"):
            for c in cp_x(i * 64, 64, SEM_A + i):
                c.wait()
        with _scope("a01"):
            run_all(ln_rows(0, 64, None, "l1", i * 64))
        return carry

    lax.fori_loop(0, 2, a01, 0)

    def a23(i, carry):
        with _scope("a_wait23"):
            for c in cp_wk(i, SEM_A + 2 + i):
                c.wait()
        with _scope("a23"):
            run_all(wk_prep(i))
            l2_side(i * 64, 64, 300, 1500)
            kproj(0, 128, [(0, i)])
            finish()
        return carry

    lax.fori_loop(0, 2, a23, 0)
    wait_group(4)
    with _scope("a4"):
        run_all(wk_prep(2))
        ln_side(128, A4N, 0, 1500)
        kproj(0, 128, [(1, 0)])
        finish()
    wait_group(5)
    with _scope("a5"):
        run_all(wk_prep(3))
        if A5 == 0:
            ln_side(160, 32, 0, 1400)
            kproj(0, 128, [(1, 1)])
            for r0 in (128, 192):
                ln_side(r0 + 64, 64, 0, 3200)
                kproj(r0, 64)
        else:
            ln_side(128 + A4N, 192 - A4N, 0, A5)
            kproj(0, 128, [(1, 1)])
            for r0, n in A5K:
                kproj(r0, n)
        finish()
    wait_group(6)
    with _scope("a6"):
        ln_side(320, 192, 0, A6[0])
        add_side(wq_perm, 128, A6[1], A6[2], A6[6])
        add_side(wq_form, 224, A6[3], A6[4], A6[6])
        add_side(route, 17, A6[5], A6[5] + 800)
        for r0 in (256, 320, 384, 448):
            kproj(r0, 64)
        finish()

    def b_body(j, carry):
        qa = BQ - QB
        with _scope("b_wait0"):
            for c in cp_b(j, 0, wait_only=True):
                c.wait()
        with _scope("b_r0"):
            z_prep()
            t1 = 49 * qa - 400
            add_side(lambda tok: ps_form(j, None), 7 * HQ // 16, 0, t1)
            if F1:
                add_side(lambda tok: ffn_part(j, 0, F1), F1 * 3 // (4 * FSTEP), 0, t1)
            for r0 in range(0, qa, QN):
                run_all(q_rows(j, r0, min(QN, qa - r0), pq_buf, den_buf, r0, r0 + QN < qa))
            finish()
        with _scope("b_wait1"):
            for c in cp_b(j, 1, wait_only=True):
                c.wait()
        with _scope("b_r1"):
            add_side(lambda tok: ffn_part(j, F1, FH), (FH - F1) * 3 // (4 * FSTEP), 0, R1T[0])
            add_side(lambda tok: normalise(pq_buf, den_buf, qa, qs, j * (qa // 2),
                                           lambda r: (r // QN + 1) * QN >= qa), 22 * (qa // 16), 0, R1T[1])
            run_all(g_kvm(j))
            finish()
        return carry

    lax.fori_loop(0, 2, b_body, 0)

    def c_body(t, carry):
        with _scope("c_body"):
            y = _rbf(jnp.sum(yacc[...], axis=0, keepdims=True))
            y = _rbf(y * _rbf(jax.nn.sigmoid(rsel[0:1, :])))
            j, h = t >> 1, t & 1
            na, nb = (BQ - QB) // 2, QB // 2
            hb = pl.ds(_mo(h * nb, 16), nb)
            add_side(lambda tok: normalise(pqb_buf.at[j, :, hb, :], denb_buf.at[j, :, hb, :], nb, qsb, 0,
                                           lambda r: True, tok),
                     4 + 22 * (nb // 16), 0, 49 * na - 800, SLAG)
            for p in range(0, na, CR):
                p0 = j * BQ + h * na + p
                run_all(out_part(p0, min(CR, na - p), y, qs, t * (na // 2) + p // 2))
            advance(clock[0] + 10 ** 6)
            flush()
            run_all(out_part(j * BQ + BQ - QB + h * nb, nb, y, qsb, 0))
            finish()
        return carry

    lax.fori_loop(0, 4, c_body, 0)
    with _scope("tail"):
        cp(out_buf, out_hbm.at[0], SEM_O).wait()


@jax.jit
def pallas_parallel_sum__linear_attn_block__moe_arch_mod__prompt_kernel(
    A_x: jax.Array,
    A_wqkv: jax.Array,
    A_wo: jax.Array,
    B_x: jax.Array,
    B_w_r: jax.Array,
    B_w_gate: jax.Array,
    B_w_up: jax.Array,
    B_w_down: jax.Array,
):
    del B_x
    V = pltpu.VMEM
    scratch = [
        V((S, D), bf16),
        V((2, D, 512), bf16),
        V((2, 512, D), bf16),
        V((8 * D,), bf16),
        V((2, D, FH), bf16),
        V((2, D, FH), bf16),
        V((2, FH, D), bf16),
        V((28, HQ // 2, 256), u32),
        V((35, HQ // 2, 256), u32),
        V((49, 128, 256), u32),
        V((S, 128), f32),
        V((S, 128), f32),
        V((8, D), f32),
        V((8, D), f32),
        V((2, 4, HQ, 512), f32),
        V((D, 128), f32),
        V((8, D), f32),
        V((8, D), f32),
        V((8, D), f32),
        V((4, 8, 128), u32),
        V((4, HD // 2, 7 * 128), u32),
        V((S, 256), f32),
        V((64, 64, 128), u32),
        V((1, HQ // 2, 49 * 128), u32),
        V((49, BQ - QB, 256), u32),
        V((49, 128, 256), u32),
        V((8, 64, 128), u32),
        V((4, 64, 128), u32),
        V((1, 4, BQ - QB, D), f32),
        V((1, 4, BQ - QB, 128), f32),
        V((2, 4, QB, D), f32),
        V((2, 4, QB, 128), f32),
        V((49, QB // 4, 256), u32),
        V((1, 4, 128, D), f32),
        V((1, FH, 128), f32),
        V((S, D), bf16),
        pltpu.SMEM((1,), i32),
        pltpu.SemaphoreType.DMA((13,)),
    ]
    return pl.pallas_call(
        _kernel,
        out_shape=jax.ShapeDtypeStruct((1, S, D), bf16),
        in_specs=[pl.BlockSpec(memory_space=pl.ANY)] * 7,
        out_specs=pl.BlockSpec(memory_space=pl.ANY),
        scratch_shapes=scratch,
        compiler_params=pltpu.CompilerParams(vmem_limit_bytes=VMEM_MB * 1024 * 1024,
                                             disable_bounds_checks=True,
                                             fuse_transposed_lhs_in_matmul=FUSE,
                                             disable_semaphore_checks=True),
    )(A_x, A_wqkv, A_wo, B_w_r, B_w_gate, B_w_up, B_w_down)
```

```python
import contextlib

import jax
import jax.numpy as jnp
from jax import lax
import jax.experimental.pallas as pl
import jax.experimental.pallas.tpu as pltpu

bf16, f32, u32, i32 = jnp.bfloat16, jnp.float32, jnp.uint32, jnp.int32

S = 2048
D = 1024
F = 3584
HP = S // 2
HD = D // 2
HQ = S // 4
BQ = HQ // 2
FH = F // 2
F1 = 0
QB = 64
QN = 48
QW = (28, 36, 36, 6, 2, 2, 2)
A6 = (0, 6400, 9600, 8600, 13900, 10800, None)
TOKEV = 2
A5K = ((128, 48), (176, 48), (224, 32))
LNLAG = 700
L4 = ([(128, 192, 0, 1500)], [])
L5 = ([(192, 320, 1000, 7200)], [(128, 176, 0, 1600), (176, 320, 1700, 8600)])
L6 = ([(320, 512, 0, 6000)], [(320, 384, 800, 3400), (384, 512, 3500, 10400)])
A6K = ((256, 64), (320, 64), (384, 64), (448, 64))
R1T = (12800, 12800)
GW = (16,) * 7
MERGE = False
FB = FH
GLAG = 0
RECQ = True
FUSE = False
QSPLIT = 6
SLAG = 400
FSTEP = 2
CR = 32
XN = 128
VMEM_MB = 120
CT = 128

L_ORD = (2, 3, 0, 1, 4, 5, 6)
R_ORD = (2, 0, 6, 5, 1, 4, 3)

K_SEQ = (1, 4, 0, 2, 3, 5, 6)
K_SEQ2 = (0, 1, 2, 5, 3, 4, 6)
W_SEQ = (0, 1, 5, 6, 4, 2, 3)

NN = (((1,), (0,)), ((), ()))
NT_ = (((1,), (1,)), ((), ()))
TN = (((0,), (0,)), ((), ()))


SCOPES = False


def _scope(name):
    return jax.named_scope(name) if SCOPES else contextlib.nullcontext()


def _mo(v, m):
    return v if isinstance(v, int) else pl.multiple_of(v, m)


def _dot(a, b, dims):
    return lax.dot_general(a, b, dims, preferred_element_type=f32)


def _pack(v):
    return pltpu.bitcast(v.astype(bf16), u32)


def _unpack(v):
    return pltpu.bitcast(v, bf16)


def _combine(m):
    m1, m2, m3, m4, m5, m6, m7 = m
    return m1 + m4 - m5 + m7, m3 + m5, m2 + m4, m1 - m2 + m3 + m6


def _lform(a11, a12, a21, a22):
    return (a11 + a22, a21 + a22, a11, a22, a11 + a12, a21 - a11, a12 - a22)


def _rform(b11, b12, b21, b22):
    return (b11 + b22, b11, b12 - b22, b21 - b11, b22, b11 + b12, b21 + b22)


def _sform(x11, x12, x21, x22):
    return (x11, x22, x11 + x22, x21 + x22, x11 + x12, x21 - x11, x12 - x22)


def _wl(a11, a12, a21, a22):
    s1 = a21 + a22
    s2 = s1 - a11
    return (a11, a12, a12 - s2, a22, s1, s2, a11 - a21)


def _wr(b11, b12, b21, b22):
    t1 = b12 - b11
    t2 = b22 - t1
    return (b11, b21, b22, t2 - b21, t1, t2, b22 - b12)


def _wc(p):
    p1, p2, p3, p4, p5, p6, p7 = p
    u2 = p1 + p6
    u3 = u2 + p7
    return p1 + p2, (u2 + p5) + p3, u3 - p4, u3 + p5


W_R = (3, 1, 0, 2, 4, 5, 6)


def _wl_swapped(a11, a12, a21, a22):
    return _wl(a12, a11, a22, a21)


def _wc_swapped(p):
    p1, p2, p3, p4, p5, p6, p7 = p
    v2 = p1 + p6
    u3 = p7 - v2
    return (p5 - v2) + p3, p1 + p2, u3 + p5, p4 - u3


class _Sym:
    def __init__(self, t):
        self.t = t

    def __add__(self, o):
        return _Sym({**self.t, **o.t})

    def __sub__(self, o):
        return _Sym({**self.t, **{k: -v for k, v in o.t.items()}})


def _st(u, ct):
    return slice((4 * ct + u) * 128, (4 * ct + u + 1) * 128)


def _to_st(v):
    return jnp.concatenate([v[:, (2 * u + ct) * 128:(2 * u + ct + 1) * 128]
                            for ct in range(2) for u in range(4)], axis=1)


def _phi(t):
    return jnp.where(t > 0, t + 1.0, jnp.exp(t)) + 1e-6


def _rbf(v):
    return v.astype(bf16).astype(f32)


def _layernorm_rows(xv):
    mf = jnp.sum(xv, axis=1, keepdims=True) * (1.0 / D)
    d = xv - mf
    var = jnp.sum(d * d, axis=1, keepdims=True) * (1.0 / D)
    sd = _rbf(jnp.sqrt(_rbf(_rbf(var) + 1e-5)))
    return _rbf(_rbf(xv - _rbf(mf)) / sd)


def _kernel(x_hbm, wqkv_hbm, wo_hbm, wr_hbm, wg_hbm, wu_hbm, wd_hbm, out_hbm,
            x_buf, wv_buf, wo_buf, wr_buf, wg_buf, wu_buf, wd_buf,
            xs1, xs2, wqs, sa, sb, zacc, zp, pk_buf, xb, yacc, rsel, wrb, zero_buf,
            wks, stats, wqt, ps_raw, qs, ms, tscr, tscr2, pq_raw, den_raw, pqb_buf, denb_buf, qsb,
            mg_raw, hb_raw, out_buf, idx_s, sem):
    wq_buf = out_buf.at[pl.ds(0, D), :]
    wk_buf = out_buf.at[pl.ds(D, D), :]

    def xs_at(k1, e, rows=None):
        r = xs1.at[k1 * 4 + (0, 1, 7, 3).index(e)] if e in (0, 1, 7, 3) else xs2.at[k1 * 4 + (2, 4, 5, 6).index(e)]
        return r if rows is None else r.at[rows, :]

    SEM_B, SEM_O, SEM_Z, SEM_A = 0, 4, 5, 6

    def cp(src, dst, s):
        return pltpu.make_async_copy(src, dst, sem.at[s])

    def cp_x(r0, n, s):
        rows = [pl.ds(_mo(q * HQ + r0, 16), n) for q in range(4)]
        return [cp(x_hbm.at[0, r, :], x_buf.at[r, :], s) for r in rows]

    def cp_wk(c, s):
        return [cp(wqkv_hbm.at[:, pl.ds(_mo(D + h * HD + c * 128, 128), 128)],
                   wk_buf.at[:, pl.ds(_mo(c * 256 + h * 128, 128), 128)], s) for h in range(2)]

    cp_wr = cp(wr_hbm, wr_buf.at[pl.ds(0, D)], SEM_Z)

    def make_a_groups():
        return [
            cp_x(0, 64, SEM_A),
            cp_x(64, 64, SEM_A + 1),
            cp_wk(0, SEM_A + 2),
            cp_wk(1, SEM_A + 3),
            cp_wk(2, SEM_A + 4) + cp_x(128, 64, SEM_A + 4),
            cp_wk(3, SEM_A + 5) + cp_x(192, 128, SEM_A + 5),
            cp_x(320, 192, SEM_A + 6) + [cp(wqkv_hbm.at[:, pl.ds(0, D)], wq_buf, SEM_A + 6)],
        ]

    def cp_b(j, part, wait_only=False):
        pairs = []
        f0, fw = (0, F1) if part == 0 else (F1, FH - F1)
        fs = pl.ds(_mo(j * FH + f0, 128), fw)
        if fw:
          pairs += [(wg_hbm.at[:, fs], wg_buf.at[j, :, pl.ds(f0, fw)]),
                  (wu_hbm.at[:, fs], wu_buf.at[j, :, pl.ds(f0, fw)]),
                  (wd_hbm.at[fs, :], wd_buf.at[j, pl.ds(f0, fw), :])]
        if part == 1:
            for a in range(4):
                c0 = _mo((2 * a + j) * 128, 128)
                pairs += [(wqkv_hbm.at[:, pl.ds(2 * D + c0, 128)], wv_buf.at[j, :, pl.ds(a * 128, 128)]),
                          (wo_hbm.at[pl.ds(c0, 128), :], wo_buf.at[j, pl.ds(a * 128, 128), :])]
        return [cp(dst if wait_only else src, dst, SEM_B + 2 * j + part) for src, dst in pairs]

    clock = [0]
    toks = []
    sides = []
    fwd = [None]

    def emit_tok(vals, stamp=None):
        t = None
        for v in vals:
            v = pltpu.bitcast(v, u32) if v.dtype != u32 else v
            t = v if t is None else t | v
        toks.append((clock[0] if stamp is None else stamp, t & zero_buf[0]))

    def gate(v):
        if fwd[0] is None:
            return v
        if fwd[0][1] is None:
            fwd[0][1] = pltpu.bitcast(fwd[0][0](), u32) & zero_buf[0]
        head = pltpu.bitcast(pltpu.bitcast(v[0:8], u32) | fwd[0][1], v.dtype)
        return head if v.shape[0] == 8 else jnp.concatenate([head, v[8:]], axis=0)

    def add_side(gen_fn, n, t0, t1, lag=None):
        st = {"i": 0, "n": n, "t0": clock[0] + t0, "t1": clock[0] + t1}

        def tok(vals, extra=0):
            if lag is not None:
                emit_tok(vals, st["t0"] + (st["i"] + 1) * (st["t1"] - st["t0"]) // st["n"] + lag + extra)
        st["g"] = gen_fn(tok)
        sides.append(st)

    def advance(until):
        for st in sides:
            while st["i"] < st["n"] and st["t0"] + st["i"] * (st["t1"] - st["t0"]) // st["n"] < until:
                next(st["g"], None)
                st["i"] += 1
                if st["i"] == st["n"]:
                    for _ in st["g"]:
                        pass

    def flush():
        for st in sides:
            for _ in st["g"]:
                pass
        sides.clear()

    def finish():
        flush()
        toks.clear()
        fwd[0] = None

    def mm(lhs, rhs, dims, cycles, nseg=1):
        due = [t for (c, t) in toks if c <= clock[0]]
        toks[:] = [(c, t) for (c, t) in toks if c > clock[0]]
        if due:
            head = rhs[0:8, 0:128]
            for t in due:
                head = head | t
            if rhs.shape[1] > 128:
                head = jnp.concatenate([head, rhs[0:8, 128:]], axis=1)
            rhs = jnp.concatenate([head, rhs[8:]], axis=0)
        res = _dot(lhs, _unpack(rhs), dims)
        ngr = res.shape[0] // 16
        for sg in range(nseg):
            for i in range(ngr):
                fwd[0] = [lambda sg=sg, i=i: res[i * 16:i * 16 + 8, sg * 128:(sg + 1) * 128], None]
                clock[0] += cycles // nseg // ngr
                advance(clock[0])
        return res

    def gate16(v):
        return jnp.concatenate([gate(v[0:8]), gate(v[8:16])], axis=0)

    def form_steps(form, form2, get, put, tok=None, keep=range(7), offdiag=False):
        terms = form(*[_Sym({i: 1}) for i in range(4)])
        for k1 in range(7):
            sub = []
            for r in range(2):
                for c in range(2):
                    v = None
                    for i, sg in sorted(terms[k1].t.items(), key=lambda e: -e[1]):
                        b = get(r + 2 * (i // 2), c + 2 * (i % 2))
                        if v is None:
                            v = gate16(b) if (r == c) != offdiag else b
                        else:
                            v = v + b if sg > 0 else v - b
                    sub.append(v)
            vals = form2(*sub) + (sub[2],)
            for k2 in keep:
                put(k1, k2, _pack(vals[k2]))
            if tok is not None and k1 % TOKEV == TOKEV - 1 - (6 % TOKEV != TOKEV - 1):
                full = vals[3 if form2 is _wr else 2]
                tok([full[0:8], full[8:16]])
            yield

    def strassen2(lhs, rhs, dims, cycles, nseg=1, wts=(16,) * 7, comb=_wc):
        m1 = [None] * 7
        for i1, k1 in enumerate(K_SEQ2):
            m2 = [None] * 7
            for k2 in W_SEQ:
                m2[k2] = mm(lhs(k1, k2), rhs(k1, k2), dims, cycles * wts[i1] // 16, nseg)
                yield
            m1[k1] = comb(m2)
        out = [[None] * 4 for _ in range(4)]
        for s2 in range(4):
            for s1, v in enumerate(_combine([m1[k1][s2] for k1 in range(7)])):
                out[(s1 // 2) * 2 + s2 // 2][(s1 % 2) * 2 + s2 % 2] = v
        return out

    made = set()

    def need(*keys):
        assert all(k in made for k in keys), keys

    def row_views(base):
        if isinstance(base, int) and base == 0:
            return x_buf, sa, sb, stats, xn_buf, None
        b = _mo(base, 64)
        return ([r.at[pl.ds(b, S - 64), :] for r in (x_buf, sa, sb, stats)]
                + [xn_buf.at[:, pl.ds(b, 64), :], pl.ds(_mo(base // 2, 32), 32)])

    def xs_form(r0, tok, which="all", base=0):
        xn_v, xs_v = row_views(base)[4:]
        rows = slice(r0 % XN, r0 % XN + 16)

        keep = {"all": range(8), "l1": (0, 1, 7, 3), "l2": (2, 4, 5, 6)}[which]
        for ct in range(2):
            def put(k1, k2, v):
                xs_at(k1, k2, xs_v)[r0 // 2:r0 // 2 + 8, ct * 128:(ct + 1) * 128] = v
            yield from form_steps(
                _sform, _wl, lambda q, u: xn_v[q, rows, _st(u, ct)], put, tok, keep)
        made.add(("xs", r0))

    def ln_stats(r_start, n_rows, tok, base=0):
        x_v, sa_v, sb_v, st_v, xn_v, _ = row_views(base)
        lane = lax.broadcasted_iota(i32, (8, 128), 1)
        for r0 in range(r_start, r_start + n_rows, 16):
            if r0 >= 2 * XN:
                need(("ln", r0 - XN))
            for g in range(8):
                q, o = g // 2, (g % 2) * 8
                rg = q * HQ + r0 + o
                xv = x_v[rg:rg + 8, :].astype(f32)
                xg = jnp.concatenate([gate(xv[:, 0:128]), xv[:, 128:]], axis=1)
                mf = jnp.sum(xg, axis=1, keepdims=True) * (1.0 / D)
                d = xv - mf
                var = jnp.sum(d * d, axis=1, keepdims=True) * (1.0 / D)
                rs = lax.rsqrt(var + 1e-5)
                xn_v.at[q][r0 % XN + o:r0 % XN + o + 8, :] = _to_st(d * rs)
                rs = jnp.broadcast_to(rs, (8, 128))
                mf = jnp.broadcast_to(mf, (8, 128))
                sa_v[rg:rg + 8, :] = 1.0 + rs
                sb_v[rg:rg + 8, :] = mf * rs
                st_v[rg:rg + 8, 0:128] = jnp.where(lane == 0, mf, jnp.broadcast_to(var, (8, 128)))
                if tok is not None:
                    tok([rs])
                if g == 7:
                    made.add(("xn", r0))
                yield

    def ln_later(r_start, n_rows, tok, which="all", base=0):
        st_v, xn_v = row_views(base)[3:5]
        for r0 in range(r_start, r_start + n_rows, 16):
            need(("xn", r0))
            form = xs_form(r0, tok, which, base)
            for g in range(8):
                for _ in range(2 if g < 7 else 0):
                    next(form)
                    yield
                q, o = g // 2, (g % 2) * 8
                t = None
                for ct in range(8):
                    v = (xn_v[q, r0 % XN + o:r0 % XN + o + 8, _st(ct // 2, ct % 2)]
                         * wrb[:, ct * 128:(ct + 1) * 128])
                    t = gate(v) if t is None else t + v
                st_v[q * HQ + r0 + o:q * HQ + r0 + o + 8, 128:256] = t
                if tok is not None:
                    tok([t])
                if g == 7:
                    next(form, None)
                    made.add(("ln", r0))
                yield

    def wk_prep(c, tok=None):
        cs = pl.ds(_mo(c * 256, 256), 256)
        for i in range(HD // 16):
            r0 = i * 16
            top = wk_buf[r0:r0 + 16, cs].astype(f32)
            bot = wk_buf[HD + r0:HD + r0 + 16, cs].astype(f32)
            ops = _rform(gate(top[:, :128]), top[:, 128:], bot[:, :128], gate(bot[:, 128:]))
            for k in range(7):
                wks.at[c][r0 // 2:r0 // 2 + 8, k * 128:(k + 1) * 128] = _pack(ops[k])
            yield

    def wq_perm(tok):
        def permute(kt):
            for g in range(8):
                tile = gate(pltpu.bitcast(wq_buf[kt * 128:(kt + 1) * 128, g * 128:(g + 1) * 128], u32))
                wqt.at[kt * 8 + g][...] = pltpu.bitcast(_unpack(tile).T, u32)
                yield

        def back(kt):
            for j in range(8):
                tile = gate(jnp.concatenate([wqt[kt * 8 + g, pl.ds(j, 8, stride=8), :] for g in range(8)],
                                            axis=0))
                v = pltpu.bitcast(_unpack(tile).T.astype(f32), u32)
                c0 = (kt // 2) * D + _st(j // 2, j % 2).start
                ps[(kt % 2) * 128:(kt % 2 + 1) * 128, c0:c0 + 128] = v
                made.add(("wqp", kt, j))
                yield

        order = (0, 2, 4, 6, 1, 3, 5, 7)
        for n in range(10):
            if n < 8:
                yield from permute(order[n])
            if n > 1:
                yield from back(order[n - 2])

    def wq_form(tok):
        for i in range(16):
            need(*[("wqp", 2 * r + i // 8, j) for r in range(4) for j in range(8)])
            for ct in range(2):
                def put(k1, k2, v):
                    wqs.at[k1 * 7 + k2][i * 8:(i + 1) * 8, ct * 128:(ct + 1) * 128] = v
                yield from form_steps(
                    _rform, _wr, lambda r, c: pltpu.bitcast(
                        ps[i * 16:(i + 1) * 16, r * D + _st(c, ct).start:r * D + _st(c, ct).stop],
                        f32), put, tok)

    def kproj(r0, n, chunks=((0, 0), (0, 1), (1, 0), (1, 1))):
        pr = pl.ds(r0 // 2, n // 2)
        need(*[("xs", r) for r in range(max(r0, 128), r0 + n, 16)])
        for ch, ct in chunks:
            c = 2 * ch + ct
            m = [None] * 7
            for k in K_SEQ:
                e11, e12, e21, e22 = [xs_at(L_ORD[k], e)[pr, :] for e in (0, 1, 7, 3)]
                lhs = jnp.concatenate([jnp.concatenate([e11, e12], axis=1),
                                       jnp.concatenate([e21, e22], axis=1)], axis=0)
                m[k] = mm(_unpack(lhs), wks[c, :, k * 128:(k + 1) * 128], NN, 2 * n)
            kk = [_phi(v) for v in _combine(m)]
            for h in range(2):
                zacc[:, pl.ds(_mo(h * HD + c * 128, 128), 128)] += (
                    (kk[h] + kk[2 + h]).reshape(n // 4, 8, 128).sum(axis=0))
            for s1 in range(4):
                u = (s1 % 2) * 2 + ch
                for h in range(2):
                    pk_buf.at[ct, (s1 // 2) * 2 + h][r0:r0 + n, u * 128:(u + 1) * 128] = (
                        kk[s1][h * n:(h + 1) * n])

    def z_prep():
        z = jnp.sum(zacc[...], axis=0, keepdims=True)
        zt = _pack(jnp.broadcast_to(z, (128, D)).astype(bf16).T)
        for g in range(8):
            tscr.at[g][...] = zt[g * 64:(g + 1) * 64, :]
        for j in range(8):
            blk = jnp.concatenate([tscr[g, pl.ds(j, 8, stride=8), :] for g in range(8)], axis=0)
            zp[:, j * 128:(j + 1) * 128] = _unpack(blk).T[0:8, :].astype(f32)

    def route(tok):
        need(*[("ln", r) for r in range(128, HQ, 16)])
        rows, dots = [], []
        for b in range(S // 128):
            rows.append(gate(stats[b * 128:(b + 1) * 128, 0:128]).T[0:8, :])
            dots.append(jnp.sum(gate(stats[b * 128:(b + 1) * 128, 128:256]).T, axis=0, keepdims=True))
            yield
        mf = jnp.concatenate([v[0:1] for v in rows], axis=0)
        var = jnp.concatenate([v[1:2] for v in rows], axis=0)
        tr = jnp.concatenate(dots, axis=0) * jnp.sqrt(var + 1e-5)
        wsum = jnp.sum(wrb[0:1, :], axis=1, keepdims=True)
        sd = _rbf(jnp.sqrt(_rbf(_rbf(var) + 1e-5)))
        rv = _rbf((tr + (mf - _rbf(mf)) * wsum) / sd)
        rmax = jnp.max(rv)
        pos = (lax.broadcasted_iota(i32, rv.shape, 0) * 128 + lax.broadcasted_iota(i32, rv.shape, 1))
        idx = jnp.min(jnp.where(rv == rmax, pos, S - 1))
        idx_s[0] = idx
        b0 = _mo((idx // 16) * 16, 16)
        xn = _layernorm_rows(x_buf[pl.ds(b0, 16), :].astype(f32))
        sel = lax.broadcasted_iota(i32, xn.shape, 0) == idx - b0
        row = jnp.sum(jnp.where(sel, xn, 0.0), axis=0, keepdims=True)
        rsel[...] = jnp.broadcast_to(_rbf(jnp.sum(row * wrb[0:1, :], axis=1, keepdims=True)), rsel.shape)
        xbv = jnp.broadcast_to(row, (128, D)).T
        xb[...] = xbv
        yacc[...] = jnp.zeros(yacc.shape, f32)
        tok([xbv[b * 128 + 120:(b + 1) * 128] for b in range(8)])
        yield

    def ps_form(j, tok):
        for c in range(HQ // 16):
            def put(k1, k2, v):
                k = k1 * 7 + k2
                ps[c * 8:(c + 1) * 8, k * 128:(k + 1) * 128] = v
            yield from form_steps(
                _lform, _wl_swapped,
                lambda r, q: pk_buf[j, q, c * 16:(c + 1) * 16, r * 128:(r + 1) * 128], put, tok, offdiag=True)

    def q_rows(j, r0, n, pq, rc, d0, rec):
        xj = pl.ds(_mo(j * (BQ // 2), BQ // 2), BQ // 2)
        pr = slice(r0 // 2, (r0 + n) // 2)
        blk = yield from strassen2(lambda k1, k2: _unpack(xs_at(L_ORD[k1], k2, xj)[pr, :]),
                                   lambda k1, k2: wqs[k1 * 7 + k2], NN, n, 1, QW)
        lane = lax.broadcasted_iota(i32, (n, 128), 1)
        for q in range(4):
            d = None
            for u in (3, 2, 1, 0):
                v = _phi(blk[q][u])
                for ct in range(2):
                    pq.at[q][d0:d0 + n, _st(u, ct)] = v[:, ct * 128:(ct + 1) * 128]
                t = v * zp[0:1, u * 256:(u + 1) * 256]
                t = t[:, :128] + t[:, 128:]
                d = t if d is None else d + t
            if rec:
                d = recip(d, lane)
            rc.at[q][d0:d0 + n, :] = d

    def recip(d, lane):
        d = d + jnp.where(lane % 2 == 0, pltpu.roll(d, 127, 1), pltpu.roll(d, 1, 1))
        d = d + jnp.where(lane % 4 < 2, pltpu.roll(d, 126, 1), pltpu.roll(d, 2, 1))
        return 1.0 / (d + 1e-6)

    def normalise(pq, rc, nr, dst, p0, raw, tok=None):
        lane = lax.broadcasted_iota(i32, (16, 128), 1)

        def fix(c):
            if c < nr // 16 and raw(c * 16):
                for q in range(4):
                    rq = slice(c * 16, (c + 1) * 16)
                    rc.at[q][rq, :] = recip(gate16(rc[q, rq, :]), lane)

        def scale(c):
            rq = slice(c * 16, (c + 1) * 16)
            fix(c + 1)
            for hf in range(2):
                for q in range(4):
                    cs = slice(hf * HD, (hf + 1) * HD)
                    pq.at[q][rq, cs] = pq[q, rq, cs] * jnp.concatenate([gate16(rc[q, rq, :])] * 4, axis=1)
                    yield

        def form(c):
            rq = slice(c * 16, (c + 1) * 16)
            p2 = pl.ds(_mo(p0 + c * 8, 8), 8)
            for ct in range(2):
                def put(k1, k2, v):
                    dst.at[k1 * 7 + k2][p2, ct * 128:(ct + 1) * 128] = v
                yield from form_steps(_lform, _wl, lambda q, u: pq[q, rq, _st(u, ct)], put, tok)

        fix(0)
        if raw(0):
            for _ in range(4):
                yield
        yield from scale(0)
        for c in range(nr // 16):
            nxt = scale(c + 1) if c + 1 < nr // 16 else iter(())
            for i, _ in enumerate(form(c)):
                yield
                if i < 8 and c + 1 < nr // 16:
                    next(nxt)
                    yield
        made.add(("qs", id(dst)))

    hist = []

    def g_lhs(k):
        v = ps[:, k * 128:(k + 1) * 128]
        hist.append(fwd[0])
        if GLAG and len(hist) > GLAG and hist[-1 - GLAG] is not None:
            cur = fwd[0]
            fwd[0] = hist[-1 - GLAG]
            v = jnp.concatenate([gate(v[i * 64:(i + 1) * 64]) for i in range(4)], axis=0)
            fwd[0] = cur
        return _unpack(v)

    def g_kvm(j):
        blk = yield from strassen2(
            lambda k1, k2: g_lhs(k1 * 7 + k2),
            lambda k1, k2: xs_at(R_ORD[k1], W_R[k2])[...], TN, 256, 2, GW, _wc_swapped)
        hm = (lax.broadcasted_iota(i32, (128, 128), 0) // 32
              == lax.broadcasted_iota(i32, (128, 128), 1) // 32)
        qb = q_rows(j, BQ - QB, QB, pqb_buf.at[j], denb_buf.at[j], 0, False)
        for _ in range(QSPLIT):
            next(qb)
        kvps = []
        for a in (3, 2, 1, 0):
            gg = jnp.concatenate(blk[a], axis=1).astype(bf16)
            clock[0] += 256
            kv = jnp.where(hm, _dot(gg, wv_buf[j, :, a * 128:(a + 1) * 128], NN), 0.0)
            tscr2.at[a][...] = _pack(kv)
            kvps.append(_unpack(jnp.concatenate(
                [tscr2[a, pl.ds(jj, 8, stride=8), :] for jj in range(8)], axis=0)))
        mg = mg_buf

        def m_form(tok):
            for a in (3, 2, 1, 0):
                need(("mg", a))
                for jl in range(2):
                    for ct in range(2):
                        def put(k1, k2, v):
                            ms.at[k1 * 7 + k2][pl.ds(_mo(jl * 64 + (2 * a + j) * 8, 8), 8),
                                               ct * 128:(ct + 1) * 128] = v
                        yield from form_steps(
                            _rform, _wr, lambda q, u: mg[a, (2 * q + jl) * 16:(2 * q + jl + 1) * 16, _st(u, ct)], put)

        for i, a in enumerate((3, 2, 1, 0)):
            wo_u = pltpu.bitcast(wo_buf[j, a * 128:(a + 1) * 128, :], u32)
            res = mm(kvps[i], wo_u, NN, 256)
            mg.at[a][...] = _to_st(res)
            made.add(("mg", a))
            if i == 0:
                add_side(m_form, 112, 128, 768 + (49 - QSPLIT) * QB - 100)
        for _ in qb:
            pass

    def out_part(p0, nr, y, src, pr0):
        pr = pl.ds(_mo(pr0, 8), nr // 2)
        rows = [pl.ds(_mo(q * HQ + p0, 16), nr) for q in range(4)]
        row = lax.broadcasted_iota(i32, (nr, 256), 0) + p0
        blk = yield from strassen2(lambda k1, k2: _unpack(src[k1 * 7 + k2, pr, :]),
                                   lambda k1, k2: ms[k1 * 7 + k2], NN, nr)
        for s1 in (3, 2, 1, 0):
            for s2 in range(4):
                q = (s1 // 2) * 2 + s2 // 2
                u = (s1 % 2) * 2 + s2 % 2
                rr, cc = rows[q], pl.ds(u * 256, 256)
                a = jnp.concatenate([sa[rr, :]] * 2, axis=1)
                b = jnp.concatenate([sb[rr, :]] * 2, axis=1)
                o = blk[q][u] + jnp.where(row + q * HQ == idx_s[0], y[:, u * 256:(u + 1) * 256], 0.0)
                out_buf[rr, cc] = (x_buf[rr, cc].astype(f32) * a - b + o).astype(bf16)
                if s2 % 2 == 1:
                    ch = pl.ds((s1 % 2) * HD, HD)
                    cp(out_buf.at[rr, ch], out_hbm.at[0, rr, ch], SEM_O).start()

    def ffn_part(j, f_lo, f_hi):
        for f0 in range(f_lo, f_hi, 256):
            fs = slice(f0, f0 + 256)
            ag = jnp.zeros((8, 256), f32)
            au = jnp.zeros((8, 256), f32)
            for kg in range(D // 8):
                xv = jnp.concatenate([gate(xb[8 * kg:8 * kg + 8, :])] * 2, axis=1)
                ag = ag + wg_buf[j, 8 * kg:8 * kg + 8, fs].astype(f32) * xv
                au = au + wu_buf[j, 8 * kg:8 * kg + 8, fs].astype(f32) * xv
                if kg % FSTEP == FSTEP - 1:
                    yield
            g = _rbf(jnp.sum(ag, axis=0, keepdims=True))
            u = _rbf(jnp.sum(au, axis=0, keepdims=True))
            h = _rbf(_rbf(g * jax.nn.sigmoid(g)) * u)
            hb_buf[fs, :] = jnp.broadcast_to(h, (128, 256)).T
        for d0 in range(0, D, 512):
            ds_ = slice(d0, d0 + 512)
            acc = yacc[:, ds_]
            for kg in range(f_lo // 8, f_hi // 8):
                hv = jnp.concatenate([gate(hb_buf[8 * kg:8 * kg + 8, :])] * 4, axis=1)
                acc = acc + wd_buf[j, 8 * kg:8 * kg + 8, ds_].astype(f32) * hv
                if kg % FSTEP == FSTEP - 1:
                    yield
            yacc[:, ds_] = acc

    def wait_group(i):
        with _scope("a_wait%d" % i):
            for c in a_groups[i]:
                c.wait()

    def run_all(gen):
        for _ in gen:
            pass

    def ln_sides(plan):
        for r0, r1, t0, t1 in plan[0]:
            add_side(lambda tok, r0=r0, r1=r1: ln_stats(r0, r1 - r0, tok), (r1 - r0) // 2, t0, t1, LNLAG)
        for r0, r1, t0, t1 in plan[1]:
            add_side(lambda tok, r0=r0, r1=r1: ln_later(r0, r1 - r0, tok), 22 * (r1 - r0) // 16, t0, t1, SLAG)

    def l2_side(base, n, t0, t1):
        def gen(tok):
            for r in range(0, n, 16):
                yield from xs_form(r, tok, "l2", base)
        add_side(gen, 14 * n // 16, t0, t1)

    a_groups = make_a_groups()
    with _scope("p0_issue"):
        cp_wr.start()
        for grp in a_groups:
            for c in grp:
                c.start()
        for j in range(2):
            for part in range(2):
                for c in cp_b(j, part):
                    c.start()
        zacc[...] = jnp.zeros(zacc.shape, f32)
        zero_buf[1] = jnp.zeros((8, 128), u32)
        cp_zero = cp(zero_buf.at[1], zero_buf.at[0], SEM_Z)
        cp_zero.start()
        cp_zero.wait()
        cp_wr.wait()
        wrb[...] = jnp.broadcast_to(wr_buf[0:D].reshape(1, D).astype(f32), (8, D))
        z0 = jnp.max(pltpu.bitcast(zero_buf[0], i32))
        ps, pq_buf, den_buf, mg_buf, hb_buf = [r.at[z0] for r in (ps_raw, pq_raw, den_raw, mg_raw, hb_raw)]
        xn_buf = mg_buf

    def a01(i, carry):
        with _scope("a_wait01"):
            for c in cp_x(i * 64, 64, SEM_A + i):
                c.wait()
        with _scope("a01"):
            for r in range(0, 64, 16):
                run_all(ln_stats(r, 16, None, i * 64))
                if r:
                    run_all(ln_later(r - 16, 16, None, "l1", i * 64))
            run_all(ln_later(48, 16, None, "l1", i * 64))
        return carry

    lax.fori_loop(0, 2, a01, 0)

    def a23(i, carry):
        with _scope("a_wait23"):
            for c in cp_wk(i, SEM_A + 2 + i):
                c.wait()
        with _scope("a23"):
            run_all(wk_prep(i))
            l2_side(i * 64, 64, 300, 1500)
            kproj(0, 128, [(0, i)])
            finish()
        return carry

    lax.fori_loop(0, 2, a23, 0)
    wait_group(4)
    with _scope("a4"):
        run_all(wk_prep(2))
        ln_sides(L4)
        kproj(0, 128, [(1, 0)])
        finish()
    wait_group(5)
    with _scope("a5"):
        run_all(wk_prep(3))
        ln_sides(L5)
        kproj(0, 128, [(1, 1)])
        for r0, n in A5K:
            kproj(r0, n)
        finish()
    wait_group(6)
    with _scope("a6"):
        ln_sides(L6)
        add_side(wq_perm, 128, A6[1], A6[2], A6[6])
        add_side(wq_form, 224, A6[3], A6[4], A6[6])
        add_side(route, 17, A6[5], A6[5] + 800)
        for r0, n in A6K:
            kproj(r0, n)
        finish()

    def b_body(j, carry):
        qa = BQ - QB
        with _scope("b_wait0"):
            for c in cp_b(j, 0, wait_only=True) + (cp_b(j, 1, wait_only=True) if MERGE else []):
                c.wait()
        with _scope("b_r0"):
            z_prep()
            t1 = 49 * qa - 400
            add_side(lambda tok: ps_form(j, tok), 7 * HQ // 16, 0, t1, SLAG if MERGE else None)
            if F1:
                add_side(lambda tok: ffn_part(j, 0, F1), F1 * 3 // (4 * FSTEP), 0, t1)
            for r0 in range(0, qa, QN):
                run_all(q_rows(j, r0, min(QN, qa - r0), pq_buf, den_buf, r0, r0 + QN < qa))
            if MERGE:
                flush()
            else:
                finish()
        if not MERGE:
            with _scope("b_wait1"):
                for c in cp_b(j, 1, wait_only=True):
                    c.wait()
        with _scope("b_r1"):
            add_side(lambda tok: ffn_part(j, F1, FB), (FB - F1) * 3 // (4 * FSTEP), 0, R1T[0])
            add_side(lambda tok: normalise(pq_buf, den_buf, qa, qs, j * (qa // 2),
                                           lambda r: (r // QN + 1) * QN >= qa), 22 * (qa // 16), 0, R1T[1])
            run_all(g_kvm(j))
            finish()
        return carry

    lax.fori_loop(0, 2, b_body, 0)

    def c_body(t, carry):
        with _scope("c_body"):
            y = _rbf(jnp.sum(yacc[...], axis=0, keepdims=True))
            y = _rbf(y * _rbf(1.0 / _rbf(1.0 + _rbf(jnp.exp(-rsel[0:1, :])))))
            j, h = t >> 1, t & 1
            na, nb = (BQ - QB) // 2, QB // 2
            hb = pl.ds(_mo(h * nb, 16), nb)
            add_side(lambda tok: normalise(pqb_buf.at[j, :, hb, :], denb_buf.at[j, :, hb, :], nb, qsb, 0,
                                           lambda r: True, tok),
                     4 + 22 * (nb // 16), 0, 49 * na - 800, SLAG)
            for p in range(0, na, CR):
                p0 = j * BQ + h * na + p
                run_all(out_part(p0, min(CR, na - p), y, qs, t * (na // 2) + p // 2))
            advance(clock[0] + 10 ** 6)
            flush()
            run_all(out_part(j * BQ + BQ - QB + h * nb, nb, y, qsb, 0))
            finish()
        return carry

    lax.fori_loop(0, 4, c_body, 0)
    with _scope("tail"):
        cp(out_buf, out_hbm.at[0], SEM_O).wait()


@jax.jit
def pallas_parallel_sum__linear_attn_block__moe_arch_mod__prompt_kernel(
    A_x: jax.Array,
    A_wqkv: jax.Array,
    A_wo: jax.Array,
    B_x: jax.Array,
    B_w_r: jax.Array,
    B_w_gate: jax.Array,
    B_w_up: jax.Array,
    B_w_down: jax.Array,
):
    del B_x
    V = pltpu.VMEM
    scratch = [
        V((S, D), bf16),
        V((2, D, 512), bf16),
        V((2, 512, D), bf16),
        V((8 * D,), bf16),
        V((2, D, FH), bf16),
        V((2, D, FH), bf16),
        V((2, FH, D), bf16),
        V((28, HQ // 2, 256), u32),
        V((28, HQ // 2, 256), u32),
        V((49, 128, 256), u32),
        V((S, 128), f32),
        V((S, 128), f32),
        V((8, D), f32),
        V((8, D), f32),
        V((2, 4, HQ, 512), f32),
        V((D, 128), f32),
        V((8, D), f32),
        V((8, D), f32),
        V((8, D), f32),
        V((4, 8, 128), u32),
        V((4, HD // 2, 7 * 128), u32),
        V((S, 256), f32),
        V((64, 64, 128), u32),
        V((1, HQ // 2, 49 * 128), u32),
        V((49, BQ - QB, 256), u32),
        V((49, 128, 256), u32),
        V((8, 64, 128), u32),
        V((4, 64, 128), u32),
        V((1, 4, BQ - QB, D), f32),
        V((1, 4, BQ - QB, 128), f32),
        V((2, 4, QB, D), f32),
        V((2, 4, QB, 128), f32),
        V((49, QB // 4, 256), u32),
        V((1, 4, 128, D), f32),
        V((1, FH, 128), f32),
        V((S, D), bf16),
        pltpu.SMEM((1,), i32),
        pltpu.SemaphoreType.DMA((13,)),
    ]
    return pl.pallas_call(
        _kernel,
        out_shape=jax.ShapeDtypeStruct((1, S, D), bf16),
        in_specs=[pl.BlockSpec(memory_space=pl.ANY)] * 7,
        out_specs=pl.BlockSpec(memory_space=pl.ANY),
        scratch_shapes=scratch,
        compiler_params=pltpu.CompilerParams(vmem_limit_bytes=VMEM_MB * 1024 * 1024,
                                             disable_bounds_checks=True,
                                             fuse_transposed_lhs_in_matmul=FUSE,
                                             disable_semaphore_checks=True),
    )(A_x, A_wqkv, A_wo, B_w_r, B_w_gate, B_w_up, B_w_down)
```

```python
import contextlib

import jax
import jax.numpy as jnp
from jax import lax
import jax.experimental.pallas as pl
import jax.experimental.pallas.tpu as pltpu

bf16, f32, u32, i32 = jnp.bfloat16, jnp.float32, jnp.uint32, jnp.int32

S = 2048
D = 1024
F = 3584
HP = S // 2
HD = D // 2
HQ = S // 4
BQ = HQ // 2
FH = F // 2
F1 = 0
QB = 64
QN = 48
QW = (28, 36, 36, 6, 2, 2, 2)
A6 = (0, 6400, 9600, 8600, 13900, 10800, None)
TOKEV = 2
A5K = ((128, 48), (176, 48), (224, 32))
LNLAG = 700
L4 = ([(128, 192, 0, 1500)], [])
L5 = ([(192, 320, 1000, 7200)], [(128, 176, 0, 1600), (176, 320, 1700, 8600)])
L6 = ([(320, 512, 0, 6000)], [(320, 384, 800, 3400), (384, 512, 3500, 10400)])
A6K = ((256, 64), (320, 64), (384, 64), (448, 64))
R1T = (12800, 12800)
GW = (16,) * 7
MERGE = False
FB = FH
GLAG = 0
RECQ = True
FUSE = False
QSPLIT = 6
SLAG = 400
FSTEP = 2
CR = 32
XN = 128
VMEM_MB = 120
CT = 128

L_ORD = (2, 3, 0, 1, 4, 5, 6)
R_ORD = (2, 0, 6, 5, 1, 4, 3)

K_SEQ = (1, 4, 0, 2, 3, 5, 6)
K_SEQ2 = (0, 1, 2, 5, 3, 4, 6)
W_SEQ = (0, 1, 5, 6, 4, 2, 3)

NN = (((1,), (0,)), ((), ()))
NT_ = (((1,), (1,)), ((), ()))
TN = (((0,), (0,)), ((), ()))


SCOPES = False


def _scope(name):
    return jax.named_scope(name) if SCOPES else contextlib.nullcontext()


def _mo(v, m):
    return v if isinstance(v, int) else pl.multiple_of(v, m)


def _dot(a, b, dims):
    return lax.dot_general(a, b, dims, preferred_element_type=f32)


def _pack(v):
    return pltpu.bitcast(v.astype(bf16), u32)


def _unpack(v):
    return pltpu.bitcast(v, bf16)


def _combine(m):
    m1, m2, m3, m4, m5, m6, m7 = m
    return m1 + m4 - m5 + m7, m3 + m5, m2 + m4, m1 - m2 + m3 + m6


def _lform(a11, a12, a21, a22):
    return (a11 + a22, a21 + a22, a11, a22, a11 + a12, a21 - a11, a12 - a22)


def _rform(b11, b12, b21, b22):
    return (b11 + b22, b11, b12 - b22, b21 - b11, b22, b11 + b12, b21 + b22)


def _sform(x11, x12, x21, x22):
    return (x11, x22, x11 + x22, x21 + x22, x11 + x12, x21 - x11, x12 - x22)


def _wl(a11, a12, a21, a22):
    s1 = a21 + a22
    s2 = s1 - a11
    return (a11, a12, a12 - s2, a22, s1, s2, a11 - a21)


def _wr(b11, b12, b21, b22):
    t1 = b12 - b11
    t2 = b22 - t1
    return (b11, b21, b22, t2 - b21, t1, t2, b22 - b12)


def _wc(p):
    p1, p2, p3, p4, p5, p6, p7 = p
    u2 = p1 + p6
    u3 = u2 + p7
    return p1 + p2, (u2 + p5) + p3, u3 - p4, u3 + p5


W_R = (3, 1, 0, 2, 4, 5, 6)


def _wl_swapped(a11, a12, a21, a22):
    return _wl(a12, a11, a22, a21)


def _wc_swapped(p):
    p1, p2, p3, p4, p5, p6, p7 = p
    v2 = p1 + p6
    u3 = p7 - v2
    return (p5 - v2) + p3, p1 + p2, u3 + p5, p4 - u3


class _Sym:
    def __init__(self, t):
        self.t = t

    def __add__(self, o):
        return _Sym({**self.t, **o.t})

    def __sub__(self, o):
        return _Sym({**self.t, **{k: -v for k, v in o.t.items()}})


def _st(u, ct):
    return slice((4 * ct + u) * 128, (4 * ct + u + 1) * 128)


def _to_st(v):
    return jnp.concatenate([v[:, (2 * u + ct) * 128:(2 * u + ct + 1) * 128]
                            for ct in range(2) for u in range(4)], axis=1)


def _phi(t):
    return jnp.where(t > 0, t + 1.0, jnp.exp(t)) + 1e-6


def _rbf(v):
    return v.astype(bf16).astype(f32)


def _layernorm_rows(xv):
    mf = jnp.sum(xv, axis=1, keepdims=True) * (1.0 / D)
    d = xv - mf
    var = jnp.sum(d * d, axis=1, keepdims=True) * (1.0 / D)
    sd = _rbf(jnp.sqrt(_rbf(_rbf(var) + 1e-5)))
    return _rbf(_rbf(xv - _rbf(mf)) / sd)


def _kernel(x_hbm, wqkv_hbm, wo_hbm, wr_hbm, wg_hbm, wu_hbm, wd_hbm, out_hbm,
            x_buf, wv_buf, wo_buf, wr_buf, wg_buf, wu_buf, wd_buf,
            xs1, xs2, wqs, sa, sb, zacc, zp, pk_buf, xb, yacc, rsel, wrb, zero_buf,
            wks, stats, wqt, ps_raw, qs, ms, tscr, tscr2, pq_raw, den_raw, pqb_buf, denb_buf, qsb,
            mg_raw, hb_raw, out_buf, idx_s, sem):
    wq_buf = out_buf.at[pl.ds(0, D), :]
    wk_buf = out_buf.at[pl.ds(D, D), :]

    def xs_at(k1, e, rows=None):
        r = xs1.at[k1 * 4 + (0, 1, 7, 3).index(e)] if e in (0, 1, 7, 3) else xs2.at[k1 * 4 + (2, 4, 5, 6).index(e)]
        return r if rows is None else r.at[rows, :]

    SEM_B, SEM_O, SEM_Z, SEM_A = 0, 4, 5, 6

    def cp(src, dst, s):
        return pltpu.make_async_copy(src, dst, sem.at[s])

    def cp_x(r0, n, s):
        rows = [pl.ds(_mo(q * HQ + r0, 16), n) for q in range(4)]
        return [cp(x_hbm.at[0, r, :], x_buf.at[r, :], s) for r in rows]

    def cp_wk(c, s):
        return [cp(wqkv_hbm.at[:, pl.ds(_mo(D + c * 256, 256), 256)],
                   wk_buf.at[:, pl.ds(_mo(c * 256, 256), 256)], s)]

    cp_wr = cp(wr_hbm, wr_buf.at[pl.ds(0, D)], SEM_Z)

    def make_a_groups():
        return [
            cp_x(0, 64, SEM_A),
            cp_x(64, 64, SEM_A + 1),
            cp_wk(0, SEM_A + 2),
            cp_wk(1, SEM_A + 3),
            cp_wk(2, SEM_A + 4) + cp_x(128, 64, SEM_A + 4),
            cp_wk(3, SEM_A + 5) + cp_x(192, 128, SEM_A + 5),
            cp_x(320, 192, SEM_A + 6) + [cp(wqkv_hbm.at[:, pl.ds(0, D)], wq_buf, SEM_A + 6)],
        ]

    def cp_b(j, part, wait_only=False):
        pairs = []
        f0, fw = (0, F1) if part == 0 else (F1, FH - F1)
        fs = pl.ds(_mo(j * FH + f0, 128), fw)
        if fw:
          pairs += [(wg_hbm.at[:, fs], wg_buf.at[j, :, pl.ds(f0, fw)]),
                  (wu_hbm.at[:, fs], wu_buf.at[j, :, pl.ds(f0, fw)]),
                  (wd_hbm.at[fs, :], wd_buf.at[j, pl.ds(f0, fw), :])]
        if part == 1:
            for a in range(4):
                c0 = _mo((2 * a + j) * 128, 128)
                pairs += [(wqkv_hbm.at[:, pl.ds(2 * D + c0, 128)], wv_buf.at[j, :, pl.ds(a * 128, 128)]),
                          (wo_hbm.at[pl.ds(c0, 128), :], wo_buf.at[j, pl.ds(a * 128, 128), :])]
        return [cp(dst if wait_only else src, dst, SEM_B + 2 * j + part) for src, dst in pairs]

    clock = [0]
    toks = []
    sides = []
    fwd = [None]

    def emit_tok(vals, stamp=None):
        t = None
        for v in vals:
            v = pltpu.bitcast(v, u32) if v.dtype != u32 else v
            t = v if t is None else t | v
        toks.append((clock[0] if stamp is None else stamp, t & zero_buf[0]))

    def gate(v):
        if fwd[0] is None:
            return v
        if fwd[0][1] is None:
            fwd[0][1] = pltpu.bitcast(fwd[0][0](), u32) & zero_buf[0]
        head = pltpu.bitcast(pltpu.bitcast(v[0:8], u32) | fwd[0][1], v.dtype)
        return head if v.shape[0] == 8 else jnp.concatenate([head, v[8:]], axis=0)

    def add_side(gen_fn, n, t0, t1, lag=None):
        st = {"i": 0, "n": n, "t0": clock[0] + t0, "t1": clock[0] + t1}

        def tok(vals, extra=0):
            if lag is not None:
                emit_tok(vals, st["t0"] + (st["i"] + 1) * (st["t1"] - st["t0"]) // st["n"] + lag + extra)
        st["g"] = gen_fn(tok)
        sides.append(st)

    def advance(until):
        for st in sides:
            while st["i"] < st["n"] and st["t0"] + st["i"] * (st["t1"] - st["t0"]) // st["n"] < until:
                next(st["g"], None)
                st["i"] += 1
                if st["i"] == st["n"]:
                    for _ in st["g"]:
                        pass

    def flush():
        for st in sides:
            for _ in st["g"]:
                pass
        sides.clear()

    def finish():
        flush()
        toks.clear()
        fwd[0] = None

    def mm(lhs, rhs, dims, cycles, nseg=1):
        due = [t for (c, t) in toks if c <= clock[0]]
        toks[:] = [(c, t) for (c, t) in toks if c > clock[0]]
        if due:
            head = rhs[0:8, 0:128]
            for t in due:
                head = head | t
            if rhs.shape[1] > 128:
                head = jnp.concatenate([head, rhs[0:8, 128:]], axis=1)
            rhs = jnp.concatenate([head, rhs[8:]], axis=0)
        res = _dot(lhs, _unpack(rhs), dims)
        ngr = res.shape[0] // 16
        for sg in range(nseg):
            for i in range(ngr):
                fwd[0] = [lambda sg=sg, i=i: res[i * 16:i * 16 + 8, sg * 128:(sg + 1) * 128], None]
                clock[0] += cycles // nseg // ngr
                advance(clock[0])
        return res

    def gate16(v):
        return jnp.concatenate([gate(v[0:8]), gate(v[8:16])], axis=0)

    def form_steps(form, form2, get, put, tok=None, keep=range(7), offdiag=False):
        terms = form(*[_Sym({i: 1}) for i in range(4)])
        for k1 in range(7):
            sub = []
            for r in range(2):
                for c in range(2):
                    v = None
                    for i, sg in sorted(terms[k1].t.items(), key=lambda e: -e[1]):
                        b = get(r + 2 * (i // 2), c + 2 * (i % 2))
                        if v is None:
                            v = gate16(b) if (r == c) != offdiag else b
                        else:
                            v = v + b if sg > 0 else v - b
                    sub.append(v)
            vals = form2(*sub) + (sub[2],)
            for k2 in keep:
                put(k1, k2, _pack(vals[k2]))
            if tok is not None and k1 % TOKEV == TOKEV - 1 - (6 % TOKEV != TOKEV - 1):
                full = vals[3 if form2 is _wr else 2]
                tok([full[0:8], full[8:16]])
            yield

    def strassen2(lhs, rhs, dims, cycles, nseg=1, wts=(16,) * 7, comb=_wc):
        m1 = [None] * 7
        for i1, k1 in enumerate(K_SEQ2):
            m2 = [None] * 7
            for k2 in W_SEQ:
                m2[k2] = mm(lhs(k1, k2), rhs(k1, k2), dims, cycles * wts[i1] // 16, nseg)
                yield
            m1[k1] = comb(m2)
        out = [[None] * 4 for _ in range(4)]
        for s2 in range(4):
            for s1, v in enumerate(_combine([m1[k1][s2] for k1 in range(7)])):
                out[(s1 // 2) * 2 + s2 // 2][(s1 % 2) * 2 + s2 % 2] = v
        return out

    made = set()

    def need(*keys):
        assert all(k in made for k in keys), keys

    def row_views(base):
        if isinstance(base, int) and base == 0:
            return x_buf, sa, sb, stats, xn_buf, None
        b = _mo(base, 64)
        return ([r.at[pl.ds(b, S - 64), :] for r in (x_buf, sa, sb, stats)]
                + [xn_buf.at[:, pl.ds(b, 64), :], pl.ds(_mo(base // 2, 32), 32)])

    def xs_form(r0, tok, which="all", base=0):
        xn_v, xs_v = row_views(base)[4:]
        rows = slice(r0 % XN, r0 % XN + 16)

        keep = {"all": range(8), "l1": (0, 1, 7, 3), "l2": (2, 4, 5, 6)}[which]
        for ct in range(2):
            def put(k1, k2, v):
                xs_at(k1, k2, xs_v)[r0 // 2:r0 // 2 + 8, ct * 128:(ct + 1) * 128] = v
            yield from form_steps(
                _sform, _wl, lambda q, u: xn_v[q, rows, _st(u, ct)], put, tok, keep)
        made.add(("xs", r0))

    def ln_stats(r_start, n_rows, tok, base=0):
        x_v, sa_v, sb_v, st_v, xn_v, _ = row_views(base)
        lane = lax.broadcasted_iota(i32, (8, 128), 1)
        for r0 in range(r_start, r_start + n_rows, 16):
            if r0 >= 2 * XN:
                need(("ln", r0 - XN))
            for g in range(8):
                q, o = g // 2, (g % 2) * 8
                rg = q * HQ + r0 + o
                xv = x_v[rg:rg + 8, :].astype(f32)
                xg = jnp.concatenate([gate(xv[:, 0:128]), xv[:, 128:]], axis=1)
                mf = jnp.sum(xg, axis=1, keepdims=True) * (1.0 / D)
                d = xv - mf
                var = jnp.sum(d * d, axis=1, keepdims=True) * (1.0 / D)
                rs = lax.rsqrt(var + 1e-5)
                xn_v.at[q][r0 % XN + o:r0 % XN + o + 8, :] = _to_st(d * rs)
                rs = jnp.broadcast_to(rs, (8, 128))
                mf = jnp.broadcast_to(mf, (8, 128))
                sa_v[rg:rg + 8, :] = 1.0 + rs
                sb_v[rg:rg + 8, :] = mf * rs
                st_v[rg:rg + 8, 0:128] = jnp.where(lane == 0, mf, jnp.broadcast_to(var, (8, 128)))
                if tok is not None:
                    tok([rs])
                if g == 7:
                    made.add(("xn", r0))
                yield

    def ln_later(r_start, n_rows, tok, which="all", base=0):
        st_v, xn_v = row_views(base)[3:5]
        for r0 in range(r_start, r_start + n_rows, 16):
            need(("xn", r0))
            form = xs_form(r0, tok, which, base)
            for g in range(8):
                for _ in range(2 if g < 7 else 0):
                    next(form)
                    yield
                q, o = g // 2, (g % 2) * 8
                t = None
                for ct in range(8 if which != "l1" else 0):
                    v = (xn_v[q, r0 % XN + o:r0 % XN + o + 8, _st(ct // 2, ct % 2)]
                         * wrb[:, ct * 128:(ct + 1) * 128])
                    t = gate(v) if t is None else t + v
                if t is not None:
                    st_v[q * HQ + r0 + o:q * HQ + r0 + o + 8, 128:256] = t
                if tok is not None:
                    tok([t])
                if g == 7:
                    next(form, None)
                    made.add(("ln", r0))
                yield

    def wk_prep(c, tok=None):
        cs = pl.ds(_mo(c * 256, 256), 256)
        for i in range(HD // 16):
            r0 = i * 16
            top = wk_buf[r0:r0 + 16, cs].astype(f32)
            bot = wk_buf[HD + r0:HD + r0 + 16, cs].astype(f32)
            ops = _rform(gate(top[:, :128]), top[:, 128:], bot[:, :128], gate(bot[:, 128:]))
            for k in range(7):
                wks.at[c][r0 // 2:r0 // 2 + 8, k * 128:(k + 1) * 128] = _pack(ops[k])
            yield

    def wq_perm(tok):
        def permute(kt):
            for g in range(8):
                tile = gate(pltpu.bitcast(wq_buf[kt * 128:(kt + 1) * 128, g * 128:(g + 1) * 128], u32))
                wqt.at[kt * 8 + g][...] = pltpu.bitcast(_unpack(tile).T, u32)
                yield

        def back(kt):
            for j in range(8):
                tile = gate(jnp.concatenate([wqt[kt * 8 + g, pl.ds(j, 8, stride=8), :] for g in range(8)],
                                            axis=0))
                v = pltpu.bitcast(_unpack(tile).T.astype(f32), u32)
                c0 = (kt // 2) * D + _st(j // 2, j % 2).start
                ps[(kt % 2) * 128:(kt % 2 + 1) * 128, c0:c0 + 128] = v
                made.add(("wqp", kt, j))
                yield

        order = (0, 2, 4, 6, 1, 3, 5, 7)
        for n in range(10):
            if n < 8:
                yield from permute(order[n])
            if n > 1:
                yield from back(order[n - 2])

    def wq_form(tok):
        for i in range(16):
            need(*[("wqp", 2 * r + i // 8, j) for r in range(4) for j in range(8)])
            for ct in range(2):
                def put(k1, k2, v):
                    wqs.at[k1 * 7 + k2][i * 8:(i + 1) * 8, ct * 128:(ct + 1) * 128] = v
                yield from form_steps(
                    _rform, _wr, lambda r, c: pltpu.bitcast(
                        ps[i * 16:(i + 1) * 16, r * D + _st(c, ct).start:r * D + _st(c, ct).stop],
                        f32), put, tok)

    def kproj(r0, n, chunks=range(4)):
        pr = pl.ds(r0 // 2, n // 2)
        need(*[("xs", r) for r in range(max(r0, 128), r0 + n, 16)])
        for c in chunks:
            m = [None] * 7
            for k in K_SEQ:
                e11, e12, e21, e22 = [xs_at(L_ORD[k], e)[pr, :] for e in (0, 1, 7, 3)]
                lhs = jnp.concatenate([jnp.concatenate([e11, e12], axis=1),
                                       jnp.concatenate([e21, e22], axis=1)], axis=0)
                m[k] = mm(_unpack(lhs), wks[c, :, k * 128:(k + 1) * 128], NN, 2 * n)
            kk = [_phi(v) for v in _combine(m)]
            for ct in range(2):
                zacc[:, pl.ds(_mo(c * 256 + ct * 128, 128), 128)] += (
                    (kk[ct] + kk[2 + ct]).reshape(n // 4, 8, 128).sum(axis=0))
            for s1 in range(4):
                for h in range(2):
                    pk_buf.at[s1 % 2, (s1 // 2) * 2 + h][r0:r0 + n, pl.ds(_mo(c * 128, 128), 128)] = (
                        kk[s1][h * n:(h + 1) * n])

    def z_prep():
        z = jnp.sum(zacc[...], axis=0, keepdims=True)
        zt = _pack(jnp.broadcast_to(z, (128, D)).astype(bf16).T)
        for g in range(8):
            tscr.at[g][...] = zt[g * 64:(g + 1) * 64, :]
        for j in range(8):
            blk = jnp.concatenate([tscr[g, pl.ds(j, 8, stride=8), :] for g in range(8)], axis=0)
            zp[:, j * 128:(j + 1) * 128] = _unpack(blk).T[0:8, :].astype(f32)

    def route(tok):
        need(*[("ln", r) for r in range(128, HQ, 16)])
        rows, dots = [], []
        for b in range(S // 128):
            rows.append(gate(stats[b * 128:(b + 1) * 128, 0:128]).T[0:8, :])
            dots.append(jnp.sum(gate(stats[b * 128:(b + 1) * 128, 128:256]).T, axis=0, keepdims=True))
            yield
        mf = jnp.concatenate([v[0:1] for v in rows], axis=0)
        var = jnp.concatenate([v[1:2] for v in rows], axis=0)
        tr = jnp.concatenate(dots, axis=0) * jnp.sqrt(var + 1e-5)
        wsum = jnp.sum(wrb[0:1, :], axis=1, keepdims=True)
        sd = _rbf(jnp.sqrt(_rbf(_rbf(var) + 1e-5)))
        rv = _rbf((tr + (mf - _rbf(mf)) * wsum) / sd)
        rmax = jnp.max(rv)
        pos = (lax.broadcasted_iota(i32, rv.shape, 0) * 128 + lax.broadcasted_iota(i32, rv.shape, 1))
        idx = jnp.min(jnp.where(rv == rmax, pos, S - 1))
        idx_s[0] = idx
        b0 = _mo((idx // 16) * 16, 16)
        xn = _layernorm_rows(x_buf[pl.ds(b0, 16), :].astype(f32))
        sel = lax.broadcasted_iota(i32, xn.shape, 0) == idx - b0
        row = jnp.sum(jnp.where(sel, xn, 0.0), axis=0, keepdims=True)
        rsel[...] = jnp.broadcast_to(_rbf(jnp.sum(row * wrb[0:1, :], axis=1, keepdims=True)), rsel.shape)
        xbv = jnp.broadcast_to(row, (128, D)).T
        xb[...] = xbv
        yacc[...] = jnp.zeros(yacc.shape, f32)
        tok([xbv[b * 128 + 120:(b + 1) * 128] for b in range(8)])
        yield

    def ps_form(j, tok):
        for c in range(HQ // 16):
            def put(k1, k2, v):
                k = k1 * 7 + k2
                ps[c * 8:(c + 1) * 8, k * 128:(k + 1) * 128] = v
            yield from form_steps(
                _lform, _wl_swapped,
                lambda r, q: pk_buf[j, q, c * 16:(c + 1) * 16, r * 128:(r + 1) * 128], put, tok, offdiag=True)

    def q_rows(j, r0, n, pq, rc, d0, rec):
        xj = pl.ds(_mo(j * (BQ // 2), BQ // 2), BQ // 2)
        pr = slice(r0 // 2, (r0 + n) // 2)
        blk = yield from strassen2(lambda k1, k2: _unpack(xs_at(L_ORD[k1], k2, xj)[pr, :]),
                                   lambda k1, k2: wqs[k1 * 7 + k2], NN, n, 1, QW)
        lane = lax.broadcasted_iota(i32, (n, 128), 1)
        for q in range(4):
            d = None
            for u in (3, 2, 1, 0):
                v = _phi(blk[q][u])
                for ct in range(2):
                    pq.at[q][d0:d0 + n, _st(u, ct)] = v[:, ct * 128:(ct + 1) * 128]
                t = v * zp[0:1, u * 256:(u + 1) * 256]
                t = t[:, :128] + t[:, 128:]
                d = t if d is None else d + t
            if rec:
                d = recip(d, lane)
            rc.at[q][d0:d0 + n, :] = d

    def recip(d, lane):
        d = d + jnp.where(lane % 2 == 0, pltpu.roll(d, 127, 1), pltpu.roll(d, 1, 1))
        d = d + jnp.where(lane % 4 < 2, pltpu.roll(d, 126, 1), pltpu.roll(d, 2, 1))
        return 1.0 / (d + 1e-6)

    def normalise(pq, rc, nr, dst, p0, raw, tok=None):
        lane = lax.broadcasted_iota(i32, (16, 128), 1)

        def fix(c):
            if c < nr // 16 and raw(c * 16):
                for q in range(4):
                    rq = slice(c * 16, (c + 1) * 16)
                    rc.at[q][rq, :] = recip(gate16(rc[q, rq, :]), lane)

        def scale(c):
            rq = slice(c * 16, (c + 1) * 16)
            fix(c + 1)
            for hf in range(2):
                for q in range(4):
                    cs = slice(hf * HD, (hf + 1) * HD)
                    pq.at[q][rq, cs] = pq[q, rq, cs] * jnp.concatenate([gate16(rc[q, rq, :])] * 4, axis=1)
                    yield

        def form(c):
            rq = slice(c * 16, (c + 1) * 16)
            p2 = pl.ds(_mo(p0 + c * 8, 8), 8)
            for ct in range(2):
                def put(k1, k2, v):
                    dst.at[k1 * 7 + k2][p2, ct * 128:(ct + 1) * 128] = v
                yield from form_steps(_lform, _wl, lambda q, u: pq[q, rq, _st(u, ct)], put, tok)

        fix(0)
        if raw(0):
            for _ in range(4):
                yield
        yield from scale(0)
        for c in range(nr // 16):
            nxt = scale(c + 1) if c + 1 < nr // 16 else iter(())
            for i, _ in enumerate(form(c)):
                yield
                if i < 8 and c + 1 < nr // 16:
                    next(nxt)
                    yield
        made.add(("qs", id(dst)))

    hist = []

    def g_lhs(k):
        v = ps[:, k * 128:(k + 1) * 128]
        hist.append(fwd[0])
        if GLAG and len(hist) > GLAG and hist[-1 - GLAG] is not None:
            cur = fwd[0]
            fwd[0] = hist[-1 - GLAG]
            v = jnp.concatenate([gate(v[i * 64:(i + 1) * 64]) for i in range(4)], axis=0)
            fwd[0] = cur
        return _unpack(v)

    def g_kvm(j):
        blk = yield from strassen2(
            lambda k1, k2: g_lhs(k1 * 7 + k2),
            lambda k1, k2: xs_at(R_ORD[k1], W_R[k2])[...], TN, 256, 2, GW, _wc_swapped)
        hm = (lax.broadcasted_iota(i32, (128, 128), 0) // 32
              == lax.broadcasted_iota(i32, (128, 128), 1) // 32)
        qb = q_rows(j, BQ - QB, QB, pqb_buf.at[j], denb_buf.at[j], 0, False)
        for _ in range(QSPLIT):
            next(qb)
        kvps = []
        for a in (3, 2, 1, 0):
            gg = jnp.concatenate(blk[a], axis=1).astype(bf16)
            clock[0] += 256
            kv = jnp.where(hm, _dot(gg, wv_buf[j, :, a * 128:(a + 1) * 128], NN), 0.0)
            tscr2.at[a][...] = _pack(kv)
            kvps.append(_unpack(jnp.concatenate(
                [tscr2[a, pl.ds(jj, 8, stride=8), :] for jj in range(8)], axis=0)))
        mg = mg_buf

        def m_form(tok):
            for a in (3, 2, 1, 0):
                need(("mg", a))
                for jl in range(2):
                    for ct in range(2):
                        def put(k1, k2, v):
                            ms.at[k1 * 7 + k2][pl.ds(_mo(jl * 64 + (2 * a + j) * 8, 8), 8),
                                               ct * 128:(ct + 1) * 128] = v
                        yield from form_steps(
                            _rform, _wr, lambda q, u: mg[a, (2 * q + jl) * 16:(2 * q + jl + 1) * 16, _st(u, ct)], put)

        for i, a in enumerate((3, 2, 1, 0)):
            wo_u = pltpu.bitcast(wo_buf[j, a * 128:(a + 1) * 128, :], u32)
            res = mm(kvps[i], wo_u, NN, 256)
            mg.at[a][...] = _to_st(res)
            made.add(("mg", a))
            if i == 0:
                add_side(m_form, 112, 128, 768 + (49 - QSPLIT) * QB - 100)
        for _ in qb:
            pass

    def out_part(p0, nr, y, src, pr0):
        pr = pl.ds(_mo(pr0, 8), nr // 2)
        rows = [pl.ds(_mo(q * HQ + p0, 16), nr) for q in range(4)]
        row = lax.broadcasted_iota(i32, (nr, 256), 0) + p0
        blk = yield from strassen2(lambda k1, k2: _unpack(src[k1 * 7 + k2, pr, :]),
                                   lambda k1, k2: ms[k1 * 7 + k2], NN, nr)
        for s1 in (3, 2, 1, 0):
            for s2 in range(4):
                q = (s1 // 2) * 2 + s2 // 2
                u = (s1 % 2) * 2 + s2 % 2
                rr, cc = rows[q], pl.ds(u * 256, 256)
                a = jnp.concatenate([sa[rr, :]] * 2, axis=1)
                b = jnp.concatenate([sb[rr, :]] * 2, axis=1)
                o = blk[q][u] + jnp.where(row + q * HQ == idx_s[0], y[:, u * 256:(u + 1) * 256], 0.0)
                out_buf[rr, cc] = (x_buf[rr, cc].astype(f32) * a - b + o).astype(bf16)
                if s2 % 2 == 1:
                    ch = pl.ds((s1 % 2) * HD, HD)
                    cp(out_buf.at[rr, ch], out_hbm.at[0, rr, ch], SEM_O).start()

    def ffn_part(j, f_lo, f_hi):
        for f0 in range(f_lo, f_hi, 256):
            fs = slice(f0, f0 + 256)
            ag = jnp.zeros((8, 256), f32)
            au = jnp.zeros((8, 256), f32)
            for kg in range(D // 8):
                xv = jnp.concatenate([gate(xb[8 * kg:8 * kg + 8, :])] * 2, axis=1)
                ag = ag + wg_buf[j, 8 * kg:8 * kg + 8, fs].astype(f32) * xv
                au = au + wu_buf[j, 8 * kg:8 * kg + 8, fs].astype(f32) * xv
                if kg % FSTEP == FSTEP - 1:
                    yield
            g = _rbf(jnp.sum(ag, axis=0, keepdims=True))
            u = _rbf(jnp.sum(au, axis=0, keepdims=True))
            h = _rbf(_rbf(g * jax.nn.sigmoid(g)) * u)
            hb_buf[fs, :] = jnp.broadcast_to(h, (128, 256)).T
        for d0 in range(0, D, 512):
            ds_ = slice(d0, d0 + 512)
            acc = yacc[:, ds_]
            for kg in range(f_lo // 8, f_hi // 8):
                hv = jnp.concatenate([gate(hb_buf[8 * kg:8 * kg + 8, :])] * 4, axis=1)
                acc = acc + wd_buf[j, 8 * kg:8 * kg + 8, ds_].astype(f32) * hv
                if kg % FSTEP == FSTEP - 1:
                    yield
            yacc[:, ds_] = acc

    def wait_group(i):
        with _scope("a_wait%d" % i):
            for c in a_groups[i]:
                c.wait()

    def run_all(gen):
        for _ in gen:
            pass

    def ln_sides(plan):
        for r0, r1, t0, t1 in plan[0]:
            add_side(lambda tok, r0=r0, r1=r1: ln_stats(r0, r1 - r0, tok), (r1 - r0) // 2, t0, t1, LNLAG)
        for r0, r1, t0, t1 in plan[1]:
            add_side(lambda tok, r0=r0, r1=r1: ln_later(r0, r1 - r0, tok), 22 * (r1 - r0) // 16, t0, t1, SLAG)

    def l2_side(base, n, t0, t1):
        add_side(lambda tok: ln_later(0, n, None, "l2", base), 22 * n // 16, t0, t1)

    a_groups = make_a_groups()
    with _scope("p0_issue"):
        cp_wr.start()
        for grp in a_groups:
            for c in grp:
                c.start()
        for j in range(2):
            for part in range(2):
                for c in cp_b(j, part):
                    c.start()
        zacc[...] = jnp.zeros(zacc.shape, f32)
        zero_buf[1] = jnp.zeros((8, 128), u32)
        cp_zero = cp(zero_buf.at[1], zero_buf.at[0], SEM_Z)
        cp_zero.start()
        cp_zero.wait()
        cp_wr.wait()
        wrb[...] = jnp.broadcast_to(wr_buf[0:D].reshape(1, D).astype(f32), (8, D))
        z0 = jnp.max(pltpu.bitcast(zero_buf[0], i32))
        ps, pq_buf, den_buf, mg_buf, hb_buf = [r.at[z0] for r in (ps_raw, pq_raw, den_raw, mg_raw, hb_raw)]
        xn_buf = mg_buf

    def a01(i, carry):
        with _scope("a_wait01"):
            for c in cp_x(i * 64, 64, SEM_A + i):
                c.wait()
        with _scope("a01"):
            for r in range(0, 64, 16):
                run_all(ln_stats(r, 16, None, i * 64))
                if r:
                    run_all(ln_later(r - 16, 16, None, "l1", i * 64))
            run_all(ln_later(48, 16, None, "l1", i * 64))
        return carry

    lax.fori_loop(0, 2, a01, 0)

    def a23(i, carry):
        with _scope("a_wait23"):
            for c in cp_wk(i, SEM_A + 2 + i):
                c.wait()
        with _scope("a23"):
            run_all(wk_prep(i))
            l2_side(i * 64, 64, 300, 1500)
            kproj(0, 128, [i])
            finish()
        return carry

    lax.fori_loop(0, 2, a23, 0)
    wait_group(4)
    with _scope("a4"):
        run_all(wk_prep(2))
        ln_sides(L4)
        kproj(0, 128, [2])
        finish()
    wait_group(5)
    with _scope("a5"):
        run_all(wk_prep(3))
        ln_sides(L5)
        kproj(0, 128, [3])
        for r0, n in A5K:
            kproj(r0, n)
        finish()
    wait_group(6)
    with _scope("a6"):
        ln_sides(L6)
        add_side(wq_perm, 128, A6[1], A6[2], A6[6])
        add_side(wq_form, 224, A6[3], A6[4], A6[6])
        add_side(route, 17, A6[5], A6[5] + 800)
        for r0, n in A6K:
            kproj(r0, n)
        finish()

    def b_body(j, carry):
        qa = BQ - QB
        with _scope("b_wait0"):
            for c in cp_b(j, 0, wait_only=True) + (cp_b(j, 1, wait_only=True) if MERGE else []):
                c.wait()
        with _scope("b_r0"):
            z_prep()
            t1 = 49 * qa - 400
            add_side(lambda tok: ps_form(j, tok), 7 * HQ // 16, 0, t1, SLAG if MERGE else None)
            if F1:
                add_side(lambda tok: ffn_part(j, 0, F1), F1 * 3 // (4 * FSTEP), 0, t1)
            for r0 in range(0, qa, QN):
                run_all(q_rows(j, r0, min(QN, qa - r0), pq_buf, den_buf, r0, r0 + QN < qa))
            if MERGE:
                flush()
            else:
                finish()
        if not MERGE:
            with _scope("b_wait1"):
                for c in cp_b(j, 1, wait_only=True):
                    c.wait()
        with _scope("b_r1"):
            add_side(lambda tok: ffn_part(j, F1, FB), (FB - F1) * 3 // (4 * FSTEP), 0, R1T[0])
            add_side(lambda tok: normalise(pq_buf, den_buf, qa, qs, j * (qa // 2),
                                           lambda r: (r // QN + 1) * QN >= qa), 22 * (qa // 16), 0, R1T[1])
            run_all(g_kvm(j))
            finish()
        return carry

    lax.fori_loop(0, 2, b_body, 0)

    def c_body(t, carry):
        with _scope("c_body"):
            y = _rbf(jnp.sum(yacc[...], axis=0, keepdims=True))
            y = _rbf(y * _rbf(1.0 / _rbf(1.0 + _rbf(jnp.exp(-rsel[0:1, :])))))
            j, h = t >> 1, t & 1
            na, nb = (BQ - QB) // 2, QB // 2
            hb = pl.ds(_mo(h * nb, 16), nb)
            add_side(lambda tok: normalise(pqb_buf.at[j, :, hb, :], denb_buf.at[j, :, hb, :], nb, qsb, 0,
                                           lambda r: True, tok),
                     4 + 22 * (nb // 16), 0, 49 * na - 800, SLAG)
            for p in range(0, na, CR):
                p0 = j * BQ + h * na + p
                run_all(out_part(p0, min(CR, na - p), y, qs, t * (na // 2) + p // 2))
            advance(clock[0] + 10 ** 6)
            flush()
            run_all(out_part(j * BQ + BQ - QB + h * nb, nb, y, qsb, 0))
            finish()
        return carry

    lax.fori_loop(0, 4, c_body, 0)
    with _scope("tail"):
        cp(out_buf, out_hbm.at[0], SEM_O).wait()


@jax.jit
def pallas_parallel_sum__linear_attn_block__moe_arch_mod__prompt_kernel(
    A_x: jax.Array,
    A_wqkv: jax.Array,
    A_wo: jax.Array,
    B_x: jax.Array,
    B_w_r: jax.Array,
    B_w_gate: jax.Array,
    B_w_up: jax.Array,
    B_w_down: jax.Array,
):
    del B_x
    V = pltpu.VMEM
    scratch = [
        V((S, D), bf16),
        V((2, D, 512), bf16),
        V((2, 512, D), bf16),
        V((8 * D,), bf16),
        V((2, D, FH), bf16),
        V((2, D, FH), bf16),
        V((2, FH, D), bf16),
        V((28, HQ // 2, 256), u32),
        V((28, HQ // 2, 256), u32),
        V((49, 128, 256), u32),
        V((S, 128), f32),
        V((S, 128), f32),
        V((8, D), f32),
        V((8, D), f32),
        V((2, 4, HQ, 512), f32),
        V((D, 128), f32),
        V((8, D), f32),
        V((8, D), f32),
        V((8, D), f32),
        V((4, 8, 128), u32),
        V((4, HD // 2, 7 * 128), u32),
        V((S, 256), f32),
        V((64, 64, 128), u32),
        V((1, HQ // 2, 49 * 128), u32),
        V((49, BQ - QB, 256), u32),
        V((49, 128, 256), u32),
        V((8, 64, 128), u32),
        V((4, 64, 128), u32),
        V((1, 4, BQ - QB, D), f32),
        V((1, 4, BQ - QB, 128), f32),
        V((2, 4, QB, D), f32),
        V((2, 4, QB, 128), f32),
        V((49, QB // 4, 256), u32),
        V((1, 4, 128, D), f32),
        V((1, FH, 128), f32),
        V((S, D), bf16),
        pltpu.SMEM((1,), i32),
        pltpu.SemaphoreType.DMA((13,)),
    ]
    return pl.pallas_call(
        _kernel,
        out_shape=jax.ShapeDtypeStruct((1, S, D), bf16),
        in_specs=[pl.BlockSpec(memory_space=pl.ANY)] * 7,
        out_specs=pl.BlockSpec(memory_space=pl.ANY),
        scratch_shapes=scratch,
        compiler_params=pltpu.CompilerParams(vmem_limit_bytes=VMEM_MB * 1024 * 1024,
                                             disable_bounds_checks=True,
                                             fuse_transposed_lhs_in_matmul=FUSE,
                                             disable_semaphore_checks=True),
    )(A_x, A_wqkv, A_wo, B_w_r, B_w_gate, B_w_up, B_w_down)
```

```python
import contextlib

import jax
import jax.numpy as jnp
from jax import lax
import jax.experimental.pallas as pl
import jax.experimental.pallas.tpu as pltpu

bf16, f32, u32, i32 = jnp.bfloat16, jnp.float32, jnp.uint32, jnp.int32

S = 2048
D = 1024
F = 3584
HP = S // 2
HD = D // 2
HQ = S // 4
BQ = HQ // 2
FH = F // 2
F1 = 0
QB = 64
QN = 48
QW = (28, 36, 36, 6, 2, 2, 2)
A6 = (0, 6400, 9600, 8600, 13900, 10800, None)
TOKEV = 2
A5K = ((128, 48), (176, 48), (224, 32))
LNLAG = 700
L4 = ([(128, 192, 0, 1500)], [])
L5 = ([(192, 320, 1000, 7200)], [(128, 176, 0, 1600), (176, 320, 1700, 8600)])
L6 = ([(320, 512, 0, 6000)], [(320, 384, 800, 3400), (384, 512, 3500, 10400)])
A6K = ((256, 64), (320, 64), (384, 64), (448, 64))
R1T = (12800, 12800)
GW = (16,) * 7
MERGE = False
FB = FH
GLAG = 0
RECQ = True
FUSE = False
QSPLIT = 6
SLAG = 400
FSTEP = 2
CR = 32
XN = 128
VMEM_MB = 120
CT = 128

L_ORD = (2, 3, 0, 1, 4, 5, 6)
R_ORD = (2, 0, 6, 5, 1, 4, 3)

K_SEQ = (1, 4, 0, 2, 3, 5, 6)
K_SEQ2 = (0, 1, 2, 5, 3, 4, 6)
W_SEQ = (0, 1, 5, 6, 4, 2, 3)

NN = (((1,), (0,)), ((), ()))
NT_ = (((1,), (1,)), ((), ()))
TN = (((0,), (0,)), ((), ()))


SCOPES = False


def _scope(name):
    return jax.named_scope(name) if SCOPES else contextlib.nullcontext()


def _mo(v, m):
    return v if isinstance(v, int) else pl.multiple_of(v, m)


def _dot(a, b, dims):
    return lax.dot_general(a, b, dims, preferred_element_type=f32)


def _pack(v):
    return pltpu.bitcast(v.astype(bf16), u32)


def _unpack(v):
    return pltpu.bitcast(v, bf16)


def _combine(m):
    m1, m2, m3, m4, m5, m6, m7 = m
    return m1 + m4 - m5 + m7, m3 + m5, m2 + m4, m1 - m2 + m3 + m6


def _lform(a11, a12, a21, a22):
    return (a11 + a22, a21 + a22, a11, a22, a11 + a12, a21 - a11, a12 - a22)


def _rform(b11, b12, b21, b22):
    return (b11 + b22, b11, b12 - b22, b21 - b11, b22, b11 + b12, b21 + b22)


def _sform(x11, x12, x21, x22):
    return (x11, x22, x11 + x22, x21 + x22, x11 + x12, x21 - x11, x12 - x22)


def _wl(a11, a12, a21, a22):
    s1 = a21 + a22
    s2 = s1 - a11
    return (a11, a12, a12 - s2, a22, s1, s2, a11 - a21)


def _wr(b11, b12, b21, b22):
    t1 = b12 - b11
    t2 = b22 - t1
    return (b11, b21, b22, t2 - b21, t1, t2, b22 - b12)


def _wc(p):
    p1, p2, p3, p4, p5, p6, p7 = p
    u2 = p1 + p6
    u3 = u2 + p7
    return p1 + p2, (u2 + p5) + p3, u3 - p4, u3 + p5


W_R = (3, 1, 0, 2, 4, 5, 6)


def _wl_swapped(a11, a12, a21, a22):
    return _wl(a12, a11, a22, a21)


def _wc_swapped(p):
    p1, p2, p3, p4, p5, p6, p7 = p
    v2 = p1 + p6
    u3 = p7 - v2
    return (p5 - v2) + p3, p1 + p2, u3 + p5, p4 - u3


class _Sym:
    def __init__(self, t):
        self.t = t

    def __add__(self, o):
        return _Sym({**self.t, **o.t})

    def __sub__(self, o):
        return _Sym({**self.t, **{k: -v for k, v in o.t.items()}})


def _st(u, ct):
    return slice((4 * ct + u) * 128, (4 * ct + u + 1) * 128)


def _to_st(v):
    return jnp.concatenate([v[:, (2 * u + ct) * 128:(2 * u + ct + 1) * 128]
                            for ct in range(2) for u in range(4)], axis=1)


def _phi(t):
    return jnp.where(t > 0, t + 1.0, jnp.exp(t)) + 1e-6


def _rbf(v):
    return v.astype(bf16).astype(f32)


def _layernorm_rows(xv):
    mf = jnp.sum(xv, axis=1, keepdims=True) * (1.0 / D)
    d = xv - mf
    var = jnp.sum(d * d, axis=1, keepdims=True) * (1.0 / D)
    sd = _rbf(jnp.sqrt(_rbf(_rbf(var) + 1e-5)))
    return _rbf(_rbf(xv - _rbf(mf)) / sd)


def _kernel(x_hbm, wqkv_hbm, wo_hbm, wr_hbm, wg_hbm, wu_hbm, wd_hbm, out_hbm,
            x_buf, wv_buf, wo_buf, wr_buf, wg_buf, wu_buf, wd_buf,
            xs1, xs2, wqs, sa, sb, zacc, zp, pk_buf, xb, yacc, rsel, wrb, zero_buf,
            wks, stats, wqt, ps_raw, qs, ms, tscr, tscr2, pq_raw, den_raw, pqb_buf, denb_buf, qsb,
            mg_raw, hb_raw, out_buf, idx_s, sem):
    wq_buf = out_buf.at[pl.ds(0, D), :]
    wk_buf = out_buf.at[pl.ds(D, D), :]

    def xs_at(k1, e, rows=None):
        r = xs1.at[k1 * 4 + (0, 1, 7, 3).index(e)] if e in (0, 1, 7, 3) else xs2.at[k1 * 4 + (2, 4, 5, 6).index(e)]
        return r if rows is None else r.at[rows, :]

    SEM_B, SEM_O, SEM_Z, SEM_A = 0, 4, 5, 6

    def cp(src, dst, s):
        return pltpu.make_async_copy(src, dst, sem.at[s])

    def cp_x(r0, n, s):
        rows = [pl.ds(_mo(q * HQ + r0, 16), n) for q in range(4)]
        return [cp(x_hbm.at[0, r, :], x_buf.at[r, :], s) for r in rows]

    def cp_wk(c, s):
        return [cp(wqkv_hbm.at[:, pl.ds(_mo(D + c * 256, 256), 256)],
                   wk_buf.at[:, pl.ds(_mo(c * 256, 256), 256)], s)]

    cp_wr = cp(wr_hbm, wr_buf.at[pl.ds(0, D)], SEM_Z)

    def make_a_groups():
        return [
            cp_x(0, 64, SEM_A),
            cp_x(64, 64, SEM_A + 1),
            cp_wk(0, SEM_A + 2),
            cp_wk(1, SEM_A + 3),
            cp_wk(2, SEM_A + 4) + cp_x(128, 64, SEM_A + 4),
            cp_wk(3, SEM_A + 5) + cp_x(192, 128, SEM_A + 5),
            cp_x(320, 192, SEM_A + 6) + [cp(wqkv_hbm.at[:, pl.ds(0, D)], wq_buf, SEM_A + 6)],
        ]

    def cp_b(j, part, wait_only=False):
        pairs = []
        f0, fw = (0, F1) if part == 0 else (F1, FH - F1)
        fs = pl.ds(_mo(j * FH + f0, 128), fw)
        if fw:
          pairs += [(wg_hbm.at[:, fs], wg_buf.at[j, :, pl.ds(f0, fw)]),
                  (wu_hbm.at[:, fs], wu_buf.at[j, :, pl.ds(f0, fw)]),
                  (wd_hbm.at[fs, :], wd_buf.at[j, pl.ds(f0, fw), :])]
        if part == 1:
            for a in range(4):
                c0 = _mo((2 * a + j) * 128, 128)
                pairs += [(wqkv_hbm.at[:, pl.ds(2 * D + c0, 128)], wv_buf.at[j, :, pl.ds(a * 128, 128)]),
                          (wo_hbm.at[pl.ds(c0, 128), :], wo_buf.at[j, pl.ds(a * 128, 128), :])]
        return [cp(dst if wait_only else src, dst, SEM_B + 2 * j + part) for src, dst in pairs]

    clock = [0]
    toks = []
    sides = []
    fwd = [None]

    def emit_tok(vals, stamp=None):
        t = None
        for v in vals:
            v = pltpu.bitcast(v, u32) if v.dtype != u32 else v
            t = v if t is None else t | v
        toks.append((clock[0] if stamp is None else stamp, t & zero_buf[0]))

    def token(kind):
        t = fwd[0]
        if "u" not in t:
            t["u"] = pltpu.bitcast(t["src"](), u32) & zero_buf[0]
        if kind != "u" and "f" not in t:
            t["f"] = pltpu.bitcast(t["u"], f32)
        if kind == "f16" and "f16" not in t:
            t["f16"] = jnp.concatenate([t["f"], t["f"]], axis=0)
        return t[kind]

    def gate(v):
        if fwd[0] is None:
            return v
        head = v if v.shape[0] == 8 else v[0:8]
        head = head | token("u") if v.dtype == u32 else head + token("f")
        return head if v.shape[0] == 8 else jnp.concatenate([head, v[8:]], axis=0)

    def gate16(v):
        return v if fwd[0] is None else v + token("f16")

    def add_side(gen_fn, n, t0, t1, lag=None):
        st = {"i": 0, "n": n, "t0": clock[0] + t0, "t1": clock[0] + t1}

        def tok(vals, extra=0):
            if lag is not None:
                emit_tok(vals, st["t0"] + (st["i"] + 1) * (st["t1"] - st["t0"]) // st["n"] + lag + extra)
        st["g"] = gen_fn(tok)
        sides.append(st)

    def advance(until):
        for st in sides:
            while st["i"] < st["n"] and st["t0"] + st["i"] * (st["t1"] - st["t0"]) // st["n"] < until:
                next(st["g"], None)
                st["i"] += 1
                if st["i"] == st["n"]:
                    for _ in st["g"]:
                        pass

    def flush():
        for st in sides:
            for _ in st["g"]:
                pass
        sides.clear()

    def finish():
        flush()
        toks.clear()
        fwd[0] = None

    def mm(lhs, rhs, dims, cycles, nseg=1):
        due = [t for (c, t) in toks if c <= clock[0]]
        toks[:] = [(c, t) for (c, t) in toks if c > clock[0]]
        if due:
            head = rhs[0:8, 0:128]
            for t in due:
                head = head | t
            if rhs.shape[1] > 128:
                head = jnp.concatenate([head, rhs[0:8, 128:]], axis=1)
            rhs = jnp.concatenate([head, rhs[8:]], axis=0)
        res = _dot(lhs, _unpack(rhs), dims)
        ngr = res.shape[0] // 16
        for sg in range(nseg):
            for i in range(ngr):
                fwd[0] = {"src": lambda sg=sg, i=i: res[i * 16:i * 16 + 8, sg * 128:(sg + 1) * 128]}
                clock[0] += cycles // nseg // ngr
                advance(clock[0])
        return res

    def form_steps(form, form2, get, put, tok=None, keep=range(7), offdiag=False):
        terms = form(*[_Sym({i: 1}) for i in range(4)])
        for k1 in range(7):
            sub = []
            for r in range(2):
                for c in range(2):
                    v = None
                    for i, sg in sorted(terms[k1].t.items(), key=lambda e: -e[1]):
                        b = get(r + 2 * (i // 2), c + 2 * (i % 2))
                        if v is None:
                            v = gate16(b) if (r == c) != offdiag else b
                        else:
                            v = v + b if sg > 0 else v - b
                    sub.append(v)
            vals = form2(*sub) + (sub[2],)
            for k2 in keep:
                put(k1, k2, _pack(vals[k2]))
            if tok is not None and k1 % TOKEV == TOKEV - 1 - (6 % TOKEV != TOKEV - 1):
                full = vals[3 if form2 is _wr else 2]
                tok([full[0:8], full[8:16]])
            yield

    def strassen2(lhs, rhs, dims, cycles, nseg=1, wts=(16,) * 7, comb=_wc):
        m1 = [None] * 7
        for i1, k1 in enumerate(K_SEQ2):
            m2 = [None] * 7
            for k2 in W_SEQ:
                m2[k2] = mm(lhs(k1, k2), rhs(k1, k2), dims, cycles * wts[i1] // 16, nseg)
                yield
            m1[k1] = comb(m2)
        out = [[None] * 4 for _ in range(4)]
        for s2 in range(4):
            for s1, v in enumerate(_combine([m1[k1][s2] for k1 in range(7)])):
                out[(s1 // 2) * 2 + s2 // 2][(s1 % 2) * 2 + s2 % 2] = v
        return out

    made = set()

    def need(*keys):
        assert all(k in made for k in keys), keys

    def row_views(base):
        if isinstance(base, int) and base == 0:
            return x_buf, sa, sb, stats, xn_buf, None
        b = _mo(base, 64)
        return ([r.at[pl.ds(b, S - 64), :] for r in (x_buf, sa, sb, stats)]
                + [xn_buf.at[:, pl.ds(b, 64), :], pl.ds(_mo(base // 2, 32), 32)])

    def xs_form(r0, tok, which="all", base=0):
        xn_v, xs_v = row_views(base)[4:]
        rows = slice(r0 % XN, r0 % XN + 16)

        keep = {"all": range(8), "l1": (0, 1, 7, 3), "l2": (2, 4, 5, 6)}[which]
        for ct in range(2):
            def put(k1, k2, v):
                xs_at(k1, k2, xs_v)[r0 // 2:r0 // 2 + 8, ct * 128:(ct + 1) * 128] = v
            yield from form_steps(
                _sform, _wl, lambda q, u: xn_v[q, rows, _st(u, ct)], put, tok, keep)
        made.add(("xs", r0))

    def ln_stats(r_start, n_rows, tok, base=0):
        x_v, sa_v, sb_v, st_v, xn_v, _ = row_views(base)
        lane = lax.broadcasted_iota(i32, (8, 128), 1)
        for r0 in range(r_start, r_start + n_rows, 16):
            if r0 >= 2 * XN:
                need(("ln", r0 - XN))
            for g in range(8):
                q, o = g // 2, (g % 2) * 8
                rg = q * HQ + r0 + o
                xv = x_v[rg:rg + 8, :].astype(f32)
                xg = jnp.concatenate([gate(xv[:, 0:128]), xv[:, 128:]], axis=1)
                mf = jnp.sum(xg, axis=1, keepdims=True) * (1.0 / D)
                d = xv - mf
                var = jnp.sum(d * d, axis=1, keepdims=True) * (1.0 / D)
                rs = lax.rsqrt(var + 1e-5)
                xn_v.at[q][r0 % XN + o:r0 % XN + o + 8, :] = _to_st(d * rs)
                rs = jnp.broadcast_to(rs, (8, 128))
                mf = jnp.broadcast_to(mf, (8, 128))
                sa_v[rg:rg + 8, :] = 1.0 + rs
                sb_v[rg:rg + 8, :] = mf * rs
                st_v[rg:rg + 8, 0:128] = jnp.where(lane == 0, mf, jnp.broadcast_to(var, (8, 128)))
                if tok is not None:
                    tok([rs])
                if g == 7:
                    made.add(("xn", r0))
                yield

    def ln_later(r_start, n_rows, tok, which="all", base=0):
        st_v, xn_v = row_views(base)[3:5]
        for r0 in range(r_start, r_start + n_rows, 16):
            need(("xn", r0))
            form = xs_form(r0, tok, which, base)
            for g in range(8):
                for _ in range(2 if g < 7 else 0):
                    next(form)
                    yield
                q, o = g // 2, (g % 2) * 8
                t = None
                if which != "l1":
                    v = xn_v[q, r0 % XN + o:r0 % XN + o + 8, :] * wrb[8:16, :]
                    for ct in range(8):
                        h = v[:, ct * 128:(ct + 1) * 128]
                        t = gate(h) if t is None else t + h
                if t is not None:
                    st_v[q * HQ + r0 + o:q * HQ + r0 + o + 8, 128:256] = t
                if tok is not None:
                    tok([t])
                if g == 7:
                    next(form, None)
                    made.add(("ln", r0))
                yield

    def wk_prep(c, tok=None):
        cs = pl.ds(_mo(c * 256, 256), 256)
        for i in range(HD // 16):
            r0 = i * 16
            top = wk_buf[r0:r0 + 16, cs].astype(f32)
            bot = wk_buf[HD + r0:HD + r0 + 16, cs].astype(f32)
            ops = _rform(gate(top[:, :128]), top[:, 128:], bot[:, :128], gate(bot[:, 128:]))
            for k in range(7):
                wks.at[c][r0 // 2:r0 // 2 + 8, k * 128:(k + 1) * 128] = _pack(ops[k])
            yield

    def wq_perm(tok):
        def permute(kt):
            for g in range(8):
                tile = gate(pltpu.bitcast(wq_buf[kt * 128:(kt + 1) * 128, g * 128:(g + 1) * 128], u32))
                wqt.at[kt * 8 + g][...] = pltpu.bitcast(_unpack(tile).T, u32)
                yield

        def back(kt):
            for j in range(8):
                tile = gate(jnp.concatenate([wqt[kt * 8 + g, pl.ds(j, 8, stride=8), :] for g in range(8)],
                                            axis=0))
                v = pltpu.bitcast(_unpack(tile).T.astype(f32), u32)
                c0 = (kt // 2) * D + _st(j // 2, j % 2).start
                ps[(kt % 2) * 128:(kt % 2 + 1) * 128, c0:c0 + 128] = v
                made.add(("wqp", kt, j))
                yield

        order = (0, 2, 4, 6, 1, 3, 5, 7)
        for n in range(10):
            if n < 8:
                yield from permute(order[n])
            if n > 1:
                yield from back(order[n - 2])

    def wq_form(tok):
        for i in range(16):
            need(*[("wqp", 2 * r + i // 8, j) for r in range(4) for j in range(8)])
            for ct in range(2):
                def put(k1, k2, v):
                    wqs.at[k1 * 7 + k2][i * 8:(i + 1) * 8, ct * 128:(ct + 1) * 128] = v
                yield from form_steps(
                    _rform, _wr, lambda r, c: pltpu.bitcast(
                        ps[i * 16:(i + 1) * 16, r * D + _st(c, ct).start:r * D + _st(c, ct).stop],
                        f32), put, tok)

    def kproj(r0, n, chunks=range(4)):
        pr = pl.ds(r0 // 2, n // 2)
        need(*[("xs", r) for r in range(max(r0, 128), r0 + n, 16)])
        for c in chunks:
            m = [None] * 7
            for k in K_SEQ:
                e11, e12, e21, e22 = [xs_at(L_ORD[k], e)[pr, :] for e in (0, 1, 7, 3)]
                lhs = jnp.concatenate([jnp.concatenate([e11, e12], axis=1),
                                       jnp.concatenate([e21, e22], axis=1)], axis=0)
                m[k] = mm(_unpack(lhs), wks[c, :, k * 128:(k + 1) * 128], NN, 2 * n)
            kk = [_phi(v) for v in _combine(m)]
            for ct in range(2):
                zacc[:, pl.ds(_mo(c * 256 + ct * 128, 128), 128)] += (
                    (kk[ct] + kk[2 + ct]).reshape(n // 4, 8, 128).sum(axis=0))
            for s1 in range(4):
                for h in range(2):
                    pk_buf.at[s1 % 2, (s1 // 2) * 2 + h][r0:r0 + n, pl.ds(_mo(c * 128, 128), 128)] = (
                        kk[s1][h * n:(h + 1) * n])

    def z_prep():
        z = jnp.sum(zacc[...], axis=0, keepdims=True)
        zt = _pack(jnp.broadcast_to(z, (128, D)).astype(bf16).T)
        for g in range(8):
            tscr.at[g][...] = zt[g * 64:(g + 1) * 64, :]
        for j in range(8):
            blk = jnp.concatenate([tscr[g, pl.ds(j, 8, stride=8), :] for g in range(8)], axis=0)
            zp[:, j * 128:(j + 1) * 128] = _unpack(blk).T[0:8, :].astype(f32)

    def route(tok):
        need(*[("ln", r) for r in range(128, HQ, 16)])
        rows, dots = [], []
        for b in range(S // 128):
            rows.append(gate(stats[b * 128:(b + 1) * 128, 0:128]).T[0:8, :])
            dots.append(jnp.sum(gate(stats[b * 128:(b + 1) * 128, 128:256]).T, axis=0, keepdims=True))
            yield
        mf = jnp.concatenate([v[0:1] for v in rows], axis=0)
        var = jnp.concatenate([v[1:2] for v in rows], axis=0)
        tr = jnp.concatenate(dots, axis=0) * jnp.sqrt(var + 1e-5)
        wsum = jnp.sum(wrb[0:1, :], axis=1, keepdims=True)
        sd = _rbf(jnp.sqrt(_rbf(_rbf(var) + 1e-5)))
        rv = _rbf((tr + (mf - _rbf(mf)) * wsum) / sd)
        rmax = jnp.max(rv)
        pos = (lax.broadcasted_iota(i32, rv.shape, 0) * 128 + lax.broadcasted_iota(i32, rv.shape, 1))
        idx = jnp.min(jnp.where(rv == rmax, pos, S - 1))
        idx_s[0] = idx
        b0 = _mo((idx // 16) * 16, 16)
        xn = _layernorm_rows(x_buf[pl.ds(b0, 16), :].astype(f32))
        sel = lax.broadcasted_iota(i32, xn.shape, 0) == idx - b0
        row = jnp.sum(jnp.where(sel, xn, 0.0), axis=0, keepdims=True)
        rsel[...] = jnp.broadcast_to(_rbf(jnp.sum(row * wrb[0:1, :], axis=1, keepdims=True)), rsel.shape)
        xbv = jnp.broadcast_to(row, (128, D)).T
        xb[...] = xbv
        yacc[...] = jnp.zeros(yacc.shape, f32)
        tok([xbv[b * 128 + 120:(b + 1) * 128] for b in range(8)])
        yield

    def ps_form(j, tok):
        for c in range(HQ // 16):
            def put(k1, k2, v):
                k = k1 * 7 + k2
                ps[c * 8:(c + 1) * 8, k * 128:(k + 1) * 128] = v
            yield from form_steps(
                _lform, _wl_swapped,
                lambda r, q: pk_buf[j, q, c * 16:(c + 1) * 16, r * 128:(r + 1) * 128], put, tok, offdiag=True)

    def q_rows(j, r0, n, pq, rc, d0, rec):
        xj = pl.ds(_mo(j * (BQ // 2), BQ // 2), BQ // 2)
        pr = slice(r0 // 2, (r0 + n) // 2)
        blk = yield from strassen2(lambda k1, k2: _unpack(xs_at(L_ORD[k1], k2, xj)[pr, :]),
                                   lambda k1, k2: wqs[k1 * 7 + k2], NN, n, 1, QW)
        lane = lax.broadcasted_iota(i32, (n, 128), 1)
        for q in range(4):
            d = None
            for u in (3, 2, 1, 0):
                v = _phi(blk[q][u])
                for ct in range(2):
                    pq.at[q][d0:d0 + n, _st(u, ct)] = v[:, ct * 128:(ct + 1) * 128]
                t = v * zp[0:1, u * 256:(u + 1) * 256]
                t = t[:, :128] + t[:, 128:]
                d = t if d is None else d + t
            if rec:
                d = recip(d, lane)
            rc.at[q][d0:d0 + n, :] = d

    def recip(d, lane):
        d = d + jnp.where(lane % 2 == 0, pltpu.roll(d, 127, 1), pltpu.roll(d, 1, 1))
        d = d + jnp.where(lane % 4 < 2, pltpu.roll(d, 126, 1), pltpu.roll(d, 2, 1))
        return 1.0 / (d + 1e-6)

    def normalise(pq, rc, nr, dst, p0, raw, tok=None):
        lane = lax.broadcasted_iota(i32, (16, 128), 1)

        def fix(c):
            if c < nr // 16 and raw(c * 16):
                for q in range(4):
                    rq = slice(c * 16, (c + 1) * 16)
                    rc.at[q][rq, :] = recip(gate16(rc[q, rq, :]), lane)

        def scale(c):
            rq = slice(c * 16, (c + 1) * 16)
            fix(c + 1)
            for hf in range(2):
                for q in range(4):
                    cs = slice(hf * HD, (hf + 1) * HD)
                    pq.at[q][rq, cs] = pq[q, rq, cs] * jnp.concatenate([gate16(rc[q, rq, :])] * 4, axis=1)
                    yield

        def form(c):
            rq = slice(c * 16, (c + 1) * 16)
            p2 = pl.ds(_mo(p0 + c * 8, 8), 8)
            for ct in range(2):
                def put(k1, k2, v):
                    dst.at[k1 * 7 + k2][p2, ct * 128:(ct + 1) * 128] = v
                yield from form_steps(_lform, _wl, lambda q, u: pq[q, rq, _st(u, ct)], put, tok)

        fix(0)
        if raw(0):
            for _ in range(4):
                yield
        yield from scale(0)
        for c in range(nr // 16):
            nxt = scale(c + 1) if c + 1 < nr // 16 else iter(())
            for i, _ in enumerate(form(c)):
                yield
                if i < 8 and c + 1 < nr // 16:
                    next(nxt)
                    yield
        made.add(("qs", id(dst)))

    hist = []

    def g_lhs(k):
        v = ps[:, k * 128:(k + 1) * 128]
        hist.append(fwd[0])
        if GLAG and len(hist) > GLAG and hist[-1 - GLAG] is not None:
            cur = fwd[0]
            fwd[0] = hist[-1 - GLAG]
            v = jnp.concatenate([gate(v[i * 64:(i + 1) * 64]) for i in range(4)], axis=0)
            fwd[0] = cur
        return _unpack(v)

    def g_kvm(j):
        blk = yield from strassen2(
            lambda k1, k2: g_lhs(k1 * 7 + k2),
            lambda k1, k2: xs_at(R_ORD[k1], W_R[k2])[...], TN, 256, 2, GW, _wc_swapped)
        hm = (lax.broadcasted_iota(i32, (128, 128), 0) // 32
              == lax.broadcasted_iota(i32, (128, 128), 1) // 32)
        qb = q_rows(j, BQ - QB, QB, pqb_buf.at[j], denb_buf.at[j], 0, False)
        for _ in range(QSPLIT):
            next(qb)
        kvps = []
        for a in (3, 2, 1, 0):
            gg = jnp.concatenate(blk[a], axis=1).astype(bf16)
            clock[0] += 256
            kv = jnp.where(hm, _dot(gg, wv_buf[j, :, a * 128:(a + 1) * 128], NN), 0.0)
            tscr2.at[a][...] = _pack(kv)
            kvps.append(_unpack(jnp.concatenate(
                [tscr2[a, pl.ds(jj, 8, stride=8), :] for jj in range(8)], axis=0)))
        mg = mg_buf

        def m_form(tok):
            for a in (3, 2, 1, 0):
                need(("mg", a))
                for jl in range(2):
                    for ct in range(2):
                        def put(k1, k2, v):
                            ms.at[k1 * 7 + k2][pl.ds(_mo(jl * 64 + (2 * a + j) * 8, 8), 8),
                                               ct * 128:(ct + 1) * 128] = v
                        yield from form_steps(
                            _rform, _wr, lambda q, u: mg[a, (2 * q + jl) * 16:(2 * q + jl + 1) * 16, _st(u, ct)], put)

        for i, a in enumerate((3, 2, 1, 0)):
            wo_u = pltpu.bitcast(wo_buf[j, a * 128:(a + 1) * 128, :], u32)
            res = mm(kvps[i], wo_u, NN, 256)
            mg.at[a][...] = _to_st(res)
            made.add(("mg", a))
            if i == 0:
                add_side(m_form, 112, 128, 768 + (49 - QSPLIT) * QB - 100)
        for _ in qb:
            pass

    def out_part(p0, nr, y, src, pr0):
        pr = pl.ds(_mo(pr0, 8), nr // 2)
        rows = [pl.ds(_mo(q * HQ + p0, 16), nr) for q in range(4)]
        row = lax.broadcasted_iota(i32, (nr, 256), 0) + p0
        blk = yield from strassen2(lambda k1, k2: _unpack(src[k1 * 7 + k2, pr, :]),
                                   lambda k1, k2: ms[k1 * 7 + k2], NN, nr)
        for s1 in (3, 2, 1, 0):
            for s2 in range(4):
                q = (s1 // 2) * 2 + s2 // 2
                u = (s1 % 2) * 2 + s2 % 2
                rr, cc = rows[q], pl.ds(u * 256, 256)
                a = jnp.concatenate([sa[rr, :]] * 2, axis=1)
                b = jnp.concatenate([sb[rr, :]] * 2, axis=1)
                o = blk[q][u] + jnp.where(row + q * HQ == idx_s[0], y[:, u * 256:(u + 1) * 256], 0.0)
                out_buf[rr, cc] = (x_buf[rr, cc].astype(f32) * a - b + o).astype(bf16)
                if s2 % 2 == 1:
                    ch = pl.ds((s1 % 2) * HD, HD)
                    cp(out_buf.at[rr, ch], out_hbm.at[0, rr, ch], SEM_O).start()

    def ffn_part(j, f_lo, f_hi):
        def fma(acc, w, v):
            p = w.astype(f32) * v
            return acc + p[0:8] + p[8:16]

        for f0 in range(f_lo, f_hi, 256):
            fs = slice(f0, f0 + 256)
            ag = jnp.zeros((8, 256), f32)
            au = jnp.zeros((8, 256), f32)
            for k in range(0, D, 16):
                xv = jnp.concatenate([gate16(xb[k:k + 16, :])] * 2, axis=1)
                ag = fma(ag, wg_buf[j, k:k + 16, fs], xv)
                au = fma(au, wu_buf[j, k:k + 16, fs], xv)
                yield
            g = _rbf(jnp.sum(ag, axis=0, keepdims=True))
            u = _rbf(jnp.sum(au, axis=0, keepdims=True))
            h = _rbf(_rbf(g * jax.nn.sigmoid(g)) * u)
            hb_buf[fs, :] = jnp.broadcast_to(h, (128, 256)).T
        for d0 in range(0, D, 512):
            ds_ = slice(d0, d0 + 512)
            acc = yacc[:, ds_]
            for k in range(f_lo, f_hi, 16):
                hv = jnp.concatenate([gate16(hb_buf[k:k + 16, :])] * 4, axis=1)
                acc = fma(acc, wd_buf[j, k:k + 16, ds_], hv)
                yield
            yacc[:, ds_] = acc

    def wait_group(i):
        with _scope("a_wait%d" % i):
            for c in a_groups[i]:
                c.wait()

    def run_all(gen):
        for _ in gen:
            pass

    def ln_sides(plan):
        for r0, r1, t0, t1 in plan[0]:
            add_side(lambda tok, r0=r0, r1=r1: ln_stats(r0, r1 - r0, tok), (r1 - r0) // 2, t0, t1, LNLAG)
        for r0, r1, t0, t1 in plan[1]:
            add_side(lambda tok, r0=r0, r1=r1: ln_later(r0, r1 - r0, tok), 22 * (r1 - r0) // 16, t0, t1, SLAG)

    def l2_side(base, n, t0, t1):
        add_side(lambda tok: ln_later(0, n, None, "l2", base), 22 * n // 16, t0, t1)

    a_groups = make_a_groups()
    with _scope("p0_issue"):
        cp_wr.start()
        for grp in a_groups:
            for c in grp:
                c.start()
        for j in range(2):
            for part in range(2):
                for c in cp_b(j, part):
                    c.start()
        zacc[...] = jnp.zeros(zacc.shape, f32)
        zero_buf[1] = jnp.zeros((8, 128), u32)
        cp_zero = cp(zero_buf.at[1], zero_buf.at[0], SEM_Z)
        cp_zero.start()
        cp_zero.wait()
        cp_wr.wait()
        wr8 = jnp.broadcast_to(wr_buf[0:D].reshape(1, D).astype(f32), (8, D))
        wrb[0:8, :] = wr8
        wrb[8:16, :] = _to_st(wr8)
        z0 = jnp.max(pltpu.bitcast(zero_buf[0], i32))
        ps, pq_buf, den_buf, mg_buf, hb_buf = [r.at[z0] for r in (ps_raw, pq_raw, den_raw, mg_raw, hb_raw)]
        xn_buf = mg_buf

    def a01(i, carry):
        with _scope("a_wait01"):
            for c in cp_x(i * 64, 64, SEM_A + i):
                c.wait()
        with _scope("a01"):
            for r in range(0, 64, 16):
                run_all(ln_stats(r, 16, None, i * 64))
                if r:
                    run_all(ln_later(r - 16, 16, None, "l1", i * 64))
            run_all(ln_later(48, 16, None, "l1", i * 64))
        return carry

    lax.fori_loop(0, 2, a01, 0)

    def a23(i, carry):
        with _scope("a_wait23"):
            for c in cp_wk(i, SEM_A + 2 + i):
                c.wait()
        with _scope("a23"):
            run_all(wk_prep(i))
            l2_side(i * 64, 64, 300, 1500)
            kproj(0, 128, [i])
            finish()
        return carry

    lax.fori_loop(0, 2, a23, 0)
    wait_group(4)
    with _scope("a4"):
        run_all(wk_prep(2))
        ln_sides(L4)
        kproj(0, 128, [2])
        finish()
    wait_group(5)
    with _scope("a5"):
        run_all(wk_prep(3))
        ln_sides(L5)
        kproj(0, 128, [3])
        for r0, n in A5K:
            kproj(r0, n)
        finish()
    wait_group(6)
    with _scope("a6"):
        ln_sides(L6)
        add_side(wq_perm, 128, A6[1], A6[2], A6[6])
        add_side(wq_form, 224, A6[3], A6[4], A6[6])
        add_side(route, 17, A6[5], A6[5] + 800)
        for r0, n in A6K:
            kproj(r0, n)
        finish()

    def b_body(j, carry):
        qa = BQ - QB
        with _scope("b_wait0"):
            for c in cp_b(j, 0, wait_only=True) + (cp_b(j, 1, wait_only=True) if MERGE else []):
                c.wait()
        with _scope("b_r0"):
            z_prep()
            t1 = 49 * qa - 400
            add_side(lambda tok: ps_form(j, tok), 7 * HQ // 16, 0, t1, SLAG if MERGE else None)
            if F1:
                add_side(lambda tok: ffn_part(j, 0, F1), F1 * 3 // (4 * FSTEP), 0, t1)
            for r0 in range(0, qa, QN):
                run_all(q_rows(j, r0, min(QN, qa - r0), pq_buf, den_buf, r0, r0 + QN < qa))
            if MERGE:
                flush()
            else:
                finish()
        if not MERGE:
            with _scope("b_wait1"):
                for c in cp_b(j, 1, wait_only=True):
                    c.wait()
        with _scope("b_r1"):
            add_side(lambda tok: ffn_part(j, F1, FB), (FB - F1) * 3 // (4 * FSTEP), 0, R1T[0])
            add_side(lambda tok: normalise(pq_buf, den_buf, qa, qs, j * (qa // 2),
                                           lambda r: (r // QN + 1) * QN >= qa), 22 * (qa // 16), 0, R1T[1])
            run_all(g_kvm(j))
            finish()
        return carry

    lax.fori_loop(0, 2, b_body, 0)

    def c_body(t, carry):
        with _scope("c_body"):
            y = _rbf(jnp.sum(yacc[...], axis=0, keepdims=True))
            y = _rbf(y * _rbf(1.0 / _rbf(1.0 + _rbf(jnp.exp(-rsel[0:1, :])))))
            j, h = t >> 1, t & 1
            na, nb = (BQ - QB) // 2, QB // 2
            hb = pl.ds(_mo(h * nb, 16), nb)
            add_side(lambda tok: normalise(pqb_buf.at[j, :, hb, :], denb_buf.at[j, :, hb, :], nb, qsb, 0,
                                           lambda r: True, tok),
                     4 + 22 * (nb // 16), 0, 49 * na - 800, SLAG)
            for p in range(0, na, CR):
                p0 = j * BQ + h * na + p
                run_all(out_part(p0, min(CR, na - p), y, qs, t * (na // 2) + p // 2))
            advance(clock[0] + 10 ** 6)
            flush()
            run_all(out_part(j * BQ + BQ - QB + h * nb, nb, y, qsb, 0))
            finish()
        return carry

    lax.fori_loop(0, 4, c_body, 0)
    with _scope("tail"):
        cp(out_buf, out_hbm.at[0], SEM_O).wait()


@jax.jit
def pallas_parallel_sum__linear_attn_block__moe_arch_mod__prompt_kernel(
    A_x: jax.Array,
    A_wqkv: jax.Array,
    A_wo: jax.Array,
    B_x: jax.Array,
    B_w_r: jax.Array,
    B_w_gate: jax.Array,
    B_w_up: jax.Array,
    B_w_down: jax.Array,
):
    del B_x
    V = pltpu.VMEM
    scratch = [
        V((S, D), bf16),
        V((2, D, 512), bf16),
        V((2, 512, D), bf16),
        V((8 * D,), bf16),
        V((2, D, FH), bf16),
        V((2, D, FH), bf16),
        V((2, FH, D), bf16),
        V((28, HQ // 2, 256), u32),
        V((28, HQ // 2, 256), u32),
        V((49, 128, 256), u32),
        V((S, 128), f32),
        V((S, 128), f32),
        V((8, D), f32),
        V((8, D), f32),
        V((2, 4, HQ, 512), f32),
        V((D, 128), f32),
        V((8, D), f32),
        V((8, D), f32),
        V((16, D), f32),
        V((4, 8, 128), u32),
        V((4, HD // 2, 7 * 128), u32),
        V((S, 256), f32),
        V((64, 64, 128), u32),
        V((1, HQ // 2, 49 * 128), u32),
        V((49, BQ - QB, 256), u32),
        V((49, 128, 256), u32),
        V((8, 64, 128), u32),
        V((4, 64, 128), u32),
        V((1, 4, BQ - QB, D), f32),
        V((1, 4, BQ - QB, 128), f32),
        V((2, 4, QB, D), f32),
        V((2, 4, QB, 128), f32),
        V((49, QB // 4, 256), u32),
        V((1, 4, 128, D), f32),
        V((1, FH, 128), f32),
        V((S, D), bf16),
        pltpu.SMEM((1,), i32),
        pltpu.SemaphoreType.DMA((13,)),
    ]
    return pl.pallas_call(
        _kernel,
        out_shape=jax.ShapeDtypeStruct((1, S, D), bf16),
        in_specs=[pl.BlockSpec(memory_space=pl.ANY)] * 7,
        out_specs=pl.BlockSpec(memory_space=pl.ANY),
        scratch_shapes=scratch,
        compiler_params=pltpu.CompilerParams(vmem_limit_bytes=VMEM_MB * 1024 * 1024,
                                             disable_bounds_checks=True,
                                             fuse_transposed_lhs_in_matmul=FUSE,
                                             disable_semaphore_checks=True),
    )(A_x, A_wqkv, A_wo, B_w_r, B_w_gate, B_w_up, B_w_down)
```

```python
import contextlib

import jax
import jax.numpy as jnp
from jax import lax
import jax.experimental.pallas as pl
import jax.experimental.pallas.tpu as pltpu

bf16, f32, u32, i32 = jnp.bfloat16, jnp.float32, jnp.uint32, jnp.int32

S = 2048
D = 1024
F = 3584
HP = S // 2
HD = D // 2
HQ = S // 4
BQ = HQ // 2
FH = F // 2
F1 = 0
QB = 64
QN = 48
QW = (28, 36, 36, 6, 2, 2, 2)
A6 = (0, 6200, 9000, 9100, 14000, 10600, None)
TOKEV = 2
A5K = ((128, 48), (176, 48), (224, 32))
LNLAG = 700
L4 = ([(128, 192, 0, 1500)], [])
L5 = ([(192, 320, 1000, 7200)], [(128, 176, 0, 1600), (176, 320, 1700, 8600)])
L6 = ([(320, 512, 0, 6000)], [(320, 384, 800, 3400), (384, 512, 3500, 10400)])
A6K = ((256, 64), (320, 64), (384, 64), (448, 64))
R1T = (12800, 12800)
GW = (16,) * 7
MERGE = False
FB = FH
MF = (128, 3420)
QWB = QW
GLAG = 0
RECQ = True
FUSE = False
QSPLIT = 6
SLAG = 400
FSTEP = 2
CR = 32
XN = 128
VMEM_MB = 120
CT = 128

L_ORD = (2, 3, 0, 1, 4, 5, 6)
R_ORD = (2, 0, 6, 5, 1, 4, 3)

K_SEQ = (1, 4, 0, 2, 3, 5, 6)
K_SEQ2 = (0, 1, 2, 5, 3, 4, 6)
W_SEQ = (0, 1, 5, 6, 4, 2, 3)

NN = (((1,), (0,)), ((), ()))
NT_ = (((1,), (1,)), ((), ()))
TN = (((0,), (0,)), ((), ()))


SCOPES = False


def _scope(name):
    return jax.named_scope(name) if SCOPES else contextlib.nullcontext()


def _mo(v, m):
    return v if isinstance(v, int) else pl.multiple_of(v, m)


def _dot(a, b, dims):
    return lax.dot_general(a, b, dims, preferred_element_type=f32)


def _pack(v):
    return pltpu.bitcast(v.astype(bf16), u32)


def _unpack(v):
    return pltpu.bitcast(v, bf16)


def _combine(m):
    m1, m2, m3, m4, m5, m6, m7 = m
    return m1 + m4 - m5 + m7, m3 + m5, m2 + m4, m1 - m2 + m3 + m6


def _lform(a11, a12, a21, a22):
    return (a11 + a22, a21 + a22, a11, a22, a11 + a12, a21 - a11, a12 - a22)


def _rform(b11, b12, b21, b22):
    return (b11 + b22, b11, b12 - b22, b21 - b11, b22, b11 + b12, b21 + b22)


def _sform(x11, x12, x21, x22):
    return (x11, x22, x11 + x22, x21 + x22, x11 + x12, x21 - x11, x12 - x22)


def _wl(a11, a12, a21, a22):
    s1 = a21 + a22
    s2 = s1 - a11
    return (a11, a12, a12 - s2, a22, s1, s2, a11 - a21)


def _wr(b11, b12, b21, b22):
    t1 = b12 - b11
    t2 = b22 - t1
    return (b11, b21, b22, t2 - b21, t1, t2, b22 - b12)


def _wc(p):
    p1, p2, p3, p4, p5, p6, p7 = p
    u2 = p1 + p6
    u3 = u2 + p7
    return p1 + p2, (u2 + p5) + p3, u3 - p4, u3 + p5


W_R = (3, 1, 0, 2, 4, 5, 6)


def _wl_swapped(a11, a12, a21, a22):
    return _wl(a12, a11, a22, a21)


def _wc_swapped(p):
    p1, p2, p3, p4, p5, p6, p7 = p
    v2 = p1 + p6
    u3 = p7 - v2
    return (p5 - v2) + p3, p1 + p2, u3 + p5, p4 - u3


class _Sym:
    def __init__(self, t):
        self.t = t

    def __add__(self, o):
        return _Sym({**self.t, **o.t})

    def __sub__(self, o):
        return _Sym({**self.t, **{k: -v for k, v in o.t.items()}})


def _st(u, ct):
    return slice((4 * ct + u) * 128, (4 * ct + u + 1) * 128)


def _to_st(v):
    return jnp.concatenate([v[:, (2 * u + ct) * 128:(2 * u + ct + 1) * 128]
                            for ct in range(2) for u in range(4)], axis=1)


def _phi(t):
    return jnp.where(t > 0, t + 1.0, jnp.exp(t)) + 1e-6


def _rbf(v):
    return v.astype(bf16).astype(f32)


def _layernorm_rows(xv):
    mf = jnp.sum(xv, axis=1, keepdims=True) * (1.0 / D)
    d = xv - mf
    var = jnp.sum(d * d, axis=1, keepdims=True) * (1.0 / D)
    sd = _rbf(jnp.sqrt(_rbf(_rbf(var) + 1e-5)))
    return _rbf(_rbf(xv - _rbf(mf)) / sd)


def _kernel(x_hbm, wqkv_hbm, wo_hbm, wr_hbm, wg_hbm, wu_hbm, wd_hbm, out_hbm,
            x_buf, wv_buf, wo_buf, wr_buf, wg_buf, wu_buf, wd_buf,
            xs1, xs2, wqs, sa, sb, zacc, zp, pk_buf, xb, yacc, rsel, wrb, zero_buf,
            wks, stats, wqt, ps_raw, qs, ms, tscr, tscr2, pq_raw, den_raw, pqb_buf, denb_buf, qsb,
            mg_raw, hb_raw, out_buf, idx_s, sem):
    wq_buf = out_buf.at[pl.ds(0, D), :]
    wk_buf = out_buf.at[pl.ds(D, D), :]

    def xs_at(k1, e, rows=None):
        r = xs1.at[k1 * 4 + (0, 1, 7, 3).index(e)] if e in (0, 1, 7, 3) else xs2.at[k1 * 4 + (2, 4, 5, 6).index(e)]
        return r if rows is None else r.at[rows, :]

    SEM_B, SEM_O, SEM_Z, SEM_A = 0, 4, 5, 6

    def cp(src, dst, s):
        return pltpu.make_async_copy(src, dst, sem.at[s])

    def cp_x(r0, n, s):
        rows = [pl.ds(_mo(q * HQ + r0, 16), n) for q in range(4)]
        return [cp(x_hbm.at[0, r, :], x_buf.at[r, :], s) for r in rows]

    def cp_wk(c, s):
        return [cp(wqkv_hbm.at[:, pl.ds(_mo(D + c * 256, 256), 256)],
                   wk_buf.at[:, pl.ds(_mo(c * 256, 256), 256)], s)]

    cp_wr = cp(wr_hbm, wr_buf.at[pl.ds(0, D)], SEM_Z)

    def make_a_groups():
        return [
            cp_x(0, 64, SEM_A),
            cp_x(64, 64, SEM_A + 1),
            cp_wk(0, SEM_A + 2),
            cp_wk(1, SEM_A + 3),
            cp_wk(2, SEM_A + 4) + cp_x(128, 64, SEM_A + 4),
            cp_wk(3, SEM_A + 5) + cp_x(192, 128, SEM_A + 5),
            cp_x(320, 192, SEM_A + 6) + [cp(wqkv_hbm.at[:, pl.ds(0, D)], wq_buf, SEM_A + 6)],
        ]

    def cp_b(j, part, wait_only=False):
        pairs = []
        f0, fw = (0, F1) if part == 0 else (F1, FH - F1)
        fs = pl.ds(_mo(j * FH + f0, 128), fw)
        if fw:
          pairs += [(wg_hbm.at[:, fs], wg_buf.at[j, :, pl.ds(f0, fw)]),
                  (wu_hbm.at[:, fs], wu_buf.at[j, :, pl.ds(f0, fw)]),
                  (wd_hbm.at[fs, :], wd_buf.at[j, pl.ds(f0, fw), :])]
        if part == 1:
            for a in range(4):
                c0 = _mo((2 * a + j) * 128, 128)
                pairs += [(wqkv_hbm.at[:, pl.ds(2 * D + c0, 128)], wv_buf.at[j, :, pl.ds(a * 128, 128)]),
                          (wo_hbm.at[pl.ds(c0, 128), :], wo_buf.at[j, pl.ds(a * 128, 128), :])]
        return [cp(dst if wait_only else src, dst, SEM_B + 2 * j + part) for src, dst in pairs]

    clock = [0]
    toks = []
    sides = []
    fwd = [None]

    def emit_tok(vals, stamp=None):
        t = None
        for v in vals:
            v = pltpu.bitcast(v, u32) if v.dtype != u32 else v
            t = v if t is None else t | v
        toks.append((clock[0] if stamp is None else stamp, t & zero_buf[0]))

    def token(kind):
        t = fwd[0]
        if "u" not in t:
            t["u"] = pltpu.bitcast(t["src"](), u32) & zero_buf[0]
        if kind != "u" and "f" not in t:
            t["f"] = pltpu.bitcast(t["u"], f32)
        if kind == "f16" and "f16" not in t:
            t["f16"] = jnp.concatenate([t["f"], t["f"]], axis=0)
        return t[kind]

    def gate(v):
        if fwd[0] is None:
            return v
        head = v if v.shape[0] == 8 else v[0:8]
        head = head | token("u") if v.dtype == u32 else head + token("f")
        return head if v.shape[0] == 8 else jnp.concatenate([head, v[8:]], axis=0)

    def gate16(v):
        return v if fwd[0] is None else v + token("f16")

    def add_side(gen_fn, n, t0, t1, lag=None):
        st = {"i": 0, "n": n, "t0": clock[0] + t0, "t1": clock[0] + t1}

        def tok(vals, extra=0):
            if lag is not None:
                emit_tok(vals, st["t0"] + (st["i"] + 1) * (st["t1"] - st["t0"]) // st["n"] + lag + extra)
        st["g"] = gen_fn(tok)
        sides.append(st)

    def advance(until):
        for st in sides:
            while st["i"] < st["n"] and st["t0"] + st["i"] * (st["t1"] - st["t0"]) // st["n"] < until:
                next(st["g"], None)
                st["i"] += 1
                if st["i"] == st["n"]:
                    for _ in st["g"]:
                        pass

    def flush():
        for st in sides:
            for _ in st["g"]:
                pass
        sides.clear()

    def finish():
        flush()
        toks.clear()
        fwd[0] = None

    def mm(lhs, rhs, dims, cycles, nseg=1):
        due = [t for (c, t) in toks if c <= clock[0]]
        toks[:] = [(c, t) for (c, t) in toks if c > clock[0]]
        if due:
            head = rhs[0:8, 0:128]
            for t in due:
                head = head | t
            if rhs.shape[1] > 128:
                head = jnp.concatenate([head, rhs[0:8, 128:]], axis=1)
            rhs = jnp.concatenate([head, rhs[8:]], axis=0)
        res = _dot(lhs, _unpack(rhs), dims)
        ngr = res.shape[0] // 16
        for sg in range(nseg):
            for i in range(ngr):
                fwd[0] = {"src": lambda sg=sg, i=i: res[i * 16:i * 16 + 8, sg * 128:(sg + 1) * 128]}
                clock[0] += cycles // nseg // ngr
                advance(clock[0])
        return res

    def form_steps(form, form2, get, put, tok=None, keep=range(7), offdiag=False):
        terms = form(*[_Sym({i: 1}) for i in range(4)])
        for k1 in range(7):
            sub = []
            for r in range(2):
                for c in range(2):
                    v = None
                    for i, sg in sorted(terms[k1].t.items(), key=lambda e: -e[1]):
                        b = get(r + 2 * (i // 2), c + 2 * (i % 2))
                        if v is None:
                            v = gate16(b) if (r == c) != offdiag else b
                        else:
                            v = v + b if sg > 0 else v - b
                    sub.append(v)
            vals = form2(*sub) + (sub[2],)
            for k2 in keep:
                put(k1, k2, _pack(vals[k2]))
            if tok is not None and k1 % TOKEV == TOKEV - 1 - (6 % TOKEV != TOKEV - 1):
                full = vals[3 if form2 is _wr else 2]
                tok([full[0:8], full[8:16]])
            yield

    def strassen2(lhs, rhs, dims, cycles, nseg=1, wts=(16,) * 7, comb=_wc):
        m1 = [None] * 7
        for i1, k1 in enumerate(K_SEQ2):
            m2 = [None] * 7
            for k2 in W_SEQ:
                m2[k2] = mm(lhs(k1, k2), rhs(k1, k2), dims, cycles * wts[i1] // 16, nseg)
                yield
            m1[k1] = comb(m2)
        out = [[None] * 4 for _ in range(4)]
        for s2 in range(4):
            for s1, v in enumerate(_combine([m1[k1][s2] for k1 in range(7)])):
                out[(s1 // 2) * 2 + s2 // 2][(s1 % 2) * 2 + s2 % 2] = v
        return out

    made = set()

    def need(*keys):
        assert all(k in made for k in keys), keys

    def row_views(base):
        if isinstance(base, int) and base == 0:
            return x_buf, sa, sb, stats, xn_buf, None
        b = _mo(base, 64)
        return ([r.at[pl.ds(b, S - 64), :] for r in (x_buf, sa, sb, stats)]
                + [xn_buf.at[:, pl.ds(b, 64), :], pl.ds(_mo(base // 2, 32), 32)])

    def xs_form(r0, tok, which="all", base=0):
        xn_v, xs_v = row_views(base)[4:]
        rows = slice(r0 % XN, r0 % XN + 16)

        keep = {"all": range(8), "l1": (0, 1, 7, 3), "l2": (2, 4, 5, 6)}[which]
        for ct in range(2):
            def put(k1, k2, v):
                xs_at(k1, k2, xs_v)[r0 // 2:r0 // 2 + 8, ct * 128:(ct + 1) * 128] = v
            yield from form_steps(
                _sform, _wl, lambda q, u: xn_v[q, rows, _st(u, ct)], put, tok, keep)
        made.add(("xs", r0))

    def ln_stats(r_start, n_rows, tok, base=0):
        x_v, sa_v, sb_v, st_v, xn_v, _ = row_views(base)
        lane = lax.broadcasted_iota(i32, (8, 128), 1)
        for r0 in range(r_start, r_start + n_rows, 16):
            if r0 >= 2 * XN:
                need(("ln", r0 - XN))
            for g in range(8):
                q, o = g // 2, (g % 2) * 8
                rg = q * HQ + r0 + o
                xv = x_v[rg:rg + 8, :].astype(f32)
                xg = jnp.concatenate([gate(xv[:, 0:128]), xv[:, 128:]], axis=1)
                mf = jnp.sum(xg, axis=1, keepdims=True) * (1.0 / D)
                d = xv - mf
                var = jnp.sum(d * d, axis=1, keepdims=True) * (1.0 / D)
                rs = lax.rsqrt(var + 1e-5)
                xn_v.at[q][r0 % XN + o:r0 % XN + o + 8, :] = _to_st(d * rs)
                rs = jnp.broadcast_to(rs, (8, 128))
                mf = jnp.broadcast_to(mf, (8, 128))
                sa_v[rg:rg + 8, :] = 1.0 + rs
                sb_v[rg:rg + 8, :] = mf * rs
                st_v[rg:rg + 8, 0:128] = jnp.where(lane == 0, mf, jnp.broadcast_to(var, (8, 128)))
                if tok is not None:
                    tok([rs])
                if g == 7:
                    made.add(("xn", r0))
                yield

    def ln_later(r_start, n_rows, tok, which="all", base=0):
        st_v, xn_v = row_views(base)[3:5]
        for r0 in range(r_start, r_start + n_rows, 16):
            need(("xn", r0))
            form = xs_form(r0, tok, which, base)
            for g in range(8):
                for _ in range(2 if g < 7 else 0):
                    next(form)
                    yield
                q, o = g // 2, (g % 2) * 8
                t = None
                if which != "l1":
                    v = xn_v[q, r0 % XN + o:r0 % XN + o + 8, :] * wrb[8:16, :]
                    for ct in range(8):
                        h = v[:, ct * 128:(ct + 1) * 128]
                        t = gate(h) if t is None else t + h
                if t is not None:
                    st_v[q * HQ + r0 + o:q * HQ + r0 + o + 8, 128:256] = t
                if tok is not None:
                    tok([t])
                if g == 7:
                    next(form, None)
                    made.add(("ln", r0))
                yield

    def wk_prep(c, tok=None):
        cs = pl.ds(_mo(c * 256, 256), 256)
        for i in range(HD // 16):
            r0 = i * 16
            top = wk_buf[r0:r0 + 16, cs].astype(f32)
            bot = wk_buf[HD + r0:HD + r0 + 16, cs].astype(f32)
            ops = _rform(gate(top[:, :128]), top[:, 128:], bot[:, :128], gate(bot[:, 128:]))
            for k in range(7):
                wks.at[c][r0 // 2:r0 // 2 + 8, k * 128:(k + 1) * 128] = _pack(ops[k])
            yield

    def wq_perm(tok):
        def permute(kt):
            for g in range(8):
                tile = gate(pltpu.bitcast(wq_buf[kt * 128:(kt + 1) * 128, g * 128:(g + 1) * 128], u32))
                wqt.at[kt * 8 + g][...] = pltpu.bitcast(_unpack(tile).T, u32)
                yield

        def back(kt):
            for j in range(8):
                tile = gate(jnp.concatenate([wqt[kt * 8 + g, pl.ds(j, 8, stride=8), :] for g in range(8)],
                                            axis=0))
                v = pltpu.bitcast(_unpack(tile).T.astype(f32), u32)
                c0 = (kt // 2) * D + _st(j // 2, j % 2).start
                ps[(kt % 2) * 128:(kt % 2 + 1) * 128, c0:c0 + 128] = v
                made.add(("wqp", kt, j))
                yield

        order = (0, 2, 4, 6, 1, 3, 5, 7)
        for n in range(10):
            if n < 8:
                yield from permute(order[n])
            if n > 1:
                yield from back(order[n - 2])

    def wq_form(tok):
        for i in range(16):
            need(*[("wqp", 2 * r + i // 8, j) for r in range(4) for j in range(8)])
            for ct in range(2):
                def put(k1, k2, v):
                    wqs.at[k1 * 7 + k2][i * 8:(i + 1) * 8, ct * 128:(ct + 1) * 128] = v
                yield from form_steps(
                    _rform, _wr, lambda r, c: pltpu.bitcast(
                        ps[i * 16:(i + 1) * 16, r * D + _st(c, ct).start:r * D + _st(c, ct).stop],
                        f32), put, tok)

    def kproj(r0, n, chunks=range(4)):
        pr = pl.ds(r0 // 2, n // 2)
        need(*[("xs", r) for r in range(max(r0, 128), r0 + n, 16)])
        for c in chunks:
            m = [None] * 7
            for k in K_SEQ:
                e11, e12, e21, e22 = [xs_at(L_ORD[k], e)[pr, :] for e in (0, 1, 7, 3)]
                lhs = jnp.concatenate([jnp.concatenate([e11, e12], axis=1),
                                       jnp.concatenate([e21, e22], axis=1)], axis=0)
                m[k] = mm(_unpack(lhs), wks[c, :, k * 128:(k + 1) * 128], NN, 2 * n)
            kk = [_phi(v) for v in _combine(m)]
            for ct in range(2):
                zacc[:, pl.ds(_mo(c * 256 + ct * 128, 128), 128)] += (
                    (kk[ct] + kk[2 + ct]).reshape(n // 4, 8, 128).sum(axis=0))
            for s1 in range(4):
                for h in range(2):
                    pk_buf.at[s1 % 2, (s1 // 2) * 2 + h][r0:r0 + n, pl.ds(_mo(c * 128, 128), 128)] = (
                        kk[s1][h * n:(h + 1) * n])

    def z_prep():
        z = jnp.sum(zacc[...], axis=0, keepdims=True)
        zt = _pack(jnp.broadcast_to(z, (128, D)).astype(bf16).T)
        for g in range(8):
            tscr.at[g][...] = zt[g * 64:(g + 1) * 64, :]
        for j in range(8):
            blk = jnp.concatenate([tscr[g, pl.ds(j, 8, stride=8), :] for g in range(8)], axis=0)
            zp[:, j * 128:(j + 1) * 128] = _unpack(blk).T[0:8, :].astype(f32)

    def route(tok):
        need(*[("ln", r) for r in range(128, HQ, 16)])
        rows, dots = [], []
        for b in range(S // 128):
            rows.append(gate(stats[b * 128:(b + 1) * 128, 0:128]).T[0:8, :])
            dots.append(jnp.sum(gate(stats[b * 128:(b + 1) * 128, 128:256]).T, axis=0, keepdims=True))
            yield
        mf = jnp.concatenate([v[0:1] for v in rows], axis=0)
        var = jnp.concatenate([v[1:2] for v in rows], axis=0)
        tr = jnp.concatenate(dots, axis=0) * jnp.sqrt(var + 1e-5)
        wsum = jnp.sum(wrb[0:1, :], axis=1, keepdims=True)
        sd = _rbf(jnp.sqrt(_rbf(_rbf(var) + 1e-5)))
        rv = _rbf((tr + (mf - _rbf(mf)) * wsum) / sd)
        rmax = jnp.max(rv)
        pos = (lax.broadcasted_iota(i32, rv.shape, 0) * 128 + lax.broadcasted_iota(i32, rv.shape, 1))
        idx = jnp.min(jnp.where(rv == rmax, pos, S - 1))
        idx_s[0] = idx
        b0 = _mo((idx // 16) * 16, 16)
        xn = _layernorm_rows(x_buf[pl.ds(b0, 16), :].astype(f32))
        sel = lax.broadcasted_iota(i32, xn.shape, 0) == idx - b0
        row = jnp.sum(jnp.where(sel, xn, 0.0), axis=0, keepdims=True)
        rsel[...] = jnp.broadcast_to(_rbf(jnp.sum(row * wrb[0:1, :], axis=1, keepdims=True)), rsel.shape)
        xbv = jnp.broadcast_to(row, (128, D)).T
        xb[...] = xbv
        yacc[...] = jnp.zeros(yacc.shape, f32)
        tok([xbv[b * 128 + 120:(b + 1) * 128] for b in range(8)])
        yield

    def ps_form(j, tok):
        for c in range(HQ // 16):
            def put(k1, k2, v):
                k = k1 * 7 + k2
                ps[c * 8:(c + 1) * 8, k * 128:(k + 1) * 128] = v
            yield from form_steps(
                _lform, _wl_swapped,
                lambda r, q: pk_buf[j, q, c * 16:(c + 1) * 16, r * 128:(r + 1) * 128], put, tok, offdiag=True)

    def q_rows(j, r0, n, pq, rc, d0, rec, wts=None):
        xj = pl.ds(_mo(j * (BQ // 2), BQ // 2), BQ // 2)
        pr = slice(r0 // 2, (r0 + n) // 2)
        blk = yield from strassen2(lambda k1, k2: _unpack(xs_at(L_ORD[k1], k2, xj)[pr, :]),
                                   lambda k1, k2: wqs[k1 * 7 + k2], NN, n, 1, wts or QW)
        lane = lax.broadcasted_iota(i32, (n, 128), 1)
        for q in range(4):
            d = None
            for u in (3, 2, 1, 0):
                v = _phi(blk[q][u])
                for ct in range(2):
                    pq.at[q][d0:d0 + n, _st(u, ct)] = v[:, ct * 128:(ct + 1) * 128]
                t = v * zp[0:1, u * 256:(u + 1) * 256]
                t = t[:, :128] + t[:, 128:]
                d = t if d is None else d + t
            if rec:
                d = recip(d, lane)
            rc.at[q][d0:d0 + n, :] = d

    def recip(d, lane):
        d = d + jnp.where(lane % 2 == 0, pltpu.roll(d, 127, 1), pltpu.roll(d, 1, 1))
        d = d + jnp.where(lane % 4 < 2, pltpu.roll(d, 126, 1), pltpu.roll(d, 2, 1))
        return 1.0 / (d + 1e-6)

    def normalise(pq, rc, nr, dst, p0, raw, tok=None):
        lane = lax.broadcasted_iota(i32, (16, 128), 1)

        def fix(c):
            if c < nr // 16 and raw(c * 16):
                for q in range(4):
                    rq = slice(c * 16, (c + 1) * 16)
                    rc.at[q][rq, :] = recip(gate16(rc[q, rq, :]), lane)

        def scale(c):
            rq = slice(c * 16, (c + 1) * 16)
            fix(c + 1)
            for hf in range(2):
                for q in range(4):
                    cs = slice(hf * HD, (hf + 1) * HD)
                    pq.at[q][rq, cs] = pq[q, rq, cs] * jnp.concatenate([gate16(rc[q, rq, :])] * 4, axis=1)
                    yield

        def form(c):
            rq = slice(c * 16, (c + 1) * 16)
            p2 = pl.ds(_mo(p0 + c * 8, 8), 8)
            for ct in range(2):
                def put(k1, k2, v):
                    dst.at[k1 * 7 + k2][p2, ct * 128:(ct + 1) * 128] = v
                yield from form_steps(_lform, _wl, lambda q, u: pq[q, rq, _st(u, ct)], put, tok)

        fix(0)
        if raw(0):
            for _ in range(4):
                yield
        yield from scale(0)
        for c in range(nr // 16):
            nxt = scale(c + 1) if c + 1 < nr // 16 else iter(())
            for i, _ in enumerate(form(c)):
                yield
                if i < 8 and c + 1 < nr // 16:
                    next(nxt)
                    yield
        made.add(("qs", id(dst)))

    hist = []

    def g_lhs(k):
        v = ps[:, k * 128:(k + 1) * 128]
        hist.append(fwd[0])
        if GLAG and len(hist) > GLAG and hist[-1 - GLAG] is not None:
            cur = fwd[0]
            fwd[0] = hist[-1 - GLAG]
            v = jnp.concatenate([gate(v[i * 64:(i + 1) * 64]) for i in range(4)], axis=0)
            fwd[0] = cur
        return _unpack(v)

    def g_kvm(j):
        blk = yield from strassen2(
            lambda k1, k2: g_lhs(k1 * 7 + k2),
            lambda k1, k2: xs_at(R_ORD[k1], W_R[k2])[...], TN, 256, 2, GW, _wc_swapped)
        hm = (lax.broadcasted_iota(i32, (128, 128), 0) // 32
              == lax.broadcasted_iota(i32, (128, 128), 1) // 32)
        qb = q_rows(j, BQ - QB, QB, pqb_buf.at[j], denb_buf.at[j], 0, False, QWB)
        for _ in range(QSPLIT):
            next(qb)
        kvps = []
        for a in (3, 2, 1, 0):
            gg = jnp.concatenate(blk[a], axis=1).astype(bf16)
            wv_u = pltpu.bitcast(wv_buf[j, :, a * 128:(a + 1) * 128], u32)
            kv = jnp.where(hm, mm(gg, wv_u, NN, 256), 0.0)
            tscr2.at[a][...] = _pack(kv)
            kvps.append(_unpack(jnp.concatenate(
                [tscr2[a, pl.ds(jj, 8, stride=8), :] for jj in range(8)], axis=0)))
        mg = mg_buf

        def m_form(tok):
            for a in (3, 2, 1, 0):
                need(("mg", a))
                for jl in range(2):
                    for ct in range(2):
                        def put(k1, k2, v):
                            ms.at[k1 * 7 + k2][pl.ds(_mo(jl * 64 + (2 * a + j) * 8, 8), 8),
                                               ct * 128:(ct + 1) * 128] = v
                        yield from form_steps(
                            _rform, _wr, lambda q, u: mg[a, (2 * q + jl) * 16:(2 * q + jl + 1) * 16, _st(u, ct)], put)

        for i, a in enumerate((3, 2, 1, 0)):
            wo_u = pltpu.bitcast(wo_buf[j, a * 128:(a + 1) * 128, :], u32)
            res = mm(kvps[i], wo_u, NN, 256)
            mg.at[a][...] = _to_st(res)
            made.add(("mg", a))
            if i == 0:
                add_side(m_form, 112, MF[0], MF[1])
        for _ in qb:
            pass

    def out_part(p0, nr, y, src, pr0):
        pr = pl.ds(_mo(pr0, 8), nr // 2)
        rows = [pl.ds(_mo(q * HQ + p0, 16), nr) for q in range(4)]
        row = lax.broadcasted_iota(i32, (nr, 256), 0) + p0
        blk = yield from strassen2(lambda k1, k2: _unpack(src[k1 * 7 + k2, pr, :]),
                                   lambda k1, k2: ms[k1 * 7 + k2], NN, nr)
        for s1 in (3, 2, 1, 0):
            for s2 in range(4):
                q = (s1 // 2) * 2 + s2 // 2
                u = (s1 % 2) * 2 + s2 % 2
                rr, cc = rows[q], pl.ds(u * 256, 256)
                a = jnp.concatenate([sa[rr, :]] * 2, axis=1)
                b = jnp.concatenate([sb[rr, :]] * 2, axis=1)
                o = blk[q][u] + jnp.where(row + q * HQ == idx_s[0], y[:, u * 256:(u + 1) * 256], 0.0)
                out_buf[rr, cc] = (x_buf[rr, cc].astype(f32) * a - b + o).astype(bf16)
                if s2 % 2 == 1:
                    ch = pl.ds((s1 % 2) * HD, HD)
                    cp(out_buf.at[rr, ch], out_hbm.at[0, rr, ch], SEM_O).start()

    def ffn_part(j, f_lo, f_hi):
        def fma(acc, w, v):
            p = w.astype(f32) * v
            return acc + p[0:8] + p[8:16]

        for f0 in range(f_lo, f_hi, 256):
            fs = slice(f0, f0 + 256)
            ag = jnp.zeros((8, 256), f32)
            au = jnp.zeros((8, 256), f32)
            for k in range(0, D, 16):
                xv = jnp.concatenate([gate16(xb[k:k + 16, :])] * 2, axis=1)
                ag = fma(ag, wg_buf[j, k:k + 16, fs], xv)
                au = fma(au, wu_buf[j, k:k + 16, fs], xv)
                yield
            g = _rbf(jnp.sum(ag, axis=0, keepdims=True))
            u = _rbf(jnp.sum(au, axis=0, keepdims=True))
            h = _rbf(_rbf(g * jax.nn.sigmoid(g)) * u)
            hb_buf[fs, :] = jnp.broadcast_to(h, (128, 256)).T
        for d0 in range(0, D, 512):
            ds_ = slice(d0, d0 + 512)
            acc = yacc[:, ds_]
            for k in range(f_lo, f_hi, 16):
                hv = jnp.concatenate([gate16(hb_buf[k:k + 16, :])] * 4, axis=1)
                acc = fma(acc, wd_buf[j, k:k + 16, ds_], hv)
                yield
            yacc[:, ds_] = acc

    def wait_group(i):
        with _scope("a_wait%d" % i):
            for c in a_groups[i]:
                c.wait()

    def run_all(gen):
        for _ in gen:
            pass

    def ln_sides(plan):
        for r0, r1, t0, t1 in plan[0]:
            add_side(lambda tok, r0=r0, r1=r1: ln_stats(r0, r1 - r0, tok), (r1 - r0) // 2, t0, t1, LNLAG)
        for r0, r1, t0, t1 in plan[1]:
            add_side(lambda tok, r0=r0, r1=r1: ln_later(r0, r1 - r0, tok), 22 * (r1 - r0) // 16, t0, t1, SLAG)

    def l2_side(base, n, t0, t1):
        add_side(lambda tok: ln_later(0, n, None, "l2", base), 22 * n // 16, t0, t1)

    a_groups = make_a_groups()
    with _scope("p0_issue"):
        cp_wr.start()
        for grp in a_groups:
            for c in grp:
                c.start()
        for j in range(2):
            for part in range(2):
                for c in cp_b(j, part):
                    c.start()
        zacc[...] = jnp.zeros(zacc.shape, f32)
        zero_buf[1] = jnp.zeros((8, 128), u32)
        cp_zero = cp(zero_buf.at[1], zero_buf.at[0], SEM_Z)
        cp_zero.start()
        cp_zero.wait()
        cp_wr.wait()
        wr8 = jnp.broadcast_to(wr_buf[0:D].reshape(1, D).astype(f32), (8, D))
        wrb[0:8, :] = wr8
        wrb[8:16, :] = _to_st(wr8)
        z0 = jnp.max(pltpu.bitcast(zero_buf[0], i32))
        ps, pq_buf, den_buf, mg_buf, hb_buf = [r.at[z0] for r in (ps_raw, pq_raw, den_raw, mg_raw, hb_raw)]
        xn_buf = mg_buf

    def a01(i, carry):
        with _scope("a_wait01"):
            for c in cp_x(i * 64, 64, SEM_A + i):
                c.wait()
        with _scope("a01"):
            for r in range(0, 64, 16):
                run_all(ln_stats(r, 16, None, i * 64))
                if r:
                    run_all(ln_later(r - 16, 16, None, "l1", i * 64))
            run_all(ln_later(48, 16, None, "l1", i * 64))
        return carry

    lax.fori_loop(0, 2, a01, 0)

    def a23(i, carry):
        with _scope("a_wait23"):
            for c in cp_wk(i, SEM_A + 2 + i):
                c.wait()
        with _scope("a23"):
            run_all(wk_prep(i))
            l2_side(i * 64, 64, 300, 1500)
            kproj(0, 128, [i])
            finish()
        return carry

    lax.fori_loop(0, 2, a23, 0)
    wait_group(4)
    with _scope("a4"):
        run_all(wk_prep(2))
        ln_sides(L4)
        kproj(0, 128, [2])
        finish()
    wait_group(5)
    with _scope("a5"):
        run_all(wk_prep(3))
        ln_sides(L5)
        kproj(0, 128, [3])
        for r0, n in A5K:
            kproj(r0, n)
        finish()
    wait_group(6)
    with _scope("a6"):
        ln_sides(L6)
        add_side(wq_perm, 128, A6[1], A6[2], A6[6])
        add_side(wq_form, 224, A6[3], A6[4], A6[6])
        add_side(route, 17, A6[5], A6[5] + 800)
        for r0, n in A6K:
            kproj(r0, n)
        finish()

    def b_body(j, carry):
        qa = BQ - QB
        with _scope("b_wait0"):
            for c in cp_b(j, 0, wait_only=True) + (cp_b(j, 1, wait_only=True) if MERGE else []):
                c.wait()
        with _scope("b_r0"):
            z_prep()
            t1 = 49 * qa - 400
            add_side(lambda tok: ps_form(j, tok), 7 * HQ // 16, 0, t1, SLAG if MERGE else None)
            if F1:
                add_side(lambda tok: ffn_part(j, 0, F1), F1 * 3 // (4 * FSTEP), 0, t1)
            for r0 in range(0, qa, QN):
                run_all(q_rows(j, r0, min(QN, qa - r0), pq_buf, den_buf, r0, r0 + QN < qa))
            if MERGE:
                flush()
            else:
                finish()
        if not MERGE:
            with _scope("b_wait1"):
                for c in cp_b(j, 1, wait_only=True):
                    c.wait()
        with _scope("b_r1"):
            add_side(lambda tok: ffn_part(j, F1, FB), (FB - F1) * 3 // (4 * FSTEP), 0, R1T[0])
            add_side(lambda tok: normalise(pq_buf, den_buf, qa, qs, j * (qa // 2),
                                           lambda r: (r // QN + 1) * QN >= qa), 22 * (qa // 16), 0, R1T[1])
            run_all(g_kvm(j))
            finish()
        return carry

    lax.fori_loop(0, 2, b_body, 0)

    def c_body(t, carry):
        with _scope("c_body"):
            y = _rbf(jnp.sum(yacc[...], axis=0, keepdims=True))
            y = _rbf(y * _rbf(1.0 / _rbf(1.0 + _rbf(jnp.exp(-rsel[0:1, :])))))
            j, h = t >> 1, t & 1
            na, nb = (BQ - QB) // 2, QB // 2
            hb = pl.ds(_mo(h * nb, 16), nb)
            add_side(lambda tok: normalise(pqb_buf.at[j, :, hb, :], denb_buf.at[j, :, hb, :], nb, qsb, 0,
                                           lambda r: True, tok),
                     4 + 22 * (nb // 16), 0, 49 * na - 800, SLAG)
            for p in range(0, na, CR):
                p0 = j * BQ + h * na + p
                run_all(out_part(p0, min(CR, na - p), y, qs, t * (na // 2) + p // 2))
            advance(clock[0] + 10 ** 6)
            flush()
            run_all(out_part(j * BQ + BQ - QB + h * nb, nb, y, qsb, 0))
            finish()
        return carry

    lax.fori_loop(0, 4, c_body, 0)
    with _scope("tail"):
        cp(out_buf, out_hbm.at[0], SEM_O).wait()


@jax.jit
def pallas_parallel_sum__linear_attn_block__moe_arch_mod__prompt_kernel(
    A_x: jax.Array,
    A_wqkv: jax.Array,
    A_wo: jax.Array,
    B_x: jax.Array,
    B_w_r: jax.Array,
    B_w_gate: jax.Array,
    B_w_up: jax.Array,
    B_w_down: jax.Array,
):
    del B_x
    V = pltpu.VMEM
    scratch = [
        V((S, D), bf16),
        V((2, D, 512), bf16),
        V((2, 512, D), bf16),
        V((8 * D,), bf16),
        V((2, D, FH), bf16),
        V((2, D, FH), bf16),
        V((2, FH, D), bf16),
        V((28, HQ // 2, 256), u32),
        V((28, HQ // 2, 256), u32),
        V((49, 128, 256), u32),
        V((S, 128), f32),
        V((S, 128), f32),
        V((8, D), f32),
        V((8, D), f32),
        V((2, 4, HQ, 512), f32),
        V((D, 128), f32),
        V((8, D), f32),
        V((8, D), f32),
        V((16, D), f32),
        V((4, 8, 128), u32),
        V((4, HD // 2, 7 * 128), u32),
        V((S, 256), f32),
        V((64, 64, 128), u32),
        V((1, HQ // 2, 49 * 128), u32),
        V((49, BQ - QB, 256), u32),
        V((49, 128, 256), u32),
        V((8, 64, 128), u32),
        V((4, 64, 128), u32),
        V((1, 4, BQ - QB, D), f32),
        V((1, 4, BQ - QB, 128), f32),
        V((2, 4, QB, D), f32),
        V((2, 4, QB, 128), f32),
        V((49, QB // 4, 256), u32),
        V((1, 4, 128, D), f32),
        V((1, FH, 128), f32),
        V((S, D), bf16),
        pltpu.SMEM((1,), i32),
        pltpu.SemaphoreType.DMA((13,)),
    ]
    return pl.pallas_call(
        _kernel,
        out_shape=jax.ShapeDtypeStruct((1, S, D), bf16),
        in_specs=[pl.BlockSpec(memory_space=pl.ANY)] * 7,
        out_specs=pl.BlockSpec(memory_space=pl.ANY),
        scratch_shapes=scratch,
        compiler_params=pltpu.CompilerParams(vmem_limit_bytes=VMEM_MB * 1024 * 1024,
                                             disable_bounds_checks=True,
                                             fuse_transposed_lhs_in_matmul=FUSE,
                                             disable_semaphore_checks=True),
    )(A_x, A_wqkv, A_wo, B_w_r, B_w_gate, B_w_up, B_w_down)
```

```python
import contextlib

import jax
import jax.numpy as jnp
from jax import lax
import jax.experimental.pallas as pl
import jax.experimental.pallas.tpu as pltpu

bf16, f32, u32, i32 = jnp.bfloat16, jnp.float32, jnp.uint32, jnp.int32

S = 2048
D = 1024
F = 3584
HP = S // 2
HD = D // 2
HQ = S // 4
BQ = HQ // 2
FH = F // 2
F1 = 0
QB = 64
QN = 48
QW = (28, 36, 36, 6, 2, 2, 2)
A6 = (0, 6200, 9000, 9100, 14000, 10600, None)
TOKEV = 2
A5K = ((128, 48), (176, 48), (224, 32))
LNLAG = 700
L4 = ([(128, 192, 0, 1500)], [])
L5 = ([(192, 320, 1000, 7200)], [(128, 176, 0, 1600), (176, 320, 1700, 8600)])
L6 = ([(320, 512, 0, 6000)], [(320, 384, 800, 3400), (384, 512, 3500, 10400)])
A6K = ((256, 64), (320, 64), (384, 64), (448, 64))
R1T = (12800, 12800)
GW = (16,) * 7
MERGE = False
FB = FH
MF = (128, 3420)
QWB = QW
G3 = ((0, 1, 3), (0, 2, 3), (1, 2), (0, 1, 2, 3))
RT = None
RW = 800
GLAG = 0
RECQ = True
FUSE = False
QSPLIT = 6
SLAG = 400
FSTEP = 2
CR = 32
XN = 128
VMEM_MB = 120
CT = 128

L_ORD = (2, 3, 0, 1, 4, 5, 6)
R_ORD = (2, 0, 6, 5, 1, 4, 3)

K_SEQ = (1, 4, 0, 2, 3, 5, 6)
K_SEQ2 = (0, 1, 2, 5, 3, 4, 6)
W_SEQ = (0, 1, 5, 6, 4, 2, 3)

NN = (((1,), (0,)), ((), ()))
NT_ = (((1,), (1,)), ((), ()))
TN = (((0,), (0,)), ((), ()))


SCOPES = False


def _scope(name):
    return jax.named_scope(name) if SCOPES else contextlib.nullcontext()


def _mo(v, m):
    return v if isinstance(v, int) else pl.multiple_of(v, m)


def _dot(a, b, dims):
    return lax.dot_general(a, b, dims, preferred_element_type=f32)


def _pack(v):
    return pltpu.bitcast(v.astype(bf16), u32)


def _unpack(v):
    return pltpu.bitcast(v, bf16)


def _combine(m):
    m1, m2, m3, m4, m5, m6, m7 = m
    return m1 + m4 - m5 + m7, m3 + m5, m2 + m4, m1 - m2 + m3 + m6


def _lform(a11, a12, a21, a22):
    return (a11 + a22, a21 + a22, a11, a22, a11 + a12, a21 - a11, a12 - a22)


def _rform(b11, b12, b21, b22):
    return (b11 + b22, b11, b12 - b22, b21 - b11, b22, b11 + b12, b21 + b22)


def _sform(x11, x12, x21, x22):
    return (x11, x22, x11 + x22, x21 + x22, x11 + x12, x21 - x11, x12 - x22)


def _wl(a11, a12, a21, a22):
    s1 = a21 + a22
    s2 = s1 - a11
    return (a11, a12, a12 - s2, a22, s1, s2, a11 - a21)


def _wr(b11, b12, b21, b22):
    t1 = b12 - b11
    t2 = b22 - t1
    return (b11, b21, b22, t2 - b21, t1, t2, b22 - b12)


def _wc(p):
    p1, p2, p3, p4, p5, p6, p7 = p
    u2 = p1 + p6
    u3 = u2 + p7
    return p1 + p2, (u2 + p5) + p3, u3 - p4, u3 + p5


W_R = (3, 1, 0, 2, 4, 5, 6)


def _wl_swapped(a11, a12, a21, a22):
    return _wl(a12, a11, a22, a21)


def _wc_swapped(p):
    p1, p2, p3, p4, p5, p6, p7 = p
    v2 = p1 + p6
    u3 = p7 - v2
    return (p5 - v2) + p3, p1 + p2, u3 + p5, p4 - u3


class _Sym:
    def __init__(self, t):
        self.t = t

    def __add__(self, o):
        return _Sym({**self.t, **o.t})

    def __sub__(self, o):
        return _Sym({**self.t, **{k: -v for k, v in o.t.items()}})


def _st(u, ct):
    return slice((4 * ct + u) * 128, (4 * ct + u + 1) * 128)


def _to_st(v):
    return jnp.concatenate([v[:, (2 * u + ct) * 128:(2 * u + ct + 1) * 128]
                            for ct in range(2) for u in range(4)], axis=1)


def _phi(t):
    return jnp.where(t > 0, t + 1.0, jnp.exp(t)) + 1e-6


def _rbf(v):
    return v.astype(bf16).astype(f32)


def _kernel(x_hbm, wqkv_hbm, wo_hbm, wr_hbm, wg_hbm, wu_hbm, wd_hbm, out_hbm,
            x_buf, wv_buf, wo_buf, wr_buf, wg_buf, wu_buf, wd_buf,
            xs1, xs2, wqs, sa, sb, zacc, zp, pk_buf, xb, yacc, rsel, wrb, zero_buf,
            wks, stats, wqt, ps_raw, qs, ms, tscr, tscr2, pq_raw, den_raw, pqb_buf, denb_buf, qsb,
            mg_raw, hb_raw, out_buf, idx_s, sem):
    wq_buf = out_buf.at[pl.ds(0, D), :]
    wk_buf = out_buf.at[pl.ds(D, D), :]

    def xs_at(k1, e, rows=None):
        r = xs1.at[k1 * 4 + (0, 1, 7, 3).index(e)] if e in (0, 1, 7, 3) else xs2.at[k1 * 4 + (2, 4, 5, 6).index(e)]
        return r if rows is None else r.at[rows, :]

    SEM_B, SEM_O, SEM_Z, SEM_A = 0, 4, 5, 6

    def cp(src, dst, s):
        return pltpu.make_async_copy(src, dst, sem.at[s])

    def cp_x(r0, n, s):
        rows = [pl.ds(_mo(q * HQ + r0, 16), n) for q in range(4)]
        return [cp(x_hbm.at[0, r, :], x_buf.at[r, :], s) for r in rows]

    def cp_wk(c, s):
        return [cp(wqkv_hbm.at[:, pl.ds(_mo(D + c * 256, 256), 256)],
                   wk_buf.at[:, pl.ds(_mo(c * 256, 256), 256)], s)]

    cp_wr = cp(wr_hbm, wr_buf.at[pl.ds(0, D)], SEM_Z)

    def make_a_groups():
        return [
            cp_x(0, 64, SEM_A),
            cp_x(64, 64, SEM_A + 1),
            cp_wk(0, SEM_A + 2),
            cp_wk(1, SEM_A + 3),
            cp_wk(2, SEM_A + 4) + cp_x(128, 64, SEM_A + 4),
            cp_wk(3, SEM_A + 5) + cp_x(192, 128, SEM_A + 5),
            cp_x(320, 192, SEM_A + 6) + [cp(wqkv_hbm.at[:, pl.ds(0, D)], wq_buf, SEM_A + 6)],
        ]

    def cp_b(j, part, wait_only=False):
        pairs = []
        f0, fw = (0, F1) if part == 0 else (F1, FH - F1)
        fs = pl.ds(_mo(j * FH + f0, 128), fw)
        if fw:
          pairs += [(wg_hbm.at[:, fs], wg_buf.at[j, :, pl.ds(f0, fw)]),
                  (wu_hbm.at[:, fs], wu_buf.at[j, :, pl.ds(f0, fw)]),
                  (wd_hbm.at[fs, :], wd_buf.at[j, pl.ds(f0, fw), :])]
        if part == 1:
            for a in range(4):
                c0 = _mo((2 * a + j) * 128, 128)
                pairs += [(wqkv_hbm.at[:, pl.ds(2 * D + c0, 128)], wv_buf.at[j, :, pl.ds(a * 128, 128)]),
                          (wo_hbm.at[pl.ds(c0, 128), :], wo_buf.at[j, pl.ds(a * 128, 128), :])]
        return [cp(dst if wait_only else src, dst, SEM_B + 2 * j + part) for src, dst in pairs]

    clock = [0]
    toks = []
    sides = []
    fwd = [None]

    def emit_tok(vals, stamp=None):
        t = None
        for v in vals:
            v = pltpu.bitcast(v, u32) if v.dtype != u32 else v
            t = v if t is None else t | v
        toks.append((clock[0] if stamp is None else stamp, t & zero_buf[0]))

    def token(kind):
        t = fwd[0]
        if "u" not in t:
            t["u"] = pltpu.bitcast(t["src"](), u32) & zero_buf[0]
        if kind != "u" and "f" not in t:
            t["f"] = pltpu.bitcast(t["u"], f32)
        if kind == "f16" and "f16" not in t:
            t["f16"] = jnp.concatenate([t["f"], t["f"]], axis=0)
        return t[kind]

    def gate(v):
        if fwd[0] is None:
            return v
        head = v if v.shape[0] == 8 else v[0:8]
        head = head | token("u") if v.dtype == u32 else head + token("f")
        return head if v.shape[0] == 8 else jnp.concatenate([head, v[8:]], axis=0)

    def gate16(v):
        return v if fwd[0] is None else v + token("f16")

    def add_side(gen_fn, n, t0, t1, lag=None):
        st = {"i": 0, "n": n, "t0": clock[0] + t0, "t1": clock[0] + t1}

        def tok(vals, extra=0):
            if lag is not None:
                emit_tok(vals, st["t0"] + (st["i"] + 1) * (st["t1"] - st["t0"]) // st["n"] + lag + extra)
        st["g"] = gen_fn(tok)
        sides.append(st)

    def advance(until):
        for st in sides:
            while st["i"] < st["n"] and st["t0"] + st["i"] * (st["t1"] - st["t0"]) // st["n"] < until:
                next(st["g"], None)
                st["i"] += 1
                if st["i"] == st["n"]:
                    for _ in st["g"]:
                        pass

    def flush():
        for st in sides:
            for _ in st["g"]:
                pass
        sides.clear()

    def finish():
        flush()
        toks.clear()
        fwd[0] = None

    def mm(lhs, rhs, dims, cycles, nseg=1):
        due = [t for (c, t) in toks if c <= clock[0]]
        toks[:] = [(c, t) for (c, t) in toks if c > clock[0]]
        if due:
            head = rhs[0:8, 0:128]
            for t in due:
                head = head | t
            if rhs.shape[1] > 128:
                head = jnp.concatenate([head, rhs[0:8, 128:]], axis=1)
            rhs = jnp.concatenate([head, rhs[8:]], axis=0)
        res = _dot(lhs, _unpack(rhs), dims)
        ngr = res.shape[0] // 16
        for sg in range(nseg):
            for i in range(ngr):
                fwd[0] = {"src": lambda sg=sg, i=i: res[i * 16:i * 16 + 8, sg * 128:(sg + 1) * 128]}
                clock[0] += cycles // nseg // ngr
                advance(clock[0])
        return res

    def form_steps(form, form2, get, put, tok=None, keep=range(7)):
        terms = form(*[_Sym({i: 1}) for i in range(4)])
        gated = {_wl: G3[0], _wr: G3[1], _wl_swapped: G3[2]}[form2]
        if 7 in keep:
            gated = G3[3]
        for k1 in range(7):
            sub = []
            for r in range(2):
                for c in range(2):
                    v = None
                    for i, sg in sorted(terms[k1].t.items(), key=lambda e: -e[1]):
                        b = get(r + 2 * (i // 2), c + 2 * (i % 2))
                        if v is None:
                            v = gate16(b) if 2 * r + c in gated else b
                        else:
                            v = v + b if sg > 0 else v - b
                    sub.append(v)
            vals = form2(*sub) + (sub[2],)
            for k2 in keep:
                put(k1, k2, _pack(vals[k2]))
            if tok is not None and k1 % TOKEV == TOKEV - 1 - (6 % TOKEV != TOKEV - 1):
                full = vals[3 if form2 is _wr else 2]
                tok([full[0:8], full[8:16]])
            yield

    def strassen2(lhs, rhs, dims, cycles, nseg=1, wts=(16,) * 7, comb=_wc):
        m1 = [None] * 7
        for i1, k1 in enumerate(K_SEQ2):
            m2 = [None] * 7
            for k2 in W_SEQ:
                m2[k2] = mm(lhs(k1, k2), rhs(k1, k2), dims, cycles * wts[i1] // 16, nseg)
                yield
            m1[k1] = comb(m2)
        out = [[None] * 4 for _ in range(4)]
        for s2 in range(4):
            for s1, v in enumerate(_combine([m1[k1][s2] for k1 in range(7)])):
                out[(s1 // 2) * 2 + s2 // 2][(s1 % 2) * 2 + s2 % 2] = v
        return out

    made = set()

    def need(*keys):
        assert all(k in made for k in keys), keys

    def row_views(base):
        if isinstance(base, int) and base == 0:
            return x_buf, sa, sb, stats, xn_buf, None
        b = _mo(base, 64)
        return ([r.at[pl.ds(b, S - 64), :] for r in (x_buf, sa, sb, stats)]
                + [xn_buf.at[:, pl.ds(b, 64), :], pl.ds(_mo(base // 2, 32), 32)])

    def xs_form(r0, tok, which="all", base=0):
        xn_v, xs_v = row_views(base)[4:]
        rows = slice(r0 % XN, r0 % XN + 16)

        keep = {"all": range(8), "l1": (0, 1, 7, 3), "l2": (2, 4, 5, 6)}[which]
        for ct in range(2):
            def put(k1, k2, v):
                xs_at(k1, k2, xs_v)[r0 // 2:r0 // 2 + 8, ct * 128:(ct + 1) * 128] = v
            yield from form_steps(
                _sform, _wl, lambda q, u: xn_v[q, rows, _st(u, ct)], put, tok, keep)
        made.add(("xs", r0))

    def ln_stats(r_start, n_rows, tok, base=0):
        x_v, sa_v, sb_v, st_v, xn_v, _ = row_views(base)
        lane = lax.broadcasted_iota(i32, (8, 128), 1)
        for r0 in range(r_start, r_start + n_rows, 16):
            if r0 >= 2 * XN:
                need(("ln", r0 - XN))
            for g in range(8):
                q, o = g // 2, (g % 2) * 8
                rg = q * HQ + r0 + o
                xv = x_v[rg:rg + 8, :].astype(f32)
                xg = jnp.concatenate([gate(xv[:, 0:128]), xv[:, 128:]], axis=1)
                mf = jnp.sum(xg, axis=1, keepdims=True) * (1.0 / D)
                d = xv - mf
                var = jnp.sum(d * d, axis=1, keepdims=True) * (1.0 / D)
                rs = lax.rsqrt(var + 1e-5)
                xn_v.at[q][r0 % XN + o:r0 % XN + o + 8, :] = _to_st(d * rs)
                rs = jnp.broadcast_to(rs, (8, 128))
                mf = jnp.broadcast_to(mf, (8, 128))
                sa_v[rg:rg + 8, :] = 1.0 + rs
                sb_v[rg:rg + 8, :] = mf * rs
                st_v[rg:rg + 8, 0:128] = jnp.where(lane == 0, mf, jnp.broadcast_to(var, (8, 128)))
                if tok is not None:
                    tok([rs])
                if g == 7:
                    made.add(("xn", r0))
                yield

    def ln_later(r_start, n_rows, tok, which="all", base=0):
        st_v, xn_v = row_views(base)[3:5]
        for r0 in range(r_start, r_start + n_rows, 16):
            need(("xn", r0))
            form = xs_form(r0, tok, which, base)
            for g in range(8):
                for _ in range(2 if g < 7 else 0):
                    next(form)
                    yield
                q, o = g // 2, (g % 2) * 8
                t = None
                if which != "l1":
                    v = xn_v[q, r0 % XN + o:r0 % XN + o + 8, :] * wrb[8:16, :]
                    for ct in range(8):
                        h = v[:, ct * 128:(ct + 1) * 128]
                        t = gate(h) if t is None else t + h
                if t is not None:
                    st_v[q * HQ + r0 + o:q * HQ + r0 + o + 8, 128:256] = t
                if tok is not None:
                    tok([t])
                if g == 7:
                    next(form, None)
                    made.add(("ln", r0))
                yield

    def wk_prep(c, tok=None):
        cs = pl.ds(_mo(c * 256, 256), 256)
        for i in range(HD // 16):
            r0 = i * 16
            top = wk_buf[r0:r0 + 16, cs].astype(f32)
            bot = wk_buf[HD + r0:HD + r0 + 16, cs].astype(f32)
            ops = _rform(gate(top[:, :128]), top[:, 128:], bot[:, :128], gate(bot[:, 128:]))
            for k in range(7):
                wks.at[c][r0 // 2:r0 // 2 + 8, k * 128:(k + 1) * 128] = _pack(ops[k])
            yield

    def wq_perm(tok):
        def permute(kt):
            for g in range(8):
                tile = gate(pltpu.bitcast(wq_buf[kt * 128:(kt + 1) * 128, g * 128:(g + 1) * 128], u32))
                wqt.at[kt * 8 + g][...] = pltpu.bitcast(_unpack(tile).T, u32)
                yield

        def back(kt):
            for j in range(8):
                tile = gate(jnp.concatenate([wqt[kt * 8 + g, pl.ds(j, 8, stride=8), :] for g in range(8)],
                                            axis=0))
                v = pltpu.bitcast(_unpack(tile).T.astype(f32), u32)
                c0 = (kt // 2) * D + _st(j // 2, j % 2).start
                ps[(kt % 2) * 128:(kt % 2 + 1) * 128, c0:c0 + 128] = v
                made.add(("wqp", kt, j))
                yield

        order = (0, 2, 4, 6, 1, 3, 5, 7)
        for n in range(10):
            if n < 8:
                yield from permute(order[n])
            if n > 1:
                yield from back(order[n - 2])

    def wq_form(tok):
        for i in range(16):
            need(*[("wqp", 2 * r + i // 8, j) for r in range(4) for j in range(8)])
            for ct in range(2):
                def put(k1, k2, v):
                    wqs.at[k1 * 7 + k2][i * 8:(i + 1) * 8, ct * 128:(ct + 1) * 128] = v
                yield from form_steps(
                    _rform, _wr, lambda r, c: pltpu.bitcast(
                        ps[i * 16:(i + 1) * 16, r * D + _st(c, ct).start:r * D + _st(c, ct).stop],
                        f32), put, tok)

    def kproj(r0, n, chunks=range(4)):
        pr = pl.ds(r0 // 2, n // 2)
        need(*[("xs", r) for r in range(max(r0, 128), r0 + n, 16)])
        for c in chunks:
            m = [None] * 7
            for k in K_SEQ:
                e11, e12, e21, e22 = [xs_at(L_ORD[k], e)[pr, :] for e in (0, 1, 7, 3)]
                lhs = jnp.concatenate([jnp.concatenate([e11, e12], axis=1),
                                       jnp.concatenate([e21, e22], axis=1)], axis=0)
                m[k] = mm(_unpack(lhs), wks[c, :, k * 128:(k + 1) * 128], NN, 2 * n)
            kk = [_phi(v) for v in _combine(m)]
            for ct in range(2):
                zacc[:, pl.ds(_mo(c * 256 + ct * 128, 128), 128)] += (
                    (kk[ct] + kk[2 + ct]).reshape(n // 4, 8, 128).sum(axis=0))
            for s1 in range(4):
                for h in range(2):
                    pk_buf.at[s1 % 2, (s1 // 2) * 2 + h][r0:r0 + n, pl.ds(_mo(c * 128, 128), 128)] = (
                        kk[s1][h * n:(h + 1) * n])

    def z_prep():
        z = jnp.sum(zacc[...], axis=0, keepdims=True)
        zt = _pack(jnp.broadcast_to(z, (128, D)).astype(bf16).T)
        for g in range(8):
            tscr.at[g][...] = zt[g * 64:(g + 1) * 64, :]
        for j in range(8):
            blk = jnp.concatenate([tscr[g, pl.ds(j, 8, stride=8), :] for g in range(8)], axis=0)
            zp[:, j * 128:(j + 1) * 128] = _unpack(blk).T[0:8, :].astype(f32)

    def route(tok):
        rows, dots = [None] * 16, [None] * 16
        for b in sorted(range(S // 128), key=lambda b: b % 4):
            need(*[("ln", r) for r in range(max(128, b % 4 * 128), b % 4 * 128 + 128, 16)])
            rows[b] = gate(stats[b * 128:(b + 1) * 128, 0:128]).T[0:8, :]
            dots[b] = jnp.sum(gate(stats[b * 128:(b + 1) * 128, 128:256]).T, axis=0, keepdims=True)
            yield
        mf = jnp.concatenate([v[0:1] for v in rows], axis=0)
        var = jnp.concatenate([v[1:2] for v in rows], axis=0)
        tr = jnp.concatenate(dots, axis=0) * jnp.sqrt(var + 1e-5)
        wsum = jnp.sum(wrb[0:1, :], axis=1, keepdims=True)
        mb = _rbf(mf)
        inv = 1.0 / _rbf(jnp.sqrt(_rbf(_rbf(var) + 1e-5)))
        rv = _rbf((tr + (mf - mb) * wsum) * inv)
        rmax = jnp.max(jnp.max(rv, axis=1, keepdims=True), axis=0, keepdims=True)
        pos = (lax.broadcasted_iota(i32, rv.shape, 0) * 128 + lax.broadcasted_iota(i32, rv.shape, 1))
        idx = jnp.min(jnp.where(rv == rmax, pos, S - 1))
        idx_s[0] = idx

        def pick(v):
            v = jnp.sum(jnp.where(pos == idx, v, 0.0), axis=1, keepdims=True)
            return jnp.sum(v, axis=0, keepdims=True)

        b0 = _mo((idx >> 4) << 4, 16)
        xv = x_buf[pl.ds(b0, 16), :].astype(f32)
        sel = lax.broadcasted_iota(i32, xv.shape, 0) == idx - b0
        row = jnp.sum(jnp.where(sel, xv, 0.0), axis=0, keepdims=True)
        row = _rbf(_rbf(row - pick(mb)) * pick(inv))
        rsel[...] = jnp.broadcast_to(_rbf(jnp.sum(row * wrb[0:1, :], axis=1, keepdims=True)), rsel.shape)
        xbv = jnp.broadcast_to(row, (128, D)).T
        xb[...] = xbv
        tok([xbv[b * 128 + 120:(b + 1) * 128] for b in range(8)])
        yield

    def ps_form(j, tok):
        for c in range(HQ // 16):
            def put(k1, k2, v):
                k = k1 * 7 + k2
                ps[c * 8:(c + 1) * 8, k * 128:(k + 1) * 128] = v
            yield from form_steps(
                _lform, _wl_swapped,
                lambda r, q: pk_buf[j, q, c * 16:(c + 1) * 16, r * 128:(r + 1) * 128], put, tok)

    def q_rows(j, r0, n, pq, rc, d0, rec, wts=None):
        xj = pl.ds(_mo(j * (BQ // 2), BQ // 2), BQ // 2)
        pr = slice(r0 // 2, (r0 + n) // 2)
        blk = yield from strassen2(lambda k1, k2: _unpack(xs_at(L_ORD[k1], k2, xj)[pr, :]),
                                   lambda k1, k2: wqs[k1 * 7 + k2], NN, n, 1, wts or QW)
        lane = lax.broadcasted_iota(i32, (n, 128), 1)
        for q in range(4):
            d = None
            for u in (3, 2, 1, 0):
                v = _phi(blk[q][u])
                for ct in range(2):
                    pq.at[q][d0:d0 + n, _st(u, ct)] = v[:, ct * 128:(ct + 1) * 128]
                t = v * zp[0:1, u * 256:(u + 1) * 256]
                t = t[:, :128] + t[:, 128:]
                d = t if d is None else d + t
            if rec:
                d = recip(d, lane)
            rc.at[q][d0:d0 + n, :] = d

    def recip(d, lane):
        d = d + jnp.where(lane % 2 == 0, pltpu.roll(d, 127, 1), pltpu.roll(d, 1, 1))
        d = d + jnp.where(lane % 4 < 2, pltpu.roll(d, 126, 1), pltpu.roll(d, 2, 1))
        return 1.0 / (d + 1e-6)

    def normalise(pq, rc, nr, dst, p0, raw, tok=None):
        lane = lax.broadcasted_iota(i32, (16, 128), 1)

        def fix(c):
            if c < nr // 16 and raw(c * 16):
                for q in range(4):
                    rq = slice(c * 16, (c + 1) * 16)
                    rc.at[q][rq, :] = recip(gate16(rc[q, rq, :]), lane)

        def scale(c):
            rq = slice(c * 16, (c + 1) * 16)
            fix(c + 1)
            for hf in range(2):
                for q in range(4):
                    cs = slice(hf * HD, (hf + 1) * HD)
                    pq.at[q][rq, cs] = pq[q, rq, cs] * jnp.concatenate([gate16(rc[q, rq, :])] * 4, axis=1)
                    yield

        def form(c):
            rq = slice(c * 16, (c + 1) * 16)
            p2 = pl.ds(_mo(p0 + c * 8, 8), 8)
            for ct in range(2):
                def put(k1, k2, v):
                    dst.at[k1 * 7 + k2][p2, ct * 128:(ct + 1) * 128] = v
                yield from form_steps(_lform, _wl, lambda q, u: pq[q, rq, _st(u, ct)], put, tok)

        fix(0)
        if raw(0):
            for _ in range(4):
                yield
        yield from scale(0)
        for c in range(nr // 16):
            nxt = scale(c + 1) if c + 1 < nr // 16 else iter(())
            for i, _ in enumerate(form(c)):
                yield
                if i < 8 and c + 1 < nr // 16:
                    next(nxt)
                    yield
        made.add(("qs", id(dst)))

    hist = []

    def g_lhs(k):
        v = ps[:, k * 128:(k + 1) * 128]
        hist.append(fwd[0])
        if GLAG and len(hist) > GLAG and hist[-1 - GLAG] is not None:
            cur = fwd[0]
            fwd[0] = hist[-1 - GLAG]
            v = jnp.concatenate([gate(v[i * 64:(i + 1) * 64]) for i in range(4)], axis=0)
            fwd[0] = cur
        return _unpack(v)

    def g_kvm(j):
        blk = yield from strassen2(
            lambda k1, k2: g_lhs(k1 * 7 + k2),
            lambda k1, k2: xs_at(R_ORD[k1], W_R[k2])[...], TN, 256, 2, GW, _wc_swapped)
        hm = (lax.broadcasted_iota(i32, (128, 128), 0) // 32
              == lax.broadcasted_iota(i32, (128, 128), 1) // 32)
        qb = q_rows(j, BQ - QB, QB, pqb_buf.at[j], denb_buf.at[j], 0, False, QWB)
        for _ in range(QSPLIT):
            next(qb)
        kvps = []
        for a in (3, 2, 1, 0):
            gg = jnp.concatenate(blk[a], axis=1).astype(bf16)
            wv_u = pltpu.bitcast(wv_buf[j, :, a * 128:(a + 1) * 128], u32)
            kv = jnp.where(hm, mm(gg, wv_u, NN, 256), 0.0)
            tscr2.at[a][...] = _pack(kv)
            kvps.append(_unpack(jnp.concatenate(
                [tscr2[a, pl.ds(jj, 8, stride=8), :] for jj in range(8)], axis=0)))
        mg = mg_buf

        def m_form(tok):
            for a in (3, 2, 1, 0):
                need(("mg", a))
                for jl in range(2):
                    for ct in range(2):
                        def put(k1, k2, v):
                            ms.at[k1 * 7 + k2][pl.ds(_mo(jl * 64 + (2 * a + j) * 8, 8), 8),
                                               ct * 128:(ct + 1) * 128] = v
                        yield from form_steps(
                            _rform, _wr, lambda q, u: mg[a, (2 * q + jl) * 16:(2 * q + jl + 1) * 16, _st(u, ct)], put)

        for i, a in enumerate((3, 2, 1, 0)):
            wo_u = pltpu.bitcast(wo_buf[j, a * 128:(a + 1) * 128, :], u32)
            res = mm(kvps[i], wo_u, NN, 256)
            mg.at[a][...] = _to_st(res)
            made.add(("mg", a))
            if i == 0:
                add_side(m_form, 112, MF[0], MF[1])
        for _ in qb:
            pass

    def out_part(p0, nr, y, src, pr0):
        pr = pl.ds(_mo(pr0, 8), nr // 2)
        rows = [pl.ds(_mo(q * HQ + p0, 16), nr) for q in range(4)]
        row = lax.broadcasted_iota(i32, (nr, 256), 0) + p0
        blk = yield from strassen2(lambda k1, k2: _unpack(src[k1 * 7 + k2, pr, :]),
                                   lambda k1, k2: ms[k1 * 7 + k2], NN, nr)
        for s1 in (3, 2, 1, 0):
            for s2 in range(4):
                q = (s1 // 2) * 2 + s2 // 2
                u = (s1 % 2) * 2 + s2 % 2
                rr, cc = rows[q], pl.ds(u * 256, 256)
                a = jnp.concatenate([sa[rr, :]] * 2, axis=1)
                b = jnp.concatenate([sb[rr, :]] * 2, axis=1)
                o = blk[q][u] + jnp.where(row + q * HQ == idx_s[0], y[:, u * 256:(u + 1) * 256], 0.0)
                out_buf[rr, cc] = (x_buf[rr, cc].astype(f32) * a - b + o).astype(bf16)
                if s2 % 2 == 1:
                    ch = pl.ds((s1 % 2) * HD, HD)
                    cp(out_buf.at[rr, ch], out_hbm.at[0, rr, ch], SEM_O).start()

    def ffn_part(j, f_lo, f_hi):
        def fma(acc, w, v):
            p = w.astype(f32) * v
            return acc + p[0:8] + p[8:16]

        for f0 in range(f_lo, f_hi, 256):
            fs = slice(f0, f0 + 256)
            ag = jnp.zeros((8, 256), f32)
            au = jnp.zeros((8, 256), f32)
            for k in range(0, D, 16):
                xv = jnp.concatenate([gate16(xb[k:k + 16, :])] * 2, axis=1)
                ag = fma(ag, wg_buf[j, k:k + 16, fs], xv)
                au = fma(au, wu_buf[j, k:k + 16, fs], xv)
                yield
            g = _rbf(jnp.sum(ag, axis=0, keepdims=True))
            u = _rbf(jnp.sum(au, axis=0, keepdims=True))
            h = _rbf(_rbf(g * jax.nn.sigmoid(g)) * u)
            hb_buf[fs, :] = jnp.broadcast_to(h, (128, 256)).T
        for d0 in range(0, D, 512):
            ds_ = slice(d0, d0 + 512)
            acc = yacc[:, ds_]
            for k in range(f_lo, f_hi, 16):
                hv = jnp.concatenate([gate16(hb_buf[k:k + 16, :])] * 4, axis=1)
                acc = fma(acc, wd_buf[j, k:k + 16, ds_], hv)
                yield
            yacc[:, ds_] = acc

    def wait_group(i):
        with _scope("a_wait%d" % i):
            for c in a_groups[i]:
                c.wait()

    def run_all(gen):
        for _ in gen:
            pass

    def ln_sides(plan):
        for r0, r1, t0, t1 in plan[0]:
            add_side(lambda tok, r0=r0, r1=r1: ln_stats(r0, r1 - r0, tok), (r1 - r0) // 2, t0, t1, LNLAG)
        for r0, r1, t0, t1 in plan[1]:
            add_side(lambda tok, r0=r0, r1=r1: ln_later(r0, r1 - r0, tok), 22 * (r1 - r0) // 16, t0, t1, SLAG)

    def l2_side(base, n, t0, t1):
        add_side(lambda tok: ln_later(0, n, None, "l2", base), 22 * n // 16, t0, t1)

    a_groups = make_a_groups()
    with _scope("p0_issue"):
        cp_wr.start()
        for grp in a_groups:
            for c in grp:
                c.start()
        for j in range(2):
            for part in range(2):
                for c in cp_b(j, part):
                    c.start()
        zacc[...] = jnp.zeros(zacc.shape, f32)
        yacc[...] = jnp.zeros(yacc.shape, f32)
        zero_buf[1] = jnp.zeros((8, 128), u32)
        cp_zero = cp(zero_buf.at[1], zero_buf.at[0], SEM_Z)
        cp_zero.start()
        cp_zero.wait()
        cp_wr.wait()
        wr8 = jnp.broadcast_to(wr_buf[0:D].reshape(1, D).astype(f32), (8, D))
        wrb[0:8, :] = wr8
        wrb[8:16, :] = _to_st(wr8)
        z0 = jnp.max(pltpu.bitcast(zero_buf[0], i32))
        ps, pq_buf, den_buf, mg_buf, hb_buf = [r.at[z0] for r in (ps_raw, pq_raw, den_raw, mg_raw, hb_raw)]
        xn_buf = mg_buf

    def a01(i, carry):
        with _scope("a_wait01"):
            for c in cp_x(i * 64, 64, SEM_A + i):
                c.wait()
        with _scope("a01"):
            for r in range(0, 64, 16):
                run_all(ln_stats(r, 16, None, i * 64))
                if r:
                    run_all(ln_later(r - 16, 16, None, "l1", i * 64))
            run_all(ln_later(48, 16, None, "l1", i * 64))
        return carry

    lax.fori_loop(0, 2, a01, 0)

    def a23(i, carry):
        with _scope("a_wait23"):
            for c in cp_wk(i, SEM_A + 2 + i):
                c.wait()
        with _scope("a23"):
            run_all(wk_prep(i))
            l2_side(i * 64, 64, 300, 1500)
            kproj(0, 128, [i])
            finish()
        return carry

    lax.fori_loop(0, 2, a23, 0)
    wait_group(4)
    with _scope("a4"):
        run_all(wk_prep(2))
        ln_sides(L4)
        kproj(0, 128, [2])
        finish()
    wait_group(5)
    with _scope("a5"):
        run_all(wk_prep(3))
        ln_sides(L5)
        kproj(0, 128, [3])
        for r0, n in A5K:
            kproj(r0, n)
        finish()
    wait_group(6)
    with _scope("a6"):
        ln_sides(L6)
        add_side(wq_perm, 128, A6[1], A6[2], A6[6])
        add_side(wq_form, 224, A6[3], A6[4], A6[6])
        if RT is None:
            add_side(route, 17, A6[5], A6[5] + RW)
        for r0, n in A6K:
            kproj(r0, n)
        finish()

    def b_body(j, carry):
        qa = BQ - QB
        with _scope("b_wait0"):
            for c in cp_b(j, 0, wait_only=True) + (cp_b(j, 1, wait_only=True) if MERGE else []):
                c.wait()
        with _scope("b_r0"):
            z_prep()
            t1 = 49 * qa - 400
            add_side(lambda tok: ps_form(j, tok), 7 * HQ // 16, 0, t1, SLAG if MERGE else None)
            if RT is not None:
                add_side(route, 17, RT[0], RT[1])
            if F1:
                add_side(lambda tok: ffn_part(j, 0, F1), F1 * 3 // (4 * FSTEP), 0, t1)
            for r0 in range(0, qa, QN):
                run_all(q_rows(j, r0, min(QN, qa - r0), pq_buf, den_buf, r0, r0 + QN < qa))
            if MERGE:
                flush()
            else:
                finish()
        if not MERGE:
            with _scope("b_wait1"):
                for c in cp_b(j, 1, wait_only=True):
                    c.wait()
        with _scope("b_r1"):
            add_side(lambda tok: ffn_part(j, F1, FB), (FB - F1) * 3 // (4 * FSTEP), 0, R1T[0])
            add_side(lambda tok: normalise(pq_buf, den_buf, qa, qs, j * (qa // 2),
                                           lambda r: (r // QN + 1) * QN >= qa), 22 * (qa // 16), 0, R1T[1])
            run_all(g_kvm(j))
            finish()
        return carry

    lax.fori_loop(0, 2, b_body, 0)

    def c_body(t, carry):
        with _scope("c_body"):
            y = _rbf(jnp.sum(yacc[...], axis=0, keepdims=True))
            y = _rbf(y * _rbf(1.0 / _rbf(1.0 + _rbf(jnp.exp(-rsel[0:1, :])))))
            j, h = t >> 1, t & 1
            na, nb = (BQ - QB) // 2, QB // 2
            hb = pl.ds(_mo(h * nb, 16), nb)
            add_side(lambda tok: normalise(pqb_buf.at[j, :, hb, :], denb_buf.at[j, :, hb, :], nb, qsb, 0,
                                           lambda r: True, tok),
                     4 + 22 * (nb // 16), 0, 49 * na - 800, SLAG)
            for p in range(0, na, CR):
                p0 = j * BQ + h * na + p
                run_all(out_part(p0, min(CR, na - p), y, qs, t * (na // 2) + p // 2))
            advance(clock[0] + 10 ** 6)
            flush()
            run_all(out_part(j * BQ + BQ - QB + h * nb, nb, y, qsb, 0))
            finish()
        return carry

    lax.fori_loop(0, 4, c_body, 0)
    with _scope("tail"):
        cp(out_buf, out_hbm.at[0], SEM_O).wait()


@jax.jit
def pallas_parallel_sum__linear_attn_block__moe_arch_mod__prompt_kernel(
    A_x: jax.Array,
    A_wqkv: jax.Array,
    A_wo: jax.Array,
    B_x: jax.Array,
    B_w_r: jax.Array,
    B_w_gate: jax.Array,
    B_w_up: jax.Array,
    B_w_down: jax.Array,
):
    del B_x
    V = pltpu.VMEM
    scratch = [
        V((S, D), bf16),
        V((2, D, 512), bf16),
        V((2, 512, D), bf16),
        V((8 * D,), bf16),
        V((2, D, FH), bf16),
        V((2, D, FH), bf16),
        V((2, FH, D), bf16),
        V((28, HQ // 2, 256), u32),
        V((28, HQ // 2, 256), u32),
        V((49, 128, 256), u32),
        V((S, 128), f32),
        V((S, 128), f32),
        V((8, D), f32),
        V((8, D), f32),
        V((2, 4, HQ, 512), f32),
        V((D, 128), f32),
        V((8, D), f32),
        V((8, D), f32),
        V((16, D), f32),
        V((4, 8, 128), u32),
        V((4, HD // 2, 7 * 128), u32),
        V((S, 256), f32),
        V((64, 64, 128), u32),
        V((1, HQ // 2, 49 * 128), u32),
        V((49, BQ - QB, 256), u32),
        V((49, 128, 256), u32),
        V((8, 64, 128), u32),
        V((4, 64, 128), u32),
        V((1, 4, BQ - QB, D), f32),
        V((1, 4, BQ - QB, 128), f32),
        V((2, 4, QB, D), f32),
        V((2, 4, QB, 128), f32),
        V((49, QB // 4, 256), u32),
        V((1, 4, 128, D), f32),
        V((1, FH, 128), f32),
        V((S, D), bf16),
        pltpu.SMEM((1,), i32),
        pltpu.SemaphoreType.DMA((13,)),
    ]
    return pl.pallas_call(
        _kernel,
        out_shape=jax.ShapeDtypeStruct((1, S, D), bf16),
        in_specs=[pl.BlockSpec(memory_space=pl.ANY)] * 7,
        out_specs=pl.BlockSpec(memory_space=pl.ANY),
        scratch_shapes=scratch,
        compiler_params=pltpu.CompilerParams(vmem_limit_bytes=VMEM_MB * 1024 * 1024,
                                             disable_bounds_checks=True,
                                             fuse_transposed_lhs_in_matmul=FUSE,
                                             disable_semaphore_checks=True),
    )(A_x, A_wqkv, A_wo, B_w_r, B_w_gate, B_w_up, B_w_down)
```

```python
import contextlib

import jax
import jax.numpy as jnp
from jax import lax
import jax.experimental.pallas as pl
import jax.experimental.pallas.tpu as pltpu

bf16, f32, u32, i32 = jnp.bfloat16, jnp.float32, jnp.uint32, jnp.int32

S = 2048
D = 1024
F = 3584
HP = S // 2
HD = D // 2
HQ = S // 4
BQ = HQ // 2
FH = F // 2
F1 = 0
QB = 64
QN = 48
QW = (28, 36, 36, 6, 2, 2, 2)
A6 = (0, 6200, 9000, 9100, 14000, 10600, None)
TOKEV = 2
A5K = ((128, 48), (176, 48), (224, 32))
LNLAG = 700
L4 = ([(128, 192, 0, 1500)], [])
L5 = ([(192, 320, 1000, 7200)], [(128, 176, 0, 1600), (176, 320, 1700, 8600)])
L6 = ([(320, 512, 0, 6000)], [(320, 384, 800, 3400), (384, 512, 3500, 10400)])
A6K = ((256, 64), (320, 64), (384, 64), (448, 64))
R1T = (12800, 12800)
GW = (16,) * 7
MERGE = False
FB = FH
MF = (128, 3420)
QWB = QW
G3 = ((0, 1, 3), (0, 2, 3), (1, 2), (0, 1, 2, 3))
X0 = 32
RT = None
RW = 800
GLAG = 0
RECQ = True
FUSE = False
QSPLIT = 6
SLAG = 400
FSTEP = 2
CR = 32
XN = 128
VMEM_MB = 120
CT = 128

L_ORD = (2, 3, 0, 1, 4, 5, 6)
R_ORD = (2, 0, 6, 5, 1, 4, 3)

K_SEQ = (1, 4, 0, 2, 3, 5, 6)
K_SEQ2 = (0, 1, 2, 5, 3, 4, 6)
W_SEQ = (0, 1, 5, 6, 4, 2, 3)

NN = (((1,), (0,)), ((), ()))
NT_ = (((1,), (1,)), ((), ()))
TN = (((0,), (0,)), ((), ()))


SCOPES = False


def _scope(name):
    return jax.named_scope(name) if SCOPES else contextlib.nullcontext()


def _mo(v, m):
    return v if isinstance(v, int) else pl.multiple_of(v, m)


def _dot(a, b, dims):
    return lax.dot_general(a, b, dims, preferred_element_type=f32)


def _pack(v):
    return pltpu.bitcast(v.astype(bf16), u32)


def _unpack(v):
    return pltpu.bitcast(v, bf16)


def _combine(m):
    m1, m2, m3, m4, m5, m6, m7 = m
    return m1 + m4 - m5 + m7, m3 + m5, m2 + m4, m1 - m2 + m3 + m6


def _lform(a11, a12, a21, a22):
    return (a11 + a22, a21 + a22, a11, a22, a11 + a12, a21 - a11, a12 - a22)


def _rform(b11, b12, b21, b22):
    return (b11 + b22, b11, b12 - b22, b21 - b11, b22, b11 + b12, b21 + b22)


def _sform(x11, x12, x21, x22):
    return (x11, x22, x11 + x22, x21 + x22, x11 + x12, x21 - x11, x12 - x22)


def _wl(a11, a12, a21, a22):
    s1 = a21 + a22
    s2 = s1 - a11
    return (a11, a12, a12 - s2, a22, s1, s2, a11 - a21)


def _wr(b11, b12, b21, b22):
    t1 = b12 - b11
    t2 = b22 - t1
    return (b11, b21, b22, t2 - b21, t1, t2, b22 - b12)


def _wc(p):
    p1, p2, p3, p4, p5, p6, p7 = p
    u2 = p1 + p6
    u3 = u2 + p7
    return p1 + p2, (u2 + p5) + p3, u3 - p4, u3 + p5


W_R = (3, 1, 0, 2, 4, 5, 6)


def _wl_swapped(a11, a12, a21, a22):
    return _wl(a12, a11, a22, a21)


def _wc_swapped(p):
    p1, p2, p3, p4, p5, p6, p7 = p
    v2 = p1 + p6
    u3 = p7 - v2
    return (p5 - v2) + p3, p1 + p2, u3 + p5, p4 - u3


class _Sym:
    def __init__(self, t):
        self.t = t

    def __add__(self, o):
        return _Sym({**self.t, **o.t})

    def __sub__(self, o):
        return _Sym({**self.t, **{k: -v for k, v in o.t.items()}})


def _st(u, ct):
    return slice((4 * ct + u) * 128, (4 * ct + u + 1) * 128)


def _to_st(v):
    return jnp.concatenate([v[:, (2 * u + ct) * 128:(2 * u + ct + 1) * 128]
                            for ct in range(2) for u in range(4)], axis=1)


def _phi(t):
    return jnp.where(t > 0, t + 1.0, jnp.exp(t)) + 1e-6


def _rbf(v):
    return v.astype(bf16).astype(f32)


def _kernel(x_hbm, wqkv_hbm, wo_hbm, wr_hbm, wg_hbm, wu_hbm, wd_hbm, out_hbm,
            x_buf, wv_buf, wo_buf, wr_buf, wg_buf, wu_buf, wd_buf,
            xs1, xs2, wqs, sa, sb, zacc, zp, pk_buf, xb, yacc, rsel, wrb, zero_buf,
            wks, stats, wqt, ps_raw, qs, ms, tscr, tscr2, pq_raw, den_raw, pqb_buf, denb_buf, qsb,
            mg_raw, hb_raw, out_buf, idx_s, sem):
    wq_buf = out_buf.at[pl.ds(0, D), :]
    wk_buf = out_buf.at[pl.ds(D, D), :]

    def xs_at(k1, e, rows=None):
        r = xs1.at[k1 * 4 + (0, 1, 7, 3).index(e)] if e in (0, 1, 7, 3) else xs2.at[k1 * 4 + (2, 4, 5, 6).index(e)]
        return r if rows is None else r.at[rows, :]

    SEM_B, SEM_O, SEM_Z, SEM_A = 0, 4, 5, 6

    def cp(src, dst, s):
        return pltpu.make_async_copy(src, dst, sem.at[s])

    def cp_x(r0, n, s):
        r = pl.ds(_mo(r0, 16), n)
        return [cp(x_hbm.at[:, r, :], x_buf.at[:, r, :], s)]

    def cp_wk(c, s):
        return [cp(wqkv_hbm.at[:, pl.ds(_mo(D + c * 256, 256), 256)],
                   wk_buf.at[:, pl.ds(_mo(c * 256, 256), 256)], s)]

    cp_wr = cp(wr_hbm, wr_buf.at[pl.ds(0, D)], SEM_Z)

    NX = 128 // X0
    SEM_W = SEM_A + NX

    def make_a_groups():
        return [cp_x(i * X0, X0, SEM_A + i) for i in range(NX)] + [
            cp_wk(0, SEM_W),
            cp_wk(1, SEM_W + 1),
            cp_wk(2, SEM_W + 2) + cp_x(128, 64, SEM_W + 2),
            cp_wk(3, SEM_W + 3) + cp_x(192, 128, SEM_W + 3),
            cp_x(320, 192, SEM_W + 4) + [cp(wqkv_hbm.at[:, pl.ds(0, D)], wq_buf, SEM_W + 4)],
        ]

    def cp_b(j, part, wait_only=False):
        pairs = []
        f0, fw = (0, F1) if part == 0 else (F1, FH - F1)
        fs = pl.ds(_mo(j * FH + f0, 128), fw)
        if fw:
          pairs += [(wg_hbm.at[:, fs], wg_buf.at[j, :, pl.ds(f0, fw)]),
                  (wu_hbm.at[:, fs], wu_buf.at[j, :, pl.ds(f0, fw)]),
                  (wd_hbm.at[fs, :], wd_buf.at[j, pl.ds(f0, fw), :])]
        if part == 1:
            for a in range(4):
                c0 = _mo((2 * a + j) * 128, 128)
                pairs += [(wqkv_hbm.at[:, pl.ds(2 * D + c0, 128)], wv_buf.at[j, :, pl.ds(a * 128, 128)]),
                          (wo_hbm.at[pl.ds(c0, 128), :], wo_buf.at[j, pl.ds(a * 128, 128), :])]
        return [cp(dst if wait_only else src, dst, SEM_B + 2 * j + part) for src, dst in pairs]

    clock = [0]
    toks = []
    sides = []
    fwd = [None]

    def emit_tok(vals, stamp=None):
        t = None
        for v in vals:
            v = pltpu.bitcast(v, u32) if v.dtype != u32 else v
            t = v if t is None else t | v
        toks.append((clock[0] if stamp is None else stamp, t & zero_buf[0]))

    def token(kind):
        t = fwd[0]
        if "u" not in t:
            t["u"] = pltpu.bitcast(t["src"](), u32) & zero_buf[0]
        if kind != "u" and "f" not in t:
            t["f"] = pltpu.bitcast(t["u"], f32)
        if kind == "f16" and "f16" not in t:
            t["f16"] = jnp.concatenate([t["f"], t["f"]], axis=0)
        return t[kind]

    def gate(v):
        if fwd[0] is None:
            return v
        head = v if v.shape[0] == 8 else v[0:8]
        head = head | token("u") if v.dtype == u32 else head + token("f")
        return head if v.shape[0] == 8 else jnp.concatenate([head, v[8:]], axis=0)

    def gate16(v):
        return v if fwd[0] is None else v + token("f16")

    def add_side(gen_fn, n, t0, t1, lag=None):
        st = {"i": 0, "n": n, "t0": clock[0] + t0, "t1": clock[0] + t1}

        def tok(vals, extra=0):
            if lag is not None:
                emit_tok(vals, st["t0"] + (st["i"] + 1) * (st["t1"] - st["t0"]) // st["n"] + lag + extra)
        st["g"] = gen_fn(tok)
        sides.append(st)

    def advance(until):
        for st in sides:
            while st["i"] < st["n"] and st["t0"] + st["i"] * (st["t1"] - st["t0"]) // st["n"] < until:
                next(st["g"], None)
                st["i"] += 1
                if st["i"] == st["n"]:
                    for _ in st["g"]:
                        pass

    def flush():
        for st in sides:
            for _ in st["g"]:
                pass
        sides.clear()

    def finish():
        flush()
        toks.clear()
        fwd[0] = None

    def mm(lhs, rhs, dims, cycles, nseg=1):
        due = [t for (c, t) in toks if c <= clock[0]]
        toks[:] = [(c, t) for (c, t) in toks if c > clock[0]]
        if due:
            head = rhs[0:8, 0:128]
            for t in due:
                head = head | t
            if rhs.shape[1] > 128:
                head = jnp.concatenate([head, rhs[0:8, 128:]], axis=1)
            rhs = jnp.concatenate([head, rhs[8:]], axis=0)
        res = _dot(lhs, _unpack(rhs), dims)
        ngr = res.shape[0] // 16
        for sg in range(nseg):
            for i in range(ngr):
                fwd[0] = {"src": lambda sg=sg, i=i: res[i * 16:i * 16 + 8, sg * 128:(sg + 1) * 128]}
                clock[0] += cycles // nseg // ngr
                advance(clock[0])
        return res

    def form_steps(form, form2, get, put, tok=None, keep=range(7)):
        terms = form(*[_Sym({i: 1}) for i in range(4)])
        gated = {_wl: G3[0], _wr: G3[1], _wl_swapped: G3[2]}[form2]
        if 7 in keep:
            gated = G3[3]
        for k1 in range(7):
            sub = []
            for r in range(2):
                for c in range(2):
                    v = None
                    for i, sg in sorted(terms[k1].t.items(), key=lambda e: -e[1]):
                        b = get(r + 2 * (i // 2), c + 2 * (i % 2))
                        if v is None:
                            v = gate16(b) if 2 * r + c in gated else b
                        else:
                            v = v + b if sg > 0 else v - b
                    sub.append(v)
            vals = form2(*sub) + (sub[2],)
            for k2 in keep:
                put(k1, k2, _pack(vals[k2]))
            if tok is not None and k1 % TOKEV == TOKEV - 1 - (6 % TOKEV != TOKEV - 1):
                full = vals[3 if form2 is _wr else 2]
                tok([full[0:8], full[8:16]])
            yield

    def strassen2(lhs, rhs, dims, cycles, nseg=1, wts=(16,) * 7, comb=_wc):
        m1 = [None] * 7
        for i1, k1 in enumerate(K_SEQ2):
            m2 = [None] * 7
            for k2 in W_SEQ:
                m2[k2] = mm(lhs(k1, k2), rhs(k1, k2), dims, cycles * wts[i1] // 16, nseg)
                yield
            m1[k1] = comb(m2)
        out = [[None] * 4 for _ in range(4)]
        for s2 in range(4):
            for s1, v in enumerate(_combine([m1[k1][s2] for k1 in range(7)])):
                out[(s1 // 2) * 2 + s2 // 2][(s1 % 2) * 2 + s2 % 2] = v
        return out

    made = set()

    def need(*keys):
        assert all(k in made for k in keys), keys

    def row_views(base):
        if base == 0:
            return x_buf, sa, sb, stats, xn_buf, None
        i, n = base
        b = _mo(i * n, n)
        return ([x_buf.at[:, pl.ds(b, n), :]] + [r.at[pl.ds(b, S - 128 + n), :] for r in (sa, sb, stats)]
                + [xn_buf.at[:, pl.ds(b, n), :], pl.ds(_mo(i * (n // 2), n // 2), n // 2)])

    def xs_form(r0, tok, which="all", base=0):
        xn_v, xs_v = row_views(base)[4:]
        rows = slice(r0 % XN, r0 % XN + 16)

        keep = {"all": range(8), "l1": (0, 1, 7, 3), "l2": (2, 4, 5, 6)}[which]
        for ct in range(2):
            def put(k1, k2, v):
                xs_at(k1, k2, xs_v)[r0 // 2:r0 // 2 + 8, ct * 128:(ct + 1) * 128] = v
            yield from form_steps(
                _sform, _wl, lambda q, u: xn_v[q, rows, _st(u, ct)], put, tok, keep)
        made.add(("xs", r0))

    def ln_stats(r_start, n_rows, tok, base=0):
        x_v, sa_v, sb_v, st_v, xn_v, _ = row_views(base)
        lane = lax.broadcasted_iota(i32, (8, 128), 1)
        for r0 in range(r_start, r_start + n_rows, 16):
            if r0 >= 2 * XN:
                need(("ln", r0 - XN))
            for g in range(8):
                q, o = g // 2, (g % 2) * 8
                rg = q * HQ + r0 + o
                xv = x_v[q, r0 + o:r0 + o + 8, :].astype(f32)
                xg = jnp.concatenate([gate(xv[:, 0:128]), xv[:, 128:]], axis=1)
                mf = jnp.sum(xg, axis=1, keepdims=True) * (1.0 / D)
                d = xv - mf
                var = jnp.sum(d * d, axis=1, keepdims=True) * (1.0 / D)
                rs = lax.rsqrt(var + 1e-5)
                xn_v.at[q][r0 % XN + o:r0 % XN + o + 8, :] = _to_st(d * rs)
                rs = jnp.broadcast_to(rs, (8, 128))
                mf = jnp.broadcast_to(mf, (8, 128))
                sa_v[rg:rg + 8, :] = 1.0 + rs
                sb_v[rg:rg + 8, :] = mf * rs
                st_v[rg:rg + 8, 0:128] = jnp.where(lane == 0, mf, jnp.broadcast_to(var, (8, 128)))
                if tok is not None:
                    tok([rs])
                if g == 7:
                    made.add(("xn", r0))
                yield

    def ln_later(r_start, n_rows, tok, which="all", base=0):
        st_v, xn_v = row_views(base)[3:5]
        for r0 in range(r_start, r_start + n_rows, 16):
            need(("xn", r0))
            form = xs_form(r0, tok, which, base)
            for g in range(8):
                for _ in range(2 if g < 7 else 0):
                    next(form)
                    yield
                q, o = g // 2, (g % 2) * 8
                t = None
                if which != "l1":
                    v = xn_v[q, r0 % XN + o:r0 % XN + o + 8, :] * wrb[8:16, :]
                    for ct in range(8):
                        h = v[:, ct * 128:(ct + 1) * 128]
                        t = gate(h) if t is None else t + h
                if t is not None:
                    st_v[q * HQ + r0 + o:q * HQ + r0 + o + 8, 128:256] = t
                if tok is not None:
                    tok([t])
                if g == 7:
                    next(form, None)
                    made.add(("ln", r0))
                yield

    def wk_prep(c, tok=None):
        cs = pl.ds(_mo(c * 256, 256), 256)
        for i in range(HD // 16):
            r0 = i * 16
            top = wk_buf[r0:r0 + 16, cs].astype(f32)
            bot = wk_buf[HD + r0:HD + r0 + 16, cs].astype(f32)
            ops = _rform(gate(top[:, :128]), top[:, 128:], bot[:, :128], gate(bot[:, 128:]))
            for k in range(7):
                wks.at[c][r0 // 2:r0 // 2 + 8, k * 128:(k + 1) * 128] = _pack(ops[k])
            yield

    def wq_perm(tok):
        def permute(kt):
            for g in range(8):
                tile = gate(pltpu.bitcast(wq_buf[kt * 128:(kt + 1) * 128, g * 128:(g + 1) * 128], u32))
                wqt.at[kt * 8 + g][...] = pltpu.bitcast(_unpack(tile).T, u32)
                yield

        def back(kt):
            for j in range(8):
                tile = gate(jnp.concatenate([wqt[kt * 8 + g, pl.ds(j, 8, stride=8), :] for g in range(8)],
                                            axis=0))
                v = pltpu.bitcast(_unpack(tile).T.astype(f32), u32)
                c0 = (kt // 2) * D + _st(j // 2, j % 2).start
                ps[(kt % 2) * 128:(kt % 2 + 1) * 128, c0:c0 + 128] = v
                made.add(("wqp", kt, j))
                yield

        order = (0, 2, 4, 6, 1, 3, 5, 7)
        for n in range(10):
            if n < 8:
                yield from permute(order[n])
            if n > 1:
                yield from back(order[n - 2])

    def wq_form(tok):
        for i in range(16):
            need(*[("wqp", 2 * r + i // 8, j) for r in range(4) for j in range(8)])
            for ct in range(2):
                def put(k1, k2, v):
                    wqs.at[k1 * 7 + k2][i * 8:(i + 1) * 8, ct * 128:(ct + 1) * 128] = v
                yield from form_steps(
                    _rform, _wr, lambda r, c: pltpu.bitcast(
                        ps[i * 16:(i + 1) * 16, r * D + _st(c, ct).start:r * D + _st(c, ct).stop],
                        f32), put, tok)

    def kproj(r0, n, chunks=range(4)):
        pr = pl.ds(r0 // 2, n // 2)
        need(*[("xs", r) for r in range(max(r0, 128), r0 + n, 16)])
        for c in chunks:
            m = [None] * 7
            for k in K_SEQ:
                e11, e12, e21, e22 = [xs_at(L_ORD[k], e)[pr, :] for e in (0, 1, 7, 3)]
                lhs = jnp.concatenate([jnp.concatenate([e11, e12], axis=1),
                                       jnp.concatenate([e21, e22], axis=1)], axis=0)
                m[k] = mm(_unpack(lhs), wks[c, :, k * 128:(k + 1) * 128], NN, 2 * n)
            kk = [_phi(v) for v in _combine(m)]
            for ct in range(2):
                zacc[:, pl.ds(_mo(c * 256 + ct * 128, 128), 128)] += (
                    (kk[ct] + kk[2 + ct]).reshape(n // 4, 8, 128).sum(axis=0))
            for s1 in range(4):
                for h in range(2):
                    pk_buf.at[s1 % 2, (s1 // 2) * 2 + h][r0:r0 + n, pl.ds(_mo(c * 128, 128), 128)] = (
                        kk[s1][h * n:(h + 1) * n])

    def z_prep():
        z = jnp.sum(zacc[...], axis=0, keepdims=True)
        zt = _pack(jnp.broadcast_to(z, (128, D)).astype(bf16).T)
        for g in range(8):
            tscr.at[g][...] = zt[g * 64:(g + 1) * 64, :]
        for j in range(8):
            blk = jnp.concatenate([tscr[g, pl.ds(j, 8, stride=8), :] for g in range(8)], axis=0)
            zp[:, j * 128:(j + 1) * 128] = _unpack(blk).T[0:8, :].astype(f32)

    def route(tok):
        rows, dots = [None] * 16, [None] * 16
        for b in sorted(range(S // 128), key=lambda b: b % 4):
            need(*[("ln", r) for r in range(max(128, b % 4 * 128), b % 4 * 128 + 128, 16)])
            rows[b] = gate(stats[b * 128:(b + 1) * 128, 0:128]).T[0:8, :]
            dots[b] = jnp.sum(gate(stats[b * 128:(b + 1) * 128, 128:256]).T, axis=0, keepdims=True)
            yield
        mf = jnp.concatenate([v[0:1] for v in rows], axis=0)
        var = jnp.concatenate([v[1:2] for v in rows], axis=0)
        tr = jnp.concatenate(dots, axis=0) * jnp.sqrt(var + 1e-5)
        wsum = jnp.sum(wrb[0:1, :], axis=1, keepdims=True)
        mb = _rbf(mf)
        inv = 1.0 / _rbf(jnp.sqrt(_rbf(_rbf(var) + 1e-5)))
        rv = _rbf((tr + (mf - mb) * wsum) * inv)
        rmax = jnp.max(jnp.max(rv, axis=1, keepdims=True), axis=0, keepdims=True)
        pos = (lax.broadcasted_iota(i32, rv.shape, 0) * 128 + lax.broadcasted_iota(i32, rv.shape, 1))
        idx = jnp.min(jnp.where(rv == rmax, pos, S - 1))
        idx_s[0] = idx

        def pick(v):
            v = jnp.sum(jnp.where(pos == idx, v, 0.0), axis=1, keepdims=True)
            return jnp.sum(v, axis=0, keepdims=True)

        xv = x_buf[(idx >> 9) & 3, pl.ds(_mo(idx & (HQ - 16), 16), 16), :].astype(f32)
        sel = lax.broadcasted_iota(i32, xv.shape, 0) == (idx & 15)
        row = jnp.sum(jnp.where(sel, xv, 0.0), axis=0, keepdims=True)
        row = _rbf(_rbf(row - pick(mb)) * pick(inv))
        rsel[...] = jnp.broadcast_to(_rbf(jnp.sum(row * wrb[0:1, :], axis=1, keepdims=True)), rsel.shape)
        xbv = jnp.broadcast_to(row, (128, D)).T
        xb[...] = xbv
        tok([xbv[b * 128 + 120:(b + 1) * 128] for b in range(8)])
        yield

    def ps_form(j, tok):
        for c in range(HQ // 16):
            def put(k1, k2, v):
                k = k1 * 7 + k2
                ps[c * 8:(c + 1) * 8, k * 128:(k + 1) * 128] = v
            yield from form_steps(
                _lform, _wl_swapped,
                lambda r, q: pk_buf[j, q, c * 16:(c + 1) * 16, r * 128:(r + 1) * 128], put, tok)

    def q_rows(j, r0, n, pq, rc, d0, rec, wts=None):
        xj = pl.ds(_mo(j * (BQ // 2), BQ // 2), BQ // 2)
        pr = slice(r0 // 2, (r0 + n) // 2)
        blk = yield from strassen2(lambda k1, k2: _unpack(xs_at(L_ORD[k1], k2, xj)[pr, :]),
                                   lambda k1, k2: wqs[k1 * 7 + k2], NN, n, 1, wts or QW)
        lane = lax.broadcasted_iota(i32, (n, 128), 1)
        for q in range(4):
            d = None
            for u in (3, 2, 1, 0):
                v = _phi(blk[q][u])
                for ct in range(2):
                    pq.at[q][d0:d0 + n, _st(u, ct)] = v[:, ct * 128:(ct + 1) * 128]
                t = v * zp[0:1, u * 256:(u + 1) * 256]
                t = t[:, :128] + t[:, 128:]
                d = t if d is None else d + t
            if rec:
                d = recip(d, lane)
            rc.at[q][d0:d0 + n, :] = d

    def recip(d, lane):
        d = d + jnp.where(lane % 2 == 0, pltpu.roll(d, 127, 1), pltpu.roll(d, 1, 1))
        d = d + jnp.where(lane % 4 < 2, pltpu.roll(d, 126, 1), pltpu.roll(d, 2, 1))
        return 1.0 / (d + 1e-6)

    def normalise(pq, rc, nr, dst, p0, raw, tok=None):
        lane = lax.broadcasted_iota(i32, (16, 128), 1)

        def fix(c):
            if c < nr // 16 and raw(c * 16):
                for q in range(4):
                    rq = slice(c * 16, (c + 1) * 16)
                    rc.at[q][rq, :] = recip(gate16(rc[q, rq, :]), lane)

        def scale(c):
            rq = slice(c * 16, (c + 1) * 16)
            fix(c + 1)
            for hf in range(2):
                for q in range(4):
                    cs = slice(hf * HD, (hf + 1) * HD)
                    pq.at[q][rq, cs] = pq[q, rq, cs] * jnp.concatenate([gate16(rc[q, rq, :])] * 4, axis=1)
                    yield

        def form(c):
            rq = slice(c * 16, (c + 1) * 16)
            p2 = pl.ds(_mo(p0 + c * 8, 8), 8)
            for ct in range(2):
                def put(k1, k2, v):
                    dst.at[k1 * 7 + k2][p2, ct * 128:(ct + 1) * 128] = v
                yield from form_steps(_lform, _wl, lambda q, u: pq[q, rq, _st(u, ct)], put, tok)

        fix(0)
        if raw(0):
            for _ in range(4):
                yield
        yield from scale(0)
        for c in range(nr // 16):
            nxt = scale(c + 1) if c + 1 < nr // 16 else iter(())
            for i, _ in enumerate(form(c)):
                yield
                if i < 8 and c + 1 < nr // 16:
                    next(nxt)
                    yield
        made.add(("qs", id(dst)))

    hist = []

    def g_lhs(k):
        v = ps[:, k * 128:(k + 1) * 128]
        hist.append(fwd[0])
        if GLAG and len(hist) > GLAG and hist[-1 - GLAG] is not None:
            cur = fwd[0]
            fwd[0] = hist[-1 - GLAG]
            v = jnp.concatenate([gate(v[i * 64:(i + 1) * 64]) for i in range(4)], axis=0)
            fwd[0] = cur
        return _unpack(v)

    def g_kvm(j):
        blk = yield from strassen2(
            lambda k1, k2: g_lhs(k1 * 7 + k2),
            lambda k1, k2: xs_at(R_ORD[k1], W_R[k2])[...], TN, 256, 2, GW, _wc_swapped)
        hm = (lax.broadcasted_iota(i32, (128, 128), 0) // 32
              == lax.broadcasted_iota(i32, (128, 128), 1) // 32)
        qb = q_rows(j, BQ - QB, QB, pqb_buf.at[j], denb_buf.at[j], 0, False, QWB)
        for _ in range(QSPLIT):
            next(qb)
        kvps = []
        for a in (3, 2, 1, 0):
            gg = jnp.concatenate(blk[a], axis=1).astype(bf16)
            wv_u = pltpu.bitcast(wv_buf[j, :, a * 128:(a + 1) * 128], u32)
            kv = jnp.where(hm, mm(gg, wv_u, NN, 256), 0.0)
            tscr2.at[a][...] = _pack(kv)
            kvps.append(_unpack(jnp.concatenate(
                [tscr2[a, pl.ds(jj, 8, stride=8), :] for jj in range(8)], axis=0)))
        mg = mg_buf

        def m_form(tok):
            for a in (3, 2, 1, 0):
                need(("mg", a))
                for jl in range(2):
                    for ct in range(2):
                        def put(k1, k2, v):
                            ms.at[k1 * 7 + k2][pl.ds(_mo(jl * 64 + (2 * a + j) * 8, 8), 8),
                                               ct * 128:(ct + 1) * 128] = v
                        yield from form_steps(
                            _rform, _wr, lambda q, u: mg[a, (2 * q + jl) * 16:(2 * q + jl + 1) * 16, _st(u, ct)], put)

        for i, a in enumerate((3, 2, 1, 0)):
            wo_u = pltpu.bitcast(wo_buf[j, a * 128:(a + 1) * 128, :], u32)
            res = mm(kvps[i], wo_u, NN, 256)
            mg.at[a][...] = _to_st(res)
            made.add(("mg", a))
            if i == 0:
                add_side(m_form, 112, MF[0], MF[1])
        for _ in qb:
            pass

    def out_part(p0, nr, y, src, pr0):
        pr = pl.ds(_mo(pr0, 8), nr // 2)
        rows = [pl.ds(_mo(q * HQ + p0, 16), nr) for q in range(4)]
        row = lax.broadcasted_iota(i32, (nr, 256), 0) + p0
        blk = yield from strassen2(lambda k1, k2: _unpack(src[k1 * 7 + k2, pr, :]),
                                   lambda k1, k2: ms[k1 * 7 + k2], NN, nr)
        for s1 in (3, 2, 1, 0):
            for s2 in range(4):
                q = (s1 // 2) * 2 + s2 // 2
                u = (s1 % 2) * 2 + s2 % 2
                rr, cc = rows[q], pl.ds(u * 256, 256)
                a = jnp.concatenate([sa[rr, :]] * 2, axis=1)
                b = jnp.concatenate([sb[rr, :]] * 2, axis=1)
                o = blk[q][u] + jnp.where(row + q * HQ == idx_s[0], y[:, u * 256:(u + 1) * 256], 0.0)
                out_buf[rr, cc] = (x_buf[q, rows[0], cc].astype(f32) * a - b + o).astype(bf16)
                if s2 % 2 == 1:
                    ch = pl.ds((s1 % 2) * HD, HD)
                    cp(out_buf.at[rr, ch], out_hbm.at[0, rr, ch], SEM_O).start()

    def ffn_part(j, f_lo, f_hi):
        def fma(acc, w, v):
            p = w.astype(f32) * v
            return acc + p[0:8] + p[8:16]

        for f0 in range(f_lo, f_hi, 256):
            fs = slice(f0, f0 + 256)
            ag = jnp.zeros((8, 256), f32)
            au = jnp.zeros((8, 256), f32)
            for k in range(0, D, 16):
                xv = jnp.concatenate([gate16(xb[k:k + 16, :])] * 2, axis=1)
                ag = fma(ag, wg_buf[j, k:k + 16, fs], xv)
                au = fma(au, wu_buf[j, k:k + 16, fs], xv)
                yield
            g = _rbf(jnp.sum(ag, axis=0, keepdims=True))
            u = _rbf(jnp.sum(au, axis=0, keepdims=True))
            h = _rbf(_rbf(g * jax.nn.sigmoid(g)) * u)
            hb_buf[fs, :] = jnp.broadcast_to(h, (128, 256)).T
        for d0 in range(0, D, 512):
            ds_ = slice(d0, d0 + 512)
            acc = yacc[:, ds_]
            for k in range(f_lo, f_hi, 16):
                hv = jnp.concatenate([gate16(hb_buf[k:k + 16, :])] * 4, axis=1)
                acc = fma(acc, wd_buf[j, k:k + 16, ds_], hv)
                yield
            yacc[:, ds_] = acc

    def wait_group(i):
        with _scope("a_wait%d" % i):
            for c in a_groups[i]:
                c.wait()

    def run_all(gen):
        for _ in gen:
            pass

    def ln_sides(plan):
        for r0, r1, t0, t1 in plan[0]:
            add_side(lambda tok, r0=r0, r1=r1: ln_stats(r0, r1 - r0, tok), (r1 - r0) // 2, t0, t1, LNLAG)
        for r0, r1, t0, t1 in plan[1]:
            add_side(lambda tok, r0=r0, r1=r1: ln_later(r0, r1 - r0, tok), 22 * (r1 - r0) // 16, t0, t1, SLAG)

    def l2_side(base, n, t0, t1):
        add_side(lambda tok: ln_later(0, n, None, "l2", base), 22 * n // 16, t0, t1)

    a_groups = make_a_groups()
    with _scope("p0_issue"):
        cp_wr.start()
        for grp in a_groups:
            for c in grp:
                c.start()
        for j in range(2):
            for part in range(2):
                for c in cp_b(j, part):
                    c.start()
        zacc[...] = jnp.zeros(zacc.shape, f32)
        yacc[...] = jnp.zeros(yacc.shape, f32)
        zero_buf[1] = jnp.zeros((8, 128), u32)
        cp_zero = cp(zero_buf.at[1], zero_buf.at[0], SEM_Z)
        cp_zero.start()
        cp_zero.wait()
        cp_wr.wait()
        wr8 = jnp.broadcast_to(wr_buf[0:D].reshape(1, D).astype(f32), (8, D))
        wrb[0:8, :] = wr8
        wrb[8:16, :] = _to_st(wr8)
        z0 = jnp.max(pltpu.bitcast(zero_buf[0], i32))
        ps, pq_buf, den_buf, mg_buf, hb_buf = [r.at[z0] for r in (ps_raw, pq_raw, den_raw, mg_raw, hb_raw)]
        xn_buf = mg_buf

    def a01(i, carry):
        with _scope("a_wait01"):
            for c in cp_x(i * X0, X0, SEM_A + i):
                c.wait()
        with _scope("a01"):
            for r in range(0, X0, 16):
                run_all(ln_stats(r, 16, None, (i, X0)))
                if r:
                    run_all(ln_later(r - 16, 16, None, "l1", (i, X0)))
            run_all(ln_later(X0 - 16, 16, None, "l1", (i, X0)))
        return carry

    lax.fori_loop(0, NX, a01, 0)
    made.update(("xn", r) for r in range(0, 64, 16))

    def a23(i, carry):
        with _scope("a_wait23"):
            for c in cp_wk(i, SEM_W + i):
                c.wait()
        with _scope("a23"):
            run_all(wk_prep(i))
            l2_side((i, 64), 64, 300, 1500)
            kproj(0, 128, [i])
            finish()
        return carry

    lax.fori_loop(0, 2, a23, 0)
    wait_group(NX + 2)
    with _scope("a4"):
        run_all(wk_prep(2))
        ln_sides(L4)
        kproj(0, 128, [2])
        finish()
    wait_group(NX + 3)
    with _scope("a5"):
        run_all(wk_prep(3))
        ln_sides(L5)
        kproj(0, 128, [3])
        for r0, n in A5K:
            kproj(r0, n)
        finish()
    wait_group(NX + 4)
    with _scope("a6"):
        ln_sides(L6)
        add_side(wq_perm, 128, A6[1], A6[2], A6[6])
        add_side(wq_form, 224, A6[3], A6[4], A6[6])
        if RT is None:
            add_side(route, 17, A6[5], A6[5] + RW)
        for r0, n in A6K:
            kproj(r0, n)
        finish()

    def b_body(j, carry):
        qa = BQ - QB
        with _scope("b_wait0"):
            for c in cp_b(j, 0, wait_only=True) + (cp_b(j, 1, wait_only=True) if MERGE else []):
                c.wait()
        with _scope("b_r0"):
            z_prep()
            t1 = 49 * qa - 400
            add_side(lambda tok: ps_form(j, tok), 7 * HQ // 16, 0, t1, SLAG if MERGE else None)
            if RT is not None:
                add_side(route, 17, RT[0], RT[1])
            if F1:
                add_side(lambda tok: ffn_part(j, 0, F1), F1 * 3 // (4 * FSTEP), 0, t1)
            for r0 in range(0, qa, QN):
                run_all(q_rows(j, r0, min(QN, qa - r0), pq_buf, den_buf, r0, r0 + QN < qa))
            if MERGE:
                flush()
            else:
                finish()
        if not MERGE:
            with _scope("b_wait1"):
                for c in cp_b(j, 1, wait_only=True):
                    c.wait()
        with _scope("b_r1"):
            add_side(lambda tok: ffn_part(j, F1, FB), (FB - F1) * 3 // (4 * FSTEP), 0, R1T[0])
            add_side(lambda tok: normalise(pq_buf, den_buf, qa, qs, j * (qa // 2),
                                           lambda r: (r // QN + 1) * QN >= qa), 22 * (qa // 16), 0, R1T[1])
            run_all(g_kvm(j))
            finish()
        return carry

    lax.fori_loop(0, 2, b_body, 0)

    def c_body(t, carry):
        with _scope("c_body"):
            y = _rbf(jnp.sum(yacc[...], axis=0, keepdims=True))
            y = _rbf(y * _rbf(1.0 / _rbf(1.0 + _rbf(jnp.exp(-rsel[0:1, :])))))
            j, h = t >> 1, t & 1
            na, nb = (BQ - QB) // 2, QB // 2
            hb = pl.ds(_mo(h * nb, 16), nb)
            add_side(lambda tok: normalise(pqb_buf.at[j, :, hb, :], denb_buf.at[j, :, hb, :], nb, qsb, 0,
                                           lambda r: True, tok),
                     4 + 22 * (nb // 16), 0, 49 * na - 800, SLAG)
            for p in range(0, na, CR):
                p0 = j * BQ + h * na + p
                run_all(out_part(p0, min(CR, na - p), y, qs, t * (na // 2) + p // 2))
            advance(clock[0] + 10 ** 6)
            flush()
            run_all(out_part(j * BQ + BQ - QB + h * nb, nb, y, qsb, 0))
            finish()
        return carry

    lax.fori_loop(0, 4, c_body, 0)
    with _scope("tail"):
        cp(out_buf, out_hbm.at[0], SEM_O).wait()


@jax.jit
def pallas_parallel_sum__linear_attn_block__moe_arch_mod__prompt_kernel(
    A_x: jax.Array,
    A_wqkv: jax.Array,
    A_wo: jax.Array,
    B_x: jax.Array,
    B_w_r: jax.Array,
    B_w_gate: jax.Array,
    B_w_up: jax.Array,
    B_w_down: jax.Array,
):
    del B_x
    V = pltpu.VMEM
    scratch = [
        V((4, HQ, D), bf16),
        V((2, D, 512), bf16),
        V((2, 512, D), bf16),
        V((8 * D,), bf16),
        V((2, D, FH), bf16),
        V((2, D, FH), bf16),
        V((2, FH, D), bf16),
        V((28, HQ // 2, 256), u32),
        V((28, HQ // 2, 256), u32),
        V((49, 128, 256), u32),
        V((S, 128), f32),
        V((S, 128), f32),
        V((8, D), f32),
        V((8, D), f32),
        V((2, 4, HQ, 512), f32),
        V((D, 128), f32),
        V((8, D), f32),
        V((8, D), f32),
        V((16, D), f32),
        V((4, 8, 128), u32),
        V((4, HD // 2, 7 * 128), u32),
        V((S, 256), f32),
        V((64, 64, 128), u32),
        V((1, HQ // 2, 49 * 128), u32),
        V((49, BQ - QB, 256), u32),
        V((49, 128, 256), u32),
        V((8, 64, 128), u32),
        V((4, 64, 128), u32),
        V((1, 4, BQ - QB, D), f32),
        V((1, 4, BQ - QB, 128), f32),
        V((2, 4, QB, D), f32),
        V((2, 4, QB, 128), f32),
        V((49, QB // 4, 256), u32),
        V((1, 4, 128, D), f32),
        V((1, FH, 128), f32),
        V((S, D), bf16),
        pltpu.SMEM((1,), i32),
        pltpu.SemaphoreType.DMA((6 + 128 // X0 + 5,)),
    ]
    return pl.pallas_call(
        _kernel,
        out_shape=jax.ShapeDtypeStruct((1, S, D), bf16),
        in_specs=[pl.BlockSpec(memory_space=pl.ANY)] * 7,
        out_specs=pl.BlockSpec(memory_space=pl.ANY),
        scratch_shapes=scratch,
        compiler_params=pltpu.CompilerParams(vmem_limit_bytes=VMEM_MB * 1024 * 1024,
                                             disable_bounds_checks=True,
                                             fuse_transposed_lhs_in_matmul=FUSE,
                                             disable_semaphore_checks=True),
    )(A_x.reshape(4, HQ, D), A_wqkv, A_wo, B_w_r, B_w_gate, B_w_up, B_w_down)
```

```python
import contextlib

import jax
import jax.numpy as jnp
from jax import lax
import jax.experimental.pallas as pl
import jax.experimental.pallas.tpu as pltpu

bf16, f32, u32, i32 = jnp.bfloat16, jnp.float32, jnp.uint32, jnp.int32

S = 2048
D = 1024
F = 3584
HD = D // 2
HQ = S // 4
BQ = HQ // 2
FH = F // 2
QB = 64
QN = 48
QSPLIT = 6
CR = 32
X0 = 32
XN = 128

SLAG = 400
LNLAG = 700
QW = (28, 36, 36, 6, 2, 2, 2)
L4 = ([(128, 192, 0, 1500)], [])
L5 = ([(192, 320, 1000, 7200)], [(128, 176, 0, 1600), (176, 320, 1700, 8600)])
L6 = ([(320, 512, 0, 6000)], [(320, 384, 800, 3400), (384, 512, 3500, 10400)])
A5K = ((128, 48), (176, 48), (224, 32))
A6K = ((256, 64), (320, 64), (384, 64), (448, 64))
WQ_PERM, WQ_FORM, ROUTE = (6200, 9000), (9100, 14000), (10600, 11400)
R1T = 12800
MF = (128, 3420)

L_ORD = (2, 3, 0, 1, 4, 5, 6)
R_ORD = (2, 0, 6, 5, 1, 4, 3)

K_SEQ = (1, 4, 0, 2, 3, 5, 6)
K_SEQ2 = (0, 1, 2, 5, 3, 4, 6)
W_SEQ = (0, 1, 5, 6, 4, 2, 3)

NN = (((1,), (0,)), ((), ()))
TN = (((0,), (0,)), ((), ()))


SCOPES = False


def _scope(name):
    return jax.named_scope(name) if SCOPES else contextlib.nullcontext()


def _mo(v, m):
    return v if isinstance(v, int) else pl.multiple_of(v, m)


def _dot(a, b, dims):
    return lax.dot_general(a, b, dims, preferred_element_type=f32)


def _pack(v):
    return pltpu.bitcast(v.astype(bf16), u32)


def _unpack(v):
    return pltpu.bitcast(v, bf16)


def _combine(m):
    m1, m2, m3, m4, m5, m6, m7 = m
    return m1 + m4 - m5 + m7, m3 + m5, m2 + m4, m1 - m2 + m3 + m6


def _lform(a11, a12, a21, a22):
    return (a11 + a22, a21 + a22, a11, a22, a11 + a12, a21 - a11, a12 - a22)


def _rform(b11, b12, b21, b22):
    return (b11 + b22, b11, b12 - b22, b21 - b11, b22, b11 + b12, b21 + b22)


def _sform(x11, x12, x21, x22):
    return (x11, x22, x11 + x22, x21 + x22, x11 + x12, x21 - x11, x12 - x22)


def _wl(a11, a12, a21, a22):
    s1 = a21 + a22
    s2 = s1 - a11
    return (a11, a12, a12 - s2, a22, s1, s2, a11 - a21)


def _wr(b11, b12, b21, b22):
    t1 = b12 - b11
    t2 = b22 - t1
    return (b11, b21, b22, t2 - b21, t1, t2, b22 - b12)


def _wc(p):
    p1, p2, p3, p4, p5, p6, p7 = p
    u2 = p1 + p6
    u3 = u2 + p7
    return p1 + p2, (u2 + p5) + p3, u3 - p4, u3 + p5


W_R = (3, 1, 0, 2, 4, 5, 6)


def _wl_swapped(a11, a12, a21, a22):
    return _wl(a12, a11, a22, a21)


def _wc_swapped(p):
    p1, p2, p3, p4, p5, p6, p7 = p
    v2 = p1 + p6
    u3 = p7 - v2
    return (p5 - v2) + p3, p1 + p2, u3 + p5, p4 - u3


class _Sym:
    def __init__(self, t):
        self.t = t

    def __add__(self, o):
        return _Sym({**self.t, **o.t})

    def __sub__(self, o):
        return _Sym({**self.t, **{k: -v for k, v in o.t.items()}})


def _st(u, ct):
    return slice((4 * ct + u) * 128, (4 * ct + u + 1) * 128)


def _to_st(v):
    return jnp.concatenate([v[:, (2 * u + ct) * 128:(2 * u + ct + 1) * 128]
                            for ct in range(2) for u in range(4)], axis=1)


def _phi(t):
    return jnp.where(t > 0, t + 1.0, jnp.exp(t)) + 1e-6


def _rbf(v):
    return v.astype(bf16).astype(f32)


def _kernel(x_hbm, wqkv_hbm, wo_hbm, wr_hbm, wg_hbm, wu_hbm, wd_hbm, out_hbm,
            x_buf, wv_buf, wo_buf, wr_buf, wg_buf, wu_buf, wd_buf,
            xs1, xs2, wqs, sa, sb, zacc, zp, pk_buf, xb, yacc, rsel, wrb, zero_buf,
            wks, stats, wqt, ps_raw, qs, ms, tscr, tscr2, pq_raw, den_raw, pqb_buf, denb_buf, qsb,
            mg_raw, hb_raw, out_buf, idx_s, sem):
    wq_buf = out_buf.at[pl.ds(0, D), :]
    wk_buf = out_buf.at[pl.ds(D, D), :]

    def xs_at(k1, e, rows=None):
        r = xs1.at[k1 * 4 + (0, 1, 7, 3).index(e)] if e in (0, 1, 7, 3) else xs2.at[k1 * 4 + (2, 4, 5, 6).index(e)]
        return r if rows is None else r.at[rows, :]

    SEM_B, SEM_O, SEM_Z, SEM_A = 0, 2, 3, 4

    def cp(src, dst, s):
        return pltpu.make_async_copy(src, dst, sem.at[s])

    def cp_x(r0, n, s):
        r = pl.ds(_mo(r0, 16), n)
        return [cp(x_hbm.at[:, r, :], x_buf.at[:, r, :], s)]

    def cp_wk(c, s):
        return [cp(wqkv_hbm.at[:, pl.ds(_mo(D + c * 256, 256), 256)],
                   wk_buf.at[:, pl.ds(_mo(c * 256, 256), 256)], s)]

    NX = 128 // X0
    SEM_W = SEM_A + NX
    cp_wr = cp(wr_hbm, wr_buf.at[pl.ds(0, D)], SEM_Z)
    a_groups = [cp_x(i * X0, X0, SEM_A + i) for i in range(NX)] + [
        cp_wk(0, SEM_W),
        cp_wk(1, SEM_W + 1),
        cp_wk(2, SEM_W + 2) + cp_x(128, 64, SEM_W + 2),
        cp_wk(3, SEM_W + 3) + cp_x(192, 128, SEM_W + 3),
        cp_x(320, 192, SEM_W + 4) + [cp(wqkv_hbm.at[:, pl.ds(0, D)], wq_buf, SEM_W + 4)],
    ]

    def cp_b(j, wait_only=False):
        dsts = [wg_buf.at[j], wu_buf.at[j], wd_buf.at[j]]
        for a in range(4):
            dsts += [wv_buf.at[j, :, pl.ds(a * 128, 128)], wo_buf.at[j, pl.ds(a * 128, 128), :]]
        if wait_only:
            return [cp(dst, dst, SEM_B + j) for dst in dsts]
        fs = pl.ds(j * FH, FH)
        srcs = [wg_hbm.at[:, fs], wu_hbm.at[:, fs], wd_hbm.at[fs, :]]
        for a in range(4):
            c0 = (2 * a + j) * 128
            srcs += [wqkv_hbm.at[:, pl.ds(2 * D + c0, 128)], wo_hbm.at[pl.ds(c0, 128), :]]
        return [cp(src, dst, SEM_B + j) for src, dst in zip(srcs, dsts)]

    clock = [0]
    toks = []
    sides = []
    fwd = [None]

    def emit_tok(vals, stamp):
        t = None
        for v in vals:
            v = pltpu.bitcast(v, u32) if v.dtype != u32 else v
            t = v if t is None else t | v
        toks.append((stamp, t & zero_buf[0]))

    def token(kind):
        t = fwd[0]
        if "u" not in t:
            t["u"] = pltpu.bitcast(t["src"](), u32) & zero_buf[0]
        if kind != "u" and "f" not in t:
            t["f"] = pltpu.bitcast(t["u"], f32)
        if kind == "f16" and "f16" not in t:
            t["f16"] = jnp.concatenate([t["f"], t["f"]], axis=0)
        return t[kind]

    def gate(v):
        if fwd[0] is None:
            return v
        head = v if v.shape[0] == 8 else v[0:8]
        head = head | token("u") if v.dtype == u32 else head + token("f")
        return head if v.shape[0] == 8 else jnp.concatenate([head, v[8:]], axis=0)

    def gate16(v):
        return v if fwd[0] is None else v + token("f16")

    def add_side(gen_fn, n, t0, t1, lag=None):
        st = {"i": 0, "n": n, "t0": clock[0] + t0, "t1": clock[0] + t1}

        def tok(vals):
            if lag is not None:
                emit_tok(vals, st["t0"] + (st["i"] + 1) * (st["t1"] - st["t0"]) // st["n"] + lag)
        st["g"] = gen_fn(tok)
        sides.append(st)

    def advance(until):
        for st in sides:
            while st["i"] < st["n"] and st["t0"] + st["i"] * (st["t1"] - st["t0"]) // st["n"] < until:
                next(st["g"], None)
                st["i"] += 1
                if st["i"] == st["n"]:
                    for _ in st["g"]:
                        pass

    def flush():
        for st in sides:
            for _ in st["g"]:
                pass
        sides.clear()

    def finish():
        flush()
        toks.clear()
        fwd[0] = None

    def mm(lhs, rhs, dims, cycles, nseg=1):
        due = [t for (c, t) in toks if c <= clock[0]]
        toks[:] = [(c, t) for (c, t) in toks if c > clock[0]]
        if due:
            head = rhs[0:8, 0:128]
            for t in due:
                head = head | t
            if rhs.shape[1] > 128:
                head = jnp.concatenate([head, rhs[0:8, 128:]], axis=1)
            rhs = jnp.concatenate([head, rhs[8:]], axis=0)
        res = _dot(lhs, _unpack(rhs), dims)
        ngr = res.shape[0] // 16
        for sg in range(nseg):
            for i in range(ngr):
                fwd[0] = {"src": lambda sg=sg, i=i: res[i * 16:i * 16 + 8, sg * 128:(sg + 1) * 128]}
                clock[0] += cycles // nseg // ngr
                advance(clock[0])
        return res

    def form_steps(form, form2, get, put, tok=None, keep=range(7)):
        terms = form(*[_Sym({i: 1}) for i in range(4)])
        gated = (0, 1, 2, 3) if 7 in keep else {_wl: (0, 1, 3), _wr: (0, 2, 3), _wl_swapped: (1, 2)}[form2]
        for k1 in range(7):
            sub = []
            for r in range(2):
                for c in range(2):
                    v = None
                    for i, sg in sorted(terms[k1].t.items(), key=lambda e: -e[1]):
                        b = get(r + 2 * (i // 2), c + 2 * (i % 2))
                        if v is None:
                            v = gate16(b) if 2 * r + c in gated else b
                        else:
                            v = v + b if sg > 0 else v - b
                    sub.append(v)
            vals = form2(*sub) + (sub[2],)
            for k2 in keep:
                put(k1, k2, _pack(vals[k2]))
            if tok is not None and k1 % 2 == 0:
                full = vals[3 if form2 is _wr else 2]
                tok([full[0:8], full[8:16]])
            yield

    def strassen2(lhs, rhs, dims, cycles, nseg=1, wts=(16,) * 7, comb=_wc):
        m1 = [None] * 7
        for i1, k1 in enumerate(K_SEQ2):
            m2 = [None] * 7
            for k2 in W_SEQ:
                m2[k2] = mm(lhs(k1, k2), rhs(k1, k2), dims, cycles * wts[i1] // 16, nseg)
                yield
            m1[k1] = comb(m2)
        out = [[None] * 4 for _ in range(4)]
        for s2 in range(4):
            for s1, v in enumerate(_combine([m1[k1][s2] for k1 in range(7)])):
                out[(s1 // 2) * 2 + s2 // 2][(s1 % 2) * 2 + s2 % 2] = v
        return out

    made = set()

    def need(*keys):
        assert all(k in made for k in keys), keys

    def row_views(base):
        if base == 0:
            return x_buf, sa, sb, stats, xn_buf, None
        i, n = base
        b = _mo(i * n, n)
        return ([x_buf.at[:, pl.ds(b, n), :]] + [r.at[pl.ds(b, S - 128 + n), :] for r in (sa, sb, stats)]
                + [xn_buf.at[:, pl.ds(b, n), :], pl.ds(_mo(i * (n // 2), n // 2), n // 2)])

    def xs_form(r0, tok, which="all", base=0):
        xn_v, xs_v = row_views(base)[4:]
        rows = slice(r0 % XN, r0 % XN + 16)

        keep = {"all": range(8), "l1": (0, 1, 7, 3), "l2": (2, 4, 5, 6)}[which]
        for ct in range(2):
            def put(k1, k2, v):
                xs_at(k1, k2, xs_v)[r0 // 2:r0 // 2 + 8, ct * 128:(ct + 1) * 128] = v
            yield from form_steps(
                _sform, _wl, lambda q, u: xn_v[q, rows, _st(u, ct)], put, tok, keep)
        made.add(("xs", r0))

    def ln_stats(r_start, n_rows, tok, base=0):
        x_v, sa_v, sb_v, st_v, xn_v, _ = row_views(base)
        lane = lax.broadcasted_iota(i32, (8, 128), 1)
        for r0 in range(r_start, r_start + n_rows, 16):
            if r0 >= 2 * XN:
                need(("ln", r0 - XN))
            for g in range(8):
                q, o = g // 2, (g % 2) * 8
                rg = q * HQ + r0 + o
                xv = x_v[q, r0 + o:r0 + o + 8, :].astype(f32)
                xg = jnp.concatenate([gate(xv[:, 0:128]), xv[:, 128:]], axis=1)
                mf = jnp.sum(xg, axis=1, keepdims=True) * (1.0 / D)
                d = xv - mf
                var = jnp.sum(d * d, axis=1, keepdims=True) * (1.0 / D)
                rs = lax.rsqrt(var + 1e-5)
                xn_v.at[q][r0 % XN + o:r0 % XN + o + 8, :] = _to_st(d * rs)
                rs = jnp.broadcast_to(rs, (8, 128))
                mf = jnp.broadcast_to(mf, (8, 128))
                sa_v[rg:rg + 8, :] = 1.0 + rs
                sb_v[rg:rg + 8, :] = mf * rs
                st_v[rg:rg + 8, 0:128] = jnp.where(lane == 0, mf, jnp.broadcast_to(var, (8, 128)))
                if tok is not None:
                    tok([rs])
                if g == 7:
                    made.add(("xn", r0))
                yield

    def ln_later(r_start, n_rows, tok, which="all", base=0):
        st_v, xn_v = row_views(base)[3:5]
        for r0 in range(r_start, r_start + n_rows, 16):
            need(("xn", r0))
            form = xs_form(r0, tok, which, base)
            for g in range(8):
                for _ in range(2 if g < 7 else 0):
                    next(form)
                    yield
                q, o = g // 2, (g % 2) * 8
                t = None
                if which != "l1":
                    v = xn_v[q, r0 % XN + o:r0 % XN + o + 8, :] * wrb[8:16, :]
                    for ct in range(8):
                        h = v[:, ct * 128:(ct + 1) * 128]
                        t = gate(h) if t is None else t + h
                if t is not None:
                    st_v[q * HQ + r0 + o:q * HQ + r0 + o + 8, 128:256] = t
                if tok is not None:
                    tok([t])
                if g == 7:
                    next(form, None)
                    made.add(("ln", r0))
                yield

    def wk_prep(c):
        cs = pl.ds(_mo(c * 256, 256), 256)
        for i in range(HD // 16):
            r0 = i * 16
            top = wk_buf[r0:r0 + 16, cs].astype(f32)
            bot = wk_buf[HD + r0:HD + r0 + 16, cs].astype(f32)
            ops = _rform(top[:, :128], top[:, 128:], bot[:, :128], bot[:, 128:])
            for k in range(7):
                wks.at[c][r0 // 2:r0 // 2 + 8, k * 128:(k + 1) * 128] = _pack(ops[k])

    def wq_perm():
        def permute(kt):
            for g in range(8):
                tile = gate(pltpu.bitcast(wq_buf[kt * 128:(kt + 1) * 128, g * 128:(g + 1) * 128], u32))
                wqt.at[kt * 8 + g][...] = pltpu.bitcast(_unpack(tile).T, u32)
                yield

        def back(kt):
            for j in range(8):
                tile = gate(jnp.concatenate([wqt[kt * 8 + g, pl.ds(j, 8, stride=8), :] for g in range(8)],
                                            axis=0))
                v = pltpu.bitcast(_unpack(tile).T.astype(f32), u32)
                c0 = (kt // 2) * D + _st(j // 2, j % 2).start
                ps[(kt % 2) * 128:(kt % 2 + 1) * 128, c0:c0 + 128] = v
                made.add(("wqp", kt, j))
                yield

        order = (0, 2, 4, 6, 1, 3, 5, 7)
        for n in range(10):
            if n < 8:
                yield from permute(order[n])
            if n > 1:
                yield from back(order[n - 2])

    def wq_form():
        for i in range(16):
            need(*[("wqp", 2 * r + i // 8, j) for r in range(4) for j in range(8)])
            for ct in range(2):
                def put(k1, k2, v):
                    wqs.at[k1 * 7 + k2][i * 8:(i + 1) * 8, ct * 128:(ct + 1) * 128] = v
                yield from form_steps(
                    _rform, _wr, lambda r, c: pltpu.bitcast(
                        ps[i * 16:(i + 1) * 16, r * D + _st(c, ct).start:r * D + _st(c, ct).stop],
                        f32), put)

    def kproj(r0, n, chunks=range(4)):
        pr = pl.ds(r0 // 2, n // 2)
        need(*[("xs", r) for r in range(max(r0, 128), r0 + n, 16)])
        for c in chunks:
            m = [None] * 7
            for k in K_SEQ:
                e11, e12, e21, e22 = [xs_at(L_ORD[k], e)[pr, :] for e in (0, 1, 7, 3)]
                lhs = jnp.concatenate([jnp.concatenate([e11, e12], axis=1),
                                       jnp.concatenate([e21, e22], axis=1)], axis=0)
                m[k] = mm(_unpack(lhs), wks[c, :, k * 128:(k + 1) * 128], NN, 2 * n)
            kk = [_phi(v) for v in _combine(m)]
            for ct in range(2):
                zacc[:, pl.ds(_mo(c * 256 + ct * 128, 128), 128)] += (
                    (kk[ct] + kk[2 + ct]).reshape(n // 4, 8, 128).sum(axis=0))
            for s1 in range(4):
                for h in range(2):
                    pk_buf.at[s1 % 2, (s1 // 2) * 2 + h][r0:r0 + n, pl.ds(_mo(c * 128, 128), 128)] = (
                        kk[s1][h * n:(h + 1) * n])

    def z_prep():
        z = jnp.sum(zacc[...], axis=0, keepdims=True)
        zt = _pack(jnp.broadcast_to(z, (128, D)).astype(bf16).T)
        for g in range(8):
            tscr.at[g][...] = zt[g * 64:(g + 1) * 64, :]
        for j in range(8):
            blk = jnp.concatenate([tscr[g, pl.ds(j, 8, stride=8), :] for g in range(8)], axis=0)
            zp[:, j * 128:(j + 1) * 128] = _unpack(blk).T[0:8, :].astype(f32)

    def route():
        rows, dots = [None] * 16, [None] * 16
        for b in sorted(range(S // 128), key=lambda b: b % 4):
            need(*[("ln", r) for r in range(max(128, b % 4 * 128), b % 4 * 128 + 128, 16)])
            rows[b] = gate(stats[b * 128:(b + 1) * 128, 0:128]).T[0:8, :]
            dots[b] = jnp.sum(gate(stats[b * 128:(b + 1) * 128, 128:256]).T, axis=0, keepdims=True)
            yield
        mf = jnp.concatenate([v[0:1] for v in rows], axis=0)
        var = jnp.concatenate([v[1:2] for v in rows], axis=0)
        tr = jnp.concatenate(dots, axis=0) * jnp.sqrt(var + 1e-5)
        wsum = jnp.sum(wrb[0:1, :], axis=1, keepdims=True)
        mb = _rbf(mf)
        inv = 1.0 / _rbf(jnp.sqrt(_rbf(_rbf(var) + 1e-5)))
        rv = _rbf((tr + (mf - mb) * wsum) * inv)
        rmax = jnp.max(jnp.max(rv, axis=1, keepdims=True), axis=0, keepdims=True)
        pos = (lax.broadcasted_iota(i32, rv.shape, 0) * 128 + lax.broadcasted_iota(i32, rv.shape, 1))
        idx = jnp.min(jnp.where(rv == rmax, pos, S - 1))
        idx_s[0] = idx

        def pick(v):
            v = jnp.sum(jnp.where(pos == idx, v, 0.0), axis=1, keepdims=True)
            return jnp.sum(v, axis=0, keepdims=True)

        xv = x_buf[(idx >> 9) & 3, pl.ds(_mo(idx & (HQ - 16), 16), 16), :].astype(f32)
        sel = lax.broadcasted_iota(i32, xv.shape, 0) == (idx & 15)
        row = jnp.sum(jnp.where(sel, xv, 0.0), axis=0, keepdims=True)
        row = _rbf(_rbf(row - pick(mb)) * pick(inv))
        rsel[...] = jnp.broadcast_to(_rbf(jnp.sum(row * wrb[0:1, :], axis=1, keepdims=True)), rsel.shape)
        xb[...] = jnp.broadcast_to(row, (128, D)).T
        yield

    def ps_form(j):
        for c in range(HQ // 16):
            def put(k1, k2, v):
                k = k1 * 7 + k2
                ps[c * 8:(c + 1) * 8, k * 128:(k + 1) * 128] = v
            yield from form_steps(
                _lform, _wl_swapped,
                lambda r, q: pk_buf[j, q, c * 16:(c + 1) * 16, r * 128:(r + 1) * 128], put)

    def q_rows(j, r0, n, pq, rc, d0, rec):
        xj = pl.ds(_mo(j * (BQ // 2), BQ // 2), BQ // 2)
        pr = slice(r0 // 2, (r0 + n) // 2)
        blk = yield from strassen2(lambda k1, k2: _unpack(xs_at(L_ORD[k1], k2, xj)[pr, :]),
                                   lambda k1, k2: wqs[k1 * 7 + k2], NN, n, 1, QW)
        lane = lax.broadcasted_iota(i32, (n, 128), 1)
        for q in range(4):
            d = None
            for u in (3, 2, 1, 0):
                v = _phi(blk[q][u])
                for ct in range(2):
                    pq.at[q][d0:d0 + n, _st(u, ct)] = v[:, ct * 128:(ct + 1) * 128]
                t = v * zp[0:1, u * 256:(u + 1) * 256]
                t = t[:, :128] + t[:, 128:]
                d = t if d is None else d + t
            if rec:
                d = recip(d, lane)
            rc.at[q][d0:d0 + n, :] = d

    def recip(d, lane):
        d = d + jnp.where(lane % 2 == 0, pltpu.roll(d, 127, 1), pltpu.roll(d, 1, 1))
        d = d + jnp.where(lane % 4 < 2, pltpu.roll(d, 126, 1), pltpu.roll(d, 2, 1))
        return 1.0 / (d + 1e-6)

    def normalise(pq, rc, nr, dst, p0, raw, tok=None):
        lane = lax.broadcasted_iota(i32, (16, 128), 1)

        def fix(c):
            if c < nr // 16 and raw(c * 16):
                for q in range(4):
                    rq = slice(c * 16, (c + 1) * 16)
                    rc.at[q][rq, :] = recip(gate16(rc[q, rq, :]), lane)

        def scale(c):
            rq = slice(c * 16, (c + 1) * 16)
            fix(c + 1)
            for hf in range(2):
                for q in range(4):
                    cs = slice(hf * HD, (hf + 1) * HD)
                    pq.at[q][rq, cs] = pq[q, rq, cs] * jnp.concatenate([gate16(rc[q, rq, :])] * 4, axis=1)
                    yield

        def form(c):
            rq = slice(c * 16, (c + 1) * 16)
            p2 = pl.ds(_mo(p0 + c * 8, 8), 8)
            for ct in range(2):
                def put(k1, k2, v):
                    dst.at[k1 * 7 + k2][p2, ct * 128:(ct + 1) * 128] = v
                yield from form_steps(_lform, _wl, lambda q, u: pq[q, rq, _st(u, ct)], put, tok)

        fix(0)
        if raw(0):
            for _ in range(4):
                yield
        yield from scale(0)
        for c in range(nr // 16):
            nxt = scale(c + 1) if c + 1 < nr // 16 else iter(())
            for i, _ in enumerate(form(c)):
                yield
                if i < 8 and c + 1 < nr // 16:
                    next(nxt)
                    yield

    def g_kvm(j):
        blk = yield from strassen2(
            lambda k1, k2: _unpack(ps[:, (k1 * 7 + k2) * 128:(k1 * 7 + k2 + 1) * 128]),
            lambda k1, k2: xs_at(R_ORD[k1], W_R[k2])[...], TN, 256, 2, comb=_wc_swapped)
        hm = (lax.broadcasted_iota(i32, (128, 128), 0) // 32
              == lax.broadcasted_iota(i32, (128, 128), 1) // 32)
        qb = q_rows(j, BQ - QB, QB, pqb_buf.at[j], denb_buf.at[j], 0, False)
        for _ in range(QSPLIT):
            next(qb)
        kvps = []
        for a in (3, 2, 1, 0):
            gg = jnp.concatenate(blk[a], axis=1).astype(bf16)
            wv_u = pltpu.bitcast(wv_buf[j, :, a * 128:(a + 1) * 128], u32)
            kv = jnp.where(hm, mm(gg, wv_u, NN, 256), 0.0)
            tscr2.at[a][...] = _pack(kv)
            kvps.append(_unpack(jnp.concatenate(
                [tscr2[a, pl.ds(jj, 8, stride=8), :] for jj in range(8)], axis=0)))

        def m_form():
            for a in (3, 2, 1, 0):
                need(("mg", a))
                for jl in range(2):
                    for ct in range(2):
                        def put(k1, k2, v):
                            ms.at[k1 * 7 + k2][pl.ds(_mo(jl * 64 + (2 * a + j) * 8, 8), 8),
                                               ct * 128:(ct + 1) * 128] = v
                        yield from form_steps(
                            _rform, _wr, lambda q, u: mg_buf[a, (2 * q + jl) * 16:(2 * q + jl + 1) * 16, _st(u, ct)], put)

        for i, a in enumerate((3, 2, 1, 0)):
            wo_u = pltpu.bitcast(wo_buf[j, a * 128:(a + 1) * 128, :], u32)
            res = mm(kvps[i], wo_u, NN, 256)
            mg_buf.at[a][...] = _to_st(res)
            made.add(("mg", a))
            if i == 0:
                add_side(lambda tok: m_form(), 112, *MF)
        for _ in qb:
            pass

    def out_part(p0, nr, y, src, pr0):
        pr = pl.ds(_mo(pr0, 8), nr // 2)
        rows = [pl.ds(_mo(q * HQ + p0, 16), nr) for q in range(4)]
        row = lax.broadcasted_iota(i32, (nr, 256), 0) + p0
        blk = yield from strassen2(lambda k1, k2: _unpack(src[k1 * 7 + k2, pr, :]),
                                   lambda k1, k2: ms[k1 * 7 + k2], NN, nr)
        for s1 in (3, 2, 1, 0):
            for s2 in range(4):
                q = (s1 // 2) * 2 + s2 // 2
                u = (s1 % 2) * 2 + s2 % 2
                rr, cc = rows[q], pl.ds(u * 256, 256)
                a = jnp.concatenate([sa[rr, :]] * 2, axis=1)
                b = jnp.concatenate([sb[rr, :]] * 2, axis=1)
                o = blk[q][u] + jnp.where(row + q * HQ == idx_s[0], y[:, u * 256:(u + 1) * 256], 0.0)
                out_buf[rr, cc] = (x_buf[q, rows[0], cc].astype(f32) * a - b + o).astype(bf16)
                if s2 % 2 == 1:
                    ch = pl.ds((s1 % 2) * HD, HD)
                    cp(out_buf.at[rr, ch], out_hbm.at[0, rr, ch], SEM_O).start()

    def ffn_part(j):
        def fma(acc, w, v):
            p = w.astype(f32) * v
            return acc + p[0:8] + p[8:16]

        for f0 in range(0, FH, 256):
            fs = slice(f0, f0 + 256)
            ag = jnp.zeros((8, 256), f32)
            au = jnp.zeros((8, 256), f32)
            for k in range(0, D, 16):
                xv = jnp.concatenate([gate16(xb[k:k + 16, :])] * 2, axis=1)
                ag = fma(ag, wg_buf[j, k:k + 16, fs], xv)
                au = fma(au, wu_buf[j, k:k + 16, fs], xv)
                yield
            g = _rbf(jnp.sum(ag, axis=0, keepdims=True))
            u = _rbf(jnp.sum(au, axis=0, keepdims=True))
            h = _rbf(_rbf(g * jax.nn.sigmoid(g)) * u)
            hb_buf[fs, :] = jnp.broadcast_to(h, (128, 256)).T
        for d0 in range(0, D, 512):
            ds_ = slice(d0, d0 + 512)
            acc = yacc[:, ds_]
            for k in range(0, FH, 16):
                hv = jnp.concatenate([gate16(hb_buf[k:k + 16, :])] * 4, axis=1)
                acc = fma(acc, wd_buf[j, k:k + 16, ds_], hv)
                yield
            yacc[:, ds_] = acc

    def wait_group(i):
        with _scope("a_wait%d" % i):
            for c in a_groups[i]:
                c.wait()

    def run_all(gen):
        for _ in gen:
            pass

    def ln_sides(plan):
        for r0, r1, t0, t1 in plan[0]:
            add_side(lambda tok, r0=r0, r1=r1: ln_stats(r0, r1 - r0, tok), (r1 - r0) // 2, t0, t1, LNLAG)
        for r0, r1, t0, t1 in plan[1]:
            add_side(lambda tok, r0=r0, r1=r1: ln_later(r0, r1 - r0, tok), 22 * (r1 - r0) // 16, t0, t1, SLAG)

    def l2_side(base, n, t0, t1):
        add_side(lambda tok: ln_later(0, n, None, "l2", base), 22 * n // 16, t0, t1)

    with _scope("p0_issue"):
        cp_wr.start()
        for grp in a_groups:
            for c in grp:
                c.start()
        for j in range(2):
            for c in cp_b(j):
                c.start()
        zacc[...] = jnp.zeros(zacc.shape, f32)
        yacc[...] = jnp.zeros(yacc.shape, f32)
        zero_buf[1] = jnp.zeros((8, 128), u32)
        cp_zero = cp(zero_buf.at[1], zero_buf.at[0], SEM_Z)
        cp_zero.start()
        cp_zero.wait()
        cp_wr.wait()
        wr8 = jnp.broadcast_to(wr_buf[0:D].reshape(1, D).astype(f32), (8, D))
        wrb[0:8, :] = wr8
        wrb[8:16, :] = _to_st(wr8)
        z0 = jnp.max(pltpu.bitcast(zero_buf[0], i32))
        ps, pq_buf, den_buf, mg_buf, hb_buf = [r.at[z0] for r in (ps_raw, pq_raw, den_raw, mg_raw, hb_raw)]
        xn_buf = mg_buf

    def a01(i, carry):
        with _scope("a_wait01"):
            for c in cp_x(i * X0, X0, SEM_A + i):
                c.wait()
        with _scope("a01"):
            for r in range(0, X0, 16):
                run_all(ln_stats(r, 16, None, (i, X0)))
                if r:
                    run_all(ln_later(r - 16, 16, None, "l1", (i, X0)))
            run_all(ln_later(X0 - 16, 16, None, "l1", (i, X0)))
        return carry

    lax.fori_loop(0, NX, a01, 0)
    made.update(("xn", r) for r in range(0, 64, 16))

    def a23(i, carry):
        with _scope("a_wait23"):
            for c in cp_wk(i, SEM_W + i):
                c.wait()
        with _scope("a23"):
            wk_prep(i)
            l2_side((i, 64), 64, 300, 1500)
            kproj(0, 128, [i])
            finish()
        return carry

    lax.fori_loop(0, 2, a23, 0)
    wait_group(NX + 2)
    with _scope("a4"):
        wk_prep(2)
        ln_sides(L4)
        kproj(0, 128, [2])
        finish()
    wait_group(NX + 3)
    with _scope("a5"):
        wk_prep(3)
        ln_sides(L5)
        kproj(0, 128, [3])
        for r0, n in A5K:
            kproj(r0, n)
        finish()
    wait_group(NX + 4)
    with _scope("a6"):
        ln_sides(L6)
        add_side(lambda tok: wq_perm(), 128, *WQ_PERM)
        add_side(lambda tok: wq_form(), 224, *WQ_FORM)
        add_side(lambda tok: route(), 17, *ROUTE)
        for r0, n in A6K:
            kproj(r0, n)
        finish()

    def b_body(j, carry):
        qa = BQ - QB
        with _scope("b_r0"):
            z_prep()
            add_side(lambda tok: ps_form(j), 7 * HQ // 16, 0, 49 * qa - 400)
            for r0 in range(0, qa, QN):
                run_all(q_rows(j, r0, QN, pq_buf, den_buf, r0, r0 + QN < qa))
            finish()
        with _scope("b_wait"):
            for c in cp_b(j, wait_only=True):
                c.wait()
        with _scope("b_r1"):
            add_side(lambda tok: ffn_part(j), FH * 3 // 8, 0, R1T)
            add_side(lambda tok: normalise(pq_buf, den_buf, qa, qs, j * (qa // 2), lambda r: r >= qa - QN),
                     22 * (qa // 16), 0, R1T)
            run_all(g_kvm(j))
            finish()
        return carry

    lax.fori_loop(0, 2, b_body, 0)

    def c_body(t, carry):
        with _scope("c_body"):
            y = _rbf(jnp.sum(yacc[...], axis=0, keepdims=True))
            y = _rbf(y * _rbf(1.0 / _rbf(1.0 + _rbf(jnp.exp(-rsel[0:1, :])))))
            j, h = t >> 1, t & 1
            na, nb = (BQ - QB) // 2, QB // 2
            hb = pl.ds(_mo(h * nb, 16), nb)
            add_side(lambda tok: normalise(pqb_buf.at[j, :, hb, :], denb_buf.at[j, :, hb, :], nb, qsb, 0,
                                           lambda r: True, tok),
                     4 + 22 * (nb // 16), 0, 49 * na - 800, SLAG)
            for p in range(0, na, CR):
                p0 = j * BQ + h * na + p
                run_all(out_part(p0, CR, y, qs, t * (na // 2) + p // 2))
            flush()
            run_all(out_part(j * BQ + BQ - QB + h * nb, nb, y, qsb, 0))
            finish()
        return carry

    lax.fori_loop(0, 4, c_body, 0)
    with _scope("tail"):
        cp(out_buf, out_hbm.at[0], SEM_O).wait()


@jax.jit
def pallas_parallel_sum__linear_attn_block__moe_arch_mod__prompt_kernel(
    A_x: jax.Array,
    A_wqkv: jax.Array,
    A_wo: jax.Array,
    B_x: jax.Array,
    B_w_r: jax.Array,
    B_w_gate: jax.Array,
    B_w_up: jax.Array,
    B_w_down: jax.Array,
):
    del B_x
    V = pltpu.VMEM
    scratch = [
        V((4, HQ, D), bf16),
        V((2, D, 512), bf16),
        V((2, 512, D), bf16),
        V((8 * D,), bf16),
        V((2, D, FH), bf16),
        V((2, D, FH), bf16),
        V((2, FH, D), bf16),
        V((28, HQ // 2, 256), u32),
        V((28, HQ // 2, 256), u32),
        V((49, 128, 256), u32),
        V((S, 128), f32),
        V((S, 128), f32),
        V((8, D), f32),
        V((8, D), f32),
        V((2, 4, HQ, 512), f32),
        V((D, 128), f32),
        V((8, D), f32),
        V((8, D), f32),
        V((16, D), f32),
        V((4, 8, 128), u32),
        V((4, HD // 2, 7 * 128), u32),
        V((S, 256), f32),
        V((64, 64, 128), u32),
        V((1, HQ // 2, 49 * 128), u32),
        V((49, BQ - QB, 256), u32),
        V((49, 128, 256), u32),
        V((8, 64, 128), u32),
        V((4, 64, 128), u32),
        V((1, 4, BQ - QB, D), f32),
        V((1, 4, BQ - QB, 128), f32),
        V((2, 4, QB, D), f32),
        V((2, 4, QB, 128), f32),
        V((49, QB // 4, 256), u32),
        V((1, 4, 128, D), f32),
        V((1, FH, 128), f32),
        V((S, D), bf16),
        pltpu.SMEM((1,), i32),
        pltpu.SemaphoreType.DMA((4 + 128 // X0 + 5,)),
    ]
    extra = {k: True for k in ("disable_bounds_checks", "disable_semaphore_checks")
             if hasattr(pltpu.CompilerParams, k)}
    return pl.pallas_call(
        _kernel,
        out_shape=jax.ShapeDtypeStruct((1, S, D), bf16),
        in_specs=[pl.BlockSpec(memory_space=pl.ANY)] * 7,
        out_specs=pl.BlockSpec(memory_space=pl.ANY),
        scratch_shapes=scratch,
        compiler_params=pltpu.CompilerParams(vmem_limit_bytes=120 * 1024 * 1024, **extra),
    )(A_x.reshape(4, HQ, D), A_wqkv, A_wo, B_w_r, B_w_gate, B_w_up, B_w_down)
```

```python
import contextlib

import jax
import jax.numpy as jnp
from jax import lax
import jax.experimental.pallas as pl
import jax.experimental.pallas.tpu as pltpu

bf16, f32, u32, i32 = jnp.bfloat16, jnp.float32, jnp.uint32, jnp.int32

S = 2048
D = 1024
F = 3584
HD = D // 2
HQ = S // 4
BQ = HQ // 2
FH = F // 2
QB = 64
QN = 48
QSPLIT = 6
CR = 32
T0 = 96
X0 = 32
XG = (160, 208)
XN = 128

SLAG = 400
LNLAG = 700
QW = (28, 36, 36, 6, 2, 2, 2)
L4 = ([(96, 144, 0, 1100)], [])
L5 = ([(144, 208, 1100, 3500)], [(96, 128, 0, 1150), (128, 144, 1250, 2000), (144, 208, 2300, 4700)])
L6 = ([(208, 512, 0, 10000)], [(208, 256, 800, 2600), (256, 448, 2700, 10500)])
L7 = ([], [(448, 512, 0, 3000)])
A5K = ((96, 32), (128, 32))
A6K = ((160, 48), (208, 48), (256, 48), (304, 48))
A7K = ((352, 48), (400, 48), (448, 64))
WQ_PERM, WQ_FORM, ROUTE = (0, 3200), (3300, 8600), (4500, 5300)
R1T = 12800
MF = (128, 3420)

L_ORD = (2, 3, 0, 1, 4, 5, 6)
R_ORD = (2, 0, 6, 5, 1, 4, 3)

K_SEQ = (1, 4, 0, 2, 3, 5, 6)
K_SEQ2 = (0, 1, 2, 5, 3, 4, 6)
W_SEQ = (0, 1, 5, 6, 4, 2, 3)

NN = (((1,), (0,)), ((), ()))
TN = (((0,), (0,)), ((), ()))


SCOPES = False


def _scope(name):
    return jax.named_scope(name) if SCOPES else contextlib.nullcontext()


def _mo(v, m):
    return v if isinstance(v, int) else pl.multiple_of(v, m)


def _dot(a, b, dims):
    return lax.dot_general(a, b, dims, preferred_element_type=f32)


def _pack(v):
    return pltpu.bitcast(v.astype(bf16), u32)


def _unpack(v):
    return pltpu.bitcast(v, bf16)


def _combine(m):
    m1, m2, m3, m4, m5, m6, m7 = m
    return m1 + m4 - m5 + m7, m3 + m5, m2 + m4, m1 - m2 + m3 + m6


def _lform(a11, a12, a21, a22):
    return (a11 + a22, a21 + a22, a11, a22, a11 + a12, a21 - a11, a12 - a22)


def _rform(b11, b12, b21, b22):
    return (b11 + b22, b11, b12 - b22, b21 - b11, b22, b11 + b12, b21 + b22)


def _sform(x11, x12, x21, x22):
    return (x11, x22, x11 + x22, x21 + x22, x11 + x12, x21 - x11, x12 - x22)


def _wl(a11, a12, a21, a22):
    s1 = a21 + a22
    s2 = s1 - a11
    return (a11, a12, a12 - s2, a22, s1, s2, a11 - a21)


def _wr(b11, b12, b21, b22):
    t1 = b12 - b11
    t2 = b22 - t1
    return (b11, b21, b22, t2 - b21, t1, t2, b22 - b12)


def _wc(p):
    p1, p2, p3, p4, p5, p6, p7 = p
    u2 = p1 + p6
    u3 = u2 + p7
    return p1 + p2, (u2 + p5) + p3, u3 - p4, u3 + p5


W_R = (3, 1, 0, 2, 4, 5, 6)


def _wl_swapped(a11, a12, a21, a22):
    return _wl(a12, a11, a22, a21)


def _wc_swapped(p):
    p1, p2, p3, p4, p5, p6, p7 = p
    v2 = p1 + p6
    u3 = p7 - v2
    return (p5 - v2) + p3, p1 + p2, u3 + p5, p4 - u3


class _Sym:
    def __init__(self, t):
        self.t = t

    def __add__(self, o):
        return _Sym({**self.t, **o.t})

    def __sub__(self, o):
        return _Sym({**self.t, **{k: -v for k, v in o.t.items()}})


def _st(u, ct):
    return slice((4 * ct + u) * 128, (4 * ct + u + 1) * 128)


def _to_st(v):
    return jnp.concatenate([v[:, (2 * u + ct) * 128:(2 * u + ct + 1) * 128]
                            for ct in range(2) for u in range(4)], axis=1)


def _phi(t):
    return jnp.where(t > 0, t + 1.0, jnp.exp(t)) + 1e-6


def _rbf(v):
    return v.astype(bf16).astype(f32)


def _kernel(x_hbm, wqkv_hbm, wo_hbm, wr_hbm, wg_hbm, wu_hbm, wd_hbm, out_hbm,
            x_buf, wv_buf, wo_buf, wr_buf, wg_buf, wu_buf, wd_buf,
            xs1, xs2, wqs, sa, sb, zacc, zp, pk_buf, xb, yacc, rsel, wrb, zero_buf,
            wks, stats, wqt, ps_raw, qs, ms, tscr, tscr2, pq_raw, den_raw, pqb_buf, denb_buf, qsb,
            mg_raw, hb_raw, out_buf, idx_s, sem):
    wq_buf = out_buf.at[pl.ds(0, D), :]
    wk_buf = out_buf.at[pl.ds(D, D), :]

    def xs_at(k1, e, rows=None):
        r = xs1.at[k1 * 4 + (0, 1, 7, 3).index(e)] if e in (0, 1, 7, 3) else xs2.at[k1 * 4 + (2, 4, 5, 6).index(e)]
        return r if rows is None else r.at[rows, :]

    SEM_B, SEM_O, SEM_Z, SEM_A = 0, 2, 3, 4

    def cp(src, dst, s):
        return pltpu.make_async_copy(src, dst, sem.at[s])

    def cp_x(r0, n, s):
        r = pl.ds(_mo(r0, 16), n)
        return [cp(x_hbm.at[:, r, :], x_buf.at[:, r, :], s)]

    def cp_wk(c, s):
        return [cp(wqkv_hbm.at[:, pl.ds(_mo(D + c * 256, 256), 256)],
                   wk_buf.at[:, pl.ds(_mo(c * 256, 256), 256)], s)]

    NX = T0 // X0
    SEM_W = SEM_A + NX
    cp_wr = cp(wr_hbm, wr_buf.at[pl.ds(0, D)], SEM_Z)
    a_groups = [cp_x(i * X0, X0, SEM_A + i) for i in range(NX)] + [
        cp_wk(0, SEM_W),
        cp_wk(1, SEM_W + 1),
        cp_wk(2, SEM_W + 2) + cp_x(T0, XG[0] - T0, SEM_W + 2),
        cp_wk(3, SEM_W + 3) + cp_x(XG[0], XG[1] - XG[0], SEM_W + 3),
        cp_x(XG[1], HQ - XG[1], SEM_W + 4),
        [cp(wqkv_hbm.at[:, pl.ds(0, D)], wq_buf, SEM_W + 5)],
    ]

    def cp_b(j, wait_only=False):
        dsts = [wg_buf.at[j], wu_buf.at[j], wd_buf.at[j]]
        for a in range(4):
            dsts += [wv_buf.at[j, :, pl.ds(a * 128, 128)], wo_buf.at[j, pl.ds(a * 128, 128), :]]
        if wait_only:
            return [cp(dst, dst, SEM_B + j) for dst in dsts]
        fs = pl.ds(j * FH, FH)
        srcs = [wg_hbm.at[:, fs], wu_hbm.at[:, fs], wd_hbm.at[fs, :]]
        for a in range(4):
            c0 = (2 * a + j) * 128
            srcs += [wqkv_hbm.at[:, pl.ds(2 * D + c0, 128)], wo_hbm.at[pl.ds(c0, 128), :]]
        return [cp(src, dst, SEM_B + j) for src, dst in zip(srcs, dsts)]

    clock = [0]
    toks = []
    sides = []
    fwd = [None]

    def emit_tok(vals, stamp):
        t = None
        for v in vals:
            v = pltpu.bitcast(v, u32) if v.dtype != u32 else v
            t = v if t is None else t | v
        toks.append((stamp, t & zero_buf[0]))

    def token(kind):
        t = fwd[0]
        if "u" not in t:
            t["u"] = pltpu.bitcast(t["src"](), u32) & zero_buf[0]
        if kind != "u" and "f" not in t:
            t["f"] = pltpu.bitcast(t["u"], f32)
        if kind == "f16" and "f16" not in t:
            t["f16"] = jnp.concatenate([t["f"], t["f"]], axis=0)
        return t[kind]

    def gate(v):
        if fwd[0] is None:
            return v
        head = v if v.shape[0] == 8 else v[0:8]
        head = head | token("u") if v.dtype == u32 else head + token("f")
        return head if v.shape[0] == 8 else jnp.concatenate([head, v[8:]], axis=0)

    def gate16(v):
        return v if fwd[0] is None else v + token("f16")

    def add_side(gen_fn, n, t0, t1, lag=None):
        st = {"i": 0, "n": n, "t0": clock[0] + t0, "t1": clock[0] + t1}

        def tok(vals):
            if lag is not None:
                emit_tok(vals, st["t0"] + (st["i"] + 1) * (st["t1"] - st["t0"]) // st["n"] + lag)
        st["g"] = gen_fn(tok)
        sides.append(st)

    def advance(until):
        for st in sides:
            while st["i"] < st["n"] and st["t0"] + st["i"] * (st["t1"] - st["t0"]) // st["n"] < until:
                next(st["g"], None)
                st["i"] += 1
                if st["i"] == st["n"]:
                    for _ in st["g"]:
                        pass

    def flush():
        for st in sides:
            for _ in st["g"]:
                pass
        sides.clear()

    def finish():
        flush()
        toks.clear()
        fwd[0] = None

    def mm(lhs, rhs, dims, cycles, nseg=1):
        due = [t for (c, t) in toks if c <= clock[0]]
        toks[:] = [(c, t) for (c, t) in toks if c > clock[0]]
        if due:
            head = rhs[0:8, 0:128]
            for t in due:
                head = head | t
            if rhs.shape[1] > 128:
                head = jnp.concatenate([head, rhs[0:8, 128:]], axis=1)
            rhs = jnp.concatenate([head, rhs[8:]], axis=0)
        res = _dot(lhs, _unpack(rhs), dims)
        ngr = res.shape[0] // 16
        for sg in range(nseg):
            for i in range(ngr):
                fwd[0] = {"src": lambda sg=sg, i=i: res[i * 16:i * 16 + 8, sg * 128:(sg + 1) * 128]}
                clock[0] += cycles // nseg // ngr
                advance(clock[0])
        return res

    def form_steps(form, form2, get, put, tok=None, keep=range(7)):
        terms = form(*[_Sym({i: 1}) for i in range(4)])
        gated = (0, 1, 2, 3) if 7 in keep else {_wl: (0, 1, 3), _wr: (0, 2, 3), _wl_swapped: (1, 2)}[form2]
        for k1 in range(7):
            sub = []
            for r in range(2):
                for c in range(2):
                    v = None
                    for i, sg in sorted(terms[k1].t.items(), key=lambda e: -e[1]):
                        b = get(r + 2 * (i // 2), c + 2 * (i % 2))
                        if v is None:
                            v = gate16(b) if 2 * r + c in gated else b
                        else:
                            v = v + b if sg > 0 else v - b
                    sub.append(v)
            vals = form2(*sub) + (sub[2],)
            for k2 in keep:
                put(k1, k2, _pack(vals[k2]))
            if tok is not None and k1 % 2 == 0:
                full = vals[3 if form2 is _wr else 2]
                tok([full[0:8], full[8:16]])
            yield

    def strassen2(lhs, rhs, dims, cycles, nseg=1, wts=(16,) * 7, comb=_wc):
        m1 = [None] * 7
        for i1, k1 in enumerate(K_SEQ2):
            m2 = [None] * 7
            for k2 in W_SEQ:
                m2[k2] = mm(lhs(k1, k2), rhs(k1, k2), dims, cycles * wts[i1] // 16, nseg)
                yield
            m1[k1] = comb(m2)
        out = [[None] * 4 for _ in range(4)]
        for s2 in range(4):
            for s1, v in enumerate(_combine([m1[k1][s2] for k1 in range(7)])):
                out[(s1 // 2) * 2 + s2 // 2][(s1 % 2) * 2 + s2 % 2] = v
        return out

    made = set()

    def need(*keys):
        assert all(k in made for k in keys), keys

    def row_views(base):
        if base == 0:
            return x_buf, sa, sb, stats, xn_buf, None
        i, n = base
        b = _mo(i * n, 16)
        return ([x_buf.at[:, pl.ds(b, n), :]] + [r.at[pl.ds(b, S - 128 + n), :] for r in (sa, sb, stats)]
                + [xn_buf.at[:, pl.ds(b, n), :], pl.ds(_mo(i * (n // 2), 8), n // 2)])

    def xs_form(r0, tok, which="all", base=0):
        xn_v, xs_v = row_views(base)[4:]
        rows = slice(r0 % XN, r0 % XN + 16)

        keep = {"all": range(8), "l1": (0, 1, 7, 3), "l2": (2, 4, 5, 6)}[which]
        for ct in range(2):
            def put(k1, k2, v):
                xs_at(k1, k2, xs_v)[r0 // 2:r0 // 2 + 8, ct * 128:(ct + 1) * 128] = v
            yield from form_steps(
                _sform, _wl, lambda q, u: xn_v[q, rows, _st(u, ct)], put, tok, keep)
        made.add(("xs", r0))

    def ln_stats(r_start, n_rows, tok, base=0):
        x_v, sa_v, sb_v, st_v, xn_v, _ = row_views(base)
        lane = lax.broadcasted_iota(i32, (8, 128), 1)
        for r0 in range(r_start, r_start + n_rows, 16):
            if r0 - XN >= T0:
                need(("ln", r0 - XN))
            for g in range(8):
                q, o = g // 2, (g % 2) * 8
                rg = q * HQ + r0 + o
                xv = x_v[q, r0 + o:r0 + o + 8, :].astype(f32)
                xg = jnp.concatenate([gate(xv[:, 0:128]), xv[:, 128:]], axis=1)
                mf = jnp.sum(xg, axis=1, keepdims=True) * (1.0 / D)
                d = xv - mf
                var = jnp.sum(d * d, axis=1, keepdims=True) * (1.0 / D)
                rs = lax.rsqrt(var + 1e-5)
                xn_v.at[q][r0 % XN + o:r0 % XN + o + 8, :] = _to_st(d * rs)
                rs = jnp.broadcast_to(rs, (8, 128))
                mf = jnp.broadcast_to(mf, (8, 128))
                sa_v[rg:rg + 8, :] = 1.0 + rs
                sb_v[rg:rg + 8, :] = mf * rs
                st_v[rg:rg + 8, 0:128] = jnp.where(lane == 0, mf, jnp.broadcast_to(var, (8, 128)))
                if tok is not None:
                    tok([rs])
                if g == 7:
                    made.add(("xn", r0))
                yield

    def ln_later(r_start, n_rows, tok, which="all", base=0):
        st_v, xn_v = row_views(base)[3:5]
        for r0 in range(r_start, r_start + n_rows, 16):
            need(("xn", r0))
            form = xs_form(r0, tok, which, base)
            for g in range(8):
                for _ in range(2 if g < 7 else 0):
                    next(form)
                    yield
                q, o = g // 2, (g % 2) * 8
                t = None
                if which != "l1":
                    v = xn_v[q, r0 % XN + o:r0 % XN + o + 8, :] * wrb[8:16, :]
                    for ct in range(8):
                        h = v[:, ct * 128:(ct + 1) * 128]
                        t = gate(h) if t is None else t + h
                if t is not None:
                    st_v[q * HQ + r0 + o:q * HQ + r0 + o + 8, 128:256] = t
                if tok is not None:
                    tok([t])
                if g == 7:
                    next(form, None)
                    made.add(("ln", r0))
                yield

    def wk_prep(c):
        cs = pl.ds(_mo(c * 256, 256), 256)
        for i in range(HD // 16):
            r0 = i * 16
            top = wk_buf[r0:r0 + 16, cs].astype(f32)
            bot = wk_buf[HD + r0:HD + r0 + 16, cs].astype(f32)
            ops = _rform(top[:, :128], top[:, 128:], bot[:, :128], bot[:, 128:])
            for k in range(7):
                wks.at[c][r0 // 2:r0 // 2 + 8, k * 128:(k + 1) * 128] = _pack(ops[k])

    def wq_perm():
        def permute(kt):
            for g in range(8):
                tile = gate(pltpu.bitcast(wq_buf[kt * 128:(kt + 1) * 128, g * 128:(g + 1) * 128], u32))
                wqt.at[kt * 8 + g][...] = pltpu.bitcast(_unpack(tile).T, u32)
                yield

        def back(kt):
            for j in range(8):
                tile = gate(jnp.concatenate([wqt[kt * 8 + g, pl.ds(j, 8, stride=8), :] for g in range(8)],
                                            axis=0))
                v = pltpu.bitcast(_unpack(tile).T.astype(f32), u32)
                c0 = (kt // 2) * D + _st(j // 2, j % 2).start
                ps[(kt % 2) * 128:(kt % 2 + 1) * 128, c0:c0 + 128] = v
                made.add(("wqp", kt, j))
                yield

        order = (0, 2, 4, 6, 1, 3, 5, 7)
        for n in range(10):
            if n < 8:
                yield from permute(order[n])
            if n > 1:
                yield from back(order[n - 2])

    def wq_form():
        for i in range(16):
            need(*[("wqp", 2 * r + i // 8, j) for r in range(4) for j in range(8)])
            for ct in range(2):
                def put(k1, k2, v):
                    wqs.at[k1 * 7 + k2][i * 8:(i + 1) * 8, ct * 128:(ct + 1) * 128] = v
                yield from form_steps(
                    _rform, _wr, lambda r, c: pltpu.bitcast(
                        ps[i * 16:(i + 1) * 16, r * D + _st(c, ct).start:r * D + _st(c, ct).stop],
                        f32), put)

    def kproj(r0, n, chunks=range(4)):
        pr = pl.ds(r0 // 2, n // 2)
        need(*[("xs", r) for r in range(max(r0, T0), r0 + n, 16)])
        for c in chunks:
            m = [None] * 7
            for k in K_SEQ:
                e11, e12, e21, e22 = [xs_at(L_ORD[k], e)[pr, :] for e in (0, 1, 7, 3)]
                lhs = jnp.concatenate([jnp.concatenate([e11, e12], axis=1),
                                       jnp.concatenate([e21, e22], axis=1)], axis=0)
                m[k] = mm(_unpack(lhs), wks[c, :, k * 128:(k + 1) * 128], NN, 2 * n)
            kk = [_phi(v) for v in _combine(m)]
            for ct in range(2):
                zacc[:, pl.ds(_mo(c * 256 + ct * 128, 128), 128)] += (
                    (kk[ct] + kk[2 + ct]).reshape(n // 4, 8, 128).sum(axis=0))
            for s1 in range(4):
                for h in range(2):
                    pk_buf.at[s1 % 2, (s1 // 2) * 2 + h][r0:r0 + n, pl.ds(_mo(c * 128, 128), 128)] = (
                        kk[s1][h * n:(h + 1) * n])

    def z_prep():
        z = jnp.sum(zacc[...], axis=0, keepdims=True)
        zt = _pack(jnp.broadcast_to(z, (128, D)).astype(bf16).T)
        for g in range(8):
            tscr.at[g][...] = zt[g * 64:(g + 1) * 64, :]
        for j in range(8):
            blk = jnp.concatenate([tscr[g, pl.ds(j, 8, stride=8), :] for g in range(8)], axis=0)
            zp[:, j * 128:(j + 1) * 128] = _unpack(blk).T[0:8, :].astype(f32)

    def route():
        rows, dots = [None] * 16, [None] * 16
        for b in sorted(range(S // 128), key=lambda b: b % 4):
            need(*[("ln", r) for r in range(max(T0, b % 4 * 128), b % 4 * 128 + 128, 16)])
            rows[b] = gate(stats[b * 128:(b + 1) * 128, 0:128]).T[0:8, :]
            dots[b] = jnp.sum(gate(stats[b * 128:(b + 1) * 128, 128:256]).T, axis=0, keepdims=True)
            yield
        mf = jnp.concatenate([v[0:1] for v in rows], axis=0)
        var = jnp.concatenate([v[1:2] for v in rows], axis=0)
        tr = jnp.concatenate(dots, axis=0) * jnp.sqrt(var + 1e-5)
        wsum = jnp.sum(wrb[0:1, :], axis=1, keepdims=True)
        mb = _rbf(mf)
        inv = 1.0 / _rbf(jnp.sqrt(_rbf(_rbf(var) + 1e-5)))
        rv = _rbf((tr + (mf - mb) * wsum) * inv)
        rmax = jnp.max(jnp.max(rv, axis=1, keepdims=True), axis=0, keepdims=True)
        pos = (lax.broadcasted_iota(i32, rv.shape, 0) * 128 + lax.broadcasted_iota(i32, rv.shape, 1))
        idx = jnp.min(jnp.where(rv == rmax, pos, S - 1))
        idx_s[0] = idx

        def pick(v):
            v = jnp.sum(jnp.where(pos == idx, v, 0.0), axis=1, keepdims=True)
            return jnp.sum(v, axis=0, keepdims=True)

        xv = x_buf[(idx >> 9) & 3, pl.ds(_mo(idx & (HQ - 16), 16), 16), :].astype(f32)
        sel = lax.broadcasted_iota(i32, xv.shape, 0) == (idx & 15)
        row = jnp.sum(jnp.where(sel, xv, 0.0), axis=0, keepdims=True)
        row = _rbf(_rbf(row - pick(mb)) * pick(inv))
        rsel[...] = jnp.broadcast_to(_rbf(jnp.sum(row * wrb[0:1, :], axis=1, keepdims=True)), rsel.shape)
        xb[...] = jnp.broadcast_to(row, (128, D)).T
        yield

    def ps_form(j):
        for c in range(HQ // 16):
            def put(k1, k2, v):
                k = k1 * 7 + k2
                ps[c * 8:(c + 1) * 8, k * 128:(k + 1) * 128] = v
            yield from form_steps(
                _lform, _wl_swapped,
                lambda r, q: pk_buf[j, q, c * 16:(c + 1) * 16, r * 128:(r + 1) * 128], put)

    def q_rows(j, r0, n, pq, rc, d0, rec):
        xj = pl.ds(_mo(j * (BQ // 2), BQ // 2), BQ // 2)
        pr = slice(r0 // 2, (r0 + n) // 2)
        blk = yield from strassen2(lambda k1, k2: _unpack(xs_at(L_ORD[k1], k2, xj)[pr, :]),
                                   lambda k1, k2: wqs[k1 * 7 + k2], NN, n, 1, QW)
        lane = lax.broadcasted_iota(i32, (n, 128), 1)
        for q in range(4):
            d = None
            for u in (3, 2, 1, 0):
                v = _phi(blk[q][u])
                for ct in range(2):
                    pq.at[q][d0:d0 + n, _st(u, ct)] = v[:, ct * 128:(ct + 1) * 128]
                t = v * zp[0:1, u * 256:(u + 1) * 256]
                t = t[:, :128] + t[:, 128:]
                d = t if d is None else d + t
            if rec:
                d = recip(d, lane)
            rc.at[q][d0:d0 + n, :] = d

    def recip(d, lane):
        d = d + jnp.where(lane % 2 == 0, pltpu.roll(d, 127, 1), pltpu.roll(d, 1, 1))
        d = d + jnp.where(lane % 4 < 2, pltpu.roll(d, 126, 1), pltpu.roll(d, 2, 1))
        return 1.0 / (d + 1e-6)

    def normalise(pq, rc, nr, dst, p0, raw, tok=None):
        lane = lax.broadcasted_iota(i32, (16, 128), 1)

        def fix(c):
            if c < nr // 16 and raw(c * 16):
                for q in range(4):
                    rq = slice(c * 16, (c + 1) * 16)
                    rc.at[q][rq, :] = recip(gate16(rc[q, rq, :]), lane)

        def scale(c):
            rq = slice(c * 16, (c + 1) * 16)
            fix(c + 1)
            for hf in range(2):
                for q in range(4):
                    cs = slice(hf * HD, (hf + 1) * HD)
                    pq.at[q][rq, cs] = pq[q, rq, cs] * jnp.concatenate([gate16(rc[q, rq, :])] * 4, axis=1)
                    yield

        def form(c):
            rq = slice(c * 16, (c + 1) * 16)
            p2 = pl.ds(_mo(p0 + c * 8, 8), 8)
            for ct in range(2):
                def put(k1, k2, v):
                    dst.at[k1 * 7 + k2][p2, ct * 128:(ct + 1) * 128] = v
                yield from form_steps(_lform, _wl, lambda q, u: pq[q, rq, _st(u, ct)], put, tok)

        fix(0)
        if raw(0):
            for _ in range(4):
                yield
        yield from scale(0)
        for c in range(nr // 16):
            nxt = scale(c + 1) if c + 1 < nr // 16 else iter(())
            for i, _ in enumerate(form(c)):
                yield
                if i < 8 and c + 1 < nr // 16:
                    next(nxt)
                    yield

    def g_kvm(j):
        blk = yield from strassen2(
            lambda k1, k2: _unpack(ps[:, (k1 * 7 + k2) * 128:(k1 * 7 + k2 + 1) * 128]),
            lambda k1, k2: xs_at(R_ORD[k1], W_R[k2])[...], TN, 256, 2, comb=_wc_swapped)
        hm = (lax.broadcasted_iota(i32, (128, 128), 0) // 32
              == lax.broadcasted_iota(i32, (128, 128), 1) // 32)
        qb = q_rows(j, BQ - QB, QB, pqb_buf.at[j], denb_buf.at[j], 0, False)
        for _ in range(QSPLIT):
            next(qb)
        kvps = []
        for a in (3, 2, 1, 0):
            gg = jnp.concatenate(blk[a], axis=1).astype(bf16)
            wv_u = pltpu.bitcast(wv_buf[j, :, a * 128:(a + 1) * 128], u32)
            kv = jnp.where(hm, mm(gg, wv_u, NN, 256), 0.0)
            tscr2.at[a][...] = _pack(kv)
            kvps.append(_unpack(jnp.concatenate(
                [tscr2[a, pl.ds(jj, 8, stride=8), :] for jj in range(8)], axis=0)))

        def m_form():
            for a in (3, 2, 1, 0):
                need(("mg", a))
                for jl in range(2):
                    for ct in range(2):
                        def put(k1, k2, v):
                            ms.at[k1 * 7 + k2][pl.ds(_mo(jl * 64 + (2 * a + j) * 8, 8), 8),
                                               ct * 128:(ct + 1) * 128] = v
                        yield from form_steps(
                            _rform, _wr, lambda q, u: mg_buf[a, (2 * q + jl) * 16:(2 * q + jl + 1) * 16, _st(u, ct)], put)

        for i, a in enumerate((3, 2, 1, 0)):
            wo_u = pltpu.bitcast(wo_buf[j, a * 128:(a + 1) * 128, :], u32)
            res = mm(kvps[i], wo_u, NN, 256)
            mg_buf.at[a][...] = _to_st(res)
            made.add(("mg", a))
            if i == 0:
                add_side(lambda tok: m_form(), 112, *MF)
        for _ in qb:
            pass

    def out_part(p0, nr, y, src, pr0):
        pr = pl.ds(_mo(pr0, 8), nr // 2)
        rows = [pl.ds(_mo(q * HQ + p0, 16), nr) for q in range(4)]
        row = lax.broadcasted_iota(i32, (nr, 256), 0) + p0
        blk = yield from strassen2(lambda k1, k2: _unpack(src[k1 * 7 + k2, pr, :]),
                                   lambda k1, k2: ms[k1 * 7 + k2], NN, nr)
        for s1 in (3, 2, 1, 0):
            for s2 in range(4):
                q = (s1 // 2) * 2 + s2 // 2
                u = (s1 % 2) * 2 + s2 % 2
                rr, cc = rows[q], pl.ds(u * 256, 256)
                a = jnp.concatenate([sa[rr, :]] * 2, axis=1)
                b = jnp.concatenate([sb[rr, :]] * 2, axis=1)
                o = blk[q][u] + jnp.where(row + q * HQ == idx_s[0], y[:, u * 256:(u + 1) * 256], 0.0)
                out_buf[rr, cc] = (x_buf[q, rows[0], cc].astype(f32) * a - b + o).astype(bf16)
                if s2 % 2 == 1:
                    ch = pl.ds((s1 % 2) * HD, HD)
                    cp(out_buf.at[rr, ch], out_hbm.at[0, rr, ch], SEM_O).start()

    def ffn_part(j):
        def fma(acc, w, v):
            p = w.astype(f32) * v
            return acc + p[0:8] + p[8:16]

        for f0 in range(0, FH, 256):
            fs = slice(f0, f0 + 256)
            ag = jnp.zeros((8, 256), f32)
            au = jnp.zeros((8, 256), f32)
            for k in range(0, D, 16):
                xv = jnp.concatenate([gate16(xb[k:k + 16, :])] * 2, axis=1)
                ag = fma(ag, wg_buf[j, k:k + 16, fs], xv)
                au = fma(au, wu_buf[j, k:k + 16, fs], xv)
                yield
            g = _rbf(jnp.sum(ag, axis=0, keepdims=True))
            u = _rbf(jnp.sum(au, axis=0, keepdims=True))
            h = _rbf(_rbf(g * jax.nn.sigmoid(g)) * u)
            hb_buf[fs, :] = jnp.broadcast_to(h, (128, 256)).T
        for d0 in range(0, D, 512):
            ds_ = slice(d0, d0 + 512)
            acc = yacc[:, ds_]
            for k in range(0, FH, 16):
                hv = jnp.concatenate([gate16(hb_buf[k:k + 16, :])] * 4, axis=1)
                acc = fma(acc, wd_buf[j, k:k + 16, ds_], hv)
                yield
            yacc[:, ds_] = acc

    def wait_group(i):
        with _scope("a_wait%d" % i):
            for c in a_groups[i]:
                c.wait()

    def run_all(gen):
        for _ in gen:
            pass

    def ln_sides(plan):
        for r0, r1, t0, t1 in plan[0]:
            add_side(lambda tok, r0=r0, r1=r1: ln_stats(r0, r1 - r0, tok), (r1 - r0) // 2, t0, t1, LNLAG)
        for r0, r1, t0, t1 in plan[1]:
            add_side(lambda tok, r0=r0, r1=r1: ln_later(r0, r1 - r0, tok), 22 * (r1 - r0) // 16, t0, t1, SLAG)

    def l2_side(base, n, t0, t1):
        add_side(lambda tok: ln_later(0, n, None, "l2", base), 22 * n // 16, t0, t1)

    with _scope("p0_issue"):
        cp_wr.start()
        for grp in a_groups:
            for c in grp:
                c.start()
        for j in range(2):
            for c in cp_b(j):
                c.start()
        zacc[...] = jnp.zeros(zacc.shape, f32)
        yacc[...] = jnp.zeros(yacc.shape, f32)
        zero_buf[1] = jnp.zeros((8, 128), u32)
        cp_zero = cp(zero_buf.at[1], zero_buf.at[0], SEM_Z)
        cp_zero.start()
        cp_zero.wait()
        cp_wr.wait()
        wr8 = jnp.broadcast_to(wr_buf[0:D].reshape(1, D).astype(f32), (8, D))
        wrb[0:8, :] = wr8
        wrb[8:16, :] = _to_st(wr8)
        z0 = jnp.max(pltpu.bitcast(zero_buf[0], i32))
        ps, pq_buf, den_buf, mg_buf, hb_buf = [r.at[z0] for r in (ps_raw, pq_raw, den_raw, mg_raw, hb_raw)]
        xn_buf = mg_buf

    def a01(i, carry):
        with _scope("a_wait01"):
            for c in cp_x(i * X0, X0, SEM_A + i):
                c.wait()
        with _scope("a01"):
            for r in range(0, X0, 16):
                run_all(ln_stats(r, 16, None, (i, X0)))
                if r:
                    run_all(ln_later(r - 16, 16, None, "l1", (i, X0)))
            run_all(ln_later(X0 - 16, 16, None, "l1", (i, X0)))
        return carry

    lax.fori_loop(0, NX, a01, 0)
    made.update(("xn", r) for r in range(0, 64, 16))

    def a23(i, carry):
        with _scope("a_wait23"):
            for c in cp_wk(i, SEM_W + i):
                c.wait()
        with _scope("a23"):
            wk_prep(i)
            l2_side((i, T0 // 2), T0 // 2, 250, 14 * T0 - 250)
            kproj(0, T0, [i])
            finish()
        return carry

    lax.fori_loop(0, 2, a23, 0)
    wait_group(NX + 2)
    with _scope("a4"):
        wk_prep(2)
        ln_sides(L4)
        kproj(0, T0, [2])
        finish()
    wait_group(NX + 3)
    with _scope("a5"):
        wk_prep(3)
        ln_sides(L5)
        kproj(0, T0, [3])
        for r0, n in A5K:
            kproj(r0, n)
        finish()
    wait_group(NX + 4)
    with _scope("a6"):
        ln_sides(L6)
        for r0, n in A6K:
            kproj(r0, n)
        finish()
    wait_group(NX + 5)
    with _scope("a7"):
        ln_sides(L7)
        add_side(lambda tok: wq_perm(), 128, *WQ_PERM)
        add_side(lambda tok: wq_form(), 224, *WQ_FORM)
        add_side(lambda tok: route(), 17, *ROUTE)
        for r0, n in A7K:
            kproj(r0, n)
        finish()

    def b_body(j, carry):
        qa = BQ - QB
        with _scope("b_r0"):
            z_prep()
            add_side(lambda tok: ps_form(j), 7 * HQ // 16, 0, 49 * qa - 400)
            for r0 in range(0, qa, QN):
                run_all(q_rows(j, r0, QN, pq_buf, den_buf, r0, r0 + QN < qa))
            finish()
        with _scope("b_wait"):
            for c in cp_b(j, wait_only=True):
                c.wait()
        with _scope("b_r1"):
            add_side(lambda tok: ffn_part(j), FH * 3 // 8, 0, R1T)
            add_side(lambda tok: normalise(pq_buf, den_buf, qa, qs, j * (qa // 2), lambda r: r >= qa - QN),
                     22 * (qa // 16), 0, R1T)
            run_all(g_kvm(j))
            finish()
        return carry

    lax.fori_loop(0, 2, b_body, 0)

    def c_body(t, carry):
        with _scope("c_body"):
            y = _rbf(jnp.sum(yacc[...], axis=0, keepdims=True))
            y = _rbf(y * _rbf(1.0 / _rbf(1.0 + _rbf(jnp.exp(-rsel[0:1, :])))))
            j, h = t >> 1, t & 1
            na, nb = (BQ - QB) // 2, QB // 2
            hb = pl.ds(_mo(h * nb, 16), nb)
            add_side(lambda tok: normalise(pqb_buf.at[j, :, hb, :], denb_buf.at[j, :, hb, :], nb, qsb, 0,
                                           lambda r: True, tok),
                     4 + 22 * (nb // 16), 0, 49 * na - 800, SLAG)
            for p in range(0, na, CR):
                p0 = j * BQ + h * na + p
                run_all(out_part(p0, CR, y, qs, t * (na // 2) + p // 2))
            flush()
            run_all(out_part(j * BQ + BQ - QB + h * nb, nb, y, qsb, 0))
            finish()
        return carry

    lax.fori_loop(0, 4, c_body, 0)
    with _scope("tail"):
        cp(out_buf, out_hbm.at[0], SEM_O).wait()


@jax.jit
def pallas_parallel_sum__linear_attn_block__moe_arch_mod__prompt_kernel(
    A_x: jax.Array,
    A_wqkv: jax.Array,
    A_wo: jax.Array,
    B_x: jax.Array,
    B_w_r: jax.Array,
    B_w_gate: jax.Array,
    B_w_up: jax.Array,
    B_w_down: jax.Array,
):
    del B_x
    V = pltpu.VMEM
    scratch = [
        V((4, HQ, D), bf16),
        V((2, D, 512), bf16),
        V((2, 512, D), bf16),
        V((8 * D,), bf16),
        V((2, D, FH), bf16),
        V((2, D, FH), bf16),
        V((2, FH, D), bf16),
        V((28, HQ // 2, 256), u32),
        V((28, HQ // 2, 256), u32),
        V((49, 128, 256), u32),
        V((S, 128), f32),
        V((S, 128), f32),
        V((8, D), f32),
        V((8, D), f32),
        V((2, 4, HQ, 512), f32),
        V((D, 128), f32),
        V((8, D), f32),
        V((8, D), f32),
        V((16, D), f32),
        V((4, 8, 128), u32),
        V((4, HD // 2, 7 * 128), u32),
        V((S, 256), f32),
        V((64, 64, 128), u32),
        V((1, HQ // 2, 49 * 128), u32),
        V((49, BQ - QB, 256), u32),
        V((49, 128, 256), u32),
        V((8, 64, 128), u32),
        V((4, 64, 128), u32),
        V((1, 4, BQ - QB, D), f32),
        V((1, 4, BQ - QB, 128), f32),
        V((2, 4, QB, D), f32),
        V((2, 4, QB, 128), f32),
        V((49, QB // 4, 256), u32),
        V((1, 4, 128, D), f32),
        V((1, FH, 128), f32),
        V((S, D), bf16),
        pltpu.SMEM((1,), i32),
        pltpu.SemaphoreType.DMA((4 + T0 // X0 + 6,)),
    ]
    extra = {k: True for k in ("disable_bounds_checks", "disable_semaphore_checks")
             if hasattr(pltpu.CompilerParams, k)}
    return pl.pallas_call(
        _kernel,
        out_shape=jax.ShapeDtypeStruct((1, S, D), bf16),
        in_specs=[pl.BlockSpec(memory_space=pl.ANY)] * 7,
        out_specs=pl.BlockSpec(memory_space=pl.ANY),
        scratch_shapes=scratch,
        compiler_params=pltpu.CompilerParams(vmem_limit_bytes=120 * 1024 * 1024, **extra),
    )(A_x.reshape(4, HQ, D), A_wqkv, A_wo, B_w_r, B_w_gate, B_w_up, B_w_down)
```

```python
import contextlib

import jax
import jax.numpy as jnp
from jax import lax
import jax.experimental.pallas as pl
import jax.experimental.pallas.tpu as pltpu

bf16, f32, u32, i32 = jnp.bfloat16, jnp.float32, jnp.uint32, jnp.int32

S = 2048
D = 1024
F = 3584
HD = D // 2
HQ = S // 4
BQ = HQ // 2
FH = F // 2
QB = 64
QN = 48
QSPLIT = 6
CR = 32
T0 = 96
X0 = 32
XG = (160, 208)
XN = 128

SLAG = 400
LNLAG = 700
QW = (28, 36, 36, 6, 2, 2, 2)
L4 = ([(96, 144, 0, 1100)], [])
L5 = ([(144, 208, 1100, 3500)], [(96, 128, 0, 1150), (128, 144, 1250, 2000), (144, 208, 2300, 4700)])
L6 = ([(208, 512, 0, 10000)], [(208, 256, 800, 2600), (256, 448, 2700, 10500)])
L7 = ([], [(448, 512, 0, 3000)])
A5K = ((96, 32), (128, 32))
A6K = ((160, 48), (208, 48), (256, 48), (304, 48))
A7K = ((352, 48), (400, 48), (448, 64))
WQ_PERM, WQ_FORM, ROUTE = (0, 3200), (3300, 8600), (4500, 5300)
R1T = 12800
MF = (128, 3420)

L_ORD = (2, 3, 0, 1, 4, 5, 6)
R_ORD = (2, 0, 6, 5, 1, 4, 3)

K_SEQ = (1, 4, 0, 2, 3, 5, 6)
K_SEQ2 = (0, 1, 2, 5, 3, 4, 6)
W_SEQ = (0, 1, 5, 6, 4, 2, 3)

NN = (((1,), (0,)), ((), ()))
TN = (((0,), (0,)), ((), ()))


SCOPES = False


def _scope(name):
    return jax.named_scope(name) if SCOPES else contextlib.nullcontext()


def _mo(v, m):
    return v if isinstance(v, int) else pl.multiple_of(v, m)


def _dot(a, b, dims):
    return lax.dot_general(a, b, dims, preferred_element_type=f32)


def _pack(v):
    return pltpu.bitcast(v.astype(bf16), u32)


def _unpack(v):
    return pltpu.bitcast(v, bf16)


def _combine(m):
    m1, m2, m3, m4, m5, m6, m7 = m
    return m1 + m4 - m5 + m7, m3 + m5, m2 + m4, m1 - m2 + m3 + m6


def _lform(a11, a12, a21, a22):
    return (a11 + a22, a21 + a22, a11, a22, a11 + a12, a21 - a11, a12 - a22)


def _rform(b11, b12, b21, b22):
    return (b11 + b22, b11, b12 - b22, b21 - b11, b22, b11 + b12, b21 + b22)


def _sform(x11, x12, x21, x22):
    return (x11, x22, x11 + x22, x21 + x22, x11 + x12, x21 - x11, x12 - x22)


def _wl(a11, a12, a21, a22):
    s1 = a21 + a22
    s2 = s1 - a11
    return (a11, a12, a12 - s2, a22, s1, s2, a11 - a21)


def _wr(b11, b12, b21, b22):
    t1 = b12 - b11
    t2 = b22 - t1
    return (b11, b21, b22, t2 - b21, t1, t2, b22 - b12)


def _wc(p):
    p1, p2, p3, p4, p5, p6, p7 = p
    u2 = p1 + p6
    u3 = u2 + p7
    return p1 + p2, (u2 + p5) + p3, u3 - p4, u3 + p5


W_R = (3, 1, 0, 2, 4, 5, 6)


def _wl_swapped(a11, a12, a21, a22):
    return _wl(a12, a11, a22, a21)


def _wc_swapped(p):
    p1, p2, p3, p4, p5, p6, p7 = p
    v2 = p1 + p6
    u3 = p7 - v2
    return (p5 - v2) + p3, p1 + p2, u3 + p5, p4 - u3


class _Sym:
    def __init__(self, t):
        self.t = t

    def __add__(self, o):
        return _Sym({**self.t, **o.t})

    def __sub__(self, o):
        return _Sym({**self.t, **{k: -v for k, v in o.t.items()}})


def _st(u, ct):
    return slice((4 * ct + u) * 128, (4 * ct + u + 1) * 128)


def _to_st(v):
    return jnp.concatenate([v[:, (2 * u + ct) * 128:(2 * u + ct + 1) * 128]
                            for ct in range(2) for u in range(4)], axis=1)


def _phi(t):
    return jnp.where(t > 0, t + 1.0, jnp.exp(t)) + 1e-6


def _rbf(v):
    return v.astype(bf16).astype(f32)


def _kernel(x_hbm, wqkv_hbm, wo_hbm, wr_hbm, wg_hbm, wu_hbm, wd_hbm, out_hbm,
            x_buf, wv_buf, wo_buf, wr_buf, wg_buf, wu_buf, wd_buf,
            xs1, xs2, wqs, sa, sb, zacc, zp, pk_buf, xb, yacc, rsel, wrb, zero_buf,
            wks, stats, wqt, ps_raw, qs, ms, tscr, tscr2, pq_raw, den_raw, pqb_buf, denb_buf, qsb,
            mg_raw, hb_raw, out_buf, idx_s, sem):
    wq_buf = out_buf.at[pl.ds(0, D), :]
    wk_buf = out_buf.at[pl.ds(D, D), :]

    def xs_at(k1, e, rows=None):
        r = xs1.at[k1 * 4 + (0, 1, 7, 3).index(e)] if e in (0, 1, 7, 3) else xs2.at[k1 * 4 + (2, 4, 5, 6).index(e)]
        return r if rows is None else r.at[rows, :]

    SEM_B, SEM_O, SEM_Z, SEM_A = 0, 2, 3, 4

    def cp(src, dst, s):
        return pltpu.make_async_copy(src, dst, sem.at[s])

    def cp_x(r0, n, s):
        r = pl.ds(_mo(r0, 16), n)
        return [cp(x_hbm.at[:, r, :], x_buf.at[:, r, :], s)]

    def cp_wk(c, s):
        return [cp(wqkv_hbm.at[:, pl.ds(_mo(D + c * 256, 256), 256)],
                   wk_buf.at[:, pl.ds(_mo(c * 256, 256), 256)], s)]

    NX = T0 // X0
    SEM_W = SEM_A + NX
    cp_wr = cp(wr_hbm, wr_buf.at[pl.ds(0, D)], SEM_Z)
    a_groups = [cp_x(i * X0, X0, SEM_A + i) for i in range(NX)] + [
        cp_wk(0, SEM_W),
        cp_wk(1, SEM_W + 1),
        cp_wk(2, SEM_W + 2) + cp_x(T0, XG[0] - T0, SEM_W + 2),
        cp_wk(3, SEM_W + 3) + cp_x(XG[0], XG[1] - XG[0], SEM_W + 3),
        cp_x(XG[1], HQ - XG[1], SEM_W + 4),
        [cp(wqkv_hbm.at[:, pl.ds(0, D)], wq_buf, SEM_W + 5)],
    ]

    def cp_b(j, wait_only=False):
        dsts = [wg_buf.at[j], wu_buf.at[j], wd_buf.at[j]]
        for a in range(4):
            dsts += [wv_buf.at[j, :, pl.ds(a * 128, 128)], wo_buf.at[j, pl.ds(a * 128, 128), :]]
        if wait_only:
            return [cp(dst, dst, SEM_B + j) for dst in dsts]
        fs = pl.ds(j * FH, FH)
        srcs = [wg_hbm.at[:, fs], wu_hbm.at[:, fs], wd_hbm.at[fs, :]]
        for a in range(4):
            c0 = (2 * a + j) * 128
            srcs += [wqkv_hbm.at[:, pl.ds(2 * D + c0, 128)], wo_hbm.at[pl.ds(c0, 128), :]]
        return [cp(src, dst, SEM_B + j) for src, dst in zip(srcs, dsts)]

    clock = [0]
    toks = []
    sides = []
    fwd = [None]

    def emit_tok(vals, stamp):
        t = None
        for v in vals:
            v = pltpu.bitcast(v, u32) if v.dtype != u32 else v
            t = v if t is None else t | v
        toks.append((stamp, t & zero_buf[0]))

    def token(kind):
        t = fwd[0]
        if "u" not in t:
            t["u"] = pltpu.bitcast(t["src"](), u32) & zero_buf[0]
        if kind != "u" and "f" not in t:
            t["f"] = pltpu.bitcast(t["u"], f32)
        if kind == "f16" and "f16" not in t:
            t["f16"] = jnp.concatenate([t["f"], t["f"]], axis=0)
        return t[kind]

    def gate(v):
        if fwd[0] is None:
            return v
        head = v if v.shape[0] == 8 else v[0:8]
        head = head | token("u") if v.dtype == u32 else head + token("f")
        return head if v.shape[0] == 8 else jnp.concatenate([head, v[8:]], axis=0)

    def gate16(v):
        return v if fwd[0] is None else v + token("f16")

    def add_side(gen_fn, n, t0, t1, lag=None):
        st = {"i": 0, "n": n, "t0": clock[0] + t0, "t1": clock[0] + t1}

        def tok(vals):
            if lag is not None:
                emit_tok(vals, st["t0"] + (st["i"] + 1) * (st["t1"] - st["t0"]) // st["n"] + lag)
        st["g"] = gen_fn(tok)
        sides.append(st)

    def advance(until):
        for st in sides:
            while st["i"] < st["n"] and st["t0"] + st["i"] * (st["t1"] - st["t0"]) // st["n"] < until:
                next(st["g"], None)
                st["i"] += 1
                if st["i"] == st["n"]:
                    for _ in st["g"]:
                        pass

    def flush():
        for st in sides:
            for _ in st["g"]:
                pass
        sides.clear()

    def finish():
        flush()
        toks.clear()
        fwd[0] = None

    def mm(lhs, rhs, dims, cycles, nseg=1):
        due = [t for (c, t) in toks if c <= clock[0]]
        toks[:] = [(c, t) for (c, t) in toks if c > clock[0]]
        if due:
            head = rhs[0:8, 0:128]
            for t in due:
                head = head | t
            if rhs.shape[1] > 128:
                head = jnp.concatenate([head, rhs[0:8, 128:]], axis=1)
            rhs = jnp.concatenate([head, rhs[8:]], axis=0)
        res = _dot(lhs, _unpack(rhs), dims)
        ngr = res.shape[0] // 16
        for sg in range(nseg):
            for i in range(ngr):
                fwd[0] = {"src": lambda sg=sg, i=i: res[i * 16:i * 16 + 8, sg * 128:(sg + 1) * 128]}
                clock[0] += cycles // nseg // ngr
                advance(clock[0])
        return res

    def form_steps(form, form2, get, put, tok=None, keep=range(7)):
        terms = form(*[_Sym({i: 1}) for i in range(4)])
        gated = (0, 1, 2, 3) if 7 in keep else {_wl: (0, 1, 3), _wr: (0, 2, 3), _wl_swapped: (1, 2)}[form2]
        for k1 in range(7):
            sub = []
            for r in range(2):
                for c in range(2):
                    v = None
                    for i, sg in sorted(terms[k1].t.items(), key=lambda e: -e[1]):
                        b = get(r + 2 * (i // 2), c + 2 * (i % 2))
                        if v is None:
                            v = gate16(b) if 2 * r + c in gated else b
                        else:
                            v = v + b if sg > 0 else v - b
                    sub.append(v)
            vals = form2(*sub) + (sub[2],)
            for k2 in keep:
                put(k1, k2, _pack(vals[k2]))
            if tok is not None and k1 % 2 == 0:
                full = vals[3 if form2 is _wr else 2]
                tok([full[0:8], full[8:16]])
            yield

    def strassen2(lhs, rhs, dims, cycles, nseg=1, wts=(16,) * 7, comb=_wc):
        m1 = [None] * 7
        for i1, k1 in enumerate(K_SEQ2):
            m2 = [None] * 7
            for k2 in W_SEQ:
                m2[k2] = mm(lhs(k1, k2), rhs(k1, k2), dims, cycles * wts[i1] // 16, nseg)
                yield
            m1[k1] = comb(m2)
        out = [[None] * 4 for _ in range(4)]
        for s2 in range(4):
            for s1, v in enumerate(_combine([m1[k1][s2] for k1 in range(7)])):
                out[(s1 // 2) * 2 + s2 // 2][(s1 % 2) * 2 + s2 % 2] = v
        return out

    made = set()

    def need(*keys):
        assert all(k in made for k in keys), keys

    def row_views(base):
        if base == 0:
            return x_buf, sa, sb, stats, xn_buf, None
        i, n = base
        b = _mo(i * n, 16)
        return ([x_buf.at[:, pl.ds(b, n), :]] + [r.at[pl.ds(b, S - 128 + n), :] for r in (sa, sb, stats)]
                + [xn_buf.at[:, pl.ds(b, n), :], pl.ds(_mo(i * (n // 2), 8), n // 2)])

    def xs_form(r0, tok, which="all", base=0):
        xn_v, xs_v = row_views(base)[4:]
        rows = slice(r0 % XN, r0 % XN + 16)

        keep = {"all": range(8), "l1": (0, 1, 7, 3), "l2": (2, 4, 5, 6)}[which]
        for ct in range(2):
            def put(k1, k2, v):
                xs_at(k1, k2, xs_v)[r0 // 2:r0 // 2 + 8, ct * 128:(ct + 1) * 128] = v
            yield from form_steps(
                _sform, _wl, lambda q, u: xn_v[q, rows, _st(u, ct)], put, tok, keep)
        made.add(("xs", r0))

    def ln_stats(r_start, n_rows, tok, base=0):
        x_v, sa_v, sb_v, st_v, xn_v, _ = row_views(base)
        lane = lax.broadcasted_iota(i32, (8, 128), 1)
        for r0 in range(r_start, r_start + n_rows, 16):
            if r0 >= T0:
                need(("in", 2 + sum(r0 >= g for g in XG)))
            if r0 - XN >= T0:
                need(("ln", r0 - XN))
            for g in range(8):
                q, o = g // 2, (g % 2) * 8
                rg = q * HQ + r0 + o
                xv = x_v[q, r0 + o:r0 + o + 8, :].astype(f32)
                xg = jnp.concatenate([gate(xv[:, 0:128]), xv[:, 128:]], axis=1)
                mf = jnp.sum(xg, axis=1, keepdims=True) * (1.0 / D)
                d = xv - mf
                var = jnp.sum(d * d, axis=1, keepdims=True) * (1.0 / D)
                rs = lax.rsqrt(var + 1e-5)
                xn_v.at[q][r0 % XN + o:r0 % XN + o + 8, :] = _to_st(d * rs)
                rs = jnp.broadcast_to(rs, (8, 128))
                mf = jnp.broadcast_to(mf, (8, 128))
                sa_v[rg:rg + 8, :] = 1.0 + rs
                sb_v[rg:rg + 8, :] = mf * rs
                st_v[rg:rg + 8, 0:128] = jnp.where(lane == 0, mf, jnp.broadcast_to(var, (8, 128)))
                if tok is not None:
                    tok([rs])
                if g == 7:
                    made.add(("xn", r0))
                yield

    def ln_later(r_start, n_rows, tok, which="all", base=0):
        st_v, xn_v = row_views(base)[3:5]
        for r0 in range(r_start, r_start + n_rows, 16):
            need(("xn", r0))
            form = xs_form(r0, tok, which, base)
            for g in range(8):
                for _ in range(2 if g < 7 else 0):
                    next(form)
                    yield
                q, o = g // 2, (g % 2) * 8
                t = None
                if which != "l1":
                    v = xn_v[q, r0 % XN + o:r0 % XN + o + 8, :] * wrb[8:16, :]
                    for ct in range(8):
                        h = v[:, ct * 128:(ct + 1) * 128]
                        t = gate(h) if t is None else t + h
                if t is not None:
                    st_v[q * HQ + r0 + o:q * HQ + r0 + o + 8, 128:256] = t
                if tok is not None:
                    tok([t])
                if g == 7:
                    next(form, None)
                    made.add(("ln", r0))
                yield

    def wk_prep(c):
        if isinstance(c, int):
            need(("in", c))
        cs = pl.ds(_mo(c * 256, 256), 256)
        for i in range(HD // 16):
            r0 = i * 16
            top = wk_buf[r0:r0 + 16, cs].astype(f32)
            bot = wk_buf[HD + r0:HD + r0 + 16, cs].astype(f32)
            ops = _rform(top[:, :128], top[:, 128:], bot[:, :128], bot[:, 128:])
            for k in range(7):
                wks.at[c][r0 // 2:r0 // 2 + 8, k * 128:(k + 1) * 128] = _pack(ops[k])

    def wq_perm():
        need(("in", 5))

        def permute(kt):
            for g in range(8):
                tile = gate(pltpu.bitcast(wq_buf[kt * 128:(kt + 1) * 128, g * 128:(g + 1) * 128], u32))
                wqt.at[kt * 8 + g][...] = pltpu.bitcast(_unpack(tile).T, u32)
                yield

        def back(kt):
            for j in range(8):
                tile = gate(jnp.concatenate([wqt[kt * 8 + g, pl.ds(j, 8, stride=8), :] for g in range(8)],
                                            axis=0))
                v = pltpu.bitcast(_unpack(tile).T.astype(f32), u32)
                c0 = (kt // 2) * D + _st(j // 2, j % 2).start
                ps[(kt % 2) * 128:(kt % 2 + 1) * 128, c0:c0 + 128] = v
                made.add(("wqp", kt, j))
                yield

        order = (0, 2, 4, 6, 1, 3, 5, 7)
        for n in range(10):
            if n < 8:
                yield from permute(order[n])
            if n > 1:
                yield from back(order[n - 2])

    def wq_form():
        for i in range(16):
            need(*[("wqp", 2 * r + i // 8, j) for r in range(4) for j in range(8)])
            for ct in range(2):
                def put(k1, k2, v):
                    wqs.at[k1 * 7 + k2][i * 8:(i + 1) * 8, ct * 128:(ct + 1) * 128] = v
                yield from form_steps(
                    _rform, _wr, lambda r, c: pltpu.bitcast(
                        ps[i * 16:(i + 1) * 16, r * D + _st(c, ct).start:r * D + _st(c, ct).stop],
                        f32), put)

    def kproj(r0, n, chunks=range(4)):
        pr = pl.ds(r0 // 2, n // 2)
        need(*[("xs", r) for r in range(max(r0, T0), r0 + n, 16)])
        for c in chunks:
            m = [None] * 7
            for k in K_SEQ:
                e11, e12, e21, e22 = [xs_at(L_ORD[k], e)[pr, :] for e in (0, 1, 7, 3)]
                lhs = jnp.concatenate([jnp.concatenate([e11, e12], axis=1),
                                       jnp.concatenate([e21, e22], axis=1)], axis=0)
                m[k] = mm(_unpack(lhs), wks[c, :, k * 128:(k + 1) * 128], NN, 2 * n)
            kk = [_phi(v) for v in _combine(m)]
            for ct in range(2):
                zacc[:, pl.ds(_mo(c * 256 + ct * 128, 128), 128)] += (
                    (kk[ct] + kk[2 + ct]).reshape(n // 4, 8, 128).sum(axis=0))
            for s1 in range(4):
                for h in range(2):
                    pk_buf.at[s1 % 2, (s1 // 2) * 2 + h][r0:r0 + n, pl.ds(_mo(c * 128, 128), 128)] = (
                        kk[s1][h * n:(h + 1) * n])

    def z_prep():
        z = jnp.sum(zacc[...], axis=0, keepdims=True)
        zt = _pack(jnp.broadcast_to(z, (128, D)).astype(bf16).T)
        for g in range(8):
            tscr.at[g][...] = zt[g * 64:(g + 1) * 64, :]
        for j in range(8):
            blk = jnp.concatenate([tscr[g, pl.ds(j, 8, stride=8), :] for g in range(8)], axis=0)
            zp[:, j * 128:(j + 1) * 128] = _unpack(blk).T[0:8, :].astype(f32)

    def route():
        rows, dots = [None] * 16, [None] * 16
        for b in sorted(range(S // 128), key=lambda b: b % 4):
            need(*[("ln", r) for r in range(max(T0, b % 4 * 128), b % 4 * 128 + 128, 16)])
            rows[b] = gate(stats[b * 128:(b + 1) * 128, 0:128]).T[0:8, :]
            dots[b] = jnp.sum(gate(stats[b * 128:(b + 1) * 128, 128:256]).T, axis=0, keepdims=True)
            yield
        mf = jnp.concatenate([v[0:1] for v in rows], axis=0)
        var = jnp.concatenate([v[1:2] for v in rows], axis=0)
        tr = jnp.concatenate(dots, axis=0) * jnp.sqrt(var + 1e-5)
        wsum = jnp.sum(wrb[0:1, :], axis=1, keepdims=True)
        mb = _rbf(mf)
        inv = 1.0 / _rbf(jnp.sqrt(_rbf(_rbf(var) + 1e-5)))
        rv = _rbf((tr + (mf - mb) * wsum) * inv)
        rmax = jnp.max(jnp.max(rv, axis=1, keepdims=True), axis=0, keepdims=True)
        pos = (lax.broadcasted_iota(i32, rv.shape, 0) * 128 + lax.broadcasted_iota(i32, rv.shape, 1))
        idx = jnp.min(jnp.where(rv == rmax, pos, S - 1))
        idx_s[0] = idx

        def pick(v):
            v = jnp.sum(jnp.where(pos == idx, v, 0.0), axis=1, keepdims=True)
            return jnp.sum(v, axis=0, keepdims=True)

        xv = x_buf[(idx >> 9) & 3, pl.ds(_mo(idx & (HQ - 16), 16), 16), :].astype(f32)
        sel = lax.broadcasted_iota(i32, xv.shape, 0) == (idx & 15)
        row = jnp.sum(jnp.where(sel, xv, 0.0), axis=0, keepdims=True)
        row = _rbf(_rbf(row - pick(mb)) * pick(inv))
        rsel[...] = jnp.broadcast_to(_rbf(jnp.sum(row * wrb[0:1, :], axis=1, keepdims=True)), rsel.shape)
        xb[...] = jnp.broadcast_to(row, (128, D)).T
        yield

    def ps_form(j):
        for c in range(HQ // 16):
            def put(k1, k2, v):
                k = k1 * 7 + k2
                ps[c * 8:(c + 1) * 8, k * 128:(k + 1) * 128] = v
            yield from form_steps(
                _lform, _wl_swapped,
                lambda r, q: pk_buf[j, q, c * 16:(c + 1) * 16, r * 128:(r + 1) * 128], put)

    def q_rows(j, r0, n, pq, rc, d0, rec):
        xj = pl.ds(_mo(j * (BQ // 2), BQ // 2), BQ // 2)
        pr = slice(r0 // 2, (r0 + n) // 2)
        blk = yield from strassen2(lambda k1, k2: _unpack(xs_at(L_ORD[k1], k2, xj)[pr, :]),
                                   lambda k1, k2: wqs[k1 * 7 + k2], NN, n, 1, QW)
        lane = lax.broadcasted_iota(i32, (n, 128), 1)
        for q in range(4):
            d = None
            for u in (3, 2, 1, 0):
                v = _phi(blk[q][u])
                for ct in range(2):
                    pq.at[q][d0:d0 + n, _st(u, ct)] = v[:, ct * 128:(ct + 1) * 128]
                t = v * zp[0:1, u * 256:(u + 1) * 256]
                t = t[:, :128] + t[:, 128:]
                d = t if d is None else d + t
            if rec:
                d = recip(d, lane)
            rc.at[q][d0:d0 + n, :] = d

    def recip(d, lane):
        d = d + jnp.where(lane % 2 == 0, pltpu.roll(d, 127, 1), pltpu.roll(d, 1, 1))
        d = d + jnp.where(lane % 4 < 2, pltpu.roll(d, 126, 1), pltpu.roll(d, 2, 1))
        return 1.0 / (d + 1e-6)

    def normalise(pq, rc, nr, dst, p0, raw, tok=None):
        lane = lax.broadcasted_iota(i32, (16, 128), 1)

        def fix(c):
            if c < nr // 16 and raw(c * 16):
                for q in range(4):
                    rq = slice(c * 16, (c + 1) * 16)
                    rc.at[q][rq, :] = recip(gate16(rc[q, rq, :]), lane)

        def scale(c):
            rq = slice(c * 16, (c + 1) * 16)
            fix(c + 1)
            for hf in range(2):
                for q in range(4):
                    cs = slice(hf * HD, (hf + 1) * HD)
                    pq.at[q][rq, cs] = pq[q, rq, cs] * jnp.concatenate([gate16(rc[q, rq, :])] * 4, axis=1)
                    yield

        def form(c):
            rq = slice(c * 16, (c + 1) * 16)
            p2 = pl.ds(_mo(p0 + c * 8, 8), 8)
            for ct in range(2):
                def put(k1, k2, v):
                    dst.at[k1 * 7 + k2][p2, ct * 128:(ct + 1) * 128] = v
                yield from form_steps(_lform, _wl, lambda q, u: pq[q, rq, _st(u, ct)], put, tok)

        fix(0)
        if raw(0):
            for _ in range(4):
                yield
        yield from scale(0)
        for c in range(nr // 16):
            nxt = scale(c + 1) if c + 1 < nr // 16 else iter(())
            for i, _ in enumerate(form(c)):
                yield
                if i < 8 and c + 1 < nr // 16:
                    next(nxt)
                    yield

    def g_kvm(j):
        blk = yield from strassen2(
            lambda k1, k2: _unpack(ps[:, (k1 * 7 + k2) * 128:(k1 * 7 + k2 + 1) * 128]),
            lambda k1, k2: xs_at(R_ORD[k1], W_R[k2])[...], TN, 256, 2, comb=_wc_swapped)
        hm = (lax.broadcasted_iota(i32, (128, 128), 0) // 32
              == lax.broadcasted_iota(i32, (128, 128), 1) // 32)
        qb = q_rows(j, BQ - QB, QB, pqb_buf.at[j], denb_buf.at[j], 0, False)
        for _ in range(QSPLIT):
            next(qb)
        kvps = []
        for a in (3, 2, 1, 0):
            gg = jnp.concatenate(blk[a], axis=1).astype(bf16)
            wv_u = pltpu.bitcast(wv_buf[j, :, a * 128:(a + 1) * 128], u32)
            kv = jnp.where(hm, mm(gg, wv_u, NN, 256), 0.0)
            tscr2.at[a][...] = _pack(kv)
            kvps.append(_unpack(jnp.concatenate(
                [tscr2[a, pl.ds(jj, 8, stride=8), :] for jj in range(8)], axis=0)))

        def m_form():
            for a in (3, 2, 1, 0):
                need(("mg", a))
                for jl in range(2):
                    for ct in range(2):
                        def put(k1, k2, v):
                            ms.at[k1 * 7 + k2][pl.ds(_mo(jl * 64 + (2 * a + j) * 8, 8), 8),
                                               ct * 128:(ct + 1) * 128] = v
                        yield from form_steps(
                            _rform, _wr, lambda q, u: mg_buf[a, (2 * q + jl) * 16:(2 * q + jl + 1) * 16, _st(u, ct)], put)

        for i, a in enumerate((3, 2, 1, 0)):
            wo_u = pltpu.bitcast(wo_buf[j, a * 128:(a + 1) * 128, :], u32)
            res = mm(kvps[i], wo_u, NN, 256)
            mg_buf.at[a][...] = _to_st(res)
            made.add(("mg", a))
            if i == 0:
                add_side(lambda tok: m_form(), 112, *MF)
        for _ in qb:
            pass

    def out_part(p0, nr, y, src, pr0):
        pr = pl.ds(_mo(pr0, 8), nr // 2)
        rows = [pl.ds(_mo(q * HQ + p0, 16), nr) for q in range(4)]
        row = lax.broadcasted_iota(i32, (nr, 256), 0) + p0
        blk = yield from strassen2(lambda k1, k2: _unpack(src[k1 * 7 + k2, pr, :]),
                                   lambda k1, k2: ms[k1 * 7 + k2], NN, nr)
        for s1 in (3, 2, 1, 0):
            for s2 in range(4):
                q = (s1 // 2) * 2 + s2 // 2
                u = (s1 % 2) * 2 + s2 % 2
                rr, cc = rows[q], pl.ds(u * 256, 256)
                a = jnp.concatenate([sa[rr, :]] * 2, axis=1)
                b = jnp.concatenate([sb[rr, :]] * 2, axis=1)
                o = blk[q][u] + jnp.where(row + q * HQ == idx_s[0], y[:, u * 256:(u + 1) * 256], 0.0)
                out_buf[rr, cc] = (x_buf[q, rows[0], cc].astype(f32) * a - b + o).astype(bf16)
                if s2 % 2 == 1:
                    ch = pl.ds((s1 % 2) * HD, HD)
                    cp(out_buf.at[rr, ch], out_hbm.at[0, rr, ch], SEM_O).start()

    def ffn_part(j):
        def fma(acc, w, v):
            p = w.astype(f32) * v
            return acc + p[0:8] + p[8:16]

        for f0 in range(0, FH, 256):
            fs = slice(f0, f0 + 256)
            ag = jnp.zeros((8, 256), f32)
            au = jnp.zeros((8, 256), f32)
            for k in range(0, D, 16):
                xv = jnp.concatenate([gate16(xb[k:k + 16, :])] * 2, axis=1)
                ag = fma(ag, wg_buf[j, k:k + 16, fs], xv)
                au = fma(au, wu_buf[j, k:k + 16, fs], xv)
                yield
            g = _rbf(jnp.sum(ag, axis=0, keepdims=True))
            u = _rbf(jnp.sum(au, axis=0, keepdims=True))
            h = _rbf(_rbf(g * jax.nn.sigmoid(g)) * u)
            hb_buf[fs, :] = jnp.broadcast_to(h, (128, 256)).T
        for d0 in range(0, D, 512):
            ds_ = slice(d0, d0 + 512)
            acc = yacc[:, ds_]
            for k in range(0, FH, 16):
                hv = jnp.concatenate([gate16(hb_buf[k:k + 16, :])] * 4, axis=1)
                acc = fma(acc, wd_buf[j, k:k + 16, ds_], hv)
                yield
            yacc[:, ds_] = acc

    def wait_group(i):
        with _scope("a_wait%d" % i):
            for c in a_groups[i]:
                c.wait()
        made.add(("in", i - NX))

    def run_all(gen):
        for _ in gen:
            pass

    def ln_sides(plan):
        for r0, r1, t0, t1 in plan[0]:
            add_side(lambda tok, r0=r0, r1=r1: ln_stats(r0, r1 - r0, tok), (r1 - r0) // 2, t0, t1, LNLAG)
        for r0, r1, t0, t1 in plan[1]:
            add_side(lambda tok, r0=r0, r1=r1: ln_later(r0, r1 - r0, tok), 22 * (r1 - r0) // 16, t0, t1, SLAG)

    def l2_side(base, n, t0, t1):
        add_side(lambda tok: ln_later(0, n, None, "l2", base), 22 * n // 16, t0, t1)

    with _scope("p0_issue"):
        cp_wr.start()
        for grp in a_groups:
            for c in grp:
                c.start()
        for j in range(2):
            for c in cp_b(j):
                c.start()
        zacc[...] = jnp.zeros(zacc.shape, f32)
        yacc[...] = jnp.zeros(yacc.shape, f32)
        zero_buf[1] = jnp.zeros((8, 128), u32)
        cp_zero = cp(zero_buf.at[1], zero_buf.at[0], SEM_Z)
        cp_zero.start()
        cp_zero.wait()
        cp_wr.wait()
        wr8 = jnp.broadcast_to(wr_buf[0:D].reshape(1, D).astype(f32), (8, D))
        wrb[0:8, :] = wr8
        wrb[8:16, :] = _to_st(wr8)
        z0 = jnp.max(pltpu.bitcast(zero_buf[0], i32))
        ps, pq_buf, den_buf, mg_buf, hb_buf = [r.at[z0] for r in (ps_raw, pq_raw, den_raw, mg_raw, hb_raw)]
        xn_buf = mg_buf

    def a01(i, carry):
        with _scope("a_wait01"):
            for c in cp_x(i * X0, X0, SEM_A + i):
                c.wait()
        with _scope("a01"):
            for r in range(0, X0, 16):
                run_all(ln_stats(r, 16, None, (i, X0)))
                if r:
                    run_all(ln_later(r - 16, 16, None, "l1", (i, X0)))
            run_all(ln_later(X0 - 16, 16, None, "l1", (i, X0)))
        return carry

    lax.fori_loop(0, NX, a01, 0)
    made.update(("xn", r) for r in range(0, 64, 16))

    def a23(i, carry):
        with _scope("a_wait23"):
            for c in cp_wk(i, SEM_W + i):
                c.wait()
        with _scope("a23"):
            wk_prep(i)
            l2_side((i, T0 // 2), T0 // 2, 250, 14 * T0 - 250)
            kproj(0, T0, [i])
            finish()
        return carry

    lax.fori_loop(0, 2, a23, 0)
    wait_group(NX + 2)
    with _scope("a4"):
        wk_prep(2)
        ln_sides(L4)
        kproj(0, T0, [2])
        finish()
    wait_group(NX + 3)
    with _scope("a5"):
        wk_prep(3)
        ln_sides(L5)
        kproj(0, T0, [3])
        for r0, n in A5K:
            kproj(r0, n)
        finish()
    wait_group(NX + 4)
    with _scope("a6"):
        ln_sides(L6)
        for r0, n in A6K:
            kproj(r0, n)
        finish()
    wait_group(NX + 5)
    with _scope("a7"):
        ln_sides(L7)
        add_side(lambda tok: wq_perm(), 128, *WQ_PERM)
        add_side(lambda tok: wq_form(), 224, *WQ_FORM)
        add_side(lambda tok: route(), 17, *ROUTE)
        for r0, n in A7K:
            kproj(r0, n)
        finish()

    def b_body(j, carry):
        qa = BQ - QB
        with _scope("b_r0"):
            z_prep()
            add_side(lambda tok: ps_form(j), 7 * HQ // 16, 0, 49 * qa - 400)
            for r0 in range(0, qa, QN):
                run_all(q_rows(j, r0, QN, pq_buf, den_buf, r0, r0 + QN < qa))
            finish()
        with _scope("b_wait"):
            for c in cp_b(j, wait_only=True):
                c.wait()
        with _scope("b_r1"):
            add_side(lambda tok: ffn_part(j), FH * 3 // 8, 0, R1T)
            add_side(lambda tok: normalise(pq_buf, den_buf, qa, qs, j * (qa // 2), lambda r: r >= qa - QN),
                     22 * (qa // 16), 0, R1T)
            run_all(g_kvm(j))
            finish()
        return carry

    lax.fori_loop(0, 2, b_body, 0)

    def c_body(t, carry):
        with _scope("c_body"):
            y = _rbf(jnp.sum(yacc[...], axis=0, keepdims=True))
            y = _rbf(y * _rbf(1.0 / _rbf(1.0 + _rbf(jnp.exp(-rsel[0:1, :])))))
            j, h = t >> 1, t & 1
            na, nb = (BQ - QB) // 2, QB // 2
            hb = pl.ds(_mo(h * nb, 16), nb)
            add_side(lambda tok: normalise(pqb_buf.at[j, :, hb, :], denb_buf.at[j, :, hb, :], nb, qsb, 0,
                                           lambda r: True, tok),
                     4 + 22 * (nb // 16), 0, 49 * na - 800, SLAG)
            for p in range(0, na, CR):
                p0 = j * BQ + h * na + p
                run_all(out_part(p0, CR, y, qs, t * (na // 2) + p // 2))
            flush()
            run_all(out_part(j * BQ + BQ - QB + h * nb, nb, y, qsb, 0))
            finish()
        return carry

    lax.fori_loop(0, 4, c_body, 0)
    with _scope("tail"):
        cp(out_buf, out_hbm.at[0], SEM_O).wait()


@jax.jit
def pallas_parallel_sum__linear_attn_block__moe_arch_mod__prompt_kernel(
    A_x: jax.Array,
    A_wqkv: jax.Array,
    A_wo: jax.Array,
    B_x: jax.Array,
    B_w_r: jax.Array,
    B_w_gate: jax.Array,
    B_w_up: jax.Array,
    B_w_down: jax.Array,
):
    del B_x
    V = pltpu.VMEM
    scratch = [
        V((4, HQ, D), bf16),
        V((2, D, 512), bf16),
        V((2, 512, D), bf16),
        V((8 * D,), bf16),
        V((2, D, FH), bf16),
        V((2, D, FH), bf16),
        V((2, FH, D), bf16),
        V((28, HQ // 2, 256), u32),
        V((28, HQ // 2, 256), u32),
        V((49, 128, 256), u32),
        V((S, 128), f32),
        V((S, 128), f32),
        V((8, D), f32),
        V((8, D), f32),
        V((2, 4, HQ, 512), f32),
        V((D, 128), f32),
        V((8, D), f32),
        V((8, D), f32),
        V((16, D), f32),
        V((4, 8, 128), u32),
        V((4, HD // 2, 7 * 128), u32),
        V((S, 256), f32),
        V((64, 64, 128), u32),
        V((1, HQ // 2, 49 * 128), u32),
        V((49, BQ - QB, 256), u32),
        V((49, 128, 256), u32),
        V((8, 64, 128), u32),
        V((4, 64, 128), u32),
        V((1, 4, BQ - QB, D), f32),
        V((1, 4, BQ - QB, 128), f32),
        V((2, 4, QB, D), f32),
        V((2, 4, QB, 128), f32),
        V((49, QB // 4, 256), u32),
        V((1, 4, 128, D), f32),
        V((1, FH, 128), f32),
        V((S, D), bf16),
        pltpu.SMEM((1,), i32),
        pltpu.SemaphoreType.DMA((4 + T0 // X0 + 6,)),
    ]
    extra = {k: True for k in ("disable_bounds_checks", "disable_semaphore_checks")
             if hasattr(pltpu.CompilerParams, k)}
    return pl.pallas_call(
        _kernel,
        out_shape=jax.ShapeDtypeStruct((1, S, D), bf16),
        in_specs=[pl.BlockSpec(memory_space=pl.ANY)] * 7,
        out_specs=pl.BlockSpec(memory_space=pl.ANY),
        scratch_shapes=scratch,
        compiler_params=pltpu.CompilerParams(vmem_limit_bytes=120 * 1024 * 1024, **extra),
    )(A_x.reshape(4, HQ, D), A_wqkv, A_wo, B_w_r, B_w_gate, B_w_up, B_w_down)
```

```python
import contextlib

import jax
import jax.numpy as jnp
from jax import lax
import jax.experimental.pallas as pl
import jax.experimental.pallas.tpu as pltpu

bf16, f32, u32, i32 = jnp.bfloat16, jnp.float32, jnp.uint32, jnp.int32

S = 2048
D = 1024
F = 3584
HD = D // 2
HQ = S // 4
BQ = HQ // 2
FH = F // 2
QB = 64
QN = 48
QSPLIT = 6
CR = 48
T0 = 96
X0 = 32
XG = (160, 208)
XN = 128

SLAG = 400
LNLAG = 700
QW = (28, 36, 36, 6, 2, 2, 2)
L4 = ([(96, 144, 0, 1100)], [])
L5 = ([(144, 208, 1100, 3500)], [(96, 128, 0, 1150), (128, 144, 1250, 2000), (144, 208, 2300, 4700)])
L6 = ([(208, 512, 0, 10000)], [(208, 256, 800, 2600), (256, 448, 2700, 10500)])
L7 = ([], [(448, 512, 0, 3000)])
A5K = ((96, 32), (128, 32))
A6K = ((160, 48), (208, 48), (256, 48), (304, 48))
A7K = ((352, 48), (400, 48), (448, 64))
WQ_PERM, WQ_FORM, ROUTE = (0, 3200), (3300, 8600), (4500, 5300)
R1T = 12800
MF = (128, 3420)

L_ORD = (2, 3, 0, 1, 4, 5, 6)
R_ORD = (2, 0, 6, 5, 1, 4, 3)

K_SEQ = (1, 4, 0, 2, 3, 5, 6)
K_SEQ2 = (0, 1, 2, 5, 3, 4, 6)
W_SEQ = (0, 1, 5, 6, 4, 2, 3)

NN = (((1,), (0,)), ((), ()))
TN = (((0,), (0,)), ((), ()))


SCOPES = False


def _scope(name):
    return jax.named_scope(name) if SCOPES else contextlib.nullcontext()


def _mo(v, m):
    return v if isinstance(v, int) else pl.multiple_of(v, m)


def _dot(a, b, dims):
    return lax.dot_general(a, b, dims, preferred_element_type=f32)


def _pack(v):
    return pltpu.bitcast(v.astype(bf16), u32)


def _unpack(v):
    return pltpu.bitcast(v, bf16)


def _combine(m):
    m1, m2, m3, m4, m5, m6, m7 = m
    return m1 + m4 - m5 + m7, m3 + m5, m2 + m4, m1 - m2 + m3 + m6


def _lform(a11, a12, a21, a22):
    return (a11 + a22, a21 + a22, a11, a22, a11 + a12, a21 - a11, a12 - a22)


def _rform(b11, b12, b21, b22):
    return (b11 + b22, b11, b12 - b22, b21 - b11, b22, b11 + b12, b21 + b22)


def _sform(x11, x12, x21, x22):
    return (x11, x22, x11 + x22, x21 + x22, x11 + x12, x21 - x11, x12 - x22)


def _wl(a11, a12, a21, a22):
    s1 = a21 + a22
    s2 = s1 - a11
    return (a11, a12, a12 - s2, a22, s1, s2, a11 - a21)


def _wr(b11, b12, b21, b22):
    t1 = b12 - b11
    t2 = b22 - t1
    return (b11, b21, b22, t2 - b21, t1, t2, b22 - b12)


def _wc(p):
    p1, p2, p3, p4, p5, p6, p7 = p
    u2 = p1 + p6
    u3 = u2 + p7
    return p1 + p2, (u2 + p5) + p3, u3 - p4, u3 + p5


W_R = (3, 1, 0, 2, 4, 5, 6)


def _wl_swapped(a11, a12, a21, a22):
    return _wl(a12, a11, a22, a21)


def _wc_swapped(p):
    p1, p2, p3, p4, p5, p6, p7 = p
    v2 = p1 + p6
    u3 = p7 - v2
    return (p5 - v2) + p3, p1 + p2, u3 + p5, p4 - u3


class _Sym:
    def __init__(self, t):
        self.t = t

    def __add__(self, o):
        return _Sym({**self.t, **o.t})

    def __sub__(self, o):
        return _Sym({**self.t, **{k: -v for k, v in o.t.items()}})


def _st(u, ct):
    return slice((4 * ct + u) * 128, (4 * ct + u + 1) * 128)


def _to_st(v):
    return jnp.concatenate([v[:, (2 * u + ct) * 128:(2 * u + ct + 1) * 128]
                            for ct in range(2) for u in range(4)], axis=1)


def _phi(t):
    return jnp.where(t > 0, t + 1.0, jnp.exp(t)) + 1e-6


def _rbf(v):
    return v.astype(bf16).astype(f32)


def _kernel(x_hbm, wqkv_hbm, wo_hbm, wr_hbm, wg_hbm, wu_hbm, wd_hbm, out_hbm,
            x_buf, wv_buf, wo_buf, wr_buf, wg_buf, wu_buf, wd_buf,
            xs1, xs2, wqs, sa, sb, zacc, zp, pk_buf, xb, yacc, rsel, wrb, zero_buf,
            wks, stats, wqt, ps_raw, qs, ms, tscr, tscr2, pq_raw, den_raw, pqb_buf, denb_buf, qsb,
            mg_raw, hb_raw, out_buf, idx_s, sem):
    wq_buf = out_buf.at[pl.ds(0, D), :]
    wk_buf = out_buf.at[pl.ds(D, D), :]

    def xs_at(k1, e, rows=None):
        r = xs1.at[k1 * 4 + (0, 1, 7, 3).index(e)] if e in (0, 1, 7, 3) else xs2.at[k1 * 4 + (2, 4, 5, 6).index(e)]
        return r if rows is None else r.at[rows, :]

    SEM_B, SEM_O, SEM_Z, SEM_A = 0, 2, 3, 4

    def cp(src, dst, s):
        return pltpu.make_async_copy(src, dst, sem.at[s])

    def cp_x(r0, n, s):
        r = pl.ds(_mo(r0, 16), n)
        return [cp(x_hbm.at[:, r, :], x_buf.at[:, r, :], s)]

    def cp_wk(c, s):
        return [cp(wqkv_hbm.at[:, pl.ds(_mo(D + c * 256, 256), 256)],
                   wk_buf.at[:, pl.ds(_mo(c * 256, 256), 256)], s)]

    NX = T0 // X0
    SEM_W = SEM_A + NX
    cp_wr = cp(wr_hbm, wr_buf.at[pl.ds(0, D)], SEM_Z)
    a_groups = [cp_x(i * X0, X0, SEM_A + i) for i in range(NX)] + [
        cp_wk(0, SEM_W),
        cp_wk(1, SEM_W + 1),
        cp_wk(2, SEM_W + 2) + cp_x(T0, XG[0] - T0, SEM_W + 2),
        cp_wk(3, SEM_W + 3) + cp_x(XG[0], XG[1] - XG[0], SEM_W + 3),
        cp_x(XG[1], HQ - XG[1], SEM_W + 4),
        [cp(wqkv_hbm.at[:, pl.ds(0, D)], wq_buf, SEM_W + 5)],
    ]

    def cp_b(j, wait_only=False):
        dsts = [wg_buf.at[j], wu_buf.at[j], wd_buf.at[j]]
        for a in range(4):
            dsts += [wv_buf.at[j, :, pl.ds(a * 128, 128)], wo_buf.at[j, pl.ds(a * 128, 128), :]]
        if wait_only:
            return [cp(dst, dst, SEM_B + j) for dst in dsts]
        fs = pl.ds(j * FH, FH)
        srcs = [wg_hbm.at[:, fs], wu_hbm.at[:, fs], wd_hbm.at[fs, :]]
        for a in range(4):
            c0 = (2 * a + j) * 128
            srcs += [wqkv_hbm.at[:, pl.ds(2 * D + c0, 128)], wo_hbm.at[pl.ds(c0, 128), :]]
        return [cp(src, dst, SEM_B + j) for src, dst in zip(srcs, dsts)]

    clock = [0]
    toks = []
    sides = []
    fwd = [None]

    def emit_tok(vals, stamp):
        t = None
        for v in vals:
            v = pltpu.bitcast(v, u32) if v.dtype != u32 else v
            t = v if t is None else t | v
        toks.append((stamp, t & zero_buf[0]))

    def token(kind):
        t = fwd[0]
        if "u" not in t:
            t["u"] = pltpu.bitcast(t["src"](), u32) & zero_buf[0]
        if kind != "u" and "f" not in t:
            t["f"] = pltpu.bitcast(t["u"], f32)
        if kind == "f16" and "f16" not in t:
            t["f16"] = jnp.concatenate([t["f"], t["f"]], axis=0)
        return t[kind]

    def gate(v):
        if fwd[0] is None:
            return v
        head = v if v.shape[0] == 8 else v[0:8]
        head = head | token("u") if v.dtype == u32 else head + token("f")
        return head if v.shape[0] == 8 else jnp.concatenate([head, v[8:]], axis=0)

    def gate16(v):
        return v if fwd[0] is None else v + token("f16")

    def add_side(gen_fn, n, t0, t1, lag=None):
        st = {"i": 0, "n": n, "t0": clock[0] + t0, "t1": clock[0] + t1}

        def tok(vals):
            if lag is not None:
                emit_tok(vals, st["t0"] + (st["i"] + 1) * (st["t1"] - st["t0"]) // st["n"] + lag)
        st["g"] = gen_fn(tok)
        sides.append(st)

    def advance(until):
        for st in sides:
            while st["i"] < st["n"] and st["t0"] + st["i"] * (st["t1"] - st["t0"]) // st["n"] < until:
                next(st["g"], None)
                st["i"] += 1
                if st["i"] == st["n"]:
                    for _ in st["g"]:
                        pass

    def flush():
        for st in sides:
            for _ in st["g"]:
                pass
        sides.clear()

    def finish():
        flush()
        toks.clear()
        fwd[0] = None

    def mm(lhs, rhs, dims, cycles, nseg=1):
        due = [t for (c, t) in toks if c <= clock[0]]
        toks[:] = [(c, t) for (c, t) in toks if c > clock[0]]
        if due:
            head = rhs[0:8, 0:128]
            for t in due:
                head = head | t
            if rhs.shape[1] > 128:
                head = jnp.concatenate([head, rhs[0:8, 128:]], axis=1)
            rhs = jnp.concatenate([head, rhs[8:]], axis=0)
        res = _dot(lhs, _unpack(rhs), dims)
        ngr = res.shape[0] // 16
        for sg in range(nseg):
            for i in range(ngr):
                fwd[0] = {"src": lambda sg=sg, i=i: res[i * 16:i * 16 + 8, sg * 128:(sg + 1) * 128]}
                clock[0] += cycles // nseg // ngr
                advance(clock[0])
        return res

    def form_steps(form, form2, get, put, tok=None, keep=range(7)):
        terms = form(*[_Sym({i: 1}) for i in range(4)])
        gated = (0, 1, 2, 3) if 7 in keep else {_wl: (0, 1, 3), _wr: (0, 2, 3), _wl_swapped: (1, 2)}[form2]
        for k1 in range(7):
            sub = []
            for r in range(2):
                for c in range(2):
                    v = None
                    for i, sg in sorted(terms[k1].t.items(), key=lambda e: -e[1]):
                        b = get(r + 2 * (i // 2), c + 2 * (i % 2))
                        if v is None:
                            v = gate16(b) if 2 * r + c in gated else b
                        else:
                            v = v + b if sg > 0 else v - b
                    sub.append(v)
            vals = form2(*sub) + (sub[2],)
            for k2 in keep:
                put(k1, k2, _pack(vals[k2]))
            if tok is not None and k1 % 2 == 0:
                full = vals[3 if form2 is _wr else 2]
                tok([full[0:8], full[8:16]])
            yield

    def strassen2(lhs, rhs, dims, cycles, nseg=1, wts=(16,) * 7, comb=_wc):
        m1 = [None] * 7
        for i1, k1 in enumerate(K_SEQ2):
            m2 = [None] * 7
            for k2 in W_SEQ:
                m2[k2] = mm(lhs(k1, k2), rhs(k1, k2), dims, cycles * wts[i1] // 16, nseg)
                yield
            m1[k1] = comb(m2)
        out = [[None] * 4 for _ in range(4)]
        for s2 in range(4):
            for s1, v in enumerate(_combine([m1[k1][s2] for k1 in range(7)])):
                out[(s1 // 2) * 2 + s2 // 2][(s1 % 2) * 2 + s2 % 2] = v
        return out

    made = set()

    def need(*keys):
        assert all(k in made for k in keys), keys

    def row_views(base):
        if base == 0:
            return x_buf, sa, sb, stats, xn_buf, None
        i, n = base
        b = _mo(i * n, 16)
        return ([x_buf.at[:, pl.ds(b, n), :]] + [r.at[pl.ds(b, S - 128 + n), :] for r in (sa, sb, stats)]
                + [xn_buf.at[:, pl.ds(b, n), :], pl.ds(_mo(i * (n // 2), 8), n // 2)])

    def xs_form(r0, tok, which="all", base=0):
        xn_v, xs_v = row_views(base)[4:]
        rows = slice(r0 % XN, r0 % XN + 16)

        keep = {"all": range(8), "l1": (0, 1, 7, 3), "l2": (2, 4, 5, 6)}[which]
        for ct in range(2):
            def put(k1, k2, v):
                xs_at(k1, k2, xs_v)[r0 // 2:r0 // 2 + 8, ct * 128:(ct + 1) * 128] = v
            yield from form_steps(
                _sform, _wl, lambda q, u: xn_v[q, rows, _st(u, ct)], put, tok, keep)
        made.add(("xs", r0))

    def ln_stats(r_start, n_rows, tok, base=0):
        x_v, sa_v, sb_v, st_v, xn_v, _ = row_views(base)
        lane = lax.broadcasted_iota(i32, (8, 128), 1)
        for r0 in range(r_start, r_start + n_rows, 16):
            if r0 >= T0:
                need(("in", 2 + sum(r0 >= g for g in XG)))
            if r0 - XN >= T0:
                need(("ln", r0 - XN))
            for g in range(8):
                q, o = g // 2, (g % 2) * 8
                rg = q * HQ + r0 + o
                xv = x_v[q, r0 + o:r0 + o + 8, :].astype(f32)
                xg = jnp.concatenate([gate(xv[:, 0:128]), xv[:, 128:]], axis=1)
                mf = jnp.sum(xg, axis=1, keepdims=True) * (1.0 / D)
                d = xv - mf
                var = jnp.sum(d * d, axis=1, keepdims=True) * (1.0 / D)
                rs = lax.rsqrt(var + 1e-5)
                xn_v.at[q][r0 % XN + o:r0 % XN + o + 8, :] = _to_st(d * rs)
                rs = jnp.broadcast_to(rs, (8, 128))
                mf = jnp.broadcast_to(mf, (8, 128))
                sa_v[rg:rg + 8, :] = 1.0 + rs
                sb_v[rg:rg + 8, :] = mf * rs
                st_v[rg:rg + 8, 0:128] = jnp.where(lane == 0, mf, jnp.broadcast_to(var, (8, 128)))
                if tok is not None:
                    tok([rs])
                if g == 7:
                    made.add(("xn", r0))
                yield

    def ln_later(r_start, n_rows, tok, which="all", base=0):
        st_v, xn_v = row_views(base)[3:5]
        for r0 in range(r_start, r_start + n_rows, 16):
            need(("xn", r0))
            form = xs_form(r0, tok, which, base)
            for g in range(8):
                for _ in range(2 if g < 7 else 0):
                    next(form)
                    yield
                q, o = g // 2, (g % 2) * 8
                t = None
                if which != "l1":
                    v = xn_v[q, r0 % XN + o:r0 % XN + o + 8, :] * wrb[8:16, :]
                    for ct in range(8):
                        h = v[:, ct * 128:(ct + 1) * 128]
                        t = gate(h) if t is None else t + h
                if t is not None:
                    st_v[q * HQ + r0 + o:q * HQ + r0 + o + 8, 128:256] = t
                if tok is not None:
                    tok([t])
                if g == 7:
                    next(form, None)
                    made.add(("ln", r0))
                yield

    def wk_prep(c):
        if isinstance(c, int):
            need(("in", c))
        cs = pl.ds(_mo(c * 256, 256), 256)
        for i in range(HD // 16):
            r0 = i * 16
            top = wk_buf[r0:r0 + 16, cs].astype(f32)
            bot = wk_buf[HD + r0:HD + r0 + 16, cs].astype(f32)
            ops = _rform(top[:, :128], top[:, 128:], bot[:, :128], bot[:, 128:])
            for k in range(7):
                wks.at[c][r0 // 2:r0 // 2 + 8, k * 128:(k + 1) * 128] = _pack(ops[k])

    def wq_perm():
        need(("in", 5))

        def permute(kt):
            for g in range(8):
                tile = gate(pltpu.bitcast(wq_buf[kt * 128:(kt + 1) * 128, g * 128:(g + 1) * 128], u32))
                wqt.at[kt * 8 + g][...] = pltpu.bitcast(_unpack(tile).T, u32)
                yield

        def back(kt):
            for j in range(8):
                tile = gate(jnp.concatenate([wqt[kt * 8 + g, pl.ds(j, 8, stride=8), :] for g in range(8)],
                                            axis=0))
                v = pltpu.bitcast(_unpack(tile).T.astype(f32), u32)
                c0 = (kt // 2) * D + _st(j // 2, j % 2).start
                ps[(kt % 2) * 128:(kt % 2 + 1) * 128, c0:c0 + 128] = v
                made.add(("wqp", kt, j))
                yield

        order = (0, 2, 4, 6, 1, 3, 5, 7)
        for n in range(10):
            if n < 8:
                yield from permute(order[n])
            if n > 1:
                yield from back(order[n - 2])

    def wq_form():
        for i in range(16):
            need(*[("wqp", 2 * r + i // 8, j) for r in range(4) for j in range(8)])
            for ct in range(2):
                def put(k1, k2, v):
                    wqs.at[k1 * 7 + k2][i * 8:(i + 1) * 8, ct * 128:(ct + 1) * 128] = v
                yield from form_steps(
                    _rform, _wr, lambda r, c: pltpu.bitcast(
                        ps[i * 16:(i + 1) * 16, r * D + _st(c, ct).start:r * D + _st(c, ct).stop],
                        f32), put)

    def kproj(r0, n, chunks=range(4)):
        pr = pl.ds(r0 // 2, n // 2)
        need(*[("xs", r) for r in range(max(r0, T0), r0 + n, 16)])
        for c in chunks:
            m = [None] * 7
            for k in K_SEQ:
                e11, e12, e21, e22 = [xs_at(L_ORD[k], e)[pr, :] for e in (0, 1, 7, 3)]
                lhs = jnp.concatenate([jnp.concatenate([e11, e12], axis=1),
                                       jnp.concatenate([e21, e22], axis=1)], axis=0)
                m[k] = mm(_unpack(lhs), wks[c, :, k * 128:(k + 1) * 128], NN, 2 * n)
            kk = [_phi(v) for v in _combine(m)]
            for ct in range(2):
                zacc[:, pl.ds(_mo(c * 256 + ct * 128, 128), 128)] += (
                    (kk[ct] + kk[2 + ct]).reshape(n // 4, 8, 128).sum(axis=0))
            for s1 in range(4):
                for h in range(2):
                    pk_buf.at[s1 % 2, (s1 // 2) * 2 + h][r0:r0 + n, pl.ds(_mo(c * 128, 128), 128)] = (
                        kk[s1][h * n:(h + 1) * n])

    def z_prep():
        z = jnp.sum(zacc[...], axis=0, keepdims=True)
        zt = _pack(jnp.broadcast_to(z, (128, D)).astype(bf16).T)
        for g in range(8):
            tscr.at[g][...] = zt[g * 64:(g + 1) * 64, :]
        for j in range(8):
            blk = jnp.concatenate([tscr[g, pl.ds(j, 8, stride=8), :] for g in range(8)], axis=0)
            zp[:, j * 128:(j + 1) * 128] = _unpack(blk).T[0:8, :].astype(f32)

    def route():
        rows, dots = [None] * 16, [None] * 16
        for b in sorted(range(S // 128), key=lambda b: b % 4):
            need(*[("ln", r) for r in range(max(T0, b % 4 * 128), b % 4 * 128 + 128, 16)])
            rows[b] = gate(stats[b * 128:(b + 1) * 128, 0:128]).T[0:8, :]
            dots[b] = jnp.sum(gate(stats[b * 128:(b + 1) * 128, 128:256]).T, axis=0, keepdims=True)
            yield
        mf = jnp.concatenate([v[0:1] for v in rows], axis=0)
        var = jnp.concatenate([v[1:2] for v in rows], axis=0)
        tr = jnp.concatenate(dots, axis=0) * jnp.sqrt(var + 1e-5)
        wsum = jnp.sum(wrb[0:1, :], axis=1, keepdims=True)
        mb = _rbf(mf)
        inv = 1.0 / _rbf(jnp.sqrt(_rbf(_rbf(var) + 1e-5)))
        rv = _rbf((tr + (mf - mb) * wsum) * inv)
        rmax = jnp.max(jnp.max(rv, axis=1, keepdims=True), axis=0, keepdims=True)
        pos = (lax.broadcasted_iota(i32, rv.shape, 0) * 128 + lax.broadcasted_iota(i32, rv.shape, 1))
        idx = jnp.min(jnp.where(rv == rmax, pos, S - 1))
        idx_s[0] = idx

        def pick(v):
            v = jnp.sum(jnp.where(pos == idx, v, 0.0), axis=1, keepdims=True)
            return jnp.sum(v, axis=0, keepdims=True)

        xv = x_buf[(idx >> 9) & 3, pl.ds(_mo(idx & (HQ - 16), 16), 16), :].astype(f32)
        sel = lax.broadcasted_iota(i32, xv.shape, 0) == (idx & 15)
        row = jnp.sum(jnp.where(sel, xv, 0.0), axis=0, keepdims=True)
        row = _rbf(_rbf(row - pick(mb)) * pick(inv))
        rsel[...] = jnp.broadcast_to(_rbf(jnp.sum(row * wrb[0:1, :], axis=1, keepdims=True)), rsel.shape)
        xb[...] = jnp.broadcast_to(row, (128, D)).T
        yield

    def ps_form(j):
        for c in range(HQ // 16):
            def put(k1, k2, v):
                k = k1 * 7 + k2
                ps[c * 8:(c + 1) * 8, k * 128:(k + 1) * 128] = v
            yield from form_steps(
                _lform, _wl_swapped,
                lambda r, q: pk_buf[j, q, c * 16:(c + 1) * 16, r * 128:(r + 1) * 128], put)

    def q_rows(j, r0, n, pq, rc, d0, rec):
        xj = pl.ds(_mo(j * (BQ // 2), BQ // 2), BQ // 2)
        pr = slice(r0 // 2, (r0 + n) // 2)
        blk = yield from strassen2(lambda k1, k2: _unpack(xs_at(L_ORD[k1], k2, xj)[pr, :]),
                                   lambda k1, k2: wqs[k1 * 7 + k2], NN, n, 1, QW)
        lane = lax.broadcasted_iota(i32, (n, 128), 1)
        for q in range(4):
            d = None
            for u in (3, 2, 1, 0):
                v = _phi(blk[q][u])
                for ct in range(2):
                    pq.at[q][d0:d0 + n, _st(u, ct)] = v[:, ct * 128:(ct + 1) * 128]
                t = v * zp[0:1, u * 256:(u + 1) * 256]
                t = t[:, :128] + t[:, 128:]
                d = t if d is None else d + t
            if rec:
                d = recip(d, lane)
            rc.at[q][d0:d0 + n, :] = d

    def recip(d, lane):
        d = d + jnp.where(lane % 2 == 0, pltpu.roll(d, 127, 1), pltpu.roll(d, 1, 1))
        d = d + jnp.where(lane % 4 < 2, pltpu.roll(d, 126, 1), pltpu.roll(d, 2, 1))
        return 1.0 / (d + 1e-6)

    def normalise(pq, rc, nr, dst, p0, raw, tok=None):
        lane = lax.broadcasted_iota(i32, (16, 128), 1)

        def fix(c):
            if c < nr // 16 and raw(c * 16):
                for q in range(4):
                    rq = slice(c * 16, (c + 1) * 16)
                    rc.at[q][rq, :] = recip(gate16(rc[q, rq, :]), lane)

        def scale(c):
            rq = slice(c * 16, (c + 1) * 16)
            fix(c + 1)
            for hf in range(2):
                for q in range(4):
                    cs = slice(hf * HD, (hf + 1) * HD)
                    pq.at[q][rq, cs] = pq[q, rq, cs] * jnp.concatenate([gate16(rc[q, rq, :])] * 4, axis=1)
                    yield

        def form(c):
            rq = slice(c * 16, (c + 1) * 16)
            p2 = pl.ds(_mo(p0 + c * 8, 8), 8)
            for ct in range(2):
                def put(k1, k2, v):
                    dst.at[k1 * 7 + k2][p2, ct * 128:(ct + 1) * 128] = v
                yield from form_steps(_lform, _wl, lambda q, u: pq[q, rq, _st(u, ct)], put, tok)

        fix(0)
        if raw(0):
            for _ in range(4):
                yield
        yield from scale(0)
        for c in range(nr // 16):
            nxt = scale(c + 1) if c + 1 < nr // 16 else iter(())
            for i, _ in enumerate(form(c)):
                yield
                if i < 8 and c + 1 < nr // 16:
                    next(nxt)
                    yield

    def g_kvm(j):
        blk = yield from strassen2(
            lambda k1, k2: _unpack(ps[:, (k1 * 7 + k2) * 128:(k1 * 7 + k2 + 1) * 128]),
            lambda k1, k2: xs_at(R_ORD[k1], W_R[k2])[...], TN, 256, 2, comb=_wc_swapped)
        hm = (lax.broadcasted_iota(i32, (128, 128), 0) // 32
              == lax.broadcasted_iota(i32, (128, 128), 1) // 32)
        qb = q_rows(j, BQ - QB, QB, pqb_buf.at[j], denb_buf.at[j], 0, False)
        for _ in range(QSPLIT):
            next(qb)
        kvps = []
        for a in (3, 2, 1, 0):
            gg = jnp.concatenate(blk[a], axis=1).astype(bf16)
            wv_u = pltpu.bitcast(wv_buf[j, :, a * 128:(a + 1) * 128], u32)
            kv = jnp.where(hm, mm(gg, wv_u, NN, 256), 0.0)
            tscr2.at[a][...] = _pack(kv)
            kvps.append(_unpack(jnp.concatenate(
                [tscr2[a, pl.ds(jj, 8, stride=8), :] for jj in range(8)], axis=0)))

        def m_form():
            for a in (3, 2, 1, 0):
                need(("mg", a))
                for jl in range(2):
                    for ct in range(2):
                        def put(k1, k2, v):
                            ms.at[k1 * 7 + k2][pl.ds(_mo(jl * 64 + (2 * a + j) * 8, 8), 8),
                                               ct * 128:(ct + 1) * 128] = v
                        yield from form_steps(
                            _rform, _wr, lambda q, u: mg_buf[a, (2 * q + jl) * 16:(2 * q + jl + 1) * 16, _st(u, ct)], put)

        for i, a in enumerate((3, 2, 1, 0)):
            wo_u = pltpu.bitcast(wo_buf[j, a * 128:(a + 1) * 128, :], u32)
            res = mm(kvps[i], wo_u, NN, 256)
            mg_buf.at[a][...] = _to_st(res)
            made.add(("mg", a))
            if i == 0:
                add_side(lambda tok: m_form(), 112, *MF)
        for _ in qb:
            pass

    def out_part(base, span, off, nr, y, src):
        b = _mo(base, 32)
        sa_v, sb_v, out_v = [r.at[pl.ds(b, 3 * HQ + span), :] for r in (sa, sb, out_buf)]
        x_v = x_buf.at[:, pl.ds(b, span), :]
        row = lax.broadcasted_iota(i32, (nr, 256), 0) + (base + off)
        blk = yield from strassen2(lambda k1, k2: _unpack(src[k1 * 7 + k2, off // 2:(off + nr) // 2, :]),
                                   lambda k1, k2: ms[k1 * 7 + k2], NN, nr)
        for s1 in (3, 2, 1, 0):
            for s2 in range(4):
                q = (s1 // 2) * 2 + s2 // 2
                u = (s1 % 2) * 2 + s2 % 2
                rr, cc = pl.ds(q * HQ + off, nr), pl.ds(u * 256, 256)
                a = jnp.concatenate([sa_v[rr, :]] * 2, axis=1)
                c = jnp.concatenate([sb_v[rr, :]] * 2, axis=1)
                o = blk[q][u] + jnp.where(row + q * HQ == idx_s[0], y[:, u * 256:(u + 1) * 256], 0.0)
                out_v[rr, cc] = (x_v[q, off:off + nr, cc].astype(f32) * a - c + o).astype(bf16)
                if s2 % 2 == 1:
                    ch = pl.ds((s1 % 2) * HD, HD)
                    ro = pl.ds(_mo(base + q * HQ + off, 16), nr)
                    cp(out_buf.at[ro, ch], out_hbm.at[0, ro, ch], SEM_O).start()

    def ffn_part(j):
        def fma(acc, w, v):
            p = w.astype(f32) * v
            return acc + p[0:8] + p[8:16]

        for f0 in range(0, FH, 256):
            fs = slice(f0, f0 + 256)
            ag = jnp.zeros((8, 256), f32)
            au = jnp.zeros((8, 256), f32)
            for k in range(0, D, 16):
                xv = jnp.concatenate([gate16(xb[k:k + 16, :])] * 2, axis=1)
                ag = fma(ag, wg_buf[j, k:k + 16, fs], xv)
                au = fma(au, wu_buf[j, k:k + 16, fs], xv)
                yield
            g = _rbf(jnp.sum(ag, axis=0, keepdims=True))
            u = _rbf(jnp.sum(au, axis=0, keepdims=True))
            h = _rbf(_rbf(g * jax.nn.sigmoid(g)) * u)
            hb_buf[fs, :] = jnp.broadcast_to(h, (128, 256)).T
        for d0 in range(0, D, 512):
            ds_ = slice(d0, d0 + 512)
            acc = yacc[:, ds_]
            for k in range(0, FH, 16):
                hv = jnp.concatenate([gate16(hb_buf[k:k + 16, :])] * 4, axis=1)
                acc = fma(acc, wd_buf[j, k:k + 16, ds_], hv)
                yield
            yacc[:, ds_] = acc

    def wait_group(i):
        with _scope("a_wait%d" % i):
            for c in a_groups[i]:
                c.wait()
        made.add(("in", i - NX))

    def run_all(gen):
        for _ in gen:
            pass

    def ln_sides(plan):
        for r0, r1, t0, t1 in plan[0]:
            add_side(lambda tok, r0=r0, r1=r1: ln_stats(r0, r1 - r0, tok), (r1 - r0) // 2, t0, t1, LNLAG)
        for r0, r1, t0, t1 in plan[1]:
            add_side(lambda tok, r0=r0, r1=r1: ln_later(r0, r1 - r0, tok), 22 * (r1 - r0) // 16, t0, t1, SLAG)

    def l2_side(base, n, t0, t1):
        add_side(lambda tok: ln_later(0, n, None, "l2", base), 22 * n // 16, t0, t1)

    with _scope("p0_issue"):
        cp_wr.start()
        for grp in a_groups:
            for c in grp:
                c.start()
        for j in range(2):
            for c in cp_b(j):
                c.start()
        zacc[...] = jnp.zeros(zacc.shape, f32)
        yacc[...] = jnp.zeros(yacc.shape, f32)
        zero_buf[1] = jnp.zeros((8, 128), u32)
        cp_zero = cp(zero_buf.at[1], zero_buf.at[0], SEM_Z)
        cp_zero.start()
        cp_zero.wait()
        cp_wr.wait()
        wr8 = jnp.broadcast_to(wr_buf[0:D].reshape(1, D).astype(f32), (8, D))
        wrb[0:8, :] = wr8
        wrb[8:16, :] = _to_st(wr8)
        z0 = jnp.max(pltpu.bitcast(zero_buf[0], i32))
        ps, pq_buf, den_buf, mg_buf, hb_buf = [r.at[z0] for r in (ps_raw, pq_raw, den_raw, mg_raw, hb_raw)]
        xn_buf = mg_buf

    def a01(i, carry):
        with _scope("a_wait01"):
            for c in cp_x(i * X0, X0, SEM_A + i):
                c.wait()
        with _scope("a01"):
            for r in range(0, X0, 16):
                run_all(ln_stats(r, 16, None, (i, X0)))
                if r:
                    run_all(ln_later(r - 16, 16, None, "l1", (i, X0)))
            run_all(ln_later(X0 - 16, 16, None, "l1", (i, X0)))
        return carry

    lax.fori_loop(0, NX, a01, 0)
    made.update(("xn", r) for r in range(0, 64, 16))

    def a23(i, carry):
        with _scope("a_wait23"):
            for c in cp_wk(i, SEM_W + i):
                c.wait()
        with _scope("a23"):
            wk_prep(i)
            l2_side((i, T0 // 2), T0 // 2, 250, 14 * T0 - 250)
            kproj(0, T0, [i])
            finish()
        return carry

    lax.fori_loop(0, 2, a23, 0)
    wait_group(NX + 2)
    with _scope("a4"):
        wk_prep(2)
        ln_sides(L4)
        kproj(0, T0, [2])
        finish()
    wait_group(NX + 3)
    with _scope("a5"):
        wk_prep(3)
        ln_sides(L5)
        kproj(0, T0, [3])
        for r0, n in A5K:
            kproj(r0, n)
        finish()
    wait_group(NX + 4)
    with _scope("a6"):
        ln_sides(L6)
        for r0, n in A6K:
            kproj(r0, n)
        finish()
    wait_group(NX + 5)
    with _scope("a7"):
        ln_sides(L7)
        add_side(lambda tok: wq_perm(), 128, *WQ_PERM)
        add_side(lambda tok: wq_form(), 224, *WQ_FORM)
        add_side(lambda tok: route(), 17, *ROUTE)
        for r0, n in A7K:
            kproj(r0, n)
        finish()

    def b_body(j, carry):
        qa = BQ - QB
        with _scope("b_r0"):
            z_prep()
            add_side(lambda tok: ps_form(j), 7 * HQ // 16, 0, 49 * qa - 400)
            for r0 in range(0, qa, QN):
                run_all(q_rows(j, r0, QN, pq_buf, den_buf, r0, r0 + QN < qa))
            finish()
        with _scope("b_wait"):
            for c in cp_b(j, wait_only=True):
                c.wait()
        with _scope("b_r1"):
            add_side(lambda tok: ffn_part(j), FH * 3 // 8, 0, R1T)
            add_side(lambda tok: normalise(pq_buf, den_buf, qa, qs, j * (qa // 2), lambda r: r >= qa - QN),
                     22 * (qa // 16), 0, R1T)
            run_all(g_kvm(j))
            finish()
        return carry

    lax.fori_loop(0, 2, b_body, 0)

    def c_body(t, carry):
        with _scope("c_body"):
            y = _rbf(jnp.sum(yacc[...], axis=0, keepdims=True))
            y = _rbf(y * _rbf(1.0 / _rbf(1.0 + _rbf(jnp.exp(-rsel[0:1, :])))))
            j, h = t >> 1, t & 1
            na, nb = (BQ - QB) // 2, QB // 2
            hb = pl.ds(_mo(h * nb, 16), nb)
            add_side(lambda tok: normalise(pqb_buf.at[j, :, hb, :], denb_buf.at[j, :, hb, :], nb, qsb, 0,
                                           lambda r: True, tok),
                     4 + 22 * (nb // 16), 0, 49 * na - 800, SLAG)
            qs_t = qs.at[:, pl.ds(_mo(t * (na // 2), 16), na // 2), :]
            for p in range(0, na, CR):
                run_all(out_part(j * BQ + h * na, na, p, CR, y, qs_t))
            flush()
            run_all(out_part(j * BQ + BQ - QB + h * nb, nb, 0, nb, y, qsb))
            finish()
        return carry

    lax.fori_loop(0, 4, c_body, 0)
    with _scope("tail"):
        cp(out_buf, out_hbm.at[0], SEM_O).wait()


@jax.jit
def pallas_parallel_sum__linear_attn_block__moe_arch_mod__prompt_kernel(
    A_x: jax.Array,
    A_wqkv: jax.Array,
    A_wo: jax.Array,
    B_x: jax.Array,
    B_w_r: jax.Array,
    B_w_gate: jax.Array,
    B_w_up: jax.Array,
    B_w_down: jax.Array,
):
    del B_x
    V = pltpu.VMEM
    scratch = [
        V((4, HQ, D), bf16),
        V((2, D, 512), bf16),
        V((2, 512, D), bf16),
        V((8 * D,), bf16),
        V((2, D, FH), bf16),
        V((2, D, FH), bf16),
        V((2, FH, D), bf16),
        V((28, HQ // 2, 256), u32),
        V((28, HQ // 2, 256), u32),
        V((49, 128, 256), u32),
        V((S, 128), f32),
        V((S, 128), f32),
        V((8, D), f32),
        V((8, D), f32),
        V((2, 4, HQ, 512), f32),
        V((D, 128), f32),
        V((8, D), f32),
        V((8, D), f32),
        V((16, D), f32),
        V((4, 8, 128), u32),
        V((4, HD // 2, 7 * 128), u32),
        V((S, 256), f32),
        V((64, 64, 128), u32),
        V((1, HQ // 2, 49 * 128), u32),
        V((49, BQ - QB, 256), u32),
        V((49, 128, 256), u32),
        V((8, 64, 128), u32),
        V((4, 64, 128), u32),
        V((1, 4, BQ - QB, D), f32),
        V((1, 4, BQ - QB, 128), f32),
        V((2, 4, QB, D), f32),
        V((2, 4, QB, 128), f32),
        V((49, QB // 4, 256), u32),
        V((1, 4, 128, D), f32),
        V((1, FH, 128), f32),
        V((S, D), bf16),
        pltpu.SMEM((1,), i32),
        pltpu.SemaphoreType.DMA((4 + T0 // X0 + 6,)),
    ]
    extra = {k: True for k in ("disable_bounds_checks", "disable_semaphore_checks")
             if hasattr(pltpu.CompilerParams, k)}
    return pl.pallas_call(
        _kernel,
        out_shape=jax.ShapeDtypeStruct((1, S, D), bf16),
        in_specs=[pl.BlockSpec(memory_space=pl.ANY)] * 7,
        out_specs=pl.BlockSpec(memory_space=pl.ANY),
        scratch_shapes=scratch,
        compiler_params=pltpu.CompilerParams(vmem_limit_bytes=120 * 1024 * 1024, **extra),
    )(A_x.reshape(4, HQ, D), A_wqkv, A_wo, B_w_r, B_w_gate, B_w_up, B_w_down)
```

```python
import contextlib

import jax
import jax.numpy as jnp
from jax import lax
import jax.experimental.pallas as pl
import jax.experimental.pallas.tpu as pltpu

bf16, f32, u32, i32 = jnp.bfloat16, jnp.float32, jnp.uint32, jnp.int32

S = 2048
D = 1024
F = 3584
HD = D // 2
HQ = S // 4
BQ = HQ // 2
FH = F // 2
QB = 64
QN = 48
QSPLIT = 6
CR = 48
T0 = 96
X0 = 32
XG = (160, 208)
XN = 128

SLAG = 400
LNLAG = 700
QW = (28, 36, 36, 6, 2, 2, 2)
L4 = ([(96, 144, 0, 1100)], [])
L5 = ([(144, 208, 1100, 3500)], [(96, 128, 0, 1150), (128, 144, 1250, 2000), (144, 208, 2300, 4700)])
L6 = ([(208, 512, 0, 10000)], [(208, 256, 800, 2600), (256, 448, 2700, 10500)])
L7 = ([], [(448, 512, 0, 3000)])
A5K = ((96, 32), (128, 32))
A6K = ((160, 48), (208, 48), (256, 48), (304, 48))
A7K = ((352, 48), (400, 48), (448, 64))
WQ_PERM, WQ_FORM, ROUTE = (0, 3200), (3300, 8600), (4500, 5300)
R1T = 12800
MF = (128, 3420)

L_ORD = (2, 3, 0, 1, 4, 5, 6)
R_ORD = (2, 0, 6, 5, 1, 4, 3)

K_SEQ = (1, 4, 0, 2, 3, 5, 6)
K_SEQ2 = (0, 1, 2, 5, 3, 4, 6)
W_SEQ = (0, 1, 5, 6, 4, 2, 3)

NN = (((1,), (0,)), ((), ()))
TN = (((0,), (0,)), ((), ()))


SCOPES = False


def _scope(name):
    return jax.named_scope(name) if SCOPES else contextlib.nullcontext()


def _mo(v, m):
    return v if isinstance(v, int) else pl.multiple_of(v, m)


def _dot(a, b, dims):
    return lax.dot_general(a, b, dims, preferred_element_type=f32)


def _pack(v):
    return pltpu.bitcast(v.astype(bf16), u32)


def _unpack(v):
    return pltpu.bitcast(v, bf16)


def _combine(m):
    m1, m2, m3, m4, m5, m6, m7 = m
    return m1 + m4 - m5 + m7, m3 + m5, m2 + m4, m1 - m2 + m3 + m6


def _lform(a11, a12, a21, a22):
    return (a11 + a22, a21 + a22, a11, a22, a11 + a12, a21 - a11, a12 - a22)


def _rform(b11, b12, b21, b22):
    return (b11 + b22, b11, b12 - b22, b21 - b11, b22, b11 + b12, b21 + b22)


def _sform(x11, x12, x21, x22):
    return (x11, x22, x11 + x22, x21 + x22, x11 + x12, x21 - x11, x12 - x22)


def _wl(a11, a12, a21, a22):
    s1 = a21 + a22
    s2 = s1 - a11
    return (a11, a12, a12 - s2, a22, s1, s2, a11 - a21)


def _wr(b11, b12, b21, b22):
    t1 = b12 - b11
    t2 = b22 - t1
    return (b11, b21, b22, t2 - b21, t1, t2, b22 - b12)


def _wc(p):
    p1, p2, p3, p4, p5, p6, p7 = p
    u2 = p1 + p6
    u3 = u2 + p7
    return p1 + p2, (u2 + p5) + p3, u3 - p4, u3 + p5


W_R = (3, 1, 0, 2, 4, 5, 6)


def _wl_swapped(a11, a12, a21, a22):
    return _wl(a12, a11, a22, a21)


def _wc_swapped(p):
    p1, p2, p3, p4, p5, p6, p7 = p
    v2 = p1 + p6
    u3 = p7 - v2
    return (p5 - v2) + p3, p1 + p2, u3 + p5, p4 - u3


class _Sym:
    def __init__(self, t):
        self.t = t

    def __add__(self, o):
        return _Sym({**self.t, **o.t})

    def __sub__(self, o):
        return _Sym({**self.t, **{k: -v for k, v in o.t.items()}})


def _st(u, ct):
    return slice((4 * ct + u) * 128, (4 * ct + u + 1) * 128)


def _to_st(v):
    return jnp.concatenate([v[:, (2 * u + ct) * 128:(2 * u + ct + 1) * 128]
                            for ct in range(2) for u in range(4)], axis=1)


def _phi(t):
    return jnp.where(t > 0, t + 1.0, jnp.exp(t)) + 1e-6


def _rbf(v):
    return v.astype(bf16).astype(f32)


def _kernel(x_hbm, wqkv_hbm, wo_hbm, wr_hbm, wg_hbm, wu_hbm, wd_hbm, out_hbm,
            x_buf, wk_buf, wv_buf, wo_buf, wr_buf, wg_buf, wu_buf, wd_buf,
            xs1, xs2, wqs, sa, sb, zacc, zp, pk_buf, xb, yacc, rsel, wrb, zero_buf,
            wks, stats, wqt, ps_raw, qs, ms, tscr, tscr2, pq_raw, den_raw, pqb_buf, denb_buf, qsb,
            mg_raw, hb_raw, out_buf, idx_s, sem):
    wq_buf = out_buf.at[pl.ds(0, D), :]

    def xs_at(k1, e, rows=None):
        r = xs1.at[k1 * 4 + (0, 1, 7, 3).index(e)] if e in (0, 1, 7, 3) else xs2.at[k1 * 4 + (2, 4, 5, 6).index(e)]
        return r if rows is None else r.at[rows, :]

    SEM_B, SEM_O, SEM_Z, SEM_A = 0, 2, 3, 4

    def cp(src, dst, s):
        return pltpu.make_async_copy(src, dst, sem.at[s])

    def cp_x(r0, n, s):
        r = pl.ds(_mo(r0, 16), n)
        return [cp(x_hbm.at[:, r, :], x_buf.at[:, r, :], s)]

    def cp_wk(c, s):
        return [cp(wqkv_hbm.at[:, pl.ds(_mo(D + c * 256, 256), 256)],
                   wk_buf.at[c], s)]

    NX = T0 // X0
    SEM_W = SEM_A + NX
    cp_wr = cp(wr_hbm, wr_buf.at[pl.ds(0, D)], SEM_Z)
    a_groups = [cp_x(i * X0, X0, SEM_A + i) for i in range(NX)] + [
        cp_wk(0, SEM_W),
        cp_wk(1, SEM_W + 1),
        cp_wk(2, SEM_W + 2) + cp_x(T0, XG[0] - T0, SEM_W + 2),
        cp_wk(3, SEM_W + 3) + cp_x(XG[0], XG[1] - XG[0], SEM_W + 3),
        cp_x(XG[1], HQ - XG[1], SEM_W + 4),
        [cp(wqkv_hbm.at[:, pl.ds(0, D)], wq_buf, SEM_W + 5)],
    ]

    def cp_b(j, wait_only=False):
        dsts = [wg_buf.at[j], wu_buf.at[j], wd_buf.at[j]]
        for a in range(4):
            dsts += [wv_buf.at[j, :, pl.ds(a * 128, 128)], wo_buf.at[j, pl.ds(a * 128, 128), :]]
        if wait_only:
            return [cp(dst, dst, SEM_B + j) for dst in dsts]
        fs = pl.ds(j * FH, FH)
        srcs = [wg_hbm.at[:, fs], wu_hbm.at[:, fs], wd_hbm.at[fs, :]]
        for a in range(4):
            c0 = (2 * a + j) * 128
            srcs += [wqkv_hbm.at[:, pl.ds(2 * D + c0, 128)], wo_hbm.at[pl.ds(c0, 128), :]]
        return [cp(src, dst, SEM_B + j) for src, dst in zip(srcs, dsts)]

    clock = [0]
    toks = []
    sides = []
    fwd = [None]

    def emit_tok(vals, stamp):
        t = None
        for v in vals:
            v = pltpu.bitcast(v, u32) if v.dtype != u32 else v
            t = v if t is None else t | v
        toks.append((stamp, t & zero_buf[0]))

    def token(kind):
        t = fwd[0]
        if "u" not in t:
            t["u"] = pltpu.bitcast(t["src"](), u32) & zero_buf[0]
        if kind != "u" and "f" not in t:
            t["f"] = pltpu.bitcast(t["u"], f32)
        if kind == "f16" and "f16" not in t:
            t["f16"] = jnp.concatenate([t["f"], t["f"]], axis=0)
        return t[kind]

    def gate(v):
        if fwd[0] is None:
            return v
        head = v if v.shape[0] == 8 else v[0:8]
        head = head | token("u") if v.dtype == u32 else head + token("f")
        return head if v.shape[0] == 8 else jnp.concatenate([head, v[8:]], axis=0)

    def gate16(v):
        return v if fwd[0] is None else v + token("f16")

    def add_side(gen_fn, n, t0, t1, lag=None):
        st = {"i": 0, "n": n, "t0": clock[0] + t0, "t1": clock[0] + t1}

        def tok(vals):
            if lag is not None:
                emit_tok(vals, st["t0"] + (st["i"] + 1) * (st["t1"] - st["t0"]) // st["n"] + lag)
        st["g"] = gen_fn(tok)
        sides.append(st)

    def advance(until):
        for st in sides:
            while st["i"] < st["n"] and st["t0"] + st["i"] * (st["t1"] - st["t0"]) // st["n"] < until:
                next(st["g"], None)
                st["i"] += 1
                if st["i"] == st["n"]:
                    for _ in st["g"]:
                        pass

    def flush():
        for st in sides:
            for _ in st["g"]:
                pass
        sides.clear()

    def finish():
        flush()
        toks.clear()
        fwd[0] = None

    def mm(lhs, rhs, dims, cycles, nseg=1):
        due = [t for (c, t) in toks if c <= clock[0]]
        toks[:] = [(c, t) for (c, t) in toks if c > clock[0]]
        if due:
            head = rhs[0:8, 0:128]
            for t in due:
                head = head | t
            if rhs.shape[1] > 128:
                head = jnp.concatenate([head, rhs[0:8, 128:]], axis=1)
            rhs = jnp.concatenate([head, rhs[8:]], axis=0)
        res = _dot(lhs, _unpack(rhs), dims)
        ngr = res.shape[0] // 16
        for sg in range(nseg):
            for i in range(ngr):
                fwd[0] = {"src": lambda sg=sg, i=i: res[i * 16:i * 16 + 8, sg * 128:(sg + 1) * 128]}
                clock[0] += cycles // nseg // ngr
                advance(clock[0])
        return res

    def form_steps(form, form2, get, put, tok=None, keep=range(7)):
        terms = form(*[_Sym({i: 1}) for i in range(4)])
        gated = (0, 1, 2, 3) if 7 in keep else {_wl: (0, 1, 3), _wr: (0, 2, 3), _wl_swapped: (1, 2)}[form2]
        for k1 in range(7):
            sub = []
            for r in range(2):
                for c in range(2):
                    v = None
                    for i, sg in sorted(terms[k1].t.items(), key=lambda e: -e[1]):
                        b = get(r + 2 * (i // 2), c + 2 * (i % 2))
                        if v is None:
                            v = gate16(b) if 2 * r + c in gated else b
                        else:
                            v = v + b if sg > 0 else v - b
                    sub.append(v)
            vals = form2(*sub) + (sub[2],)
            for k2 in keep:
                put(k1, k2, _pack(vals[k2]))
            if tok is not None and k1 % 2 == 0:
                full = vals[3 if form2 is _wr else 2]
                tok([full[0:8], full[8:16]])
            yield

    def strassen2(lhs, rhs, dims, cycles, nseg=1, wts=(16,) * 7, comb=_wc):
        m1 = [None] * 7
        for i1, k1 in enumerate(K_SEQ2):
            m2 = [None] * 7
            for k2 in W_SEQ:
                m2[k2] = mm(lhs(k1, k2), rhs(k1, k2), dims, cycles * wts[i1] // 16, nseg)
                yield
            m1[k1] = comb(m2)
        out = [[None] * 4 for _ in range(4)]
        for s2 in range(4):
            for s1, v in enumerate(_combine([m1[k1][s2] for k1 in range(7)])):
                out[(s1 // 2) * 2 + s2 // 2][(s1 % 2) * 2 + s2 % 2] = v
        return out

    made = set()

    def need(*keys):
        assert all(k in made for k in keys), keys

    def row_views(base):
        if base == 0:
            return x_buf, sa, sb, stats, xn_buf, None
        i, n = base
        b = _mo(i * n, 16)
        return ([x_buf.at[:, pl.ds(b, n), :]] + [r.at[pl.ds(b, S - 128 + n), :] for r in (sa, sb, stats)]
                + [xn_buf.at[:, pl.ds(b, n), :], pl.ds(_mo(i * (n // 2), 8), n // 2)])

    def xs_form(r0, tok, which="all", base=0):
        xn_v, xs_v = row_views(base)[4:]
        rows = slice(r0 % XN, r0 % XN + 16)

        keep = {"all": range(8), "l1": (0, 1, 7, 3), "l2": (2, 4, 5, 6)}[which]
        for ct in range(2):
            def put(k1, k2, v):
                xs_at(k1, k2, xs_v)[r0 // 2:r0 // 2 + 8, ct * 128:(ct + 1) * 128] = v
            yield from form_steps(
                _sform, _wl, lambda q, u: xn_v[q, rows, _st(u, ct)], put, tok, keep)
        made.add(("xs", r0))

    def ln_stats(r_start, n_rows, tok, base=0):
        x_v, sa_v, sb_v, st_v, xn_v, _ = row_views(base)
        lane = lax.broadcasted_iota(i32, (8, 128), 1)
        for r0 in range(r_start, r_start + n_rows, 16):
            if r0 >= T0:
                need(("in", 2 + sum(r0 >= g for g in XG)))
            if r0 - XN >= T0:
                need(("ln", r0 - XN))
            for g in range(8):
                q, o = g // 2, (g % 2) * 8
                rg = q * HQ + r0 + o
                xv = x_v[q, r0 + o:r0 + o + 8, :].astype(f32)
                xg = jnp.concatenate([gate(xv[:, 0:128]), xv[:, 128:]], axis=1)
                mf = jnp.sum(xg, axis=1, keepdims=True) * (1.0 / D)
                d = xv - mf
                var = jnp.sum(d * d, axis=1, keepdims=True) * (1.0 / D)
                rs = lax.rsqrt(var + 1e-5)
                xn_v.at[q][r0 % XN + o:r0 % XN + o + 8, :] = _to_st(d * rs)
                rs = jnp.broadcast_to(rs, (8, 128))
                mf = jnp.broadcast_to(mf, (8, 128))
                sa_v[rg:rg + 8, :] = 1.0 + rs
                sb_v[rg:rg + 8, :] = mf * rs
                st_v[rg:rg + 8, 0:128] = jnp.where(lane == 0, mf, jnp.broadcast_to(var, (8, 128)))
                if tok is not None:
                    tok([rs])
                if g == 7:
                    made.add(("xn", r0))
                yield

    def ln_later(r_start, n_rows, tok, which="all", base=0):
        st_v, xn_v = row_views(base)[3:5]
        for r0 in range(r_start, r_start + n_rows, 16):
            need(("xn", r0))
            form = xs_form(r0, tok, which, base)
            for g in range(8):
                for _ in range(2 if g < 7 else 0):
                    next(form)
                    yield
                q, o = g // 2, (g % 2) * 8
                t = None
                if which != "l1":
                    v = xn_v[q, r0 % XN + o:r0 % XN + o + 8, :] * wrb[8:16, :]
                    for ct in range(8):
                        h = v[:, ct * 128:(ct + 1) * 128]
                        t = gate(h) if t is None else t + h
                if t is not None:
                    st_v[q * HQ + r0 + o:q * HQ + r0 + o + 8, 128:256] = t
                if tok is not None:
                    tok([t])
                if g == 7:
                    next(form, None)
                    made.add(("ln", r0))
                yield

    def wk_prep(c):
        if isinstance(c, int):
            need(("in", c))
        wks.at[c][:, 128:256] = pltpu.bitcast(wk_buf[c, 0:HD, 0:128], u32)
        wks.at[c][:, 512:640] = pltpu.bitcast(wk_buf[c, HD:D, 128:256], u32)
        for i in range(HD // 16):
            r0 = i * 16
            top = wk_buf[c, r0:r0 + 16, :].astype(f32)
            bot = wk_buf[c, HD + r0:HD + r0 + 16, :].astype(f32)
            ops = _rform(top[:, :128], top[:, 128:], bot[:, :128], bot[:, 128:])
            for k in (0, 2, 3, 5, 6):
                wks.at[c][r0 // 2:r0 // 2 + 8, k * 128:(k + 1) * 128] = _pack(ops[k])

    def wq_perm():
        need(("in", 5))

        def permute(kt):
            for g in range(8):
                tile = gate(pltpu.bitcast(wq_buf[kt * 128:(kt + 1) * 128, g * 128:(g + 1) * 128], u32))
                wqt.at[kt * 8 + g][...] = pltpu.bitcast(_unpack(tile).T, u32)
                yield

        def back(kt):
            for j in range(8):
                tile = gate(jnp.concatenate([wqt[kt * 8 + g, pl.ds(j, 8, stride=8), :] for g in range(8)],
                                            axis=0))
                v = pltpu.bitcast(_unpack(tile).T.astype(f32), u32)
                c0 = (kt // 2) * D + _st(j // 2, j % 2).start
                ps[(kt % 2) * 128:(kt % 2 + 1) * 128, c0:c0 + 128] = v
                made.add(("wqp", kt, j))
                yield

        order = (0, 2, 4, 6, 1, 3, 5, 7)
        for n in range(10):
            if n < 8:
                yield from permute(order[n])
            if n > 1:
                yield from back(order[n - 2])

    def wq_form():
        for i in range(16):
            need(*[("wqp", 2 * r + i // 8, j) for r in range(4) for j in range(8)])
            for ct in range(2):
                def put(k1, k2, v):
                    wqs.at[k1 * 7 + k2][i * 8:(i + 1) * 8, ct * 128:(ct + 1) * 128] = v
                yield from form_steps(
                    _rform, _wr, lambda r, c: pltpu.bitcast(
                        ps[i * 16:(i + 1) * 16, r * D + _st(c, ct).start:r * D + _st(c, ct).stop],
                        f32), put)

    def kproj(r0, n, chunks=range(4)):
        pr = pl.ds(r0 // 2, n // 2)
        need(*[("xs", r) for r in range(max(r0, T0), r0 + n, 16)])
        for c in chunks:
            m = [None] * 7
            for k in K_SEQ:
                e11, e12, e21, e22 = [xs_at(L_ORD[k], e)[pr, :] for e in (0, 1, 7, 3)]
                lhs = jnp.concatenate([jnp.concatenate([e11, e12], axis=1),
                                       jnp.concatenate([e21, e22], axis=1)], axis=0)
                m[k] = mm(_unpack(lhs), wks[c, :, k * 128:(k + 1) * 128], NN, 2 * n)
            kk = [_phi(v) for v in _combine(m)]
            for ct in range(2):
                zacc[:, pl.ds(_mo(c * 256 + ct * 128, 128), 128)] += (
                    (kk[ct] + kk[2 + ct]).reshape(n // 4, 8, 128).sum(axis=0))
            for s1 in range(4):
                for h in range(2):
                    pk_buf.at[s1 % 2, (s1 // 2) * 2 + h][r0:r0 + n, pl.ds(_mo(c * 128, 128), 128)] = (
                        kk[s1][h * n:(h + 1) * n])

    def z_prep():
        z = jnp.sum(zacc[...], axis=0, keepdims=True)
        zt = _pack(jnp.broadcast_to(z, (128, D)).astype(bf16).T)
        for g in range(8):
            tscr.at[g][...] = zt[g * 64:(g + 1) * 64, :]
        for j in range(8):
            blk = jnp.concatenate([tscr[g, pl.ds(j, 8, stride=8), :] for g in range(8)], axis=0)
            zp[:, j * 128:(j + 1) * 128] = _unpack(blk).T[0:8, :].astype(f32)

    def route():
        rows, dots = [None] * 16, [None] * 16
        for b in sorted(range(S // 128), key=lambda b: b % 4):
            need(*[("ln", r) for r in range(max(T0, b % 4 * 128), b % 4 * 128 + 128, 16)])
            rows[b] = gate(stats[b * 128:(b + 1) * 128, 0:128]).T[0:8, :]
            dots[b] = jnp.sum(gate(stats[b * 128:(b + 1) * 128, 128:256]).T, axis=0, keepdims=True)
            yield
        mf = jnp.concatenate([v[0:1] for v in rows], axis=0)
        var = jnp.concatenate([v[1:2] for v in rows], axis=0)
        tr = jnp.concatenate(dots, axis=0) * jnp.sqrt(var + 1e-5)
        wsum = jnp.sum(wrb[0:1, :], axis=1, keepdims=True)
        mb = _rbf(mf)
        inv = 1.0 / _rbf(jnp.sqrt(_rbf(_rbf(var) + 1e-5)))
        rv = _rbf((tr + (mf - mb) * wsum) * inv)
        rmax = jnp.max(jnp.max(rv, axis=1, keepdims=True), axis=0, keepdims=True)
        pos = (lax.broadcasted_iota(i32, rv.shape, 0) * 128 + lax.broadcasted_iota(i32, rv.shape, 1))
        idx = jnp.min(jnp.where(rv == rmax, pos, S - 1))
        idx_s[0] = idx

        def pick(v):
            v = jnp.sum(jnp.where(pos == idx, v, 0.0), axis=1, keepdims=True)
            return jnp.sum(v, axis=0, keepdims=True)

        xv = x_buf[(idx >> 9) & 3, pl.ds(_mo(idx & (HQ - 16), 16), 16), :].astype(f32)
        sel = lax.broadcasted_iota(i32, xv.shape, 0) == (idx & 15)
        row = jnp.sum(jnp.where(sel, xv, 0.0), axis=0, keepdims=True)
        row = _rbf(_rbf(row - pick(mb)) * pick(inv))
        rsel[...] = jnp.broadcast_to(_rbf(jnp.sum(row * wrb[0:1, :], axis=1, keepdims=True)), rsel.shape)
        xb[...] = jnp.broadcast_to(row, (128, D)).T
        yield

    def ps_form(j):
        for c in range(HQ // 16):
            def put(k1, k2, v):
                k = k1 * 7 + k2
                ps[c * 8:(c + 1) * 8, k * 128:(k + 1) * 128] = v
            yield from form_steps(
                _lform, _wl_swapped,
                lambda r, q: pk_buf[j, q, c * 16:(c + 1) * 16, r * 128:(r + 1) * 128], put)

    def q_rows(j, r0, n, pq, rc, d0, rec):
        xj = pl.ds(_mo(j * (BQ // 2), BQ // 2), BQ // 2)
        pr = slice(r0 // 2, (r0 + n) // 2)
        blk = yield from strassen2(lambda k1, k2: _unpack(xs_at(L_ORD[k1], k2, xj)[pr, :]),
                                   lambda k1, k2: wqs[k1 * 7 + k2], NN, n, 1, QW)
        lane = lax.broadcasted_iota(i32, (n, 128), 1)
        for q in range(4):
            d = None
            for u in (3, 2, 1, 0):
                v = _phi(blk[q][u])
                for ct in range(2):
                    pq.at[q][d0:d0 + n, _st(u, ct)] = v[:, ct * 128:(ct + 1) * 128]
                t = v * zp[0:1, u * 256:(u + 1) * 256]
                t = t[:, :128] + t[:, 128:]
                d = t if d is None else d + t
            if rec:
                d = recip(d, lane)
            rc.at[q][d0:d0 + n, :] = d

    def recip(d, lane):
        d = d + jnp.where(lane % 2 == 0, pltpu.roll(d, 127, 1), pltpu.roll(d, 1, 1))
        d = d + jnp.where(lane % 4 < 2, pltpu.roll(d, 126, 1), pltpu.roll(d, 2, 1))
        return 1.0 / (d + 1e-6)

    def normalise(pq, rc, nr, dst, p0, raw, tok=None):
        lane = lax.broadcasted_iota(i32, (16, 128), 1)

        def fix(c):
            if c < nr // 16 and raw(c * 16):
                for q in range(4):
                    rq = slice(c * 16, (c + 1) * 16)
                    rc.at[q][rq, :] = recip(gate16(rc[q, rq, :]), lane)

        def scale(c):
            rq = slice(c * 16, (c + 1) * 16)
            fix(c + 1)
            for hf in range(2):
                for q in range(4):
                    cs = slice(hf * HD, (hf + 1) * HD)
                    pq.at[q][rq, cs] = pq[q, rq, cs] * jnp.concatenate([gate16(rc[q, rq, :])] * 4, axis=1)
                    yield

        def form(c):
            rq = slice(c * 16, (c + 1) * 16)
            p2 = pl.ds(_mo(p0 + c * 8, 8), 8)
            for ct in range(2):
                def put(k1, k2, v):
                    dst.at[k1 * 7 + k2][p2, ct * 128:(ct + 1) * 128] = v
                yield from form_steps(_lform, _wl, lambda q, u: pq[q, rq, _st(u, ct)], put, tok)

        fix(0)
        if raw(0):
            for _ in range(4):
                yield
        yield from scale(0)
        for c in range(nr // 16):
            nxt = scale(c + 1) if c + 1 < nr // 16 else iter(())
            for i, _ in enumerate(form(c)):
                yield
                if i < 8 and c + 1 < nr // 16:
                    next(nxt)
                    yield

    def g_kvm(j):
        blk = yield from strassen2(
            lambda k1, k2: _unpack(ps[:, (k1 * 7 + k2) * 128:(k1 * 7 + k2 + 1) * 128]),
            lambda k1, k2: xs_at(R_ORD[k1], W_R[k2])[...], TN, 256, 2, comb=_wc_swapped)
        hm = (lax.broadcasted_iota(i32, (128, 128), 0) // 32
              == lax.broadcasted_iota(i32, (128, 128), 1) // 32)
        qb = q_rows(j, BQ - QB, QB, pqb_buf.at[j], denb_buf.at[j], 0, False)
        for _ in range(QSPLIT):
            next(qb)
        kvps = []
        for a in (3, 2, 1, 0):
            gg = jnp.concatenate(blk[a], axis=1).astype(bf16)
            wv_u = pltpu.bitcast(wv_buf[j, :, a * 128:(a + 1) * 128], u32)
            kv = jnp.where(hm, mm(gg, wv_u, NN, 256), 0.0)
            tscr2.at[a][...] = _pack(kv)
            kvps.append(_unpack(jnp.concatenate(
                [tscr2[a, pl.ds(jj, 8, stride=8), :] for jj in range(8)], axis=0)))

        def m_form():
            for a in (3, 2, 1, 0):
                need(("mg", a))
                for jl in range(2):
                    for ct in range(2):
                        def put(k1, k2, v):
                            ms.at[k1 * 7 + k2][pl.ds(_mo(jl * 64 + (2 * a + j) * 8, 8), 8),
                                               ct * 128:(ct + 1) * 128] = v
                        yield from form_steps(
                            _rform, _wr, lambda q, u: mg_buf[a, (2 * q + jl) * 16:(2 * q + jl + 1) * 16, _st(u, ct)], put)

        for i, a in enumerate((3, 2, 1, 0)):
            wo_u = pltpu.bitcast(wo_buf[j, a * 128:(a + 1) * 128, :], u32)
            res = mm(kvps[i], wo_u, NN, 256)
            mg_buf.at[a][...] = _to_st(res)
            made.add(("mg", a))
            if i == 0:
                add_side(lambda tok: m_form(), 112, *MF)
        for _ in qb:
            pass

    def out_part(base, span, off, nr, y, src):
        b = _mo(base, 32)
        sa_v, sb_v, out_v = [r.at[pl.ds(b, 3 * HQ + span), :] for r in (sa, sb, out_buf)]
        x_v = x_buf.at[:, pl.ds(b, span), :]
        row = lax.broadcasted_iota(i32, (nr, 256), 0) + (base + off)
        blk = yield from strassen2(lambda k1, k2: _unpack(src[k1 * 7 + k2, off // 2:(off + nr) // 2, :]),
                                   lambda k1, k2: ms[k1 * 7 + k2], NN, nr)
        for s1 in (3, 2, 1, 0):
            for s2 in range(4):
                q = (s1 // 2) * 2 + s2 // 2
                u = (s1 % 2) * 2 + s2 % 2
                rr, cc = pl.ds(q * HQ + off, nr), pl.ds(u * 256, 256)
                a = jnp.concatenate([sa_v[rr, :]] * 2, axis=1)
                c = jnp.concatenate([sb_v[rr, :]] * 2, axis=1)
                o = blk[q][u] + jnp.where(row + q * HQ == idx_s[0], y[:, u * 256:(u + 1) * 256], 0.0)
                out_v[rr, cc] = (x_v[q, off:off + nr, cc].astype(f32) * a - c + o).astype(bf16)
                if s2 % 2 == 1:
                    ch = pl.ds((s1 % 2) * HD, HD)
                    ro = pl.ds(_mo(base + q * HQ + off, 16), nr)
                    cp(out_buf.at[ro, ch], out_hbm.at[0, ro, ch], SEM_O).start()

    def ffn_part(j):
        def fma(acc, w, v):
            p = w.astype(f32) * v
            return acc + p[0:8] + p[8:16]

        for f0 in range(0, FH, 256):
            fs = slice(f0, f0 + 256)
            ag = jnp.zeros((8, 256), f32)
            au = jnp.zeros((8, 256), f32)
            for k in range(0, D, 16):
                xv = jnp.concatenate([gate16(xb[k:k + 16, :])] * 2, axis=1)
                ag = fma(ag, wg_buf[j, k:k + 16, fs], xv)
                au = fma(au, wu_buf[j, k:k + 16, fs], xv)
                yield
            g = _rbf(jnp.sum(ag, axis=0, keepdims=True))
            u = _rbf(jnp.sum(au, axis=0, keepdims=True))
            h = _rbf(_rbf(g * jax.nn.sigmoid(g)) * u)
            hb_buf[fs, :] = jnp.broadcast_to(h, (128, 256)).T
        for d0 in range(0, D, 512):
            ds_ = slice(d0, d0 + 512)
            acc = yacc[:, ds_]
            for k in range(0, FH, 16):
                hv = jnp.concatenate([gate16(hb_buf[k:k + 16, :])] * 4, axis=1)
                acc = fma(acc, wd_buf[j, k:k + 16, ds_], hv)
                yield
            yacc[:, ds_] = acc

    def wait_group(i):
        with _scope("a_wait%d" % i):
            for c in a_groups[i]:
                c.wait()
        made.add(("in", i - NX))

    def run_all(gen):
        for _ in gen:
            pass

    def ln_sides(plan):
        for r0, r1, t0, t1 in plan[0]:
            add_side(lambda tok, r0=r0, r1=r1: ln_stats(r0, r1 - r0, tok), (r1 - r0) // 2, t0, t1, LNLAG)
        for r0, r1, t0, t1 in plan[1]:
            add_side(lambda tok, r0=r0, r1=r1: ln_later(r0, r1 - r0, tok), 22 * (r1 - r0) // 16, t0, t1, SLAG)

    def l2_side(base, n, t0, t1):
        add_side(lambda tok: ln_later(0, n, None, "l2", base), 22 * n // 16, t0, t1)

    with _scope("p0_issue"):
        cp_wr.start()
        for grp in a_groups:
            for c in grp:
                c.start()
        for j in range(2):
            for c in cp_b(j):
                c.start()
        zacc[...] = jnp.zeros(zacc.shape, f32)
        yacc[...] = jnp.zeros(yacc.shape, f32)
        zero_buf[1] = jnp.zeros((8, 128), u32)
        cp_zero = cp(zero_buf.at[1], zero_buf.at[0], SEM_Z)
        cp_zero.start()
        cp_zero.wait()
        cp_wr.wait()
        wr8 = jnp.broadcast_to(wr_buf[0:D].reshape(1, D).astype(f32), (8, D))
        wrb[0:8, :] = wr8
        wrb[8:16, :] = _to_st(wr8)
        z0 = jnp.max(pltpu.bitcast(zero_buf[0], i32))
        ps, pq_buf, den_buf, mg_buf, hb_buf = [r.at[z0] for r in (ps_raw, pq_raw, den_raw, mg_raw, hb_raw)]
        xn_buf = mg_buf

    def a01(i, carry):
        with _scope("a_wait01"):
            for c in cp_x(i * X0, X0, SEM_A + i):
                c.wait()
        with _scope("a01"):
            for r in range(0, X0, 16):
                run_all(ln_stats(r, 16, None, (i, X0)))
                if r:
                    run_all(ln_later(r - 16, 16, None, "l1", (i, X0)))
            run_all(ln_later(X0 - 16, 16, None, "l1", (i, X0)))
        return carry

    lax.fori_loop(0, NX, a01, 0)
    made.update(("xn", r) for r in range(0, 64, 16))

    def a23(i, carry):
        with _scope("a_wait23"):
            for c in cp_wk(i, SEM_W + i):
                c.wait()
        with _scope("a23"):
            wk_prep(i)
            l2_side((i, T0 // 2), T0 // 2, 250, 14 * T0 - 250)
            kproj(0, T0, [i])
            finish()
        return carry

    lax.fori_loop(0, 2, a23, 0)
    wait_group(NX + 2)
    with _scope("a4"):
        wk_prep(2)
        ln_sides(L4)
        kproj(0, T0, [2])
        finish()
    wait_group(NX + 3)
    with _scope("a5"):
        wk_prep(3)
        ln_sides(L5)
        kproj(0, T0, [3])
        for r0, n in A5K:
            kproj(r0, n)
        finish()
    wait_group(NX + 4)
    with _scope("a6"):
        ln_sides(L6)
        for r0, n in A6K:
            kproj(r0, n)
        finish()
    wait_group(NX + 5)
    with _scope("a7"):
        ln_sides(L7)
        add_side(lambda tok: wq_perm(), 128, *WQ_PERM)
        add_side(lambda tok: wq_form(), 224, *WQ_FORM)
        add_side(lambda tok: route(), 17, *ROUTE)
        for r0, n in A7K:
            kproj(r0, n)
        finish()

    def b_body(j, carry):
        qa = BQ - QB
        with _scope("b_r0"):
            z_prep()
            add_side(lambda tok: ps_form(j), 7 * HQ // 16, 0, 49 * qa - 400)
            for r0 in range(0, qa, QN):
                run_all(q_rows(j, r0, QN, pq_buf, den_buf, r0, r0 + QN < qa))
            finish()
        with _scope("b_wait"):
            for c in cp_b(j, wait_only=True):
                c.wait()
        with _scope("b_r1"):
            add_side(lambda tok: ffn_part(j), FH * 3 // 8, 0, R1T)
            add_side(lambda tok: normalise(pq_buf, den_buf, qa, qs, j * (qa // 2), lambda r: r >= qa - QN),
                     22 * (qa // 16), 0, R1T)
            run_all(g_kvm(j))
            finish()
        return carry

    lax.fori_loop(0, 2, b_body, 0)

    def c_body(t, carry):
        with _scope("c_body"):
            y = _rbf(jnp.sum(yacc[...], axis=0, keepdims=True))
            y = _rbf(y * _rbf(1.0 / _rbf(1.0 + _rbf(jnp.exp(-rsel[0:1, :])))))
            j, h = t >> 1, t & 1
            na, nb = (BQ - QB) // 2, QB // 2
            hb = pl.ds(_mo(h * nb, 16), nb)
            add_side(lambda tok: normalise(pqb_buf.at[j, :, hb, :], denb_buf.at[j, :, hb, :], nb, qsb, 0,
                                           lambda r: True, tok),
                     4 + 22 * (nb // 16), 0, 49 * na - 800, SLAG)
            qs_t = qs.at[:, pl.ds(_mo(t * (na // 2), 16), na // 2), :]
            for p in range(0, na, CR):
                run_all(out_part(j * BQ + h * na, na, p, CR, y, qs_t))
            flush()
            run_all(out_part(j * BQ + BQ - QB + h * nb, nb, 0, nb, y, qsb))
            finish()
        return carry

    lax.fori_loop(0, 4, c_body, 0)
    with _scope("tail"):
        cp(out_buf, out_hbm.at[0], SEM_O).wait()


@jax.jit
def pallas_parallel_sum__linear_attn_block__moe_arch_mod__prompt_kernel(
    A_x: jax.Array,
    A_wqkv: jax.Array,
    A_wo: jax.Array,
    B_x: jax.Array,
    B_w_r: jax.Array,
    B_w_gate: jax.Array,
    B_w_up: jax.Array,
    B_w_down: jax.Array,
):
    del B_x
    V = pltpu.VMEM
    scratch = [
        V((4, HQ, D), bf16),
        V((4, D, 256), bf16),
        V((2, D, 512), bf16),
        V((2, 512, D), bf16),
        V((8 * D,), bf16),
        V((2, D, FH), bf16),
        V((2, D, FH), bf16),
        V((2, FH, D), bf16),
        V((28, HQ // 2, 256), u32),
        V((28, HQ // 2, 256), u32),
        V((49, 128, 256), u32),
        V((S, 128), f32),
        V((S, 128), f32),
        V((8, D), f32),
        V((8, D), f32),
        V((2, 4, HQ, 512), f32),
        V((D, 128), f32),
        V((8, D), f32),
        V((8, D), f32),
        V((16, D), f32),
        V((4, 8, 128), u32),
        V((4, HD // 2, 7 * 128), u32),
        V((S, 256), f32),
        V((64, 64, 128), u32),
        V((1, HQ // 2, 49 * 128), u32),
        V((49, BQ - QB, 256), u32),
        V((49, 128, 256), u32),
        V((8, 64, 128), u32),
        V((4, 64, 128), u32),
        V((1, 4, BQ - QB, D), f32),
        V((1, 4, BQ - QB, 128), f32),
        V((2, 4, QB, D), f32),
        V((2, 4, QB, 128), f32),
        V((49, QB // 4, 256), u32),
        V((1, 4, 128, D), f32),
        V((1, FH, 128), f32),
        V((S, D), bf16),
        pltpu.SMEM((1,), i32),
        pltpu.SemaphoreType.DMA((4 + T0 // X0 + 6,)),
    ]
    extra = {k: True for k in ("disable_bounds_checks", "disable_semaphore_checks")
             if hasattr(pltpu.CompilerParams, k)}
    return pl.pallas_call(
        _kernel,
        out_shape=jax.ShapeDtypeStruct((1, S, D), bf16),
        in_specs=[pl.BlockSpec(memory_space=pl.ANY)] * 7,
        out_specs=pl.BlockSpec(memory_space=pl.ANY),
        scratch_shapes=scratch,
        compiler_params=pltpu.CompilerParams(vmem_limit_bytes=120 * 1024 * 1024, **extra),
    )(A_x.reshape(4, HQ, D), A_wqkv, A_wo, B_w_r, B_w_gate, B_w_up, B_w_down)
```

```python
import contextlib

import jax
import jax.numpy as jnp
from jax import lax
import jax.experimental.pallas as pl
import jax.experimental.pallas.tpu as pltpu

bf16, f32, u32, i32 = jnp.bfloat16, jnp.float32, jnp.uint32, jnp.int32

S = 2048
D = 1024
F = 3584
HD = D // 2
HQ = S // 4
BQ = HQ // 2
FH = F // 2
QB = 64
QN = 48
QPRE = 3
QSPLIT = 6
CR = 48
T0 = 96
X0 = 32
XG = (160, 208)
XN = 128

SLAG = 400
LNLAG = 700
QW = (28, 36, 36, 6, 2, 2, 2)
L4 = ([(96, 144, 0, 1100)], [])
L5 = ([(144, 208, 1100, 3500)], [(96, 128, 300, 1250), (128, 144, 1300, 2000), (144, 208, 2300, 4700)])
L6 = ([(208, 512, 0, 10000)], [(208, 256, 800, 2600), (256, 448, 2700, 10500)])
L7 = ([], [(448, 512, 0, 3000)])
A5K = ((96, 32), (128, 32))
A6K = ((160, 48), (208, 48), (256, 48), (304, 48))
A7K = ((352, 48), (400, 48), (448, 64))
WQ_PERM, WQ_FORM, ROUTE = (0, 3200), (3300, 8600), (4500, 5300)
R1T = 12800
MF = (128, 3420)

L_ORD = (2, 3, 0, 1, 4, 5, 6)
R_ORD = (2, 0, 6, 5, 1, 4, 3)

K_SEQ = (1, 4, 0, 2, 3, 5, 6)
K_SEQ2 = (0, 1, 2, 5, 3, 4, 6)
W_SEQ = (0, 1, 5, 6, 4, 2, 3)

NN = (((1,), (0,)), ((), ()))
TN = (((0,), (0,)), ((), ()))


SCOPES = False


def _scope(name):
    return jax.named_scope(name) if SCOPES else contextlib.nullcontext()


def _mo(v, m):
    return v if isinstance(v, int) else pl.multiple_of(v, m)


def _dot(a, b, dims):
    return lax.dot_general(a, b, dims, preferred_element_type=f32)


def _pack(v):
    return pltpu.bitcast(v.astype(bf16), u32)


def _unpack(v):
    return pltpu.bitcast(v, bf16)


def _combine(m):
    m1, m2, m3, m4, m5, m6, m7 = m
    return m1 + m4 - m5 + m7, m3 + m5, m2 + m4, m1 - m2 + m3 + m6


def _lform(a11, a12, a21, a22):
    return (a11 + a22, a21 + a22, a11, a22, a11 + a12, a21 - a11, a12 - a22)


def _rform(b11, b12, b21, b22):
    return (b11 + b22, b11, b12 - b22, b21 - b11, b22, b11 + b12, b21 + b22)


def _sform(x11, x12, x21, x22):
    return (x11, x22, x11 + x22, x21 + x22, x11 + x12, x21 - x11, x12 - x22)


def _wl(a11, a12, a21, a22):
    s1 = a21 + a22
    s2 = s1 - a11
    return (a11, a12, a12 - s2, a22, s1, s2, a11 - a21)


def _wr(b11, b12, b21, b22):
    t1 = b12 - b11
    t2 = b22 - t1
    return (b11, b21, b22, t2 - b21, t1, t2, b22 - b12)


def _wc(p):
    p1, p2, p3, p4, p5, p6, p7 = p
    u2 = p1 + p6
    u3 = u2 + p7
    return p1 + p2, (u2 + p5) + p3, u3 - p4, u3 + p5


W_R = (3, 1, 0, 2, 4, 5, 6)


def _wl_swapped(a11, a12, a21, a22):
    return _wl(a12, a11, a22, a21)


def _wc_swapped(p):
    p1, p2, p3, p4, p5, p6, p7 = p
    v2 = p1 + p6
    u3 = p7 - v2
    return (p5 - v2) + p3, p1 + p2, u3 + p5, p4 - u3


class _Sym:
    def __init__(self, t):
        self.t = t

    def __add__(self, o):
        return _Sym({**self.t, **o.t})

    def __sub__(self, o):
        return _Sym({**self.t, **{k: -v for k, v in o.t.items()}})


def _st(u, ct):
    return slice((4 * ct + u) * 128, (4 * ct + u + 1) * 128)


def _to_st(v):
    return jnp.concatenate([v[:, (2 * u + ct) * 128:(2 * u + ct + 1) * 128]
                            for ct in range(2) for u in range(4)], axis=1)


def _phi(t):
    return jnp.where(t > 0, t + 1.0, jnp.exp(t)) + 1e-6


def _rbf(v):
    return v.astype(bf16).astype(f32)


def _kernel(x_hbm, wqkv_hbm, wo_hbm, wr_hbm, wg_hbm, wu_hbm, wd_hbm, out_hbm,
            x_buf, wk_buf, wv_buf, wo_buf, wr_buf, wg_buf, wu_buf, wd_buf,
            xs1, xs2, wqs, sa, sb, zacc, zp, pk_buf, xb, yacc, rsel, wrb, zero_buf,
            wks, stats, wqt, ps_raw, qs, ms, tscr, tscr2, pq_raw, den_raw, pqb_buf, denb_buf, qsb,
            mg_raw, hb_raw, out_buf, idx_s, sem):
    wq_buf = out_buf.at[pl.ds(0, D), :]

    def xs_at(k1, e, rows=None):
        r = xs1.at[k1 * 4 + (0, 1, 7, 3).index(e)] if e in (0, 1, 7, 3) else xs2.at[k1 * 4 + (2, 4, 5, 6).index(e)]
        return r if rows is None else r.at[rows, :]

    SEM_B, SEM_O, SEM_Z, SEM_A = 0, 2, 3, 4

    def cp(src, dst, s):
        return pltpu.make_async_copy(src, dst, sem.at[s])

    def cp_x(r0, n, s):
        r = pl.ds(_mo(r0, 16), n)
        return [cp(x_hbm.at[:, r, :], x_buf.at[:, r, :], s)]

    def cp_wk(c, s):
        return [cp(wqkv_hbm.at[:, pl.ds(_mo(D + c * 256, 256), 256)],
                   wk_buf.at[c], s)]

    NX = T0 // X0
    SEM_W = SEM_A + NX
    cp_wr = cp(wr_hbm, wr_buf.at[pl.ds(0, D)], SEM_Z)
    a_groups = [cp_x(i * X0, X0, SEM_A + i) for i in range(NX)] + [
        cp_wk(0, SEM_W),
        cp_wk(1, SEM_W + 1),
        cp_wk(2, SEM_W + 2) + cp_x(T0, XG[0] - T0, SEM_W + 2),
        cp_wk(3, SEM_W + 3) + cp_x(XG[0], XG[1] - XG[0], SEM_W + 3),
        cp_x(XG[1], HQ - XG[1], SEM_W + 4),
        [cp(wqkv_hbm.at[:, pl.ds(0, D)], wq_buf, SEM_W + 5)],
    ]

    def cp_b(j, wait_only=False):
        dsts = [wg_buf.at[j], wu_buf.at[j], wd_buf.at[j]]
        for a in range(4):
            dsts += [wv_buf.at[j, :, pl.ds(a * 128, 128)], wo_buf.at[j, pl.ds(a * 128, 128), :]]
        if wait_only:
            return [cp(dst, dst, SEM_B + j) for dst in dsts]
        fs = pl.ds(j * FH, FH)
        srcs = [wg_hbm.at[:, fs], wu_hbm.at[:, fs], wd_hbm.at[fs, :]]
        for a in range(4):
            c0 = (2 * a + j) * 128
            srcs += [wqkv_hbm.at[:, pl.ds(2 * D + c0, 128)], wo_hbm.at[pl.ds(c0, 128), :]]
        return [cp(src, dst, SEM_B + j) for src, dst in zip(srcs, dsts)]

    clock = [0]
    toks = []
    sides = []
    fwd = [None]

    def emit_tok(vals, stamp):
        t = None
        for v in vals:
            v = pltpu.bitcast(v, u32) if v.dtype != u32 else v
            t = v if t is None else t | v
        toks.append((stamp, t & zero_buf[0]))

    def token(kind):
        t = fwd[0]
        if "u" not in t:
            t["u"] = pltpu.bitcast(t["src"](), u32) & zero_buf[0]
        if kind != "u" and "f" not in t:
            t["f"] = pltpu.bitcast(t["u"], f32)
        if kind == "f16" and "f16" not in t:
            t["f16"] = jnp.concatenate([t["f"], t["f"]], axis=0)
        return t[kind]

    def gate(v):
        if fwd[0] is None:
            return v
        head = v if v.shape[0] == 8 else v[0:8]
        head = head | token("u") if v.dtype == u32 else head + token("f")
        return head if v.shape[0] == 8 else jnp.concatenate([head, v[8:]], axis=0)

    def gate16(v):
        return v if fwd[0] is None else v + token("f16")

    def add_side(gen_fn, n, t0, t1, lag=None):
        st = {"i": 0, "n": n, "t0": clock[0] + t0, "t1": clock[0] + t1}

        def tok(vals):
            if lag is not None:
                emit_tok(vals, st["t0"] + (st["i"] + 1) * (st["t1"] - st["t0"]) // st["n"] + lag)
        st["g"] = gen_fn(tok)
        sides.append(st)

    def advance(until):
        for st in sides:
            while st["i"] < st["n"] and st["t0"] + st["i"] * (st["t1"] - st["t0"]) // st["n"] < until:
                next(st["g"], None)
                st["i"] += 1
                if st["i"] == st["n"]:
                    for _ in st["g"]:
                        pass

    def flush():
        for st in sides:
            for _ in st["g"]:
                pass
        sides.clear()

    def finish():
        flush()
        toks.clear()
        fwd[0] = None

    def mm(lhs, rhs, dims, cycles, nseg=1):
        due = [t for (c, t) in toks if c <= clock[0]]
        toks[:] = [(c, t) for (c, t) in toks if c > clock[0]]
        if due:
            head = rhs[0:8, 0:128]
            for t in due:
                head = head | t
            if rhs.shape[1] > 128:
                head = jnp.concatenate([head, rhs[0:8, 128:]], axis=1)
            rhs = jnp.concatenate([head, rhs[8:]], axis=0)
        res = _dot(lhs, _unpack(rhs), dims)
        ngr = res.shape[0] // 16
        for sg in range(nseg):
            for i in range(ngr):
                fwd[0] = {"src": lambda sg=sg, i=i: res[i * 16:i * 16 + 8, sg * 128:(sg + 1) * 128]}
                clock[0] += cycles // nseg // ngr
                advance(clock[0])
        return res

    def form_steps(form, form2, get, put, tok=None, keep=range(7)):
        terms = form(*[_Sym({i: 1}) for i in range(4)])
        gated = (0, 1, 2, 3) if 7 in keep else {_wl: (0, 1, 3), _wr: (0, 2, 3), _wl_swapped: (1, 2)}[form2]
        for k1 in range(7):
            sub = []
            for r in range(2):
                for c in range(2):
                    v = None
                    for i, sg in sorted(terms[k1].t.items(), key=lambda e: -e[1]):
                        b = get(r + 2 * (i // 2), c + 2 * (i % 2))
                        if v is None:
                            v = gate16(b) if 2 * r + c in gated else b
                        else:
                            v = v + b if sg > 0 else v - b
                    sub.append(v)
            vals = form2(*sub) + (sub[2],)
            for k2 in keep:
                put(k1, k2, _pack(vals[k2]))
            if tok is not None and k1 % 2 == 0:
                full = vals[3 if form2 is _wr else 2]
                tok([full[0:8], full[8:16]])
            yield

    def strassen2(lhs, rhs, dims, cycles, nseg=1, wts=(16,) * 7, comb=_wc):
        m1 = [None] * 7
        for i1, k1 in enumerate(K_SEQ2):
            m2 = [None] * 7
            for k2 in W_SEQ:
                m2[k2] = mm(lhs(k1, k2), rhs(k1, k2), dims, cycles * wts[i1] // 16, nseg)
                yield
            m1[k1] = comb(m2)
        out = [[None] * 4 for _ in range(4)]
        for s2 in range(4):
            for s1, v in enumerate(_combine([m1[k1][s2] for k1 in range(7)])):
                out[(s1 // 2) * 2 + s2 // 2][(s1 % 2) * 2 + s2 % 2] = v
        return out

    made = set()

    def need(*keys):
        assert all(k in made for k in keys), keys

    def row_views(base):
        if base == 0:
            return x_buf, sa, sb, stats, xn_buf, None
        i, n = base
        b = _mo(i * n, 16)
        return ([x_buf.at[:, pl.ds(b, n), :]] + [r.at[pl.ds(b, S - 128 + n), :] for r in (sa, sb, stats)]
                + [xn_buf.at[:, pl.ds(b, n), :], pl.ds(_mo(i * (n // 2), 8), n // 2)])

    def xs_form(r0, tok, which="all", base=0):
        xn_v, xs_v = row_views(base)[4:]
        rows = slice(r0 % XN, r0 % XN + 16)

        keep = {"all": range(8), "l1": (0, 1, 7, 3), "l2": (2, 4, 5, 6)}[which]
        for ct in range(2):
            def put(k1, k2, v):
                xs_at(k1, k2, xs_v)[r0 // 2:r0 // 2 + 8, ct * 128:(ct + 1) * 128] = v
            yield from form_steps(
                _sform, _wl, lambda q, u: xn_v[q, rows, _st(u, ct)], put, tok, keep)
        made.add(("xs", r0))

    def ln_stats(r_start, n_rows, tok, base=0):
        x_v, sa_v, sb_v, st_v, xn_v, _ = row_views(base)
        lane = lax.broadcasted_iota(i32, (8, 128), 1)
        for r0 in range(r_start, r_start + n_rows, 16):
            if r0 >= T0:
                need(("in", 2 + sum(r0 >= g for g in XG)))
            if r0 - XN >= T0:
                need(("ln", r0 - XN))
            for g in range(8):
                q, o = g // 2, (g % 2) * 8
                rg = q * HQ + r0 + o
                xv = x_v[q, r0 + o:r0 + o + 8, :].astype(f32)
                xg = jnp.concatenate([gate(xv[:, 0:128]), xv[:, 128:]], axis=1)
                mf = jnp.sum(xg, axis=1, keepdims=True) * (1.0 / D)
                d = xv - mf
                var = jnp.sum(d * d, axis=1, keepdims=True) * (1.0 / D)
                rs = lax.rsqrt(var + 1e-5)
                xn_v.at[q][r0 % XN + o:r0 % XN + o + 8, :] = _to_st(d * rs)
                rs = jnp.broadcast_to(rs, (8, 128))
                mf = jnp.broadcast_to(mf, (8, 128))
                sa_v[rg:rg + 8, :] = 1.0 + rs
                sb_v[rg:rg + 8, :] = mf * rs
                st_v[rg:rg + 8, 0:128] = jnp.where(lane == 0, mf, jnp.broadcast_to(var, (8, 128)))
                if tok is not None:
                    tok([rs])
                if g == 7:
                    made.add(("xn", r0))
                yield

    def ln_later(r_start, n_rows, tok, which="all", base=0):
        st_v, xn_v = row_views(base)[3:5]
        for r0 in range(r_start, r_start + n_rows, 16):
            need(("xn", r0))
            form = xs_form(r0, tok, which, base)
            for g in range(8):
                for _ in range(2 if g < 7 else 0):
                    next(form)
                    yield
                q, o = g // 2, (g % 2) * 8
                t = None
                if which != "l1":
                    v = xn_v[q, r0 % XN + o:r0 % XN + o + 8, :] * wrb[8:16, :]
                    for ct in range(8):
                        h = v[:, ct * 128:(ct + 1) * 128]
                        t = gate(h) if t is None else t + h
                if t is not None:
                    st_v[q * HQ + r0 + o:q * HQ + r0 + o + 8, 128:256] = t
                if tok is not None:
                    tok([t])
                if g == 7:
                    next(form, None)
                    made.add(("ln", r0))
                yield

    def wk_prep(c):
        if isinstance(c, int):
            need(("in", c))
        wks.at[c][:, 128:256] = pltpu.bitcast(wk_buf[c, 0:HD, 0:128], u32)
        wks.at[c][:, 512:640] = pltpu.bitcast(wk_buf[c, HD:D, 128:256], u32)
        for i in range(HD // 16):
            r0 = i * 16
            top = wk_buf[c, r0:r0 + 16, :].astype(f32)
            bot = wk_buf[c, HD + r0:HD + r0 + 16, :].astype(f32)
            ops = _rform(top[:, :128], top[:, 128:], bot[:, :128], bot[:, 128:])
            for k in (0, 2, 3, 5, 6):
                wks.at[c][r0 // 2:r0 // 2 + 8, k * 128:(k + 1) * 128] = _pack(ops[k])

    def wq_perm():
        need(("in", 5))

        def permute(kt):
            for g in range(8):
                tile = gate(pltpu.bitcast(wq_buf[kt * 128:(kt + 1) * 128, g * 128:(g + 1) * 128], u32))
                wqt.at[kt * 8 + g][...] = pltpu.bitcast(_unpack(tile).T, u32)
                yield

        def back(kt):
            for j in range(8):
                tile = gate(jnp.concatenate([wqt[kt * 8 + g, pl.ds(j, 8, stride=8), :] for g in range(8)],
                                            axis=0))
                v = pltpu.bitcast(_unpack(tile).T.astype(f32), u32)
                c0 = (kt // 2) * D + _st(j // 2, j % 2).start
                ps[(kt % 2) * 128:(kt % 2 + 1) * 128, c0:c0 + 128] = v
                made.add(("wqp", kt, j))
                yield

        order = (0, 2, 4, 6, 1, 3, 5, 7)
        for n in range(10):
            if n < 8:
                yield from permute(order[n])
            if n > 1:
                yield from back(order[n - 2])

    def wq_form():
        for i in range(16):
            need(*[("wqp", 2 * r + i // 8, j) for r in range(4) for j in range(8)])
            for ct in range(2):
                def put(k1, k2, v):
                    wqs.at[k1 * 7 + k2][i * 8:(i + 1) * 8, ct * 128:(ct + 1) * 128] = v
                yield from form_steps(
                    _rform, _wr, lambda r, c: pltpu.bitcast(
                        ps[i * 16:(i + 1) * 16, r * D + _st(c, ct).start:r * D + _st(c, ct).stop],
                        f32), put)

    def kproj(r0, n, chunks=range(4)):
        pr = pl.ds(r0 // 2, n // 2)
        need(*[("xs", r) for r in range(max(r0, T0), r0 + n, 16)])
        for c in chunks:
            m = [None] * 7
            for k in K_SEQ:
                e11, e12, e21, e22 = [xs_at(L_ORD[k], e)[pr, :] for e in (0, 1, 7, 3)]
                lhs = jnp.concatenate([jnp.concatenate([e11, e12], axis=1),
                                       jnp.concatenate([e21, e22], axis=1)], axis=0)
                m[k] = mm(_unpack(lhs), wks[c, :, k * 128:(k + 1) * 128], NN, 2 * n)
            kk = [_phi(v) for v in _combine(m)]
            for ct in range(2):
                zacc[:, pl.ds(_mo(c * 256 + ct * 128, 128), 128)] += (
                    (kk[ct] + kk[2 + ct]).reshape(n // 4, 8, 128).sum(axis=0))
            for s1 in range(4):
                for h in range(2):
                    pk_buf.at[s1 % 2, (s1 // 2) * 2 + h][r0:r0 + n, pl.ds(_mo(c * 128, 128), 128)] = (
                        kk[s1][h * n:(h + 1) * n])

    def z_prep():
        z = jnp.sum(zacc[...], axis=0, keepdims=True)
        zt = _pack(jnp.broadcast_to(z, (128, D)).astype(bf16).T)
        for g in range(8):
            tscr.at[g][...] = zt[g * 64:(g + 1) * 64, :]
        for j in range(8):
            blk = jnp.concatenate([tscr[g, pl.ds(j, 8, stride=8), :] for g in range(8)], axis=0)
            zp[:, j * 128:(j + 1) * 128] = _unpack(blk).T[0:8, :].astype(f32)

    def route():
        rows, dots = [None] * 16, [None] * 16
        for b in sorted(range(S // 128), key=lambda b: b % 4):
            need(*[("ln", r) for r in range(max(T0, b % 4 * 128), b % 4 * 128 + 128, 16)])
            rows[b] = gate(stats[b * 128:(b + 1) * 128, 0:128]).T[0:8, :]
            dots[b] = jnp.sum(gate(stats[b * 128:(b + 1) * 128, 128:256]).T, axis=0, keepdims=True)
            yield
        mf = jnp.concatenate([v[0:1] for v in rows], axis=0)
        var = jnp.concatenate([v[1:2] for v in rows], axis=0)
        tr = jnp.concatenate(dots, axis=0) * jnp.sqrt(var + 1e-5)
        wsum = jnp.sum(wrb[0:1, :], axis=1, keepdims=True)
        mb = _rbf(mf)
        inv = 1.0 / _rbf(jnp.sqrt(_rbf(_rbf(var) + 1e-5)))
        rv = _rbf((tr + (mf - mb) * wsum) * inv)
        rmax = jnp.max(jnp.max(rv, axis=1, keepdims=True), axis=0, keepdims=True)
        pos = (lax.broadcasted_iota(i32, rv.shape, 0) * 128 + lax.broadcasted_iota(i32, rv.shape, 1))
        idx = jnp.min(jnp.where(rv == rmax, pos, S - 1))
        idx_s[0] = idx

        def pick(v):
            v = jnp.sum(jnp.where(pos == idx, v, 0.0), axis=1, keepdims=True)
            return jnp.sum(v, axis=0, keepdims=True)

        xv = x_buf[(idx >> 9) & 3, pl.ds(_mo(idx & (HQ - 16), 16), 16), :].astype(f32)
        sel = lax.broadcasted_iota(i32, xv.shape, 0) == (idx & 15)
        row = jnp.sum(jnp.where(sel, xv, 0.0), axis=0, keepdims=True)
        row = _rbf(_rbf(row - pick(mb)) * pick(inv))
        rsel[...] = jnp.broadcast_to(_rbf(jnp.sum(row * wrb[0:1, :], axis=1, keepdims=True)), rsel.shape)
        xb[...] = jnp.broadcast_to(row, (128, D)).T
        yield

    def ps_form(j):
        for c in range(HQ // 16):
            def put(k1, k2, v):
                k = k1 * 7 + k2
                ps[c * 8:(c + 1) * 8, k * 128:(k + 1) * 128] = v
            yield from form_steps(
                _lform, _wl_swapped,
                lambda r, q: pk_buf[j, q, c * 16:(c + 1) * 16, r * 128:(r + 1) * 128], put)

    def q_rows(j, r0, n, pq, rc, d0, rec):
        xj = pl.ds(_mo(j * (BQ // 2), BQ // 2), BQ // 2)
        pr = slice(r0 // 2, (r0 + n) // 2)
        blk = yield from strassen2(lambda k1, k2: _unpack(xs_at(L_ORD[k1], k2, xj)[pr, :]),
                                   lambda k1, k2: wqs[k1 * 7 + k2], NN, n, 1, QW)
        lane = lax.broadcasted_iota(i32, (n, 128), 1)
        for q in range(4):
            d = None
            for u in (3, 2, 1, 0):
                v = _phi(blk[q][u])
                for ct in range(2):
                    pq.at[q][d0:d0 + n, _st(u, ct)] = v[:, ct * 128:(ct + 1) * 128]
                t = v * zp[0:1, u * 256:(u + 1) * 256]
                t = t[:, :128] + t[:, 128:]
                d = t if d is None else d + t
            if rec:
                d = recip(d, lane)
            rc.at[q][d0:d0 + n, :] = d

    def recip(d, lane):
        d = d + jnp.where(lane % 2 == 0, pltpu.roll(d, 127, 1), pltpu.roll(d, 1, 1))
        d = d + jnp.where(lane % 4 < 2, pltpu.roll(d, 126, 1), pltpu.roll(d, 2, 1))
        return 1.0 / (d + 1e-6)

    def normalise(pq, rc, nr, dst, p0, raw, tok=None):
        lane = lax.broadcasted_iota(i32, (16, 128), 1)

        def fix(c):
            if c < nr // 16 and raw(c * 16):
                for q in range(4):
                    rq = slice(c * 16, (c + 1) * 16)
                    rc.at[q][rq, :] = recip(gate16(rc[q, rq, :]), lane)

        def scale(c):
            rq = slice(c * 16, (c + 1) * 16)
            fix(c + 1)
            for hf in range(2):
                for q in range(4):
                    cs = slice(hf * HD, (hf + 1) * HD)
                    pq.at[q][rq, cs] = pq[q, rq, cs] * jnp.concatenate([gate16(rc[q, rq, :])] * 4, axis=1)
                    yield

        def form(c):
            rq = slice(c * 16, (c + 1) * 16)
            p2 = pl.ds(_mo(p0 + c * 8, 8), 8)
            for ct in range(2):
                def put(k1, k2, v):
                    dst.at[k1 * 7 + k2][p2, ct * 128:(ct + 1) * 128] = v
                yield from form_steps(_lform, _wl, lambda q, u: pq[q, rq, _st(u, ct)], put, tok)

        fix(0)
        if raw(0):
            for _ in range(4):
                yield
        yield from scale(0)
        for c in range(nr // 16):
            nxt = scale(c + 1) if c + 1 < nr // 16 else iter(())
            for i, _ in enumerate(form(c)):
                yield
                if i < 8 and c + 1 < nr // 16:
                    next(nxt)
                    yield

    def g_kvm(j):
        qb = q_rows(j, BQ - QB, QB, pqb_buf.at[j], denb_buf.at[j], 0, False)
        for _ in range(QPRE):
            next(qb)
        blk = yield from strassen2(
            lambda k1, k2: _unpack(ps[:, (k1 * 7 + k2) * 128:(k1 * 7 + k2 + 1) * 128]),
            lambda k1, k2: xs_at(R_ORD[k1], W_R[k2])[...], TN, 256, 2, comb=_wc_swapped)
        hm = (lax.broadcasted_iota(i32, (128, 128), 0) // 32
              == lax.broadcasted_iota(i32, (128, 128), 1) // 32)
        for _ in range(QSPLIT - QPRE):
            next(qb)
        kvps = []
        for a in (3, 2, 1, 0):
            gg = jnp.concatenate(blk[a], axis=1).astype(bf16)
            wv_u = pltpu.bitcast(wv_buf[j, :, a * 128:(a + 1) * 128], u32)
            kv = jnp.where(hm, mm(gg, wv_u, NN, 256), 0.0)
            tscr2.at[a][...] = _pack(kv)
            kvps.append(_unpack(jnp.concatenate(
                [tscr2[a, pl.ds(jj, 8, stride=8), :] for jj in range(8)], axis=0)))

        def m_form():
            for a in (3, 2, 1, 0):
                need(("mg", a))
                for jl in range(2):
                    for ct in range(2):
                        def put(k1, k2, v):
                            ms.at[k1 * 7 + k2][pl.ds(_mo(jl * 64 + (2 * a + j) * 8, 8), 8),
                                               ct * 128:(ct + 1) * 128] = v
                        yield from form_steps(
                            _rform, _wr, lambda q, u: mg_buf[a, (2 * q + jl) * 16:(2 * q + jl + 1) * 16, _st(u, ct)], put)

        for i, a in enumerate((3, 2, 1, 0)):
            wo_u = pltpu.bitcast(wo_buf[j, a * 128:(a + 1) * 128, :], u32)
            res = mm(kvps[i], wo_u, NN, 256)
            mg_buf.at[a][...] = _to_st(res)
            made.add(("mg", a))
            if i == 0:
                add_side(lambda tok: m_form(), 112, *MF)
        for _ in qb:
            pass

    def out_part(base, span, off, nr, y, src):
        b = _mo(base, 32)
        sa_v, sb_v, out_v = [r.at[pl.ds(b, 3 * HQ + span), :] for r in (sa, sb, out_buf)]
        x_v = x_buf.at[:, pl.ds(b, span), :]
        row = lax.broadcasted_iota(i32, (nr, 256), 0) + (base + off)
        blk = yield from strassen2(lambda k1, k2: _unpack(src[k1 * 7 + k2, off // 2:(off + nr) // 2, :]),
                                   lambda k1, k2: ms[k1 * 7 + k2], NN, nr)
        for s1 in (3, 2, 1, 0):
            for s2 in range(4):
                q = (s1 // 2) * 2 + s2 // 2
                u = (s1 % 2) * 2 + s2 % 2
                rr, cc = pl.ds(q * HQ + off, nr), pl.ds(u * 256, 256)
                a = jnp.concatenate([sa_v[rr, :]] * 2, axis=1)
                c = jnp.concatenate([sb_v[rr, :]] * 2, axis=1)
                o = blk[q][u] + jnp.where(row + q * HQ == idx_s[0], y[:, u * 256:(u + 1) * 256], 0.0)
                out_v[rr, cc] = (x_v[q, off:off + nr, cc].astype(f32) * a - c + o).astype(bf16)
                if s2 % 2 == 1:
                    ch = pl.ds((s1 % 2) * HD, HD)
                    ro = pl.ds(_mo(base + q * HQ + off, 16), nr)
                    cp(out_buf.at[ro, ch], out_hbm.at[0, ro, ch], SEM_O).start()

    def ffn_part(j):
        def fma(acc, w, v):
            p = w.astype(f32) * v
            return acc + p[0:8] + p[8:16]

        for f0 in range(0, FH, 256):
            fs = slice(f0, f0 + 256)
            ag = jnp.zeros((8, 256), f32)
            au = jnp.zeros((8, 256), f32)
            for k in range(0, D, 16):
                xv = jnp.concatenate([gate16(xb[k:k + 16, :])] * 2, axis=1)
                ag = fma(ag, wg_buf[j, k:k + 16, fs], xv)
                au = fma(au, wu_buf[j, k:k + 16, fs], xv)
                yield
            g = _rbf(jnp.sum(ag, axis=0, keepdims=True))
            u = _rbf(jnp.sum(au, axis=0, keepdims=True))
            h = _rbf(_rbf(g * jax.nn.sigmoid(g)) * u)
            hb_buf[fs, :] = jnp.broadcast_to(h, (128, 256)).T
        for d0 in range(0, D, 512):
            ds_ = slice(d0, d0 + 512)
            acc = yacc[:, ds_]
            for k in range(0, FH, 16):
                hv = jnp.concatenate([gate16(hb_buf[k:k + 16, :])] * 4, axis=1)
                acc = fma(acc, wd_buf[j, k:k + 16, ds_], hv)
                yield
            yacc[:, ds_] = acc

    def wait_group(i):
        with _scope("a_wait%d" % i):
            for c in a_groups[i]:
                c.wait()
        made.add(("in", i - NX))

    def run_all(gen):
        for _ in gen:
            pass

    def ln_sides(plan):
        for r0, r1, t0, t1 in plan[0]:
            add_side(lambda tok, r0=r0, r1=r1: ln_stats(r0, r1 - r0, tok), (r1 - r0) // 2, t0, t1, LNLAG)
        for r0, r1, t0, t1 in plan[1]:
            add_side(lambda tok, r0=r0, r1=r1: ln_later(r0, r1 - r0, tok), 22 * (r1 - r0) // 16, t0, t1, SLAG)

    def l2_side(base, n, t0, t1):
        add_side(lambda tok: ln_later(0, n, None, "l2", base), 22 * n // 16, t0, t1)

    with _scope("p0_issue"):
        cp_wr.start()
        for grp in a_groups:
            for c in grp:
                c.start()
        for j in range(2):
            for c in cp_b(j):
                c.start()
        zacc[...] = jnp.zeros(zacc.shape, f32)
        yacc[...] = jnp.zeros(yacc.shape, f32)
        zero_buf[1] = jnp.zeros((8, 128), u32)
        cp_zero = cp(zero_buf.at[1], zero_buf.at[0], SEM_Z)
        cp_zero.start()
        cp_zero.wait()
        cp_wr.wait()
        wr8 = jnp.broadcast_to(wr_buf[0:D].reshape(1, D).astype(f32), (8, D))
        wrb[0:8, :] = wr8
        wrb[8:16, :] = _to_st(wr8)
        z0 = jnp.max(pltpu.bitcast(zero_buf[0], i32))
        ps, pq_buf, den_buf, mg_buf, hb_buf = [r.at[z0] for r in (ps_raw, pq_raw, den_raw, mg_raw, hb_raw)]
        xn_buf = mg_buf

    def a01(i, carry):
        with _scope("a_wait01"):
            for c in cp_x(i * X0, X0, SEM_A + i):
                c.wait()
        with _scope("a01"):
            for r in range(0, X0, 16):
                run_all(ln_stats(r, 16, None, (i, X0)))
                if r:
                    run_all(ln_later(r - 16, 16, None, "l1", (i, X0)))
            run_all(ln_later(X0 - 16, 16, None, "l1", (i, X0)))
        return carry

    lax.fori_loop(0, NX, a01, 0)
    made.update(("xn", r) for r in range(0, 64, 16))

    def a23(i, carry):
        with _scope("a_wait23"):
            for c in cp_wk(i, SEM_W + i):
                c.wait()
        with _scope("a23"):
            wk_prep(i)
            l2_side((i, T0 // 2), T0 // 2, 250, 14 * T0 - 250)
            kproj(0, T0, [i])
            finish()
        return carry

    lax.fori_loop(0, 2, a23, 0)
    wait_group(NX + 2)
    with _scope("a4"):
        wk_prep(2)
        ln_sides(L4)
        kproj(0, T0, [2])
        finish()
    wait_group(NX + 3)
    with _scope("a5"):
        wk_prep(3)
        ln_sides(L5)
        kproj(0, T0, [3])
        for r0, n in A5K:
            kproj(r0, n)
        finish()
    wait_group(NX + 4)
    with _scope("a6"):
        ln_sides(L6)
        for r0, n in A6K:
            kproj(r0, n)
        finish()
    wait_group(NX + 5)
    with _scope("a7"):
        ln_sides(L7)
        add_side(lambda tok: wq_perm(), 128, *WQ_PERM)
        add_side(lambda tok: wq_form(), 224, *WQ_FORM)
        add_side(lambda tok: route(), 17, *ROUTE)
        for r0, n in A7K:
            kproj(r0, n)
        finish()

    def b_body(j, carry):
        qa = BQ - QB
        with _scope("b_r0"):
            z_prep()
            add_side(lambda tok: ps_form(j), 7 * HQ // 16, 0, 49 * qa - 400)
            for r0 in range(0, qa, QN):
                run_all(q_rows(j, r0, QN, pq_buf, den_buf, r0, r0 + QN < qa))
            finish()
        with _scope("b_wait"):
            for c in cp_b(j, wait_only=True):
                c.wait()
        with _scope("b_r1"):
            add_side(lambda tok: ffn_part(j), FH * 3 // 8, 0, R1T)
            add_side(lambda tok: normalise(pq_buf, den_buf, qa, qs, j * (qa // 2), lambda r: r >= qa - QN),
                     22 * (qa // 16), 0, R1T)
            run_all(g_kvm(j))
            finish()
        return carry

    lax.fori_loop(0, 2, b_body, 0)

    def c_body(t, carry):
        with _scope("c_body"):
            y = _rbf(jnp.sum(yacc[...], axis=0, keepdims=True))
            y = _rbf(y * _rbf(1.0 / _rbf(1.0 + _rbf(jnp.exp(-rsel[0:1, :])))))
            j, h = t >> 1, t & 1
            na, nb = (BQ - QB) // 2, QB // 2
            hb = pl.ds(_mo(h * nb, 16), nb)
            add_side(lambda tok: normalise(pqb_buf.at[j, :, hb, :], denb_buf.at[j, :, hb, :], nb, qsb, 0,
                                           lambda r: True, tok),
                     4 + 22 * (nb // 16), 0, 49 * na - 800, SLAG)
            qs_t = qs.at[:, pl.ds(_mo(t * (na // 2), 16), na // 2), :]
            for p in range(0, na, CR):
                run_all(out_part(j * BQ + h * na, na, p, CR, y, qs_t))
            flush()
            run_all(out_part(j * BQ + BQ - QB + h * nb, nb, 0, nb, y, qsb))
            finish()
        return carry

    lax.fori_loop(0, 4, c_body, 0)
    with _scope("tail"):
        cp(out_buf, out_hbm.at[0], SEM_O).wait()


@jax.jit
def pallas_parallel_sum__linear_attn_block__moe_arch_mod__prompt_kernel(
    A_x: jax.Array,
    A_wqkv: jax.Array,
    A_wo: jax.Array,
    B_x: jax.Array,
    B_w_r: jax.Array,
    B_w_gate: jax.Array,
    B_w_up: jax.Array,
    B_w_down: jax.Array,
):
    del B_x
    V = pltpu.VMEM
    scratch = [
        V((4, HQ, D), bf16),
        V((4, D, 256), bf16),
        V((2, D, 512), bf16),
        V((2, 512, D), bf16),
        V((8 * D,), bf16),
        V((2, D, FH), bf16),
        V((2, D, FH), bf16),
        V((2, FH, D), bf16),
        V((28, HQ // 2, 256), u32),
        V((28, HQ // 2, 256), u32),
        V((49, 128, 256), u32),
        V((S, 128), f32),
        V((S, 128), f32),
        V((8, D), f32),
        V((8, D), f32),
        V((2, 4, HQ, 512), f32),
        V((D, 128), f32),
        V((8, D), f32),
        V((8, D), f32),
        V((16, D), f32),
        V((4, 8, 128), u32),
        V((4, HD // 2, 7 * 128), u32),
        V((S, 256), f32),
        V((64, 64, 128), u32),
        V((1, HQ // 2, 49 * 128), u32),
        V((49, BQ - QB, 256), u32),
        V((49, 128, 256), u32),
        V((8, 64, 128), u32),
        V((4, 64, 128), u32),
        V((1, 4, BQ - QB, D), f32),
        V((1, 4, BQ - QB, 128), f32),
        V((2, 4, QB, D), f32),
        V((2, 4, QB, 128), f32),
        V((49, QB // 4, 256), u32),
        V((1, 4, 128, D), f32),
        V((1, FH, 128), f32),
        V((S, D), bf16),
        pltpu.SMEM((1,), i32),
        pltpu.SemaphoreType.DMA((4 + T0 // X0 + 6,)),
    ]
    extra = {k: True for k in ("disable_bounds_checks", "disable_semaphore_checks")
             if hasattr(pltpu.CompilerParams, k)}
    return pl.pallas_call(
        _kernel,
        out_shape=jax.ShapeDtypeStruct((1, S, D), bf16),
        in_specs=[pl.BlockSpec(memory_space=pl.ANY)] * 7,
        out_specs=pl.BlockSpec(memory_space=pl.ANY),
        scratch_shapes=scratch,
        compiler_params=pltpu.CompilerParams(vmem_limit_bytes=120 * 1024 * 1024, **extra),
    )(A_x.reshape(4, HQ, D), A_wqkv, A_wo, B_w_r, B_w_gate, B_w_up, B_w_down)
```

```python
import contextlib

import jax
import jax.numpy as jnp
from jax import lax
import jax.experimental.pallas as pl
import jax.experimental.pallas.tpu as pltpu

bf16, f32, u32, i32 = jnp.bfloat16, jnp.float32, jnp.uint32, jnp.int32

S = 2048
D = 1024
F = 3584
HD = D // 2
HQ = S // 4
BQ = HQ // 2
FH = F // 2
QB = 64
QN = 48
QPRE = 3
QSPLIT = 6
CR = 48
T0 = 96
X0 = 32
XG = (160, 208)
XN = 128

SLAG = 400
LNLAG = 700
QW = (28, 36, 36, 6, 2, 2, 2)
L4 = ([(96, 144, 0, 1100)], [])
L5 = ([(144, 208, 1100, 3500)], [(96, 128, 300, 1250), (128, 144, 1300, 2000), (144, 208, 2300, 4700)])
L6 = ([(208, 512, 0, 10000)], [(208, 256, 800, 2600), (256, 448, 2700, 10500)])
L7 = ([], [(448, 512, 0, 3000)])
A5K = ((96, 32), (128, 32))
A6K = ((160, 48), (208, 48), (256, 48), (304, 48))
A7K = ((352, 48), (400, 48), (448, 64))
WQ_PERM, WQ_FORM, ROUTE = (0, 3200), (3300, 8600), (4500, 5300)
R1T = 12800
MF = (128, 3420)

L_ORD = (2, 3, 0, 1, 4, 5, 6)
R_ORD = (2, 0, 6, 5, 1, 4, 3)

K_SEQ = (1, 4, 0, 2, 3, 5, 6)
K_SEQ2 = (0, 1, 2, 5, 3, 4, 6)
W_SEQ = (0, 1, 5, 6, 4, 2, 3)

NN = (((1,), (0,)), ((), ()))
TN = (((0,), (0,)), ((), ()))


SCOPES = False


def _scope(name):
    return jax.named_scope(name) if SCOPES else contextlib.nullcontext()


def _mo(v, m):
    return v if isinstance(v, int) else pl.multiple_of(v, m)


def _dot(a, b, dims):
    return lax.dot_general(a, b, dims, preferred_element_type=f32)


def _pack(v):
    return pltpu.bitcast(v.astype(bf16), u32)


def _unpack(v):
    return pltpu.bitcast(v, bf16)


def _combine(m):
    m1, m2, m3, m4, m5, m6, m7 = m
    return m1 + m4 - m5 + m7, m3 + m5, m2 + m4, m1 - m2 + m3 + m6


def _lform(a11, a12, a21, a22):
    return (a11 + a22, a21 + a22, a11, a22, a11 + a12, a21 - a11, a12 - a22)


def _rform(b11, b12, b21, b22):
    return (b11 + b22, b11, b12 - b22, b21 - b11, b22, b11 + b12, b21 + b22)


def _sform(x11, x12, x21, x22):
    return (x11, x22, x11 + x22, x21 + x22, x11 + x12, x21 - x11, x12 - x22)


def _wl(a11, a12, a21, a22):
    s1 = a21 + a22
    s2 = s1 - a11
    return (a11, a12, a12 - s2, a22, s1, s2, a11 - a21)


def _wr(b11, b12, b21, b22):
    t1 = b12 - b11
    t2 = b22 - t1
    return (b11, b21, b22, t2 - b21, t1, t2, b22 - b12)


def _wc(p):
    p1, p2, p3, p4, p5, p6, p7 = p
    u2 = p1 + p6
    u3 = u2 + p7
    return p1 + p2, (u2 + p5) + p3, u3 - p4, u3 + p5


W_R = (3, 1, 0, 2, 4, 5, 6)


def _wl_swapped(a11, a12, a21, a22):
    return _wl(a12, a11, a22, a21)


def _wc_swapped(p):
    p1, p2, p3, p4, p5, p6, p7 = p
    v2 = p1 + p6
    u3 = p7 - v2
    return (p5 - v2) + p3, p1 + p2, u3 + p5, p4 - u3


class _Sym:
    def __init__(self, t):
        self.t = t

    def __add__(self, o):
        return _Sym({**self.t, **o.t})

    def __sub__(self, o):
        return _Sym({**self.t, **{k: -v for k, v in o.t.items()}})


def _st(u, ct):
    return slice((4 * ct + u) * 128, (4 * ct + u + 1) * 128)


def _to_st(v):
    return jnp.concatenate([v[:, (2 * u + ct) * 128:(2 * u + ct + 1) * 128]
                            for ct in range(2) for u in range(4)], axis=1)


def _phi(t):
    return jnp.where(t > 0, t + 1.0, jnp.exp(t)) + 1e-6


def _rbf(v):
    return v.astype(bf16).astype(f32)


def _kernel(x_hbm, wqkv_hbm, wo_hbm, wr_hbm, wg_hbm, wu_hbm, wd_hbm, out_hbm,
            x_buf, wk_buf, wv_buf, wo_buf, wr_buf, wg_buf, wu_buf, wd_buf,
            xs1, xs2, wqs, sa, sb, zacc, zp, pk_buf, xb, yacc, rsel, wrb, zero_buf,
            wks, stats, wqt, ps_raw, qs, ms, tscr, tscr2, pq_raw, den_raw, pqb_buf, denb_buf, qsb,
            mg_raw, hb_raw, out_buf, idx_s, sem):
    wq_buf = out_buf.at[pl.ds(0, D), :]

    def xs_at(k1, e, rows=None):
        r = xs1.at[k1 * 4 + (0, 1, 7, 3).index(e)] if e in (0, 1, 7, 3) else xs2.at[k1 * 4 + (2, 4, 5, 6).index(e)]
        return r if rows is None else r.at[rows, :]

    SEM_B, SEM_O, SEM_Z, SEM_A = 0, 2, 3, 4

    def cp(src, dst, s):
        return pltpu.make_async_copy(src, dst, sem.at[s])

    def cp_x(r0, n, s):
        r = pl.ds(_mo(r0, 16), n)
        return [cp(x_hbm.at[:, r, :], x_buf.at[:, r, :], s)]

    def cp_wk(c, s):
        return [cp(wqkv_hbm.at[:, pl.ds(_mo(D + c * 256, 256), 256)],
                   wk_buf.at[c], s)]

    NX = T0 // X0
    SEM_W = SEM_A + NX
    cp_wr = cp(wr_hbm, wr_buf.at[pl.ds(0, D)], SEM_Z)
    a_groups = [cp_x(i * X0, X0, SEM_A + i) for i in range(NX)] + [
        cp_wk(0, SEM_W),
        cp_wk(1, SEM_W + 1),
        cp_wk(2, SEM_W + 2) + cp_x(T0, XG[0] - T0, SEM_W + 2),
        cp_wk(3, SEM_W + 3) + cp_x(XG[0], XG[1] - XG[0], SEM_W + 3),
        cp_x(XG[1], HQ - XG[1], SEM_W + 4),
        [cp(wqkv_hbm.at[:, pl.ds(0, D)], wq_buf, SEM_W + 5)],
    ]

    def cp_b(j, wait_only=False):
        dsts = [r.at[j] for r in (wg_buf, wu_buf, wd_buf, wv_buf, wo_buf)]
        if wait_only:
            return [cp(dst, dst, SEM_B + j) for dst in dsts]
        fs = pl.ds(j * FH, FH)
        srcs = [wg_hbm.at[:, fs], wu_hbm.at[:, fs], wd_hbm.at[fs, :],
                wqkv_hbm.at[:, pl.ds(2 * D + j * HD, HD)], wo_hbm.at[pl.ds(j * HD, HD), :]]
        return [cp(src, dst, SEM_B + j) for src, dst in zip(srcs, dsts)]

    clock = [0]
    toks = []
    sides = []
    fwd = [None]

    def emit_tok(vals, stamp):
        t = None
        for v in vals:
            v = pltpu.bitcast(v, u32) if v.dtype != u32 else v
            t = v if t is None else t | v
        toks.append((stamp, t & zero_buf[0]))

    def token(kind):
        t = fwd[0]
        if "u" not in t:
            t["u"] = pltpu.bitcast(t["src"](), u32) & zero_buf[0]
        if kind != "u" and "f" not in t:
            t["f"] = pltpu.bitcast(t["u"], f32)
        if kind == "f16" and "f16" not in t:
            t["f16"] = jnp.concatenate([t["f"], t["f"]], axis=0)
        return t[kind]

    def gate(v):
        if fwd[0] is None:
            return v
        head = v if v.shape[0] == 8 else v[0:8]
        head = head | token("u") if v.dtype == u32 else head + token("f")
        return head if v.shape[0] == 8 else jnp.concatenate([head, v[8:]], axis=0)

    def gate16(v):
        return v if fwd[0] is None else v + token("f16")

    def add_side(gen_fn, n, t0, t1, lag=None):
        st = {"i": 0, "n": n, "t0": clock[0] + t0, "t1": clock[0] + t1}

        def tok(vals):
            if lag is not None:
                emit_tok(vals, st["t0"] + (st["i"] + 1) * (st["t1"] - st["t0"]) // st["n"] + lag)
        st["g"] = gen_fn(tok)
        sides.append(st)

    def advance(until):
        for st in sides:
            while st["i"] < st["n"] and st["t0"] + st["i"] * (st["t1"] - st["t0"]) // st["n"] < until:
                next(st["g"], None)
                st["i"] += 1
                if st["i"] == st["n"]:
                    for _ in st["g"]:
                        pass

    def flush():
        for st in sides:
            for _ in st["g"]:
                pass
        sides.clear()

    def finish():
        flush()
        toks.clear()
        fwd[0] = None

    def mm(lhs, rhs, dims, cycles, nseg=1):
        due = [t for (c, t) in toks if c <= clock[0]]
        toks[:] = [(c, t) for (c, t) in toks if c > clock[0]]
        if due:
            head = rhs[0:8, 0:128]
            for t in due:
                head = head | t
            if rhs.shape[1] > 128:
                head = jnp.concatenate([head, rhs[0:8, 128:]], axis=1)
            rhs = jnp.concatenate([head, rhs[8:]], axis=0)
        res = _dot(lhs, _unpack(rhs), dims)
        ngr = res.shape[0] // 16
        for sg in range(nseg):
            for i in range(ngr):
                fwd[0] = {"src": lambda sg=sg, i=i: res[i * 16:i * 16 + 8, sg * 128:(sg + 1) * 128]}
                clock[0] += cycles // nseg // ngr
                advance(clock[0])
        return res

    def form_steps(form, form2, get, put, tok=None, keep=range(7)):
        terms = form(*[_Sym({i: 1}) for i in range(4)])
        gated = (0, 1, 2, 3) if 7 in keep else {_wl: (0, 1, 3), _wr: (0, 2, 3), _wl_swapped: (1, 2)}[form2]
        for k1 in range(7):
            sub = []
            for r in range(2):
                for c in range(2):
                    v = None
                    for i, sg in sorted(terms[k1].t.items(), key=lambda e: -e[1]):
                        b = get(r + 2 * (i // 2), c + 2 * (i % 2))
                        if v is None:
                            v = gate16(b) if 2 * r + c in gated else b
                        else:
                            v = v + b if sg > 0 else v - b
                    sub.append(v)
            vals = form2(*sub) + (sub[2],)
            for k2 in keep:
                put(k1, k2, _pack(vals[k2]))
            if tok is not None and k1 % 2 == 0:
                full = vals[3 if form2 is _wr else 2]
                tok([full[0:8], full[8:16]])
            yield

    def strassen2(lhs, rhs, dims, cycles, nseg=1, wts=(16,) * 7, comb=_wc):
        m1 = [None] * 7
        for i1, k1 in enumerate(K_SEQ2):
            m2 = [None] * 7
            for k2 in W_SEQ:
                m2[k2] = mm(lhs(k1, k2), rhs(k1, k2), dims, cycles * wts[i1] // 16, nseg)
                yield
            m1[k1] = comb(m2)
        out = [[None] * 4 for _ in range(4)]
        for s2 in range(4):
            for s1, v in enumerate(_combine([m1[k1][s2] for k1 in range(7)])):
                out[(s1 // 2) * 2 + s2 // 2][(s1 % 2) * 2 + s2 % 2] = v
        return out

    made = set()

    def need(*keys):
        assert all(k in made for k in keys), keys

    def row_views(base):
        if base == 0:
            return x_buf, sa, sb, stats, xn_buf, None
        i, n = base
        b = _mo(i * n, 16)
        return ([x_buf.at[:, pl.ds(b, n), :]] + [r.at[pl.ds(b, S - 128 + n), :] for r in (sa, sb, stats)]
                + [xn_buf.at[:, pl.ds(b, n), :], pl.ds(_mo(i * (n // 2), 8), n // 2)])

    def xs_form(r0, tok, which="all", base=0):
        xn_v, xs_v = row_views(base)[4:]
        rows = slice(r0 % XN, r0 % XN + 16)

        keep = {"all": range(8), "l1": (0, 1, 7, 3), "l2": (2, 4, 5, 6)}[which]
        for ct in range(2):
            def put(k1, k2, v):
                xs_at(k1, k2, xs_v)[r0 // 2:r0 // 2 + 8, ct * 128:(ct + 1) * 128] = v
            yield from form_steps(
                _sform, _wl, lambda q, u: xn_v[q, rows, _st(u, ct)], put, tok, keep)
        made.add(("xs", r0))

    def ln_stats(r_start, n_rows, tok, base=0):
        x_v, sa_v, sb_v, st_v, xn_v, _ = row_views(base)
        lane = lax.broadcasted_iota(i32, (8, 128), 1)
        for r0 in range(r_start, r_start + n_rows, 16):
            if r0 >= T0:
                need(("in", 2 + sum(r0 >= g for g in XG)))
            if r0 - XN >= T0:
                need(("ln", r0 - XN))
            for g in range(8):
                q, o = g // 2, (g % 2) * 8
                rg = q * HQ + r0 + o
                xv = x_v[q, r0 + o:r0 + o + 8, :].astype(f32)
                xg = jnp.concatenate([gate(xv[:, 0:128]), xv[:, 128:]], axis=1)
                mf = jnp.sum(xg, axis=1, keepdims=True) * (1.0 / D)
                d = xv - mf
                var = jnp.sum(d * d, axis=1, keepdims=True) * (1.0 / D)
                rs = lax.rsqrt(var + 1e-5)
                xn_v.at[q][r0 % XN + o:r0 % XN + o + 8, :] = _to_st(d * rs)
                rs = jnp.broadcast_to(rs, (8, 128))
                mf = jnp.broadcast_to(mf, (8, 128))
                sa_v[rg:rg + 8, :] = 1.0 + rs
                sb_v[rg:rg + 8, :] = mf * rs
                st_v[rg:rg + 8, 0:128] = jnp.where(lane == 0, mf, jnp.broadcast_to(var, (8, 128)))
                if tok is not None:
                    tok([rs])
                if g == 7:
                    made.add(("xn", r0))
                yield

    def ln_later(r_start, n_rows, tok, which="all", base=0):
        st_v, xn_v = row_views(base)[3:5]
        for r0 in range(r_start, r_start + n_rows, 16):
            need(("xn", r0))
            form = xs_form(r0, tok, which, base)
            for g in range(8):
                for _ in range(2 if g < 7 else 0):
                    next(form)
                    yield
                q, o = g // 2, (g % 2) * 8
                t = None
                if which != "l1":
                    v = xn_v[q, r0 % XN + o:r0 % XN + o + 8, :] * wrb[8:16, :]
                    for ct in range(8):
                        h = v[:, ct * 128:(ct + 1) * 128]
                        t = gate(h) if t is None else t + h
                if t is not None:
                    st_v[q * HQ + r0 + o:q * HQ + r0 + o + 8, 128:256] = t
                if tok is not None:
                    tok([t])
                if g == 7:
                    next(form, None)
                    made.add(("ln", r0))
                yield

    def wk_prep(c):
        if isinstance(c, int):
            need(("in", c))
        wks.at[c][:, 128:256] = pltpu.bitcast(wk_buf[c, 0:HD, 0:128], u32)
        wks.at[c][:, 512:640] = pltpu.bitcast(wk_buf[c, HD:D, 128:256], u32)
        for i in range(HD // 16):
            r0 = i * 16
            top = wk_buf[c, r0:r0 + 16, :].astype(f32)
            bot = wk_buf[c, HD + r0:HD + r0 + 16, :].astype(f32)
            ops = _rform(top[:, :128], top[:, 128:], bot[:, :128], bot[:, 128:])
            for k in (0, 2, 3, 5, 6):
                wks.at[c][r0 // 2:r0 // 2 + 8, k * 128:(k + 1) * 128] = _pack(ops[k])

    def wq_perm():
        need(("in", 5))

        def permute(kt):
            for g in range(8):
                tile = gate(pltpu.bitcast(wq_buf[kt * 128:(kt + 1) * 128, g * 128:(g + 1) * 128], u32))
                wqt.at[kt * 8 + g][...] = pltpu.bitcast(_unpack(tile).T, u32)
                yield

        def back(kt):
            for j in range(8):
                tile = gate(jnp.concatenate([wqt[kt * 8 + g, pl.ds(j, 8, stride=8), :] for g in range(8)],
                                            axis=0))
                v = pltpu.bitcast(_unpack(tile).T.astype(f32), u32)
                c0 = (kt // 2) * D + _st(j // 2, j % 2).start
                ps[(kt % 2) * 128:(kt % 2 + 1) * 128, c0:c0 + 128] = v
                made.add(("wqp", kt, j))
                yield

        order = (0, 2, 4, 6, 1, 3, 5, 7)
        for n in range(10):
            if n < 8:
                yield from permute(order[n])
            if n > 1:
                yield from back(order[n - 2])

    def wq_form():
        for i in range(16):
            need(*[("wqp", 2 * r + i // 8, j) for r in range(4) for j in range(8)])
            for ct in range(2):
                def put(k1, k2, v):
                    wqs.at[k1 * 7 + k2][i * 8:(i + 1) * 8, ct * 128:(ct + 1) * 128] = v
                yield from form_steps(
                    _rform, _wr, lambda r, c: pltpu.bitcast(
                        ps[i * 16:(i + 1) * 16, r * D + _st(c, ct).start:r * D + _st(c, ct).stop],
                        f32), put)

    def kproj(r0, n, chunks=range(4)):
        pr = pl.ds(r0 // 2, n // 2)
        need(*[("xs", r) for r in range(max(r0, T0), r0 + n, 16)])
        for c in chunks:
            m = [None] * 7
            for k in K_SEQ:
                e11, e12, e21, e22 = [xs_at(L_ORD[k], e)[pr, :] for e in (0, 1, 7, 3)]
                lhs = jnp.concatenate([jnp.concatenate([e11, e12], axis=1),
                                       jnp.concatenate([e21, e22], axis=1)], axis=0)
                m[k] = mm(_unpack(lhs), wks[c, :, k * 128:(k + 1) * 128], NN, 2 * n)
            kk = [_phi(v) for v in _combine(m)]
            for ct in range(2):
                zacc[:, pl.ds(_mo(c * 256 + ct * 128, 128), 128)] += (
                    (kk[ct] + kk[2 + ct]).reshape(n // 4, 8, 128).sum(axis=0))
            j, c2 = (c // 2, c % 2) if isinstance(c, int) else (0, c)
            pk_v = pk_buf.at[j, :, :, pl.ds(_mo(c2 * 256, 256), 256)]
            for s1 in range(4):
                for h in range(2):
                    pk_v.at[(s1 // 2) * 2 + h][r0:r0 + n, (s1 % 2) * 128:(s1 % 2 + 1) * 128] = (
                        kk[s1][h * n:(h + 1) * n])

    def z_prep():
        z = jnp.sum(zacc[...], axis=0, keepdims=True)
        zt = _pack(jnp.broadcast_to(z, (128, D)).astype(bf16).T)
        for g in range(8):
            tscr.at[g][...] = zt[g * 64:(g + 1) * 64, :]
        for j in range(8):
            blk = jnp.concatenate([tscr[g, pl.ds(j, 8, stride=8), :] for g in range(8)], axis=0)
            zp[:, j * 128:(j + 1) * 128] = _unpack(blk).T[0:8, :].astype(f32)

    def route():
        rows, dots = [None] * 16, [None] * 16
        for b in sorted(range(S // 128), key=lambda b: b % 4):
            need(*[("ln", r) for r in range(max(T0, b % 4 * 128), b % 4 * 128 + 128, 16)])
            rows[b] = gate(stats[b * 128:(b + 1) * 128, 0:128]).T[0:8, :]
            dots[b] = jnp.sum(gate(stats[b * 128:(b + 1) * 128, 128:256]).T, axis=0, keepdims=True)
            yield
        mf = jnp.concatenate([v[0:1] for v in rows], axis=0)
        var = jnp.concatenate([v[1:2] for v in rows], axis=0)
        tr = jnp.concatenate(dots, axis=0) * jnp.sqrt(var + 1e-5)
        wsum = jnp.sum(wrb[0:1, :], axis=1, keepdims=True)
        mb = _rbf(mf)
        inv = 1.0 / _rbf(jnp.sqrt(_rbf(_rbf(var) + 1e-5)))
        rv = _rbf((tr + (mf - mb) * wsum) * inv)
        rmax = jnp.max(jnp.max(rv, axis=1, keepdims=True), axis=0, keepdims=True)
        pos = (lax.broadcasted_iota(i32, rv.shape, 0) * 128 + lax.broadcasted_iota(i32, rv.shape, 1))
        idx = jnp.min(jnp.where(rv == rmax, pos, S - 1))
        idx_s[0] = idx

        def pick(v):
            v = jnp.sum(jnp.where(pos == idx, v, 0.0), axis=1, keepdims=True)
            return jnp.sum(v, axis=0, keepdims=True)

        xv = x_buf[(idx >> 9) & 3, pl.ds(_mo(idx & (HQ - 16), 16), 16), :].astype(f32)
        sel = lax.broadcasted_iota(i32, xv.shape, 0) == (idx & 15)
        row = jnp.sum(jnp.where(sel, xv, 0.0), axis=0, keepdims=True)
        row = _rbf(_rbf(row - pick(mb)) * pick(inv))
        rsel[...] = jnp.broadcast_to(_rbf(jnp.sum(row * wrb[0:1, :], axis=1, keepdims=True)), rsel.shape)
        xb[...] = jnp.broadcast_to(row, (128, D)).T
        yield

    def ps_form(j):
        for c in range(HQ // 16):
            def put(k1, k2, v):
                k = k1 * 7 + k2
                ps[c * 8:(c + 1) * 8, k * 128:(k + 1) * 128] = v
            yield from form_steps(
                _lform, _wl_swapped,
                lambda r, q: pk_buf[j, q, c * 16:(c + 1) * 16, r * 128:(r + 1) * 128], put)

    def q_rows(j, r0, n, pq, rc, d0, rec):
        xj = pl.ds(_mo(j * (BQ // 2), BQ // 2), BQ // 2)
        pr = slice(r0 // 2, (r0 + n) // 2)
        blk = yield from strassen2(lambda k1, k2: _unpack(xs_at(L_ORD[k1], k2, xj)[pr, :]),
                                   lambda k1, k2: wqs[k1 * 7 + k2], NN, n, 1, QW)
        lane = lax.broadcasted_iota(i32, (n, 128), 1)
        for q in range(4):
            d = None
            for u in (3, 2, 1, 0):
                v = _phi(blk[q][u])
                for ct in range(2):
                    pq.at[q][d0:d0 + n, _st(u, ct)] = v[:, ct * 128:(ct + 1) * 128]
                t = v * zp[0:1, u * 256:(u + 1) * 256]
                t = t[:, :128] + t[:, 128:]
                d = t if d is None else d + t
            if rec:
                d = recip(d, lane)
            rc.at[q][d0:d0 + n, :] = d

    def recip(d, lane):
        d = d + jnp.where(lane % 2 == 0, pltpu.roll(d, 127, 1), pltpu.roll(d, 1, 1))
        d = d + jnp.where(lane % 4 < 2, pltpu.roll(d, 126, 1), pltpu.roll(d, 2, 1))
        return 1.0 / (d + 1e-6)

    def normalise(pq, rc, nr, dst, raw, tok=None):
        lane = lax.broadcasted_iota(i32, (16, 128), 1)

        def fix(c):
            if c < nr // 16 and raw(c * 16):
                for q in range(4):
                    rq = slice(c * 16, (c + 1) * 16)
                    rc.at[q][rq, :] = recip(gate16(rc[q, rq, :]), lane)

        def scale(c):
            rq = slice(c * 16, (c + 1) * 16)
            fix(c + 1)
            for hf in range(2):
                for q in range(4):
                    cs = slice(hf * HD, (hf + 1) * HD)
                    pq.at[q][rq, cs] = pq[q, rq, cs] * jnp.concatenate([gate16(rc[q, rq, :])] * 4, axis=1)
                    yield

        def form(c):
            rq = slice(c * 16, (c + 1) * 16)
            for ct in range(2):
                def put(k1, k2, v):
                    dst.at[k1 * 7 + k2][c * 8:(c + 1) * 8, ct * 128:(ct + 1) * 128] = v
                yield from form_steps(_lform, _wl, lambda q, u: pq[q, rq, _st(u, ct)], put, tok)

        fix(0)
        if raw(0):
            for _ in range(4):
                yield
        yield from scale(0)
        for c in range(nr // 16):
            nxt = scale(c + 1) if c + 1 < nr // 16 else iter(())
            for i, _ in enumerate(form(c)):
                yield
                if i < 8 and c + 1 < nr // 16:
                    next(nxt)
                    yield

    def g_kvm(j):
        qb = q_rows(j, BQ - QB, QB, pqb_buf.at[j], denb_buf.at[j], 0, False)
        for _ in range(QPRE):
            next(qb)
        blk = yield from strassen2(
            lambda k1, k2: _unpack(ps[:, (k1 * 7 + k2) * 128:(k1 * 7 + k2 + 1) * 128]),
            lambda k1, k2: xs_at(R_ORD[k1], W_R[k2])[...], TN, 256, 2, comb=_wc_swapped)
        hm = (lax.broadcasted_iota(i32, (128, 128), 0) // 32
              == lax.broadcasted_iota(i32, (128, 128), 1) // 32)
        for _ in range(QSPLIT - QPRE):
            next(qb)
        kvps = []
        for a in (3, 2, 1, 0):
            gg = jnp.concatenate(blk[a], axis=1).astype(bf16)
            wv_u = pltpu.bitcast(wv_buf[j, :, a * 128:(a + 1) * 128], u32)
            kv = jnp.where(hm, mm(gg, wv_u, NN, 256), 0.0)
            tscr2.at[a][...] = _pack(kv)
            kvps.append(_unpack(jnp.concatenate(
                [tscr2[a, pl.ds(jj, 8, stride=8), :] for jj in range(8)], axis=0)))

        ms_j = ms.at[:, pl.ds(_mo(j * 32, 32), 96), :]

        def m_form():
            for a in (3, 2, 1, 0):
                need(("mg", a))
                for jl in range(2):
                    for ct in range(2):
                        def put(k1, k2, v):
                            ms_j.at[k1 * 7 + k2][jl * 64 + a * 8:jl * 64 + (a + 1) * 8,
                                                 ct * 128:(ct + 1) * 128] = v
                        yield from form_steps(
                            _rform, _wr, lambda q, u: mg_buf[a, (2 * q + jl) * 16:(2 * q + jl + 1) * 16, _st(u, ct)], put)

        for i, a in enumerate((3, 2, 1, 0)):
            wo_u = pltpu.bitcast(wo_buf[j, a * 128:(a + 1) * 128, :], u32)
            res = mm(kvps[i], wo_u, NN, 256)
            mg_buf.at[a][...] = _to_st(res)
            made.add(("mg", a))
            if i == 0:
                add_side(lambda tok: m_form(), 112, *MF)
        for _ in qb:
            pass

    def out_part(base, span, off, nr, y, src):
        b = _mo(base, 32)
        sa_v, sb_v, out_v = [r.at[pl.ds(b, 3 * HQ + span), :] for r in (sa, sb, out_buf)]
        x_v = x_buf.at[:, pl.ds(b, span), :]
        row = lax.broadcasted_iota(i32, (nr, 256), 0) + (base + off)
        blk = yield from strassen2(lambda k1, k2: _unpack(src[k1 * 7 + k2, off // 2:(off + nr) // 2, :]),
                                   lambda k1, k2: ms[k1 * 7 + k2], NN, nr)
        for s1 in (3, 2, 1, 0):
            for s2 in range(4):
                q = (s1 // 2) * 2 + s2 // 2
                u = (s1 % 2) * 2 + s2 % 2
                rr, cc = pl.ds(q * HQ + off, nr), pl.ds(u * 256, 256)
                a = jnp.concatenate([sa_v[rr, :]] * 2, axis=1)
                c = jnp.concatenate([sb_v[rr, :]] * 2, axis=1)
                o = blk[q][u] + jnp.where(row + q * HQ == idx_s[0], y[:, u * 256:(u + 1) * 256], 0.0)
                out_v[rr, cc] = (x_v[q, off:off + nr, cc].astype(f32) * a - c + o).astype(bf16)
                if s2 % 2 == 1:
                    ch = pl.ds((s1 % 2) * HD, HD)
                    ro = pl.ds(_mo(base + q * HQ + off, 16), nr)
                    cp(out_buf.at[ro, ch], out_hbm.at[0, ro, ch], SEM_O).start()

    def ffn_part(j):
        def fma(acc, w, v):
            p = w.astype(f32) * v
            return acc + p[0:8] + p[8:16]

        for f0 in range(0, FH, 256):
            fs = slice(f0, f0 + 256)
            ag = jnp.zeros((8, 256), f32)
            au = jnp.zeros((8, 256), f32)
            for k in range(0, D, 16):
                xv = jnp.concatenate([gate16(xb[k:k + 16, :])] * 2, axis=1)
                ag = fma(ag, wg_buf[j, k:k + 16, fs], xv)
                au = fma(au, wu_buf[j, k:k + 16, fs], xv)
                yield
            g = _rbf(jnp.sum(ag, axis=0, keepdims=True))
            u = _rbf(jnp.sum(au, axis=0, keepdims=True))
            h = _rbf(_rbf(g * jax.nn.sigmoid(g)) * u)
            hb_buf[fs, :] = jnp.broadcast_to(h, (128, 256)).T
        for d0 in range(0, D, 512):
            ds_ = slice(d0, d0 + 512)
            acc = yacc[:, ds_]
            for k in range(0, FH, 16):
                hv = jnp.concatenate([gate16(hb_buf[k:k + 16, :])] * 4, axis=1)
                acc = fma(acc, wd_buf[j, k:k + 16, ds_], hv)
                yield
            yacc[:, ds_] = acc

    def wait_group(i):
        with _scope("a_wait%d" % i):
            for c in a_groups[i]:
                c.wait()
        made.add(("in", i - NX))

    def run_all(gen):
        for _ in gen:
            pass

    def ln_sides(plan):
        for r0, r1, t0, t1 in plan[0]:
            add_side(lambda tok, r0=r0, r1=r1: ln_stats(r0, r1 - r0, tok), (r1 - r0) // 2, t0, t1, LNLAG)
        for r0, r1, t0, t1 in plan[1]:
            add_side(lambda tok, r0=r0, r1=r1: ln_later(r0, r1 - r0, tok), 22 * (r1 - r0) // 16, t0, t1, SLAG)

    def l2_side(base, n, t0, t1):
        add_side(lambda tok: ln_later(0, n, None, "l2", base), 22 * n // 16, t0, t1)

    with _scope("p0_issue"):
        cp_wr.start()
        for grp in a_groups:
            for c in grp:
                c.start()
        for j in range(2):
            for c in cp_b(j):
                c.start()
        zacc[...] = jnp.zeros(zacc.shape, f32)
        yacc[...] = jnp.zeros(yacc.shape, f32)
        zero_buf[1] = jnp.zeros((8, 128), u32)
        cp_zero = cp(zero_buf.at[1], zero_buf.at[0], SEM_Z)
        cp_zero.start()
        cp_zero.wait()
        cp_wr.wait()
        wr8 = jnp.broadcast_to(wr_buf[0:D].reshape(1, D).astype(f32), (8, D))
        wrb[0:8, :] = wr8
        wrb[8:16, :] = _to_st(wr8)
        z0 = jnp.max(pltpu.bitcast(zero_buf[0], i32))
        ps, pq_buf, den_buf, mg_buf, hb_buf = [r.at[z0] for r in (ps_raw, pq_raw, den_raw, mg_raw, hb_raw)]
        xn_buf = mg_buf

    def a01(i, carry):
        with _scope("a_wait01"):
            for c in cp_x(i * X0, X0, SEM_A + i):
                c.wait()
        with _scope("a01"):
            for r in range(0, X0, 16):
                run_all(ln_stats(r, 16, None, (i, X0)))
                if r:
                    run_all(ln_later(r - 16, 16, None, "l1", (i, X0)))
            run_all(ln_later(X0 - 16, 16, None, "l1", (i, X0)))
        return carry

    lax.fori_loop(0, NX, a01, 0)
    made.update(("xn", r) for r in range(0, 64, 16))

    def a23(i, carry):
        with _scope("a_wait23"):
            for c in cp_wk(i, SEM_W + i):
                c.wait()
        with _scope("a23"):
            wk_prep(i)
            l2_side((i, T0 // 2), T0 // 2, 250, 14 * T0 - 250)
            kproj(0, T0, [i])
            finish()
        return carry

    lax.fori_loop(0, 2, a23, 0)
    wait_group(NX + 2)
    with _scope("a4"):
        wk_prep(2)
        ln_sides(L4)
        kproj(0, T0, [2])
        finish()
    wait_group(NX + 3)
    with _scope("a5"):
        wk_prep(3)
        ln_sides(L5)
        kproj(0, T0, [3])
        for r0, n in A5K:
            kproj(r0, n)
        finish()
    wait_group(NX + 4)
    with _scope("a6"):
        ln_sides(L6)
        for r0, n in A6K:
            kproj(r0, n)
        finish()
    wait_group(NX + 5)
    with _scope("a7"):
        ln_sides(L7)
        add_side(lambda tok: wq_perm(), 128, *WQ_PERM)
        add_side(lambda tok: wq_form(), 224, *WQ_FORM)
        add_side(lambda tok: route(), 17, *ROUTE)
        for r0, n in A7K:
            kproj(r0, n)
        finish()

    def b_body(j, carry):
        qa = BQ - QB
        with _scope("b_r0"):
            z_prep()
            add_side(lambda tok: ps_form(j), 7 * HQ // 16, 0, 49 * qa - 400)
            for r0 in range(0, qa, QN):
                run_all(q_rows(j, r0, QN, pq_buf, den_buf, r0, r0 + QN < qa))
            finish()
        with _scope("b_wait"):
            for c in cp_b(j, wait_only=True):
                c.wait()
        with _scope("b_r1"):
            add_side(lambda tok: ffn_part(j), FH * 3 // 8, 0, R1T)
            qs_j = qs.at[:, pl.ds(_mo(j * (qa // 2), 16), qa // 2), :]
            add_side(lambda tok: normalise(pq_buf, den_buf, qa, qs_j, lambda r: r >= qa - QN),
                     22 * (qa // 16), 0, R1T)
            run_all(g_kvm(j))
            finish()
        return carry

    lax.fori_loop(0, 2, b_body, 0)

    def c_body(t, carry):
        with _scope("c_body"):
            y = _rbf(jnp.sum(yacc[...], axis=0, keepdims=True))
            y = _rbf(y * _rbf(1.0 / _rbf(1.0 + _rbf(jnp.exp(-rsel[0:1, :])))))
            j, h = t >> 1, t & 1
            na, nb = (BQ - QB) // 2, QB // 2
            hb = pl.ds(_mo(h * nb, 16), nb)
            add_side(lambda tok: normalise(pqb_buf.at[j, :, hb, :], denb_buf.at[j, :, hb, :], nb, qsb,
                                           lambda r: True, tok),
                     4 + 22 * (nb // 16), 0, 49 * na - 800, SLAG)
            qs_t = qs.at[:, pl.ds(_mo(t * (na // 2), 16), na // 2), :]
            for p in range(0, na, CR):
                run_all(out_part(j * BQ + h * na, na, p, CR, y, qs_t))
            flush()
            run_all(out_part(j * BQ + BQ - QB + h * nb, nb, 0, nb, y, qsb))
            finish()
        return carry

    lax.fori_loop(0, 4, c_body, 0)
    with _scope("tail"):
        cp(out_buf, out_hbm.at[0], SEM_O).wait()


@jax.jit
def pallas_parallel_sum__linear_attn_block__moe_arch_mod__prompt_kernel(
    A_x: jax.Array,
    A_wqkv: jax.Array,
    A_wo: jax.Array,
    B_x: jax.Array,
    B_w_r: jax.Array,
    B_w_gate: jax.Array,
    B_w_up: jax.Array,
    B_w_down: jax.Array,
):
    del B_x
    V = pltpu.VMEM
    scratch = [
        V((4, HQ, D), bf16),
        V((4, D, 256), bf16),
        V((2, D, 512), bf16),
        V((2, 512, D), bf16),
        V((8 * D,), bf16),
        V((2, D, FH), bf16),
        V((2, D, FH), bf16),
        V((2, FH, D), bf16),
        V((28, HQ // 2, 256), u32),
        V((28, HQ // 2, 256), u32),
        V((49, 128, 256), u32),
        V((S, 128), f32),
        V((S, 128), f32),
        V((8, D), f32),
        V((8, D), f32),
        V((2, 4, HQ, 512), f32),
        V((D, 128), f32),
        V((8, D), f32),
        V((8, D), f32),
        V((16, D), f32),
        V((4, 8, 128), u32),
        V((4, HD // 2, 7 * 128), u32),
        V((S, 256), f32),
        V((64, 64, 128), u32),
        V((1, HQ // 2, 49 * 128), u32),
        V((49, BQ - QB, 256), u32),
        V((49, 128, 256), u32),
        V((8, 64, 128), u32),
        V((4, 64, 128), u32),
        V((1, 4, BQ - QB, D), f32),
        V((1, 4, BQ - QB, 128), f32),
        V((2, 4, QB, D), f32),
        V((2, 4, QB, 128), f32),
        V((49, QB // 4, 256), u32),
        V((1, 4, 128, D), f32),
        V((1, FH, 128), f32),
        V((S, D), bf16),
        pltpu.SMEM((1,), i32),
        pltpu.SemaphoreType.DMA((4 + T0 // X0 + 6,)),
    ]
    extra = {k: True for k in ("disable_bounds_checks", "disable_semaphore_checks")
             if hasattr(pltpu.CompilerParams, k)}
    return pl.pallas_call(
        _kernel,
        out_shape=jax.ShapeDtypeStruct((1, S, D), bf16),
        in_specs=[pl.BlockSpec(memory_space=pl.ANY)] * 7,
        out_specs=pl.BlockSpec(memory_space=pl.ANY),
        scratch_shapes=scratch,
        compiler_params=pltpu.CompilerParams(vmem_limit_bytes=120 * 1024 * 1024, **extra),
    )(A_x.reshape(4, HQ, D), A_wqkv, A_wo, B_w_r, B_w_gate, B_w_up, B_w_down)
```

```python
import contextlib

import jax
import jax.numpy as jnp
from jax import lax
import jax.experimental.pallas as pl
import jax.experimental.pallas.tpu as pltpu

bf16, f32, u32, i32 = jnp.bfloat16, jnp.float32, jnp.uint32, jnp.int32

S = 2048
D = 1024
F = 3584
HD = D // 2
HQ = S // 4
BQ = HQ // 2
FH = F // 2
QB = 64
QN = 48
QPRE = 3
QSPLIT = 6
CR = 48
T0 = 96
X0 = 32
XG = (160, 208)
XN = 128

SLAG = 400
LNLAG = 700
QW = (28, 36, 36, 6, 2, 2, 2)
L4 = ([(96, 144, 0, 1100)], [])
L5 = ([(144, 208, 1100, 3500)], [(96, 128, 300, 1250), (128, 144, 1300, 2000), (144, 208, 2300, 4700)])
L6 = ([(208, 512, 0, 10000)], [(208, 256, 800, 2600), (256, 448, 2700, 10500)])
L7 = ([], [(448, 512, 0, 3000)])
A5K = ((96, 32), (128, 32))
A6K = ((160, 48), (208, 48), (256, 48), (304, 48))
A7K = ((352, 48), (400, 48), (448, 64))
WQ_PERM, WQ_FORM, ROUTE = (0, 3200), (3300, 8600), (4500, 5300)
R1T = 12800
MF = (128, 3420)

L_ORD = (2, 3, 0, 1, 4, 5, 6)
R_ORD = (2, 0, 6, 5, 1, 4, 3)

K_SEQ = (1, 4, 0, 2, 3, 5, 6)
K_SEQ2 = (0, 1, 2, 5, 3, 4, 6)
W_SEQ = (0, 1, 5, 6, 4, 2, 3)

NN = (((1,), (0,)), ((), ()))
TN = (((0,), (0,)), ((), ()))


SCOPES = False


def _scope(name):
    return jax.named_scope(name) if SCOPES else contextlib.nullcontext()


def _mo(v, m):
    return v if isinstance(v, int) else pl.multiple_of(v, m)


def _dot(a, b, dims):
    return lax.dot_general(a, b, dims, preferred_element_type=f32)


def _pack(v):
    return pltpu.bitcast(v.astype(bf16), u32)


def _unpack(v):
    return pltpu.bitcast(v, bf16)


def _combine(m):
    m1, m2, m3, m4, m5, m6, m7 = m
    return m1 + m4 - m5 + m7, m3 + m5, m2 + m4, m1 - m2 + m3 + m6


def _lform(a11, a12, a21, a22):
    return (a11 + a22, a21 + a22, a11, a22, a11 + a12, a21 - a11, a12 - a22)


def _rform(b11, b12, b21, b22):
    return (b11 + b22, b11, b12 - b22, b21 - b11, b22, b11 + b12, b21 + b22)


def _sform(x11, x12, x21, x22):
    return (x11, x22, x11 + x22, x21 + x22, x11 + x12, x21 - x11, x12 - x22)


def _wl(a11, a12, a21, a22):
    s1 = a21 + a22
    s2 = s1 - a11
    return (a11, a12, a12 - s2, a22, s1, s2, a11 - a21)


def _wr(b11, b12, b21, b22):
    t1 = b12 - b11
    t2 = b22 - t1
    return (b11, b21, b22, t2 - b21, t1, t2, b22 - b12)


def _wc(p):
    p1, p2, p3, p4, p5, p6, p7 = p
    u2 = p1 + p6
    u3 = u2 + p7
    return p1 + p2, (u2 + p5) + p3, u3 - p4, u3 + p5


W_R = (3, 1, 0, 2, 4, 5, 6)


def _wl_swapped(a11, a12, a21, a22):
    return _wl(a12, a11, a22, a21)


def _wc_swapped(p):
    p1, p2, p3, p4, p5, p6, p7 = p
    v2 = p1 + p6
    u3 = p7 - v2
    return (p5 - v2) + p3, p1 + p2, u3 + p5, p4 - u3


class _Sym:
    def __init__(self, t):
        self.t = t

    def __add__(self, o):
        return _Sym({**self.t, **o.t})

    def __sub__(self, o):
        return _Sym({**self.t, **{k: -v for k, v in o.t.items()}})


def _st(u, ct):
    return slice((4 * ct + u) * 128, (4 * ct + u + 1) * 128)


def _to_st(v):
    return jnp.concatenate([v[:, (2 * u + ct) * 128:(2 * u + ct + 1) * 128]
                            for ct in range(2) for u in range(4)], axis=1)


def _phi(t):
    return jnp.where(t > 0, t + 1.0, jnp.exp(t)) + 1e-6


def _rbf(v):
    return v.astype(bf16).astype(f32)


def _kernel(x_hbm, wqkv_hbm, wo_hbm, wr_hbm, wg_hbm, wu_hbm, wd_hbm, out_hbm,
            x_buf, wk_buf, wv_buf, wo_buf, wr_buf, wg_buf, wu_buf, wd_buf,
            xs1, xs2, wqs, sa, sb, zacc, zp, pk_buf, xb, yacc, rsel, wrb, zero_buf,
            wks, stats, wqt, ps_raw, qs, ms, tscr, tscr2, pq_raw, den_raw, pqb_buf, denb_buf, qsb,
            mg_raw, hb_raw, out_buf, idx_s, sem):
    wq_buf = out_buf.at[pl.ds(0, D), :]

    def xs_at(k1, e, rows=None):
        r = xs1.at[k1 * 4 + (0, 1, 7, 3).index(e)] if e in (0, 1, 7, 3) else xs2.at[k1 * 4 + (2, 4, 5, 6).index(e)]
        return r if rows is None else r.at[rows, :]

    SEM_B, SEM_O, SEM_Z, SEM_A = 0, 2, 3, 4

    def cp(src, dst, s):
        return pltpu.make_async_copy(src, dst, sem.at[s])

    def cp_x(r0, n, s):
        r = pl.ds(_mo(r0, 16), n)
        return [cp(x_hbm.at[:, r, :], x_buf.at[:, r, :], s)]

    def cp_wk(c, s):
        return [cp(wqkv_hbm.at[:, pl.ds(_mo(D + c * 256, 256), 256)],
                   wk_buf.at[c], s)]

    NX = T0 // X0
    SEM_W = SEM_A + NX
    cp_wr = cp(wr_hbm, wr_buf.at[pl.ds(0, D)], SEM_Z)
    a_groups = [cp_x(i * X0, X0, SEM_A + i) for i in range(NX)] + [
        cp_wk(0, SEM_W),
        cp_wk(1, SEM_W + 1),
        cp_wk(2, SEM_W + 2) + cp_x(T0, XG[0] - T0, SEM_W + 2),
        cp_wk(3, SEM_W + 3) + cp_x(XG[0], XG[1] - XG[0], SEM_W + 3),
        cp_x(XG[1], HQ - XG[1], SEM_W + 4),
        [cp(wqkv_hbm.at[:, pl.ds(0, D)], wq_buf, SEM_W + 5)],
    ]

    def cp_b(j, wait_only=False):
        dsts = [r.at[j] for r in (wg_buf, wu_buf, wd_buf, wv_buf, wo_buf)]
        if wait_only:
            return [cp(dst, dst, SEM_B + j) for dst in dsts]
        fs = pl.ds(j * FH, FH)
        srcs = [wg_hbm.at[:, fs], wu_hbm.at[:, fs], wd_hbm.at[fs, :],
                wqkv_hbm.at[:, pl.ds(2 * D + j * HD, HD)], wo_hbm.at[pl.ds(j * HD, HD), :]]
        return [cp(src, dst, SEM_B + j) for src, dst in zip(srcs, dsts)]

    clock = [0]
    toks = []
    sides = []
    fwd = [None]

    def emit_tok(vals, stamp):
        t = None
        for v in vals:
            v = pltpu.bitcast(v, u32) if v.dtype != u32 else v
            t = v if t is None else t | v
        toks.append((stamp, t & zero_buf[0]))

    def token(kind):
        t = fwd[0]
        if "u" not in t:
            t["u"] = pltpu.bitcast(t["src"](), u32) & zero_buf[0]
        if kind != "u" and "f" not in t:
            t["f"] = pltpu.bitcast(t["u"], f32)
        if kind == "f16" and "f16" not in t:
            t["f16"] = jnp.concatenate([t["f"], t["f"]], axis=0)
        return t[kind]

    def gate(v):
        if fwd[0] is None:
            return v
        head = v if v.shape[0] == 8 else v[0:8]
        head = head | token("u") if v.dtype == u32 else head + token("f")
        return head if v.shape[0] == 8 else jnp.concatenate([head, v[8:]], axis=0)

    def gate16(v):
        return v if fwd[0] is None else v + token("f16")

    def add_side(gen_fn, n, t0, t1, lag=None):
        st = {"i": 0, "n": n, "t0": clock[0] + t0, "t1": clock[0] + t1}

        def tok(vals):
            if lag is not None:
                emit_tok(vals, st["t0"] + (st["i"] + 1) * (st["t1"] - st["t0"]) // st["n"] + lag)
        st["g"] = gen_fn(tok)
        sides.append(st)

    def advance(until):
        for st in sides:
            while st["i"] < st["n"] and st["t0"] + st["i"] * (st["t1"] - st["t0"]) // st["n"] < until:
                next(st["g"], None)
                st["i"] += 1
                if st["i"] == st["n"]:
                    for _ in st["g"]:
                        pass

    def flush():
        for st in sides:
            for _ in st["g"]:
                pass
        sides.clear()

    def finish():
        flush()
        toks.clear()
        fwd[0] = None

    def mm(lhs, rhs, dims, cycles, nseg=1):
        due = [t for (c, t) in toks if c <= clock[0]]
        toks[:] = [(c, t) for (c, t) in toks if c > clock[0]]
        if due:
            head = rhs[0:8, 0:128]
            for t in due:
                head = head | t
            if rhs.shape[1] > 128:
                head = jnp.concatenate([head, rhs[0:8, 128:]], axis=1)
            rhs = jnp.concatenate([head, rhs[8:]], axis=0)
        res = _dot(lhs, _unpack(rhs), dims)
        ngr = res.shape[0] // 16
        for sg in range(nseg):
            for i in range(ngr):
                fwd[0] = {"src": lambda sg=sg, i=i: res[i * 16:i * 16 + 8, sg * 128:(sg + 1) * 128]}
                clock[0] += cycles // nseg // ngr
                advance(clock[0])
        return res

    def form_steps(form, form2, get, put, tok=None, keep=range(7)):
        terms = form(*[_Sym({i: 1}) for i in range(4)])
        gated = (0, 1, 2, 3) if 7 in keep else {_wl: (0, 1, 3), _wr: (0, 2, 3), _wl_swapped: (1, 2)}[form2]
        for k1 in range(7):
            sub = []
            for r in range(2):
                for c in range(2):
                    v = None
                    for i, sg in sorted(terms[k1].t.items(), key=lambda e: -e[1]):
                        b = get(r + 2 * (i // 2), c + 2 * (i % 2))
                        if v is None:
                            v = gate16(b) if 2 * r + c in gated else b
                        else:
                            v = v + b if sg > 0 else v - b
                    sub.append(v)
            vals = form2(*sub) + (sub[2],)
            for k2 in keep:
                put(k1, k2, _pack(vals[k2]))
            if tok is not None and k1 % 2 == 0:
                full = vals[3 if form2 is _wr else 2]
                tok([full[0:8], full[8:16]])
            yield

    def strassen2(lhs, rhs, dims, cycles, nseg=1, wts=(16,) * 7, comb=_wc):
        m1 = [None] * 7
        for i1, k1 in enumerate(K_SEQ2):
            m2 = [None] * 7
            for k2 in W_SEQ:
                m2[k2] = mm(lhs(k1, k2), rhs(k1, k2), dims, cycles * wts[i1] // 16, nseg)
                yield
            m1[k1] = comb(m2)
        out = [[None] * 4 for _ in range(4)]
        for s2 in range(4):
            for s1, v in enumerate(_combine([m1[k1][s2] for k1 in range(7)])):
                out[(s1 // 2) * 2 + s2 // 2][(s1 % 2) * 2 + s2 % 2] = v
        return out

    made = set()

    def need(*keys):
        assert all(k in made for k in keys), keys

    def row_views(base):
        if base == 0:
            return x_buf, sa, sb, stats, xn_buf, None
        i, n = base
        b = _mo(i * n, 16)
        return ([x_buf.at[:, pl.ds(b, n), :]] + [r.at[pl.ds(b, S - 128 + n), :] for r in (sa, sb, stats)]
                + [xn_buf.at[:, pl.ds(b, n), :], pl.ds(_mo(i * (n // 2), 8), n // 2)])

    def xs_form(r0, tok, which="all", base=0):
        xn_v, xs_v = row_views(base)[4:]
        rows = slice(r0 % XN, r0 % XN + 16)

        keep = {"all": range(8), "l1": (0, 1, 7, 3), "l2": (2, 4, 5, 6)}[which]
        for ct in range(2):
            def put(k1, k2, v):
                xs_at(k1, k2, xs_v)[r0 // 2:r0 // 2 + 8, ct * 128:(ct + 1) * 128] = v
            yield from form_steps(
                _sform, _wl, lambda q, u: xn_v[q, rows, _st(u, ct)], put, tok, keep)
        made.add(("xs", r0))

    def ln_stats(r_start, n_rows, tok, base=0):
        x_v, sa_v, sb_v, st_v, xn_v, _ = row_views(base)
        lane = lax.broadcasted_iota(i32, (8, 128), 1)
        for r0 in range(r_start, r_start + n_rows, 16):
            if r0 >= T0:
                need(("in", 2 + sum(r0 >= g for g in XG)))
            if r0 - XN >= T0:
                need(("ln", r0 - XN))
            for g in range(8):
                q, o = g // 2, (g % 2) * 8
                rg = q * HQ + r0 + o
                xv = x_v[q, r0 + o:r0 + o + 8, :].astype(f32)
                xg = jnp.concatenate([gate(xv[:, 0:128]), xv[:, 128:]], axis=1)
                mf = jnp.sum(xg, axis=1, keepdims=True) * (1.0 / D)
                d = xv - mf
                var = jnp.sum(d * d, axis=1, keepdims=True) * (1.0 / D)
                rs = lax.rsqrt(var + 1e-5)
                xn_v.at[q][r0 % XN + o:r0 % XN + o + 8, :] = _to_st(d * rs)
                rs = jnp.broadcast_to(rs, (8, 128))
                mf = jnp.broadcast_to(mf, (8, 128))
                sa_v[rg:rg + 8, :] = 1.0 + rs
                sb_v[rg:rg + 8, :] = mf * rs
                st_v[rg:rg + 8, 0:128] = jnp.where(lane == 0, mf, jnp.broadcast_to(var, (8, 128)))
                if tok is not None:
                    tok([rs])
                if g == 7:
                    made.add(("xn", r0))
                yield

    def ln_later(r_start, n_rows, tok, which="all", base=0):
        st_v, xn_v = row_views(base)[3:5]
        for r0 in range(r_start, r_start + n_rows, 16):
            need(("xn", r0))
            form = xs_form(r0, tok, which, base)
            for g in range(8):
                for _ in range(2 if g < 7 else 0):
                    next(form)
                    yield
                q, o = g // 2, (g % 2) * 8
                t = None
                if which != "l1":
                    v = xn_v[q, r0 % XN + o:r0 % XN + o + 8, :] * wrb[8:16, :]
                    for ct in range(8):
                        h = v[:, ct * 128:(ct + 1) * 128]
                        t = gate(h) if t is None else t + h
                if t is not None:
                    st_v[q * HQ + r0 + o:q * HQ + r0 + o + 8, 128:256] = t
                if tok is not None:
                    tok([t])
                if g == 7:
                    next(form, None)
                    made.add(("ln", r0))
                yield

    def wk_prep(c):
        if isinstance(c, int):
            need(("in", c))
        wks.at[c][:, 128:256] = pltpu.bitcast(wk_buf[c, 0:HD, 0:128], u32)
        wks.at[c][:, 512:640] = pltpu.bitcast(wk_buf[c, HD:D, 128:256], u32)
        for i in range(HD // 16):
            r0 = i * 16
            top = wk_buf[c, r0:r0 + 16, :].astype(f32)
            bot = wk_buf[c, HD + r0:HD + r0 + 16, :].astype(f32)
            ops = _rform(top[:, :128], top[:, 128:], bot[:, :128], bot[:, 128:])
            for k in (0, 2, 3, 5, 6):
                wks.at[c][r0 // 2:r0 // 2 + 8, k * 128:(k + 1) * 128] = _pack(ops[k])

    def wq_perm():
        need(("in", 5))

        def permute(kt):
            for g in range(8):
                tile = gate(pltpu.bitcast(wq_buf[kt * 128:(kt + 1) * 128, g * 128:(g + 1) * 128], u32))
                wqt.at[kt * 8 + g][...] = pltpu.bitcast(_unpack(tile).T, u32)
                yield

        def back(kt):
            for j in range(8):
                tile = gate(jnp.concatenate([wqt[kt * 8 + g, pl.ds(j, 8, stride=8), :] for g in range(8)],
                                            axis=0))
                v = pltpu.bitcast(_unpack(tile).T.astype(f32), u32)
                c0 = (kt // 2) * D + _st(j // 2, j % 2).start
                ps[(kt % 2) * 128:(kt % 2 + 1) * 128, c0:c0 + 128] = v
                made.add(("wqp", kt, j))
                yield

        order = (0, 2, 4, 6, 1, 3, 5, 7)
        for n in range(10):
            if n < 8:
                yield from permute(order[n])
            if n > 1:
                yield from back(order[n - 2])

    def wq_form():
        for i in range(16):
            need(*[("wqp", 2 * r + i // 8, j) for r in range(4) for j in range(8)])
            for ct in range(2):
                def put(k1, k2, v):
                    wqs.at[k1 * 7 + k2][i * 8:(i + 1) * 8, ct * 128:(ct + 1) * 128] = v
                yield from form_steps(
                    _rform, _wr, lambda r, c: pltpu.bitcast(
                        ps[i * 16:(i + 1) * 16, r * D + _st(c, ct).start:r * D + _st(c, ct).stop],
                        f32), put)

    def kproj(r0, n, chunks=range(4)):
        pr = pl.ds(r0 // 2, n // 2)
        need(*[("xs", r) for r in range(max(r0, T0), r0 + n, 16)])
        for c in chunks:
            m = [None] * 7
            for k in K_SEQ:
                e11, e12, e21, e22 = [xs_at(L_ORD[k], e)[pr, :] for e in (0, 1, 7, 3)]
                lhs = jnp.concatenate([jnp.concatenate([e11, e12], axis=1),
                                       jnp.concatenate([e21, e22], axis=1)], axis=0)
                m[k] = mm(_unpack(lhs), wks[c, :, k * 128:(k + 1) * 128], NN, 2 * n)
            kk = [_phi(v) for v in _combine(m)]
            for ct in range(2):
                zacc[:, pl.ds(_mo(c * 256 + ct * 128, 128), 128)] += (
                    (kk[ct] + kk[2 + ct]).reshape(n // 4, 8, 128).sum(axis=0))
            j, c2 = (c // 2, c % 2) if isinstance(c, int) else (0, c)
            pk_v = pk_buf.at[j, :, :, pl.ds(_mo(c2 * 256, 256), 256)]
            for s1 in range(4):
                for h in range(2):
                    pk_v.at[(s1 // 2) * 2 + h][r0:r0 + n, (s1 % 2) * 128:(s1 % 2 + 1) * 128] = (
                        kk[s1][h * n:(h + 1) * n])

    def z_prep():
        z = jnp.sum(zacc[...], axis=0, keepdims=True)
        zt = _pack(jnp.broadcast_to(z, (128, D)).astype(bf16).T)
        for g in range(8):
            tscr.at[g][...] = zt[g * 64:(g + 1) * 64, :]
        for j in range(8):
            blk = jnp.concatenate([tscr[g, pl.ds(j, 8, stride=8), :] for g in range(8)], axis=0)
            zp[:, j * 128:(j + 1) * 128] = _unpack(blk).T[0:8, :].astype(f32)

    def route():
        rows, dots = [None] * 16, [None] * 16
        for b in sorted(range(S // 128), key=lambda b: b % 4):
            need(*[("ln", r) for r in range(max(T0, b % 4 * 128), b % 4 * 128 + 128, 16)])
            rows[b] = gate(stats[b * 128:(b + 1) * 128, 0:128]).T[0:8, :]
            dots[b] = jnp.sum(gate(stats[b * 128:(b + 1) * 128, 128:256]).T, axis=0, keepdims=True)
            yield
        mf = jnp.concatenate([v[0:1] for v in rows], axis=0)
        var = jnp.concatenate([v[1:2] for v in rows], axis=0)
        tr = jnp.concatenate(dots, axis=0) * jnp.sqrt(var + 1e-5)
        wsum = jnp.sum(wrb[0:1, :], axis=1, keepdims=True)
        mb = _rbf(mf)
        inv = 1.0 / _rbf(jnp.sqrt(_rbf(_rbf(var) + 1e-5)))
        rv = _rbf((tr + (mf - mb) * wsum) * inv)
        rmax = jnp.max(jnp.max(rv, axis=1, keepdims=True), axis=0, keepdims=True)
        pos = (lax.broadcasted_iota(i32, rv.shape, 0) * 128 + lax.broadcasted_iota(i32, rv.shape, 1))
        idx = jnp.min(jnp.where(rv == rmax, pos, S - 1))
        idx_s[0] = idx

        def pick(v):
            v = jnp.sum(jnp.where(pos == idx, v, 0.0), axis=1, keepdims=True)
            return jnp.sum(v, axis=0, keepdims=True)

        xv = x_buf[(idx >> 9) & 3, pl.ds(_mo(idx & (HQ - 16), 16), 16), :].astype(f32)
        sel = lax.broadcasted_iota(i32, xv.shape, 0) == (idx & 15)
        row = jnp.sum(jnp.where(sel, xv, 0.0), axis=0, keepdims=True)
        row = _rbf(_rbf(row - pick(mb)) * pick(inv))
        rsel[...] = jnp.broadcast_to(_rbf(jnp.sum(row * wrb[0:1, :], axis=1, keepdims=True)), rsel.shape)
        xb[...] = jnp.broadcast_to(row, (128, D)).T
        yield

    def ps_form(j):
        for c in range(HQ // 16):
            def put(k1, k2, v):
                k = k1 * 7 + k2
                ps[c * 8:(c + 1) * 8, k * 128:(k + 1) * 128] = v
            yield from form_steps(
                _lform, _wl_swapped,
                lambda r, q: pk_buf[j, q, c * 16:(c + 1) * 16, r * 128:(r + 1) * 128], put)

    def q_rows(j, r0, n, pq, rc, d0, rec):
        xj = pl.ds(_mo(j * (BQ // 2), BQ // 2), BQ // 2)
        pr = slice(r0 // 2, (r0 + n) // 2)
        blk = yield from strassen2(lambda k1, k2: _unpack(xs_at(L_ORD[k1], k2, xj)[pr, :]),
                                   lambda k1, k2: wqs[k1 * 7 + k2], NN, n, 1, QW)
        lane = lax.broadcasted_iota(i32, (n, 128), 1)
        for q in range(4):
            d = None
            for u in (3, 2, 1, 0):
                v = _phi(blk[q][u])
                for ct in range(2):
                    pq.at[q][d0:d0 + n, _st(u, ct)] = v[:, ct * 128:(ct + 1) * 128]
                t = v * zp[0:1, u * 256:(u + 1) * 256]
                t = t[:, :128] + t[:, 128:]
                d = t if d is None else d + t
            if rec:
                d = recip(d, lane)
            rc.at[q][d0:d0 + n, :] = d

    def recip(d, lane):
        d = d + jnp.where(lane % 2 == 0, pltpu.roll(d, 127, 1), pltpu.roll(d, 1, 1))
        d = d + jnp.where(lane % 4 < 2, pltpu.roll(d, 126, 1), pltpu.roll(d, 2, 1))
        return 1.0 / (d + 1e-6)

    def normalise(pq, rc, nr, dst, raw, tok=None):
        lane = lax.broadcasted_iota(i32, (16, 128), 1)

        def fix(c):
            if c < nr // 16 and raw(c * 16):
                for q in range(4):
                    rq = slice(c * 16, (c + 1) * 16)
                    rc.at[q][rq, :] = recip(gate16(rc[q, rq, :]), lane)

        def scale(c):
            rq = slice(c * 16, (c + 1) * 16)
            fix(c + 1)
            for hf in range(2):
                for q in range(4):
                    cs = slice(hf * HD, (hf + 1) * HD)
                    pq.at[q][rq, cs] = pq[q, rq, cs] * jnp.concatenate([gate16(rc[q, rq, :])] * 4, axis=1)
                    yield

        def form(c):
            rq = slice(c * 16, (c + 1) * 16)
            for ct in range(2):
                def put(k1, k2, v):
                    dst.at[k1 * 7 + k2][c * 8:(c + 1) * 8, ct * 128:(ct + 1) * 128] = v
                yield from form_steps(_lform, _wl, lambda q, u: pq[q, rq, _st(u, ct)], put, tok)

        fix(0)
        if raw(0):
            for _ in range(4):
                yield
        yield from scale(0)
        for c in range(nr // 16):
            nxt = scale(c + 1) if c + 1 < nr // 16 else iter(())
            for i, _ in enumerate(form(c)):
                yield
                if i < 8 and c + 1 < nr // 16:
                    next(nxt)
                    yield

    def g_kvm(j):
        qb = q_rows(j, BQ - QB, QB, pqb_buf.at[j], denb_buf.at[j], 0, False)
        for _ in range(QPRE):
            next(qb)
        blk = yield from strassen2(
            lambda k1, k2: _unpack(ps[:, (k1 * 7 + k2) * 128:(k1 * 7 + k2 + 1) * 128]),
            lambda k1, k2: xs_at(R_ORD[k1], W_R[k2])[...], TN, 256, 2, comb=_wc_swapped)
        hm = (lax.broadcasted_iota(i32, (128, 128), 0) // 32
              == lax.broadcasted_iota(i32, (128, 128), 1) // 32)
        for _ in range(QSPLIT - QPRE):
            next(qb)
        kvps = []
        for a in (3, 2, 1, 0):
            gg = jnp.concatenate(blk[a], axis=1).astype(bf16)
            wv_u = pltpu.bitcast(wv_buf[j, :, a * 128:(a + 1) * 128], u32)
            kv = jnp.where(hm, mm(gg, wv_u, NN, 256), 0.0)
            tscr2.at[a][...] = _pack(kv)
            kvps.append(_unpack(jnp.concatenate(
                [tscr2[a, pl.ds(jj, 8, stride=8), :] for jj in range(8)], axis=0)))

        ms_j = ms.at[:, pl.ds(_mo(j * 32, 32), 96), :]

        def m_form():
            for a in (3, 2, 1, 0):
                need(("mg", a))
                for jl in range(2):
                    for ct in range(2):
                        def put(k1, k2, v):
                            ms_j.at[k1 * 7 + k2][jl * 64 + a * 8:jl * 64 + (a + 1) * 8,
                                                 ct * 128:(ct + 1) * 128] = v
                        yield from form_steps(
                            _rform, _wr, lambda q, u: mg_buf[a, (2 * q + jl) * 16:(2 * q + jl + 1) * 16, _st(u, ct)], put)

        for i, a in enumerate((3, 2, 1, 0)):
            wo_u = pltpu.bitcast(wo_buf[j, a * 128:(a + 1) * 128, :], u32)
            res = mm(kvps[i], wo_u, NN, 256)
            mg_buf.at[a][...] = _to_st(res)
            made.add(("mg", a))
            if i == 0:
                add_side(lambda tok: m_form(), 112, *MF)
        for _ in qb:
            pass

    def out_part(base, span, off, nr, y, src):
        b = _mo(base, 32)
        sa_v, sb_v, out_v = [r.at[pl.ds(b, 3 * HQ + span), :] for r in (sa, sb, out_buf)]
        x_v = x_buf.at[:, pl.ds(b, span), :]
        row = lax.broadcasted_iota(i32, (nr, 256), 0) + (base + off)
        blk = yield from strassen2(lambda k1, k2: _unpack(src[k1 * 7 + k2, off // 2:(off + nr) // 2, :]),
                                   lambda k1, k2: ms[k1 * 7 + k2], NN, nr)
        for s1 in (3, 2, 1, 0):
            for s2 in range(4):
                q = (s1 // 2) * 2 + s2 // 2
                u = (s1 % 2) * 2 + s2 % 2
                rr, cc = pl.ds(q * HQ + off, nr), pl.ds(u * 256, 256)
                a = jnp.concatenate([sa_v[rr, :]] * 2, axis=1)
                c = jnp.concatenate([sb_v[rr, :]] * 2, axis=1)
                o = blk[q][u] + jnp.where(row + q * HQ == idx_s[0], y[:, u * 256:(u + 1) * 256], 0.0)
                out_v[rr, cc] = (x_v[q, off:off + nr, cc].astype(f32) * a - c + o).astype(bf16)
                if s2 % 2 == 1:
                    ch = pl.ds((s1 % 2) * HD, HD)
                    ro = pl.ds(_mo(base + q * HQ + off, 16), nr)
                    cp(out_buf.at[ro, ch], out_hbm.at[0, ro, ch], SEM_O).start()

    def ffn_part(j):
        def fma(acc, w, v):
            p = w.astype(f32) * v
            return acc + p[0:8] + p[8:16]

        for f0 in range(0, FH, 256):
            fs = slice(f0, f0 + 256)
            ag = jnp.zeros((8, 256), f32)
            au = jnp.zeros((8, 256), f32)
            for k in range(0, D, 16):
                xv = jnp.concatenate([gate16(xb[k:k + 16, :])] * 2, axis=1)
                ag = fma(ag, wg_buf[j, k:k + 16, fs], xv)
                au = fma(au, wu_buf[j, k:k + 16, fs], xv)
                yield
            g = _rbf(jnp.sum(ag, axis=0, keepdims=True))
            u = _rbf(jnp.sum(au, axis=0, keepdims=True))
            h = _rbf(_rbf(g * jax.nn.sigmoid(g)) * u)
            hb_buf[fs, :] = jnp.broadcast_to(h, (128, 256)).T
        for d0 in range(0, D, 512):
            ds_ = slice(d0, d0 + 512)
            acc = yacc[:, ds_]
            for k in range(0, FH, 16):
                hv = jnp.concatenate([gate16(hb_buf[k:k + 16, :])] * 4, axis=1)
                acc = fma(acc, wd_buf[j, k:k + 16, ds_], hv)
                yield
            yacc[:, ds_] = acc

    def wait_group(i):
        with _scope("a_wait%d" % i):
            for c in a_groups[i]:
                c.wait()
        made.add(("in", i - NX))

    def run_all(gen):
        for _ in gen:
            pass

    def ln_sides(plan):
        for r0, r1, t0, t1 in plan[0]:
            add_side(lambda tok, r0=r0, r1=r1: ln_stats(r0, r1 - r0, tok), (r1 - r0) // 2, t0, t1, LNLAG)
        for r0, r1, t0, t1 in plan[1]:
            add_side(lambda tok, r0=r0, r1=r1: ln_later(r0, r1 - r0, tok), 22 * (r1 - r0) // 16, t0, t1, SLAG)

    def l2_side(base, n, t0, t1):
        add_side(lambda tok: ln_later(0, n, None, "l2", base), 22 * n // 16, t0, t1)

    with _scope("p0_issue"):
        cp_wr.start()
        for grp in a_groups:
            for c in grp:
                c.start()
        for j in range(2):
            for c in cp_b(j):
                c.start()
        zacc[...] = jnp.zeros(zacc.shape, f32)
        yacc[...] = jnp.zeros(yacc.shape, f32)
        zero_buf[1] = jnp.zeros((8, 128), u32)
        cp_zero = cp(zero_buf.at[1], zero_buf.at[0], SEM_Z)
        cp_zero.start()
        cp_zero.wait()
        cp_wr.wait()
        wr8 = jnp.broadcast_to(wr_buf[0:D].reshape(1, D).astype(f32), (8, D))
        wrb[0:8, :] = wr8
        wrb[8:16, :] = _to_st(wr8)
        z0 = jnp.max(pltpu.bitcast(zero_buf[0], i32))
        ps, pq_buf, den_buf, mg_buf, hb_buf = [r.at[z0] for r in (ps_raw, pq_raw, den_raw, mg_raw, hb_raw)]
        xn_buf = mg_buf

    def main(_, carry0):
        def a01(i, carry):
            with _scope("a_wait01"):
                for c in cp_x(i * X0, X0, SEM_A + i):
                    c.wait()
            with _scope("a01"):
                for r in range(0, X0, 16):
                    run_all(ln_stats(r, 16, None, (i, X0)))
                    if r:
                        run_all(ln_later(r - 16, 16, None, "l1", (i, X0)))
                run_all(ln_later(X0 - 16, 16, None, "l1", (i, X0)))
            return carry

        lax.fori_loop(0, NX, a01, 0)
        made.update(("xn", r) for r in range(0, 64, 16))

        def a23(i, carry):
            with _scope("a_wait23"):
                for c in cp_wk(i, SEM_W + i):
                    c.wait()
            with _scope("a23"):
                wk_prep(i)
                l2_side((i, T0 // 2), T0 // 2, 250, 14 * T0 - 250)
                kproj(0, T0, [i])
                finish()
            return carry

        lax.fori_loop(0, 2, a23, 0)
        wait_group(NX + 2)
        with _scope("a4"):
            wk_prep(2)
            ln_sides(L4)
            kproj(0, T0, [2])
            finish()
        wait_group(NX + 3)
        with _scope("a5"):
            wk_prep(3)
            ln_sides(L5)
            kproj(0, T0, [3])
            for r0, n in A5K:
                kproj(r0, n)
            finish()
        wait_group(NX + 4)
        with _scope("a6"):
            ln_sides(L6)
            for r0, n in A6K:
                kproj(r0, n)
            finish()
        wait_group(NX + 5)
        with _scope("a7"):
            ln_sides(L7)
            add_side(lambda tok: wq_perm(), 128, *WQ_PERM)
            add_side(lambda tok: wq_form(), 224, *WQ_FORM)
            add_side(lambda tok: route(), 17, *ROUTE)
            for r0, n in A7K:
                kproj(r0, n)
            finish()

        def b_body(j, carry):
            qa = BQ - QB
            with _scope("b_r0"):
                z_prep()
                add_side(lambda tok: ps_form(j), 7 * HQ // 16, 0, 49 * qa - 400)
                for r0 in range(0, qa, QN):
                    run_all(q_rows(j, r0, QN, pq_buf, den_buf, r0, r0 + QN < qa))
                finish()
            with _scope("b_wait"):
                for c in cp_b(j, wait_only=True):
                    c.wait()
            with _scope("b_r1"):
                add_side(lambda tok: ffn_part(j), FH * 3 // 8, 0, R1T)
                qs_j = qs.at[:, pl.ds(_mo(j * (qa // 2), 16), qa // 2), :]
                add_side(lambda tok: normalise(pq_buf, den_buf, qa, qs_j, lambda r: r >= qa - QN),
                         22 * (qa // 16), 0, R1T)
                run_all(g_kvm(j))
                finish()
            return carry

        lax.fori_loop(0, 2, b_body, 0)

        def c_body(t, carry):
            with _scope("c_body"):
                y = _rbf(jnp.sum(yacc[...], axis=0, keepdims=True))
                y = _rbf(y * _rbf(1.0 / _rbf(1.0 + _rbf(jnp.exp(-rsel[0:1, :])))))
                j, h = t >> 1, t & 1
                na, nb = (BQ - QB) // 2, QB // 2
                hb = pl.ds(_mo(h * nb, 16), nb)
                add_side(lambda tok: normalise(pqb_buf.at[j, :, hb, :], denb_buf.at[j, :, hb, :], nb, qsb,
                                               lambda r: True, tok),
                         4 + 22 * (nb // 16), 0, 49 * na - 800, SLAG)
                qs_t = qs.at[:, pl.ds(_mo(t * (na // 2), 16), na // 2), :]
                for p in range(0, na, CR):
                    run_all(out_part(j * BQ + h * na, na, p, CR, y, qs_t))
                flush()
                run_all(out_part(j * BQ + BQ - QB + h * nb, nb, 0, nb, y, qsb))
                finish()
            return carry

        lax.fori_loop(0, 4, c_body, 0)
        return carry0

    lax.fori_loop(0, z0 + 1, main, 0)
    with _scope("tail"):
        cp(out_buf, out_hbm.at[0], SEM_O).wait()


@jax.jit
def pallas_parallel_sum__linear_attn_block__moe_arch_mod__prompt_kernel(
    A_x: jax.Array,
    A_wqkv: jax.Array,
    A_wo: jax.Array,
    B_x: jax.Array,
    B_w_r: jax.Array,
    B_w_gate: jax.Array,
    B_w_up: jax.Array,
    B_w_down: jax.Array,
):
    del B_x
    V = pltpu.VMEM
    scratch = [
        V((4, HQ, D), bf16),
        V((4, D, 256), bf16),
        V((2, D, 512), bf16),
        V((2, 512, D), bf16),
        V((8 * D,), bf16),
        V((2, D, FH), bf16),
        V((2, D, FH), bf16),
        V((2, FH, D), bf16),
        V((28, HQ // 2, 256), u32),
        V((28, HQ // 2, 256), u32),
        V((49, 128, 256), u32),
        V((S, 128), f32),
        V((S, 128), f32),
        V((8, D), f32),
        V((8, D), f32),
        V((2, 4, HQ, 512), f32),
        V((D, 128), f32),
        V((8, D), f32),
        V((8, D), f32),
        V((16, D), f32),
        V((4, 8, 128), u32),
        V((4, HD // 2, 7 * 128), u32),
        V((S, 256), f32),
        V((64, 64, 128), u32),
        V((1, HQ // 2, 49 * 128), u32),
        V((49, BQ - QB, 256), u32),
        V((49, 128, 256), u32),
        V((8, 64, 128), u32),
        V((4, 64, 128), u32),
        V((1, 4, BQ - QB, D), f32),
        V((1, 4, BQ - QB, 128), f32),
        V((2, 4, QB, D), f32),
        V((2, 4, QB, 128), f32),
        V((49, QB // 4, 256), u32),
        V((1, 4, 128, D), f32),
        V((1, FH, 128), f32),
        V((S, D), bf16),
        pltpu.SMEM((1,), i32),
        pltpu.SemaphoreType.DMA((4 + T0 // X0 + 6,)),
    ]
    extra = {k: True for k in ("disable_bounds_checks", "disable_semaphore_checks")
             if hasattr(pltpu.CompilerParams, k)}
    return pl.pallas_call(
        _kernel,
        out_shape=jax.ShapeDtypeStruct((1, S, D), bf16),
        in_specs=[pl.BlockSpec(memory_space=pl.ANY)] * 7,
        out_specs=pl.BlockSpec(memory_space=pl.ANY),
        scratch_shapes=scratch,
        compiler_params=pltpu.CompilerParams(vmem_limit_bytes=120 * 1024 * 1024, **extra),
    )(A_x.reshape(4, HQ, D), A_wqkv, A_wo, B_w_r, B_w_gate, B_w_up, B_w_down)
```

```python
import contextlib

import jax
import jax.numpy as jnp
from jax import lax
import jax.experimental.pallas as pl
import jax.experimental.pallas.tpu as pltpu

bf16, f32, u32, i32 = jnp.bfloat16, jnp.float32, jnp.uint32, jnp.int32

S = 2048
D = 1024
F = 3584
HD = D // 2
HQ = S // 4
BQ = HQ // 2
FH = F // 2
QB = 64
QN = 48
QPRE = 3
QSPLIT = 6
CR = 48
T0 = 96
X0 = 32
XG = (144, 176, 384)
XN = 128

SLAG = 400
LNLAG = 700
QW = (28, 36, 36, 6, 2, 2, 2)
L4 = ([(96, 144, 0, 1100)], [])
L5 = ([(144, 176, 500, 1600)], [(96, 128, 300, 1250), (128, 144, 1300, 1900), (144, 176, 2000, 2950)])
L6 = ([(176, 384, 0, 7200)], [(176, 224, 800, 2600), (224, 352, 2700, 7800)])
L7 = ([(384, 512, 0, 4400)], [(352, 384, 0, 1500), (384, 512, 1600, 8800)])
A5K = ((96, 32),)
A6K = ((128, 48), (176, 48), (224, 48))
A7K = ((272, 64), (336, 48), (384, 64), (448, 64))
WQ_PERM, WQ_FORM, ROUTE = (4700, 7600), (7700, 13100), (9200, 10000)
R1T = 12800
MF = (128, 3420)

L_ORD = (2, 3, 0, 1, 4, 5, 6)
R_ORD = (2, 0, 6, 5, 1, 4, 3)

K_SEQ = (1, 4, 0, 2, 3, 5, 6)
K_SEQ2 = (0, 1, 2, 5, 3, 4, 6)
W_SEQ = (0, 1, 5, 6, 4, 2, 3)

NN = (((1,), (0,)), ((), ()))
TN = (((0,), (0,)), ((), ()))


SCOPES = False


def _scope(name):
    return jax.named_scope(name) if SCOPES else contextlib.nullcontext()


def _mo(v, m):
    return v if isinstance(v, int) else pl.multiple_of(v, m)


def _dot(a, b, dims):
    return lax.dot_general(a, b, dims, preferred_element_type=f32)


def _pack(v):
    return pltpu.bitcast(v.astype(bf16), u32)


def _unpack(v):
    return pltpu.bitcast(v, bf16)


def _combine(m):
    m1, m2, m3, m4, m5, m6, m7 = m
    return m1 + m4 - m5 + m7, m3 + m5, m2 + m4, m1 - m2 + m3 + m6


def _lform(a11, a12, a21, a22):
    return (a11 + a22, a21 + a22, a11, a22, a11 + a12, a21 - a11, a12 - a22)


def _rform(b11, b12, b21, b22):
    return (b11 + b22, b11, b12 - b22, b21 - b11, b22, b11 + b12, b21 + b22)


def _sform(x11, x12, x21, x22):
    return (x11, x22, x11 + x22, x21 + x22, x11 + x12, x21 - x11, x12 - x22)


def _wl(a11, a12, a21, a22):
    s1 = a21 + a22
    s2 = s1 - a11
    return (a11, a12, a12 - s2, a22, s1, s2, a11 - a21)


def _wr(b11, b12, b21, b22):
    t1 = b12 - b11
    t2 = b22 - t1
    return (b11, b21, b22, t2 - b21, t1, t2, b22 - b12)


def _wc(p):
    p1, p2, p3, p4, p5, p6, p7 = p
    u2 = p1 + p6
    u3 = u2 + p7
    return p1 + p2, (u2 + p5) + p3, u3 - p4, u3 + p5


W_R = (3, 1, 0, 2, 4, 5, 6)


def _wl_swapped(a11, a12, a21, a22):
    return _wl(a12, a11, a22, a21)


def _wc_swapped(p):
    p1, p2, p3, p4, p5, p6, p7 = p
    v2 = p1 + p6
    u3 = p7 - v2
    return (p5 - v2) + p3, p1 + p2, u3 + p5, p4 - u3


class _Sym:
    def __init__(self, t):
        self.t = t

    def __add__(self, o):
        return _Sym({**self.t, **o.t})

    def __sub__(self, o):
        return _Sym({**self.t, **{k: -v for k, v in o.t.items()}})


def _st(u, ct):
    return slice((4 * ct + u) * 128, (4 * ct + u + 1) * 128)


def _to_st(v):
    return jnp.concatenate([v[:, (2 * u + ct) * 128:(2 * u + ct + 1) * 128]
                            for ct in range(2) for u in range(4)], axis=1)


def _phi(t):
    return jnp.where(t > 0, t + 1.0, jnp.exp(t)) + 1e-6


def _rbf(v):
    return v.astype(bf16).astype(f32)


def _kernel(x_hbm, wqkv_hbm, wo_hbm, wr_hbm, wg_hbm, wu_hbm, wd_hbm, out_hbm,
            x_buf, wk_buf, wv_buf, wo_buf, wr_buf, wg_buf, wu_buf, wd_buf,
            xs1, xs2, wqs, sa, sb, zacc, zp, pk_buf, xb, yacc, rsel, wrb, zero_buf,
            wks, stats, wqt, ps_raw, qs, ms, tscr, tscr2, pq_raw, den_raw, pqb_buf, denb_buf, qsb,
            mg_raw, hb_raw, out_buf, idx_s, sem):
    wq_buf = out_buf.at[pl.ds(0, D), :]

    def xs_at(k1, e, rows=None):
        r = xs1.at[k1 * 4 + (0, 1, 7, 3).index(e)] if e in (0, 1, 7, 3) else xs2.at[k1 * 4 + (2, 4, 5, 6).index(e)]
        return r if rows is None else r.at[rows, :]

    SEM_B, SEM_O, SEM_Z, SEM_A = 0, 2, 3, 4

    def cp(src, dst, s):
        return pltpu.make_async_copy(src, dst, sem.at[s])

    def cp_x(r0, n, s):
        r = pl.ds(_mo(r0, 16), n)
        return [cp(x_hbm.at[:, r, :], x_buf.at[:, r, :], s)]

    def cp_wk(c, s):
        return [cp(wqkv_hbm.at[:, pl.ds(_mo(D + c * 256, 256), 256)],
                   wk_buf.at[c], s)]

    NX = T0 // X0
    SEM_W = SEM_A + NX
    cp_wr = cp(wr_hbm, wr_buf.at[pl.ds(0, D)], SEM_Z)
    a_groups = [cp_x(i * X0, X0, SEM_A + i) for i in range(NX)] + [
        cp_wk(0, SEM_W),
        cp_wk(1, SEM_W + 1),
        cp_wk(2, SEM_W + 2) + cp_x(T0, XG[0] - T0, SEM_W + 2),
        cp_wk(3, SEM_W + 3) + cp_x(XG[0], XG[1] - XG[0], SEM_W + 3),
        cp_x(XG[1], XG[2] - XG[1], SEM_W + 4),
        (cp_x(XG[2], HQ - XG[2], SEM_W + 5) if XG[2] < HQ else [])
        + [cp(wqkv_hbm.at[:, pl.ds(0, D)], wq_buf, SEM_W + 5)],
    ]

    def cp_b(j, wait_only=False):
        dsts = [r.at[j] for r in (wg_buf, wu_buf, wd_buf, wv_buf, wo_buf)]
        if wait_only:
            return [cp(dst, dst, SEM_B + j) for dst in dsts]
        fs = pl.ds(j * FH, FH)
        srcs = [wg_hbm.at[:, fs], wu_hbm.at[:, fs], wd_hbm.at[fs, :],
                wqkv_hbm.at[:, pl.ds(2 * D + j * HD, HD)], wo_hbm.at[pl.ds(j * HD, HD), :]]
        return [cp(src, dst, SEM_B + j) for src, dst in zip(srcs, dsts)]

    clock = [0]
    toks = []
    sides = []
    fwd = [None]

    def emit_tok(vals, stamp):
        t = None
        for v in vals:
            v = pltpu.bitcast(v, u32) if v.dtype != u32 else v
            t = v if t is None else t | v
        toks.append((stamp, t & zero_buf[0]))

    def token(kind):
        t = fwd[0]
        if "u" not in t:
            t["u"] = pltpu.bitcast(t["src"](), u32) & zero_buf[0]
        if kind != "u" and "f" not in t:
            t["f"] = pltpu.bitcast(t["u"], f32)
        if kind == "f16" and "f16" not in t:
            t["f16"] = jnp.concatenate([t["f"], t["f"]], axis=0)
        return t[kind]

    def gate(v):
        if fwd[0] is None:
            return v
        head = v if v.shape[0] == 8 else v[0:8]
        head = head | token("u") if v.dtype == u32 else head + token("f")
        return head if v.shape[0] == 8 else jnp.concatenate([head, v[8:]], axis=0)

    def gate16(v):
        return v if fwd[0] is None else v + token("f16")

    def add_side(gen_fn, n, t0, t1, lag=None):
        st = {"i": 0, "n": n, "t0": clock[0] + t0, "t1": clock[0] + t1}

        def tok(vals):
            if lag is not None:
                emit_tok(vals, st["t0"] + (st["i"] + 1) * (st["t1"] - st["t0"]) // st["n"] + lag)
        st["g"] = gen_fn(tok)
        sides.append(st)

    def advance(until):
        for st in sides:
            while st["i"] < st["n"] and st["t0"] + st["i"] * (st["t1"] - st["t0"]) // st["n"] < until:
                next(st["g"], None)
                st["i"] += 1
                if st["i"] == st["n"]:
                    for _ in st["g"]:
                        pass

    def flush():
        for st in sides:
            for _ in st["g"]:
                pass
        sides.clear()

    def finish():
        flush()
        toks.clear()
        fwd[0] = None

    def mm(lhs, rhs, dims, cycles, nseg=1):
        due = [t for (c, t) in toks if c <= clock[0]]
        toks[:] = [(c, t) for (c, t) in toks if c > clock[0]]
        if due:
            head = rhs[0:8, 0:128]
            for t in due:
                head = head | t
            if rhs.shape[1] > 128:
                head = jnp.concatenate([head, rhs[0:8, 128:]], axis=1)
            rhs = jnp.concatenate([head, rhs[8:]], axis=0)
        res = _dot(lhs, _unpack(rhs), dims)
        ngr = res.shape[0] // 16
        for sg in range(nseg):
            for i in range(ngr):
                fwd[0] = {"src": lambda sg=sg, i=i: res[i * 16:i * 16 + 8, sg * 128:(sg + 1) * 128]}
                clock[0] += cycles // nseg // ngr
                advance(clock[0])
        return res

    def form_steps(form, form2, get, put, tok=None, keep=range(7)):
        terms = form(*[_Sym({i: 1}) for i in range(4)])
        gated = (0, 1, 2, 3) if 7 in keep else {_wl: (0, 1, 3), _wr: (0, 2, 3), _wl_swapped: (1, 2)}[form2]
        for k1 in range(7):
            sub = []
            for r in range(2):
                for c in range(2):
                    v = None
                    for i, sg in sorted(terms[k1].t.items(), key=lambda e: -e[1]):
                        b = get(r + 2 * (i // 2), c + 2 * (i % 2))
                        if v is None:
                            v = gate16(b) if 2 * r + c in gated else b
                        else:
                            v = v + b if sg > 0 else v - b
                    sub.append(v)
            vals = form2(*sub) + (sub[2],)
            for k2 in keep:
                put(k1, k2, _pack(vals[k2]))
            if tok is not None and k1 % 2 == 0:
                full = vals[3 if form2 is _wr else 2]
                tok([full[0:8], full[8:16]])
            yield

    def strassen2(lhs, rhs, dims, cycles, nseg=1, wts=(16,) * 7, comb=_wc):
        m1 = [None] * 7
        for i1, k1 in enumerate(K_SEQ2):
            m2 = [None] * 7
            for k2 in W_SEQ:
                m2[k2] = mm(lhs(k1, k2), rhs(k1, k2), dims, cycles * wts[i1] // 16, nseg)
                yield
            m1[k1] = comb(m2)
        out = [[None] * 4 for _ in range(4)]
        for s2 in range(4):
            for s1, v in enumerate(_combine([m1[k1][s2] for k1 in range(7)])):
                out[(s1 // 2) * 2 + s2 // 2][(s1 % 2) * 2 + s2 % 2] = v
        return out

    made = set()

    def need(*keys):
        assert all(k in made for k in keys), keys

    def row_views(base):
        if base == 0:
            return x_buf, sa, sb, stats, xn_buf, None
        i, n = base
        b = _mo(i * n, 16)
        return ([x_buf.at[:, pl.ds(b, n), :]] + [r.at[pl.ds(b, S - 128 + n), :] for r in (sa, sb, stats)]
                + [xn_buf.at[:, pl.ds(b, n), :], pl.ds(_mo(i * (n // 2), 8), n // 2)])

    def xs_form(r0, tok, which="all", base=0):
        xn_v, xs_v = row_views(base)[4:]
        rows = slice(r0 % XN, r0 % XN + 16)

        keep = {"all": range(8), "l1": (0, 1, 7, 3), "l2": (2, 4, 5, 6)}[which]
        for ct in range(2):
            def put(k1, k2, v):
                xs_at(k1, k2, xs_v)[r0 // 2:r0 // 2 + 8, ct * 128:(ct + 1) * 128] = v
            yield from form_steps(
                _sform, _wl, lambda q, u: xn_v[q, rows, _st(u, ct)], put, tok, keep)
        made.add(("xs", r0))

    def ln_stats(r_start, n_rows, tok, base=0):
        x_v, sa_v, sb_v, st_v, xn_v, _ = row_views(base)
        lane = lax.broadcasted_iota(i32, (8, 128), 1)
        for r0 in range(r_start, r_start + n_rows, 16):
            if r0 >= T0:
                need(("in", 2 + sum(r0 >= g for g in XG)))
            if r0 - XN >= T0:
                need(("ln", r0 - XN))
            for g in range(8):
                q, o = g // 2, (g % 2) * 8
                rg = q * HQ + r0 + o
                xv = x_v[q, r0 + o:r0 + o + 8, :].astype(f32)
                xg = jnp.concatenate([gate(xv[:, 0:128]), xv[:, 128:]], axis=1)
                mf = jnp.sum(xg, axis=1, keepdims=True) * (1.0 / D)
                d = xv - mf
                var = jnp.sum(d * d, axis=1, keepdims=True) * (1.0 / D)
                rs = lax.rsqrt(var + 1e-5)
                xn_v.at[q][r0 % XN + o:r0 % XN + o + 8, :] = _to_st(d * rs)
                rs = jnp.broadcast_to(rs, (8, 128))
                mf = jnp.broadcast_to(mf, (8, 128))
                sa_v[rg:rg + 8, :] = 1.0 + rs
                sb_v[rg:rg + 8, :] = mf * rs
                st_v[rg:rg + 8, 0:128] = jnp.where(lane == 0, mf, jnp.broadcast_to(var, (8, 128)))
                if tok is not None:
                    tok([rs])
                if g == 7:
                    made.add(("xn", r0))
                yield

    def ln_later(r_start, n_rows, tok, which="all", base=0):
        st_v, xn_v = row_views(base)[3:5]
        for r0 in range(r_start, r_start + n_rows, 16):
            need(("xn", r0))
            form = xs_form(r0, tok, which, base)
            for g in range(8):
                for _ in range(2 if g < 7 else 0):
                    next(form)
                    yield
                q, o = g // 2, (g % 2) * 8
                t = None
                if which != "l1":
                    v = xn_v[q, r0 % XN + o:r0 % XN + o + 8, :] * wrb[8:16, :]
                    for ct in range(8):
                        h = v[:, ct * 128:(ct + 1) * 128]
                        t = gate(h) if t is None else t + h
                if t is not None:
                    st_v[q * HQ + r0 + o:q * HQ + r0 + o + 8, 128:256] = t
                if tok is not None:
                    tok([t])
                if g == 7:
                    next(form, None)
                    made.add(("ln", r0))
                yield

    def wk_prep(c):
        if isinstance(c, int):
            need(("in", c))
        wks.at[c][:, 128:256] = pltpu.bitcast(wk_buf[c, 0:HD, 0:128], u32)
        wks.at[c][:, 512:640] = pltpu.bitcast(wk_buf[c, HD:D, 128:256], u32)
        for i in range(HD // 16):
            r0 = i * 16
            top = wk_buf[c, r0:r0 + 16, :].astype(f32)
            bot = wk_buf[c, HD + r0:HD + r0 + 16, :].astype(f32)
            ops = _rform(top[:, :128], top[:, 128:], bot[:, :128], bot[:, 128:])
            for k in (0, 2, 3, 5, 6):
                wks.at[c][r0 // 2:r0 // 2 + 8, k * 128:(k + 1) * 128] = _pack(ops[k])

    def wq_perm():
        need(("in", 5))

        def permute(kt):
            for g in range(8):
                tile = gate(pltpu.bitcast(wq_buf[kt * 128:(kt + 1) * 128, g * 128:(g + 1) * 128], u32))
                wqt.at[kt * 8 + g][...] = pltpu.bitcast(_unpack(tile).T, u32)
                yield

        def back(kt):
            for j in range(8):
                tile = gate(jnp.concatenate([wqt[kt * 8 + g, pl.ds(j, 8, stride=8), :] for g in range(8)],
                                            axis=0))
                v = pltpu.bitcast(_unpack(tile).T.astype(f32), u32)
                c0 = (kt // 2) * D + _st(j // 2, j % 2).start
                ps[(kt % 2) * 128:(kt % 2 + 1) * 128, c0:c0 + 128] = v
                made.add(("wqp", kt, j))
                yield

        order = (0, 2, 4, 6, 1, 3, 5, 7)
        for n in range(10):
            if n < 8:
                yield from permute(order[n])
            if n > 1:
                yield from back(order[n - 2])

    def wq_form():
        for i in range(16):
            need(*[("wqp", 2 * r + i // 8, j) for r in range(4) for j in range(8)])
            for ct in range(2):
                def put(k1, k2, v):
                    wqs.at[k1 * 7 + k2][i * 8:(i + 1) * 8, ct * 128:(ct + 1) * 128] = v
                yield from form_steps(
                    _rform, _wr, lambda r, c: pltpu.bitcast(
                        ps[i * 16:(i + 1) * 16, r * D + _st(c, ct).start:r * D + _st(c, ct).stop],
                        f32), put)

    def kproj(r0, n, chunks=range(4)):
        pr = pl.ds(r0 // 2, n // 2)
        need(*[("xs", r) for r in range(max(r0, T0), r0 + n, 16)])
        for c in chunks:
            m = [None] * 7
            for k in K_SEQ:
                e11, e12, e21, e22 = [xs_at(L_ORD[k], e)[pr, :] for e in (0, 1, 7, 3)]
                lhs = jnp.concatenate([jnp.concatenate([e11, e12], axis=1),
                                       jnp.concatenate([e21, e22], axis=1)], axis=0)
                m[k] = mm(_unpack(lhs), wks[c, :, k * 128:(k + 1) * 128], NN, 2 * n)
            kk = [_phi(v) for v in _combine(m)]
            for ct in range(2):
                zacc[:, pl.ds(_mo(c * 256 + ct * 128, 128), 128)] += (
                    (kk[ct] + kk[2 + ct]).reshape(n // 4, 8, 128).sum(axis=0))
            j, c2 = (c // 2, c % 2) if isinstance(c, int) else (0, c)
            pk_v = pk_buf.at[j, :, :, pl.ds(_mo(c2 * 256, 256), 256)]
            for s1 in range(4):
                for h in range(2):
                    pk_v.at[(s1 // 2) * 2 + h][r0:r0 + n, (s1 % 2) * 128:(s1 % 2 + 1) * 128] = (
                        kk[s1][h * n:(h + 1) * n])

    def z_prep():
        z = jnp.sum(zacc[...], axis=0, keepdims=True)
        zt = _pack(jnp.broadcast_to(z, (128, D)).astype(bf16).T)
        for g in range(8):
            tscr.at[g][...] = zt[g * 64:(g + 1) * 64, :]
        for j in range(8):
            blk = jnp.concatenate([tscr[g, pl.ds(j, 8, stride=8), :] for g in range(8)], axis=0)
            zp[:, j * 128:(j + 1) * 128] = _unpack(blk).T[0:8, :].astype(f32)

    def route():
        rows, dots = [None] * 16, [None] * 16
        for b in sorted(range(S // 128), key=lambda b: b % 4):
            need(*[("ln", r) for r in range(max(T0, b % 4 * 128), b % 4 * 128 + 128, 16)])
            rows[b] = gate(stats[b * 128:(b + 1) * 128, 0:128]).T[0:8, :]
            dots[b] = jnp.sum(gate(stats[b * 128:(b + 1) * 128, 128:256]).T, axis=0, keepdims=True)
            yield
        mf = jnp.concatenate([v[0:1] for v in rows], axis=0)
        var = jnp.concatenate([v[1:2] for v in rows], axis=0)
        tr = jnp.concatenate(dots, axis=0) * jnp.sqrt(var + 1e-5)
        wsum = jnp.sum(wrb[0:1, :], axis=1, keepdims=True)
        mb = _rbf(mf)
        inv = 1.0 / _rbf(jnp.sqrt(_rbf(_rbf(var) + 1e-5)))
        rv = _rbf((tr + (mf - mb) * wsum) * inv)
        rmax = jnp.max(jnp.max(rv, axis=1, keepdims=True), axis=0, keepdims=True)
        pos = (lax.broadcasted_iota(i32, rv.shape, 0) * 128 + lax.broadcasted_iota(i32, rv.shape, 1))
        idx = jnp.min(jnp.where(rv == rmax, pos, S - 1))
        idx_s[0] = idx

        def pick(v):
            v = jnp.sum(jnp.where(pos == idx, v, 0.0), axis=1, keepdims=True)
            return jnp.sum(v, axis=0, keepdims=True)

        xv = x_buf[(idx >> 9) & 3, pl.ds(_mo(idx & (HQ - 16), 16), 16), :].astype(f32)
        sel = lax.broadcasted_iota(i32, xv.shape, 0) == (idx & 15)
        row = jnp.sum(jnp.where(sel, xv, 0.0), axis=0, keepdims=True)
        row = _rbf(_rbf(row - pick(mb)) * pick(inv))
        rsel[...] = jnp.broadcast_to(_rbf(jnp.sum(row * wrb[0:1, :], axis=1, keepdims=True)), rsel.shape)
        xb[...] = jnp.broadcast_to(row, (128, D)).T
        yield

    def ps_form(j):
        for c in range(HQ // 16):
            def put(k1, k2, v):
                k = k1 * 7 + k2
                ps[c * 8:(c + 1) * 8, k * 128:(k + 1) * 128] = v
            yield from form_steps(
                _lform, _wl_swapped,
                lambda r, q: pk_buf[j, q, c * 16:(c + 1) * 16, r * 128:(r + 1) * 128], put)

    def q_rows(j, r0, n, pq, rc, d0, rec):
        xj = pl.ds(_mo(j * (BQ // 2), BQ // 2), BQ // 2)
        pr = slice(r0 // 2, (r0 + n) // 2)
        blk = yield from strassen2(lambda k1, k2: _unpack(xs_at(L_ORD[k1], k2, xj)[pr, :]),
                                   lambda k1, k2: wqs[k1 * 7 + k2], NN, n, 1, QW)
        lane = lax.broadcasted_iota(i32, (n, 128), 1)
        for q in range(4):
            d = None
            for u in (3, 2, 1, 0):
                v = _phi(blk[q][u])
                for ct in range(2):
                    pq.at[q][d0:d0 + n, _st(u, ct)] = v[:, ct * 128:(ct + 1) * 128]
                t = v * zp[0:1, u * 256:(u + 1) * 256]
                t = t[:, :128] + t[:, 128:]
                d = t if d is None else d + t
            if rec:
                d = recip(d, lane)
            rc.at[q][d0:d0 + n, :] = d

    def recip(d, lane):
        d = d + jnp.where(lane % 2 == 0, pltpu.roll(d, 127, 1), pltpu.roll(d, 1, 1))
        d = d + jnp.where(lane % 4 < 2, pltpu.roll(d, 126, 1), pltpu.roll(d, 2, 1))
        return 1.0 / (d + 1e-6)

    def normalise(pq, rc, nr, dst, raw, tok=None):
        lane = lax.broadcasted_iota(i32, (16, 128), 1)

        def fix(c):
            if c < nr // 16 and raw(c * 16):
                for q in range(4):
                    rq = slice(c * 16, (c + 1) * 16)
                    rc.at[q][rq, :] = recip(gate16(rc[q, rq, :]), lane)

        def scale(c):
            rq = slice(c * 16, (c + 1) * 16)
            fix(c + 1)
            for hf in range(2):
                for q in range(4):
                    cs = slice(hf * HD, (hf + 1) * HD)
                    pq.at[q][rq, cs] = pq[q, rq, cs] * jnp.concatenate([gate16(rc[q, rq, :])] * 4, axis=1)
                    yield

        def form(c):
            rq = slice(c * 16, (c + 1) * 16)
            for ct in range(2):
                def put(k1, k2, v):
                    dst.at[k1 * 7 + k2][c * 8:(c + 1) * 8, ct * 128:(ct + 1) * 128] = v
                yield from form_steps(_lform, _wl, lambda q, u: pq[q, rq, _st(u, ct)], put, tok)

        fix(0)
        if raw(0):
            for _ in range(4):
                yield
        yield from scale(0)
        for c in range(nr // 16):
            nxt = scale(c + 1) if c + 1 < nr // 16 else iter(())
            for i, _ in enumerate(form(c)):
                yield
                if i < 8 and c + 1 < nr // 16:
                    next(nxt)
                    yield

    def g_kvm(j):
        qb = q_rows(j, BQ - QB, QB, pqb_buf.at[j], denb_buf.at[j], 0, False)
        for _ in range(QPRE):
            next(qb)
        blk = yield from strassen2(
            lambda k1, k2: _unpack(ps[:, (k1 * 7 + k2) * 128:(k1 * 7 + k2 + 1) * 128]),
            lambda k1, k2: xs_at(R_ORD[k1], W_R[k2])[...], TN, 256, 2, comb=_wc_swapped)
        hm = (lax.broadcasted_iota(i32, (128, 128), 0) // 32
              == lax.broadcasted_iota(i32, (128, 128), 1) // 32)
        for _ in range(QSPLIT - QPRE):
            next(qb)
        kvps = []
        for a in (3, 2, 1, 0):
            gg = jnp.concatenate(blk[a], axis=1).astype(bf16)
            wv_u = pltpu.bitcast(wv_buf[j, :, a * 128:(a + 1) * 128], u32)
            kv = jnp.where(hm, mm(gg, wv_u, NN, 256), 0.0)
            tscr2.at[a][...] = _pack(kv)
            kvps.append(_unpack(jnp.concatenate(
                [tscr2[a, pl.ds(jj, 8, stride=8), :] for jj in range(8)], axis=0)))

        ms_j = ms.at[:, pl.ds(_mo(j * 32, 32), 96), :]

        def m_form():
            for a in (3, 2, 1, 0):
                need(("mg", a))
                for jl in range(2):
                    for ct in range(2):
                        def put(k1, k2, v):
                            ms_j.at[k1 * 7 + k2][jl * 64 + a * 8:jl * 64 + (a + 1) * 8,
                                                 ct * 128:(ct + 1) * 128] = v
                        yield from form_steps(
                            _rform, _wr, lambda q, u: mg_buf[a, (2 * q + jl) * 16:(2 * q + jl + 1) * 16, _st(u, ct)], put)

        for i, a in enumerate((3, 2, 1, 0)):
            wo_u = pltpu.bitcast(wo_buf[j, a * 128:(a + 1) * 128, :], u32)
            res = mm(kvps[i], wo_u, NN, 256)
            mg_buf.at[a][...] = _to_st(res)
            made.add(("mg", a))
            if i == 0:
                add_side(lambda tok: m_form(), 112, *MF)
        for _ in qb:
            pass

    def out_part(base, span, off, nr, y, src):
        b = _mo(base, 32)
        sa_v, sb_v, out_v = [r.at[pl.ds(b, 3 * HQ + span), :] for r in (sa, sb, out_buf)]
        x_v = x_buf.at[:, pl.ds(b, span), :]
        row = lax.broadcasted_iota(i32, (nr, 256), 0) + (base + off)
        blk = yield from strassen2(lambda k1, k2: _unpack(src[k1 * 7 + k2, off // 2:(off + nr) // 2, :]),
                                   lambda k1, k2: ms[k1 * 7 + k2], NN, nr)
        for s1 in (3, 2, 1, 0):
            for s2 in range(4):
                q = (s1 // 2) * 2 + s2 // 2
                u = (s1 % 2) * 2 + s2 % 2
                rr, cc = pl.ds(q * HQ + off, nr), pl.ds(u * 256, 256)
                a = jnp.concatenate([sa_v[rr, :]] * 2, axis=1)
                c = jnp.concatenate([sb_v[rr, :]] * 2, axis=1)
                o = blk[q][u] + jnp.where(row + q * HQ == idx_s[0], y[:, u * 256:(u + 1) * 256], 0.0)
                out_v[rr, cc] = (x_v[q, off:off + nr, cc].astype(f32) * a - c + o).astype(bf16)
                if s2 % 2 == 1:
                    ch = pl.ds((s1 % 2) * HD, HD)
                    ro = pl.ds(_mo(base + q * HQ + off, 16), nr)
                    cp(out_buf.at[ro, ch], out_hbm.at[0, ro, ch], SEM_O).start()

    def ffn_part(j):
        def fma(acc, w, v):
            p = w.astype(f32) * v
            return acc + p[0:8] + p[8:16]

        for f0 in range(0, FH, 256):
            fs = slice(f0, f0 + 256)
            ag = jnp.zeros((8, 256), f32)
            au = jnp.zeros((8, 256), f32)
            for k in range(0, D, 16):
                xv = jnp.concatenate([gate16(xb[k:k + 16, :])] * 2, axis=1)
                ag = fma(ag, wg_buf[j, k:k + 16, fs], xv)
                au = fma(au, wu_buf[j, k:k + 16, fs], xv)
                yield
            g = _rbf(jnp.sum(ag, axis=0, keepdims=True))
            u = _rbf(jnp.sum(au, axis=0, keepdims=True))
            h = _rbf(_rbf(g * jax.nn.sigmoid(g)) * u)
            hb_buf[fs, :] = jnp.broadcast_to(h, (128, 256)).T
        for d0 in range(0, D, 512):
            ds_ = slice(d0, d0 + 512)
            acc = yacc[:, ds_]
            for k in range(0, FH, 16):
                hv = jnp.concatenate([gate16(hb_buf[k:k + 16, :])] * 4, axis=1)
                acc = fma(acc, wd_buf[j, k:k + 16, ds_], hv)
                yield
            yacc[:, ds_] = acc

    def wait_group(i):
        with _scope("a_wait%d" % i):
            for c in a_groups[i]:
                c.wait()
        made.add(("in", i - NX))

    def run_all(gen):
        for _ in gen:
            pass

    def ln_sides(plan):
        for r0, r1, t0, t1 in plan[0]:
            add_side(lambda tok, r0=r0, r1=r1: ln_stats(r0, r1 - r0, tok), (r1 - r0) // 2, t0, t1, LNLAG)
        for r0, r1, t0, t1 in plan[1]:
            add_side(lambda tok, r0=r0, r1=r1: ln_later(r0, r1 - r0, tok), 22 * (r1 - r0) // 16, t0, t1, SLAG)

    def l2_side(base, n, t0, t1):
        add_side(lambda tok: ln_later(0, n, None, "l2", base), 22 * n // 16, t0, t1)

    with _scope("p0_issue"):
        cp_wr.start()
        for grp in a_groups:
            for c in grp:
                c.start()
        for j in range(2):
            for c in cp_b(j):
                c.start()
        zacc[...] = jnp.zeros(zacc.shape, f32)
        yacc[...] = jnp.zeros(yacc.shape, f32)
        zero_buf[1] = jnp.zeros((8, 128), u32)
        cp_zero = cp(zero_buf.at[1], zero_buf.at[0], SEM_Z)
        cp_zero.start()
        cp_zero.wait()
        cp_wr.wait()
        wr8 = jnp.broadcast_to(wr_buf[0:D].reshape(1, D).astype(f32), (8, D))
        wrb[0:8, :] = wr8
        wrb[8:16, :] = _to_st(wr8)
        z0 = jnp.max(pltpu.bitcast(zero_buf[0], i32))
        ps, pq_buf, den_buf, mg_buf, hb_buf = [r.at[z0] for r in (ps_raw, pq_raw, den_raw, mg_raw, hb_raw)]
        xn_buf = mg_buf

    def main(_, carry0):
        def a01(i, carry):
            with _scope("a_wait01"):
                for c in cp_x(i * X0, X0, SEM_A + i):
                    c.wait()
            with _scope("a01"):
                for r in range(0, X0, 16):
                    run_all(ln_stats(r, 16, None, (i, X0)))
                    if r:
                        run_all(ln_later(r - 16, 16, None, "l1", (i, X0)))
                run_all(ln_later(X0 - 16, 16, None, "l1", (i, X0)))
            return carry

        lax.fori_loop(0, NX, a01, 0)
        made.update(("xn", r) for r in range(0, 64, 16))

        def a23(i, carry):
            with _scope("a_wait23"):
                for c in cp_wk(i, SEM_W + i):
                    c.wait()
            with _scope("a23"):
                wk_prep(i)
                l2_side((i, T0 // 2), T0 // 2, 250, 14 * T0 - 250)
                kproj(0, T0, [i])
                finish()
            return carry

        lax.fori_loop(0, 2, a23, 0)
        wait_group(NX + 2)
        with _scope("a4"):
            wk_prep(2)
            ln_sides(L4)
            kproj(0, T0, [2])
            finish()
        wait_group(NX + 3)
        with _scope("a5"):
            wk_prep(3)
            ln_sides(L5)
            kproj(0, T0, [3])
            for r0, n in A5K:
                kproj(r0, n)
            finish()
        wait_group(NX + 4)
        with _scope("a6"):
            ln_sides(L6)
            for r0, n in A6K:
                kproj(r0, n)
            finish()
        wait_group(NX + 5)
        with _scope("a7"):
            ln_sides(L7)
            add_side(lambda tok: wq_perm(), 128, *WQ_PERM)
            add_side(lambda tok: wq_form(), 224, *WQ_FORM)
            add_side(lambda tok: route(), 17, *ROUTE)
            for r0, n in A7K:
                kproj(r0, n)
            finish()

        def b_body(j, carry):
            qa = BQ - QB
            with _scope("b_r0"):
                z_prep()
                add_side(lambda tok: ps_form(j), 7 * HQ // 16, 0, 49 * qa - 400)
                for r0 in range(0, qa, QN):
                    run_all(q_rows(j, r0, QN, pq_buf, den_buf, r0, r0 + QN < qa))
                finish()
            with _scope("b_wait"):
                for c in cp_b(j, wait_only=True):
                    c.wait()
            with _scope("b_r1"):
                add_side(lambda tok: ffn_part(j), FH * 3 // 8, 0, R1T)
                qs_j = qs.at[:, pl.ds(_mo(j * (qa // 2), 16), qa // 2), :]
                add_side(lambda tok: normalise(pq_buf, den_buf, qa, qs_j, lambda r: r >= qa - QN),
                         22 * (qa // 16), 0, R1T)
                run_all(g_kvm(j))
                finish()
            return carry

        lax.fori_loop(0, 2, b_body, 0)

        def c_body(t, carry):
            with _scope("c_body"):
                y = _rbf(jnp.sum(yacc[...], axis=0, keepdims=True))
                y = _rbf(y * _rbf(1.0 / _rbf(1.0 + _rbf(jnp.exp(-rsel[0:1, :])))))
                j, h = t >> 1, t & 1
                na, nb = (BQ - QB) // 2, QB // 2
                hb = pl.ds(_mo(h * nb, 16), nb)
                add_side(lambda tok: normalise(pqb_buf.at[j, :, hb, :], denb_buf.at[j, :, hb, :], nb, qsb,
                                               lambda r: True, tok),
                         4 + 22 * (nb // 16), 0, 49 * na - 800, SLAG)
                qs_t = qs.at[:, pl.ds(_mo(t * (na // 2), 16), na // 2), :]
                for p in range(0, na, CR):
                    run_all(out_part(j * BQ + h * na, na, p, CR, y, qs_t))
                flush()
                run_all(out_part(j * BQ + BQ - QB + h * nb, nb, 0, nb, y, qsb))
                finish()
            return carry

        lax.fori_loop(0, 4, c_body, 0)
        return carry0

    lax.fori_loop(0, z0 + 1, main, 0)
    with _scope("tail"):
        cp(out_buf, out_hbm.at[0], SEM_O).wait()


@jax.jit
def pallas_parallel_sum__linear_attn_block__moe_arch_mod__prompt_kernel(
    A_x: jax.Array,
    A_wqkv: jax.Array,
    A_wo: jax.Array,
    B_x: jax.Array,
    B_w_r: jax.Array,
    B_w_gate: jax.Array,
    B_w_up: jax.Array,
    B_w_down: jax.Array,
):
    del B_x
    V = pltpu.VMEM
    scratch = [
        V((4, HQ, D), bf16),
        V((4, D, 256), bf16),
        V((2, D, 512), bf16),
        V((2, 512, D), bf16),
        V((8 * D,), bf16),
        V((2, D, FH), bf16),
        V((2, D, FH), bf16),
        V((2, FH, D), bf16),
        V((28, HQ // 2, 256), u32),
        V((28, HQ // 2, 256), u32),
        V((49, 128, 256), u32),
        V((S, 128), f32),
        V((S, 128), f32),
        V((8, D), f32),
        V((8, D), f32),
        V((2, 4, HQ, 512), f32),
        V((D, 128), f32),
        V((8, D), f32),
        V((8, D), f32),
        V((16, D), f32),
        V((4, 8, 128), u32),
        V((4, HD // 2, 7 * 128), u32),
        V((S, 256), f32),
        V((64, 64, 128), u32),
        V((1, HQ // 2, 49 * 128), u32),
        V((49, BQ - QB, 256), u32),
        V((49, 128, 256), u32),
        V((8, 64, 128), u32),
        V((4, 64, 128), u32),
        V((1, 4, BQ - QB, D), f32),
        V((1, 4, BQ - QB, 128), f32),
        V((2, 4, QB, D), f32),
        V((2, 4, QB, 128), f32),
        V((49, QB // 4, 256), u32),
        V((1, 4, 128, D), f32),
        V((1, FH, 128), f32),
        V((S, D), bf16),
        pltpu.SMEM((1,), i32),
        pltpu.SemaphoreType.DMA((4 + T0 // X0 + 6,)),
    ]
    extra = {k: True for k in ("disable_bounds_checks", "disable_semaphore_checks")
             if hasattr(pltpu.CompilerParams, k)}
    return pl.pallas_call(
        _kernel,
        out_shape=jax.ShapeDtypeStruct((1, S, D), bf16),
        in_specs=[pl.BlockSpec(memory_space=pl.ANY)] * 7,
        out_specs=pl.BlockSpec(memory_space=pl.ANY),
        scratch_shapes=scratch,
        compiler_params=pltpu.CompilerParams(vmem_limit_bytes=120 * 1024 * 1024, **extra),
    )(A_x.reshape(4, HQ, D), A_wqkv, A_wo, B_w_r, B_w_gate, B_w_up, B_w_down)
```

```python
import contextlib

import jax
import jax.numpy as jnp
from jax import lax
import jax.experimental.pallas as pl
import jax.experimental.pallas.tpu as pltpu

bf16, f32, u32, i32 = jnp.bfloat16, jnp.float32, jnp.uint32, jnp.int32

S = 2048
D = 1024
F = 3584
HD = D // 2
HQ = S // 4
BQ = HQ // 2
FH = F // 2
QB = 64
QN = 48
QPRE = 3
QSPLIT = 6
CR = 48
T0 = 96
X0 = 32
XG = (144, 176, 368)
XN = 128

SLAG = 400
LNLAG = 700
QW = (28, 36, 36, 6, 2, 2, 2)
L4 = ([(96, 144, 0, 1100)], [])
L5 = ([(144, 176, 500, 1600)], [(96, 128, 300, 1250), (128, 144, 1300, 1900), (144, 176, 2000, 2950)])
L6 = ([(176, 368, 0, 7400)], [(176, 224, 800, 2600), (224, 336, 2700, 7800)])
L7 = ([(368, 512, 0, 4800)], [(336, 384, 0, 2400), (384, 512, 2500, 9000)])
A5K = ((96, 32),)
A6K = ((128, 48), (176, 48), (224, 48))
A7K = ((272, 64), (336, 48), (384, 64), (448, 64))
WQ_PERM, WQ_FORM, ROUTE = (5100, 7900), (8000, 13100), (9400, 10200)
R1T = 12800
MF = (128, 3420)

L_ORD = (2, 3, 0, 1, 4, 5, 6)
R_ORD = (2, 0, 6, 5, 1, 4, 3)

K_SEQ = (1, 4, 0, 2, 3, 5, 6)
K_SEQ2 = (0, 1, 2, 5, 3, 4, 6)
W_SEQ = (0, 1, 5, 6, 4, 2, 3)

NN = (((1,), (0,)), ((), ()))
TN = (((0,), (0,)), ((), ()))


SCOPES = False


def _scope(name):
    return jax.named_scope(name) if SCOPES else contextlib.nullcontext()


def _mo(v, m):
    return v if isinstance(v, int) else pl.multiple_of(v, m)


def _dot(a, b, dims):
    return lax.dot_general(a, b, dims, preferred_element_type=f32)


def _pack(v):
    return pltpu.bitcast(v.astype(bf16), u32)


def _unpack(v):
    return pltpu.bitcast(v, bf16)


def _combine(m):
    m1, m2, m3, m4, m5, m6, m7 = m
    return m1 + m4 - m5 + m7, m3 + m5, m2 + m4, m1 - m2 + m3 + m6


def _lform(a11, a12, a21, a22):
    return (a11 + a22, a21 + a22, a11, a22, a11 + a12, a21 - a11, a12 - a22)


def _rform(b11, b12, b21, b22):
    return (b11 + b22, b11, b12 - b22, b21 - b11, b22, b11 + b12, b21 + b22)


def _sform(x11, x12, x21, x22):
    return (x11, x22, x11 + x22, x21 + x22, x11 + x12, x21 - x11, x12 - x22)


def _wl(a11, a12, a21, a22):
    s1 = a21 + a22
    s2 = s1 - a11
    return (a11, a12, a12 - s2, a22, s1, s2, a11 - a21)


def _wr(b11, b12, b21, b22):
    t1 = b12 - b11
    t2 = b22 - t1
    return (b11, b21, b22, t2 - b21, t1, t2, b22 - b12)


def _wc(p):
    p1, p2, p3, p4, p5, p6, p7 = p
    u2 = p1 + p6
    u3 = u2 + p7
    return p1 + p2, (u2 + p5) + p3, u3 - p4, u3 + p5


W_R = (3, 1, 0, 2, 4, 5, 6)


def _wl_swapped(a11, a12, a21, a22):
    return _wl(a12, a11, a22, a21)


def _wc_swapped(p):
    p1, p2, p3, p4, p5, p6, p7 = p
    v2 = p1 + p6
    u3 = p7 - v2
    return (p5 - v2) + p3, p1 + p2, u3 + p5, p4 - u3


class _Sym:
    def __init__(self, t):
        self.t = t

    def __add__(self, o):
        return _Sym({**self.t, **o.t})

    def __sub__(self, o):
        return _Sym({**self.t, **{k: -v for k, v in o.t.items()}})


def _st(u, ct):
    return slice((4 * ct + u) * 128, (4 * ct + u + 1) * 128)


def _to_st(v):
    return jnp.concatenate([v[:, (2 * u + ct) * 128:(2 * u + ct + 1) * 128]
                            for ct in range(2) for u in range(4)], axis=1)


def _phi(t):
    return jnp.where(t > 0, t + 1.0, jnp.exp(t)) + 1e-6


def _rbf(v):
    return v.astype(bf16).astype(f32)


def _kernel(x_hbm, wqkv_hbm, wo_hbm, wr_hbm, wg_hbm, wu_hbm, wd_hbm, out_hbm,
            x_buf, wk_buf, wv_buf, wo_buf, wr_buf, wg_buf, wu_buf, wd_buf,
            xs1, xs2, wqs, sa, sb, zacc, zp, pk_buf, xb, yacc, rsel, wrb, zero_buf,
            wks, stats, wqt, ps_raw, qs, ms, tscr, tscr2, pq_raw, den_raw, pqb_buf, denb_buf, qsb,
            mg_raw, hb_raw, out_buf, idx_s, sem):
    wq_buf = out_buf.at[pl.ds(0, D), :]

    def xs_at(k1, e, rows=None):
        r = xs1.at[k1 * 4 + (0, 1, 7, 3).index(e)] if e in (0, 1, 7, 3) else xs2.at[k1 * 4 + (2, 4, 5, 6).index(e)]
        return r if rows is None else r.at[rows, :]

    SEM_B, SEM_O, SEM_Z, SEM_A = 0, 2, 3, 4

    def cp(src, dst, s):
        return pltpu.make_async_copy(src, dst, sem.at[s])

    def cp_x(r0, n, s):
        r = pl.ds(_mo(r0, 16), n)
        return [cp(x_hbm.at[:, r, :], x_buf.at[:, r, :], s)]

    def cp_wk(c, s):
        return [cp(wqkv_hbm.at[:, pl.ds(_mo(D + c * 256, 256), 256)],
                   wk_buf.at[c], s)]

    NX = T0 // X0
    SEM_W = SEM_A + NX
    cp_wr = cp(wr_hbm, wr_buf.at[pl.ds(0, D)], SEM_Z)
    a_groups = [cp_x(i * X0, X0, SEM_A + i) for i in range(NX)] + [
        cp_wk(0, SEM_W),
        cp_wk(1, SEM_W + 1),
        cp_wk(2, SEM_W + 2) + cp_x(T0, XG[0] - T0, SEM_W + 2),
        cp_wk(3, SEM_W + 3) + cp_x(XG[0], XG[1] - XG[0], SEM_W + 3),
        cp_x(XG[1], XG[2] - XG[1], SEM_W + 4),
        (cp_x(XG[2], HQ - XG[2], SEM_W + 5) if XG[2] < HQ else [])
        + [cp(wqkv_hbm.at[:, pl.ds(0, D)], wq_buf, SEM_W + 5)],
    ]

    def cp_b(j, wait_only=False):
        dsts = [r.at[j] for r in (wg_buf, wu_buf, wd_buf, wv_buf, wo_buf)]
        if wait_only:
            return [cp(dst, dst, SEM_B + j) for dst in dsts]
        fs = pl.ds(j * FH, FH)
        srcs = [wg_hbm.at[:, fs], wu_hbm.at[:, fs], wd_hbm.at[fs, :],
                wqkv_hbm.at[:, pl.ds(2 * D + j * HD, HD)], wo_hbm.at[pl.ds(j * HD, HD), :]]
        return [cp(src, dst, SEM_B + j) for src, dst in zip(srcs, dsts)]

    clock = [0]
    toks = []
    sides = []
    fwd = [None]

    def emit_tok(vals, stamp):
        t = None
        for v in vals:
            v = pltpu.bitcast(v, u32) if v.dtype != u32 else v
            t = v if t is None else t | v
        toks.append((stamp, t & zero_buf[0]))

    def token(kind):
        t = fwd[0]
        if "u" not in t:
            t["u"] = pltpu.bitcast(t["src"](), u32) & zero_buf[0]
        if kind != "u" and "f" not in t:
            t["f"] = pltpu.bitcast(t["u"], f32)
        if kind == "f16" and "f16" not in t:
            t["f16"] = jnp.concatenate([t["f"], t["f"]], axis=0)
        return t[kind]

    def gate(v):
        if fwd[0] is None:
            return v
        head = v if v.shape[0] == 8 else v[0:8]
        head = head | token("u") if v.dtype == u32 else head + token("f")
        return head if v.shape[0] == 8 else jnp.concatenate([head, v[8:]], axis=0)

    def gate16(v):
        return v if fwd[0] is None else v + token("f16")

    def add_side(gen_fn, n, t0, t1, lag=None):
        st = {"i": 0, "n": n, "t0": clock[0] + t0, "t1": clock[0] + t1}

        def tok(vals):
            if lag is not None:
                emit_tok(vals, st["t0"] + (st["i"] + 1) * (st["t1"] - st["t0"]) // st["n"] + lag)
        st["g"] = gen_fn(tok)
        sides.append(st)

    def advance(until):
        for st in sides:
            while st["i"] < st["n"] and st["t0"] + st["i"] * (st["t1"] - st["t0"]) // st["n"] < until:
                next(st["g"], None)
                st["i"] += 1
                if st["i"] == st["n"]:
                    for _ in st["g"]:
                        pass

    def flush():
        for st in sides:
            for _ in st["g"]:
                pass
        sides.clear()

    def finish():
        flush()
        toks.clear()
        fwd[0] = None

    def mm(lhs, rhs, dims, cycles, nseg=1):
        due = [t for (c, t) in toks if c <= clock[0]]
        toks[:] = [(c, t) for (c, t) in toks if c > clock[0]]
        if due:
            head = rhs[0:8, 0:128]
            for t in due:
                head = head | t
            if rhs.shape[1] > 128:
                head = jnp.concatenate([head, rhs[0:8, 128:]], axis=1)
            rhs = jnp.concatenate([head, rhs[8:]], axis=0)
        res = _dot(lhs, _unpack(rhs), dims)
        ngr = res.shape[0] // 16
        for sg in range(nseg):
            for i in range(ngr):
                fwd[0] = {"src": lambda sg=sg, i=i: res[i * 16:i * 16 + 8, sg * 128:(sg + 1) * 128]}
                clock[0] += cycles // nseg // ngr
                advance(clock[0])
        return res

    def form_steps(form, form2, get, put, tok=None, keep=range(7)):
        terms = form(*[_Sym({i: 1}) for i in range(4)])
        gated = (0, 1, 2, 3) if 7 in keep else {_wl: (0, 1, 3), _wr: (0, 2, 3), _wl_swapped: (1, 2)}[form2]
        for k1 in range(7):
            sub = []
            for r in range(2):
                for c in range(2):
                    v = None
                    for i, sg in sorted(terms[k1].t.items(), key=lambda e: -e[1]):
                        b = get(r + 2 * (i // 2), c + 2 * (i % 2))
                        if v is None:
                            v = gate16(b) if 2 * r + c in gated else b
                        else:
                            v = v + b if sg > 0 else v - b
                    sub.append(v)
            vals = form2(*sub) + (sub[2],)
            for k2 in keep:
                put(k1, k2, _pack(vals[k2]))
            if tok is not None and k1 % 2 == 0:
                full = vals[3 if form2 is _wr else 2]
                tok([full[0:8], full[8:16]])
            yield

    def strassen2(lhs, rhs, dims, cycles, nseg=1, wts=(16,) * 7, comb=_wc):
        m1 = [None] * 7
        for i1, k1 in enumerate(K_SEQ2):
            m2 = [None] * 7
            for k2 in W_SEQ:
                m2[k2] = mm(lhs(k1, k2), rhs(k1, k2), dims, cycles * wts[i1] // 16, nseg)
                yield
            m1[k1] = comb(m2)
        out = [[None] * 4 for _ in range(4)]
        for s2 in range(4):
            for s1, v in enumerate(_combine([m1[k1][s2] for k1 in range(7)])):
                out[(s1 // 2) * 2 + s2 // 2][(s1 % 2) * 2 + s2 % 2] = v
        return out

    made = set()

    def need(*keys):
        assert all(k in made for k in keys), keys

    def row_views(base):
        if base == 0:
            return x_buf, sa, sb, stats, xn_buf, None
        i, n = base
        b = _mo(i * n, 16)
        return ([x_buf.at[:, pl.ds(b, n), :]] + [r.at[pl.ds(b, S - 128 + n), :] for r in (sa, sb, stats)]
                + [xn_buf.at[:, pl.ds(b, n), :], pl.ds(_mo(i * (n // 2), 8), n // 2)])

    def xs_form(r0, tok, which="all", base=0):
        xn_v, xs_v = row_views(base)[4:]
        rows = slice(r0 % XN, r0 % XN + 16)

        keep = {"all": range(8), "l1": (0, 1, 7, 3), "l2": (2, 4, 5, 6)}[which]
        for ct in range(2):
            def put(k1, k2, v):
                xs_at(k1, k2, xs_v)[r0 // 2:r0 // 2 + 8, ct * 128:(ct + 1) * 128] = v
            yield from form_steps(
                _sform, _wl, lambda q, u: xn_v[q, rows, _st(u, ct)], put, tok, keep)
        made.add(("xs", r0))

    def ln_stats(r_start, n_rows, tok, base=0):
        x_v, sa_v, sb_v, st_v, xn_v, _ = row_views(base)
        lane = lax.broadcasted_iota(i32, (8, 128), 1)
        for r0 in range(r_start, r_start + n_rows, 16):
            if r0 >= T0:
                need(("in", 2 + sum(r0 >= g for g in XG)))
            if r0 - XN >= T0:
                need(("ln", r0 - XN))
            for g in range(8):
                q, o = g // 2, (g % 2) * 8
                rg = q * HQ + r0 + o
                xv = x_v[q, r0 + o:r0 + o + 8, :].astype(f32)
                xg = jnp.concatenate([gate(xv[:, 0:128]), xv[:, 128:]], axis=1)
                mf = jnp.sum(xg, axis=1, keepdims=True) * (1.0 / D)
                d = xv - mf
                var = jnp.sum(d * d, axis=1, keepdims=True) * (1.0 / D)
                rs = lax.rsqrt(var + 1e-5)
                xn_v.at[q][r0 % XN + o:r0 % XN + o + 8, :] = _to_st(d * rs)
                rs = jnp.broadcast_to(rs, (8, 128))
                mf = jnp.broadcast_to(mf, (8, 128))
                sa_v[rg:rg + 8, :] = 1.0 + rs
                sb_v[rg:rg + 8, :] = mf * rs
                st_v[rg:rg + 8, 0:128] = jnp.where(lane == 0, mf, jnp.broadcast_to(var, (8, 128)))
                if tok is not None:
                    tok([rs])
                if g == 7:
                    made.add(("xn", r0))
                yield

    def ln_later(r_start, n_rows, tok, which="all", base=0):
        st_v, xn_v = row_views(base)[3:5]
        for r0 in range(r_start, r_start + n_rows, 16):
            need(("xn", r0))
            form = xs_form(r0, tok, which, base)
            for g in range(8):
                for _ in range(2 if g < 7 else 0):
                    next(form)
                    yield
                q, o = g // 2, (g % 2) * 8
                t = None
                if which != "l1":
                    v = xn_v[q, r0 % XN + o:r0 % XN + o + 8, :] * wrb[8:16, :]
                    for ct in range(8):
                        h = v[:, ct * 128:(ct + 1) * 128]
                        t = gate(h) if t is None else t + h
                if t is not None:
                    st_v[q * HQ + r0 + o:q * HQ + r0 + o + 8, 128:256] = t
                if tok is not None:
                    tok([t])
                if g == 7:
                    next(form, None)
                    made.add(("ln", r0))
                yield

    def wk_prep(c):
        if isinstance(c, int):
            need(("in", c))
        wks.at[c][:, 128:256] = pltpu.bitcast(wk_buf[c, 0:HD, 0:128], u32)
        wks.at[c][:, 512:640] = pltpu.bitcast(wk_buf[c, HD:D, 128:256], u32)
        for i in range(HD // 16):
            r0 = i * 16
            top = wk_buf[c, r0:r0 + 16, :].astype(f32)
            bot = wk_buf[c, HD + r0:HD + r0 + 16, :].astype(f32)
            ops = _rform(top[:, :128], top[:, 128:], bot[:, :128], bot[:, 128:])
            for k in (0, 2, 3, 5, 6):
                wks.at[c][r0 // 2:r0 // 2 + 8, k * 128:(k + 1) * 128] = _pack(ops[k])

    def wq_perm():
        need(("in", 5))

        def permute(kt):
            for g in range(8):
                tile = gate(pltpu.bitcast(wq_buf[kt * 128:(kt + 1) * 128, g * 128:(g + 1) * 128], u32))
                wqt.at[kt * 8 + g][...] = pltpu.bitcast(_unpack(tile).T, u32)
                yield

        def back(kt):
            for j in range(8):
                tile = gate(jnp.concatenate([wqt[kt * 8 + g, pl.ds(j, 8, stride=8), :] for g in range(8)],
                                            axis=0))
                v = pltpu.bitcast(_unpack(tile).T.astype(f32), u32)
                c0 = (kt // 2) * D + _st(j // 2, j % 2).start
                ps[(kt % 2) * 128:(kt % 2 + 1) * 128, c0:c0 + 128] = v
                made.add(("wqp", kt, j))
                yield

        order = (0, 2, 4, 6, 1, 3, 5, 7)
        for n in range(10):
            if n < 8:
                yield from permute(order[n])
            if n > 1:
                yield from back(order[n - 2])

    def wq_form():
        for i in range(16):
            need(*[("wqp", 2 * r + i // 8, j) for r in range(4) for j in range(8)])
            for ct in range(2):
                def put(k1, k2, v):
                    wqs.at[k1 * 7 + k2][i * 8:(i + 1) * 8, ct * 128:(ct + 1) * 128] = v
                yield from form_steps(
                    _rform, _wr, lambda r, c: pltpu.bitcast(
                        ps[i * 16:(i + 1) * 16, r * D + _st(c, ct).start:r * D + _st(c, ct).stop],
                        f32), put)

    def kproj(r0, n, chunks=range(4)):
        pr = pl.ds(r0 // 2, n // 2)
        need(*[("xs", r) for r in range(max(r0, T0), r0 + n, 16)])
        for c in chunks:
            m = [None] * 7
            for k in K_SEQ:
                e11, e12, e21, e22 = [xs_at(L_ORD[k], e)[pr, :] for e in (0, 1, 7, 3)]
                lhs = jnp.concatenate([jnp.concatenate([e11, e12], axis=1),
                                       jnp.concatenate([e21, e22], axis=1)], axis=0)
                m[k] = mm(_unpack(lhs), wks[c, :, k * 128:(k + 1) * 128], NN, 2 * n)
            kk = [_phi(v) for v in _combine(m)]
            for ct in range(2):
                zacc[:, pl.ds(_mo(c * 256 + ct * 128, 128), 128)] += (
                    (kk[ct] + kk[2 + ct]).reshape(n // 4, 8, 128).sum(axis=0))
            j, c2 = (c // 2, c % 2) if isinstance(c, int) else (0, c)
            pk_v = pk_buf.at[j, :, :, pl.ds(_mo(c2 * 256, 256), 256)]
            for s1 in range(4):
                for h in range(2):
                    pk_v.at[(s1 // 2) * 2 + h][r0:r0 + n, (s1 % 2) * 128:(s1 % 2 + 1) * 128] = (
                        kk[s1][h * n:(h + 1) * n])

    def z_prep():
        z = jnp.sum(zacc[...], axis=0, keepdims=True)
        zt = _pack(jnp.broadcast_to(z, (128, D)).astype(bf16).T)
        for g in range(8):
            tscr.at[g][...] = zt[g * 64:(g + 1) * 64, :]
        for j in range(8):
            blk = jnp.concatenate([tscr[g, pl.ds(j, 8, stride=8), :] for g in range(8)], axis=0)
            zp[:, j * 128:(j + 1) * 128] = _unpack(blk).T[0:8, :].astype(f32)

    def route():
        rows, dots = [None] * 16, [None] * 16
        for b in sorted(range(S // 128), key=lambda b: b % 4):
            need(*[("ln", r) for r in range(max(T0, b % 4 * 128), b % 4 * 128 + 128, 16)])
            rows[b] = gate(stats[b * 128:(b + 1) * 128, 0:128]).T[0:8, :]
            dots[b] = jnp.sum(gate(stats[b * 128:(b + 1) * 128, 128:256]).T, axis=0, keepdims=True)
            yield
        mf = jnp.concatenate([v[0:1] for v in rows], axis=0)
        var = jnp.concatenate([v[1:2] for v in rows], axis=0)
        tr = jnp.concatenate(dots, axis=0) * jnp.sqrt(var + 1e-5)
        wsum = jnp.sum(wrb[0:1, :], axis=1, keepdims=True)
        mb = _rbf(mf)
        inv = 1.0 / _rbf(jnp.sqrt(_rbf(_rbf(var) + 1e-5)))
        rv = _rbf((tr + (mf - mb) * wsum) * inv)
        rmax = jnp.max(jnp.max(rv, axis=1, keepdims=True), axis=0, keepdims=True)
        pos = (lax.broadcasted_iota(i32, rv.shape, 0) * 128 + lax.broadcasted_iota(i32, rv.shape, 1))
        idx = jnp.min(jnp.where(rv == rmax, pos, S - 1))
        idx_s[0] = idx

        def pick(v):
            v = jnp.sum(jnp.where(pos == idx, v, 0.0), axis=1, keepdims=True)
            return jnp.sum(v, axis=0, keepdims=True)

        xv = x_buf[(idx >> 9) & 3, pl.ds(_mo(idx & (HQ - 16), 16), 16), :].astype(f32)
        sel = lax.broadcasted_iota(i32, xv.shape, 0) == (idx & 15)
        row = jnp.sum(jnp.where(sel, xv, 0.0), axis=0, keepdims=True)
        row = _rbf(_rbf(row - pick(mb)) * pick(inv))
        rsel[...] = jnp.broadcast_to(_rbf(jnp.sum(row * wrb[0:1, :], axis=1, keepdims=True)), rsel.shape)
        xb[...] = jnp.broadcast_to(row, (128, D)).T
        yield

    def ps_form(j):
        for c in range(HQ // 16):
            def put(k1, k2, v):
                k = k1 * 7 + k2
                ps[c * 8:(c + 1) * 8, k * 128:(k + 1) * 128] = v
            yield from form_steps(
                _lform, _wl_swapped,
                lambda r, q: pk_buf[j, q, c * 16:(c + 1) * 16, r * 128:(r + 1) * 128], put)

    def q_rows(j, r0, n, pq, rc, d0, rec):
        xj = pl.ds(_mo(j * (BQ // 2), BQ // 2), BQ // 2)
        pr = slice(r0 // 2, (r0 + n) // 2)
        blk = yield from strassen2(lambda k1, k2: _unpack(xs_at(L_ORD[k1], k2, xj)[pr, :]),
                                   lambda k1, k2: wqs[k1 * 7 + k2], NN, n, 1, QW)
        lane = lax.broadcasted_iota(i32, (n, 128), 1)
        for q in range(4):
            d = None
            for u in (3, 2, 1, 0):
                v = _phi(blk[q][u])
                for ct in range(2):
                    pq.at[q][d0:d0 + n, _st(u, ct)] = v[:, ct * 128:(ct + 1) * 128]
                t = v * zp[0:1, u * 256:(u + 1) * 256]
                t = t[:, :128] + t[:, 128:]
                d = t if d is None else d + t
            if rec:
                d = recip(d, lane)
            rc.at[q][d0:d0 + n, :] = d

    def recip(d, lane):
        d = d + jnp.where(lane % 2 == 0, pltpu.roll(d, 127, 1), pltpu.roll(d, 1, 1))
        d = d + jnp.where(lane % 4 < 2, pltpu.roll(d, 126, 1), pltpu.roll(d, 2, 1))
        return 1.0 / (d + 1e-6)

    def normalise(pq, rc, nr, dst, raw, tok=None):
        lane = lax.broadcasted_iota(i32, (16, 128), 1)

        def fix(c):
            if c < nr // 16 and raw(c * 16):
                for q in range(4):
                    rq = slice(c * 16, (c + 1) * 16)
                    rc.at[q][rq, :] = recip(gate16(rc[q, rq, :]), lane)

        def scale(c):
            rq = slice(c * 16, (c + 1) * 16)
            fix(c + 1)
            for hf in range(2):
                for q in range(4):
                    cs = slice(hf * HD, (hf + 1) * HD)
                    pq.at[q][rq, cs] = pq[q, rq, cs] * jnp.concatenate([gate16(rc[q, rq, :])] * 4, axis=1)
                    yield

        def form(c):
            rq = slice(c * 16, (c + 1) * 16)
            for ct in range(2):
                def put(k1, k2, v):
                    dst.at[k1 * 7 + k2][c * 8:(c + 1) * 8, ct * 128:(ct + 1) * 128] = v
                yield from form_steps(_lform, _wl, lambda q, u: pq[q, rq, _st(u, ct)], put, tok)

        fix(0)
        if raw(0):
            for _ in range(4):
                yield
        yield from scale(0)
        for c in range(nr // 16):
            nxt = scale(c + 1) if c + 1 < nr // 16 else iter(())
            for i, _ in enumerate(form(c)):
                yield
                if i < 8 and c + 1 < nr // 16:
                    next(nxt)
                    yield

    def g_kvm(j):
        qb = q_rows(j, BQ - QB, QB, pqb_buf.at[j], denb_buf.at[j], 0, False)
        for _ in range(QPRE):
            next(qb)
        blk = yield from strassen2(
            lambda k1, k2: _unpack(ps[:, (k1 * 7 + k2) * 128:(k1 * 7 + k2 + 1) * 128]),
            lambda k1, k2: xs_at(R_ORD[k1], W_R[k2])[...], TN, 256, 2, comb=_wc_swapped)
        hm = (lax.broadcasted_iota(i32, (128, 128), 0) // 32
              == lax.broadcasted_iota(i32, (128, 128), 1) // 32)
        for _ in range(QSPLIT - QPRE):
            next(qb)
        kvps = []
        for a in (3, 2, 1, 0):
            gg = jnp.concatenate(blk[a], axis=1).astype(bf16)
            wv_u = pltpu.bitcast(wv_buf[j, :, a * 128:(a + 1) * 128], u32)
            kv = jnp.where(hm, mm(gg, wv_u, NN, 256), 0.0)
            tscr2.at[a][...] = _pack(kv)
            kvps.append(_unpack(jnp.concatenate(
                [tscr2[a, pl.ds(jj, 8, stride=8), :] for jj in range(8)], axis=0)))

        ms_j = ms.at[:, pl.ds(_mo(j * 32, 32), 96), :]

        def m_form():
            for a in (3, 2, 1, 0):
                need(("mg", a))
                for jl in range(2):
                    for ct in range(2):
                        def put(k1, k2, v):
                            ms_j.at[k1 * 7 + k2][jl * 64 + a * 8:jl * 64 + (a + 1) * 8,
                                                 ct * 128:(ct + 1) * 128] = v
                        yield from form_steps(
                            _rform, _wr, lambda q, u: mg_buf[a, (2 * q + jl) * 16:(2 * q + jl + 1) * 16, _st(u, ct)], put)

        for i, a in enumerate((3, 2, 1, 0)):
            wo_u = pltpu.bitcast(wo_buf[j, a * 128:(a + 1) * 128, :], u32)
            res = mm(kvps[i], wo_u, NN, 256)
            mg_buf.at[a][...] = _to_st(res)
            made.add(("mg", a))
            if i == 0:
                add_side(lambda tok: m_form(), 112, *MF)
        for _ in qb:
            pass

    def out_part(base, span, off, nr, y, src):
        b = _mo(base, 32)
        sa_v, sb_v, out_v = [r.at[pl.ds(b, 3 * HQ + span), :] for r in (sa, sb, out_buf)]
        x_v = x_buf.at[:, pl.ds(b, span), :]
        row = lax.broadcasted_iota(i32, (nr, 256), 0) + (base + off)
        blk = yield from strassen2(lambda k1, k2: _unpack(src[k1 * 7 + k2, off // 2:(off + nr) // 2, :]),
                                   lambda k1, k2: ms[k1 * 7 + k2], NN, nr)
        for s1 in (3, 2, 1, 0):
            for s2 in range(4):
                q = (s1 // 2) * 2 + s2 // 2
                u = (s1 % 2) * 2 + s2 % 2
                rr, cc = pl.ds(q * HQ + off, nr), pl.ds(u * 256, 256)
                a = jnp.concatenate([sa_v[rr, :]] * 2, axis=1)
                c = jnp.concatenate([sb_v[rr, :]] * 2, axis=1)
                o = blk[q][u] + jnp.where(row + q * HQ == idx_s[0], y[:, u * 256:(u + 1) * 256], 0.0)
                out_v[rr, cc] = (x_v[q, off:off + nr, cc].astype(f32) * a - c + o).astype(bf16)
                if s2 % 2 == 1:
                    ch = pl.ds((s1 % 2) * HD, HD)
                    ro = pl.ds(_mo(base + q * HQ + off, 16), nr)
                    cp(out_buf.at[ro, ch], out_hbm.at[0, ro, ch], SEM_O).start()

    def ffn_part(j):
        def fma(acc, w, v):
            p = w.astype(f32) * v
            return acc + p[0:8] + p[8:16]

        for f0 in range(0, FH, 256):
            fs = slice(f0, f0 + 256)
            ag = jnp.zeros((8, 256), f32)
            au = jnp.zeros((8, 256), f32)
            for k in range(0, D, 16):
                xv = jnp.concatenate([gate16(xb[k:k + 16, :])] * 2, axis=1)
                ag = fma(ag, wg_buf[j, k:k + 16, fs], xv)
                au = fma(au, wu_buf[j, k:k + 16, fs], xv)
                yield
            g = _rbf(jnp.sum(ag, axis=0, keepdims=True))
            u = _rbf(jnp.sum(au, axis=0, keepdims=True))
            h = _rbf(_rbf(g * jax.nn.sigmoid(g)) * u)
            hb_buf[fs, :] = jnp.broadcast_to(h, (128, 256)).T
        for d0 in range(0, D, 512):
            ds_ = slice(d0, d0 + 512)
            acc = yacc[:, ds_]
            for k in range(0, FH, 16):
                hv = jnp.concatenate([gate16(hb_buf[k:k + 16, :])] * 4, axis=1)
                acc = fma(acc, wd_buf[j, k:k + 16, ds_], hv)
                yield
            yacc[:, ds_] = acc

    def wait_group(i):
        with _scope("a_wait%d" % i):
            for c in a_groups[i]:
                c.wait()
        made.add(("in", i - NX))

    def run_all(gen):
        for _ in gen:
            pass

    def ln_sides(plan):
        for r0, r1, t0, t1 in plan[0]:
            add_side(lambda tok, r0=r0, r1=r1: ln_stats(r0, r1 - r0, tok), (r1 - r0) // 2, t0, t1, LNLAG)
        for r0, r1, t0, t1 in plan[1]:
            add_side(lambda tok, r0=r0, r1=r1: ln_later(r0, r1 - r0, tok), 22 * (r1 - r0) // 16, t0, t1, SLAG)

    def l2_side(base, n, t0, t1):
        add_side(lambda tok: ln_later(0, n, None, "l2", base), 22 * n // 16, t0, t1)

    with _scope("p0_issue"):
        cp_wr.start()
        for grp in a_groups:
            for c in grp:
                c.start()
        for j in range(2):
            for c in cp_b(j):
                c.start()
        zacc[...] = jnp.zeros(zacc.shape, f32)
        yacc[...] = jnp.zeros(yacc.shape, f32)
        zero_buf[1] = jnp.zeros((8, 128), u32)
        cp_zero = cp(zero_buf.at[1], zero_buf.at[0], SEM_Z)
        cp_zero.start()
        cp_zero.wait()
        cp_wr.wait()
        wr8 = jnp.broadcast_to(wr_buf[0:D].reshape(1, D).astype(f32), (8, D))
        wrb[0:8, :] = wr8
        wrb[8:16, :] = _to_st(wr8)
        z0 = jnp.max(pltpu.bitcast(zero_buf[0], i32))
        ps, pq_buf, den_buf, mg_buf, hb_buf = [r.at[z0] for r in (ps_raw, pq_raw, den_raw, mg_raw, hb_raw)]
        xn_buf = mg_buf

    def main(_, carry0):
        def a01(i, carry):
            with _scope("a_wait01"):
                for c in cp_x(i * X0, X0, SEM_A + i):
                    c.wait()
            with _scope("a01"):
                for r in range(0, X0, 16):
                    run_all(ln_stats(r, 16, None, (i, X0)))
                    if r:
                        run_all(ln_later(r - 16, 16, None, "l1", (i, X0)))
                run_all(ln_later(X0 - 16, 16, None, "l1", (i, X0)))
            return carry

        lax.fori_loop(0, NX, a01, 0)
        made.update(("xn", r) for r in range(0, 64, 16))

        def a23(i, carry):
            with _scope("a_wait23"):
                for c in cp_wk(i, SEM_W + i):
                    c.wait()
            with _scope("a23"):
                wk_prep(i)
                l2_side((i, T0 // 2), T0 // 2, 250, 14 * T0 - 250)
                kproj(0, T0, [i])
                finish()
            return carry

        lax.fori_loop(0, 2, a23, 0)
        wait_group(NX + 2)
        with _scope("a4"):
            wk_prep(2)
            ln_sides(L4)
            kproj(0, T0, [2])
            finish()
        wait_group(NX + 3)
        with _scope("a5"):
            wk_prep(3)
            ln_sides(L5)
            kproj(0, T0, [3])
            for r0, n in A5K:
                kproj(r0, n)
            finish()
        wait_group(NX + 4)
        with _scope("a6"):
            ln_sides(L6)
            for r0, n in A6K:
                kproj(r0, n)
            finish()
        wait_group(NX + 5)
        with _scope("a7"):
            ln_sides(L7)
            add_side(lambda tok: wq_perm(), 128, *WQ_PERM)
            add_side(lambda tok: wq_form(), 224, *WQ_FORM)
            add_side(lambda tok: route(), 17, *ROUTE)
            for r0, n in A7K:
                kproj(r0, n)
            finish()

        def b_body(j, carry):
            qa = BQ - QB
            with _scope("b_r0"):
                z_prep()
                add_side(lambda tok: ps_form(j), 7 * HQ // 16, 0, 49 * qa - 400)
                for r0 in range(0, qa, QN):
                    run_all(q_rows(j, r0, QN, pq_buf, den_buf, r0, r0 + QN < qa))
                finish()
            with _scope("b_wait"):
                for c in cp_b(j, wait_only=True):
                    c.wait()
            with _scope("b_r1"):
                add_side(lambda tok: ffn_part(j), FH * 3 // 8, 0, R1T)
                qs_j = qs.at[:, pl.ds(_mo(j * (qa // 2), 16), qa // 2), :]
                add_side(lambda tok: normalise(pq_buf, den_buf, qa, qs_j, lambda r: r >= qa - QN),
                         22 * (qa // 16), 0, R1T)
                run_all(g_kvm(j))
                finish()
            return carry

        lax.fori_loop(0, 2, b_body, 0)

        def c_body(t, carry):
            with _scope("c_body"):
                y = _rbf(jnp.sum(yacc[...], axis=0, keepdims=True))
                y = _rbf(y * _rbf(1.0 / _rbf(1.0 + _rbf(jnp.exp(-rsel[0:1, :])))))
                j, h = t >> 1, t & 1
                na, nb = (BQ - QB) // 2, QB // 2
                hb = pl.ds(_mo(h * nb, 16), nb)
                add_side(lambda tok: normalise(pqb_buf.at[j, :, hb, :], denb_buf.at[j, :, hb, :], nb, qsb,
                                               lambda r: True, tok),
                         4 + 22 * (nb // 16), 0, 49 * na - 800, SLAG)
                qs_t = qs.at[:, pl.ds(_mo(t * (na // 2), 16), na // 2), :]
                for p in range(0, na, CR):
                    run_all(out_part(j * BQ + h * na, na, p, CR, y, qs_t))
                flush()
                run_all(out_part(j * BQ + BQ - QB + h * nb, nb, 0, nb, y, qsb))
                finish()
            return carry

        lax.fori_loop(0, 4, c_body, 0)
        return carry0

    lax.fori_loop(0, z0 + 1, main, 0)
    with _scope("tail"):
        cp(out_buf, out_hbm.at[0], SEM_O).wait()


@jax.jit
def pallas_parallel_sum__linear_attn_block__moe_arch_mod__prompt_kernel(
    A_x: jax.Array,
    A_wqkv: jax.Array,
    A_wo: jax.Array,
    B_x: jax.Array,
    B_w_r: jax.Array,
    B_w_gate: jax.Array,
    B_w_up: jax.Array,
    B_w_down: jax.Array,
):
    del B_x
    V = pltpu.VMEM
    scratch = [
        V((4, HQ, D), bf16),
        V((4, D, 256), bf16),
        V((2, D, 512), bf16),
        V((2, 512, D), bf16),
        V((8 * D,), bf16),
        V((2, D, FH), bf16),
        V((2, D, FH), bf16),
        V((2, FH, D), bf16),
        V((28, HQ // 2, 256), u32),
        V((28, HQ // 2, 256), u32),
        V((49, 128, 256), u32),
        V((S, 128), f32),
        V((S, 128), f32),
        V((8, D), f32),
        V((8, D), f32),
        V((2, 4, HQ, 512), f32),
        V((D, 128), f32),
        V((8, D), f32),
        V((8, D), f32),
        V((16, D), f32),
        V((4, 8, 128), u32),
        V((4, HD // 2, 7 * 128), u32),
        V((S, 256), f32),
        V((64, 64, 128), u32),
        V((1, HQ // 2, 49 * 128), u32),
        V((49, BQ - QB, 256), u32),
        V((49, 128, 256), u32),
        V((8, 64, 128), u32),
        V((4, 64, 128), u32),
        V((1, 4, BQ - QB, D), f32),
        V((1, 4, BQ - QB, 128), f32),
        V((2, 4, QB, D), f32),
        V((2, 4, QB, 128), f32),
        V((49, QB // 4, 256), u32),
        V((1, 4, 128, D), f32),
        V((1, FH, 128), f32),
        V((S, D), bf16),
        pltpu.SMEM((1,), i32),
        pltpu.SemaphoreType.DMA((4 + T0 // X0 + 6,)),
    ]
    extra = {k: True for k in ("disable_bounds_checks", "disable_semaphore_checks")
             if hasattr(pltpu.CompilerParams, k)}
    return pl.pallas_call(
        _kernel,
        out_shape=jax.ShapeDtypeStruct((1, S, D), bf16),
        in_specs=[pl.BlockSpec(memory_space=pl.ANY)] * 7,
        out_specs=pl.BlockSpec(memory_space=pl.ANY),
        scratch_shapes=scratch,
        compiler_params=pltpu.CompilerParams(vmem_limit_bytes=120 * 1024 * 1024, **extra),
    )(A_x.reshape(4, HQ, D), A_wqkv, A_wo, B_w_r, B_w_gate, B_w_up, B_w_down)
```

```python
import contextlib

import jax
import jax.numpy as jnp
from jax import lax
import jax.experimental.pallas as pl
import jax.experimental.pallas.tpu as pltpu

bf16, f32, u32, i32 = jnp.bfloat16, jnp.float32, jnp.uint32, jnp.int32

S = 2048
D = 1024
F = 3584
HD = D // 2
HQ = S // 4
BQ = HQ // 2
FH = F // 2
QB = 64
QN = 48
QPRE = 3
QSPLIT = 6
CR = 48
T0 = 96
X0 = 32
XG = (144, 176, 368)
XN = 128

SLAG = 400
LNLAG = 700
QW = (28, 36, 36, 6, 2, 2, 2)
L4 = ([(96, 144, 0, 1070)], [])
L5 = ([(144, 176, 310, 1750)], [(96, 128, 220, 1170), (128, 144, 1340, 2060), (144, 176, 2010, 2910)])
L6 = ([(176, 368, 0, 7410)], [(176, 224, 740, 2510), (224, 336, 2800, 7870)])
L7 = ([(368, 512, 0, 4800)], [(336, 384, 0, 2400), (384, 512, 2500, 9000)])
A5K = ((96, 32),)
A6K = ((128, 48), (176, 48), (224, 48))
A7K = ((272, 64), (336, 48), (384, 64), (448, 64))
WQ_PERM, WQ_FORM, ROUTE = (5100, 7900), (8000, 13100), (9400, 10200)
L2W, PSW, FFW, NRW, CNW = (270, 1304), (0, 9008), (0, 12800), (0, 12800), (0, 3614)
MF = (128, 3420)

L_ORD = (2, 3, 0, 1, 4, 5, 6)
R_ORD = (2, 0, 6, 5, 1, 4, 3)

K_SEQ = (1, 4, 0, 2, 3, 5, 6)
K_SEQ2 = (0, 1, 2, 5, 3, 4, 6)
W_SEQ = (0, 1, 5, 6, 4, 2, 3)

NN = (((1,), (0,)), ((), ()))
TN = (((0,), (0,)), ((), ()))


SCOPES = False


def _scope(name):
    return jax.named_scope(name) if SCOPES else contextlib.nullcontext()


def _mo(v, m):
    return v if isinstance(v, int) else pl.multiple_of(v, m)


def _dot(a, b, dims):
    return lax.dot_general(a, b, dims, preferred_element_type=f32)


def _pack(v):
    return pltpu.bitcast(v.astype(bf16), u32)


def _unpack(v):
    return pltpu.bitcast(v, bf16)


def _combine(m):
    m1, m2, m3, m4, m5, m6, m7 = m
    return m1 + m4 - m5 + m7, m3 + m5, m2 + m4, m1 - m2 + m3 + m6


def _lform(a11, a12, a21, a22):
    return (a11 + a22, a21 + a22, a11, a22, a11 + a12, a21 - a11, a12 - a22)


def _rform(b11, b12, b21, b22):
    return (b11 + b22, b11, b12 - b22, b21 - b11, b22, b11 + b12, b21 + b22)


def _sform(x11, x12, x21, x22):
    return (x11, x22, x11 + x22, x21 + x22, x11 + x12, x21 - x11, x12 - x22)


def _wl(a11, a12, a21, a22):
    s1 = a21 + a22
    s2 = s1 - a11
    return (a11, a12, a12 - s2, a22, s1, s2, a11 - a21)


def _wr(b11, b12, b21, b22):
    t1 = b12 - b11
    t2 = b22 - t1
    return (b11, b21, b22, t2 - b21, t1, t2, b22 - b12)


def _wc(p):
    p1, p2, p3, p4, p5, p6, p7 = p
    u2 = p1 + p6
    u3 = u2 + p7
    return p1 + p2, (u2 + p5) + p3, u3 - p4, u3 + p5


W_R = (3, 1, 0, 2, 4, 5, 6)


def _wl_swapped(a11, a12, a21, a22):
    return _wl(a12, a11, a22, a21)


def _wc_swapped(p):
    p1, p2, p3, p4, p5, p6, p7 = p
    v2 = p1 + p6
    u3 = p7 - v2
    return (p5 - v2) + p3, p1 + p2, u3 + p5, p4 - u3


class _Sym:
    def __init__(self, t):
        self.t = t

    def __add__(self, o):
        return _Sym({**self.t, **o.t})

    def __sub__(self, o):
        return _Sym({**self.t, **{k: -v for k, v in o.t.items()}})


def _st(u, ct):
    return slice((4 * ct + u) * 128, (4 * ct + u + 1) * 128)


def _to_st(v):
    return jnp.concatenate([v[:, (2 * u + ct) * 128:(2 * u + ct + 1) * 128]
                            for ct in range(2) for u in range(4)], axis=1)


def _phi(t):
    return jnp.where(t > 0, t + 1.0, jnp.exp(t)) + 1e-6


def _rbf(v):
    return v.astype(bf16).astype(f32)


def _kernel(x_hbm, wqkv_hbm, wo_hbm, wr_hbm, wg_hbm, wu_hbm, wd_hbm, out_hbm,
            x_buf, wk_buf, wv_buf, wo_buf, wr_buf, wg_buf, wu_buf, wd_buf,
            xs1, xs2, wqs, sa, sb, zacc, zp, pk_buf, xb, yacc, rsel, wrb, zero_buf,
            wks, stats, wqt, ps_raw, qs, ms, tscr, tscr2, pq_raw, den_raw, pqb_buf, denb_buf, qsb,
            mg_raw, hb_raw, out_buf, idx_s, sem):
    wq_buf = out_buf.at[pl.ds(0, D), :]

    def xs_at(k1, e, rows=None):
        r = xs1.at[k1 * 4 + (0, 1, 7, 3).index(e)] if e in (0, 1, 7, 3) else xs2.at[k1 * 4 + (2, 4, 5, 6).index(e)]
        return r if rows is None else r.at[rows, :]

    SEM_B, SEM_O, SEM_Z, SEM_A = 0, 2, 3, 4

    def cp(src, dst, s):
        return pltpu.make_async_copy(src, dst, sem.at[s])

    def cp_x(r0, n, s):
        r = pl.ds(_mo(r0, 16), n)
        return [cp(x_hbm.at[:, r, :], x_buf.at[:, r, :], s)]

    def cp_wk(c, s):
        return [cp(wqkv_hbm.at[:, pl.ds(_mo(D + c * 256, 256), 256)],
                   wk_buf.at[c], s)]

    NX = T0 // X0
    SEM_W = SEM_A + NX
    cp_wr = cp(wr_hbm, wr_buf.at[pl.ds(0, D)], SEM_Z)
    a_groups = [cp_x(i * X0, X0, SEM_A + i) for i in range(NX)] + [
        cp_wk(0, SEM_W),
        cp_wk(1, SEM_W + 1),
        cp_wk(2, SEM_W + 2) + cp_x(T0, XG[0] - T0, SEM_W + 2),
        cp_wk(3, SEM_W + 3) + cp_x(XG[0], XG[1] - XG[0], SEM_W + 3),
        cp_x(XG[1], XG[2] - XG[1], SEM_W + 4),
        (cp_x(XG[2], HQ - XG[2], SEM_W + 5) if XG[2] < HQ else [])
        + [cp(wqkv_hbm.at[:, pl.ds(0, D)], wq_buf, SEM_W + 5)],
    ]

    def cp_b(j, wait_only=False):
        dsts = [r.at[j] for r in (wg_buf, wu_buf, wd_buf, wv_buf, wo_buf)]
        if wait_only:
            return [cp(dst, dst, SEM_B + j) for dst in dsts]
        fs = pl.ds(j * FH, FH)
        srcs = [wg_hbm.at[:, fs], wu_hbm.at[:, fs], wd_hbm.at[fs, :],
                wqkv_hbm.at[:, pl.ds(2 * D + j * HD, HD)], wo_hbm.at[pl.ds(j * HD, HD), :]]
        return [cp(src, dst, SEM_B + j) for src, dst in zip(srcs, dsts)]

    clock = [0]
    toks = []
    sides = []
    fwd = [None]

    def emit_tok(vals, stamp):
        t = None
        for v in vals:
            v = pltpu.bitcast(v, u32) if v.dtype != u32 else v
            t = v if t is None else t | v
        toks.append((stamp, t & zero_buf[0]))

    def token(kind):
        t = fwd[0]
        if "u" not in t:
            t["u"] = pltpu.bitcast(t["src"](), u32) & zero_buf[0]
        if kind != "u" and "f" not in t:
            t["f"] = pltpu.bitcast(t["u"], f32)
        if kind == "f16" and "f16" not in t:
            t["f16"] = jnp.concatenate([t["f"], t["f"]], axis=0)
        return t[kind]

    def gate(v):
        if fwd[0] is None:
            return v
        head = v if v.shape[0] == 8 else v[0:8]
        head = head | token("u") if v.dtype == u32 else head + token("f")
        return head if v.shape[0] == 8 else jnp.concatenate([head, v[8:]], axis=0)

    def gate16(v):
        return v if fwd[0] is None else v + token("f16")

    def add_side(gen_fn, n, t0, t1, lag=None):
        st = {"i": 0, "n": n, "t0": clock[0] + t0, "t1": clock[0] + t1}

        def tok(vals):
            if lag is not None:
                emit_tok(vals, st["t0"] + (st["i"] + 1) * (st["t1"] - st["t0"]) // st["n"] + lag)
        st["g"] = gen_fn(tok)
        sides.append(st)

    def advance(until):
        for st in sides:
            while st["i"] < st["n"] and st["t0"] + st["i"] * (st["t1"] - st["t0"]) // st["n"] < until:
                next(st["g"], None)
                st["i"] += 1
                if st["i"] == st["n"]:
                    for _ in st["g"]:
                        pass

    def flush():
        for st in sides:
            for _ in st["g"]:
                pass
        sides.clear()

    def finish():
        flush()
        toks.clear()
        fwd[0] = None

    def mm(lhs, rhs, dims, cycles, nseg=1):
        due = [t for (c, t) in toks if c <= clock[0]]
        toks[:] = [(c, t) for (c, t) in toks if c > clock[0]]
        if due:
            head = rhs[0:8, 0:128]
            for t in due:
                head = head | t
            if rhs.shape[1] > 128:
                head = jnp.concatenate([head, rhs[0:8, 128:]], axis=1)
            rhs = jnp.concatenate([head, rhs[8:]], axis=0)
        res = _dot(lhs, _unpack(rhs), dims)
        ngr = res.shape[0] // 16
        for sg in range(nseg):
            for i in range(ngr):
                fwd[0] = {"src": lambda sg=sg, i=i: res[i * 16:i * 16 + 8, sg * 128:(sg + 1) * 128]}
                clock[0] += cycles // nseg // ngr
                advance(clock[0])
        return res

    def form_steps(form, form2, get, put, tok=None, keep=range(7)):
        terms = form(*[_Sym({i: 1}) for i in range(4)])
        gated = (0, 1, 2, 3) if 7 in keep else {_wl: (0, 1, 3), _wr: (0, 2, 3), _wl_swapped: (1, 2)}[form2]
        for k1 in range(7):
            sub = []
            for r in range(2):
                for c in range(2):
                    v = None
                    for i, sg in sorted(terms[k1].t.items(), key=lambda e: -e[1]):
                        b = get(r + 2 * (i // 2), c + 2 * (i % 2))
                        if v is None:
                            v = gate16(b) if 2 * r + c in gated else b
                        else:
                            v = v + b if sg > 0 else v - b
                    sub.append(v)
            vals = form2(*sub) + (sub[2],)
            for k2 in keep:
                put(k1, k2, _pack(vals[k2]))
            if tok is not None and k1 % 2 == 0:
                full = vals[3 if form2 is _wr else 2]
                tok([full[0:8], full[8:16]])
            yield

    def strassen2(lhs, rhs, dims, cycles, nseg=1, wts=(16,) * 7, comb=_wc):
        m1 = [None] * 7
        for i1, k1 in enumerate(K_SEQ2):
            m2 = [None] * 7
            for k2 in W_SEQ:
                m2[k2] = mm(lhs(k1, k2), rhs(k1, k2), dims, cycles * wts[i1] // 16, nseg)
                yield
            m1[k1] = comb(m2)
        out = [[None] * 4 for _ in range(4)]
        for s2 in range(4):
            for s1, v in enumerate(_combine([m1[k1][s2] for k1 in range(7)])):
                out[(s1 // 2) * 2 + s2 // 2][(s1 % 2) * 2 + s2 % 2] = v
        return out

    made = set()

    def need(*keys):
        assert all(k in made for k in keys), keys

    def row_views(base):
        if base == 0:
            return x_buf, sa, sb, stats, xn_buf, None
        i, n = base
        b = _mo(i * n, 16)
        return ([x_buf.at[:, pl.ds(b, n), :]] + [r.at[pl.ds(b, S - 128 + n), :] for r in (sa, sb, stats)]
                + [xn_buf.at[:, pl.ds(b, n), :], pl.ds(_mo(i * (n // 2), 8), n // 2)])

    def xs_form(r0, tok, which="all", base=0):
        xn_v, xs_v = row_views(base)[4:]
        rows = slice(r0 % XN, r0 % XN + 16)

        keep = {"all": range(8), "l1": (0, 1, 7, 3), "l2": (2, 4, 5, 6)}[which]
        for ct in range(2):
            def put(k1, k2, v):
                xs_at(k1, k2, xs_v)[r0 // 2:r0 // 2 + 8, ct * 128:(ct + 1) * 128] = v
            yield from form_steps(
                _sform, _wl, lambda q, u: xn_v[q, rows, _st(u, ct)], put, tok, keep)
        made.add(("xs", r0))

    def ln_stats(r_start, n_rows, tok, base=0):
        x_v, sa_v, sb_v, st_v, xn_v, _ = row_views(base)
        lane = lax.broadcasted_iota(i32, (8, 128), 1)
        for r0 in range(r_start, r_start + n_rows, 16):
            if r0 >= T0:
                need(("in", 2 + sum(r0 >= g for g in XG)))
            if r0 - XN >= T0:
                need(("ln", r0 - XN))
            for g in range(8):
                q, o = g // 2, (g % 2) * 8
                rg = q * HQ + r0 + o
                xv = x_v[q, r0 + o:r0 + o + 8, :].astype(f32)
                xg = jnp.concatenate([gate(xv[:, 0:128]), xv[:, 128:]], axis=1)
                mf = jnp.sum(xg, axis=1, keepdims=True) * (1.0 / D)
                d = xv - mf
                var = jnp.sum(d * d, axis=1, keepdims=True) * (1.0 / D)
                rs = lax.rsqrt(var + 1e-5)
                xn_v.at[q][r0 % XN + o:r0 % XN + o + 8, :] = _to_st(d * rs)
                rs = jnp.broadcast_to(rs, (8, 128))
                mf = jnp.broadcast_to(mf, (8, 128))
                sa_v[rg:rg + 8, :] = 1.0 + rs
                sb_v[rg:rg + 8, :] = mf * rs
                st_v[rg:rg + 8, 0:128] = jnp.where(lane == 0, mf, jnp.broadcast_to(var, (8, 128)))
                if tok is not None:
                    tok([rs])
                if g == 7:
                    made.add(("xn", r0))
                yield

    def ln_later(r_start, n_rows, tok, which="all", base=0):
        st_v, xn_v = row_views(base)[3:5]
        for r0 in range(r_start, r_start + n_rows, 16):
            need(("xn", r0))
            form = xs_form(r0, tok, which, base)
            for g in range(8):
                for _ in range(2 if g < 7 else 0):
                    next(form)
                    yield
                q, o = g // 2, (g % 2) * 8
                t = None
                if which != "l1":
                    v = xn_v[q, r0 % XN + o:r0 % XN + o + 8, :] * wrb[8:16, :]
                    for ct in range(8):
                        h = v[:, ct * 128:(ct + 1) * 128]
                        t = gate(h) if t is None else t + h
                if t is not None:
                    st_v[q * HQ + r0 + o:q * HQ + r0 + o + 8, 128:256] = t
                if tok is not None:
                    tok([t])
                if g == 7:
                    next(form, None)
                    made.add(("ln", r0))
                yield

    def wk_prep(c):
        if isinstance(c, int):
            need(("in", c))
        wks.at[c][:, 128:256] = pltpu.bitcast(wk_buf[c, 0:HD, 0:128], u32)
        wks.at[c][:, 512:640] = pltpu.bitcast(wk_buf[c, HD:D, 128:256], u32)
        for i in range(HD // 16):
            r0 = i * 16
            top = wk_buf[c, r0:r0 + 16, :].astype(f32)
            bot = wk_buf[c, HD + r0:HD + r0 + 16, :].astype(f32)
            ops = _rform(top[:, :128], top[:, 128:], bot[:, :128], bot[:, 128:])
            for k in (0, 2, 3, 5, 6):
                wks.at[c][r0 // 2:r0 // 2 + 8, k * 128:(k + 1) * 128] = _pack(ops[k])

    def wq_perm():
        need(("in", 5))

        def permute(kt):
            for g in range(8):
                tile = gate(pltpu.bitcast(wq_buf[kt * 128:(kt + 1) * 128, g * 128:(g + 1) * 128], u32))
                wqt.at[kt * 8 + g][...] = pltpu.bitcast(_unpack(tile).T, u32)
                yield

        def back(kt):
            for j in range(8):
                tile = gate(jnp.concatenate([wqt[kt * 8 + g, pl.ds(j, 8, stride=8), :] for g in range(8)],
                                            axis=0))
                v = pltpu.bitcast(_unpack(tile).T.astype(f32), u32)
                c0 = (kt // 2) * D + _st(j // 2, j % 2).start
                ps[(kt % 2) * 128:(kt % 2 + 1) * 128, c0:c0 + 128] = v
                made.add(("wqp", kt, j))
                yield

        order = (0, 2, 4, 6, 1, 3, 5, 7)
        for n in range(10):
            if n < 8:
                yield from permute(order[n])
            if n > 1:
                yield from back(order[n - 2])

    def wq_form():
        for i in range(16):
            need(*[("wqp", 2 * r + i // 8, j) for r in range(4) for j in range(8)])
            for ct in range(2):
                def put(k1, k2, v):
                    wqs.at[k1 * 7 + k2][i * 8:(i + 1) * 8, ct * 128:(ct + 1) * 128] = v
                yield from form_steps(
                    _rform, _wr, lambda r, c: pltpu.bitcast(
                        ps[i * 16:(i + 1) * 16, r * D + _st(c, ct).start:r * D + _st(c, ct).stop],
                        f32), put)

    def kproj(r0, n, chunks=range(4)):
        pr = pl.ds(r0 // 2, n // 2)
        need(*[("xs", r) for r in range(max(r0, T0), r0 + n, 16)])
        for c in chunks:
            m = [None] * 7
            for k in K_SEQ:
                e11, e12, e21, e22 = [xs_at(L_ORD[k], e)[pr, :] for e in (0, 1, 7, 3)]
                lhs = jnp.concatenate([jnp.concatenate([e11, e12], axis=1),
                                       jnp.concatenate([e21, e22], axis=1)], axis=0)
                m[k] = mm(_unpack(lhs), wks[c, :, k * 128:(k + 1) * 128], NN, 2 * n)
            kk = [_phi(v) for v in _combine(m)]
            for ct in range(2):
                zacc[:, pl.ds(_mo(c * 256 + ct * 128, 128), 128)] += (
                    (kk[ct] + kk[2 + ct]).reshape(n // 4, 8, 128).sum(axis=0))
            j, c2 = (c // 2, c % 2) if isinstance(c, int) else (0, c)
            pk_v = pk_buf.at[j, :, :, pl.ds(_mo(c2 * 256, 256), 256)]
            for s1 in range(4):
                for h in range(2):
                    pk_v.at[(s1 // 2) * 2 + h][r0:r0 + n, (s1 % 2) * 128:(s1 % 2 + 1) * 128] = (
                        kk[s1][h * n:(h + 1) * n])

    def z_prep():
        z = jnp.sum(zacc[...], axis=0, keepdims=True)
        zt = _pack(jnp.broadcast_to(z, (128, D)).astype(bf16).T)
        for g in range(8):
            tscr.at[g][...] = zt[g * 64:(g + 1) * 64, :]
        for j in range(8):
            blk = jnp.concatenate([tscr[g, pl.ds(j, 8, stride=8), :] for g in range(8)], axis=0)
            zp[:, j * 128:(j + 1) * 128] = _unpack(blk).T[0:8, :].astype(f32)

    def route():
        rows, dots = [None] * 16, [None] * 16
        for b in sorted(range(S // 128), key=lambda b: b % 4):
            need(*[("ln", r) for r in range(max(T0, b % 4 * 128), b % 4 * 128 + 128, 16)])
            rows[b] = gate(stats[b * 128:(b + 1) * 128, 0:128]).T[0:8, :]
            dots[b] = jnp.sum(gate(stats[b * 128:(b + 1) * 128, 128:256]).T, axis=0, keepdims=True)
            yield
        mf = jnp.concatenate([v[0:1] for v in rows], axis=0)
        var = jnp.concatenate([v[1:2] for v in rows], axis=0)
        tr = jnp.concatenate(dots, axis=0) * jnp.sqrt(var + 1e-5)
        wsum = jnp.sum(wrb[0:1, :], axis=1, keepdims=True)
        mb = _rbf(mf)
        inv = 1.0 / _rbf(jnp.sqrt(_rbf(_rbf(var) + 1e-5)))
        rv = _rbf((tr + (mf - mb) * wsum) * inv)
        rmax = jnp.max(jnp.max(rv, axis=1, keepdims=True), axis=0, keepdims=True)
        pos = (lax.broadcasted_iota(i32, rv.shape, 0) * 128 + lax.broadcasted_iota(i32, rv.shape, 1))
        idx = jnp.min(jnp.where(rv == rmax, pos, S - 1))
        idx_s[0] = idx

        def pick(v):
            v = jnp.sum(jnp.where(pos == idx, v, 0.0), axis=1, keepdims=True)
            return jnp.sum(v, axis=0, keepdims=True)

        xv = x_buf[(idx >> 9) & 3, pl.ds(_mo(idx & (HQ - 16), 16), 16), :].astype(f32)
        sel = lax.broadcasted_iota(i32, xv.shape, 0) == (idx & 15)
        row = jnp.sum(jnp.where(sel, xv, 0.0), axis=0, keepdims=True)
        row = _rbf(_rbf(row - pick(mb)) * pick(inv))
        rsel[...] = jnp.broadcast_to(_rbf(jnp.sum(row * wrb[0:1, :], axis=1, keepdims=True)), rsel.shape)
        xb[...] = jnp.broadcast_to(row, (128, D)).T
        yield

    def ps_form(j):
        for c in range(HQ // 16):
            def put(k1, k2, v):
                k = k1 * 7 + k2
                ps[c * 8:(c + 1) * 8, k * 128:(k + 1) * 128] = v
            yield from form_steps(
                _lform, _wl_swapped,
                lambda r, q: pk_buf[j, q, c * 16:(c + 1) * 16, r * 128:(r + 1) * 128], put)

    def q_rows(j, r0, n, pq, rc, d0, rec):
        xj = pl.ds(_mo(j * (BQ // 2), BQ // 2), BQ // 2)
        pr = slice(r0 // 2, (r0 + n) // 2)
        blk = yield from strassen2(lambda k1, k2: _unpack(xs_at(L_ORD[k1], k2, xj)[pr, :]),
                                   lambda k1, k2: wqs[k1 * 7 + k2], NN, n, 1, QW)
        lane = lax.broadcasted_iota(i32, (n, 128), 1)
        for q in range(4):
            d = None
            for u in (3, 2, 1, 0):
                v = _phi(blk[q][u])
                for ct in range(2):
                    pq.at[q][d0:d0 + n, _st(u, ct)] = v[:, ct * 128:(ct + 1) * 128]
                t = v * zp[0:1, u * 256:(u + 1) * 256]
                t = t[:, :128] + t[:, 128:]
                d = t if d is None else d + t
            if rec:
                d = recip(d, lane)
            rc.at[q][d0:d0 + n, :] = d

    def recip(d, lane):
        d = d + jnp.where(lane % 2 == 0, pltpu.roll(d, 127, 1), pltpu.roll(d, 1, 1))
        d = d + jnp.where(lane % 4 < 2, pltpu.roll(d, 126, 1), pltpu.roll(d, 2, 1))
        return 1.0 / (d + 1e-6)

    def normalise(pq, rc, nr, dst, raw, tok=None):
        lane = lax.broadcasted_iota(i32, (16, 128), 1)

        def fix(c):
            if c < nr // 16 and raw(c * 16):
                for q in range(4):
                    rq = slice(c * 16, (c + 1) * 16)
                    rc.at[q][rq, :] = recip(gate16(rc[q, rq, :]), lane)

        def scale(c):
            rq = slice(c * 16, (c + 1) * 16)
            fix(c + 1)
            for hf in range(2):
                for q in range(4):
                    cs = slice(hf * HD, (hf + 1) * HD)
                    pq.at[q][rq, cs] = pq[q, rq, cs] * jnp.concatenate([gate16(rc[q, rq, :])] * 4, axis=1)
                    yield

        def form(c):
            rq = slice(c * 16, (c + 1) * 16)
            for ct in range(2):
                def put(k1, k2, v):
                    dst.at[k1 * 7 + k2][c * 8:(c + 1) * 8, ct * 128:(ct + 1) * 128] = v
                yield from form_steps(_lform, _wl, lambda q, u: pq[q, rq, _st(u, ct)], put, tok)

        fix(0)
        if raw(0):
            for _ in range(4):
                yield
        yield from scale(0)
        for c in range(nr // 16):
            nxt = scale(c + 1) if c + 1 < nr // 16 else iter(())
            for i, _ in enumerate(form(c)):
                yield
                if i < 8 and c + 1 < nr // 16:
                    next(nxt)
                    yield

    def g_kvm(j):
        qb = q_rows(j, BQ - QB, QB, pqb_buf.at[j], denb_buf.at[j], 0, False)
        for _ in range(QPRE):
            next(qb)
        blk = yield from strassen2(
            lambda k1, k2: _unpack(ps[:, (k1 * 7 + k2) * 128:(k1 * 7 + k2 + 1) * 128]),
            lambda k1, k2: xs_at(R_ORD[k1], W_R[k2])[...], TN, 256, 2, comb=_wc_swapped)
        hm = (lax.broadcasted_iota(i32, (128, 128), 0) // 32
              == lax.broadcasted_iota(i32, (128, 128), 1) // 32)
        for _ in range(QSPLIT - QPRE):
            next(qb)
        kvps = []
        for a in (3, 2, 1, 0):
            gg = jnp.concatenate(blk[a], axis=1).astype(bf16)
            wv_u = pltpu.bitcast(wv_buf[j, :, a * 128:(a + 1) * 128], u32)
            kv = jnp.where(hm, mm(gg, wv_u, NN, 256), 0.0)
            tscr2.at[a][...] = _pack(kv)
            kvps.append(_unpack(jnp.concatenate(
                [tscr2[a, pl.ds(jj, 8, stride=8), :] for jj in range(8)], axis=0)))

        ms_j = ms.at[:, pl.ds(_mo(j * 32, 32), 96), :]

        def m_form():
            for a in (3, 2, 1, 0):
                need(("mg", a))
                for jl in range(2):
                    for ct in range(2):
                        def put(k1, k2, v):
                            ms_j.at[k1 * 7 + k2][jl * 64 + a * 8:jl * 64 + (a + 1) * 8,
                                                 ct * 128:(ct + 1) * 128] = v
                        yield from form_steps(
                            _rform, _wr, lambda q, u: mg_buf[a, (2 * q + jl) * 16:(2 * q + jl + 1) * 16, _st(u, ct)], put)

        for i, a in enumerate((3, 2, 1, 0)):
            wo_u = pltpu.bitcast(wo_buf[j, a * 128:(a + 1) * 128, :], u32)
            res = mm(kvps[i], wo_u, NN, 256)
            mg_buf.at[a][...] = _to_st(res)
            made.add(("mg", a))
            if i == 0:
                add_side(lambda tok: m_form(), 112, *MF)
        for _ in qb:
            pass

    def out_part(base, span, off, nr, y, src):
        b = _mo(base, 32)
        sa_v, sb_v, out_v = [r.at[pl.ds(b, 3 * HQ + span), :] for r in (sa, sb, out_buf)]
        x_v = x_buf.at[:, pl.ds(b, span), :]
        row = lax.broadcasted_iota(i32, (nr, 256), 0) + (base + off)
        blk = yield from strassen2(lambda k1, k2: _unpack(src[k1 * 7 + k2, off // 2:(off + nr) // 2, :]),
                                   lambda k1, k2: ms[k1 * 7 + k2], NN, nr)
        for s1 in (3, 2, 1, 0):
            for s2 in range(4):
                q = (s1 // 2) * 2 + s2 // 2
                u = (s1 % 2) * 2 + s2 % 2
                rr, cc = pl.ds(q * HQ + off, nr), pl.ds(u * 256, 256)
                a = jnp.concatenate([sa_v[rr, :]] * 2, axis=1)
                c = jnp.concatenate([sb_v[rr, :]] * 2, axis=1)
                o = blk[q][u] + jnp.where(row + q * HQ == idx_s[0], y[:, u * 256:(u + 1) * 256], 0.0)
                out_v[rr, cc] = (x_v[q, off:off + nr, cc].astype(f32) * a - c + o).astype(bf16)
                if s2 % 2 == 1:
                    ch = pl.ds((s1 % 2) * HD, HD)
                    ro = pl.ds(_mo(base + q * HQ + off, 16), nr)
                    cp(out_buf.at[ro, ch], out_hbm.at[0, ro, ch], SEM_O).start()

    def ffn_part(j):
        def fma(acc, w, v):
            p = w.astype(f32) * v
            return acc + p[0:8] + p[8:16]

        for f0 in range(0, FH, 256):
            fs = slice(f0, f0 + 256)
            ag = jnp.zeros((8, 256), f32)
            au = jnp.zeros((8, 256), f32)
            for k in range(0, D, 16):
                xv = jnp.concatenate([gate16(xb[k:k + 16, :])] * 2, axis=1)
                ag = fma(ag, wg_buf[j, k:k + 16, fs], xv)
                au = fma(au, wu_buf[j, k:k + 16, fs], xv)
                yield
            g = _rbf(jnp.sum(ag, axis=0, keepdims=True))
            u = _rbf(jnp.sum(au, axis=0, keepdims=True))
            h = _rbf(_rbf(g * jax.nn.sigmoid(g)) * u)
            hb_buf[fs, :] = jnp.broadcast_to(h, (128, 256)).T
        for d0 in range(0, D, 512):
            ds_ = slice(d0, d0 + 512)
            acc = yacc[:, ds_]
            for k in range(0, FH, 16):
                hv = jnp.concatenate([gate16(hb_buf[k:k + 16, :])] * 4, axis=1)
                acc = fma(acc, wd_buf[j, k:k + 16, ds_], hv)
                yield
            yacc[:, ds_] = acc

    def wait_group(i):
        with _scope("a_wait%d" % i):
            for c in a_groups[i]:
                c.wait()
        made.add(("in", i - NX))

    def run_all(gen):
        for _ in gen:
            pass

    def ln_sides(plan):
        for r0, r1, t0, t1 in plan[0]:
            add_side(lambda tok, r0=r0, r1=r1: ln_stats(r0, r1 - r0, tok), (r1 - r0) // 2, t0, t1, LNLAG)
        for r0, r1, t0, t1 in plan[1]:
            add_side(lambda tok, r0=r0, r1=r1: ln_later(r0, r1 - r0, tok), 22 * (r1 - r0) // 16, t0, t1, SLAG)

    def l2_side(base, n, t0, t1):
        add_side(lambda tok: ln_later(0, n, None, "l2", base), 22 * n // 16, t0, t1)

    with _scope("p0_issue"):
        cp_wr.start()
        for grp in a_groups:
            for c in grp:
                c.start()
        for j in range(2):
            for c in cp_b(j):
                c.start()
        zacc[...] = jnp.zeros(zacc.shape, f32)
        yacc[...] = jnp.zeros(yacc.shape, f32)
        zero_buf[1] = jnp.zeros((8, 128), u32)
        cp_zero = cp(zero_buf.at[1], zero_buf.at[0], SEM_Z)
        cp_zero.start()
        cp_zero.wait()
        cp_wr.wait()
        wr8 = jnp.broadcast_to(wr_buf[0:D].reshape(1, D).astype(f32), (8, D))
        wrb[0:8, :] = wr8
        wrb[8:16, :] = _to_st(wr8)
        z0 = jnp.max(pltpu.bitcast(zero_buf[0], i32))
        ps, pq_buf, den_buf, mg_buf, hb_buf = [r.at[z0] for r in (ps_raw, pq_raw, den_raw, mg_raw, hb_raw)]
        xn_buf = mg_buf

    def main(_, carry0):
        def a01(i, carry):
            with _scope("a_wait01"):
                for c in cp_x(i * X0, X0, SEM_A + i):
                    c.wait()
            with _scope("a01"):
                for r in range(0, X0, 16):
                    run_all(ln_stats(r, 16, None, (i, X0)))
                    if r:
                        run_all(ln_later(r - 16, 16, None, "l1", (i, X0)))
                run_all(ln_later(X0 - 16, 16, None, "l1", (i, X0)))
            return carry

        lax.fori_loop(0, NX, a01, 0)
        made.update(("xn", r) for r in range(0, 64, 16))

        def a23(i, carry):
            with _scope("a_wait23"):
                for c in cp_wk(i, SEM_W + i):
                    c.wait()
            with _scope("a23"):
                wk_prep(i)
                l2_side((i, T0 // 2), T0 // 2, *L2W)
                kproj(0, T0, [i])
                finish()
            return carry

        lax.fori_loop(0, 2, a23, 0)
        wait_group(NX + 2)
        with _scope("a4"):
            wk_prep(2)
            ln_sides(L4)
            kproj(0, T0, [2])
            finish()
        wait_group(NX + 3)
        with _scope("a5"):
            wk_prep(3)
            ln_sides(L5)
            kproj(0, T0, [3])
            for r0, n in A5K:
                kproj(r0, n)
            finish()
        wait_group(NX + 4)
        with _scope("a6"):
            ln_sides(L6)
            for r0, n in A6K:
                kproj(r0, n)
            finish()
        wait_group(NX + 5)
        with _scope("a7"):
            ln_sides(L7)
            add_side(lambda tok: wq_perm(), 128, *WQ_PERM)
            add_side(lambda tok: wq_form(), 224, *WQ_FORM)
            add_side(lambda tok: route(), 17, *ROUTE)
            for r0, n in A7K:
                kproj(r0, n)
            finish()

        def b_body(j, carry):
            qa = BQ - QB
            with _scope("b_r0"):
                z_prep()
                add_side(lambda tok: ps_form(j), 7 * HQ // 16, *PSW)
                for r0 in range(0, qa, QN):
                    run_all(q_rows(j, r0, QN, pq_buf, den_buf, r0, r0 + QN < qa))
                finish()
            with _scope("b_wait"):
                for c in cp_b(j, wait_only=True):
                    c.wait()
            with _scope("b_r1"):
                add_side(lambda tok: ffn_part(j), FH * 3 // 8, *FFW)
                qs_j = qs.at[:, pl.ds(_mo(j * (qa // 2), 16), qa // 2), :]
                add_side(lambda tok: normalise(pq_buf, den_buf, qa, qs_j, lambda r: r >= qa - QN),
                         22 * (qa // 16), *NRW)
                run_all(g_kvm(j))
                finish()
            return carry

        lax.fori_loop(0, 2, b_body, 0)

        def c_body(t, carry):
            with _scope("c_body"):
                y = _rbf(jnp.sum(yacc[...], axis=0, keepdims=True))
                y = _rbf(y * _rbf(1.0 / _rbf(1.0 + _rbf(jnp.exp(-rsel[0:1, :])))))
                j, h = t >> 1, t & 1
                na, nb = (BQ - QB) // 2, QB // 2
                hb = pl.ds(_mo(h * nb, 16), nb)
                add_side(lambda tok: normalise(pqb_buf.at[j, :, hb, :], denb_buf.at[j, :, hb, :], nb, qsb,
                                               lambda r: True, tok),
                         4 + 22 * (nb // 16), *CNW, SLAG)
                qs_t = qs.at[:, pl.ds(_mo(t * (na // 2), 16), na // 2), :]
                for p in range(0, na, CR):
                    run_all(out_part(j * BQ + h * na, na, p, CR, y, qs_t))
                flush()
                run_all(out_part(j * BQ + BQ - QB + h * nb, nb, 0, nb, y, qsb))
                finish()
            return carry

        lax.fori_loop(0, 4, c_body, 0)
        return carry0

    lax.fori_loop(0, z0 + 1, main, 0)
    with _scope("tail"):
        cp(out_buf, out_hbm.at[0], SEM_O).wait()


@jax.jit
def pallas_parallel_sum__linear_attn_block__moe_arch_mod__prompt_kernel(
    A_x: jax.Array,
    A_wqkv: jax.Array,
    A_wo: jax.Array,
    B_x: jax.Array,
    B_w_r: jax.Array,
    B_w_gate: jax.Array,
    B_w_up: jax.Array,
    B_w_down: jax.Array,
):
    del B_x
    V = pltpu.VMEM
    scratch = [
        V((4, HQ, D), bf16),
        V((4, D, 256), bf16),
        V((2, D, 512), bf16),
        V((2, 512, D), bf16),
        V((8 * D,), bf16),
        V((2, D, FH), bf16),
        V((2, D, FH), bf16),
        V((2, FH, D), bf16),
        V((28, HQ // 2, 256), u32),
        V((28, HQ // 2, 256), u32),
        V((49, 128, 256), u32),
        V((S, 128), f32),
        V((S, 128), f32),
        V((8, D), f32),
        V((8, D), f32),
        V((2, 4, HQ, 512), f32),
        V((D, 128), f32),
        V((8, D), f32),
        V((8, D), f32),
        V((16, D), f32),
        V((4, 8, 128), u32),
        V((4, HD // 2, 7 * 128), u32),
        V((S, 256), f32),
        V((64, 64, 128), u32),
        V((1, HQ // 2, 49 * 128), u32),
        V((49, BQ - QB, 256), u32),
        V((49, 128, 256), u32),
        V((8, 64, 128), u32),
        V((4, 64, 128), u32),
        V((1, 4, BQ - QB, D), f32),
        V((1, 4, BQ - QB, 128), f32),
        V((2, 4, QB, D), f32),
        V((2, 4, QB, 128), f32),
        V((49, QB // 4, 256), u32),
        V((1, 4, 128, D), f32),
        V((1, FH, 128), f32),
        V((S, D), bf16),
        pltpu.SMEM((1,), i32),
        pltpu.SemaphoreType.DMA((4 + T0 // X0 + 6,)),
    ]
    extra = {k: True for k in ("disable_bounds_checks", "disable_semaphore_checks")
             if hasattr(pltpu.CompilerParams, k)}
    return pl.pallas_call(
        _kernel,
        out_shape=jax.ShapeDtypeStruct((1, S, D), bf16),
        in_specs=[pl.BlockSpec(memory_space=pl.ANY)] * 7,
        out_specs=pl.BlockSpec(memory_space=pl.ANY),
        scratch_shapes=scratch,
        compiler_params=pltpu.CompilerParams(vmem_limit_bytes=120 * 1024 * 1024, **extra),
    )(A_x.reshape(4, HQ, D), A_wqkv, A_wo, B_w_r, B_w_gate, B_w_up, B_w_down)
```

```python
import contextlib

import jax
import jax.numpy as jnp
from jax import lax
import jax.experimental.pallas as pl
import jax.experimental.pallas.tpu as pltpu

bf16, f32, u32, i32 = jnp.bfloat16, jnp.float32, jnp.uint32, jnp.int32

S = 2048
D = 1024
F = 3584
HD = D // 2
HQ = S // 4
BQ = HQ // 2
FH = F // 2
QB = 64
QN = 48
QSPLIT = 5
CR = 48
T0 = 96
X0 = 32
XG = (144, 176, 368)
XN = 128

SLAG = 400
LNLAG = 700
QW = (22, 12, 22, 12, 22, 12, 10)
QWB = (26, 10, 26, 10, 26, 8, 6)
L4 = ([(96, 144, 0, 1070)], [])
L5 = ([(144, 176, 310, 1750)], [(96, 128, 220, 1170), (128, 144, 1340, 2060), (144, 176, 2010, 2910)])
L6 = ([(176, 368, 0, 7410)], [(176, 224, 740, 2510), (224, 336, 2800, 7870)])
L7 = ([(368, 512, 0, 4800)], [(336, 384, 0, 2400), (384, 512, 2500, 9000)])
A5K = ((96, 32),)
A6K = ((128, 48), (176, 48), (224, 48))
A7K = ((272, 64), (336, 48), (384, 64), (448, 64))
WQ_PERM, WQ_FORM, ROUTE = (5100, 7900), (8000, 13100), (9400, 10200)
L2W, PSW, FFW, NRW, CNW = (270, 1304), (0, 7400), (0, 12800), (0, 12800), (0, 3614)
MF = (128, 3540)
PFW = ((2100, 3900), (4000, 5800), (5850, 7600), (7650, 9200))

L_ORD = (2, 3, 0, 1, 4, 5, 6)
R_ORD = (2, 0, 6, 5, 1, 4, 3)

K_SEQ = (1, 4, 0, 2, 3, 5, 6)
K_SEQ2 = (1, 3, 2, 4, 0, 5, 6)
W_SEQ = (0, 1, 5, 6, 4, 2, 3)

SCOPES = False


def _scope(name):
    return jax.named_scope(name) if SCOPES else contextlib.nullcontext()


def _mo(v, m):
    return v if isinstance(v, int) else pl.multiple_of(v, m)


def _pack(v):
    return pltpu.bitcast(v.astype(bf16), u32)


def _unpack(v):
    return pltpu.bitcast(v, bf16)


def _combine(m):
    m1, m2, m3, m4, m5, m6, m7 = m
    return m1 + m4 - m5 + m7, m3 + m5, m2 + m4, m1 - m2 + m3 + m6


def _combine2(m):
    m1, m2, m3, m4, m5, m6, m7 = m
    return (m4 - m5) + m1 + m7, m3 + m5, m2 + m4, (m3 - m2) + m1 + m6


def _lform(a11, a12, a21, a22):
    return (a11 + a22, a21 + a22, a11, a22, a11 + a12, a21 - a11, a12 - a22)


def _rform(b11, b12, b21, b22):
    return (b11 + b22, b11, b12 - b22, b21 - b11, b22, b11 + b12, b21 + b22)


def _sform(x11, x12, x21, x22):
    return (x11, x22, x11 + x22, x21 + x22, x11 + x12, x21 - x11, x12 - x22)


def _wl(a11, a12, a21, a22):
    s1 = a21 + a22
    s2 = s1 - a11
    return (a11, a12, a12 - s2, a22, s1, s2, a11 - a21)


def _wr(b11, b12, b21, b22):
    t1 = b12 - b11
    t2 = b22 - t1
    return (b11, b21, b22, t2 - b21, t1, t2, b22 - b12)


def _wc(p):
    p1, p2, p3, p4, p5, p6, p7 = p
    u2 = p1 + p6
    u3 = u2 + p7
    return p1 + p2, (u2 + p5) + p3, u3 - p4, u3 + p5


W_R = (3, 1, 0, 2, 4, 5, 6)


def _wl_swapped(a11, a12, a21, a22):
    return _wl(a12, a11, a22, a21)


def _wc_swapped(p):
    p1, p2, p3, p4, p5, p6, p7 = p
    v2 = p1 + p6
    u3 = p7 - v2
    return (p5 - v2) + p3, p1 + p2, u3 + p5, p4 - u3


class _Sym:
    def __init__(self, t):
        self.t = t

    def __add__(self, o):
        return _Sym({**self.t, **o.t})

    def __sub__(self, o):
        return _Sym({**self.t, **{k: -v for k, v in o.t.items()}})


def _st(u, ct):
    return slice((4 * ct + u) * 128, (4 * ct + u + 1) * 128)


def _to_st(v):
    return jnp.concatenate([v[:, (2 * u + ct) * 128:(2 * u + ct + 1) * 128]
                            for ct in range(2) for u in range(4)], axis=1)


def _phi(t):
    return jnp.where(t > 0, t + 1.0, jnp.exp(t)) + 1e-6


def _rbf(v):
    return v.astype(bf16).astype(f32)


def _kernel(x_hbm, wqkv_hbm, wo_hbm, wr_hbm, wg_hbm, wu_hbm, wd_hbm, out_hbm,
            x_buf, wk_buf, wv_buf, wo_buf, wr_buf, wg_buf, wu_buf, wd_buf,
            xs1, xs2, wqs, sa, sb, zacc, zp, pk_buf, xb, yacc, rsel, wrb, zero_buf,
            wks, stats, wqt, ps_raw, qs, ms, tscr, tscr2, pq_raw, den_raw, pqb_buf, denb_buf, qsb,
            mg_raw, hb_raw, out_buf, idx_s, sem):
    wq_buf = out_buf.at[pl.ds(0, D), :]

    def xs_at(k1, e, rows=None):
        r = xs1.at[k1 * 4 + (0, 1, 7, 3).index(e)] if e in (0, 1, 7, 3) else xs2.at[k1 * 4 + (2, 4, 5, 6).index(e)]
        return r if rows is None else r.at[rows, :]

    SEM_B, SEM_O, SEM_Z, SEM_A = 0, 2, 3, 4

    def cp(src, dst, s):
        return pltpu.make_async_copy(src, dst, sem.at[s])

    def cp_x(r0, n, s):
        r = pl.ds(_mo(r0, 16), n)
        return [cp(x_hbm.at[:, r, :], x_buf.at[:, r, :], s)]

    def cp_wk(c, s):
        return [cp(wqkv_hbm.at[:, pl.ds(_mo(D + c * 256, 256), 256)],
                   wk_buf.at[c], s)]

    NX = T0 // X0
    SEM_W = SEM_A + NX
    cp_wr = cp(wr_hbm, wr_buf.at[pl.ds(0, D)], SEM_Z)
    a_groups = [cp_x(i * X0, X0, SEM_A + i) for i in range(NX)] + [
        cp_wk(0, SEM_W),
        cp_wk(1, SEM_W + 1),
        cp_wk(2, SEM_W + 2) + cp_x(T0, XG[0] - T0, SEM_W + 2),
        cp_wk(3, SEM_W + 3) + cp_x(XG[0], XG[1] - XG[0], SEM_W + 3),
        cp_x(XG[1], XG[2] - XG[1], SEM_W + 4),
        (cp_x(XG[2], HQ - XG[2], SEM_W + 5) if XG[2] < HQ else [])
        + [cp(wqkv_hbm.at[:, pl.ds(0, D)], wq_buf, SEM_W + 5)],
    ]

    def cp_b(j, wait_only=False):
        dsts = [r.at[j] for r in (wg_buf, wu_buf, wd_buf, wv_buf, wo_buf)]
        if wait_only:
            return [cp(dst, dst, SEM_B + j) for dst in dsts]
        fs = pl.ds(j * FH, FH)
        srcs = [wg_hbm.at[:, fs], wu_hbm.at[:, fs], wd_hbm.at[fs, :],
                wqkv_hbm.at[:, pl.ds(2 * D + j * HD, HD)], wo_hbm.at[pl.ds(j * HD, HD), :]]
        return [cp(src, dst, SEM_B + j) for src, dst in zip(srcs, dsts)]

    clock = [0]
    toks = []
    sides = []
    fwd = [None]

    def emit_tok(vals, stamp):
        t = None
        for v in vals:
            v = pltpu.bitcast(v, u32) if v.dtype != u32 else v
            t = v if t is None else t | v
        toks.append((stamp, t & zero_buf[0]))

    def token(kind):
        t = fwd[0]
        if "u" not in t:
            t["u"] = pltpu.bitcast(t["src"](), u32) & zero_buf[0]
        if kind != "u" and "f" not in t:
            t["f"] = pltpu.bitcast(t["u"], f32)
        if kind == "f16" and "f16" not in t:
            t["f16"] = jnp.concatenate([t["f"], t["f"]], axis=0)
        return t[kind]

    def gate(v):
        if fwd[0] is None:
            return v
        head = v if v.shape[0] == 8 else v[0:8]
        head = head | token("u") if v.dtype == u32 else head + token("f")
        return head if v.shape[0] == 8 else jnp.concatenate([head, v[8:]], axis=0)

    def gate16(v):
        return v if fwd[0] is None else v + token("f16")

    def add_side(gen_fn, n, t0, t1, lag=None):
        st = {"i": 0, "n": n, "t0": clock[0] + t0, "t1": clock[0] + t1}

        def tok(vals):
            if lag is not None:
                emit_tok(vals, st["t0"] + (st["i"] + 1) * (st["t1"] - st["t0"]) // st["n"] + lag)
        st["g"] = gen_fn(tok)
        sides.append(st)

    def advance(until):
        for st in sides:
            while st["i"] < st["n"] and st["t0"] + st["i"] * (st["t1"] - st["t0"]) // st["n"] < until:
                next(st["g"], None)
                st["i"] += 1
                if st["i"] == st["n"]:
                    for _ in st["g"]:
                        pass

    def flush():
        for st in sides:
            for _ in st["g"]:
                pass
        sides.clear()

    def finish():
        flush()
        toks.clear()
        fwd[0] = None

    def mm(lhs, rhs, cycles, nseg=1):
        due = [t for (c, t) in toks if c <= clock[0]]
        toks[:] = [(c, t) for (c, t) in toks if c > clock[0]]
        if due:
            head = rhs[0:8, 0:128]
            for t in due:
                head = head | t
            if rhs.shape[1] > 128:
                head = jnp.concatenate([head, rhs[0:8, 128:]], axis=1)
            rhs = jnp.concatenate([head, rhs[8:]], axis=0)
        res = jnp.dot(lhs, _unpack(rhs), preferred_element_type=f32)
        ngr = res.shape[0] // 16
        for sg in range(nseg):
            for i in range(ngr):
                fwd[0] = {"src": lambda sg=sg, i=i: res[i * 16:i * 16 + 8, sg * 128:(sg + 1) * 128]}
                clock[0] += cycles // nseg // ngr
                advance(clock[0])
        return res

    def form_steps(form, form2, get, put, tok=None, keep=range(7)):
        terms = form(*[_Sym({i: 1}) for i in range(4)])
        gated = (0, 1, 2, 3) if 7 in keep else {_wl: (0, 1, 3), _wr: (0, 2, 3), _wl_swapped: (1, 2)}[form2]
        for k1 in range(7):
            sub = []
            for r in range(2):
                for c in range(2):
                    v = None
                    for i, sg in sorted(terms[k1].t.items(), key=lambda e: -e[1]):
                        b = get(r + 2 * (i // 2), c + 2 * (i % 2))
                        if v is None:
                            v = gate16(b) if 2 * r + c in gated else b
                        else:
                            v = v + b if sg > 0 else v - b
                    sub.append(v)
            vals = form2(*sub) + (sub[2],)
            for k2 in keep:
                put(k1, k2, _pack(vals[k2]))
            if tok is not None and k1 % 2 == 0:
                full = vals[3 if form2 is _wr else 2]
                tok([full[0:8], full[8:16]])
            yield

    def strassen2(lhs, rhs, cycles, nseg=1, wts=(16,) * 7, comb=_wc):
        m1 = [None] * 7
        for i1, k1 in enumerate(K_SEQ2):
            m2 = [None] * 7
            for k2 in W_SEQ:
                m2[k2] = mm(lhs(k1, k2), rhs(k1, k2), cycles * wts[i1] // 16, nseg)
                yield
            m1[k1] = comb(m2)
        out = [[None] * 4 for _ in range(4)]
        for s2 in range(4):
            for s1, v in enumerate(_combine2([m1[k1][s2] for k1 in range(7)])):
                out[(s1 // 2) * 2 + s2 // 2][(s1 % 2) * 2 + s2 % 2] = v
        return out

    made = set()

    def need(*keys):
        assert all(k in made for k in keys), keys

    def row_views(base):
        if base == 0:
            return x_buf, sa, sb, stats, xn_buf, None
        i, n = base
        b = _mo(i * n, 16)
        return ([x_buf.at[:, pl.ds(b, n), :]] + [r.at[pl.ds(b, S - 128 + n), :] for r in (sa, sb, stats)]
                + [xn_buf.at[:, pl.ds(b, n), :], pl.ds(_mo(i * (n // 2), 8), n // 2)])

    def xs_form(r0, tok, which="all", base=0):
        xn_v, xs_v = row_views(base)[4:]
        rows = slice(r0 % XN, r0 % XN + 16)

        keep = {"all": range(8), "l1": (0, 1, 7, 3), "l2": (2, 4, 5, 6)}[which]
        for ct in range(2):
            def put(k1, k2, v):
                xs_at(k1, k2, xs_v)[r0 // 2:r0 // 2 + 8, ct * 128:(ct + 1) * 128] = v
            yield from form_steps(
                _sform, _wl, lambda q, u: xn_v[q, rows, _st(u, ct)], put, tok, keep)
        made.add(("xs", r0))

    def ln_stats(r_start, n_rows, tok, base=0):
        x_v, sa_v, sb_v, st_v, xn_v, _ = row_views(base)
        lane = lax.broadcasted_iota(i32, (8, 128), 1)
        for r0 in range(r_start, r_start + n_rows, 16):
            if r0 >= T0:
                need(("in", 2 + sum(r0 >= g for g in XG)))
            if r0 - XN >= T0:
                need(("ln", r0 - XN))
            for g in range(8):
                q, o = g // 2, (g % 2) * 8
                rg = q * HQ + r0 + o
                xv = x_v[q, r0 + o:r0 + o + 8, :].astype(f32)
                xg = jnp.concatenate([gate(xv[:, 0:128]), xv[:, 128:]], axis=1)
                mf = jnp.sum(xg, axis=1, keepdims=True) * (1.0 / D)
                d = xv - mf
                var = jnp.sum(d * d, axis=1, keepdims=True) * (1.0 / D)
                rs = lax.rsqrt(var + 1e-5)
                xn_v.at[q][r0 % XN + o:r0 % XN + o + 8, :] = _to_st(d * rs)
                rs = jnp.broadcast_to(rs, (8, 128))
                mf = jnp.broadcast_to(mf, (8, 128))
                sa_v[rg:rg + 8, :] = 1.0 + rs
                sb_v[rg:rg + 8, :] = mf * rs
                st_v[rg:rg + 8, 0:128] = jnp.where(lane == 0, mf, jnp.broadcast_to(var, (8, 128)))
                if tok is not None:
                    tok([rs])
                if g == 7:
                    made.add(("xn", r0))
                yield

    def ln_later(r_start, n_rows, tok, which="all", base=0):
        st_v, xn_v = row_views(base)[3:5]
        for r0 in range(r_start, r_start + n_rows, 16):
            need(("xn", r0))
            form = xs_form(r0, tok, which, base)
            for g in range(8):
                for _ in range(2 if g < 7 else 0):
                    next(form)
                    yield
                q, o = g // 2, (g % 2) * 8
                t = None
                if which != "l1":
                    v = xn_v[q, r0 % XN + o:r0 % XN + o + 8, :] * wrb[8:16, :]
                    for ct in range(8):
                        h = v[:, ct * 128:(ct + 1) * 128]
                        t = gate(h) if t is None else t + h
                if t is not None:
                    st_v[q * HQ + r0 + o:q * HQ + r0 + o + 8, 128:256] = t
                if tok is not None:
                    tok([t])
                if g == 7:
                    next(form, None)
                    made.add(("ln", r0))
                yield

    def wk_prep(c):
        if isinstance(c, int):
            need(("in", c))
        wks.at[c][:, 128:256] = pltpu.bitcast(wk_buf[c, 0:HD, 0:128], u32)
        wks.at[c][:, 512:640] = pltpu.bitcast(wk_buf[c, HD:D, 128:256], u32)
        for i in range(HD // 16):
            r0 = i * 16
            top = wk_buf[c, r0:r0 + 16, :].astype(f32)
            bot = wk_buf[c, HD + r0:HD + r0 + 16, :].astype(f32)
            ops = _rform(top[:, :128], top[:, 128:], bot[:, :128], bot[:, 128:])
            for k in (0, 2, 3, 5, 6):
                wks.at[c][r0 // 2:r0 // 2 + 8, k * 128:(k + 1) * 128] = _pack(ops[k])

    def wq_perm():
        need(("in", 5))

        def permute(kt):
            for g in range(8):
                tile = gate(pltpu.bitcast(wq_buf[kt * 128:(kt + 1) * 128, g * 128:(g + 1) * 128], u32))
                wqt.at[kt * 8 + g][...] = pltpu.bitcast(_unpack(tile).T, u32)
                yield

        def back(kt):
            for j in range(8):
                tile = gate(jnp.concatenate([wqt[kt * 8 + g, pl.ds(j, 8, stride=8), :] for g in range(8)],
                                            axis=0))
                v = pltpu.bitcast(_unpack(tile).T.astype(f32), u32)
                c0 = (kt // 2) * D + _st(j // 2, j % 2).start
                ps[(kt % 2) * 128:(kt % 2 + 1) * 128, c0:c0 + 128] = v
                made.add(("wqp", kt, j))
                yield

        order = (0, 2, 4, 6, 1, 3, 5, 7)
        for n in range(10):
            if n < 8:
                yield from permute(order[n])
            if n > 1:
                yield from back(order[n - 2])

    def wq_form():
        for i in range(16):
            need(*[("wqp", 2 * r + i // 8, j) for r in range(4) for j in range(8)])
            for ct in range(2):
                def put(k1, k2, v):
                    wqs.at[k1 * 7 + k2][i * 8:(i + 1) * 8, ct * 128:(ct + 1) * 128] = v
                yield from form_steps(
                    _rform, _wr, lambda r, c: pltpu.bitcast(
                        ps[i * 16:(i + 1) * 16, r * D + _st(c, ct).start:r * D + _st(c, ct).stop],
                        f32), put)

    def kproj(r0, n, chunks=range(4)):
        pr = pl.ds(r0 // 2, n // 2)
        need(*[("xs", r) for r in range(max(r0, T0), r0 + n, 16)])
        for c in chunks:
            m = [None] * 7
            for k in K_SEQ:
                e11, e12, e21, e22 = [xs_at(L_ORD[k], e)[pr, :] for e in (0, 1, 7, 3)]
                lhs = jnp.concatenate([jnp.concatenate([e11, e12], axis=1),
                                       jnp.concatenate([e21, e22], axis=1)], axis=0)
                m[k] = mm(_unpack(lhs), wks[c, :, k * 128:(k + 1) * 128], 2 * n)
            kk = [_phi(v) for v in _combine(m)]
            for ct in range(2):
                zacc[:, pl.ds(_mo(c * 256 + ct * 128, 128), 128)] += (
                    (kk[ct] + kk[2 + ct]).reshape(n // 4, 8, 128).sum(axis=0))
            j, c2 = (c // 2, c % 2) if isinstance(c, int) else (0, c)
            pk_v = pk_buf.at[j, :, :, pl.ds(_mo(c2 * 256, 256), 256)]
            for s1 in range(4):
                for h in range(2):
                    pk_v.at[(s1 // 2) * 2 + h][r0:r0 + n, (s1 % 2) * 128:(s1 % 2 + 1) * 128] = (
                        kk[s1][h * n:(h + 1) * n])

    def z_prep():
        z = jnp.sum(zacc[...], axis=0, keepdims=True)
        zt = _pack(jnp.broadcast_to(z, (128, D)).astype(bf16).T)
        for g in range(8):
            tscr.at[g][...] = zt[g * 64:(g + 1) * 64, :]
        for j in range(8):
            blk = jnp.concatenate([tscr[g, pl.ds(j, 8, stride=8), :] for g in range(8)], axis=0)
            zp[:, j * 128:(j + 1) * 128] = _unpack(blk).T[0:8, :].astype(f32)

    def route():
        rows, dots = [None] * 16, [None] * 16
        for b in sorted(range(S // 128), key=lambda b: b % 4):
            need(*[("ln", r) for r in range(max(T0, b % 4 * 128), b % 4 * 128 + 128, 16)])
            rows[b] = gate(stats[b * 128:(b + 1) * 128, 0:128]).T[0:8, :]
            dots[b] = jnp.sum(gate(stats[b * 128:(b + 1) * 128, 128:256]).T, axis=0, keepdims=True)
            yield
        mf = jnp.concatenate([v[0:1] for v in rows], axis=0)
        var = jnp.concatenate([v[1:2] for v in rows], axis=0)
        tr = jnp.concatenate(dots, axis=0) * jnp.sqrt(var + 1e-5)
        wsum = jnp.sum(wrb[0:1, :], axis=1, keepdims=True)
        mb = _rbf(mf)
        inv = 1.0 / _rbf(jnp.sqrt(_rbf(_rbf(var) + 1e-5)))
        rv = _rbf((tr + (mf - mb) * wsum) * inv)
        rmax = jnp.max(jnp.max(rv, axis=1, keepdims=True), axis=0, keepdims=True)
        pos = (lax.broadcasted_iota(i32, rv.shape, 0) * 128 + lax.broadcasted_iota(i32, rv.shape, 1))
        idx = jnp.min(jnp.where(rv == rmax, pos, S - 1))
        idx_s[0] = idx

        def pick(v):
            v = jnp.sum(jnp.where(pos == idx, v, 0.0), axis=1, keepdims=True)
            return jnp.sum(v, axis=0, keepdims=True)

        xv = x_buf[(idx >> 9) & 3, pl.ds(_mo(idx & (HQ - 16), 16), 16), :].astype(f32)
        sel = lax.broadcasted_iota(i32, xv.shape, 0) == (idx & 15)
        row = jnp.sum(jnp.where(sel, xv, 0.0), axis=0, keepdims=True)
        row = _rbf(_rbf(row - pick(mb)) * pick(inv))
        rsel[...] = jnp.broadcast_to(_rbf(jnp.sum(row * wrb[0:1, :], axis=1, keepdims=True)), rsel.shape)
        xb[...] = jnp.broadcast_to(row, (128, D)).T
        yield

    def ps_form(j):
        for c in range(HQ // 16):
            def put(k1, k2, v):
                k = k1 * 7 + k2
                ps[c * 8:(c + 1) * 8, k * 128:(k + 1) * 128] = v
            yield from form_steps(
                _lform, _wl_swapped,
                lambda r, q: pk_buf[j, q, c * 16:(c + 1) * 16, r * 128:(r + 1) * 128], put)
            made.add(("ps", c))

    def ps_flip(t):
        need(*[("ps", c) for c in range(8 * t, 8 * t + 8)])
        for k in range(49):
            at = (slice(t * 64, (t + 1) * 64), slice(k * 128, (k + 1) * 128))
            ps[at] = pltpu.bitcast(_unpack(gate(ps[at])).T, u32)
            yield

    def q_rows(j, r0, n, pq, rc, d0, wts):
        xj = pl.ds(_mo(j * (BQ // 2), BQ // 2), BQ // 2)
        pr = slice(r0 // 2, (r0 + n) // 2)
        blk = yield from strassen2(lambda k1, k2: _unpack(xs_at(L_ORD[k1], k2, xj)[pr, :]),
                                   lambda k1, k2: wqs[k1 * 7 + k2], n, 1, wts)
        for q in range(4):
            d = None
            for u in ((0, 1, 2, 3) if q >= 2 else (3, 2, 1, 0)):
                v = _phi(blk[q][u])
                for ct in range(2):
                    pq.at[q][d0:d0 + n, _st(u, ct)] = v[:, ct * 128:(ct + 1) * 128]
                t = v * zp[0:1, u * 256:(u + 1) * 256]
                t = t[:, :128] + t[:, 128:]
                d = t if d is None else d + t
            rc.at[q][d0:d0 + n, :] = d

    def normalise(pq, rc, nr, dst, tok=None):
        lane = lax.broadcasted_iota(i32, (16, 128), 1)
        nc = nr // 16

        def recips(c):
            rq = slice(c * 16, (c + 1) * 16)
            for q in range(4):
                d = gate16(rc[q, rq, :])
                d = d + jnp.where(lane % 2 == 0, pltpu.roll(d, 127, 1), pltpu.roll(d, 1, 1))
                d = d + jnp.where(lane % 4 < 2, pltpu.roll(d, 126, 1), pltpu.roll(d, 2, 1))
                rc.at[q][rq, :] = 1.0 / (d + 1e-6)
                yield

        def scale(c):
            rq = slice(c * 16, (c + 1) * 16)
            for hf in range(2):
                for q in range(4):
                    cs = slice(hf * HD, (hf + 1) * HD)
                    pq.at[q][rq, cs] = pq[q, rq, cs] * jnp.concatenate([gate16(rc[q, rq, :])] * 4, axis=1)
                    yield

        def form(c):
            rq = slice(c * 16, (c + 1) * 16)
            for ct in range(2):
                def put(k1, k2, v):
                    dst.at[k1 * 7 + k2][c * 8:(c + 1) * 8, ct * 128:(ct + 1) * 128] = v
                yield from form_steps(_lform, _wl, lambda q, u: pq[q, rq, _st(u, ct)], put, tok)

        def ahead(c):
            if c + 2 < nc:
                yield from recips(c + 2)
            if c + 1 < nc:
                yield from scale(c + 1)

        yield from recips(0)
        yield from recips(1)
        for _ in range(4):
            yield
        yield from scale(0)
        for c in range(nc):
            nxt = ahead(c)
            for _ in form(c):
                yield
                if next(nxt, 0) is None:
                    yield

    def g_kvm(j):
        qb = q_rows(j, BQ - QB, QB, pqb_buf.at[j], denb_buf.at[j], 0, QWB)
        blk = yield from strassen2(
            lambda k1, k2: _unpack(jnp.concatenate(
                [ps[t * 64:(t + 1) * 64, (k1 * 7 + k2) * 128:(k1 * 7 + k2 + 1) * 128] for t in range(4)], axis=1)),
            lambda k1, k2: xs_at(R_ORD[k1], W_R[k2])[...], 256, 2, comb=_wc_swapped)
        hm = (lax.broadcasted_iota(i32, (128, 128), 0) // 32
              == lax.broadcasted_iota(i32, (128, 128), 1) // 32)
        for _ in range(QSPLIT):
            next(qb)
        kvps = []
        for a in (3, 2, 1, 0):
            gg = jnp.concatenate(blk[a], axis=1).astype(bf16)
            wv_u = pltpu.bitcast(wv_buf[j, :, a * 128:(a + 1) * 128], u32)
            kv = jnp.where(hm, mm(gg, wv_u, 256), 0.0)
            tscr2.at[a][...] = _pack(kv)
            kvps.append(_unpack(jnp.concatenate(
                [tscr2[a, pl.ds(jj, 8, stride=8), :] for jj in range(8)], axis=0)))

        ms_j = ms.at[:, pl.ds(_mo(j * 32, 32), 96), :]

        def m_form():
            for a in (3, 2, 1, 0):
                need(("mg", a))
                for jl in range(2):
                    for ct in range(2):
                        def put(k1, k2, v):
                            ms_j.at[k1 * 7 + k2][jl * 64 + a * 8:jl * 64 + (a + 1) * 8,
                                                 ct * 128:(ct + 1) * 128] = v
                        yield from form_steps(
                            _rform, _wr, lambda q, u: mg_buf[a, (2 * q + jl) * 16:(2 * q + jl + 1) * 16, _st(u, ct)], put)

        for i, a in enumerate((3, 2, 1, 0)):
            wo_u = pltpu.bitcast(wo_buf[j, a * 128:(a + 1) * 128, :], u32)
            res = mm(kvps[i], wo_u, 256)
            mg_buf.at[a][...] = _to_st(res)
            made.add(("mg", a))
            if i == 0:
                add_side(lambda tok: m_form(), 112, *MF)
        for _ in qb:
            pass

    def out_part(base, span, off, nr, y, src):
        b = _mo(base, 32)
        sa_v, sb_v, out_v = [r.at[pl.ds(b, 3 * HQ + span), :] for r in (sa, sb, out_buf)]
        x_v = x_buf.at[:, pl.ds(b, span), :]
        row = lax.broadcasted_iota(i32, (nr, 256), 0) + (base + off)
        blk = yield from strassen2(lambda k1, k2: _unpack(src[k1 * 7 + k2, off // 2:(off + nr) // 2, :]),
                                   lambda k1, k2: ms[k1 * 7 + k2], nr)
        for s1 in (2, 1, 3, 0):
            for s2 in range(4):
                q = (s1 // 2) * 2 + s2 // 2
                u = (s1 % 2) * 2 + s2 % 2
                rr, cc = pl.ds(q * HQ + off, nr), pl.ds(u * 256, 256)
                a = jnp.concatenate([sa_v[rr, :]] * 2, axis=1)
                c = jnp.concatenate([sb_v[rr, :]] * 2, axis=1)
                o = blk[q][u] + jnp.where(row + q * HQ == idx_s[0], y[:, u * 256:(u + 1) * 256], 0.0)
                out_v[rr, cc] = (x_v[q, off:off + nr, cc].astype(f32) * a - c + o).astype(bf16)
                if s2 % 2 == 1:
                    ch = pl.ds((s1 % 2) * HD, HD)
                    ro = pl.ds(_mo(base + q * HQ + off, 16), nr)
                    cp(out_buf.at[ro, ch], out_hbm.at[0, ro, ch], SEM_O).start()

    def ffn_part(j):
        def fma(acc, w, v):
            p = w.astype(f32) * v
            return acc + p[0:8] + p[8:16]

        for f0 in range(0, FH, 256):
            fs = slice(f0, f0 + 256)
            ag = jnp.zeros((8, 256), f32)
            au = jnp.zeros((8, 256), f32)
            for k in range(0, D, 16):
                xv = jnp.concatenate([gate16(xb[k:k + 16, :])] * 2, axis=1)
                ag = fma(ag, wg_buf[j, k:k + 16, fs], xv)
                au = fma(au, wu_buf[j, k:k + 16, fs], xv)
                yield
            g = _rbf(jnp.sum(ag, axis=0, keepdims=True))
            u = _rbf(jnp.sum(au, axis=0, keepdims=True))
            h = _rbf(_rbf(g * jax.nn.sigmoid(g)) * u)
            hb_buf[fs, :] = jnp.broadcast_to(h, (128, 256)).T
        for d0 in range(0, D, 512):
            ds_ = slice(d0, d0 + 512)
            acc = yacc[:, ds_]
            for k in range(0, FH, 16):
                hv = jnp.concatenate([gate16(hb_buf[k:k + 16, :])] * 4, axis=1)
                acc = fma(acc, wd_buf[j, k:k + 16, ds_], hv)
                yield
            yacc[:, ds_] = acc

    def wait_group(i):
        with _scope("a_wait%d" % i):
            for c in a_groups[i]:
                c.wait()
        made.add(("in", i - NX))

    def run_all(gen):
        for _ in gen:
            pass

    def ln_sides(plan):
        for r0, r1, t0, t1 in plan[0]:
            add_side(lambda tok, r0=r0, r1=r1: ln_stats(r0, r1 - r0, tok), (r1 - r0) // 2, t0, t1, LNLAG)
        for r0, r1, t0, t1 in plan[1]:
            add_side(lambda tok, r0=r0, r1=r1: ln_later(r0, r1 - r0, tok), 22 * (r1 - r0) // 16, t0, t1, SLAG)

    def l2_side(base, n, t0, t1):
        add_side(lambda tok: ln_later(0, n, None, "l2", base), 22 * n // 16, t0, t1)

    with _scope("p0_issue"):
        cp_wr.start()
        for grp in a_groups:
            for c in grp:
                c.start()
        for j in range(2):
            for c in cp_b(j):
                c.start()
        zacc[...] = jnp.zeros(zacc.shape, f32)
        yacc[...] = jnp.zeros(yacc.shape, f32)
        zero_buf[1] = jnp.zeros((8, 128), u32)
        cp_zero = cp(zero_buf.at[1], zero_buf.at[0], SEM_Z)
        cp_zero.start()
        cp_zero.wait()
        cp_wr.wait()
        wr8 = jnp.broadcast_to(wr_buf[0:D].reshape(1, D).astype(f32), (8, D))
        wrb[0:8, :] = wr8
        wrb[8:16, :] = _to_st(wr8)
        z0 = jnp.max(pltpu.bitcast(zero_buf[0], i32))
        ps, pq_buf, den_buf, mg_buf, hb_buf = [r.at[z0] for r in (ps_raw, pq_raw, den_raw, mg_raw, hb_raw)]
        xn_buf = mg_buf

    def main(_, carry0):
        def a01(i, carry):
            with _scope("a_wait01"):
                for c in cp_x(i * X0, X0, SEM_A + i):
                    c.wait()
            with _scope("a01"):
                for r in range(0, X0, 16):
                    run_all(ln_stats(r, 16, None, (i, X0)))
                    if r:
                        run_all(ln_later(r - 16, 16, None, "l1", (i, X0)))
                run_all(ln_later(X0 - 16, 16, None, "l1", (i, X0)))
            return carry

        lax.fori_loop(0, NX, a01, 0)
        made.update(("xn", r) for r in range(0, 64, 16))

        def a23(i, carry):
            with _scope("a_wait23"):
                for c in cp_wk(i, SEM_W + i):
                    c.wait()
            with _scope("a23"):
                wk_prep(i)
                l2_side((i, T0 // 2), T0 // 2, *L2W)
                kproj(0, T0, [i])
                finish()
            return carry

        lax.fori_loop(0, 2, a23, 0)
        wait_group(NX + 2)
        with _scope("a4"):
            wk_prep(2)
            ln_sides(L4)
            kproj(0, T0, [2])
            finish()
        wait_group(NX + 3)
        with _scope("a5"):
            wk_prep(3)
            ln_sides(L5)
            kproj(0, T0, [3])
            for r0, n in A5K:
                kproj(r0, n)
            finish()
        wait_group(NX + 4)
        with _scope("a6"):
            ln_sides(L6)
            for r0, n in A6K:
                kproj(r0, n)
            finish()
        wait_group(NX + 5)
        with _scope("a7"):
            ln_sides(L7)
            add_side(lambda tok: wq_perm(), 128, *WQ_PERM)
            add_side(lambda tok: wq_form(), 224, *WQ_FORM)
            add_side(lambda tok: route(), 17, *ROUTE)
            for r0, n in A7K:
                kproj(r0, n)
            finish()

        def b_body(j, carry):
            qa = BQ - QB
            with _scope("b_r0"):
                z_prep()
                add_side(lambda tok: ps_form(j), 7 * HQ // 16, *PSW)
                for t in range(4):
                    add_side(lambda tok, t=t: ps_flip(t), 49, *PFW[t])
                for r0 in range(0, qa, QN):
                    run_all(q_rows(j, r0, QN, pq_buf, den_buf, r0, QW))
                finish()
            with _scope("b_wait"):
                for c in cp_b(j, wait_only=True):
                    c.wait()
            with _scope("b_r1"):
                add_side(lambda tok: ffn_part(j), FH * 3 // 8, *FFW)
                qs_j = qs.at[:, pl.ds(_mo(j * (qa // 2), 16), qa // 2), :]
                add_side(lambda tok: normalise(pq_buf, den_buf, qa, qs_j), 4 + 26 * (qa // 16), *NRW)
                run_all(g_kvm(j))
                finish()
            return carry

        lax.fori_loop(0, 2, b_body, 0)

        def c_body(t, carry):
            with _scope("c_body"):
                y = _rbf(jnp.sum(yacc[...], axis=0, keepdims=True))
                y = _rbf(y * _rbf(1.0 / _rbf(1.0 + _rbf(jnp.exp(-rsel[0:1, :])))))
                j, h = t >> 1, t & 1
                na, nb = (BQ - QB) // 2, QB // 2
                hb = pl.ds(_mo(h * nb, 16), nb)
                add_side(lambda tok: normalise(pqb_buf.at[j, :, hb, :], denb_buf.at[j, :, hb, :], nb, qsb, tok),
                         4 + 26 * (nb // 16), *CNW, SLAG)
                qs_t = qs.at[:, pl.ds(_mo(t * (na // 2), 16), na // 2), :]
                for p in range(0, na, CR):
                    run_all(out_part(j * BQ + h * na, na, p, CR, y, qs_t))
                flush()
                run_all(out_part(j * BQ + BQ - QB + h * nb, nb, 0, nb, y, qsb))
                finish()
            return carry

        lax.fori_loop(0, 4, c_body, 0)
        return carry0

    lax.fori_loop(0, z0 + 1, main, 0)
    with _scope("tail"):
        cp(out_buf, out_hbm.at[0], SEM_O).wait()


@jax.jit
def pallas_parallel_sum__linear_attn_block__moe_arch_mod__prompt_kernel(
    A_x: jax.Array,
    A_wqkv: jax.Array,
    A_wo: jax.Array,
    B_x: jax.Array,
    B_w_r: jax.Array,
    B_w_gate: jax.Array,
    B_w_up: jax.Array,
    B_w_down: jax.Array,
):
    del B_x
    V = pltpu.VMEM
    scratch = [
        V((4, HQ, D), bf16),
        V((4, D, 256), bf16),
        V((2, D, 512), bf16),
        V((2, 512, D), bf16),
        V((8 * D,), bf16),
        V((2, D, FH), bf16),
        V((2, D, FH), bf16),
        V((2, FH, D), bf16),
        V((28, HQ // 2, 256), u32),
        V((28, HQ // 2, 256), u32),
        V((49, 128, 256), u32),
        V((S, 128), f32),
        V((S, 128), f32),
        V((8, D), f32),
        V((8, D), f32),
        V((2, 4, HQ, 512), f32),
        V((D, 128), f32),
        V((8, D), f32),
        V((8, D), f32),
        V((16, D), f32),
        V((4, 8, 128), u32),
        V((4, HD // 2, 7 * 128), u32),
        V((S, 256), f32),
        V((64, 64, 128), u32),
        V((1, HQ // 2, 49 * 128), u32),
        V((49, BQ - QB, 256), u32),
        V((49, 128, 256), u32),
        V((8, 64, 128), u32),
        V((4, 64, 128), u32),
        V((1, 4, BQ - QB, D), f32),
        V((1, 4, BQ - QB, 128), f32),
        V((2, 4, QB, D), f32),
        V((2, 4, QB, 128), f32),
        V((49, QB // 4, 256), u32),
        V((1, 4, 128, D), f32),
        V((1, FH, 128), f32),
        V((S, D), bf16),
        pltpu.SMEM((1,), i32),
        pltpu.SemaphoreType.DMA((4 + T0 // X0 + 6,)),
    ]
    extra = {k: True for k in ("disable_bounds_checks", "disable_semaphore_checks")
             if hasattr(pltpu.CompilerParams, k)}
    return pl.pallas_call(
        _kernel,
        out_shape=jax.ShapeDtypeStruct((1, S, D), bf16),
        in_specs=[pl.BlockSpec(memory_space=pl.ANY)] * 7,
        out_specs=pl.BlockSpec(memory_space=pl.ANY),
        scratch_shapes=scratch,
        compiler_params=pltpu.CompilerParams(vmem_limit_bytes=120 * 1024 * 1024, **extra),
    )(A_x.reshape(4, HQ, D), A_wqkv, A_wo, B_w_r, B_w_gate, B_w_up, B_w_down)
```

```python
import contextlib

import jax
import jax.numpy as jnp
from jax import lax
import jax.experimental.pallas as pl
import jax.experimental.pallas.tpu as pltpu

bf16, f32, u32, i32 = jnp.bfloat16, jnp.float32, jnp.uint32, jnp.int32

S = 2048
D = 1024
F = 3584
HD = D // 2
HQ = S // 4
BQ = HQ // 2
FH = F // 2
QB = 64
QN = 48
QSPLIT = 5
CR = 48
T0 = 96
X0 = 32
XG = (144, 176, 368)
XN = 128

SLAG = 400
LNLAG = 700
QW = (24, 10, 25, 13, 19, 9, 12)
QWB = (23, 16, 26, 10, 23, 8, 6)
L4 = ([(96, 144, 0, 1070)], [])
L5 = ([(144, 176, 340, 1770)], [(96, 128, 130, 1370), (128, 144, 1310, 1960), (144, 176, 1940, 2900)])
L6 = ([(176, 368, 20, 7430)], [(176, 224, 780, 2600), (224, 336, 2780, 7890)])
L7 = ([(368, 512, 0, 4800)], [(336, 384, 0, 2400), (384, 512, 2500, 9000)])
A5K = ((96, 32),)
A6K = ((128, 48), (176, 48), (224, 48))
A7K = ((272, 64), (336, 48), (384, 64), (448, 64))
WQ_PERM, WQ_FORM, ROUTE = (5100, 7900), (8000, 13100), (9400, 10200)
L2W, PSW, FFW, NRW, CNW = (270, 1284), (210, 7300), (0, 13100), (0, 12710), (0, 3624)
MF = (178, 3530)
PFW = ((2042, 3650), (4040, 5830), (5920, 7680), (7820, 9220))

L_ORD = (2, 3, 0, 1, 4, 5, 6)
R_ORD = (2, 0, 6, 5, 1, 4, 3)

K_SEQ = (1, 4, 0, 2, 3, 5, 6)
K_SEQ2 = (1, 3, 2, 4, 0, 5, 6)
W_SEQ = (0, 1, 5, 6, 4, 2, 3)

SCOPES = False


def _scope(name):
    return jax.named_scope(name) if SCOPES else contextlib.nullcontext()


def _mo(v, m):
    return v if isinstance(v, int) else pl.multiple_of(v, m)


def _pack(v):
    return pltpu.bitcast(v.astype(bf16), u32)


def _unpack(v):
    return pltpu.bitcast(v, bf16)


def _combine(m):
    m1, m2, m3, m4, m5, m6, m7 = m
    return m1 + m4 - m5 + m7, m3 + m5, m2 + m4, m1 - m2 + m3 + m6


def _combine2(m):
    m1, m2, m3, m4, m5, m6, m7 = m
    return (m4 - m5) + m1 + m7, m3 + m5, m2 + m4, (m3 - m2) + m1 + m6


def _lform(a11, a12, a21, a22):
    return (a11 + a22, a21 + a22, a11, a22, a11 + a12, a21 - a11, a12 - a22)


def _rform(b11, b12, b21, b22):
    return (b11 + b22, b11, b12 - b22, b21 - b11, b22, b11 + b12, b21 + b22)


def _sform(x11, x12, x21, x22):
    return (x11, x22, x11 + x22, x21 + x22, x11 + x12, x21 - x11, x12 - x22)


def _wl(a11, a12, a21, a22):
    s1 = a21 + a22
    s2 = s1 - a11
    return (a11, a12, a12 - s2, a22, s1, s2, a11 - a21)


def _wr(b11, b12, b21, b22):
    t1 = b12 - b11
    t2 = b22 - t1
    return (b11, b21, b22, t2 - b21, t1, t2, b22 - b12)


def _wc(p):
    p1, p2, p3, p4, p5, p6, p7 = p
    u2 = p1 + p6
    u3 = u2 + p7
    return p1 + p2, (u2 + p5) + p3, u3 - p4, u3 + p5


W_R = (3, 1, 0, 2, 4, 5, 6)


def _wl_swapped(a11, a12, a21, a22):
    return _wl(a12, a11, a22, a21)


def _wc_swapped(p):
    p1, p2, p3, p4, p5, p6, p7 = p
    v2 = p1 + p6
    u3 = p7 - v2
    return (p5 - v2) + p3, p1 + p2, u3 + p5, p4 - u3


class _Sym:
    def __init__(self, t):
        self.t = t

    def __add__(self, o):
        return _Sym({**self.t, **o.t})

    def __sub__(self, o):
        return _Sym({**self.t, **{k: -v for k, v in o.t.items()}})


def _st(u, ct):
    return slice((4 * ct + u) * 128, (4 * ct + u + 1) * 128)


def _to_st(v):
    return jnp.concatenate([v[:, (2 * u + ct) * 128:(2 * u + ct + 1) * 128]
                            for ct in range(2) for u in range(4)], axis=1)


def _phi(t):
    return jnp.where(t > 0, t + 1.0, jnp.exp(t)) + 1e-6


def _rbf(v):
    return v.astype(bf16).astype(f32)


def _kernel(x_hbm, wqkv_hbm, wo_hbm, wr_hbm, wg_hbm, wu_hbm, wd_hbm, out_hbm,
            x_buf, wk_buf, wv_buf, wo_buf, wr_buf, wg_buf, wu_buf, wd_buf,
            xs1, xs2, wqs, sa, sb, zacc, zp, pk_buf, xb, yacc, rsel, wrb, zero_buf,
            wks, stats, wqt, ps_raw, qs, ms, tscr, tscr2, pq_raw, den_raw, pqb_buf, denb_buf, qsb,
            mg_raw, hb_raw, out_buf, idx_s, sem):
    wq_buf = out_buf.at[pl.ds(0, D), :]

    def xs_at(k1, e, rows=None):
        r = xs1.at[k1 * 4 + (0, 1, 7, 3).index(e)] if e in (0, 1, 7, 3) else xs2.at[k1 * 4 + (2, 4, 5, 6).index(e)]
        return r if rows is None else r.at[rows, :]

    SEM_B, SEM_O, SEM_Z, SEM_A = 0, 2, 3, 4

    def cp(src, dst, s):
        return pltpu.make_async_copy(src, dst, sem.at[s])

    def cp_x(r0, n, s):
        r = pl.ds(_mo(r0, 16), n)
        return [cp(x_hbm.at[:, r, :], x_buf.at[:, r, :], s)]

    def cp_wk(c, s):
        return [cp(wqkv_hbm.at[:, pl.ds(_mo(D + c * 256, 256), 256)],
                   wk_buf.at[c], s)]

    NX = T0 // X0
    SEM_W = SEM_A + NX
    cp_wr = cp(wr_hbm, wr_buf.at[pl.ds(0, D)], SEM_Z)
    a_groups = [cp_x(i * X0, X0, SEM_A + i) for i in range(NX)] + [
        cp_wk(0, SEM_W),
        cp_wk(1, SEM_W + 1),
        cp_wk(2, SEM_W + 2) + cp_x(T0, XG[0] - T0, SEM_W + 2),
        cp_wk(3, SEM_W + 3) + cp_x(XG[0], XG[1] - XG[0], SEM_W + 3),
        cp_x(XG[1], XG[2] - XG[1], SEM_W + 4),
        (cp_x(XG[2], HQ - XG[2], SEM_W + 5) if XG[2] < HQ else [])
        + [cp(wqkv_hbm.at[:, pl.ds(0, D)], wq_buf, SEM_W + 5)],
    ]

    def cp_b(j, wait_only=False):
        dsts = [r.at[j] for r in (wg_buf, wu_buf, wd_buf, wv_buf, wo_buf)]
        if wait_only:
            return [cp(dst, dst, SEM_B + j) for dst in dsts]
        fs = pl.ds(j * FH, FH)
        srcs = [wg_hbm.at[:, fs], wu_hbm.at[:, fs], wd_hbm.at[fs, :],
                wqkv_hbm.at[:, pl.ds(2 * D + j * HD, HD)], wo_hbm.at[pl.ds(j * HD, HD), :]]
        return [cp(src, dst, SEM_B + j) for src, dst in zip(srcs, dsts)]

    clock = [0]
    toks = []
    sides = []
    fwd = [None]

    def emit_tok(vals, stamp):
        t = None
        for v in vals:
            v = pltpu.bitcast(v, u32) if v.dtype != u32 else v
            t = v if t is None else t | v
        toks.append((stamp, t & zero_buf[0]))

    def token(kind):
        t = fwd[0]
        if "u" not in t:
            t["u"] = pltpu.bitcast(t["src"](), u32) & zero_buf[0]
        if kind != "u" and "f" not in t:
            t["f"] = pltpu.bitcast(t["u"], f32)
        if kind == "f16" and "f16" not in t:
            t["f16"] = jnp.concatenate([t["f"], t["f"]], axis=0)
        return t[kind]

    def gate(v):
        if fwd[0] is None:
            return v
        head = v if v.shape[0] == 8 else v[0:8]
        head = head | token("u") if v.dtype == u32 else head + token("f")
        return head if v.shape[0] == 8 else jnp.concatenate([head, v[8:]], axis=0)

    def gate16(v):
        return v if fwd[0] is None else v + token("f16")

    def add_side(gen_fn, n, t0, t1, lag=None):
        st = {"i": 0, "n": n, "t0": clock[0] + t0, "t1": clock[0] + t1}

        def tok(vals):
            if lag is not None:
                emit_tok(vals, st["t0"] + (st["i"] + 1) * (st["t1"] - st["t0"]) // st["n"] + lag)
        st["g"] = gen_fn(tok)
        sides.append(st)

    def advance(until):
        for st in sides:
            while st["i"] < st["n"] and st["t0"] + st["i"] * (st["t1"] - st["t0"]) // st["n"] < until:
                next(st["g"], None)
                st["i"] += 1
                if st["i"] == st["n"]:
                    for _ in st["g"]:
                        pass

    def flush():
        for st in sides:
            for _ in st["g"]:
                pass
        sides.clear()

    def finish():
        flush()
        toks.clear()
        fwd[0] = None

    def mm(lhs, rhs, cycles, nseg=1):
        due = [t for (c, t) in toks if c <= clock[0]]
        toks[:] = [(c, t) for (c, t) in toks if c > clock[0]]
        if due:
            head = rhs[0:8, 0:128]
            for t in due:
                head = head | t
            if rhs.shape[1] > 128:
                head = jnp.concatenate([head, rhs[0:8, 128:]], axis=1)
            rhs = jnp.concatenate([head, rhs[8:]], axis=0)
        res = jnp.dot(lhs, _unpack(rhs), preferred_element_type=f32)
        ngr = res.shape[0] // 16
        for sg in range(nseg):
            for i in range(ngr):
                fwd[0] = {"src": lambda sg=sg, i=i: res[i * 16:i * 16 + 8, sg * 128:(sg + 1) * 128]}
                clock[0] += cycles // nseg // ngr
                advance(clock[0])
        return res

    def form_steps(form, form2, get, put, tok=None, keep=range(7)):
        terms = form(*[_Sym({i: 1}) for i in range(4)])
        gated = (0, 1, 2, 3) if 7 in keep else {_wl: (0, 1, 3), _wr: (0, 2, 3), _wl_swapped: (1, 2)}[form2]
        for k1 in range(7):
            sub = []
            for r in range(2):
                for c in range(2):
                    v = None
                    for i, sg in sorted(terms[k1].t.items(), key=lambda e: -e[1]):
                        b = get(r + 2 * (i // 2), c + 2 * (i % 2))
                        if v is None:
                            v = gate16(b) if 2 * r + c in gated else b
                        else:
                            v = v + b if sg > 0 else v - b
                    sub.append(v)
            vals = form2(*sub) + (sub[2],)
            for k2 in keep:
                put(k1, k2, _pack(vals[k2]))
            if tok is not None and k1 % 2 == 0:
                full = vals[3 if form2 is _wr else 2]
                tok([full[0:8], full[8:16]])
            yield

    def strassen2(lhs, rhs, cycles, nseg=1, wts=(16,) * 7, comb=_wc):
        m1 = [None] * 7
        for i1, k1 in enumerate(K_SEQ2):
            m2 = [None] * 7
            for k2 in W_SEQ:
                m2[k2] = mm(lhs(k1, k2), rhs(k1, k2), cycles * wts[i1] // 16, nseg)
                yield
            m1[k1] = comb(m2)
        out = [[None] * 4 for _ in range(4)]
        for s2 in range(4):
            for s1, v in enumerate(_combine2([m1[k1][s2] for k1 in range(7)])):
                out[(s1 // 2) * 2 + s2 // 2][(s1 % 2) * 2 + s2 % 2] = v
        return out

    made = set()

    def need(*keys):
        assert all(k in made for k in keys), keys

    def row_views(base):
        if base == 0:
            return x_buf, sa, sb, stats, xn_buf, None
        i, n = base
        b = _mo(i * n, 16)
        return ([x_buf.at[:, pl.ds(b, n), :]] + [r.at[pl.ds(b, S - 128 + n), :] for r in (sa, sb, stats)]
                + [xn_buf.at[:, pl.ds(b, n), :], pl.ds(_mo(i * (n // 2), 8), n // 2)])

    def xs_form(r0, tok, which="all", base=0):
        xn_v, xs_v = row_views(base)[4:]
        rows = slice(r0 % XN, r0 % XN + 16)

        keep = {"all": range(8), "l1": (0, 1, 7, 3), "l2": (2, 4, 5, 6)}[which]
        for ct in range(2):
            def put(k1, k2, v):
                xs_at(k1, k2, xs_v)[r0 // 2:r0 // 2 + 8, ct * 128:(ct + 1) * 128] = v
            yield from form_steps(
                _sform, _wl, lambda q, u: xn_v[q, rows, _st(u, ct)], put, tok, keep)
        made.add(("xs", r0))

    def ln_stats(r_start, n_rows, tok, base=0):
        x_v, sa_v, sb_v, st_v, xn_v, _ = row_views(base)
        lane = lax.broadcasted_iota(i32, (8, 128), 1)
        for r0 in range(r_start, r_start + n_rows, 16):
            if r0 >= T0:
                need(("in", 2 + sum(r0 >= g for g in XG)))
            if r0 - XN >= T0:
                need(("ln", r0 - XN))
            for g in range(8):
                q, o = g // 2, (g % 2) * 8
                rg = q * HQ + r0 + o
                xv = x_v[q, r0 + o:r0 + o + 8, :].astype(f32)
                xg = jnp.concatenate([gate(xv[:, 0:128]), xv[:, 128:]], axis=1)
                mf = jnp.sum(xg, axis=1, keepdims=True) * (1.0 / D)
                d = xv - mf
                var = jnp.sum(d * d, axis=1, keepdims=True) * (1.0 / D)
                rs = lax.rsqrt(var + 1e-5)
                xn_v.at[q][r0 % XN + o:r0 % XN + o + 8, :] = _to_st(d * rs)
                rs = jnp.broadcast_to(rs, (8, 128))
                mf = jnp.broadcast_to(mf, (8, 128))
                sa_v[rg:rg + 8, :] = 1.0 + rs
                sb_v[rg:rg + 8, :] = mf * rs
                st_v[rg:rg + 8, 0:128] = jnp.where(lane == 0, mf, jnp.broadcast_to(var, (8, 128)))
                if tok is not None:
                    tok([rs])
                if g == 7:
                    made.add(("xn", r0))
                yield

    def ln_later(r_start, n_rows, tok, which="all", base=0):
        st_v, xn_v = row_views(base)[3:5]
        for r0 in range(r_start, r_start + n_rows, 16):
            need(("xn", r0))
            form = xs_form(r0, tok, which, base)
            for g in range(8):
                for _ in range(2 if g < 7 else 0):
                    next(form)
                    yield
                q, o = g // 2, (g % 2) * 8
                t = None
                if which != "l1":
                    v = xn_v[q, r0 % XN + o:r0 % XN + o + 8, :] * wrb[8:16, :]
                    for ct in range(8):
                        h = v[:, ct * 128:(ct + 1) * 128]
                        t = gate(h) if t is None else t + h
                if t is not None:
                    st_v[q * HQ + r0 + o:q * HQ + r0 + o + 8, 128:256] = t
                if tok is not None:
                    tok([t])
                if g == 7:
                    next(form, None)
                    made.add(("ln", r0))
                yield

    def wk_prep(c):
        if isinstance(c, int):
            need(("in", c))
        wks.at[c][:, 128:256] = pltpu.bitcast(wk_buf[c, 0:HD, 0:128], u32)
        wks.at[c][:, 512:640] = pltpu.bitcast(wk_buf[c, HD:D, 128:256], u32)
        for i in range(HD // 16):
            r0 = i * 16
            top = wk_buf[c, r0:r0 + 16, :].astype(f32)
            bot = wk_buf[c, HD + r0:HD + r0 + 16, :].astype(f32)
            ops = _rform(top[:, :128], top[:, 128:], bot[:, :128], bot[:, 128:])
            for k in (0, 2, 3, 5, 6):
                wks.at[c][r0 // 2:r0 // 2 + 8, k * 128:(k + 1) * 128] = _pack(ops[k])

    def wq_perm():
        need(("in", 5))

        def permute(kt):
            for g in range(8):
                tile = gate(pltpu.bitcast(wq_buf[kt * 128:(kt + 1) * 128, g * 128:(g + 1) * 128], u32))
                wqt.at[kt * 8 + g][...] = pltpu.bitcast(_unpack(tile).T, u32)
                yield

        def back(kt):
            for j in range(8):
                tile = gate(jnp.concatenate([wqt[kt * 8 + g, pl.ds(j, 8, stride=8), :] for g in range(8)],
                                            axis=0))
                v = pltpu.bitcast(_unpack(tile).T.astype(f32), u32)
                c0 = (kt // 2) * D + _st(j // 2, j % 2).start
                ps[(kt % 2) * 128:(kt % 2 + 1) * 128, c0:c0 + 128] = v
                made.add(("wqp", kt, j))
                yield

        order = (0, 2, 4, 6, 1, 3, 5, 7)
        for n in range(10):
            if n < 8:
                yield from permute(order[n])
            if n > 1:
                yield from back(order[n - 2])

    def wq_form():
        for i in range(16):
            need(*[("wqp", 2 * r + i // 8, j) for r in range(4) for j in range(8)])
            for ct in range(2):
                def put(k1, k2, v):
                    wqs.at[k1 * 7 + k2][i * 8:(i + 1) * 8, ct * 128:(ct + 1) * 128] = v
                yield from form_steps(
                    _rform, _wr, lambda r, c: pltpu.bitcast(
                        ps[i * 16:(i + 1) * 16, r * D + _st(c, ct).start:r * D + _st(c, ct).stop],
                        f32), put)

    def kproj(r0, n, chunks=range(4)):
        pr = pl.ds(r0 // 2, n // 2)
        need(*[("xs", r) for r in range(max(r0, T0), r0 + n, 16)])
        for c in chunks:
            m = [None] * 7
            for k in K_SEQ:
                e11, e12, e21, e22 = [xs_at(L_ORD[k], e)[pr, :] for e in (0, 1, 7, 3)]
                lhs = jnp.concatenate([jnp.concatenate([e11, e12], axis=1),
                                       jnp.concatenate([e21, e22], axis=1)], axis=0)
                m[k] = mm(_unpack(lhs), wks[c, :, k * 128:(k + 1) * 128], 2 * n)
            kk = [_phi(v) for v in _combine(m)]
            for ct in range(2):
                zacc[:, pl.ds(_mo(c * 256 + ct * 128, 128), 128)] += (
                    (kk[ct] + kk[2 + ct]).reshape(n // 4, 8, 128).sum(axis=0))
            j, c2 = (c // 2, c % 2) if isinstance(c, int) else (0, c)
            pk_v = pk_buf.at[j, :, :, pl.ds(_mo(c2 * 256, 256), 256)]
            for s1 in range(4):
                for h in range(2):
                    pk_v.at[(s1 // 2) * 2 + h][r0:r0 + n, (s1 % 2) * 128:(s1 % 2 + 1) * 128] = (
                        kk[s1][h * n:(h + 1) * n])

    def z_prep():
        z = jnp.sum(zacc[...], axis=0, keepdims=True)
        zt = _pack(jnp.broadcast_to(z, (128, D)).astype(bf16).T)
        for g in range(8):
            tscr.at[g][...] = zt[g * 64:(g + 1) * 64, :]
        for j in range(8):
            blk = jnp.concatenate([tscr[g, pl.ds(j, 8, stride=8), :] for g in range(8)], axis=0)
            zp[:, j * 128:(j + 1) * 128] = _unpack(blk).T[0:8, :].astype(f32)

    def route():
        rows, dots = [None] * 16, [None] * 16
        for b in sorted(range(S // 128), key=lambda b: b % 4):
            need(*[("ln", r) for r in range(max(T0, b % 4 * 128), b % 4 * 128 + 128, 16)])
            rows[b] = gate(stats[b * 128:(b + 1) * 128, 0:128]).T[0:8, :]
            dots[b] = jnp.sum(gate(stats[b * 128:(b + 1) * 128, 128:256]).T, axis=0, keepdims=True)
            yield
        mf = jnp.concatenate([v[0:1] for v in rows], axis=0)
        var = jnp.concatenate([v[1:2] for v in rows], axis=0)
        tr = jnp.concatenate(dots, axis=0) * jnp.sqrt(var + 1e-5)
        wsum = jnp.sum(wrb[0:1, :], axis=1, keepdims=True)
        mb = _rbf(mf)
        inv = 1.0 / _rbf(jnp.sqrt(_rbf(_rbf(var) + 1e-5)))
        rv = _rbf((tr + (mf - mb) * wsum) * inv)
        rmax = jnp.max(jnp.max(rv, axis=1, keepdims=True), axis=0, keepdims=True)
        pos = (lax.broadcasted_iota(i32, rv.shape, 0) * 128 + lax.broadcasted_iota(i32, rv.shape, 1))
        idx = jnp.min(jnp.where(rv == rmax, pos, S - 1))
        idx_s[0] = idx

        def pick(v):
            v = jnp.sum(jnp.where(pos == idx, v, 0.0), axis=1, keepdims=True)
            return jnp.sum(v, axis=0, keepdims=True)

        xv = x_buf[(idx >> 9) & 3, pl.ds(_mo(idx & (HQ - 16), 16), 16), :].astype(f32)
        sel = lax.broadcasted_iota(i32, xv.shape, 0) == (idx & 15)
        row = jnp.sum(jnp.where(sel, xv, 0.0), axis=0, keepdims=True)
        row = _rbf(_rbf(row - pick(mb)) * pick(inv))
        rsel[...] = jnp.broadcast_to(_rbf(jnp.sum(row * wrb[0:1, :], axis=1, keepdims=True)), rsel.shape)
        xb[...] = jnp.broadcast_to(row, (128, D)).T
        yield

    def ps_form(j):
        for c in range(HQ // 16):
            def put(k1, k2, v):
                k = k1 * 7 + k2
                ps[c * 8:(c + 1) * 8, k * 128:(k + 1) * 128] = v
            yield from form_steps(
                _lform, _wl_swapped,
                lambda r, q: pk_buf[j, q, c * 16:(c + 1) * 16, r * 128:(r + 1) * 128], put)
            made.add(("ps", c))

    def ps_flip(t):
        need(*[("ps", c) for c in range(8 * t, 8 * t + 8)])
        for k in range(49):
            at = (slice(t * 64, (t + 1) * 64), slice(k * 128, (k + 1) * 128))
            ps[at] = pltpu.bitcast(_unpack(gate(ps[at])).T, u32)
            yield

    def q_rows(j, r0, n, pq, rc, d0, wts):
        xj = pl.ds(_mo(j * (BQ // 2), BQ // 2), BQ // 2)
        pr = slice(r0 // 2, (r0 + n) // 2)
        blk = yield from strassen2(lambda k1, k2: _unpack(xs_at(L_ORD[k1], k2, xj)[pr, :]),
                                   lambda k1, k2: wqs[k1 * 7 + k2], n, 1, wts)
        for q in range(4):
            d = None
            for u in ((0, 1, 2, 3) if q >= 2 else (3, 2, 1, 0)):
                v = _phi(blk[q][u])
                for ct in range(2):
                    pq.at[q][d0:d0 + n, _st(u, ct)] = v[:, ct * 128:(ct + 1) * 128]
                t = v * zp[0:1, u * 256:(u + 1) * 256]
                t = t[:, :128] + t[:, 128:]
                d = t if d is None else d + t
            rc.at[q][d0:d0 + n, :] = d

    def normalise(pq, rc, nr, dst, tok=None):
        lane = lax.broadcasted_iota(i32, (16, 128), 1)
        nc = nr // 16

        def recips(c):
            rq = slice(c * 16, (c + 1) * 16)
            for q in range(4):
                d = gate16(rc[q, rq, :])
                d = d + jnp.where(lane % 2 == 0, pltpu.roll(d, 127, 1), pltpu.roll(d, 1, 1))
                d = d + jnp.where(lane % 4 < 2, pltpu.roll(d, 126, 1), pltpu.roll(d, 2, 1))
                rc.at[q][rq, :] = 1.0 / (d + 1e-6)
                yield

        def scale(c):
            rq = slice(c * 16, (c + 1) * 16)
            for hf in range(2):
                for q in range(4):
                    cs = slice(hf * HD, (hf + 1) * HD)
                    pq.at[q][rq, cs] = pq[q, rq, cs] * jnp.concatenate([gate16(rc[q, rq, :])] * 4, axis=1)
                    yield

        def form(c):
            rq = slice(c * 16, (c + 1) * 16)
            for ct in range(2):
                def put(k1, k2, v):
                    dst.at[k1 * 7 + k2][c * 8:(c + 1) * 8, ct * 128:(ct + 1) * 128] = v
                yield from form_steps(_lform, _wl, lambda q, u: pq[q, rq, _st(u, ct)], put, tok)

        def ahead(c):
            if c + 2 < nc:
                yield from recips(c + 2)
            if c + 1 < nc:
                yield from scale(c + 1)

        yield from recips(0)
        yield from recips(1)
        for _ in range(4):
            yield
        yield from scale(0)
        for c in range(nc):
            nxt = ahead(c)
            for _ in form(c):
                yield
                if next(nxt, 0) is None:
                    yield

    def g_kvm(j):
        qb = q_rows(j, BQ - QB, QB, pqb_buf.at[j], denb_buf.at[j], 0, QWB)
        blk = yield from strassen2(
            lambda k1, k2: _unpack(jnp.concatenate(
                [ps[t * 64:(t + 1) * 64, (k1 * 7 + k2) * 128:(k1 * 7 + k2 + 1) * 128] for t in range(4)], axis=1)),
            lambda k1, k2: xs_at(R_ORD[k1], W_R[k2])[...], 256, 2, comb=_wc_swapped)
        hm = (lax.broadcasted_iota(i32, (128, 128), 0) // 32
              == lax.broadcasted_iota(i32, (128, 128), 1) // 32)
        for _ in range(QSPLIT):
            next(qb)
        kvps = []
        for a in (3, 2, 1, 0):
            gg = jnp.concatenate(blk[a], axis=1).astype(bf16)
            wv_u = pltpu.bitcast(wv_buf[j, :, a * 128:(a + 1) * 128], u32)
            kv = jnp.where(hm, mm(gg, wv_u, 256), 0.0)
            tscr2.at[a][...] = _pack(kv)
            kvps.append(_unpack(jnp.concatenate(
                [tscr2[a, pl.ds(jj, 8, stride=8), :] for jj in range(8)], axis=0)))

        ms_j = ms.at[:, pl.ds(_mo(j * 32, 32), 96), :]

        def m_form():
            for a in (3, 2, 1, 0):
                need(("mg", a))
                for jl in range(2):
                    for ct in range(2):
                        def put(k1, k2, v):
                            ms_j.at[k1 * 7 + k2][jl * 64 + a * 8:jl * 64 + (a + 1) * 8,
                                                 ct * 128:(ct + 1) * 128] = v
                        yield from form_steps(
                            _rform, _wr, lambda q, u: mg_buf[a, (2 * q + jl) * 16:(2 * q + jl + 1) * 16, _st(u, ct)], put)

        for i, a in enumerate((3, 2, 1, 0)):
            wo_u = pltpu.bitcast(wo_buf[j, a * 128:(a + 1) * 128, :], u32)
            res = mm(kvps[i], wo_u, 256)
            mg_buf.at[a][...] = _to_st(res)
            made.add(("mg", a))
            if i == 0:
                add_side(lambda tok: m_form(), 112, *MF)
        for _ in qb:
            pass

    def out_part(base, span, off, nr, y, src):
        b = _mo(base, 32)
        sa_v, sb_v, out_v = [r.at[pl.ds(b, 3 * HQ + span), :] for r in (sa, sb, out_buf)]
        x_v = x_buf.at[:, pl.ds(b, span), :]
        row = lax.broadcasted_iota(i32, (nr, 256), 0) + (base + off)
        blk = yield from strassen2(lambda k1, k2: _unpack(src[k1 * 7 + k2, off // 2:(off + nr) // 2, :]),
                                   lambda k1, k2: ms[k1 * 7 + k2], nr)
        for s1 in (2, 1, 3, 0):
            for s2 in range(4):
                q = (s1 // 2) * 2 + s2 // 2
                u = (s1 % 2) * 2 + s2 % 2
                rr, cc = pl.ds(q * HQ + off, nr), pl.ds(u * 256, 256)
                a = jnp.concatenate([sa_v[rr, :]] * 2, axis=1)
                c = jnp.concatenate([sb_v[rr, :]] * 2, axis=1)
                o = blk[q][u] + jnp.where(row + q * HQ == idx_s[0], y[:, u * 256:(u + 1) * 256], 0.0)
                out_v[rr, cc] = (x_v[q, off:off + nr, cc].astype(f32) * a - c + o).astype(bf16)
                if s2 % 2 == 1:
                    ch = pl.ds((s1 % 2) * HD, HD)
                    ro = pl.ds(_mo(base + q * HQ + off, 16), nr)
                    cp(out_buf.at[ro, ch], out_hbm.at[0, ro, ch], SEM_O).start()

    def ffn_part(j):
        def fma(acc, w, v):
            p = w.astype(f32) * v
            return acc + p[0:8] + p[8:16]

        for f0 in range(0, FH, 256):
            fs = slice(f0, f0 + 256)
            ag = jnp.zeros((8, 256), f32)
            au = jnp.zeros((8, 256), f32)
            for k in range(0, D, 16):
                xv = jnp.concatenate([gate16(xb[k:k + 16, :])] * 2, axis=1)
                ag = fma(ag, wg_buf[j, k:k + 16, fs], xv)
                au = fma(au, wu_buf[j, k:k + 16, fs], xv)
                yield
            g = _rbf(jnp.sum(ag, axis=0, keepdims=True))
            u = _rbf(jnp.sum(au, axis=0, keepdims=True))
            h = _rbf(_rbf(g * jax.nn.sigmoid(g)) * u)
            hb_buf[fs, :] = jnp.broadcast_to(h, (128, 256)).T
        for d0 in range(0, D, 512):
            ds_ = slice(d0, d0 + 512)
            acc = yacc[:, ds_]
            for k in range(0, FH, 16):
                hv = jnp.concatenate([gate16(hb_buf[k:k + 16, :])] * 4, axis=1)
                acc = fma(acc, wd_buf[j, k:k + 16, ds_], hv)
                yield
            yacc[:, ds_] = acc

    def wait_group(i):
        with _scope("a_wait%d" % i):
            for c in a_groups[i]:
                c.wait()
        made.add(("in", i - NX))

    def run_all(gen):
        for _ in gen:
            pass

    def ln_sides(plan):
        for r0, r1, t0, t1 in plan[0]:
            add_side(lambda tok, r0=r0, r1=r1: ln_stats(r0, r1 - r0, tok), (r1 - r0) // 2, t0, t1, LNLAG)
        for r0, r1, t0, t1 in plan[1]:
            add_side(lambda tok, r0=r0, r1=r1: ln_later(r0, r1 - r0, tok), 22 * (r1 - r0) // 16, t0, t1, SLAG)

    def l2_side(base, n, t0, t1):
        add_side(lambda tok: ln_later(0, n, None, "l2", base), 22 * n // 16, t0, t1)

    with _scope("p0_issue"):
        cp_wr.start()
        for grp in a_groups:
            for c in grp:
                c.start()
        for j in range(2):
            for c in cp_b(j):
                c.start()
        zacc[...] = jnp.zeros(zacc.shape, f32)
        yacc[...] = jnp.zeros(yacc.shape, f32)
        zero_buf[1] = jnp.zeros((8, 128), u32)
        cp_zero = cp(zero_buf.at[1], zero_buf.at[0], SEM_Z)
        cp_zero.start()
        cp_zero.wait()
        cp_wr.wait()
        wr8 = jnp.broadcast_to(wr_buf[0:D].reshape(1, D).astype(f32), (8, D))
        wrb[0:8, :] = wr8
        wrb[8:16, :] = _to_st(wr8)
        z0 = jnp.max(pltpu.bitcast(zero_buf[0], i32))
        ps, pq_buf, den_buf, mg_buf, hb_buf = [r.at[z0] for r in (ps_raw, pq_raw, den_raw, mg_raw, hb_raw)]
        xn_buf = mg_buf

    def main(_, carry0):
        def a01(i, carry):
            with _scope("a_wait01"):
                for c in cp_x(i * X0, X0, SEM_A + i):
                    c.wait()
            with _scope("a01"):
                for r in range(0, X0, 16):
                    run_all(ln_stats(r, 16, None, (i, X0)))
                    if r:
                        run_all(ln_later(r - 16, 16, None, "l1", (i, X0)))
                run_all(ln_later(X0 - 16, 16, None, "l1", (i, X0)))
            return carry

        lax.fori_loop(0, NX, a01, 0)
        made.update(("xn", r) for r in range(0, 64, 16))

        def a23(i, carry):
            with _scope("a_wait23"):
                for c in cp_wk(i, SEM_W + i):
                    c.wait()
            with _scope("a23"):
                wk_prep(i)
                l2_side((i, T0 // 2), T0 // 2, *L2W)
                kproj(0, T0, [i])
                finish()
            return carry

        lax.fori_loop(0, 2, a23, 0)
        wait_group(NX + 2)
        with _scope("a4"):
            wk_prep(2)
            ln_sides(L4)
            kproj(0, T0, [2])
            finish()
        wait_group(NX + 3)
        with _scope("a5"):
            wk_prep(3)
            ln_sides(L5)
            kproj(0, T0, [3])
            for r0, n in A5K:
                kproj(r0, n)
            finish()
        wait_group(NX + 4)
        with _scope("a6"):
            ln_sides(L6)
            for r0, n in A6K:
                kproj(r0, n)
            finish()
        wait_group(NX + 5)
        with _scope("a7"):
            ln_sides(L7)
            add_side(lambda tok: wq_perm(), 128, *WQ_PERM)
            add_side(lambda tok: wq_form(), 224, *WQ_FORM)
            add_side(lambda tok: route(), 17, *ROUTE)
            for r0, n in A7K:
                kproj(r0, n)
            finish()

        def b_body(j, carry):
            qa = BQ - QB
            with _scope("b_r0"):
                z_prep()
                add_side(lambda tok: ps_form(j), 7 * HQ // 16, *PSW)
                for t in range(4):
                    add_side(lambda tok, t=t: ps_flip(t), 49, *PFW[t])
                for r0 in range(0, qa, QN):
                    run_all(q_rows(j, r0, QN, pq_buf, den_buf, r0, QW))
                finish()
            with _scope("b_wait"):
                for c in cp_b(j, wait_only=True):
                    c.wait()
            with _scope("b_r1"):
                add_side(lambda tok: ffn_part(j), FH * 3 // 8, *FFW)
                qs_j = qs.at[:, pl.ds(_mo(j * (qa // 2), 16), qa // 2), :]
                add_side(lambda tok: normalise(pq_buf, den_buf, qa, qs_j), 4 + 26 * (qa // 16), *NRW)
                run_all(g_kvm(j))
                finish()
            return carry

        lax.fori_loop(0, 2, b_body, 0)

        def c_body(t, carry):
            with _scope("c_body"):
                y = _rbf(jnp.sum(yacc[...], axis=0, keepdims=True))
                y = _rbf(y * _rbf(1.0 / _rbf(1.0 + _rbf(jnp.exp(-rsel[0:1, :])))))
                j, h = t >> 1, t & 1
                na, nb = (BQ - QB) // 2, QB // 2
                hb = pl.ds(_mo(h * nb, 16), nb)
                add_side(lambda tok: normalise(pqb_buf.at[j, :, hb, :], denb_buf.at[j, :, hb, :], nb, qsb, tok),
                         4 + 26 * (nb // 16), *CNW, SLAG)
                qs_t = qs.at[:, pl.ds(_mo(t * (na // 2), 16), na // 2), :]
                for p in range(0, na, CR):
                    run_all(out_part(j * BQ + h * na, na, p, CR, y, qs_t))
                flush()
                run_all(out_part(j * BQ + BQ - QB + h * nb, nb, 0, nb, y, qsb))
                finish()
            return carry

        lax.fori_loop(0, 4, c_body, 0)
        return carry0

    lax.fori_loop(0, z0 + 1, main, 0)
    with _scope("tail"):
        cp(out_buf, out_hbm.at[0], SEM_O).wait()


@jax.jit
def pallas_parallel_sum__linear_attn_block__moe_arch_mod__prompt_kernel(
    A_x: jax.Array,
    A_wqkv: jax.Array,
    A_wo: jax.Array,
    B_x: jax.Array,
    B_w_r: jax.Array,
    B_w_gate: jax.Array,
    B_w_up: jax.Array,
    B_w_down: jax.Array,
):
    del B_x
    V = pltpu.VMEM
    scratch = [
        V((4, HQ, D), bf16),
        V((4, D, 256), bf16),
        V((2, D, 512), bf16),
        V((2, 512, D), bf16),
        V((8 * D,), bf16),
        V((2, D, FH), bf16),
        V((2, D, FH), bf16),
        V((2, FH, D), bf16),
        V((28, HQ // 2, 256), u32),
        V((28, HQ // 2, 256), u32),
        V((49, 128, 256), u32),
        V((S, 128), f32),
        V((S, 128), f32),
        V((8, D), f32),
        V((8, D), f32),
        V((2, 4, HQ, 512), f32),
        V((D, 128), f32),
        V((8, D), f32),
        V((8, D), f32),
        V((16, D), f32),
        V((4, 8, 128), u32),
        V((4, HD // 2, 7 * 128), u32),
        V((S, 256), f32),
        V((64, 64, 128), u32),
        V((1, HQ // 2, 49 * 128), u32),
        V((49, BQ - QB, 256), u32),
        V((49, 128, 256), u32),
        V((8, 64, 128), u32),
        V((4, 64, 128), u32),
        V((1, 4, BQ - QB, D), f32),
        V((1, 4, BQ - QB, 128), f32),
        V((2, 4, QB, D), f32),
        V((2, 4, QB, 128), f32),
        V((49, QB // 4, 256), u32),
        V((1, 4, 128, D), f32),
        V((1, FH, 128), f32),
        V((S, D), bf16),
        pltpu.SMEM((1,), i32),
        pltpu.SemaphoreType.DMA((4 + T0 // X0 + 6,)),
    ]
    extra = {k: True for k in ("disable_bounds_checks", "disable_semaphore_checks")
             if hasattr(pltpu.CompilerParams, k)}
    return pl.pallas_call(
        _kernel,
        out_shape=jax.ShapeDtypeStruct((1, S, D), bf16),
        in_specs=[pl.BlockSpec(memory_space=pl.ANY)] * 7,
        out_specs=pl.BlockSpec(memory_space=pl.ANY),
        scratch_shapes=scratch,
        compiler_params=pltpu.CompilerParams(vmem_limit_bytes=120 * 1024 * 1024, **extra),
    )(A_x.reshape(4, HQ, D), A_wqkv, A_wo, B_w_r, B_w_gate, B_w_up, B_w_down)
```

```python
import contextlib

import jax
import jax.numpy as jnp
from jax import lax
import jax.experimental.pallas as pl
import jax.experimental.pallas.tpu as pltpu

bf16, f32, u32, i32 = jnp.bfloat16, jnp.float32, jnp.uint32, jnp.int32

S = 2048
D = 1024
F = 3584
HD = D // 2
HQ = S // 4
BQ = HQ // 2
FH = F // 2
QB = 64
QN = 48
QSPLIT = 5
CR = 48
T0 = 96
X0 = 32
XG = (144, 176, 368)
XN = 128

SLAG = 400
LNLAG = 700
QW = (24, 10, 25, 13, 19, 9, 12)
KW5 = (20, 20, 20, 13, 13, 13, 13)
KW6 = (22, 22, 20, 12, 12, 12, 12)
KW7 = (16, 16, 16, 16, 16, 16, 16)
QWB = (23, 16, 26, 10, 23, 8, 6)
L4 = ([(96, 144, 0, 1070)], [])
L5 = ([(144, 176, 340, 1770)], [(96, 128, 130, 1370), (128, 144, 1310, 1960), (144, 176, 1940, 2900)])
L6 = ([(176, 368, 20, 7430)], [(176, 224, 780, 2600), (224, 336, 2780, 7890)])
L7 = ([(368, 512, 0, 4800)], [(336, 384, 0, 2400), (384, 512, 2500, 9000)])
A5K = ((96, 32),)
A6K = ((128, 48), (176, 48), (224, 48))
A7K = ((272, 64), (336, 48), (384, 64), (448, 64))
WQ_PERM, WQ_FORM, ROUTE = (5100, 7900), (8000, 13100), (9400, 10200)
L2W, PSW, FFW, NRW, CNW = (270, 1284), (210, 7300), (0, 13100), (0, 12710), (0, 3624)
MF = (178, 3530)
PFW = ((2042, 3650), (4040, 5830), (5920, 7680), (7820, 9220))

L_ORD = (2, 3, 0, 1, 4, 5, 6)
R_ORD = (2, 0, 6, 5, 1, 4, 3)

K_SEQ = (1, 4, 0, 2, 3, 5, 6)
K_SEQ2 = (1, 3, 2, 4, 0, 5, 6)
W_SEQ = (0, 1, 5, 6, 4, 2, 3)

SCOPES = False


def _scope(name):
    return jax.named_scope(name) if SCOPES else contextlib.nullcontext()


def _mo(v, m):
    return v if isinstance(v, int) else pl.multiple_of(v, m)


def _pack(v):
    return pltpu.bitcast(v.astype(bf16), u32)


def _unpack(v):
    return pltpu.bitcast(v, bf16)


def _combine(m):
    m1, m2, m3, m4, m5, m6, m7 = m
    return m1 + m4 - m5 + m7, m3 + m5, m2 + m4, m1 - m2 + m3 + m6


def _combine2(m):
    m1, m2, m3, m4, m5, m6, m7 = m
    return (m4 - m5) + m1 + m7, m3 + m5, m2 + m4, (m3 - m2) + m1 + m6


def _lform(a11, a12, a21, a22):
    return (a11 + a22, a21 + a22, a11, a22, a11 + a12, a21 - a11, a12 - a22)


def _rform(b11, b12, b21, b22):
    return (b11 + b22, b11, b12 - b22, b21 - b11, b22, b11 + b12, b21 + b22)


def _sform(x11, x12, x21, x22):
    return (x11, x22, x11 + x22, x21 + x22, x11 + x12, x21 - x11, x12 - x22)


def _wl(a11, a12, a21, a22):
    s1 = a21 + a22
    s2 = s1 - a11
    return (a11, a12, a12 - s2, a22, s1, s2, a11 - a21)


def _wr(b11, b12, b21, b22):
    t1 = b12 - b11
    t2 = b22 - t1
    return (b11, b21, b22, t2 - b21, t1, t2, b22 - b12)


def _wc(p):
    p1, p2, p3, p4, p5, p6, p7 = p
    u2 = p1 + p6
    u3 = u2 + p7
    return p1 + p2, (u2 + p5) + p3, u3 - p4, u3 + p5


W_R = (3, 1, 0, 2, 4, 5, 6)


def _wl_swapped(a11, a12, a21, a22):
    return _wl(a12, a11, a22, a21)


def _wc_swapped(p):
    p1, p2, p3, p4, p5, p6, p7 = p
    v2 = p1 + p6
    u3 = p7 - v2
    return (p5 - v2) + p3, p1 + p2, u3 + p5, p4 - u3


class _Sym:
    def __init__(self, t):
        self.t = t

    def __add__(self, o):
        return _Sym({**self.t, **o.t})

    def __sub__(self, o):
        return _Sym({**self.t, **{k: -v for k, v in o.t.items()}})


def _st(u, ct):
    return slice((4 * ct + u) * 128, (4 * ct + u + 1) * 128)


def _to_st(v):
    return jnp.concatenate([v[:, (2 * u + ct) * 128:(2 * u + ct + 1) * 128]
                            for ct in range(2) for u in range(4)], axis=1)


def _phi(t):
    return jnp.where(t > 0, t + 1.0, jnp.exp(t)) + 1e-6


def _rbf(v):
    return v.astype(bf16).astype(f32)


def _kernel(x_hbm, wqkv_hbm, wo_hbm, wr_hbm, wg_hbm, wu_hbm, wd_hbm, out_hbm,
            x_buf, wk_buf, wv_buf, wo_buf, wr_buf, wg_buf, wu_buf, wd_buf,
            xs1, xs2, wqs, sa, sb, zacc, zp, pk_buf, xb, yacc, rsel, wrb, zero_buf,
            wks, stats, wqt, ps_raw, qs, ms, tscr, tscr2, pq_raw, den_raw, pqb_buf, denb_buf, qsb,
            mg_raw, hb_raw, out_buf, idx_s, sem):
    wq_buf = out_buf.at[pl.ds(0, D), :]

    def xs_at(k1, e, rows=None):
        r = xs1.at[k1 * 4 + (0, 1, 7, 3).index(e)] if e in (0, 1, 7, 3) else xs2.at[k1 * 4 + (2, 4, 5, 6).index(e)]
        return r if rows is None else r.at[rows, :]

    SEM_B, SEM_O, SEM_Z, SEM_A = 0, 2, 3, 4

    def cp(src, dst, s):
        return pltpu.make_async_copy(src, dst, sem.at[s])

    def cp_x(r0, n, s):
        r = pl.ds(_mo(r0, 16), n)
        return [cp(x_hbm.at[:, r, :], x_buf.at[:, r, :], s)]

    def cp_wk(c, s):
        return [cp(wqkv_hbm.at[:, pl.ds(_mo(D + c * 256, 256), 256)],
                   wk_buf.at[c], s)]

    NX = T0 // X0
    SEM_W = SEM_A + NX
    cp_wr = cp(wr_hbm, wr_buf.at[pl.ds(0, D)], SEM_Z)
    a_groups = [cp_x(i * X0, X0, SEM_A + i) for i in range(NX)] + [
        cp_wk(0, SEM_W),
        cp_wk(1, SEM_W + 1),
        cp_wk(2, SEM_W + 2) + cp_x(T0, XG[0] - T0, SEM_W + 2),
        cp_wk(3, SEM_W + 3) + cp_x(XG[0], XG[1] - XG[0], SEM_W + 3),
        cp_x(XG[1], XG[2] - XG[1], SEM_W + 4),
        (cp_x(XG[2], HQ - XG[2], SEM_W + 5) if XG[2] < HQ else [])
        + [cp(wqkv_hbm.at[:, pl.ds(0, D)], wq_buf, SEM_W + 5)],
    ]

    def cp_b(j, wait_only=False):
        dsts = [r.at[j] for r in (wg_buf, wu_buf, wd_buf, wv_buf, wo_buf)]
        if wait_only:
            return [cp(dst, dst, SEM_B + j) for dst in dsts]
        fs = pl.ds(j * FH, FH)
        srcs = [wg_hbm.at[:, fs], wu_hbm.at[:, fs], wd_hbm.at[fs, :],
                wqkv_hbm.at[:, pl.ds(2 * D + j * HD, HD)], wo_hbm.at[pl.ds(j * HD, HD), :]]
        return [cp(src, dst, SEM_B + j) for src, dst in zip(srcs, dsts)]

    clock = [0]
    toks = []
    sides = []
    fwd = [None]

    def emit_tok(vals, stamp):
        t = None
        for v in vals:
            v = pltpu.bitcast(v, u32) if v.dtype != u32 else v
            t = v if t is None else t | v
        toks.append((stamp, t & zero_buf[0]))

    def token(kind):
        t = fwd[0]
        if "u" not in t:
            t["u"] = pltpu.bitcast(t["src"](), u32) & zero_buf[0]
        if kind != "u" and "f" not in t:
            t["f"] = pltpu.bitcast(t["u"], f32)
        if kind == "f16" and "f16" not in t:
            t["f16"] = jnp.concatenate([t["f"], t["f"]], axis=0)
        return t[kind]

    def gate(v):
        if fwd[0] is None:
            return v
        head = v if v.shape[0] == 8 else v[0:8]
        head = head | token("u") if v.dtype == u32 else head + token("f")
        return head if v.shape[0] == 8 else jnp.concatenate([head, v[8:]], axis=0)

    def gate16(v):
        return v if fwd[0] is None else v + token("f16")

    def add_side(gen_fn, n, t0, t1, lag=None):
        st = {"i": 0, "n": n, "t0": clock[0] + t0, "t1": clock[0] + t1}

        def tok(vals):
            if lag is not None:
                emit_tok(vals, st["t0"] + (st["i"] + 1) * (st["t1"] - st["t0"]) // st["n"] + lag)
        st["g"] = gen_fn(tok)
        sides.append(st)

    def advance(until):
        for st in sides:
            while st["i"] < st["n"] and st["t0"] + st["i"] * (st["t1"] - st["t0"]) // st["n"] < until:
                next(st["g"], None)
                st["i"] += 1
                if st["i"] == st["n"]:
                    for _ in st["g"]:
                        pass

    def flush():
        for st in sides:
            for _ in st["g"]:
                pass
        sides.clear()

    def finish():
        flush()
        toks.clear()
        fwd[0] = None

    def mm(lhs, rhs, cycles, nseg=1):
        due = [t for (c, t) in toks if c <= clock[0]]
        toks[:] = [(c, t) for (c, t) in toks if c > clock[0]]
        if due:
            head = rhs[0:8, 0:128]
            for t in due:
                head = head | t
            if rhs.shape[1] > 128:
                head = jnp.concatenate([head, rhs[0:8, 128:]], axis=1)
            rhs = jnp.concatenate([head, rhs[8:]], axis=0)
        res = jnp.dot(lhs, _unpack(rhs), preferred_element_type=f32)
        ngr = res.shape[0] // 16
        for sg in range(nseg):
            for i in range(ngr):
                fwd[0] = {"src": lambda sg=sg, i=i: res[i * 16:i * 16 + 8, sg * 128:(sg + 1) * 128]}
                clock[0] += cycles // nseg // ngr
                advance(clock[0])
        return res

    def form_steps(form, form2, get, put, tok=None, keep=range(7)):
        terms = form(*[_Sym({i: 1}) for i in range(4)])
        gated = (0, 1, 2, 3) if 7 in keep else {_wl: (0, 1, 3), _wr: (0, 2, 3), _wl_swapped: (1, 2)}[form2]
        for k1 in range(7):
            sub = []
            for r in range(2):
                for c in range(2):
                    v = None
                    for i, sg in sorted(terms[k1].t.items(), key=lambda e: -e[1]):
                        b = get(r + 2 * (i // 2), c + 2 * (i % 2))
                        if v is None:
                            v = gate16(b) if 2 * r + c in gated else b
                        else:
                            v = v + b if sg > 0 else v - b
                    sub.append(v)
            vals = form2(*sub) + (sub[2],)
            for k2 in keep:
                put(k1, k2, _pack(vals[k2]))
            if tok is not None and k1 % 2 == 0:
                full = vals[3 if form2 is _wr else 2]
                tok([full[0:8], full[8:16]])
            yield

    def strassen2(lhs, rhs, cycles, nseg=1, wts=(16,) * 7, comb=_wc):
        m1 = [None] * 7
        for i1, k1 in enumerate(K_SEQ2):
            m2 = [None] * 7
            for k2 in W_SEQ:
                m2[k2] = mm(lhs(k1, k2), rhs(k1, k2), cycles * wts[i1] // 16, nseg)
                yield
            m1[k1] = comb(m2)
        out = [[None] * 4 for _ in range(4)]
        for s2 in range(4):
            for s1, v in enumerate(_combine2([m1[k1][s2] for k1 in range(7)])):
                out[(s1 // 2) * 2 + s2 // 2][(s1 % 2) * 2 + s2 % 2] = v
        return out

    made = set()

    def need(*keys):
        assert all(k in made for k in keys), keys

    def row_views(base):
        if base == 0:
            return x_buf, sa, sb, stats, xn_buf, None
        i, n = base
        b = _mo(i * n, 16)
        return ([x_buf.at[:, pl.ds(b, n), :]] + [r.at[pl.ds(b, S - 128 + n), :] for r in (sa, sb, stats)]
                + [xn_buf.at[:, pl.ds(b, n), :], pl.ds(_mo(i * (n // 2), 8), n // 2)])

    def xs_form(r0, tok, which="all", base=0):
        xn_v, xs_v = row_views(base)[4:]
        rows = slice(r0 % XN, r0 % XN + 16)

        keep = {"all": range(8), "l1": (0, 1, 7, 3), "l2": (2, 4, 5, 6)}[which]
        for ct in range(2):
            def put(k1, k2, v):
                xs_at(k1, k2, xs_v)[r0 // 2:r0 // 2 + 8, ct * 128:(ct + 1) * 128] = v
            yield from form_steps(
                _sform, _wl, lambda q, u: xn_v[q, rows, _st(u, ct)], put, tok, keep)
        made.add(("xs", r0))

    def ln_stats(r_start, n_rows, tok, base=0):
        x_v, sa_v, sb_v, st_v, xn_v, _ = row_views(base)
        lane = lax.broadcasted_iota(i32, (8, 128), 1)
        for r0 in range(r_start, r_start + n_rows, 16):
            if r0 >= T0:
                need(("in", 2 + sum(r0 >= g for g in XG)))
            if r0 - XN >= T0:
                need(("ln", r0 - XN))
            for g in range(8):
                q, o = g // 2, (g % 2) * 8
                rg = q * HQ + r0 + o
                xv = x_v[q, r0 + o:r0 + o + 8, :].astype(f32)
                xg = jnp.concatenate([gate(xv[:, 0:128]), xv[:, 128:]], axis=1)
                mf = jnp.sum(xg, axis=1, keepdims=True) * (1.0 / D)
                d = xv - mf
                var = jnp.sum(d * d, axis=1, keepdims=True) * (1.0 / D)
                rs = lax.rsqrt(var + 1e-5)
                xn_v.at[q][r0 % XN + o:r0 % XN + o + 8, :] = _to_st(d * rs)
                rs = jnp.broadcast_to(rs, (8, 128))
                mf = jnp.broadcast_to(mf, (8, 128))
                sa_v[rg:rg + 8, :] = 1.0 + rs
                sb_v[rg:rg + 8, :] = mf * rs
                st_v[rg:rg + 8, 0:128] = jnp.where(lane == 0, mf, jnp.broadcast_to(var, (8, 128)))
                if tok is not None:
                    tok([rs])
                if g == 7:
                    made.add(("xn", r0))
                yield

    def ln_later(r_start, n_rows, tok, which="all", base=0):
        st_v, xn_v = row_views(base)[3:5]
        for r0 in range(r_start, r_start + n_rows, 16):
            need(("xn", r0))
            form = xs_form(r0, tok, which, base)
            for g in range(8):
                for _ in range(2 if g < 7 else 0):
                    next(form)
                    yield
                q, o = g // 2, (g % 2) * 8
                t = None
                if which != "l1":
                    v = xn_v[q, r0 % XN + o:r0 % XN + o + 8, :] * wrb[8:16, :]
                    for ct in range(8):
                        h = v[:, ct * 128:(ct + 1) * 128]
                        t = gate(h) if t is None else t + h
                if t is not None:
                    st_v[q * HQ + r0 + o:q * HQ + r0 + o + 8, 128:256] = t
                if tok is not None:
                    tok([t])
                if g == 7:
                    next(form, None)
                    made.add(("ln", r0))
                yield

    def wk_prep(c):
        if isinstance(c, int):
            need(("in", c))
        wks.at[c][:, 128:256] = pltpu.bitcast(wk_buf[c, 0:HD, 0:128], u32)
        wks.at[c][:, 512:640] = pltpu.bitcast(wk_buf[c, HD:D, 128:256], u32)
        for i in range(HD // 16):
            r0 = i * 16
            top = wk_buf[c, r0:r0 + 16, :].astype(f32)
            bot = wk_buf[c, HD + r0:HD + r0 + 16, :].astype(f32)
            ops = _rform(top[:, :128], top[:, 128:], bot[:, :128], bot[:, 128:])
            for k in (0, 2, 3, 5, 6):
                wks.at[c][r0 // 2:r0 // 2 + 8, k * 128:(k + 1) * 128] = _pack(ops[k])

    def wq_perm():
        need(("in", 5))

        def permute(kt):
            for g in range(8):
                tile = gate(pltpu.bitcast(wq_buf[kt * 128:(kt + 1) * 128, g * 128:(g + 1) * 128], u32))
                wqt.at[kt * 8 + g][...] = pltpu.bitcast(_unpack(tile).T, u32)
                yield

        def back(kt):
            for j in range(8):
                tile = gate(jnp.concatenate([wqt[kt * 8 + g, pl.ds(j, 8, stride=8), :] for g in range(8)],
                                            axis=0))
                v = pltpu.bitcast(_unpack(tile).T.astype(f32), u32)
                c0 = (kt // 2) * D + _st(j // 2, j % 2).start
                ps[(kt % 2) * 128:(kt % 2 + 1) * 128, c0:c0 + 128] = v
                made.add(("wqp", kt, j))
                yield

        order = (0, 2, 4, 6, 1, 3, 5, 7)
        for n in range(10):
            if n < 8:
                yield from permute(order[n])
            if n > 1:
                yield from back(order[n - 2])

    def wq_form():
        for i in range(16):
            need(*[("wqp", 2 * r + i // 8, j) for r in range(4) for j in range(8)])
            for ct in range(2):
                def put(k1, k2, v):
                    wqs.at[k1 * 7 + k2][i * 8:(i + 1) * 8, ct * 128:(ct + 1) * 128] = v
                yield from form_steps(
                    _rform, _wr, lambda r, c: pltpu.bitcast(
                        ps[i * 16:(i + 1) * 16, r * D + _st(c, ct).start:r * D + _st(c, ct).stop],
                        f32), put)

    def kproj(r0, n, chunks=range(4), wts=(16,) * 7):
        pr = pl.ds(r0 // 2, n // 2)
        need(*[("xs", r) for r in range(max(r0, T0), r0 + n, 16)])
        for c in chunks:
            m = [None] * 7
            for i, k in enumerate(K_SEQ):
                e11, e12, e21, e22 = [xs_at(L_ORD[k], e)[pr, :] for e in (0, 1, 7, 3)]
                lhs = jnp.concatenate([jnp.concatenate([e11, e12], axis=1),
                                       jnp.concatenate([e21, e22], axis=1)], axis=0)
                m[k] = mm(_unpack(lhs), wks[c, :, k * 128:(k + 1) * 128], 2 * n * wts[i] // 16)
            kk = [_phi(v) for v in _combine(m)]
            for ct in range(2):
                zacc[:, pl.ds(_mo(c * 256 + ct * 128, 128), 128)] += (
                    (kk[ct] + kk[2 + ct]).reshape(n // 4, 8, 128).sum(axis=0))
            j, c2 = (c // 2, c % 2) if isinstance(c, int) else (0, c)
            pk_v = pk_buf.at[j, :, :, pl.ds(_mo(c2 * 256, 256), 256)]
            for s1 in range(4):
                for h in range(2):
                    pk_v.at[(s1 // 2) * 2 + h][r0:r0 + n, (s1 % 2) * 128:(s1 % 2 + 1) * 128] = (
                        kk[s1][h * n:(h + 1) * n])

    def z_prep():
        z = jnp.sum(zacc[...], axis=0, keepdims=True)
        zt = _pack(jnp.broadcast_to(z, (128, D)).astype(bf16).T)
        for g in range(8):
            tscr.at[g][...] = zt[g * 64:(g + 1) * 64, :]
        for j in range(8):
            blk = jnp.concatenate([tscr[g, pl.ds(j, 8, stride=8), :] for g in range(8)], axis=0)
            zp[:, j * 128:(j + 1) * 128] = _unpack(blk).T[0:8, :].astype(f32)

    def route():
        rows, dots = [None] * 16, [None] * 16
        for b in sorted(range(S // 128), key=lambda b: b % 4):
            need(*[("ln", r) for r in range(max(T0, b % 4 * 128), b % 4 * 128 + 128, 16)])
            rows[b] = gate(stats[b * 128:(b + 1) * 128, 0:128]).T[0:8, :]
            dots[b] = jnp.sum(gate(stats[b * 128:(b + 1) * 128, 128:256]).T, axis=0, keepdims=True)
            yield
        mf = jnp.concatenate([v[0:1] for v in rows], axis=0)
        var = jnp.concatenate([v[1:2] for v in rows], axis=0)
        tr = jnp.concatenate(dots, axis=0) * jnp.sqrt(var + 1e-5)
        wsum = jnp.sum(wrb[0:1, :], axis=1, keepdims=True)
        mb = _rbf(mf)
        inv = 1.0 / _rbf(jnp.sqrt(_rbf(_rbf(var) + 1e-5)))
        rv = _rbf((tr + (mf - mb) * wsum) * inv)
        rmax = jnp.max(jnp.max(rv, axis=1, keepdims=True), axis=0, keepdims=True)
        pos = (lax.broadcasted_iota(i32, rv.shape, 0) * 128 + lax.broadcasted_iota(i32, rv.shape, 1))
        idx = jnp.min(jnp.where(rv == rmax, pos, S - 1))
        idx_s[0] = idx

        def pick(v):
            v = jnp.sum(jnp.where(pos == idx, v, 0.0), axis=1, keepdims=True)
            return jnp.sum(v, axis=0, keepdims=True)

        xv = x_buf[(idx >> 9) & 3, pl.ds(_mo(idx & (HQ - 16), 16), 16), :].astype(f32)
        sel = lax.broadcasted_iota(i32, xv.shape, 0) == (idx & 15)
        row = jnp.sum(jnp.where(sel, xv, 0.0), axis=0, keepdims=True)
        row = _rbf(_rbf(row - pick(mb)) * pick(inv))
        rsel[...] = jnp.broadcast_to(_rbf(jnp.sum(row * wrb[0:1, :], axis=1, keepdims=True)), rsel.shape)
        xb[...] = jnp.broadcast_to(row, (128, D)).T
        yield

    def ps_form(j):
        for c in range(HQ // 16):
            def put(k1, k2, v):
                k = k1 * 7 + k2
                ps[c * 8:(c + 1) * 8, k * 128:(k + 1) * 128] = v
            yield from form_steps(
                _lform, _wl_swapped,
                lambda r, q: pk_buf[j, q, c * 16:(c + 1) * 16, r * 128:(r + 1) * 128], put)
            made.add(("ps", c))

    def ps_flip(t):
        need(*[("ps", c) for c in range(8 * t, 8 * t + 8)])
        for k in range(49):
            at = (slice(t * 64, (t + 1) * 64), slice(k * 128, (k + 1) * 128))
            ps[at] = pltpu.bitcast(_unpack(gate(ps[at])).T, u32)
            yield

    def q_rows(j, r0, n, pq, rc, d0, wts):
        xj = pl.ds(_mo(j * (BQ // 2), BQ // 2), BQ // 2)
        pr = slice(r0 // 2, (r0 + n) // 2)
        blk = yield from strassen2(lambda k1, k2: _unpack(xs_at(L_ORD[k1], k2, xj)[pr, :]),
                                   lambda k1, k2: wqs[k1 * 7 + k2], n, 1, wts)
        for q in range(4):
            d = None
            for u in ((0, 1, 2, 3) if q >= 2 else (3, 2, 1, 0)):
                v = _phi(blk[q][u])
                for ct in range(2):
                    pq.at[q][d0:d0 + n, _st(u, ct)] = v[:, ct * 128:(ct + 1) * 128]
                t = v * zp[0:1, u * 256:(u + 1) * 256]
                t = t[:, :128] + t[:, 128:]
                d = t if d is None else d + t
            rc.at[q][d0:d0 + n, :] = d

    def normalise(pq, rc, nr, dst, tok=None):
        lane = lax.broadcasted_iota(i32, (16, 128), 1)
        nc = nr // 16

        def recips(c):
            rq = slice(c * 16, (c + 1) * 16)
            for q in range(4):
                d = gate16(rc[q, rq, :])
                d = d + jnp.where(lane % 2 == 0, pltpu.roll(d, 127, 1), pltpu.roll(d, 1, 1))
                d = d + jnp.where(lane % 4 < 2, pltpu.roll(d, 126, 1), pltpu.roll(d, 2, 1))
                rc.at[q][rq, :] = 1.0 / (d + 1e-6)
                yield

        def scale(c):
            rq = slice(c * 16, (c + 1) * 16)
            for hf in range(2):
                for q in range(4):
                    cs = slice(hf * HD, (hf + 1) * HD)
                    pq.at[q][rq, cs] = pq[q, rq, cs] * jnp.concatenate([gate16(rc[q, rq, :])] * 4, axis=1)
                    yield

        def form(c):
            rq = slice(c * 16, (c + 1) * 16)
            for ct in range(2):
                def put(k1, k2, v):
                    dst.at[k1 * 7 + k2][c * 8:(c + 1) * 8, ct * 128:(ct + 1) * 128] = v
                yield from form_steps(_lform, _wl, lambda q, u: pq[q, rq, _st(u, ct)], put, tok)

        def ahead(c):
            if c + 2 < nc:
                yield from recips(c + 2)
            if c + 1 < nc:
                yield from scale(c + 1)

        yield from recips(0)
        yield from recips(1)
        for _ in range(4):
            yield
        yield from scale(0)
        for c in range(nc):
            nxt = ahead(c)
            for _ in form(c):
                yield
                if next(nxt, 0) is None:
                    yield

    def g_kvm(j):
        qb = q_rows(j, BQ - QB, QB, pqb_buf.at[j], denb_buf.at[j], 0, QWB)
        blk = yield from strassen2(
            lambda k1, k2: _unpack(jnp.concatenate(
                [ps[t * 64:(t + 1) * 64, (k1 * 7 + k2) * 128:(k1 * 7 + k2 + 1) * 128] for t in range(4)], axis=1)),
            lambda k1, k2: xs_at(R_ORD[k1], W_R[k2])[...], 256, 2, comb=_wc_swapped)
        hm = (lax.broadcasted_iota(i32, (128, 128), 0) // 32
              == lax.broadcasted_iota(i32, (128, 128), 1) // 32)
        for _ in range(QSPLIT):
            next(qb)
        kvps = []
        for a in (3, 2, 1, 0):
            gg = jnp.concatenate(blk[a], axis=1).astype(bf16)
            wv_u = pltpu.bitcast(wv_buf[j, :, a * 128:(a + 1) * 128], u32)
            kv = jnp.where(hm, mm(gg, wv_u, 256), 0.0)
            tscr2.at[a][...] = _pack(kv)
            kvps.append(_unpack(jnp.concatenate(
                [tscr2[a, pl.ds(jj, 8, stride=8), :] for jj in range(8)], axis=0)))

        ms_j = ms.at[:, pl.ds(_mo(j * 32, 32), 96), :]

        def m_form():
            for a in (3, 2, 1, 0):
                need(("mg", a))
                for jl in range(2):
                    for ct in range(2):
                        def put(k1, k2, v):
                            ms_j.at[k1 * 7 + k2][jl * 64 + a * 8:jl * 64 + (a + 1) * 8,
                                                 ct * 128:(ct + 1) * 128] = v
                        yield from form_steps(
                            _rform, _wr, lambda q, u: mg_buf[a, (2 * q + jl) * 16:(2 * q + jl + 1) * 16, _st(u, ct)], put)

        for i, a in enumerate((3, 2, 1, 0)):
            wo_u = pltpu.bitcast(wo_buf[j, a * 128:(a + 1) * 128, :], u32)
            res = mm(kvps[i], wo_u, 256)
            mg_buf.at[a][...] = _to_st(res)
            made.add(("mg", a))
            if i == 0:
                add_side(lambda tok: m_form(), 112, *MF)
        for _ in qb:
            pass

    def out_part(base, span, off, nr, y, src):
        b = _mo(base, 32)
        sa_v, sb_v, out_v = [r.at[pl.ds(b, 3 * HQ + span), :] for r in (sa, sb, out_buf)]
        x_v = x_buf.at[:, pl.ds(b, span), :]
        row = lax.broadcasted_iota(i32, (nr, 256), 0) + (base + off)
        blk = yield from strassen2(lambda k1, k2: _unpack(src[k1 * 7 + k2, off // 2:(off + nr) // 2, :]),
                                   lambda k1, k2: ms[k1 * 7 + k2], nr)
        for s1 in (2, 1, 3, 0):
            for s2 in range(4):
                q = (s1 // 2) * 2 + s2 // 2
                u = (s1 % 2) * 2 + s2 % 2
                rr, cc = pl.ds(q * HQ + off, nr), pl.ds(u * 256, 256)
                a = jnp.concatenate([sa_v[rr, :]] * 2, axis=1)
                c = jnp.concatenate([sb_v[rr, :]] * 2, axis=1)
                o = blk[q][u] + jnp.where(row + q * HQ == idx_s[0], y[:, u * 256:(u + 1) * 256], 0.0)
                out_v[rr, cc] = (x_v[q, off:off + nr, cc].astype(f32) * a - c + o).astype(bf16)
                if s2 % 2 == 1:
                    ch = pl.ds((s1 % 2) * HD, HD)
                    ro = pl.ds(_mo(base + q * HQ + off, 16), nr)
                    cp(out_buf.at[ro, ch], out_hbm.at[0, ro, ch], SEM_O).start()

    def ffn_part(j):
        def fma(acc, w, v):
            p = w.astype(f32) * v
            return acc + p[0:8] + p[8:16]

        for f0 in range(0, FH, 256):
            fs = slice(f0, f0 + 256)
            ag = jnp.zeros((8, 256), f32)
            au = jnp.zeros((8, 256), f32)
            for k in range(0, D, 16):
                xv = jnp.concatenate([gate16(xb[k:k + 16, :])] * 2, axis=1)
                ag = fma(ag, wg_buf[j, k:k + 16, fs], xv)
                au = fma(au, wu_buf[j, k:k + 16, fs], xv)
                yield
            g = _rbf(jnp.sum(ag, axis=0, keepdims=True))
            u = _rbf(jnp.sum(au, axis=0, keepdims=True))
            h = _rbf(_rbf(g * jax.nn.sigmoid(g)) * u)
            hb_buf[fs, :] = jnp.broadcast_to(h, (128, 256)).T
        for d0 in range(0, D, 512):
            ds_ = slice(d0, d0 + 512)
            acc = yacc[:, ds_]
            for k in range(0, FH, 16):
                hv = jnp.concatenate([gate16(hb_buf[k:k + 16, :])] * 4, axis=1)
                acc = fma(acc, wd_buf[j, k:k + 16, ds_], hv)
                yield
            yacc[:, ds_] = acc

    def wait_group(i):
        with _scope("a_wait%d" % i):
            for c in a_groups[i]:
                c.wait()
        made.add(("in", i - NX))

    def run_all(gen):
        for _ in gen:
            pass

    def ln_sides(plan):
        for r0, r1, t0, t1 in plan[0]:
            add_side(lambda tok, r0=r0, r1=r1: ln_stats(r0, r1 - r0, tok), (r1 - r0) // 2, t0, t1, LNLAG)
        for r0, r1, t0, t1 in plan[1]:
            add_side(lambda tok, r0=r0, r1=r1: ln_later(r0, r1 - r0, tok), 22 * (r1 - r0) // 16, t0, t1, SLAG)

    def l2_side(base, n, t0, t1):
        add_side(lambda tok: ln_later(0, n, None, "l2", base), 22 * n // 16, t0, t1)

    with _scope("p0_issue"):
        cp_wr.start()
        for grp in a_groups:
            for c in grp:
                c.start()
        for j in range(2):
            for c in cp_b(j):
                c.start()
        zacc[...] = jnp.zeros(zacc.shape, f32)
        yacc[...] = jnp.zeros(yacc.shape, f32)
        zero_buf[1] = jnp.zeros((8, 128), u32)
        cp_zero = cp(zero_buf.at[1], zero_buf.at[0], SEM_Z)
        cp_zero.start()
        cp_zero.wait()
        cp_wr.wait()
        wr8 = jnp.broadcast_to(wr_buf[0:D].reshape(1, D).astype(f32), (8, D))
        wrb[0:8, :] = wr8
        wrb[8:16, :] = _to_st(wr8)
        z0 = jnp.max(pltpu.bitcast(zero_buf[0], i32))
        ps, pq_buf, den_buf, mg_buf, hb_buf = [r.at[z0] for r in (ps_raw, pq_raw, den_raw, mg_raw, hb_raw)]
        xn_buf = mg_buf

    def main(_, carry0):
        def a01(i, carry):
            with _scope("a_wait01"):
                for c in cp_x(i * X0, X0, SEM_A + i):
                    c.wait()
            with _scope("a01"):
                for r in range(0, X0, 16):
                    run_all(ln_stats(r, 16, None, (i, X0)))
                    if r:
                        run_all(ln_later(r - 16, 16, None, "l1", (i, X0)))
                run_all(ln_later(X0 - 16, 16, None, "l1", (i, X0)))
            return carry

        lax.fori_loop(0, NX, a01, 0)
        made.update(("xn", r) for r in range(0, 64, 16))

        def a23(i, carry):
            with _scope("a_wait23"):
                for c in cp_wk(i, SEM_W + i):
                    c.wait()
            with _scope("a23"):
                wk_prep(i)
                l2_side((i, T0 // 2), T0 // 2, *L2W)
                kproj(0, T0, [i])
                finish()
            return carry

        lax.fori_loop(0, 2, a23, 0)
        wait_group(NX + 2)
        with _scope("a4"):
            wk_prep(2)
            ln_sides(L4)
            kproj(0, T0, [2])
            finish()
        wait_group(NX + 3)
        with _scope("a5"):
            wk_prep(3)
            ln_sides(L5)
            kproj(0, T0, [3])
            for r0, n in A5K:
                kproj(r0, n, wts=KW5)
            finish()
        wait_group(NX + 4)
        with _scope("a6"):
            ln_sides(L6)
            for r0, n in A6K:
                kproj(r0, n, wts=KW6)
            finish()
        wait_group(NX + 5)
        with _scope("a7"):
            ln_sides(L7)
            add_side(lambda tok: wq_perm(), 128, *WQ_PERM)
            add_side(lambda tok: wq_form(), 224, *WQ_FORM)
            add_side(lambda tok: route(), 17, *ROUTE)
            for r0, n in A7K:
                kproj(r0, n, wts=KW7)
            finish()

        def b_body(j, carry):
            qa = BQ - QB
            with _scope("b_r0"):
                z_prep()
                add_side(lambda tok: ps_form(j), 7 * HQ // 16, *PSW)
                for t in range(4):
                    add_side(lambda tok, t=t: ps_flip(t), 49, *PFW[t])
                for r0 in range(0, qa, QN):
                    run_all(q_rows(j, r0, QN, pq_buf, den_buf, r0, QW))
                finish()
            with _scope("b_wait"):
                for c in cp_b(j, wait_only=True):
                    c.wait()
            with _scope("b_r1"):
                add_side(lambda tok: ffn_part(j), FH * 3 // 8, *FFW)
                qs_j = qs.at[:, pl.ds(_mo(j * (qa // 2), 16), qa // 2), :]
                add_side(lambda tok: normalise(pq_buf, den_buf, qa, qs_j), 4 + 26 * (qa // 16), *NRW)
                run_all(g_kvm(j))
                finish()
            return carry

        lax.fori_loop(0, 2, b_body, 0)

        def c_body(t, carry):
            with _scope("c_body"):
                y = _rbf(jnp.sum(yacc[...], axis=0, keepdims=True))
                y = _rbf(y * _rbf(1.0 / _rbf(1.0 + _rbf(jnp.exp(-rsel[0:1, :])))))
                j, h = t >> 1, t & 1
                na, nb = (BQ - QB) // 2, QB // 2
                hb = pl.ds(_mo(h * nb, 16), nb)
                add_side(lambda tok: normalise(pqb_buf.at[j, :, hb, :], denb_buf.at[j, :, hb, :], nb, qsb, tok),
                         4 + 26 * (nb // 16), *CNW, SLAG)
                qs_t = qs.at[:, pl.ds(_mo(t * (na // 2), 16), na // 2), :]
                for p in range(0, na, CR):
                    run_all(out_part(j * BQ + h * na, na, p, CR, y, qs_t))
                flush()
                run_all(out_part(j * BQ + BQ - QB + h * nb, nb, 0, nb, y, qsb))
                finish()
            return carry

        lax.fori_loop(0, 4, c_body, 0)
        return carry0

    lax.fori_loop(0, z0 + 1, main, 0)
    with _scope("tail"):
        cp(out_buf, out_hbm.at[0], SEM_O).wait()


@jax.jit
def pallas_parallel_sum__linear_attn_block__moe_arch_mod__prompt_kernel(
    A_x: jax.Array,
    A_wqkv: jax.Array,
    A_wo: jax.Array,
    B_x: jax.Array,
    B_w_r: jax.Array,
    B_w_gate: jax.Array,
    B_w_up: jax.Array,
    B_w_down: jax.Array,
):
    del B_x
    V = pltpu.VMEM
    scratch = [
        V((4, HQ, D), bf16),
        V((4, D, 256), bf16),
        V((2, D, 512), bf16),
        V((2, 512, D), bf16),
        V((8 * D,), bf16),
        V((2, D, FH), bf16),
        V((2, D, FH), bf16),
        V((2, FH, D), bf16),
        V((28, HQ // 2, 256), u32),
        V((28, HQ // 2, 256), u32),
        V((49, 128, 256), u32),
        V((S, 128), f32),
        V((S, 128), f32),
        V((8, D), f32),
        V((8, D), f32),
        V((2, 4, HQ, 512), f32),
        V((D, 128), f32),
        V((8, D), f32),
        V((8, D), f32),
        V((16, D), f32),
        V((4, 8, 128), u32),
        V((4, HD // 2, 7 * 128), u32),
        V((S, 256), f32),
        V((64, 64, 128), u32),
        V((1, HQ // 2, 49 * 128), u32),
        V((49, BQ - QB, 256), u32),
        V((49, 128, 256), u32),
        V((8, 64, 128), u32),
        V((4, 64, 128), u32),
        V((1, 4, BQ - QB, D), f32),
        V((1, 4, BQ - QB, 128), f32),
        V((2, 4, QB, D), f32),
        V((2, 4, QB, 128), f32),
        V((49, QB // 4, 256), u32),
        V((1, 4, 128, D), f32),
        V((1, FH, 128), f32),
        V((S, D), bf16),
        pltpu.SMEM((1,), i32),
        pltpu.SemaphoreType.DMA((4 + T0 // X0 + 6,)),
    ]
    extra = {k: True for k in ("disable_bounds_checks", "disable_semaphore_checks")
             if hasattr(pltpu.CompilerParams, k)}
    return pl.pallas_call(
        _kernel,
        out_shape=jax.ShapeDtypeStruct((1, S, D), bf16),
        in_specs=[pl.BlockSpec(memory_space=pl.ANY)] * 7,
        out_specs=pl.BlockSpec(memory_space=pl.ANY),
        scratch_shapes=scratch,
        compiler_params=pltpu.CompilerParams(vmem_limit_bytes=120 * 1024 * 1024, **extra),
    )(A_x.reshape(4, HQ, D), A_wqkv, A_wo, B_w_r, B_w_gate, B_w_up, B_w_down)
```
